```python
import jax
import jax.numpy as jnp

def _softmax(x, axis=-1):
    return jax.nn.softmax(x, axis=axis)
def _gelu(x):
    return jax.nn.gelu(x, approximate=True)
def _silu(x):
    return jax.nn.silu(x)
def _sigmoid(x):
    return jax.nn.sigmoid(x)
def _layernorm(x, axis=-1, eps=1e-5):
    m = jnp.mean(x, axis=axis, keepdims=True)
    v = jnp.var(x, axis=axis, keepdims=True)
    return (x - m) / jnp.sqrt(v + eps)
def _scatter_add(tgt, idx, src, axis=0):
    return tgt.at[idx].add(src)
def _segment_sum(src, seg, n):
    return jax.ops.segment_sum(src, seg, n)
class _Rng:
    def __init__(self, key):
        self._k = key
    def _next(self):
        self._k, sub = jax.random.split(self._k)
        return sub
    def normal(self, shape):
        return jax.random.normal(self._next(), shape, dtype=jnp.bfloat16)
    def randint(self, lo, hi, shape):
        return jax.random.randint(self._next(), shape, lo, hi, dtype=jnp.int32)
    def uniform(self, shape, lo=0.0, hi=1.0):
        return jax.random.uniform(self._next(), shape, jnp.bfloat16, lo, hi)
    def permutation(self, n):
        return jax.random.permutation(self._next(), n)


kernel_name = 'concat_heads__ssm_conv_h3__compressed_kv_cla__prompt'

def setup_inputs():
    _rng = _Rng(jax.random.key(int.from_bytes(__import__("os").urandom(4), "little")))
    _w = (lambda a: (lambda t: t.astype(jnp.bfloat16) if jnp.issubdtype(t.dtype, jnp.floating) else t)(jnp.asarray(a)))
    def _A_setup():
        B, S, D = 1, 2048, 448
        ks = 4
        return {
            "q": _w((lambda *s: _rng.normal(s) * 0.05)(B, S, D)),
            "k": _w((lambda *s: _rng.normal(s) * 0.05)(B, S, D)),
            "v": _w((lambda *s: _rng.normal(s) * 0.05)(B, S, D)),
            "shift_k": _w((lambda *s: _rng.normal(s) * 0.05)(D, ks) * 0.5),
            "ssm_k": _w((lambda *s: _rng.normal(s) * 0.05)(D, S) * (1.0 / S ** 0.5)),
            "ssm_D": _w((lambda *s: _rng.normal(s) * 0.05)(D)),
        }
    _A_in = _A_setup()

    def _B_setup():
        B, H, Sq, Sk, D, M = 1, 16, 2048, 2048, 256, 448
        Dc = 4 * D
        return {
            "x": _w((lambda *s: _rng.normal(s) * 0.05)(B, Sq, M)),
            "c_kv": _w((lambda *s: _rng.normal(s) * 0.05)(B, Sk, Dc)),
            "w_q": _w((lambda *s: _rng.normal(s) * 0.05)(M, H, D) * (M ** -0.5)),
            "w_uk": _w((lambda *s: _rng.normal(s) * 0.05)(Dc, H, D) * (Dc ** -0.5)),
            "w_uv": _w((lambda *s: _rng.normal(s) * 0.05)(Dc, H, D) * (Dc ** -0.5)),
            "w_o": _w((lambda *s: _rng.normal(s) * 0.05)(H, D, M) * ((H * D) ** -0.5)),
        }
    _B_in = _B_setup()

    return {
        "A_q": _A_in["q"],
        "A_k": _A_in["k"],
        "A_v": _A_in["v"],
        "A_shift_k": _A_in["shift_k"],
        "A_ssm_k": _A_in["ssm_k"],
        "A_ssm_D": _A_in["ssm_D"],
        "B_x": _B_in["x"],
        "B_c_kv": _B_in["c_kv"],
        "B_w_q": _B_in["w_q"],
        "B_w_uk": _B_in["w_uk"],
        "B_w_uv": _B_in["w_uv"],
        "B_w_o": _B_in["w_o"],
    }

def reference(A_q, A_k, A_v, A_shift_k, A_ssm_k, A_ssm_D, B_x, B_c_kv, B_w_q, B_w_uk, B_w_uv, B_w_o):
    def _A_ref(q, k, v, shift_k, ssm_k, ssm_D):
        B, S, D = q.shape
        ks = shift_k.shape[-1]
        k_pad = jnp.pad(k, ((0, 0), (ks - 1, 0), (0, 0)))
        k_shift = jnp.zeros_like(k)
        for t in range(ks):
            k_shift = k_shift + k_pad[:, t:t + S, :] * shift_k[:, ks - 1 - t][None, None, :]
        kv = k_shift * v
        L = 2 * S
        kv_pad = jnp.pad(kv, ((0, 0), (0, S), (0, 0)))
        kf_pad = jnp.pad(ssm_k, ((0, 0), (0, S)))
        kv_f = (lambda x, axes=(-2,-1): jnp.fft.rfft2(x.astype(jnp.float32), axes=axes))(kv_pad[:, None, :, :], axes=(1, 2))
        kf_f = (lambda x, axes=(-2,-1): jnp.fft.rfft2(x.astype(jnp.float32), axes=axes))(kf_pad[:, None, :], axes=(1, 2))
        kf_f = (lambda x, *d: x.transpose(*d))(kf_f, 1, 2, 0)
        y_f = kv_f * kf_f[None, :, :, :]
        y = (lambda x, s, axes=(-2,-1): jnp.fft.irfft2(x, s=s, axes=axes).astype(jnp.bfloat16))(y_f, (1, L), axes=(1, 2))[:, 0, :S, :]
        y = y + kv * ssm_D[None, None, :]
        return q * y

    def _B_ref(x, c_kv, w_q, w_uk, w_uv, w_o):
        B, Sq, M = x.shape[0], x.shape[1], x.shape[2]
        Sk = c_kv.shape[1]
        H, D = w_q.shape[1], w_q.shape[2]
        q = jnp.einsum("bqm,mhd->bhqd", x, w_q)
        k = jnp.einsum("bkc,chd->bhkd", c_kv, w_uk)
        v = jnp.einsum("bkc,chd->bhkd", c_kv, w_uv)
        scores = jnp.einsum("bhqd,bhkd->bhqk", q, k) * (D ** -0.5)
        off = Sk - Sq
        qi = jnp.arange(Sq)[:, None]
        kj = jnp.arange(Sk)[None, :]
        cmask = kj <= (qi + off)
        scores = jnp.where(cmask[None, None], scores, -1e9)
        p = _softmax(scores, axis=-1)
        ctx = jnp.einsum("bhqk,bhkd->bhqd", p, v)
        return jnp.einsum("bhqd,hdm->bqm", ctx, w_o)

    a = _A_ref(A_q, A_k, A_v, A_shift_k, A_ssm_k, A_ssm_D)
    b = _B_ref(B_x, B_c_kv, B_w_q, B_w_uk, B_w_uv, B_w_o)
    return jnp.concatenate([a, b], axis=-1)
```

```python
import functools

import jax
import jax.numpy as jnp
from jax import lax
import jax.experimental.pallas as pl
import jax.experimental.pallas.tpu as pltpu

F32 = jnp.float32
BF16 = jnp.bfloat16
U32 = jnp.uint32

S = 2048
M = 448
C = 1024
H = 16
D = 256
KS = 4
LANE = 128
NB = S // LANE
AR = 32
A_STEPS = M // AR
LOG2E = 1.4426950408889634
NEG = -1e30

NT = (((1,), (1,)), ((), ()))


def _dot(a, b):
    return jnp.dot(a, b, preferred_element_type=F32)


def _dot_nt(a, b):
    return lax.dot_general(a, b, NT, preferred_element_type=F32)


def _unpack_pair(w):
    lo = pltpu.bitcast(w << 16, F32).astype(BF16)
    hi = pltpu.bitcast(w & jnp.uint32(0xFFFF0000), F32).astype(BF16)
    return lo, hi


def _make_kernel(tq, wq_chunks, x_chunks):
    nq = S // tq
    nsub = tq // LANE
    wq_rows = M // wq_chunks
    x_cols = S // x_chunks
    WCH = 128
    n_wch = 2 * C // WCH
    QIT = 8

    def kernel(aq_hbm, ak_hbm, av_hbm, sh_hbm, ssm_hbm, dd_hbm, x_hbm, c_hbm,
               wq_hbm, wk_hbm, wv_hbm, wo_hbm,
               out_hbm,
               aq_v, ak_v, av_v, ssm_v, sh_v, dd_v, par_v, f_v,
               xt_v, x_v, c_v, wqs_v, wq_v, ws_v, wkv_v, wo_v,
               q_all, k_s, v_s, p_s, r_t, out_v,
               sem_x, sem_wq, sem_w, sem_misc, sem_out):
        h = pl.program_id(0)

        def x_copy(i):
            return pltpu.make_async_copy(
                x_hbm.at[:, pl.ds(i * x_cols, x_cols)],
                xt_v.at[:, pl.ds(i * x_cols, x_cols)], sem_x.at[i])

        def wq_copy(i, half):
            return pltpu.make_async_copy(
                wq_hbm.at[pl.ds(i * wq_rows * H, wq_rows * H), pl.ds(half * LANE, LANE)],
                wqs_v.at[half, pl.ds(i * wq_rows * H, wq_rows * H)],
                sem_wq.at[2 * i + half])

        def w_copy(src, row0, slot, half):
            return pltpu.make_async_copy(
                src.at[pl.ds(row0, WCH * H), pl.ds(half * LANE, LANE)],
                ws_v.at[slot, half], sem_w.at[2 * slot + half])

        misc = [(c_hbm, c_v), (ak_hbm, ak_v), (av_hbm, av_v), (ssm_hbm, ssm_v),
                (aq_hbm, aq_v), (wo_hbm, wo_v), (sh_hbm, sh_v), (dd_hbm, dd_v)]

        def misc_copy(i):
            return pltpu.make_async_copy(misc[i][0], misc[i][1], sem_misc.at[i])

        @pl.when(h == 0)
        def _prologue():
            misc_copy(6).start()
            misc_copy(7).start()
            for i in range(max(wq_chunks, x_chunks)):
                if i < wq_chunks:
                    wq_copy(i, 0).start()
                    wq_copy(i, 1).start()
                if i < x_chunks:
                    x_copy(i).start()

            bi = lax.broadcasted_iota(jnp.int32, (LANE, LANE), 0)
            mi = lax.broadcasted_iota(jnp.int32, (LANE, LANE), 1)
            ph = ((4 * mi + 1) * bi) & 511
            ang = ph.astype(F32) * (2.0 * 3.141592653589793 / 512.0)
            f_v[:, 0:LANE] = jnp.cos(ang).astype(BF16)
            f_v[:, LANE:2 * LANE] = (-jnp.sin(ang)).astype(BF16)

            r_t[M:, :] = jnp.zeros((M, S), F32)

            misc_copy(6).wait()
            misc_copy(7).wait()
            sh = sh_v[...].astype(F32)
            for j in range(KS):
                par_v[j] = jnp.broadcast_to(sh[j:j + 1, :], (LANE, M)).T
            dd = dd_v[...].astype(F32).reshape(1, M)
            par_v[KS] = jnp.broadcast_to(dd, (LANE, M)).T

            wqs32 = wqs_v.bitcast(U32)
            for i in range(max(wq_chunks, x_chunks)):
                if i < wq_chunks:
                    for half in range(2):
                        wq_copy(i, half).wait()
                        for j in range(H // 2):
                            w = wqs32[half, pl.ds(i * wq_rows * 8 + j, wq_rows, stride=8), :]
                            lo, hi = _unpack_pair(w)
                            rows = pl.ds(i * wq_rows, wq_rows)
                            wq_v[j, rows, pl.ds(half * LANE, LANE)] = lo
                            wq_v[j, rows, pl.ds(D + half * LANE, LANE)] = hi
                if i < x_chunks:
                    x_copy(i).wait()
                    cols = pl.ds(i * x_cols, x_cols)
                    x_v[cols, :] = xt_v[:, cols].astype(F32).T.astype(BF16)

            def start_w(it, slot):
                row0 = pl.multiple_of(it * (WCH * H), WCH * H)
                for half in range(2):
                    w_copy(wk_hbm, row0, 2 * slot, half).start()
                    w_copy(wv_hbm, row0, 2 * slot + 1, half).start()

            start_w(0, 0)
            start_w(1, 1)
            ws32 = ws_v.bitcast(U32)

            def q_body(it, carry):
                slot = it % 2
                for which in range(2):
                    for half in range(2):
                        w_copy(wk_hbm, 0, 2 * slot + which, half).wait()
                for k in range(6):
                    @pl.when(it == k)
                    def _():
                        misc_copy(k).start()
                rows = pl.ds(pl.multiple_of(it * WCH, WCH), WCH)
                for which in range(2):
                    for half in range(2):
                        for j in range(H // 2):
                            w = ws32[2 * slot + which, half, pl.ds(j, WCH, stride=8), :]
                            lo, hi = _unpack_pair(w)
                            cols = pl.ds(which * D + half * LANE, LANE)
                            wkv_v[2 * j, rows, cols] = lo
                            wkv_v[2 * j + 1, rows, cols] = hi
                q2 = _dot(x_v[...], wq_v[it]) * (D ** -0.5 * LOG2E)
                q_all[2 * it] = q2[:, :D].astype(BF16)
                q_all[2 * it + 1] = q2[:, D:].astype(BF16)

                @pl.when(it + 2 < QIT)
                def _():
                    start_w(it + 2, slot)
                return carry

            lax.fori_loop(0, QIT, q_body, 0)
            for k in range(6):
                misc_copy(k).wait()

        def branch_a():
            a0 = pl.multiple_of(jnp.minimum(h, A_STEPS - 1) * AR, AR)
            rows = pl.ds(a0, AR)
            kk = ak_v[rows, :].astype(F32)
            lane = lax.broadcasted_iota(jnp.int32, (AR, LANE), 1)
            coef = [par_v[j, rows, :] for j in range(KS + 1)]
            kv_blocks = []
            rolled = [kk] + [pltpu.roll(kk, j, 1) for j in range(1, KS)]
            vv = av_v[rows, :].astype(F32)
            for a in range(NB):
                cs = slice(a * LANE, (a + 1) * LANE)
                acc = rolled[0][:, cs] * coef[0]
                for j in range(1, KS):
                    t = rolled[j][:, cs]
                    if a == 0:
                        t = jnp.where(lane >= j, t, 0.0)
                    acc = acc + t * coef[j]
                kv_blocks.append((acc * vv[:, cs]).astype(BF16))
            hk = ssm_v[rows, :]
            lhs = jnp.concatenate(
                kv_blocks + [hk[:, a * LANE:(a + 1) * LANE] for a in range(NB)], axis=0)
            spec = _dot(lhs, f_v[...])
            xr = [spec[a * AR:(a + 1) * AR, :LANE] for a in range(NB)]
            xi = [spec[a * AR:(a + 1) * AR, LANE:] for a in range(NB)]
            hr0 = [spec[(NB + a) * AR:(NB + a + 1) * AR, :LANE] for a in range(NB)]
            hi0 = [spec[(NB + a) * AR:(NB + a + 1) * AR, LANE:] for a in range(NB)]
            hr = [hr0[0]] + [hr0[j] - hi0[j - 1] for j in range(1, NB)]
            hi = [hi0[0]] + [hi0[j] + hr0[j - 1] for j in range(1, NB)]
            zs = []
            for c in range(NB):
                zr = zi = None
                for a in range(c + 1):
                    j = c - a
                    tr = xr[a] * hr[j] - xi[a] * hi[j]
                    ti = xr[a] * hi[j] + xi[a] * hr[j]
                    zr = tr if zr is None else zr + tr
                    zi = ti if zi is None else zi + ti
                zs.append(jnp.concatenate([zr, zi], axis=1).astype(BF16))
            z = jnp.concatenate(zs, axis=0)
            y = _dot_nt(z, f_v[...])
            qq = aq_v[rows, :].astype(F32)
            for c in range(NB):
                cs = slice(c * LANE, (c + 1) * LANE)
                yc = y[c * AR:(c + 1) * AR, :] * (1.0 / LANE)
                yc = yc + kv_blocks[c].astype(F32) * coef[KS]
                r_t[rows, cs] = qq[:, cs] * yc

        def proj(r0, n):
            kv = _dot(c_v[r0:r0 + n, :], wkv_v[h]).astype(BF16)
            k_s[r0:r0 + n, :] = kv[:, :D]
            v_s[r0:r0 + n, :] = kv[:, D:]

        q_h = q_all.at[h]
        tri = (lax.broadcasted_iota(jnp.int32, (LANE, LANE), 1)
               <= lax.broadcasted_iota(jnp.int32, (LANE, LANE), 0))
        proj(0, tq)
        for i in range(nq):
            r0 = i * tq
            pb = p_s.at[i % 2]
            s0 = _dot_nt(q_h[r0:r0 + tq, :], k_s[0:r0 + LANE, :])
            parts = [
                _dot_nt(q_h[r0 + LANE * j:r0 + tq, :],
                        k_s[r0 + LANE * j:r0 + LANE * (j + 1), :])
                for j in range(1, nsub)]
            if i + 1 < nq:
                proj(r0 + tq, tq)
            else:
                branch_a()
            ls = []
            for a in range(nsub):
                rows = slice(LANE * a, LANE * (a + 1))
                sa = s0[rows, :]
                if a == 0:
                    dg = jnp.where(tri, sa[:, r0:], NEG)
                    blocks = ([(0, sa[:, :r0])] if r0 > 0 else []) + [(r0, dg)]
                else:
                    blocks = [(0, sa)]
                    for j in range(1, a + 1):
                        b = parts[j - 1][LANE * (a - j):LANE * (a - j + 1), :]
                        if j == a:
                            b = jnp.where(tri, b, NEG)
                        blocks.append((r0 + LANE * j, b))
                m = functools.reduce(
                    jnp.maximum, [jnp.max(b, axis=1, keepdims=True) for _, b in blocks])
                l = None
                for c0, b in blocks:
                    p = jnp.exp2(b - m)
                    ps = jnp.sum(p, axis=1, keepdims=True)
                    l = ps if l is None else l + ps
                    pb[rows, c0:c0 + b.shape[1]] = p.astype(BF16)
                ls.append(l)
            ctx = _dot(pb[:, 0:r0 + LANE], v_s[0:r0 + LANE, :])
            cs = [ctx[LANE * a:LANE * (a + 1)] for a in range(nsub)]
            for j in range(1, nsub):
                cj = _dot(pb[LANE * j:, r0 + LANE * j:r0 + LANE * (j + 1)],
                          v_s[r0 + LANE * j:r0 + LANE * (j + 1), :])
                for a in range(j, nsub):
                    cs[a] = cs[a] + cj[LANE * (a - j):LANE * (a - j + 1)]
            for a in range(nsub):
                r = pl.reciprocal(ls[a], approx=True)
                r = r * (2.0 - ls[a] * r)
                cs[a] = cs[a] * r
            ctx = jnp.concatenate(cs, axis=0).astype(BF16)
            r_t[M:, r0:r0 + tq] += _dot_nt(wo_v[h], ctx)

        @pl.when(h == H - 1)
        def _epilogue():
            n_out = 8
            rows_per = S // n_out

            def out_copy(i):
                rs = pl.ds(i * rows_per, rows_per)
                return pltpu.make_async_copy(out_v.at[rs], out_hbm.at[rs], sem_out.at[i])

            for i in range(n_out):
                cols = slice(i * rows_per, (i + 1) * rows_per)
                out_v[cols, :] = r_t[:, cols].T.astype(BF16)
                out_copy(i).start()
            for i in range(n_out):
                out_copy(i).wait()

    scratch = [
        pltpu.VMEM((M, S), BF16),
        pltpu.VMEM((M, S), BF16),
        pltpu.VMEM((M, S), BF16),
        pltpu.VMEM((M, S), BF16),
        pltpu.VMEM((KS, M), BF16),
        pltpu.VMEM((M,), BF16),
        pltpu.VMEM((KS + 1, M, LANE), F32),
        pltpu.VMEM((LANE, 2 * LANE), BF16),
        pltpu.VMEM((M, S), BF16),
        pltpu.VMEM((S, M), BF16),
        pltpu.VMEM((S, C), BF16),
        pltpu.VMEM((2, M * H, LANE), BF16),
        pltpu.VMEM((H // 2, M, 2 * D), BF16),
        pltpu.VMEM((4, 2, WCH * H, LANE), BF16),
        pltpu.VMEM((H, C, 2 * D), BF16),
        pltpu.VMEM((H, M, D), BF16),
        pltpu.VMEM((H, S, D), BF16),
        pltpu.VMEM((S, D), BF16),
        pltpu.VMEM((S, D), BF16),
        pltpu.VMEM((2, tq, S), BF16),
        pltpu.VMEM((2 * M, S), F32),
        pltpu.VMEM((S, 2 * M), BF16),
        pltpu.SemaphoreType.DMA((x_chunks,)),
        pltpu.SemaphoreType.DMA((2 * wq_chunks,)),
        pltpu.SemaphoreType.DMA((8,)),
        pltpu.SemaphoreType.DMA((8,)),
        pltpu.SemaphoreType.DMA((8,)),
    ]
    return kernel, scratch


def _build(tq=512, wq_chunks=4, x_chunks=4):
    kernel, scratch = _make_kernel(tq, wq_chunks, x_chunks)

    def run(A_q, A_k, A_v, A_shift_k, A_ssm_k, A_ssm_D, B_x, B_c_kv, B_w_q, B_w_uk,
            B_w_uv, B_w_o):
        tr = lambda a: jnp.swapaxes(a, 1, 2).reshape(M, S)
        args = (
            tr(A_q), tr(A_k), tr(A_v), A_shift_k.T, A_ssm_k, A_ssm_D, tr(B_x),
            B_c_kv.reshape(S, C),
            B_w_q.reshape(M * H, D), B_w_uk.reshape(C * H, D), B_w_uv.reshape(C * H, D),
            jnp.swapaxes(B_w_o, 1, 2),
        )
        out = pl.pallas_call(
            kernel,
            grid=(H,),
            in_specs=[pl.BlockSpec(memory_space=pl.ANY)] * len(args),
            out_specs=pl.BlockSpec(memory_space=pl.ANY),
            out_shape=jax.ShapeDtypeStruct((S, 2 * M), BF16),
            scratch_shapes=scratch,
            compiler_params=pltpu.CompilerParams(
                dimension_semantics=("arbitrary",),
                vmem_limit_bytes=120 * 1024 * 1024),
        )(*args)
        return out.reshape(1, S, 2 * M)

    return run


_run = _build()


@jax.jit
def pallas_concat_heads__ssm_conv_h3__compressed_kv_cla__prompt_kernel(
    A_q: jax.Array,
    A_k: jax.Array,
    A_v: jax.Array,
    A_shift_k: jax.Array,
    A_ssm_k: jax.Array,
    A_ssm_D: jax.Array,
    B_x: jax.Array,
    B_c_kv: jax.Array,
    B_w_q: jax.Array,
    B_w_uk: jax.Array,
    B_w_uv: jax.Array,
    B_w_o: jax.Array,
):
    return _run(A_q, A_k, A_v, A_shift_k, A_ssm_k, A_ssm_D, B_x, B_c_kv, B_w_q,
                B_w_uk, B_w_uv, B_w_o)
```

```python
import functools

import jax
import jax.numpy as jnp
from jax import lax
import jax.experimental.pallas as pl
import jax.experimental.pallas.tpu as pltpu

F32 = jnp.float32
BF16 = jnp.bfloat16
U32 = jnp.uint32

S = 2048
M = 448
MP = 512
C = 1024
H = 16
D = 256
KS = 4
LANE = 128
NB = S // LANE
AR = 32
A_STEPS = M // AR
LOG2E = 1.4426950408889634
NEG = -1e30

NT = (((1,), (1,)), ((), ()))


def _dot(a, b):
    return jnp.dot(a, b, preferred_element_type=F32)


def _dot_nt(a, b):
    return lax.dot_general(a, b, NT, preferred_element_type=F32)


def _bf(x):
    return pltpu.bitcast(x, BF16)


def _u32(x):
    return pltpu.bitcast(x, U32)


def _h(r0, n):
    return pl.ds(r0 // 2, n // 2)


def _repack(ev, od):
    lo = (ev & jnp.uint32(0xFFFF)) | (od << 16)
    hi = (ev >> 16) | (od & jnp.uint32(0xFFFF0000))
    return lo, hi


def _opaque_zero(vals):
    acc = None
    for v in vals:
        b = v if v.dtype == U32 else pltpu.bitcast(v, U32)
        for r in range(0, b.shape[0], 8):
            for c in range(0, b.shape[1], LANE):
                t = b[r:r + 8, c:c + LANE]
                acc = t if acc is None else acc | t
    return jnp.minimum((acc >> 1).astype(jnp.int32), 0)


def _pin(x, zero, r=0, c=0):
    t = pltpu.bitcast(pltpu.bitcast(x[r:r + 8, c:c + LANE], jnp.int32) + zero, x.dtype)
    row = ([x[r:r + 8, :c]] if c > 0 else []) + [t] + (
        [x[r:r + 8, c + LANE:]] if c + LANE < x.shape[1] else [])
    row = jnp.concatenate(row, axis=1) if len(row) > 1 else row[0]
    col = ([x[:r, :]] if r > 0 else []) + [row] + ([x[r + 8:, :]] if r + 8 < x.shape[0] else [])
    return jnp.concatenate(col, axis=0) if len(col) > 1 else col[0]


def _make_kernel(cfg):
    wq_chunks, x_chunks = cfg["wq_chunks"], cfg["x_chunks"]
    nsteps = cfg["nsteps"]
    tq = cfg["tq"]
    nq = S // tq
    nsub = tq // LANE
    wq_rows = M // wq_chunks
    x_cols = S // x_chunks
    WCH = 128
    QIT = 8

    def kernel(aq_hbm, ak_hbm, av_hbm, sh_hbm, ssm_hbm, dd_hbm, x_hbm, c_hbm,
               wq_hbm, wk_hbm, wv_hbm, wo_hbm,
               out_hbm,
               aq_v, ak_v, av_v, ssm_v, sh_v, dd_v, par_v, f_v,
               xt_v, x_v, c_v, wqs_v, wq_v, ws_v, wkv_v, wo_v,
               q_all, k_s, v_s, p_s, r_t, ra_t, out_v,
               sem_x, sem_wq, sem_w, sem_misc, sem_out):
        h = pl.program_id(0)
        x32, wq32, wk32, wv32 = (r.bitcast(U32) for r in (x_hbm, wq_hbm, wk_hbm, wv_hbm))

        def x_copy(i):
            return pltpu.make_async_copy(
                x32.at[:, pl.ds(i * x_cols, x_cols)],
                xt_v.at[pl.ds(0, M // 2), pl.ds(i * x_cols, x_cols)], sem_x.at[i])

        def wq_copy(i, half):
            rs = pl.ds(i * wq_rows * 8, wq_rows * 8)
            return pltpu.make_async_copy(
                wq32.at[rs, pl.ds(half * LANE, LANE)], wqs_v.at[half, rs],
                sem_wq.at[2 * i + half])

        def w_copy(src, row0, slot, half):
            return pltpu.make_async_copy(
                src.at[pl.ds(row0, WCH * 8), pl.ds(half * LANE, LANE)],
                ws_v.at[slot, half], sem_w.at[2 * slot + half])

        misc = [(c_hbm.bitcast(U32), c_v), (wo_hbm.bitcast(U32), wo_v),
                (ak_hbm.bitcast(U32), ak_v), (av_hbm.bitcast(U32), av_v),
                (ssm_hbm.bitcast(U32), ssm_v), (aq_hbm.bitcast(U32), aq_v),
                (sh_hbm, sh_v), (dd_hbm, dd_v)]

        def misc_copy(i):
            return pltpu.make_async_copy(misc[i][0], misc[i][1], sem_misc.at[i])

        @pl.when(h == 0)
        def _prologue():
            misc_copy(6).start()
            misc_copy(7).start()
            for i in range(max(wq_chunks, x_chunks)):
                if i < wq_chunks:
                    wq_copy(i, 0).start()
                    wq_copy(i, 1).start()
                if i < x_chunks:
                    x_copy(i).start()

            bi = lax.broadcasted_iota(jnp.int32, (LANE, LANE), 0)
            mi = lax.broadcasted_iota(jnp.int32, (LANE, LANE), 1)
            ph = ((4 * mi + 1) * bi) & 511
            ang = ph.astype(F32) * (2.0 * 3.141592653589793 / 512.0)
            f_v[:, 0:LANE] = _u32(jnp.cos(ang).astype(BF16))
            f_v[:, LANE:] = _u32((-jnp.sin(ang)).astype(BF16))

            r_t[M:, :] = jnp.zeros((M, S), F32)
            xt_v[M // 2:, :] = jnp.zeros(((MP - M) // 2, S), U32)
            wq_v[:, M // 2:, :] = jnp.zeros((H // 2, (MP - M) // 2, 2 * D), U32)

            misc_copy(6).wait()
            misc_copy(7).wait()
            sh = sh_v[...].astype(F32)
            for j in range(KS):
                par_v[j] = jnp.broadcast_to(sh[j:j + 1, :], (LANE, M)).T
            dd = dd_v[...].astype(F32).reshape(1, M)
            par_v[KS] = jnp.broadcast_to(dd, (LANE, M)).T

            for i in range(max(wq_chunks, x_chunks)):
                if i < wq_chunks:
                    for half in range(2):
                        wq_copy(i, half).wait()
                        for j in range(H // 2):
                            b0 = i * wq_rows * 8 + j
                            lo, hi = _repack(
                                wqs_v[half, pl.ds(b0, wq_rows // 2, stride=16), :],
                                wqs_v[half, pl.ds(b0 + 8, wq_rows // 2, stride=16), :])
                            rows = _h(i * wq_rows, wq_rows)
                            wq_v[j, rows, pl.ds(half * LANE, LANE)] = lo
                            wq_v[j, rows, pl.ds(D + half * LANE, LANE)] = hi
                if i < x_chunks:
                    x_copy(i).wait()
                    xt = _bf(xt_v[:, pl.ds(i * x_cols, x_cols)])
                    x_v[_h(i * x_cols, x_cols), :] = _u32(xt.astype(F32).T.astype(BF16))

            def start_w(it, slot):
                row0 = pl.multiple_of(it * (WCH * 8), WCH * 8)
                for half in range(2):
                    w_copy(wk32, row0, 2 * slot, half).start()
                    w_copy(wv32, row0, 2 * slot + 1, half).start()

            start_w(0, 0)

            def q_body(it, carry):
                slot = it % 2
                rows = pl.ds(pl.multiple_of(it * (WCH // 2), WCH // 2), WCH // 2)

                def unpack(which, half, j):
                    lo, hi = _repack(
                        ws_v[2 * slot + which, half, pl.ds(j, WCH // 2, stride=16), :],
                        ws_v[2 * slot + which, half, pl.ds(j + 8, WCH // 2, stride=16), :])
                    cols = pl.ds(which * D + half * LANE, LANE)
                    wkv_v[2 * j, rows, cols] = lo
                    wkv_v[2 * j + 1, rows, cols] = hi
                    return [lo, hi]

                def qproj(r0, n, t, zero):
                    lhs = _bf(x_v[_h(r0, n), :])
                    q2 = jnp.concatenate(
                        [_dot(lhs, _bf(wq_v[it, :, pl.ds(t * D + u * LANE, LANE)])) for u in range(2)],
                        axis=1)
                    if zero is not None:
                        q2 = _pin(q2, zero)
                    q_all[2 * it + t, _h(r0, n), :] = _u32((q2 * (D ** -0.5 * LOG2E)).astype(BF16))

                units = [(w_, h_, j_) for w_ in range(2) for h_ in range(2) for j_ in range(H // 2)]
                npc = cfg["q_pieces"]
                pieces = [(pc, t) for pc in range(npc) for t in range(2)]
                first = len(pieces) // 2
                per = len(units) // (len(pieces) - first)
                for k, (pc, t) in enumerate(pieces):
                    zero = None
                    if k == first:
                        for which in range(2):
                            for half in range(2):
                                w_copy(wk32, 0, 2 * slot + which, half).wait()

                        @pl.when(it == 0)
                        def _():
                            start_w(1, 1)
                    if k >= first:
                        outs = []
                        for (w_, h_, j_) in units[(k - first) * per:(k - first + 1) * per]:
                            outs += unpack(w_, h_, j_)
                        zero = _opaque_zero(outs)
                    qproj(pc * (S // npc), S // npc, t, zero)

                @pl.when(it + 2 < QIT)
                def _():
                    start_w(it + 2, slot)
                for k in range(6):
                    @pl.when(it == k)
                    def _():
                        misc_copy(k).start()
                return carry

            lax.fori_loop(0, QIT, q_body, 0)
            for i in range(6):
                misc_copy(i).wait()

        link = [None]

        def set_link(res, row=None):
            if row is None:
                row = res.shape[0] - cfg["link_back"]
            link[0] = _opaque_zero([res[row:row + 8, res.shape[1] - LANE:]])

        def linked(x, r=0, c=0):
            return x if link[0] is None or not cfg["mxu_chain"] else _pin(x, link[0], r, c)

        a_idx = jnp.minimum(h, A_STEPS - 1)
        a_rows = pl.ds(pl.multiple_of(a_idx * AR, AR), AR)
        a_rows2 = pl.ds(pl.multiple_of(a_idx * (AR // 2), AR // 2), AR // 2)

        def a_fwd():
            kk = _bf(ak_v[a_rows2, :]).astype(F32)
            lane = lax.broadcasted_iota(jnp.int32, (AR, LANE), 1)
            coef = [par_v[j, a_rows, :] for j in range(KS)]
            kv_blocks = []
            rolled = [kk] + [pltpu.roll(kk, j, 1) for j in range(1, KS)]
            vv = _bf(av_v[a_rows2, :]).astype(F32)
            for a in range(NB):
                cs = slice(a * LANE, (a + 1) * LANE)
                acc = rolled[0][:, cs] * coef[0]
                for j in range(1, KS):
                    t = rolled[j][:, cs]
                    if a == 0:
                        t = jnp.where(lane >= j, t, 0.0)
                    acc = acc + t * coef[j]
                kv_blocks.append(acc * vv[:, cs])
            kv = jnp.concatenate(kv_blocks, axis=0)
            hk = ssm_v[a_rows2, :]
            hk = jnp.concatenate([hk[:, a * LANE:(a + 1) * LANE] for a in range(NB)], axis=0)
            fm = _bf(f_v[...])
            hs = _dot(_bf(linked(hk)), fm)
            kv = linked(kv).astype(BF16)
            xs = _dot(kv, fm)
            set_link(xs)
            return kv, xs, hs

        def a_conv(xs, hs):
            def tile(v, a, g, part):
                r = a * AR + 8 * g
                return v[r:r + 8, part * LANE:(part + 1) * LANE]

            prev = [None]

            def make(g):
                xr = [tile(xs, a, g, 0) for a in range(NB)]
                xi = [tile(xs, a, g, 1) for a in range(NB)]
                hr0 = [tile(hs, a, g, 0) for a in range(NB)]
                hi0 = [tile(hs, a, g, 1) for a in range(NB)]
                hr = [hr0[0]] + [hr0[j] - hi0[j - 1] for j in range(1, NB)]
                hi = [hi0[0]] + [hi0[j] + hr0[j - 1] for j in range(1, NB)]
                out = {}
                for c in range(NB):
                    zr = zi = None
                    if cfg["a_serial"] and prev[0] is not None:
                        zero = pltpu.bitcast(prev[0], F32)
                        zr = zi = zero
                    for a in range(c + 1):
                        j = c - a
                        if cfg["a_serial"] == 2 and zr is not None:
                            zr = zr + xr[a] * hr[j]
                            zi = zi + xr[a] * hi[j]
                            zr = zr - xi[a] * hi[j]
                            zi = zi + xi[a] * hr[j]
                        else:
                            tr = xr[a] * hr[j] - xi[a] * hi[j]
                            ti = xr[a] * hi[j] + xi[a] * hr[j]
                            zr = tr if zr is None else zr + tr
                            zi = ti if zi is None else zi + ti
                    out[c, g] = (zr, zi)
                    prev[0] = _opaque_zero([zr, zi])
                return out

            z = {}
            for g in range(AR // 8):
                z.update(make(g))
            pieces = [[*z[c, g], *z[NB - 1 - c, g]] for g in range(AR // 8) for c in range(NB // 2)]
            zs = [jnp.concatenate(
                [jnp.concatenate(z[c, g], axis=1) for g in range(AR // 8)], axis=0)
                for c in range(NB)]
            return zs, pieces

        def a_inv(kv, zs):
            half = NB // 2
            fm = _bf(f_v[...])
            y = jnp.concatenate(
                [_dot_nt(linked(jnp.concatenate(zs[u * half:(u + 1) * half], axis=0)).astype(BF16), fm)
                 for u in range(2)], axis=0)
            if cfg["a_inv_link"]:
                set_link(y, cfg["a_inv_link"])
            qq = _bf(aq_v[a_rows2, :]).astype(F32)
            dd = par_v[KS, a_rows, :]
            kvf = kv.astype(F32)
            for c in range(NB):
                cs = slice(c * LANE, (c + 1) * LANE)
                yc = y[c * AR:(c + 1) * AR, :] * (1.0 / LANE) + kvf[c * AR:(c + 1) * AR, :] * dd
                if cfg["a_sep"]:
                    ra_t[a_rows, cs] = qq[:, cs] * yc
                else:
                    r_t[a_rows, cs] = qq[:, cs] * yc

        def proj(dst, which, r0, n, pins=()):
            outs = []
            npass = cfg["proj_pass"]
            kw = C // npass
            for t in range(2):
                acc = None
                for u in range(npass):
                    lhs = linked(c_v[_h(r0, n), pl.ds(u * kw, kw)])
                    d = _dot(_bf(lhs), _bf(wkv_v[h, _h(u * kw, kw), pl.ds(which * D + t * LANE, LANE)]))
                    set_link(d)
                    acc = d if acc is None else acc + d
                outs.append(acc)
            dst[r0:r0 + n, :] = jnp.concatenate(outs, axis=1).astype(BF16)

        tri = (lax.broadcasted_iota(jnp.int32, (LANE, LANE), 1)
               <= lax.broadcasted_iota(jnp.int32, (LANE, LANE), 0))

        def rowcat(xs):
            return jnp.concatenate(xs, axis=0) if len(xs) > 1 else xs[0]

        def qk(i):
            r0 = i * tq
            parts = [_dot_nt(_bf(linked(q_all[h, _h(r0, tq), :])), k_s[0:r0 + LANE, :])]
            if i > 0:
                link[0] = _opaque_zero([parts[0][0:8, r0 - LANE:r0]])
            for j in range(1, nsub):
                parts.append(_dot_nt(_bf(linked(q_all[h, _h(r0 + LANE * j, tq - LANE * j), :])),
                                     k_s[r0 + LANE * j:r0 + LANE * (j + 1), :]))
            set_link(parts[2], cfg["link_part"])
            return parts

        def softmax(i, parts, pins=()):
            pb = p_s.at[i % 2]
            ngroups = tq // 8
            pin_at = {(k + 1) * ngroups // (len(pins) + 1): piece for k, piece in enumerate(pins)}
            par = cfg["exp_par"]
            chain = []
            if cfg["exp_start"]:
                chain = [_opaque_zero([b[b.shape[0] - 8:, b.shape[1] - LANE:] for b in parts])] * par
            ls = []
            for a in range(nsub):
                blocks = [parts[j][LANE * (a - j):LANE * (a - j + 1), :] for j in range(a + 1)]
                last = blocks[-1]
                w = last.shape[1]
                dg = jnp.where(tri, last[:, w - LANE:], NEG)
                blocks[-1] = dg if w == LANE else jnp.concatenate([last[:, :w - LANE], dg], axis=1)
                sa = jnp.concatenate(blocks, axis=1) if a > 0 else blocks[0]
                m = jnp.max(sa, axis=1, keepdims=True)
                mb = jnp.broadcast_to(m, (LANE, LANE))
                nt = sa.shape[1] // LANE
                ptiles, psums = [], []
                for g in range(0, LANE, 8):
                    mg = mb[g:g + 8, :]
                    if len(chain) >= par:
                        mg = _pin(mg, chain[-par])
                    if (LANE * a + g) // 8 in pin_at:
                        mg = _pin(mg, _opaque_zero(pin_at[(LANE * a + g) // 8]))
                    pg = [jnp.exp2(sa[g:g + 8, t * LANE:(t + 1) * LANE] - mg) for t in range(nt)]
                    ps = functools.reduce(jnp.add, pg)
                    chain.append(_opaque_zero([ps]))
                    psums.append(ps)
                    ptiles.append(jnp.concatenate(pg, axis=1) if nt > 1 else pg[0])
                ls.append(jnp.sum(rowcat(psums), axis=1, keepdims=True))
                p = _pin(rowcat(ptiles), link[0], 0, 0 if a == 0 else sa.shape[1] - LANE)
                pb[LANE * a:LANE * (a + 1), 0:sa.shape[1]] = p.astype(BF16)
            return ls

        def pv(i, ls):
            r0 = i * tq
            pb = p_s.at[i % 2]
            ctx = [_dot(pb[:, 0:r0 + LANE], v_s[0:r0 + LANE, :])]
            for j in range(1, nsub):
                ctx.append(_dot(pb[LANE * j:, r0 + LANE * j:r0 + LANE * (j + 1)],
                                v_s[r0 + LANE * j:r0 + LANE * (j + 1), :]))
            set_link(ctx[2], cfg["link_part"])
            cs = []
            for a in range(nsub):
                sl = lambda j: slice(LANE * (a - j), LANE * (a - j + 1))
                r = pl.reciprocal(ls[a], approx=True)
                r = r * (2.0 - ls[a] * r)
                cs.append(functools.reduce(jnp.add, [ctx[j][sl(j)] for j in range(a + 1)]) * r)
            return rowcat(cs).astype(BF16)

        def oproj(i, ctx):
            for u in range(tq // D):
                res = _dot_nt(_bf(linked(wo_v[h])), ctx[u * D:(u + 1) * D, :])
                set_link(res)
                r_t[M:, i * tq + u * D:i * tq + (u + 1) * D] += res

        use_a = cfg["use_a"]

        a_state = {}

        def a_hook(tag):
            if not use_a:
                return
            if tag == cfg["a_fwd_at"]:
                a_state["kv"], xs, hs = a_fwd()
                a_state["zs"], a_state["pieces"] = a_conv(xs, hs)
            if tag == cfg["a_inv_at"]:
                a_inv(a_state["kv"], a_state["zs"])

        a_hook(0)
        proj(k_s, 0, 0, tq)
        a_hook(1)
        parts = qk(0)
        ctx_prev = None
        for i in range(nq):
            r0 = i * tq
            a_hook(10 * (i + 1))
            if ctx_prev is not None:
                oproj(i - 1, ctx_prev)
            a_hook(10 * (i + 1) + 1)
            if i + 1 < nq:
                proj(k_s, 0, r0 + tq, tq)
            a_hook(10 * (i + 1) + 2)
            proj(v_s, 1, r0, tq)
            a_hook(10 * (i + 1) + 3)
            ls = softmax(i, parts)
            ctx_prev = pv(i, ls)
            a_hook(10 * (i + 1) + 4)
            if i + 1 < nq:
                parts = qk(i + 1)
        oproj(nq - 1, ctx_prev)

        @pl.when(h == nsteps - 1)
        def _epilogue():
            n_out = 8
            rows_per = S // n_out

            def out_copy(i):
                rs = pl.ds(i * rows_per, rows_per)
                return pltpu.make_async_copy(out_v.at[rs], out_hbm.at[rs], sem_out.at[i])

            for i in range(n_out):
                cols = slice(i * rows_per, (i + 1) * rows_per)
                if cfg["a_sep"]:
                    full = jnp.concatenate([ra_t[:, cols], r_t[M:, cols]], axis=0)
                else:
                    full = r_t[:, cols]
                out_v[cols, :] = full.T.astype(BF16)
                out_copy(i).start()
            for i in range(n_out):
                out_copy(i).wait()

    scratch = [
        pltpu.VMEM((M // 2, S), U32),
        pltpu.VMEM((M // 2, S), U32),
        pltpu.VMEM((M // 2, S), U32),
        pltpu.VMEM((M // 2, S), U32),
        pltpu.VMEM((KS, M), BF16),
        pltpu.VMEM((M,), BF16),
        pltpu.VMEM((KS + 1, M, LANE), F32),
        pltpu.VMEM((LANE // 2, 2 * LANE), U32),
        pltpu.VMEM((MP // 2, S), U32),
        pltpu.VMEM((S // 2, MP), U32),
        pltpu.VMEM((S // 2, C), U32),
        pltpu.VMEM((2, M * 8, LANE), U32),
        pltpu.VMEM((H // 2, MP // 2, 2 * D), U32),
        pltpu.VMEM((4, 2, WCH * 8, LANE), U32),
        pltpu.VMEM((H, C // 2, 2 * D), U32),
        pltpu.VMEM((H, M // 2, D), U32),
        pltpu.VMEM((H, S // 2, D), U32),
        pltpu.VMEM((S, D), BF16),
        pltpu.VMEM((S, D), BF16),
        pltpu.VMEM((2, tq, S), BF16),
        pltpu.VMEM((2 * M, S), F32),
        pltpu.VMEM((M, S), F32),
        pltpu.VMEM((S, 2 * M), BF16),
        pltpu.SemaphoreType.DMA((x_chunks,)),
        pltpu.SemaphoreType.DMA((2 * wq_chunks,)),
        pltpu.SemaphoreType.DMA((8,)),
        pltpu.SemaphoreType.DMA((8,)),
        pltpu.SemaphoreType.DMA((8,)),
    ]
    return kernel, scratch


_DEFAULT = dict(wq_chunks=4, x_chunks=4, q_pieces=4, tq=512, use_a=1, proj_pass=2,
                a_serial=0, a_sep=1, a_fwd_at=1, a_inv_at=44, a_inv_link=0,
                mxu_chain=1, link_back=176, link_part=64, exp_par=1, exp_start=1, nsteps=H)


def _build(**kw):
    cfg = dict(_DEFAULT)
    cfg.update(kw)
    kernel, scratch = _make_kernel(cfg)

    def run(A_q, A_k, A_v, A_shift_k, A_ssm_k, A_ssm_D, B_x, B_c_kv, B_w_q, B_w_uk,
            B_w_uv, B_w_o):
        tr = lambda a: jnp.swapaxes(a, 1, 2).reshape(M, S)
        args = (
            tr(A_q), tr(A_k), tr(A_v), A_shift_k.T, A_ssm_k, A_ssm_D, tr(B_x),
            B_c_kv.reshape(S, C),
            B_w_q.reshape(M * H, D), B_w_uk.reshape(C * H, D), B_w_uv.reshape(C * H, D),
            jnp.swapaxes(B_w_o, 1, 2),
        )
        out = pl.pallas_call(
            kernel,
            grid=(cfg["nsteps"],),
            in_specs=[pl.BlockSpec(memory_space=pl.ANY)] * len(args),
            out_specs=pl.BlockSpec(memory_space=pl.ANY),
            out_shape=jax.ShapeDtypeStruct((S, 2 * M), BF16),
            scratch_shapes=scratch,
            compiler_params=pltpu.CompilerParams(
                dimension_semantics=("arbitrary",),
                vmem_limit_bytes=120 * 1024 * 1024),
        )(*args)
        return out.reshape(1, S, 2 * M)

    return run


_run = _build()


@jax.jit
def pallas_concat_heads__ssm_conv_h3__compressed_kv_cla__prompt_kernel(
    A_q: jax.Array,
    A_k: jax.Array,
    A_v: jax.Array,
    A_shift_k: jax.Array,
    A_ssm_k: jax.Array,
    A_ssm_D: jax.Array,
    B_x: jax.Array,
    B_c_kv: jax.Array,
    B_w_q: jax.Array,
    B_w_uk: jax.Array,
    B_w_uv: jax.Array,
    B_w_o: jax.Array,
):
    return _run(A_q, A_k, A_v, A_shift_k, A_ssm_k, A_ssm_D, B_x, B_c_kv, B_w_q,
                B_w_uk, B_w_uv, B_w_o)
```

```python
import functools

import jax
import jax.numpy as jnp
from jax import lax
import jax.experimental.pallas as pl
import jax.experimental.pallas.tpu as pltpu

F32 = jnp.float32
BF16 = jnp.bfloat16
U32 = jnp.uint32

S = 2048
M = 448
MP = 512
C = 1024
H = 16
D = 256
KS = 4
LANE = 128
NB = S // LANE
AR = 32
A_STEPS = M // AR
LOG2E = 1.4426950408889634
NEG = -1e30

NT = (((1,), (1,)), ((), ()))


def _dot(a, b):
    return jnp.dot(a, b, preferred_element_type=F32)


def _dot_nt(a, b):
    return lax.dot_general(a, b, NT, preferred_element_type=F32)


def _bf(x):
    return pltpu.bitcast(x, BF16)


def _u32(x):
    return pltpu.bitcast(x, U32)


def _h(r0, n):
    return pl.ds(r0 // 2, n // 2)


def _repack(ev, od):
    lo = (ev & jnp.uint32(0xFFFF)) | (od << 16)
    hi = (ev >> 16) | (od & jnp.uint32(0xFFFF0000))
    return lo, hi


def _opaque_zero(vals):
    acc = None
    for v in vals:
        b = v if v.dtype == U32 else pltpu.bitcast(v, U32)
        for r in range(0, b.shape[0], 8):
            for c in range(0, b.shape[1], LANE):
                t = b[r:r + 8, c:c + LANE]
                acc = t if acc is None else acc | t
    return jnp.minimum((acc >> 1).astype(jnp.int32), 0)


def _pin(x, zero, r=0, c=0):
    t = pltpu.bitcast(pltpu.bitcast(x[r:r + 8, c:c + LANE], jnp.int32) + zero, x.dtype)
    row = ([x[r:r + 8, :c]] if c > 0 else []) + [t] + (
        [x[r:r + 8, c + LANE:]] if c + LANE < x.shape[1] else [])
    row = jnp.concatenate(row, axis=1) if len(row) > 1 else row[0]
    col = ([x[:r, :]] if r > 0 else []) + [row] + ([x[r + 8:, :]] if r + 8 < x.shape[0] else [])
    return jnp.concatenate(col, axis=0) if len(col) > 1 else col[0]


def _rowcat(xs):
    return jnp.concatenate(xs, axis=0) if len(xs) > 1 else xs[0]


def _lanecat(xs):
    return jnp.concatenate(xs, axis=1) if len(xs) > 1 else xs[0]


def _make_kernel(cfg):
    tq = cfg["tq"]
    nq = S // tq
    nsub = tq // LANE
    WQC = cfg["wq_chunks"]
    wq_pairs = M // 2 // WQC
    XC = 4
    x_cols = S // XC
    WCH = 128
    QIT = 8
    AT = 3

    def kernel(aq_hbm, ak_hbm, av_hbm, sh_hbm, ssm_hbm, dd_hbm, x_hbm, c_hbm,
               wq_hbm, wk_hbm, wv_hbm, wo_hbm,
               out_hbm,
               a_v, sh_v, dd_v, par_v, f_v,
               xt_v, x_v, c_v, wqs_v, wq_v, ws_v, wkv_v, wo_v,
               q_all, k_s, v_s, p_s, ra_t, rb_t, out_v,
               sem_x, sem_wq, sem_w, sem_c, sem_s, sem_a, sem_out):
        x32, c32, wq32, wk32, wv32, wo32 = (
            r.bitcast(U32) for r in (x_hbm, c_hbm, wq_hbm, wk_hbm, wv_hbm, wo_hbm))
        a32 = [r.bitcast(U32) for r in (ak_hbm, av_hbm, ssm_hbm, aq_hbm)]

        def x_copy(i):
            return pltpu.make_async_copy(
                x32.at[:, pl.ds(i * x_cols, x_cols)],
                xt_v.at[pl.ds(0, M // 2), pl.ds(i * x_cols, x_cols)], sem_x.at[i])

        def wq_copy(i, par, half):
            k = 2 * par + half
            dst = wqs_v.reshape(4, M // 2, 8, LANE)
            rs = pl.ds(i * wq_pairs, wq_pairs)
            return pltpu.make_async_copy(
                wq32.at[rs, pl.ds(8 * par, 8), pl.ds(half * LANE, LANE)],
                dst.at[k, rs], sem_wq.at[4 * i + k])

        def w_copies(it, slot):
            dst = ws_v.reshape(16, WCH // 2, 8, LANE)
            rs = pl.ds(it * (WCH // 2), WCH // 2)
            out = []
            for which, src in enumerate((wk32, wv32)):
                for par in range(2):
                    for half in range(2):
                        k = 8 * slot + 4 * which + 2 * par + half
                        out.append(pltpu.make_async_copy(
                            src.at[rs, pl.ds(8 * par, 8), pl.ds(half * LANE, LANE)],
                            dst.at[k], sem_w.at[k]))
            return out

        def c_copy(it):
            n = S // 2 // QIT
            rs = pl.ds(pl.multiple_of(it * n, n), n)
            return pltpu.make_async_copy(c32.at[rs], c_v.at[rs], sem_c.at[it])

        def step_copies(h):
            slot = h % 2
            out = [pltpu.make_async_copy(wo32.at[h], wo_v.at[slot], sem_a.at[5 * slot])]
            n = AR // 2
            rs = pl.ds(pl.multiple_of(jnp.minimum(h, A_STEPS - 1) * n, n), n)
            for k in range(4):
                out.append(pltpu.make_async_copy(
                    a32[k].at[rs], a_v.at[slot, k], sem_a.at[5 * slot + 1 + k]))
            return out

        small = [pltpu.make_async_copy(sh_hbm, sh_v, sem_s.at[0]),
                 pltpu.make_async_copy(dd_hbm, dd_v, sem_s.at[1])]

        link = [None]

        def set_link(res, row=None):
            if row is None:
                row = res.shape[0] - cfg["link_back"]
            link[0] = _opaque_zero([res[row:row + 8, res.shape[1] - LANE:]])

        def linked(x):
            return x if link[0] is None else _pin(x, link[0])

        with jax.named_scope("first_starts"):
            for cp in small:
                cp.start()
        for i in range(WQC):
            for k in range(4):
                wq_copy(i, k // 2, k % 2).start()
        x_copy(0).start()

        bi = lax.broadcasted_iota(jnp.int32, (LANE, LANE), 0)
        mi = lax.broadcasted_iota(jnp.int32, (LANE, LANE), 1)
        ph = ((4 * mi + 1) * bi) & 511
        ang = ph.astype(F32) * (2.0 * 3.141592653589793 / 512.0)
        f_v[:, 0:LANE] = _u32(jnp.cos(ang).astype(BF16))
        f_v[:, LANE:] = _u32((-jnp.sin(ang)).astype(BF16))

        rb_t[...] = jnp.zeros((M, S), F32)
        xt_v[M // 2:, :] = jnp.zeros(((MP - M) // 2, S), U32)
        wq_v[:, M // 2:, :] = jnp.zeros((H // 2, (MP - M) // 2, 2 * D), U32)

        with jax.named_scope("small_wait"):
            for cp in small:
                cp.wait()
        sh = sh_v[...].astype(F32)
        for j in range(KS):
            par_v[j] = jnp.broadcast_to(sh[j:j + 1, :], (LANE, M)).T
        dd = dd_v[...].astype(F32).reshape(1, M)
        par_v[KS] = jnp.broadcast_to(dd, (LANE, M)).T

        for i in range(WQC):
            if i == WQC - 1:
                for i2 in range(1, XC):
                    x_copy(i2).start()
            with jax.named_scope("wq_wait"):
                for k in range(4):
                    wq_copy(i, k // 2, k % 2).wait()
            rows = pl.ds(i * wq_pairs, wq_pairs)
            for half in range(2):
                for j in range(H // 2):
                    ev, od = (
                        wqs_v[pl.ds((2 * par + half) * (M // 2) * 8 + i * wq_pairs * 8 + j,
                                    wq_pairs, stride=8), :] for par in range(2))
                    lo, hi = _repack(ev, od)
                    wq_v[j, rows, pl.ds(half * LANE, LANE)] = lo
                    wq_v[j, rows, pl.ds(D + half * LANE, LANE)] = hi

        def unpack(it, slot, which, half, j):
            ev, od = (
                ws_v[slot, pl.ds((4 * which + 2 * par + half) * (WCH // 2) * 8 + j,
                                 WCH // 2, stride=8), :] for par in range(2))
            lo, hi = _repack(ev, od)
            rows = pl.ds(pl.multiple_of(it * (WCH // 2), WCH // 2), WCH // 2)
            cols = pl.ds(which * D + half * LANE, LANE)
            wkv_v[2 * j, rows, cols] = lo
            wkv_v[2 * j + 1, rows, cols] = hi
            return [lo, hi]

        units = [(w_, h_, j_) for w_ in range(2) for h_ in range(2) for j_ in range(H // 2)]

        def qproj(it, r0, n, t, zero=None):
            outs = []
            for u in range(2):
                lhs = _bf(linked(x_v[_h(r0, n), :]))
                outs.append(_dot(lhs, _bf(wq_v[it, :, pl.ds(t * D + u * LANE, LANE)])))
                set_link(outs[-1])
            q2 = _lanecat(outs)
            if zero is not None:
                q2 = _pin(q2, zero)
            q_all[2 * it + t, _h(r0, n), :] = _u32((q2 * (D ** -0.5 * LOG2E)).astype(BF16))

        def q_pieces(it, slot, pieces):
            per = len(units) // len(pieces)
            for k, (pc, t) in enumerate(pieces):
                outs = []
                for u_ in units[k * per:(k + 1) * per]:
                    outs += unpack(it, slot, *u_)
                qproj(it, pc * x_cols, x_cols, t, _opaque_zero(outs))

        def x_transpose(i):
            xt = _bf(xt_v[:, pl.ds(i * x_cols, x_cols)])
            x_v[_h(i * x_cols, x_cols), :] = _u32(xt.astype(F32).T.astype(BF16))

        for cp in w_copies(0, 0):
            cp.start()
        with jax.named_scope("x_wait"):
            x_copy(0).wait()
        x_transpose(0)
        for t in range(2):
            qproj(0, 0, x_cols, t)
        for cp in w_copies(1, 1):
            cp.start()
        with jax.named_scope("x_wait"):
            for i in range(1, XC):
                x_copy(i).wait()
        link[0] = None
        for i in range(1, XC):
            x_transpose(i)
        for i in range(1, XC - 1):
            for t in range(2):
                qproj(0, i * x_cols, x_cols, t)
        c_copy(0).start()
        with jax.named_scope("w0_wait"):
            for cp in w_copies(0, 0):
                cp.wait()
        link[0] = None
        q_pieces(0, 0, [(XC - 1, 0), (XC - 1, 1)])
        for cp in w_copies(2, 0):
            cp.start()

        def q_body(it, carry):
            slot = it % 2
            with jax.named_scope("w_wait"):
                for cp in w_copies(0, slot):
                    cp.wait()
            c_copy(it).start()
            link[0] = None
            q_pieces(it, slot, [(pc, t) for pc in range(XC) for t in range(2)])

            @pl.when(it + 2 < QIT)
            def _():
                for cp in w_copies(it + 2, slot):
                    cp.start()
            return carry

        for cp in step_copies(0):
            cp.start()
        with jax.named_scope("q_loop"):
            lax.fori_loop(1, QIT, q_body, 0)
        for it in range(QIT):
            c_copy(it).wait()

        tri = (lax.broadcasted_iota(jnp.int32, (LANE, LANE), 1)
               <= lax.broadcasted_iota(jnp.int32, (LANE, LANE), 0))

        def out_copy(i):
            if i == S // D:
                cs = pl.ds(0, AT * LANE)
                return pltpu.make_async_copy(out_v.at[:, cs], out_hbm.at[:, cs], sem_out.at[i])
            rs, cs = pl.ds(i * D, D), pl.ds(AT * LANE, 2 * M - AT * LANE)
            return pltpu.make_async_copy(out_v.at[rs, cs], out_hbm.at[rs, cs], sem_out.at[i])

        def head_step(h, carry):
            slot = h % 2
            with_a = cfg["use_a"]

            @pl.when(h == A_STEPS)
            def _():
                for i in range(S // tq):
                    cols = slice(i * tq, (i + 1) * tq)
                    out_v[cols, 0:AT * LANE] = ra_t[0:AT * LANE, cols].T.astype(BF16)
                out_copy(S // D).start()

            for cp in step_copies(h):
                cp.wait()

            @pl.when(h + 1 < H)
            def _():
                for cp in step_copies(h + 1):
                    cp.start()
            link[0] = None

            a_rows = pl.ds(pl.multiple_of(jnp.minimum(h, A_STEPS - 1) * AR, AR), AR)

            def a_fwd():
                kk = _bf(a_v[slot, 0]).astype(F32)
                lane = lax.broadcasted_iota(jnp.int32, (AR, LANE), 1)
                coef = [par_v[j, a_rows, :] for j in range(KS)]
                rolled = [kk] + [pltpu.roll(kk, j, 1) for j in range(1, KS)]
                vv = _bf(a_v[slot, 1]).astype(F32)
                kv_blocks = []
                for a in range(NB):
                    cs = slice(a * LANE, (a + 1) * LANE)
                    acc = rolled[0][:, cs] * coef[0]
                    for j in range(1, KS):
                        t = rolled[j][:, cs]
                        if a == 0:
                            t = jnp.where(lane >= j, t, 0.0)
                        acc = acc + t * coef[j]
                    kv_blocks.append(acc * vv[:, cs])
                hk = a_v[slot, 2]
                hk = _rowcat([hk[:, a * LANE:(a + 1) * LANE] for a in range(NB)])
                fm = _bf(f_v[...])
                hs = _dot(_bf(linked(hk)), fm)
                kv = linked(_rowcat(kv_blocks)).astype(BF16)
                xs = _dot(kv, fm)
                set_link(xs)
                return kv, xs, hs

            def a_conv(xs, hs):
                blk = lambda v, a, part: v[a * AR:(a + 1) * AR, part * LANE:(part + 1) * LANE]
                xr = [blk(xs, a, 0) for a in range(NB)]
                xi = [blk(xs, a, 1) for a in range(NB)]
                hr = [blk(hs, 0, 0)] + [blk(hs, j, 0) - blk(hs, j - 1, 1) for j in range(1, NB)]
                hi = [blk(hs, 0, 1)] + [blk(hs, j, 1) + blk(hs, j - 1, 0) for j in range(1, NB)]
                zs = []
                for c in range(NB):
                    zr = zi = None
                    for a in range(c + 1):
                        j = c - a
                        tr = xr[a] * hr[j] - xi[a] * hi[j]
                        ti = xr[a] * hi[j] + xi[a] * hr[j]
                        zr = tr if zr is None else zr + tr
                        zi = ti if zi is None else zi + ti
                    zs.append(_lanecat([zr, zi]))
                return zs

            def a_inv(kv, zs):
                half = NB // 2
                fm = _bf(f_v[...])
                y = _rowcat([
                    _dot_nt(linked(_rowcat(zs[u * half:(u + 1) * half])).astype(BF16), fm)
                    for u in range(2)])
                qq = _bf(a_v[slot, 3]).astype(F32)
                dd = par_v[KS, a_rows, :]
                kvf = kv.astype(F32)
                for c in range(NB):
                    cs = slice(c * LANE, (c + 1) * LANE)
                    rs = slice(c * AR, (c + 1) * AR)
                    ra_t[a_rows, cs] = qq[:, cs] * (y[rs, :] * (1.0 / LANE) + kvf[rs, :] * dd)

            def proj(dst, which, r0, n):
                outs = []
                kw = C // 2
                for t in range(2):
                    acc = None
                    for u in range(2):
                        lhs = linked(c_v[_h(r0, n), pl.ds(u * kw, kw)])
                        w = wkv_v[h, _h(u * kw, kw), pl.ds(which * D + t * LANE, LANE)]
                        d = _dot(_bf(lhs), _bf(w))
                        set_link(d)
                        acc = d if acc is None else acc + d
                    outs.append(acc)
                dst[r0:r0 + n, :] = _lanecat(outs).astype(BF16)

            def qk(i):
                r0 = i * tq
                parts = [_dot_nt(_bf(linked(q_all[h, _h(r0, tq), :])), k_s[0:r0 + LANE, :])]
                if i > 0:
                    link[0] = _opaque_zero([parts[0][0:8, r0 - LANE:r0]])
                for j in range(1, nsub):
                    q = linked(q_all[h, _h(r0 + LANE * j, tq - LANE * j), :])
                    parts.append(_dot_nt(_bf(q), k_s[r0 + LANE * j:r0 + LANE * (j + 1), :]))
                set_link(parts[2], cfg["link_part"])
                return parts

            def softmax(i, parts):
                pb = p_s.at[i % 2]
                chain = _opaque_zero([b[b.shape[0] - 8:, b.shape[1] - LANE:] for b in parts])
                ls = []
                for a in range(nsub):
                    blocks = [parts[j][LANE * (a - j):LANE * (a - j + 1), :] for j in range(a + 1)]
                    last = blocks[-1]
                    w = last.shape[1]
                    dg = jnp.where(tri, last[:, w - LANE:], NEG)
                    blocks[-1] = dg if w == LANE else _lanecat([last[:, :w - LANE], dg])
                    sa = _lanecat(blocks)
                    mb = jnp.broadcast_to(jnp.max(sa, axis=1, keepdims=True), (LANE, LANE))
                    nt = sa.shape[1] // LANE
                    ptiles, psums = [], []
                    for g in range(0, LANE, 8):
                        mg = _pin(mb[g:g + 8, :], chain)
                        pg = [jnp.exp2(sa[g:g + 8, t * LANE:(t + 1) * LANE] - mg) for t in range(nt)]
                        ps = functools.reduce(jnp.add, pg)
                        chain = _opaque_zero([ps])
                        psums.append(ps)
                        ptiles.append(_lanecat(pg))
                    ls.append(jnp.sum(_rowcat(psums), axis=1, keepdims=True))
                    p = _pin(_rowcat(ptiles), link[0], 0, 0 if a == 0 else sa.shape[1] - LANE)
                    pb[LANE * a:LANE * (a + 1), 0:sa.shape[1]] = p.astype(BF16)
                return ls

            def pv(i, ls):
                r0 = i * tq
                pb = p_s.at[i % 2]
                ctx = [_dot(pb[:, 0:r0 + LANE], v_s[0:r0 + LANE, :])]
                for j in range(1, nsub):
                    ctx.append(_dot(pb[LANE * j:, r0 + LANE * j:r0 + LANE * (j + 1)],
                                    v_s[r0 + LANE * j:r0 + LANE * (j + 1), :]))
                set_link(ctx[2], cfg["link_part"])
                cs = []
                for a in range(nsub):
                    sl = lambda j: slice(LANE * (a - j), LANE * (a - j + 1))
                    r = pl.reciprocal(ls[a], approx=True)
                    r = r * (2.0 - ls[a] * r)
                    cs.append(functools.reduce(jnp.add, [ctx[j][sl(j)] for j in range(a + 1)]) * r)
                return _rowcat(cs).astype(BF16)

            def oproj(i, ctx):
                for u in range(tq // D):
                    res = _dot_nt(_bf(linked(wo_v[slot])), ctx[u * D:(u + 1) * D, :])
                    set_link(res)
                    c0 = i * tq + u * D
                    rb_t[:, c0:c0 + D] += res

            a_state = {}

            def a_hook(tag):
                if with_a and tag == cfg["a_fwd_at"]:
                    a_state["kv"], xs, hs = a_fwd()
                    a_state["zs"] = a_conv(xs, hs)
                if with_a and tag == cfg["a_inv_at"]:
                    a_inv(a_state["kv"], a_state["zs"])

            a_hook(0)
            proj(k_s, 0, 0, tq)
            a_hook(1)
            parts = qk(0)
            ctx_prev = None
            for i in range(nq):
                r0 = i * tq
                a_hook(10 * (i + 1))
                if ctx_prev is not None:
                    oproj(i - 1, ctx_prev)
                a_hook(10 * (i + 1) + 1)
                if i + 1 < nq:
                    proj(k_s, 0, r0 + tq, tq)
                a_hook(10 * (i + 1) + 2)
                proj(v_s, 1, r0, tq)
                a_hook(10 * (i + 1) + 3)
                ls = softmax(i, parts)
                ctx_prev = pv(i, ls)
                a_hook(10 * (i + 1) + 4)
                if i + 1 < nq:
                    parts = qk(i + 1)
            oproj(nq - 1, ctx_prev)
            return carry

        with jax.named_scope("loop_a"):
            lax.fori_loop(cfg["h0"], H, head_step, 0)
        with jax.named_scope("tail"):
            for i in range(S // D):
                cols = slice(i * D, (i + 1) * D)
                full = _rowcat([ra_t[AT * LANE:, cols], rb_t[:, cols]])
                out_v[cols, AT * LANE:] = full.T.astype(BF16)
                out_copy(i).start()
            for i in range(S // D + 1):
                out_copy(i).wait()

    scratch = [
        pltpu.VMEM((2, 4, AR // 2, S), U32),
        pltpu.VMEM((KS, M), BF16),
        pltpu.VMEM((M,), BF16),
        pltpu.VMEM((KS + 1, M, LANE), F32),
        pltpu.VMEM((LANE // 2, 2 * LANE), U32),
        pltpu.VMEM((MP // 2, S), U32),
        pltpu.VMEM((S // 2, MP), U32),
        pltpu.VMEM((S // 2, C), U32),
        pltpu.VMEM((4 * (M // 2) * 8, LANE), U32),
        pltpu.VMEM((H // 2, MP // 2, 2 * D), U32),
        pltpu.VMEM((2, 8 * (WCH // 2) * 8, LANE), U32),
        pltpu.VMEM((H, C // 2, 2 * D), U32),
        pltpu.VMEM((2, M // 2, D), U32),
        pltpu.VMEM((H, S // 2, D), U32),
        pltpu.VMEM((S, D), BF16),
        pltpu.VMEM((S, D), BF16),
        pltpu.VMEM((2, tq, S), BF16),
        pltpu.VMEM((M, S), F32),
        pltpu.VMEM((M, S), F32),
        pltpu.VMEM((S, 2 * M), BF16),
        pltpu.SemaphoreType.DMA((XC,)),
        pltpu.SemaphoreType.DMA((4 * WQC,)),
        pltpu.SemaphoreType.DMA((16,)),
        pltpu.SemaphoreType.DMA((QIT,)),
        pltpu.SemaphoreType.DMA((2,)),
        pltpu.SemaphoreType.DMA((10,)),
        pltpu.SemaphoreType.DMA((S // D + 1,)),
    ]
    return kernel, scratch


_DEFAULT = dict(wq_chunks=4, tq=512, a_fwd_at=1, a_inv_at=44,
                link_back=176, link_part=64, use_a=1, h0=0)


def _build(**kw):
    cfg = dict(_DEFAULT)
    cfg.update(kw)
    kernel, scratch = _make_kernel(cfg)

    def run(A_q, A_k, A_v, A_shift_k, A_ssm_k, A_ssm_D, B_x, B_c_kv, B_w_q, B_w_uk,
            B_w_uv, B_w_o):
        tr = lambda a: jnp.swapaxes(a, 1, 2).reshape(M, S)
        args = (
            tr(A_q), tr(A_k), tr(A_v), A_shift_k.T, A_ssm_k, A_ssm_D, tr(B_x),
            B_c_kv.reshape(S, C),
            B_w_q.reshape(M // 2, 2 * H, D), B_w_uk.reshape(C // 2, 2 * H, D),
            B_w_uv.reshape(C // 2, 2 * H, D),
            jnp.swapaxes(B_w_o, 1, 2),
        )
        out = pl.pallas_call(
            kernel,
            in_specs=[pl.BlockSpec(memory_space=pl.ANY)] * len(args),
            out_specs=pl.BlockSpec(memory_space=pl.ANY),
            out_shape=jax.ShapeDtypeStruct((S, 2 * M), BF16),
            scratch_shapes=scratch,
            compiler_params=pltpu.CompilerParams(
                vmem_limit_bytes=120 * 1024 * 1024,
                disable_bounds_checks=True),
        )(*args)
        return out.reshape(1, S, 2 * M)

    return run


_run = _build()


@jax.jit
def pallas_concat_heads__ssm_conv_h3__compressed_kv_cla__prompt_kernel(
    A_q: jax.Array,
    A_k: jax.Array,
    A_v: jax.Array,
    A_shift_k: jax.Array,
    A_ssm_k: jax.Array,
    A_ssm_D: jax.Array,
    B_x: jax.Array,
    B_c_kv: jax.Array,
    B_w_q: jax.Array,
    B_w_uk: jax.Array,
    B_w_uv: jax.Array,
    B_w_o: jax.Array,
):
    return _run(A_q, A_k, A_v, A_shift_k, A_ssm_k, A_ssm_D, B_x, B_c_kv, B_w_q,
                B_w_uk, B_w_uv, B_w_o)
```

```python
import functools

import jax
import jax.numpy as jnp
from jax import lax
import jax.experimental.pallas as pl
import jax.experimental.pallas.tpu as pltpu

F32 = jnp.float32
BF16 = jnp.bfloat16
U32 = jnp.uint32

S = 2048
M = 448
MP = 512
C = 1024
H = 16
D = 256
KS = 4
LANE = 128
NB = S // LANE
AR = 32
A_STEPS = M // AR
LOG2E = 1.4426950408889634
NEG = -1e30

NT = (((1,), (1,)), ((), ()))


def _dot(a, b):
    return jnp.dot(a, b, preferred_element_type=F32)


def _dot_nt(a, b):
    return lax.dot_general(a, b, NT, preferred_element_type=F32)


def _bf(x):
    return pltpu.bitcast(x, BF16)


def _u32(x):
    return pltpu.bitcast(x, U32)


def _h(r0, n):
    return pl.ds(r0 // 2, n // 2)


def _repack(ev, od):
    lo = (ev & jnp.uint32(0xFFFF)) | (od << 16)
    hi = (ev >> 16) | (od & jnp.uint32(0xFFFF0000))
    return lo, hi


def _opaque_zero(vals):
    acc = None
    for v in vals:
        b = v if v.dtype == U32 else pltpu.bitcast(v, U32)
        for r in range(0, b.shape[0], 8):
            for c in range(0, b.shape[1], LANE):
                t = b[r:r + 8, c:c + LANE]
                acc = t if acc is None else acc | t
    return jnp.minimum((acc >> 1).astype(jnp.int32), 0)


def _pin(x, zero, r=0, c=0):
    t = pltpu.bitcast(pltpu.bitcast(x[r:r + 8, c:c + LANE], jnp.int32) + zero, x.dtype)
    row = ([x[r:r + 8, :c]] if c > 0 else []) + [t] + (
        [x[r:r + 8, c + LANE:]] if c + LANE < x.shape[1] else [])
    row = jnp.concatenate(row, axis=1) if len(row) > 1 else row[0]
    col = ([x[:r, :]] if r > 0 else []) + [row] + ([x[r + 8:, :]] if r + 8 < x.shape[0] else [])
    return jnp.concatenate(col, axis=0) if len(col) > 1 else col[0]


def _rowcat(xs):
    return jnp.concatenate(xs, axis=0) if len(xs) > 1 else xs[0]


def _lanecat(xs):
    return jnp.concatenate(xs, axis=1) if len(xs) > 1 else xs[0]


def _make_kernel(cfg):
    tq = cfg["tq"]
    nq = S // tq
    nsub = tq // LANE
    WQC = cfg["wq_chunks"]
    wq_pairs = M // 2 // WQC
    XC = 4
    x_cols = S // XC
    WP = 80
    QIT = 8
    AT = 3

    def kernel(aq_hbm, ak_hbm, av_hbm, sh_hbm, ssm_hbm, dd_hbm, x_hbm, c_hbm,
               wq_hbm, wk_hbm, wv_hbm, wo_hbm,
               out_hbm,
               a_v, sh_v, dd_v, par_v, f_v,
               xt_v, x_v, c_v, wqs_v, wq_v, ws_v, wkv_v, wo_v,
               q_all, k_s, v_s, p_s, ra_t, rb_t, out_v,
               sem_x, sem_wq, sem_w, sem_c, sem_s, sem_a, sem_out):
        x32, c32, wq32, wk32, wv32, wo32 = (
            r.bitcast(U32) for r in (x_hbm, c_hbm, wq_hbm, wk_hbm, wv_hbm, wo_hbm))
        a32 = [r.bitcast(U32) for r in (ak_hbm, av_hbm, ssm_hbm, aq_hbm)]

        def x_copy(i):
            return pltpu.make_async_copy(
                x32.at[:, pl.ds(i * x_cols, x_cols)],
                xt_v.at[pl.ds(0, M // 2), pl.ds(i * x_cols, x_cols)], sem_x.at[i])

        def wq_copy(i, par, half):
            k = 2 * par + half
            dst = wqs_v.reshape(4, M // 2, 8, LANE)
            rs = pl.ds(i * wq_pairs, wq_pairs)
            return pltpu.make_async_copy(
                wq32.at[rs, pl.ds(8 * par, 8), pl.ds(half * LANE, LANE)],
                dst.at[k, rs], sem_wq.at[4 * i + k])

        def w_rows(chunk):
            r0 = chunk * WP
            if isinstance(r0, int):
                return pl.ds(min(r0, C // 2 - WP), WP)
            return pl.ds(pl.multiple_of(jnp.minimum(r0, C // 2 - WP), 8), WP)

        def w_copies(chunk, slot):
            dst = ws_v.reshape(16, WP, 8, LANE)
            rs = w_rows(chunk)
            out = []
            for which, src in enumerate((wk32, wv32)):
                for par in range(2):
                    for half in range(2):
                        k = 8 * slot + 4 * which + 2 * par + half
                        out.append(pltpu.make_async_copy(
                            src.at[rs, pl.ds(8 * par, 8), pl.ds(half * LANE, LANE)],
                            dst.at[k], sem_w.at[k]))
            return out

        def c_copy(it):
            n = S // 2 // QIT
            rs = pl.ds(pl.multiple_of(it * n, n), n)
            return pltpu.make_async_copy(c32.at[rs], c_v.at[rs], sem_c.at[it])

        def step_copies(h):
            slot = h % 2
            out = [pltpu.make_async_copy(wo32.at[h], wo_v.at[slot], sem_a.at[5 * slot])]
            n = AR // 2
            rs = pl.ds(pl.multiple_of(jnp.minimum(h, A_STEPS - 1) * n, n), n)
            for k in range(4):
                out.append(pltpu.make_async_copy(
                    a32[k].at[rs], a_v.at[slot, k], sem_a.at[5 * slot + 1 + k]))
            return out

        small = [pltpu.make_async_copy(sh_hbm, sh_v, sem_s.at[0]),
                 pltpu.make_async_copy(dd_hbm, dd_v, sem_s.at[1])]

        link = [None]

        def set_link(res, row=None):
            if row is None:
                row = res.shape[0] - cfg["link_back"]
            link[0] = _opaque_zero([res[row:row + 8, res.shape[1] - LANE:]])

        def linked(x):
            return x if link[0] is None or cfg["dbg"] & 2 else _pin(x, link[0])

        with jax.named_scope("first_starts"):
            for cp in small:
                cp.start()
        x_copy(0).start()
        for i in range(WQC):
            for k in range(4):
                wq_copy(i, k // 2, k % 2).start()

        bi = lax.broadcasted_iota(jnp.int32, (LANE, LANE), 0)
        mi = lax.broadcasted_iota(jnp.int32, (LANE, LANE), 1)
        ph = ((4 * mi + 1) * bi) & 511
        ang = ph.astype(F32) * (2.0 * 3.141592653589793 / 512.0)
        f_v[:, 0:LANE] = _u32(jnp.cos(ang).astype(BF16))
        f_v[:, LANE:] = _u32((-jnp.sin(ang)).astype(BF16))

        rb_t[...] = jnp.zeros((M, S), F32)
        xt_v[M // 2:, :] = jnp.zeros(((MP - M) // 2, S), U32)
        wq_v[:, M // 2:, :] = jnp.zeros((H // 2, (MP - M) // 2, 2 * D), U32)

        with jax.named_scope("small_wait"):
            for cp in small:
                cp.wait()
        sh = sh_v[...].astype(F32)
        for j in range(KS):
            par_v[j] = jnp.broadcast_to(sh[j:j + 1, :], (LANE, M)).T
        dd = dd_v[...].astype(F32).reshape(1, M)
        par_v[KS] = jnp.broadcast_to(dd, (LANE, M)).T

        def x_transpose(i):
            xt = _bf(xt_v[:, pl.ds(i * x_cols, x_cols)])
            x_v[_h(i * x_cols, x_cols), :] = _u32(xt.astype(F32).T.astype(BF16))

        x_copy(0).wait()
        x_transpose(0)
        for i in range(WQC):
            if i == WQC - cfg["x_early"]:
                for i2 in range(1, XC):
                    x_copy(i2).start()
            with jax.named_scope("wq_wait"):
                for k in range(4):
                    wq_copy(i, k // 2, k % 2).wait()
            rows = pl.ds(i * wq_pairs, wq_pairs)
            for half in range(2):
                for j in range(H // 2):
                    ev, od = (
                        wqs_v[pl.ds((2 * par + half) * (M // 2) * 8 + i * wq_pairs * 8 + j,
                                    wq_pairs, stride=8), :] for par in range(2))
                    lo, hi = _repack(ev, od)
                    wq_v[j, rows, pl.ds(half * LANE, LANE)] = lo
                    wq_v[j, rows, pl.ds(D + half * LANE, LANE)] = hi

        def unpack(chunk, slot, which, half, j):
            ev, od = (
                ws_v[slot, pl.ds((4 * which + 2 * par + half) * WP * 8 + j, WP, stride=8), :]
                for par in range(2))
            lo, hi = _repack(ev, od)
            rows = w_rows(chunk)
            cols = pl.ds(which * D + half * LANE, LANE)
            wkv_v[2 * j, rows, cols] = lo
            wkv_v[2 * j + 1, rows, cols] = hi
            return [lo, hi]

        units = [(w_, h_, j_) for w_ in range(2) for h_ in range(2) for j_ in range(H // 2)]

        def qproj(it, r0, n, t, zeros=(None, None)):
            outs = []
            for u in range(2):
                lhs = _bf(linked(x_v[_h(r0, n), :]))
                d = _dot(lhs, _bf(wq_v[it, :, pl.ds(t * D + u * LANE, LANE)]))
                set_link(d)
                if zeros[u] is not None:
                    for k, z in enumerate(zeros[u]):
                        d = _pin(d, z, 8 * ((k * (n // 8)) // len(zeros[u])))
                outs.append(d)
            q2 = _lanecat(outs)
            q_all[2 * it + t, _h(r0, n), :] = _u32((q2 * (D ** -0.5 * LOG2E)).astype(BF16))

        def q_pieces(it, chunk, slot, pieces):
            per = len(units) // (2 * len(pieces))
            grp = cfg["unp_grp"]
            for k, (pc, t) in enumerate(pieces):
                zeros = []
                for u in range(2):
                    mine = units[(2 * k + u) * per:(2 * k + u + 1) * per]
                    zeros.append([
                        _opaque_zero(sum([unpack(chunk, slot, *u_) for u_ in mine[g:g + grp]], []))
                        for g in range(0, per, grp)])
                qproj(it, pc * x_cols, x_cols, t, zeros)

        for t in range(2):
            qproj(0, 0, x_cols, t)
        for cp in w_copies(0, 0):
            cp.start()
        with jax.named_scope("x_wait"):
            for i in range(1, XC):
                x_copy(i).wait()
        link[0] = None
        for i in range(1, XC):
            x_transpose(i)
        for i in range(1, XC):
            for t in range(2):
                qproj(0, i * x_cols, x_cols, t)
        for cp in w_copies(1, 1):
            cp.start()
        c_copy(0).start()

        def q_body(it, carry):
            slot = (it - 1) % 2
            with jax.named_scope("w_wait"):
                for cp in w_copies(0, slot):
                    cp.wait()
            c_copy(it).start()
            link[0] = None
            q_pieces(it, it - 1, slot, [(pc, t) for pc in range(XC) for t in range(2)])

            @pl.when(it + 2 < QIT)
            def _():
                for cp in w_copies(it + 1, slot):
                    cp.start()
            return carry

        for cp in step_copies(0):
            cp.start()
        with jax.named_scope("q_loop"):
            lax.fori_loop(1, QIT, q_body, 0)
        for it in range(QIT):
            c_copy(it).wait()

        tri = (lax.broadcasted_iota(jnp.int32, (LANE, LANE), 1)
               <= lax.broadcasted_iota(jnp.int32, (LANE, LANE), 0))

        def out_copy(i):
            if i == S // D:
                cs = pl.ds(0, AT * LANE)
                return pltpu.make_async_copy(out_v.at[:, cs], out_hbm.at[:, cs], sem_out.at[i])
            rs, cs = pl.ds(i * D, D), pl.ds(AT * LANE, 2 * M - AT * LANE)
            return pltpu.make_async_copy(out_v.at[rs, cs], out_hbm.at[rs, cs], sem_out.at[i])

        def a_out():
            for i in range(S // tq):
                cols = slice(i * tq, (i + 1) * tq)
                out_v[cols, 0:AT * LANE] = ra_t[0:AT * LANE, cols].T.astype(BF16)
            out_copy(S // D).start()

        def head_step(h, carry):
            slot = h % 2
            with_a = cfg["use_a"]

            if cfg["a_out"] == 0:
                pl.when(h == A_STEPS)(a_out)

            if not cfg["no_step_dma"]:
                for cp in step_copies(h):
                    cp.wait()

                @pl.when(h + 1 < H)
                def _():
                    for cp in step_copies(h + 1):
                        cp.start()
            link[0] = None

            a_rows = pl.ds(pl.multiple_of(jnp.minimum(h, A_STEPS - 1) * AR, AR), AR)

            def a_fwd():
                kk = _bf(a_v[slot, 0]).astype(F32)
                lane = lax.broadcasted_iota(jnp.int32, (AR, LANE), 1)
                coef = [par_v[j, a_rows, :] for j in range(KS)]
                rolled = [kk] + [pltpu.roll(kk, j, 1) for j in range(1, KS)]
                vv = _bf(a_v[slot, 1]).astype(F32)
                kv_blocks = []
                for a in range(NB):
                    cs = slice(a * LANE, (a + 1) * LANE)
                    acc = rolled[0][:, cs] * coef[0]
                    for j in range(1, KS):
                        t = rolled[j][:, cs]
                        if a == 0:
                            t = jnp.where(lane >= j, t, 0.0)
                        acc = acc + t * coef[j]
                    kv_blocks.append(acc * vv[:, cs])
                hk = a_v[slot, 2]
                hk = _rowcat([hk[:, a * LANE:(a + 1) * LANE] for a in range(NB)])
                fm = _bf(f_v[...])
                hs = _dot(_bf(linked(hk)), fm)
                kv = linked(_rowcat(kv_blocks)).astype(BF16)
                xs = _dot(kv, fm)
                set_link(xs)
                return kv, xs, hs

            def a_conv(xs, hs):
                blk = lambda v, a, part: v[a * AR:(a + 1) * AR, part * LANE:(part + 1) * LANE]
                xr = [blk(xs, a, 0) for a in range(NB)]
                xi = [blk(xs, a, 1) for a in range(NB)]
                hr = [blk(hs, 0, 0)] + [blk(hs, j, 0) - blk(hs, j - 1, 1) for j in range(1, NB)]
                hi = [blk(hs, 0, 1)] + [blk(hs, j, 1) + blk(hs, j - 1, 0) for j in range(1, NB)]
                def z_of(c, prev):
                    zr = zi = None if prev is None else pltpu.bitcast(prev, F32)
                    for a in range(c + 1):
                        j = c - a
                        tr = xr[a] * hr[j] - xi[a] * hi[j]
                        ti = xr[a] * hi[j] + xi[a] * hr[j]
                        zr = tr if zr is None else zr + tr
                        zi = ti if zi is None else zi + ti
                    return _lanecat([zr, zi])
                return z_of

            def a_inv(kv, z_of, cs_):
                half = len(cs_) // 2
                fm = _bf(f_v[...])
                zs, prev = [], None
                for c in cs_:
                    zs.append(z_of(c, prev))
                    if cfg["a_serial"]:
                        prev = jnp.concatenate([_opaque_zero([zs[-1]])] * (AR // 8), axis=0)
                y = _rowcat([
                    _dot_nt(linked(_rowcat(zs[u * half:(u + 1) * half])).astype(BF16), fm)
                    for u in range(2)])
                dd = par_v[KS, a_rows, :]
                for k, c in enumerate(cs_):
                    cs = slice(c * LANE, (c + 1) * LANE)
                    qq = _bf(a_v[slot, 3, :, cs]).astype(F32)
                    kvf = kv[c * AR:(c + 1) * AR, :].astype(F32)
                    ra_t[a_rows, cs] = qq * (y[k * AR:(k + 1) * AR, :] * (1.0 / LANE) + kvf * dd)

            def proj(dst, which, r0, n):
                outs = []
                kw = C // 2
                for t in range(2):
                    acc = None
                    for u in range(2):
                        lhs = linked(c_v[_h(r0, n), pl.ds(u * kw, kw)])
                        w = wkv_v[h, _h(u * kw, kw), pl.ds(which * D + t * LANE, LANE)]
                        d = _dot(_bf(lhs), _bf(w))
                        set_link(d)
                        acc = d if acc is None else acc + d
                    outs.append(acc)
                dst[r0:r0 + n, :] = _lanecat(outs).astype(BF16)

            def qk(i):
                r0 = i * tq
                parts = [_dot_nt(_bf(linked(q_all[h, _h(r0, tq), :])), k_s[0:r0 + LANE, :])]
                if i > 0:
                    link[0] = _opaque_zero([parts[0][0:8, r0 - LANE:r0]])
                for j in range(1, nsub):
                    q = linked(q_all[h, _h(r0 + LANE * j, tq - LANE * j), :])
                    parts.append(_dot_nt(_bf(q), k_s[r0 + LANE * j:r0 + LANE * (j + 1), :]))
                set_link(parts[2], cfg["link_part"])
                return parts

            def softmax(i, parts):
                pb = p_s.at[i % 2]
                chain = _opaque_zero([b[b.shape[0] - 8:, b.shape[1] - LANE:] for b in parts])
                ls = []
                for a in range(nsub):
                    blocks = [parts[j][LANE * (a - j):LANE * (a - j + 1), :] for j in range(a + 1)]
                    last = blocks[-1]
                    w = last.shape[1]
                    dg = jnp.where(tri, last[:, w - LANE:], NEG)
                    blocks[-1] = dg if w == LANE else _lanecat([last[:, :w - LANE], dg])
                    sa = _lanecat(blocks)
                    mb = jnp.broadcast_to(jnp.max(sa, axis=1, keepdims=True), (LANE, LANE))
                    nt = sa.shape[1] // LANE
                    ptiles, psums = [], []
                    for g in range(0, LANE, 8):
                        mg = _pin(mb[g:g + 8, :], chain)
                        pg = [jnp.exp2(sa[g:g + 8, t * LANE:(t + 1) * LANE] - mg) for t in range(nt)]
                        ps = functools.reduce(jnp.add, pg)
                        chain = _opaque_zero([ps])
                        psums.append(ps)
                        ptiles.append(_lanecat(pg))
                    ls.append(jnp.sum(_rowcat(psums), axis=1, keepdims=True))
                    p = _pin(_rowcat(ptiles), link[0], 0, 0 if a == 0 else sa.shape[1] - LANE)
                    pb[LANE * a:LANE * (a + 1), 0:sa.shape[1]] = p.astype(BF16)
                return ls

            def pv(i, ls):
                r0 = i * tq
                pb = p_s.at[i % 2]
                ctx = [_dot(pb[:, 0:r0 + LANE], v_s[0:r0 + LANE, :])]
                for j in range(1, nsub):
                    ctx.append(_dot(pb[LANE * j:, r0 + LANE * j:r0 + LANE * (j + 1)],
                                    v_s[r0 + LANE * j:r0 + LANE * (j + 1), :]))
                set_link(ctx[2], cfg["link_part"])
                cs = []
                for a in range(nsub):
                    sl = lambda j: slice(LANE * (a - j), LANE * (a - j + 1))
                    r = pl.reciprocal(ls[a], approx=True)
                    r = r * (2.0 - ls[a] * r)
                    cs.append(functools.reduce(jnp.add, [ctx[j][sl(j)] for j in range(a + 1)]) * r)
                return _rowcat(cs).astype(BF16)

            def oproj(i, ctx):
                for u in range(tq // D):
                    res = _dot_nt(_bf(linked(wo_v[slot])), ctx[u * D:(u + 1) * D, :])
                    set_link(res)
                    c0 = i * tq + u * D
                    rb_t[:, c0:c0 + D] += res

            a_state = {}

            inv_at = cfg["a_inv_at"]
            ngrp = len(inv_at)
            if cfg["a_balance"]:
                order = [c for k in range(NB // 2) for c in (k, NB - 1 - k)]
                groups = [sorted(order[g * (NB // ngrp):(g + 1) * (NB // ngrp)]) for g in range(ngrp)]
            else:
                groups = [list(range(g * (NB // ngrp), (g + 1) * (NB // ngrp))) for g in range(ngrp)]

            def a_hook(tag):
                if with_a and tag == cfg["a_fwd_at"]:
                    a_state["kv"], xs, hs = a_fwd()
                    a_state["z_of"] = a_conv(xs, hs)
                if with_a and tag in inv_at:
                    a_inv(a_state["kv"], a_state["z_of"], groups[inv_at.index(tag)])

            a_hook(0)
            proj(k_s, 0, 0, tq)
            a_hook(1)
            parts = qk(0)
            ctx_prev = None
            for i in range(nq):
                r0 = i * tq
                a_hook(10 * (i + 1))
                if ctx_prev is not None:
                    oproj(i - 1, ctx_prev)
                a_hook(10 * (i + 1) + 1)
                if i + 1 < nq:
                    proj(k_s, 0, r0 + tq, tq)
                a_hook(10 * (i + 1) + 2)
                proj(v_s, 1, r0, tq)
                a_hook(10 * (i + 1) + 3)
                ls = softmax(i, parts)
                ctx_prev = pv(i, ls)
                a_hook(10 * (i + 1) + 4)
                if i + 1 < nq:
                    parts = qk(i + 1)
            oproj(nq - 1, ctx_prev)
            return carry

        if cfg["no_step_dma"]:
            for cp in step_copies(0):
                cp.wait()
        with jax.named_scope("loop_a"):
            lax.fori_loop(cfg["h0"], H, head_step, 0)
        with jax.named_scope("tail"):
            if cfg["a_out"] == 1:
                a_out()
            for i in range(S // D):
                cols = slice(i * D, (i + 1) * D)
                full = _rowcat([ra_t[AT * LANE:, cols], rb_t[:, cols]])
                out_v[cols, AT * LANE:] = full.T.astype(BF16)
                out_copy(i).start()
            for i in range(S // D + 1):
                out_copy(i).wait()

    scratch = [
        pltpu.VMEM((2, 4, AR // 2, S), U32),
        pltpu.VMEM((KS, M), BF16),
        pltpu.VMEM((M,), BF16),
        pltpu.VMEM((KS + 1, M, LANE), F32),
        pltpu.VMEM((LANE // 2, 2 * LANE), U32),
        pltpu.VMEM((MP // 2, S), U32),
        pltpu.VMEM((S // 2, MP), U32),
        pltpu.VMEM((S // 2, C), U32),
        pltpu.VMEM((4 * (M // 2) * 8, LANE), U32),
        pltpu.VMEM((H // 2, MP // 2, 2 * D), U32),
        pltpu.VMEM((2, 8 * WP * 8, LANE), U32),
        pltpu.VMEM((H, C // 2, 2 * D), U32),
        pltpu.VMEM((2, M // 2, D), U32),
        pltpu.VMEM((H, S // 2, D), U32),
        pltpu.VMEM((S, D), BF16),
        pltpu.VMEM((S, D), BF16),
        pltpu.VMEM((2, tq, S), BF16),
        pltpu.VMEM((M, S), F32),
        pltpu.VMEM((M, S), F32),
        pltpu.VMEM((S, 2 * M), BF16),
        pltpu.SemaphoreType.DMA((XC,)),
        pltpu.SemaphoreType.DMA((4 * WQC,)),
        pltpu.SemaphoreType.DMA((16,)),
        pltpu.SemaphoreType.DMA((QIT,)),
        pltpu.SemaphoreType.DMA((2,)),
        pltpu.SemaphoreType.DMA((10,)),
        pltpu.SemaphoreType.DMA((S // D + 1,)),
    ]
    return kernel, scratch


_DEFAULT = dict(wq_chunks=7, tq=512, a_fwd_at=13, a_inv_at=(44,), no_step_dma=0, a_out=0, dbg=0, unp_grp=1, x_early=3, a_serial=0, a_balance=1,
                link_back=176, link_part=32, use_a=1, h0=0)


def _build(**kw):
    cfg = dict(_DEFAULT)
    cfg.update(kw)
    kernel, scratch = _make_kernel(cfg)

    def run(A_q, A_k, A_v, A_shift_k, A_ssm_k, A_ssm_D, B_x, B_c_kv, B_w_q, B_w_uk,
            B_w_uv, B_w_o):
        tr = lambda a: jnp.swapaxes(a, 1, 2).reshape(M, S)
        args = (
            tr(A_q), tr(A_k), tr(A_v), A_shift_k.T, A_ssm_k, A_ssm_D, tr(B_x),
            B_c_kv.reshape(S, C),
            B_w_q.reshape(M // 2, 2 * H, D), B_w_uk.reshape(C // 2, 2 * H, D),
            B_w_uv.reshape(C // 2, 2 * H, D),
            jnp.swapaxes(B_w_o, 1, 2),
        )
        out = pl.pallas_call(
            kernel,
            in_specs=[pl.BlockSpec(memory_space=pl.ANY)] * len(args),
            out_specs=pl.BlockSpec(memory_space=pl.ANY),
            out_shape=jax.ShapeDtypeStruct((S, 2 * M), BF16),
            scratch_shapes=scratch,
            compiler_params=pltpu.CompilerParams(
                vmem_limit_bytes=120 * 1024 * 1024,
                disable_bounds_checks=True),
        )(*args)
        return out.reshape(1, S, 2 * M)

    return run


_run = _build()


@jax.jit
def pallas_concat_heads__ssm_conv_h3__compressed_kv_cla__prompt_kernel(
    A_q: jax.Array,
    A_k: jax.Array,
    A_v: jax.Array,
    A_shift_k: jax.Array,
    A_ssm_k: jax.Array,
    A_ssm_D: jax.Array,
    B_x: jax.Array,
    B_c_kv: jax.Array,
    B_w_q: jax.Array,
    B_w_uk: jax.Array,
    B_w_uv: jax.Array,
    B_w_o: jax.Array,
):
    return _run(A_q, A_k, A_v, A_shift_k, A_ssm_k, A_ssm_D, B_x, B_c_kv, B_w_q,
                B_w_uk, B_w_uv, B_w_o)
```

```python
import functools

import jax
import jax.numpy as jnp
from jax import lax
import jax.experimental.pallas as pl
import jax.experimental.pallas.tpu as pltpu

F32 = jnp.float32
BF16 = jnp.bfloat16
U32 = jnp.uint32

S = 2048
M = 448
MP = 512
C = 1024
H = 16
D = 256
KS = 4
LANE = 128
NB = S // LANE
AR = 32
A_STEPS = M // AR
LOG2E = 1.4426950408889634
NEG = -1e30

NT = (((1,), (1,)), ((), ()))


def _dot(a, b):
    return jnp.dot(a, b, preferred_element_type=F32)


def _dot_nt(a, b):
    return lax.dot_general(a, b, NT, preferred_element_type=F32)


def _bf(x):
    return pltpu.bitcast(x, BF16)


def _u32(x):
    return pltpu.bitcast(x, U32)


def _h(r0, n):
    return pl.ds(r0 // 2, n // 2)


def _repack(ev, od):
    lo = (ev & jnp.uint32(0xFFFF)) | (od << 16)
    hi = (ev >> 16) | (od & jnp.uint32(0xFFFF0000))
    return lo, hi


def _opaque_zero(vals):
    acc = None
    for v in vals:
        b = v if v.dtype == U32 else pltpu.bitcast(v, U32)
        for r in range(0, b.shape[0], 8):
            for c in range(0, b.shape[1], LANE):
                t = b[r:r + 8, c:c + LANE]
                acc = t if acc is None else acc | t
    return jnp.minimum((acc >> 1).astype(jnp.int32), 0)


def _pin(x, zero, r=0, c=0):
    t = pltpu.bitcast(pltpu.bitcast(x[r:r + 8, c:c + LANE], jnp.int32) + zero, x.dtype)
    row = ([x[r:r + 8, :c]] if c > 0 else []) + [t] + (
        [x[r:r + 8, c + LANE:]] if c + LANE < x.shape[1] else [])
    row = jnp.concatenate(row, axis=1) if len(row) > 1 else row[0]
    col = ([x[:r, :]] if r > 0 else []) + [row] + ([x[r + 8:, :]] if r + 8 < x.shape[0] else [])
    return jnp.concatenate(col, axis=0) if len(col) > 1 else col[0]


def _rowcat(xs):
    return jnp.concatenate(xs, axis=0) if len(xs) > 1 else xs[0]


def _lanecat(xs):
    return jnp.concatenate(xs, axis=1) if len(xs) > 1 else xs[0]


def _make_kernel(cfg):
    tq = cfg["tq"]
    nq = S // tq
    nsub = tq // LANE
    WQC = cfg["wq_chunks"]
    wq_pairs = M // 2 // WQC
    XC = 4
    x_cols = S // XC
    WP = 80
    QIT = 8
    AT = 3

    def kernel(aq_hbm, ak_hbm, av_hbm, sh_hbm, ssm_hbm, dd_hbm, x_hbm, c_hbm,
               wq_hbm, wk_hbm, wv_hbm, wo_hbm,
               out_hbm,
               a_v, sh_v, dd_v, par_v, f_v,
               xt_v, x_v, c_v, wqs_v, wq_v, ws_v, wkv_v, wo_v,
               q_all, k_s, v_s, p_s, ra_t, rb_t, out_v,
               sem_x, sem_wq, sem_w, sem_c, sem_s, sem_a, sem_out):
        x32, c32, wq32, wk32, wv32, wo32 = (
            r.bitcast(U32) for r in (x_hbm, c_hbm, wq_hbm, wk_hbm, wv_hbm, wo_hbm))
        a32 = [r.bitcast(U32) for r in (ak_hbm, av_hbm, ssm_hbm, aq_hbm)]

        def x_copy(i):
            return pltpu.make_async_copy(
                x32.at[:, pl.ds(i * x_cols, x_cols)],
                xt_v.at[pl.ds(0, M // 2), pl.ds(i * x_cols, x_cols)], sem_x.at[i])

        def wq_copy(i, par, half):
            k = 2 * par + half
            dst = wqs_v.reshape(4, M // 2, 8, LANE)
            rs = pl.ds(i * wq_pairs, wq_pairs)
            return pltpu.make_async_copy(
                wq32.at[rs, pl.ds(8 * par, 8), pl.ds(half * LANE, LANE)],
                dst.at[k, rs], sem_wq.at[4 * i + k])

        def w_rows(chunk):
            r0 = chunk * WP
            if isinstance(r0, int):
                return pl.ds(min(r0, C // 2 - WP), WP)
            return pl.ds(pl.multiple_of(jnp.minimum(r0, C // 2 - WP), 8), WP)

        def w_copies(chunk, slot):
            dst = ws_v.reshape(16, WP, 8, LANE)
            rs = w_rows(chunk)
            out = []
            for which, src in enumerate((wk32, wv32)):
                for par in range(2):
                    for half in range(2):
                        k = 8 * slot + 4 * which + 2 * par + half
                        out.append(pltpu.make_async_copy(
                            src.at[rs, pl.ds(8 * par, 8), pl.ds(half * LANE, LANE)],
                            dst.at[k], sem_w.at[k]))
            return out

        def c_copy(it):
            n = S // 2 // QIT
            rs = pl.ds(pl.multiple_of(it * n, n), n)
            return pltpu.make_async_copy(c32.at[rs], c_v.at[rs], sem_c.at[it])

        def step_copies(h):
            slot = h % 2
            out = [pltpu.make_async_copy(wo32.at[h], wo_v.at[slot], sem_a.at[2 * slot])]
            n = AR // 2
            rs = pl.ds(pl.multiple_of(jnp.minimum(h, A_STEPS - 1) * n, n), n)
            for k in range(4):
                out.append(pltpu.make_async_copy(
                    a32[k].at[rs], a_v.at[slot, k], sem_a.at[2 * slot + 1]))
            return out

        def step_wait(h):
            slot = h % 2
            pltpu.make_async_copy(wo_v.at[slot], wo_v.at[slot], sem_a.at[2 * slot]).wait()
            pltpu.make_async_copy(a_v.at[slot], a_v.at[slot], sem_a.at[2 * slot + 1]).wait()

        small = [pltpu.make_async_copy(sh_hbm, sh_v, sem_s.at[0]),
                 pltpu.make_async_copy(dd_hbm, dd_v, sem_s.at[1])]

        link = [None]

        def set_link(res, row=None):
            if row is None:
                row = res.shape[0] - cfg["link_back"]
            link[0] = _opaque_zero([res[row:row + 8, res.shape[1] - LANE:]])

        def linked(x):
            return x if link[0] is None or cfg["dbg"] & 2 else _pin(x, link[0])

        with jax.named_scope("first_starts"):
            for cp in small:
                cp.start()
        x_copy(0).start()
        for i in range(WQC):
            for k in range(4):
                wq_copy(i, k // 2, k % 2).start()

        bi = lax.broadcasted_iota(jnp.int32, (LANE, LANE), 0)
        mi = lax.broadcasted_iota(jnp.int32, (LANE, LANE), 1)
        ph = ((4 * mi + 1) * bi) & 511
        ang = ph.astype(F32) * (2.0 * 3.141592653589793 / 512.0)
        f_v[:, 0:LANE] = _u32(jnp.cos(ang).astype(BF16))
        f_v[:, LANE:] = _u32((-jnp.sin(ang)).astype(BF16))

        rb_t[...] = jnp.zeros((M, S), F32)
        xt_v[M // 2:, :] = jnp.zeros(((MP - M) // 2, S), U32)
        wq_v[:, M // 2:, :] = jnp.zeros((H // 2, (MP - M) // 2, 2 * D), U32)

        with jax.named_scope("small_wait"):
            for cp in small:
                cp.wait()
        sh = sh_v[...].astype(F32)
        for j in range(KS):
            par_v[j] = jnp.broadcast_to(sh[j:j + 1, :], (LANE, M)).T
        dd = dd_v[...].astype(F32).reshape(1, M)
        par_v[KS] = jnp.broadcast_to(dd, (LANE, M)).T

        def x_transpose(i):
            xt = _bf(xt_v[:, pl.ds(i * x_cols, x_cols)])
            x_v[_h(i * x_cols, x_cols), :] = _u32(xt.astype(F32).T.astype(BF16))

        x_copy(0).wait()
        x_transpose(0)
        for i in range(WQC):
            if i == WQC - cfg["x_early"]:
                for i2 in range(1, XC):
                    x_copy(i2).start()
            with jax.named_scope("wq_wait"):
                for k in range(4):
                    wq_copy(i, k // 2, k % 2).wait()
            rows = pl.ds(i * wq_pairs, wq_pairs)
            for half in range(2):
                for j in range(H // 2):
                    ev, od = (
                        wqs_v[pl.ds((2 * par + half) * (M // 2) * 8 + i * wq_pairs * 8 + j,
                                    wq_pairs, stride=8), :] for par in range(2))
                    lo, hi = _repack(ev, od)
                    wq_v[j, rows, pl.ds(half * LANE, LANE)] = lo
                    wq_v[j, rows, pl.ds(D + half * LANE, LANE)] = hi

        def unpack(chunk, slot, which, half, j):
            ev, od = (
                ws_v[slot, pl.ds((4 * which + 2 * par + half) * WP * 8 + j, WP, stride=8), :]
                for par in range(2))
            lo, hi = _repack(ev, od)
            rows = w_rows(chunk)
            cols = pl.ds(which * D + half * LANE, LANE)
            wkv_v[2 * j, rows, cols] = lo
            wkv_v[2 * j + 1, rows, cols] = hi
            return [lo, hi]

        units = [(w_, h_, j_) for w_ in range(2) for h_ in range(2) for j_ in range(H // 2)]

        def qproj(it, r0, n, t, zeros=(None, None)):
            outs = []
            for u in range(2):
                lhs = _bf(linked(x_v[_h(r0, n), :]))
                d = _dot(lhs, _bf(wq_v[it, :, pl.ds(t * D + u * LANE, LANE)]))
                set_link(d)
                if zeros[u] is not None:
                    for k, z in enumerate(zeros[u]):
                        d = _pin(d, z, 8 * ((k * (n // 8)) // len(zeros[u])))
                outs.append(d)
            q2 = _lanecat(outs)
            q_all[2 * it + t, _h(r0, n), :] = _u32((q2 * (D ** -0.5 * LOG2E)).astype(BF16))

        def q_pieces(it, chunk, slot, pieces):
            per = len(units) // (2 * len(pieces))
            grp = cfg["unp_grp"]
            for k, (pc, t) in enumerate(pieces):
                zeros = []
                for u in range(2):
                    mine = units[(2 * k + u) * per:(2 * k + u + 1) * per]
                    zeros.append([
                        _opaque_zero(sum([unpack(chunk, slot, *u_) for u_ in mine[g:g + grp]], []))
                        for g in range(0, per, grp)])
                qproj(it, pc * x_cols, x_cols, t, zeros)

        for t in range(2):
            qproj(0, 0, x_cols, t)
        for cp in w_copies(0, 0):
            cp.start()
        with jax.named_scope("x_wait"):
            for i in range(1, XC):
                x_copy(i).wait()
        link[0] = None
        for i in range(1, XC):
            x_transpose(i)
        for i in range(1, XC):
            for t in range(2):
                qproj(0, i * x_cols, x_cols, t)
        for cp in w_copies(1, 1):
            cp.start()
        c_copy(0).start()

        def q_body(it, carry):
            slot = (it - 1) % 2
            with jax.named_scope("w_wait"):
                for cp in w_copies(0, slot):
                    cp.wait()
            c_copy(it).start()
            link[0] = None
            q_pieces(it, it - 1, slot, [(pc, t) for pc in range(XC) for t in range(2)])

            @pl.when(it + 2 < QIT)
            def _():
                for cp in w_copies(it + 1, slot):
                    cp.start()
            return carry

        for cp in step_copies(0):
            cp.start()
        with jax.named_scope("q_loop"):
            lax.fori_loop(1, QIT, q_body, 0)
        for it in range(QIT):
            c_copy(it).wait()

        tri = (lax.broadcasted_iota(jnp.int32, (LANE, LANE), 1)
               <= lax.broadcasted_iota(jnp.int32, (LANE, LANE), 0))

        def out_copy(i):
            if i == S // D:
                cs = pl.ds(0, AT * LANE)
                return pltpu.make_async_copy(out_v.at[:, cs], out_hbm.at[:, cs], sem_out.at[i])
            rs, cs = pl.ds(i * D, D), pl.ds(AT * LANE, 2 * M - AT * LANE)
            return pltpu.make_async_copy(out_v.at[rs, cs], out_hbm.at[rs, cs], sem_out.at[i])

        def a_out():
            for i in range(S // tq):
                cols = slice(i * tq, (i + 1) * tq)
                out_v[cols, 0:AT * LANE] = ra_t[0:AT * LANE, cols].T.astype(BF16)
            out_copy(S // D).start()

        def head_step(h, carry):
            slot = h % 2
            with_a = cfg["use_a"]

            if cfg["a_out"] == 0:
                pl.when(h == A_STEPS)(a_out)

            step_wait(h)
            link[0] = None

            def prefetch():
                @pl.when(h + 1 < H)
                def _():
                    for cp in step_copies(h + 1):
                        cp.start()

            a_rows = pl.ds(pl.multiple_of(jnp.minimum(h, A_STEPS - 1) * AR, AR), AR)

            def a_fwd():
                kk = _bf(a_v[slot, 0]).astype(F32)
                lane = lax.broadcasted_iota(jnp.int32, (AR, LANE), 1)
                coef = [par_v[j, a_rows, :] for j in range(KS)]
                rolled = [kk] + [pltpu.roll(kk, j, 1) for j in range(1, KS)]
                vv = _bf(a_v[slot, 1]).astype(F32)
                kv_blocks = []
                for a in range(NB):
                    cs = slice(a * LANE, (a + 1) * LANE)
                    acc = rolled[0][:, cs] * coef[0]
                    for j in range(1, KS):
                        t = rolled[j][:, cs]
                        if a == 0:
                            t = jnp.where(lane >= j, t, 0.0)
                        acc = acc + t * coef[j]
                    kv_blocks.append(acc * vv[:, cs])
                hk = a_v[slot, 2]
                hk = _rowcat([hk[:, a * LANE:(a + 1) * LANE] for a in range(NB)])
                fm = _bf(f_v[...])
                hs = _dot(_bf(linked(hk)), fm)
                kv = linked(_rowcat(kv_blocks)).astype(BF16)
                xs = _dot(kv, fm)
                set_link(xs)
                return kv, xs, hs

            def a_conv(xs, hs):
                def tile(v, a, g, part):
                    r = a * AR + 8 * g
                    return v[r:r + 8, part * LANE:(part + 1) * LANE]

                z = {}
                nch = cfg["a_chains"]
                gates = [None] * nch
                width = cfg["a_width"]
                k = 0
                for g in range(AR // 8):
                    hr = [tile(hs, 0, g, 0)] + [
                        tile(hs, j, g, 0) - tile(hs, j - 1, g, 1) for j in range(1, NB)]
                    hi = [tile(hs, 0, g, 1)] + [
                        tile(hs, j, g, 1) + tile(hs, j - 1, g, 0) for j in range(1, NB)]
                    for c0 in range(0, NB, width):
                        ch = k % nch
                        k += 1
                        for a in range(c0 + width):
                            xr, xi = tile(xs, a, g, 0), tile(xs, a, g, 1)
                            if gates[ch] is not None and cfg["a_gate"]:
                                xr, xi = _pin(xr, gates[ch]), _pin(xi, gates[ch])
                            for c in range(max(c0, a), c0 + width):
                                j = c - a
                                tr = xr * hr[j] - xi * hi[j]
                                ti = xr * hi[j] + xi * hr[j]
                                z[c, g] = (tr, ti) if a == 0 else (z[c, g][0] + tr, z[c, g][1] + ti)
                            gates[ch] = _opaque_zero(list(z[c0 + width - 1, g]))
                return z

            def a_inv(kv, z):
                fm = _bf(f_v[...])
                ng = AR // 8
                ys = []
                for u in range(2):
                    rows = [_lanecat(z[c, g]) for g in range(u * ng // 2, (u + 1) * ng // 2)
                            for c in range(NB)]
                    ys.append(_dot_nt(linked(_rowcat(rows)).astype(BF16), fm))
                y = _rowcat(ys)
                dd = par_v[KS, a_rows, :]
                for c in range(NB):
                    cs = slice(c * LANE, (c + 1) * LANE)
                    yc = _rowcat([y[(g * NB + c) * 8:(g * NB + c + 1) * 8, :] for g in range(ng)])
                    qq = _bf(a_v[slot, 3, :, cs]).astype(F32)
                    kvf = kv[c * AR:(c + 1) * AR, :].astype(F32)
                    ra_t[a_rows, cs] = qq * (yc * (1.0 / LANE) + kvf * dd)

            def proj(dst, which, r0, n):
                outs = []
                kw = C // 2
                for t in range(2):
                    acc = None
                    for u in range(2):
                        lhs = linked(c_v[_h(r0, n), pl.ds(u * kw, kw)])
                        w = wkv_v[h, _h(u * kw, kw), pl.ds(which * D + t * LANE, LANE)]
                        d = _dot(_bf(lhs), _bf(w))
                        set_link(d)
                        acc = d if acc is None else acc + d
                    outs.append(acc)
                dst[r0:r0 + n, :] = _lanecat(outs).astype(BF16)

            def qk(i):
                r0 = i * tq
                parts = [_dot_nt(_bf(linked(q_all[h, _h(r0, tq), :])), k_s[0:r0 + LANE, :])]
                if i > 0:
                    link[0] = _opaque_zero([parts[0][0:8, r0 - LANE:r0]])
                for j in range(1, nsub):
                    q = linked(q_all[h, _h(r0 + LANE * j, tq - LANE * j), :])
                    parts.append(_dot_nt(_bf(q), k_s[r0 + LANE * j:r0 + LANE * (j + 1), :]))
                set_link(parts[2], cfg["link_part"])
                return parts

            def softmax(i, parts):
                pb = p_s.at[i % 2]
                chain = _opaque_zero([b[b.shape[0] - 8:, b.shape[1] - LANE:] for b in parts])
                ls = []
                for a in range(nsub):
                    blocks = [parts[j][LANE * (a - j):LANE * (a - j + 1), :] for j in range(a + 1)]
                    last = blocks[-1]
                    w = last.shape[1]
                    dg = jnp.where(tri, last[:, w - LANE:], NEG)
                    blocks[-1] = dg if w == LANE else _lanecat([last[:, :w - LANE], dg])
                    sa = _lanecat(blocks)
                    if cfg["dbg"] & 4:
                        ls.append(jnp.ones((LANE, 1), F32))
                        p = _pin(sa, link[0], 0, 0 if a == 0 else sa.shape[1] - LANE)
                        pb[LANE * a:LANE * (a + 1), 0:sa.shape[1]] = p.astype(BF16)
                        continue
                    mb = jnp.broadcast_to(jnp.max(sa, axis=1, keepdims=True), (LANE, LANE))
                    nt = sa.shape[1] // LANE
                    ptiles, psums = [], []
                    for g in range(0, LANE, 8):
                        mg = _pin(mb[g:g + 8, :], chain)
                        pg = [jnp.exp2(sa[g:g + 8, t * LANE:(t + 1) * LANE] - mg) for t in range(nt)]
                        ps = functools.reduce(jnp.add, pg)
                        chain = _opaque_zero([ps])
                        psums.append(ps)
                        ptiles.append(_lanecat(pg))
                    ls.append(jnp.sum(_rowcat(psums), axis=1, keepdims=True))
                    p = _pin(_rowcat(ptiles), link[0], 0, 0 if a == 0 else sa.shape[1] - LANE)
                    pb[LANE * a:LANE * (a + 1), 0:sa.shape[1]] = p.astype(BF16)
                return ls

            def pv(i, ls):
                r0 = i * tq
                pb = p_s.at[i % 2]
                ctx = [_dot(pb[:, 0:r0 + LANE], v_s[0:r0 + LANE, :])]
                for j in range(1, nsub):
                    ctx.append(_dot(pb[LANE * j:, r0 + LANE * j:r0 + LANE * (j + 1)],
                                    v_s[r0 + LANE * j:r0 + LANE * (j + 1), :]))
                set_link(ctx[2], cfg["link_part"])
                cs = []
                for a in range(nsub):
                    sl = lambda j: slice(LANE * (a - j), LANE * (a - j + 1))
                    r = pl.reciprocal(ls[a], approx=True)
                    r = r * (2.0 - ls[a] * r)
                    cs.append(functools.reduce(jnp.add, [ctx[j][sl(j)] for j in range(a + 1)]) * r)
                return _rowcat(cs).astype(BF16)

            def oproj(i, ctx):
                for u in range(tq // D):
                    res = _dot_nt(_bf(linked(wo_v[slot])), ctx[u * D:(u + 1) * D, :])
                    set_link(res)
                    c0 = i * tq + u * D
                    rb_t[:, c0:c0 + D] += res

            a_state = {}

            def a_hook(tag):
                if tag == cfg["pf_at"]:
                    prefetch()
                if with_a and tag == cfg["a_fwd_at"]:
                    a_state["kv"], xs, hs = a_fwd()
                    a_state["z"] = a_conv(xs, hs)
                if with_a and tag == cfg["a_inv_at"]:
                    a_inv(a_state["kv"], a_state["z"])

            import contextlib
            sc = (lambda n: jax.named_scope(n)) if cfg["dbg"] & 8 else (lambda n: contextlib.nullcontext())
            with sc("s_kp0"):
                a_hook(0)
                proj(k_s, 0, 0, tq)
                a_hook(1)
            with sc("s_qk"):
                parts = qk(0)
            ctx_prev = None
            for i in range(nq):
                r0 = i * tq
                with sc("s_mid"):
                    a_hook(10 * (i + 1))
                    if ctx_prev is not None:
                        oproj(i - 1, ctx_prev)
                    a_hook(10 * (i + 1) + 1)
                    if i + 1 < nq:
                        proj(k_s, 0, r0 + tq, tq)
                    a_hook(10 * (i + 1) + 2)
                    proj(v_s, 1, r0, tq)
                    a_hook(10 * (i + 1) + 3)
                    ls = softmax(i, parts)
                with sc("s_pv"):
                    ctx_prev = pv(i, ls)
                    a_hook(10 * (i + 1) + 4)
                if i + 1 < nq:
                    with sc("s_qk"):
                        parts = qk(i + 1)
            with sc("s_o"):
                oproj(nq - 1, ctx_prev)
            return carry

        with jax.named_scope("loop_a"):
            lax.fori_loop(cfg["h0"], H, head_step, 0)
        with jax.named_scope("tail"):
            if cfg["a_out"] == 1:
                a_out()
            for i in range(S // D):
                cols = slice(i * D, (i + 1) * D)
                full = _rowcat([ra_t[AT * LANE:, cols], rb_t[:, cols]])
                out_v[cols, AT * LANE:] = full.T.astype(BF16)
                out_copy(i).start()
            for i in range(S // D + 1):
                out_copy(i).wait()

    scratch = [
        pltpu.VMEM((2, 4, AR // 2, S), U32),
        pltpu.VMEM((KS, M), BF16),
        pltpu.VMEM((M,), BF16),
        pltpu.VMEM((KS + 1, M, LANE), F32),
        pltpu.VMEM((LANE // 2, 2 * LANE), U32),
        pltpu.VMEM((MP // 2, S), U32),
        pltpu.VMEM((S // 2, MP), U32),
        pltpu.VMEM((S // 2, C), U32),
        pltpu.VMEM((4 * (M // 2) * 8, LANE), U32),
        pltpu.VMEM((H // 2, MP // 2, 2 * D), U32),
        pltpu.VMEM((2, 8 * WP * 8, LANE), U32),
        pltpu.VMEM((H, C // 2, 2 * D), U32),
        pltpu.VMEM((2, M // 2, D), U32),
        pltpu.VMEM((H, S // 2, D), U32),
        pltpu.VMEM((S, D), BF16),
        pltpu.VMEM((S, D), BF16),
        pltpu.VMEM((2, tq, S), BF16),
        pltpu.VMEM((M, S), F32),
        pltpu.VMEM((M, S), F32),
        pltpu.VMEM((S, 2 * M), BF16),
        pltpu.SemaphoreType.DMA((XC,)),
        pltpu.SemaphoreType.DMA((4 * WQC,)),
        pltpu.SemaphoreType.DMA((16,)),
        pltpu.SemaphoreType.DMA((QIT,)),
        pltpu.SemaphoreType.DMA((2,)),
        pltpu.SemaphoreType.DMA((4,)),
        pltpu.SemaphoreType.DMA((S // D + 1,)),
    ]
    return kernel, scratch


_DEFAULT = dict(wq_chunks=7, tq=512, a_fwd_at=13, a_inv_at=44, pf_at=0, a_gate=1, a_chains=1, a_width=4, a_out=0, dbg=0, unp_grp=1, x_early=3,
                link_back=176, link_part=32, use_a=1, h0=0)


def _build(**kw):
    cfg = dict(_DEFAULT)
    cfg.update(kw)
    kernel, scratch = _make_kernel(cfg)

    def run(A_q, A_k, A_v, A_shift_k, A_ssm_k, A_ssm_D, B_x, B_c_kv, B_w_q, B_w_uk,
            B_w_uv, B_w_o):
        tr = lambda a: jnp.swapaxes(a, 1, 2).reshape(M, S)
        args = (
            tr(A_q), tr(A_k), tr(A_v), A_shift_k.T, A_ssm_k, A_ssm_D, tr(B_x),
            B_c_kv.reshape(S, C),
            B_w_q.reshape(M // 2, 2 * H, D), B_w_uk.reshape(C // 2, 2 * H, D),
            B_w_uv.reshape(C // 2, 2 * H, D),
            jnp.swapaxes(B_w_o, 1, 2),
        )
        out = pl.pallas_call(
            kernel,
            in_specs=[pl.BlockSpec(memory_space=pl.ANY)] * len(args),
            out_specs=pl.BlockSpec(memory_space=pl.ANY),
            out_shape=jax.ShapeDtypeStruct((S, 2 * M), BF16),
            scratch_shapes=scratch,
            compiler_params=pltpu.CompilerParams(
                vmem_limit_bytes=120 * 1024 * 1024,
                disable_bounds_checks=True),
        )(*args)
        return out.reshape(1, S, 2 * M)

    return run


_run = _build()


@jax.jit
def pallas_concat_heads__ssm_conv_h3__compressed_kv_cla__prompt_kernel(
    A_q: jax.Array,
    A_k: jax.Array,
    A_v: jax.Array,
    A_shift_k: jax.Array,
    A_ssm_k: jax.Array,
    A_ssm_D: jax.Array,
    B_x: jax.Array,
    B_c_kv: jax.Array,
    B_w_q: jax.Array,
    B_w_uk: jax.Array,
    B_w_uv: jax.Array,
    B_w_o: jax.Array,
):
    return _run(A_q, A_k, A_v, A_shift_k, A_ssm_k, A_ssm_D, B_x, B_c_kv, B_w_q,
                B_w_uk, B_w_uv, B_w_o)
```

```python
import functools

import jax
import jax.numpy as jnp
from jax import lax
import jax.experimental.pallas as pl
import jax.experimental.pallas.tpu as pltpu

F32 = jnp.float32
BF16 = jnp.bfloat16
U32 = jnp.uint32

S = 2048
M = 448
MP = 512
C = 1024
H = 16
D = 256
KS = 4
LANE = 128
NB = S // LANE
AR = 32
A_STEPS = M // AR
LOG2E = 1.4426950408889634
NEG = -1e30

NT = (((1,), (1,)), ((), ()))


def _dot(a, b):
    return jnp.dot(a, b, preferred_element_type=F32)


def _dot_nt(a, b):
    return lax.dot_general(a, b, NT, preferred_element_type=F32)


def _bf(x):
    return pltpu.bitcast(x, BF16)


def _u32(x):
    return pltpu.bitcast(x, U32)


def _h(r0, n):
    return pl.ds(r0 // 2, n // 2)


def _repack(ev, od):
    lo = (ev & jnp.uint32(0xFFFF)) | (od << 16)
    hi = (ev >> 16) | (od & jnp.uint32(0xFFFF0000))
    return lo, hi


def _opaque_zero(vals):
    acc = None
    for v in vals:
        b = v if v.dtype == U32 else pltpu.bitcast(v, U32)
        for r in range(0, b.shape[0], 8):
            for c in range(0, b.shape[1], LANE):
                t = b[r:r + 8, c:c + LANE]
                acc = t if acc is None else acc | t
    return jnp.minimum((acc >> 1).astype(jnp.int32), 0)


def _pin(x, zero, r=0, c=0):
    t = pltpu.bitcast(pltpu.bitcast(x[r:r + 8, c:c + LANE], jnp.int32) + zero, x.dtype)
    row = ([x[r:r + 8, :c]] if c > 0 else []) + [t] + (
        [x[r:r + 8, c + LANE:]] if c + LANE < x.shape[1] else [])
    row = jnp.concatenate(row, axis=1) if len(row) > 1 else row[0]
    col = ([x[:r, :]] if r > 0 else []) + [row] + ([x[r + 8:, :]] if r + 8 < x.shape[0] else [])
    return jnp.concatenate(col, axis=0) if len(col) > 1 else col[0]


def _rowcat(xs):
    return jnp.concatenate(xs, axis=0) if len(xs) > 1 else xs[0]


def _lanecat(xs):
    return jnp.concatenate(xs, axis=1) if len(xs) > 1 else xs[0]


def _make_kernel(cfg):
    tq = cfg["tq"]
    nq = S // tq
    nsub = tq // LANE
    KT = MP // LANE
    TP = LANE // 2
    XC = 4
    x_cols = S // XC
    WP = 64
    QIT = 8
    AT = 3

    def kernel(aq_hbm, ak_hbm, av_hbm, sh_hbm, ssm_hbm, dd_hbm, x_hbm, c_hbm,
               wq_hbm, wk_hbm, wv_hbm, wo_hbm,
               out_hbm,
               a_v, sh_v, dd_v, par_v, f_v,
               xt_v, x_v, c_v, wqs_v, wq_v, qacc, ws_v, wkv_v, wo_v,
               q_all, k_s, v_s, p_s, ra_t, rb_t, out_v,
               sem_x, sem_wq, sem_w, sem_c, sem_s, sem_a, sem_out):
        x32, c32, wq32, wk32, wv32, wo32 = (
            r.bitcast(U32) for r in (x_hbm, c_hbm, wq_hbm, wk_hbm, wv_hbm, wo_hbm))
        a32 = [r.bitcast(U32) for r in (ak_hbm, av_hbm, ssm_hbm, aq_hbm)]

        def x_copy(i):
            cs = pl.ds(i * x_cols, x_cols)
            return pltpu.make_async_copy(x32.at[:, cs], xt_v.at[:, cs], sem_x.at[i])

        def wq_copies(kt):
            dst = wqs_v.reshape(4 * KT, TP, 8, LANE)
            if isinstance(kt, int):
                rs = pl.ds(min(kt * TP, M // 2 - TP), TP)
            else:
                rs = pl.ds(kt * TP, TP)
            return [pltpu.make_async_copy(
                wq32.at[rs, pl.ds(8 * (k // 2), 8), pl.ds((k % 2) * LANE, LANE)],
                dst.at[4 * kt + k], sem_wq.at[4 * kt + k]) for k in range(4)]

        def w_rows(chunk):
            r0 = chunk * WP
            return pl.ds(r0 if isinstance(r0, int) else pl.multiple_of(r0, WP), WP)

        def w_copies(chunk, slot):
            dst = ws_v.reshape(16, WP, 8, LANE)
            rs = w_rows(chunk)
            out = []
            for which, src in enumerate((wk32, wv32)):
                for par in range(2):
                    for half in range(2):
                        k = 8 * slot + 4 * which + 2 * par + half
                        out.append(pltpu.make_async_copy(
                            src.at[rs, pl.ds(8 * par, 8), pl.ds(half * LANE, LANE)],
                            dst.at[k], sem_w.at[k]))
            return out

        def c_copy(it):
            n = S // 2 // QIT
            rs = pl.ds(pl.multiple_of(it * n, n), n)
            return pltpu.make_async_copy(c32.at[rs], c_v.at[rs], sem_c.at[it])

        def step_copies(h):
            slot = h % 2
            out = [pltpu.make_async_copy(wo32.at[h], wo_v.at[slot], sem_a.at[2 * slot])]
            n = AR // 2
            rs = pl.ds(pl.multiple_of(jnp.minimum(h, A_STEPS - 1) * n, n), n)
            for k in range(4):
                out.append(pltpu.make_async_copy(
                    a32[k].at[rs], a_v.at[slot, k], sem_a.at[2 * slot + 1]))
            return out

        def step_wait(h):
            slot = h % 2
            pltpu.make_async_copy(wo_v.at[slot], wo_v.at[slot], sem_a.at[2 * slot]).wait()
            pltpu.make_async_copy(a_v.at[slot], a_v.at[slot], sem_a.at[2 * slot + 1]).wait()

        small = [pltpu.make_async_copy(sh_hbm, sh_v, sem_s.at[0]),
                 pltpu.make_async_copy(dd_hbm, dd_v, sem_s.at[1])]

        link = [None]

        def set_link(res, row=None):
            if row is None:
                row = res.shape[0] - cfg["link_back"]
            link[0] = _opaque_zero([res[row:row + 8, res.shape[1] - LANE:]])

        def linked(x):
            return x if link[0] is None or cfg["dbg"] & 2 else _pin(x, link[0])

        with jax.named_scope("first_starts"):
            for cp in small:
                cp.start()
        x_copy(0).start()
        for kt in range(KT):
            for cp in wq_copies(kt):
                cp.start()

        bi = lax.broadcasted_iota(jnp.int32, (LANE, LANE), 0)
        mi = lax.broadcasted_iota(jnp.int32, (LANE, LANE), 1)
        ph = ((4 * mi + 1) * bi) & 511
        ang = ph.astype(F32) * (2.0 * 3.141592653589793 / 512.0)
        f_v[:, 0:LANE] = _u32(jnp.cos(ang).astype(BF16))
        f_v[:, LANE:] = _u32((-jnp.sin(ang)).astype(BF16))

        rb_t[...] = jnp.zeros((M, S), F32)

        with jax.named_scope("small_wait"):
            for cp in small:
                cp.wait()
        sh = sh_v[...].astype(F32)
        for j in range(KS):
            par_v[j] = jnp.broadcast_to(sh[j:j + 1, :], (LANE, M)).T
        dd = dd_v[...].astype(F32).reshape(1, M)
        par_v[KS] = jnp.broadcast_to(dd, (LANE, M)).T

        def x_transpose(i):
            xt = xt_v[:, pl.ds(i * x_cols, x_cols)]
            nfull = (KT - 1) * TP
            xt = _rowcat([xt[:nfull], jnp.zeros((MP // 2 - M // 2, x_cols), U32), xt[nfull:]])
            x_v[_h(i * x_cols, x_cols), :] = _u32(_bf(xt).astype(F32).T.astype(BF16))

        def q_early(kt, first, last):
            r0 = kt * TP
            rows = pl.ds(r0 if isinstance(r0, int) else pl.multiple_of(r0, TP), TP)
            c0 = kt * LANE
            cols = pl.ds(c0 if isinstance(c0, int) else pl.multiple_of(c0, LANE), LANE)
            link[0] = None
            for j in range(H // 2):
                ws = []
                for half in range(2):
                    ev, od = (
                        wqs_v[kt, pl.ds((2 * par + half) * TP * 8 + j, TP, stride=8), :]
                        for par in range(2))
                    ws.append(_repack(ev, od))
                w = _lanecat([ws[0][0], ws[1][0], ws[0][1], ws[1][1]])
                wq_v[j, rows, :] = w
                d = _dot(_bf(linked(x_v[_h(0, x_cols), cols])), _bf(w))
                set_link(d)
                if not first:
                    d = d + qacc[j]
                if last:
                    d = (d * (D ** -0.5 * LOG2E)).astype(BF16)
                    for t in range(2):
                        q_all[2 * j + t, _h(0, x_cols), :] = _u32(d[:, t * D:(t + 1) * D])
                else:
                    qacc[j] = d

        with jax.named_scope("x_wait"):
            x_copy(0).wait()
        x_transpose(0)
        with jax.named_scope("wq_wait"):
            for cp in wq_copies(0):
                cp.wait()
        q_early(0, True, False)
        for i in range(1, XC):
            x_copy(i).start()

        def early_body(kt, carry):
            with jax.named_scope("wq_wait"):
                for cp in wq_copies(kt):
                    cp.wait()
            q_early(kt, False, False)
            for cp in w_copies(kt - 1, kt - 1):
                cp.start()
            return carry

        lax.fori_loop(1, KT - 1, early_body, 0)
        with jax.named_scope("wq_wait"):
            for cp in wq_copies(KT - 1):
                cp.wait()
            for i in range(1, XC):
                x_copy(i).wait()
        q_early(KT - 1, False, True)
        for i in range(1, XC):
            x_transpose(i)

        def unpack(chunk, slot, which, half, j):
            ev, od = (
                ws_v[slot, pl.ds((4 * which + 2 * par + half) * WP * 8 + j, WP, stride=8), :]
                for par in range(2))
            lo, hi = _repack(ev, od)
            rows = w_rows(chunk)
            cols = pl.ds(which * D + half * LANE, LANE)
            wkv_v[2 * j, rows, cols] = lo
            wkv_v[2 * j + 1, rows, cols] = hi
            return [lo, hi]

        units = [(w_, h_, j_) for w_ in range(2) for h_ in range(2) for j_ in range(H // 2)]

        def qproj(it, r0, n, t, zeros=(None, None)):
            outs = []
            for u in range(2):
                lhs = _bf(linked(x_v[_h(r0, n), :]))
                d = _dot(lhs, _bf(wq_v[it, :, pl.ds(t * D + u * LANE, LANE)]))
                set_link(d)
                if zeros[u] is not None:
                    for k, z in enumerate(zeros[u]):
                        d = _pin(d, z, 8 * ((k * (n // 8)) // len(zeros[u])))
                outs.append(d)
            q2 = _lanecat(outs)
            q_all[2 * it + t, _h(r0, n), :] = _u32((q2 * (D ** -0.5 * LOG2E)).astype(BF16))

        def q_body(it, carry):
            slot = it % 2
            with jax.named_scope("w_wait"):
                for cp in w_copies(0, slot):
                    cp.wait()
            c_copy(it).start()
            link[0] = None
            pieces = [(pc, t) for pc in range(1, XC) for t in range(2)]
            nd = 2 * len(pieces)
            for k, (pc, t) in enumerate(pieces):
                zeros = []
                for u in range(2):
                    d = 2 * k + u
                    mine = units[d * len(units) // nd:(d + 1) * len(units) // nd]
                    zeros.append([_opaque_zero(unpack(it, slot, *u_)) for u_ in mine])
                qproj(it, pc * x_cols, x_cols, t, zeros)

            @pl.when(it + 2 < QIT)
            def _():
                for cp in w_copies(it + 2, slot):
                    cp.start()
            return carry

        for cp in step_copies(0):
            cp.start()
        with jax.named_scope("q_loop"):
            lax.fori_loop(0, QIT, q_body, 0)
        for it in range(QIT):
            c_copy(it).wait()

        tri = (lax.broadcasted_iota(jnp.int32, (LANE, LANE), 1)
               <= lax.broadcasted_iota(jnp.int32, (LANE, LANE), 0))

        def out_copy(i):
            if i == S // D:
                cs = pl.ds(0, AT * LANE)
                return pltpu.make_async_copy(out_v.at[:, cs], out_hbm.at[:, cs], sem_out.at[i])
            rs, cs = pl.ds(i * D, D), pl.ds(AT * LANE, 2 * M - AT * LANE)
            return pltpu.make_async_copy(out_v.at[rs, cs], out_hbm.at[rs, cs], sem_out.at[i])

        def a_out():
            for i in range(S // tq):
                cols = slice(i * tq, (i + 1) * tq)
                out_v[cols, 0:AT * LANE] = ra_t[0:AT * LANE, cols].T.astype(BF16)
            out_copy(S // D).start()

        def head_step(h, carry):
            slot = h % 2
            with_a = cfg["use_a"]

            if cfg["a_out"] == 0:
                pl.when(h == A_STEPS)(a_out)

            step_wait(h)
            link[0] = None

            def prefetch():
                @pl.when(h + 1 < H)
                def _():
                    for cp in step_copies(h + 1):
                        cp.start()

            a_rows = pl.ds(pl.multiple_of(jnp.minimum(h, A_STEPS - 1) * AR, AR), AR)

            def a_fwd():
                kk = _bf(a_v[slot, 0]).astype(F32)
                lane = lax.broadcasted_iota(jnp.int32, (AR, LANE), 1)
                coef = [par_v[j, a_rows, :] for j in range(KS)]
                rolled = [kk] + [pltpu.roll(kk, j, 1) for j in range(1, KS)]
                vv = _bf(a_v[slot, 1]).astype(F32)
                kv_blocks = []
                for a in range(NB):
                    cs = slice(a * LANE, (a + 1) * LANE)
                    acc = rolled[0][:, cs] * coef[0]
                    for j in range(1, KS):
                        t = rolled[j][:, cs]
                        if a == 0:
                            t = jnp.where(lane >= j, t, 0.0)
                        acc = acc + t * coef[j]
                    kv_blocks.append(acc * vv[:, cs])
                hk = a_v[slot, 2]
                hk = _rowcat([hk[:, a * LANE:(a + 1) * LANE] for a in range(NB)])
                fm = _bf(f_v[...])
                hs = _dot(_bf(linked(hk)), fm)
                kv = linked(_rowcat(kv_blocks)).astype(BF16)
                xs = _dot(kv, fm)
                set_link(xs)
                return kv, xs, hs

            def a_conv(xs, hs):
                def tile(v, a, g, part):
                    r = a * AR + 8 * g
                    return v[r:r + 8, part * LANE:(part + 1) * LANE]

                z = {}
                nch = cfg["a_chains"]
                gates = [None] * nch
                width = cfg["a_width"]
                k = 0
                for g in range(AR // 8):
                    hr = [tile(hs, 0, g, 0)] + [
                        tile(hs, j, g, 0) - tile(hs, j - 1, g, 1) for j in range(1, NB)]
                    hi = [tile(hs, 0, g, 1)] + [
                        tile(hs, j, g, 1) + tile(hs, j - 1, g, 0) for j in range(1, NB)]
                    for c0 in range(0, NB, width):
                        ch = k % nch
                        k += 1
                        for a in range(c0 + width):
                            xr, xi = tile(xs, a, g, 0), tile(xs, a, g, 1)
                            if gates[ch] is not None and cfg["a_gate"]:
                                xr, xi = _pin(xr, gates[ch]), _pin(xi, gates[ch])
                            for c in range(max(c0, a), c0 + width):
                                j = c - a
                                tr = xr * hr[j] - xi * hi[j]
                                ti = xr * hi[j] + xi * hr[j]
                                z[c, g] = (tr, ti) if a == 0 else (z[c, g][0] + tr, z[c, g][1] + ti)
                            gates[ch] = _opaque_zero(list(z[c0 + width - 1, g]))
                return z

            def a_inv(kv, z):
                fm = _bf(f_v[...])
                ng = AR // 8
                ys = []
                for u in range(2):
                    rows = [_lanecat(z[c, g]) for g in range(u * ng // 2, (u + 1) * ng // 2)
                            for c in range(NB)]
                    ys.append(_dot_nt(linked(_rowcat(rows)).astype(BF16), fm))
                y = _rowcat(ys)
                dd = par_v[KS, a_rows, :]
                for c in range(NB):
                    cs = slice(c * LANE, (c + 1) * LANE)
                    yc = _rowcat([y[(g * NB + c) * 8:(g * NB + c + 1) * 8, :] for g in range(ng)])
                    qq = _bf(a_v[slot, 3, :, cs]).astype(F32)
                    kvf = kv[c * AR:(c + 1) * AR, :].astype(F32)
                    ra_t[a_rows, cs] = qq * (yc * (1.0 / LANE) + kvf * dd)

            def proj(dst, which, r0, n):
                outs = []
                kw = C // 2
                for t in range(2):
                    acc = None
                    for u in range(2):
                        lhs = linked(c_v[_h(r0, n), pl.ds(u * kw, kw)])
                        w = wkv_v[h, _h(u * kw, kw), pl.ds(which * D + t * LANE, LANE)]
                        d = _dot(_bf(lhs), _bf(w))
                        set_link(d)
                        acc = d if acc is None else acc + d
                    outs.append(acc)
                dst[r0:r0 + n, :] = _lanecat(outs).astype(BF16)

            def qk(i):
                r0 = i * tq
                parts = [_dot_nt(_bf(linked(q_all[h, _h(r0, tq), :])), k_s[0:r0 + LANE, :])]
                if i > 0:
                    link[0] = _opaque_zero([parts[0][0:8, r0 - LANE:r0]])
                for j in range(1, nsub):
                    q = linked(q_all[h, _h(r0 + LANE * j, tq - LANE * j), :])
                    parts.append(_dot_nt(_bf(q), k_s[r0 + LANE * j:r0 + LANE * (j + 1), :]))
                set_link(parts[2], cfg["link_part"])
                return parts

            def softmax(i, parts):
                pb = p_s.at[i % 2]
                chain = _opaque_zero([b[b.shape[0] - 8:, b.shape[1] - LANE:] for b in parts])
                ls = []
                for a in range(nsub):
                    blocks = [parts[j][LANE * (a - j):LANE * (a - j + 1), :] for j in range(a + 1)]
                    last = blocks[-1]
                    w = last.shape[1]
                    dg = jnp.where(tri, last[:, w - LANE:], NEG)
                    blocks[-1] = dg if w == LANE else _lanecat([last[:, :w - LANE], dg])
                    sa = _lanecat(blocks)
                    if cfg["dbg"] & 4:
                        ls.append(jnp.ones((LANE, 1), F32))
                        p = _pin(sa, link[0], 0, 0 if a == 0 else sa.shape[1] - LANE)
                        pb[LANE * a:LANE * (a + 1), 0:sa.shape[1]] = p.astype(BF16)
                        continue
                    mb = jnp.broadcast_to(jnp.max(sa, axis=1, keepdims=True), (LANE, LANE))
                    nt = sa.shape[1] // LANE
                    ptiles, psums = [], []
                    for g in range(0, LANE, 8):
                        mg = _pin(mb[g:g + 8, :], chain)
                        pg = [jnp.exp2(sa[g:g + 8, t * LANE:(t + 1) * LANE] - mg) for t in range(nt)]
                        ps = functools.reduce(jnp.add, pg)
                        chain = _opaque_zero([ps])
                        psums.append(ps)
                        ptiles.append(_lanecat(pg))
                    ls.append(jnp.sum(_rowcat(psums), axis=1, keepdims=True))
                    p = _pin(_rowcat(ptiles), link[0], 0, 0 if a == 0 else sa.shape[1] - LANE)
                    pb[LANE * a:LANE * (a + 1), 0:sa.shape[1]] = p.astype(BF16)
                return ls

            def pv(i, ls):
                r0 = i * tq
                pb = p_s.at[i % 2]
                ctx = [_dot(pb[:, 0:r0 + LANE], v_s[0:r0 + LANE, :])]
                for j in range(1, nsub):
                    ctx.append(_dot(pb[LANE * j:, r0 + LANE * j:r0 + LANE * (j + 1)],
                                    v_s[r0 + LANE * j:r0 + LANE * (j + 1), :]))
                set_link(ctx[2], cfg["link_part"])
                cs = []
                for a in range(nsub):
                    sl = lambda j: slice(LANE * (a - j), LANE * (a - j + 1))
                    r = pl.reciprocal(ls[a], approx=True)
                    r = r * (2.0 - ls[a] * r)
                    cs.append(functools.reduce(jnp.add, [ctx[j][sl(j)] for j in range(a + 1)]) * r)
                return _rowcat(cs).astype(BF16)

            def oproj(i, ctx):
                for u in range(tq // D):
                    res = _dot_nt(_bf(linked(wo_v[slot])), ctx[u * D:(u + 1) * D, :])
                    set_link(res)
                    c0 = i * tq + u * D
                    rb_t[:, c0:c0 + D] += res

            a_state = {}

            def a_hook(tag):
                if tag == cfg["pf_at"]:
                    prefetch()
                if with_a and tag == cfg["a_fwd_at"]:
                    a_state["kv"], xs, hs = a_fwd()
                    a_state["z"] = a_conv(xs, hs)
                if with_a and tag == cfg["a_inv_at"]:
                    a_inv(a_state["kv"], a_state["z"])

            import contextlib
            sc = (lambda n: jax.named_scope(n)) if cfg["dbg"] & 8 else (lambda n: contextlib.nullcontext())
            with sc("s_kp0"):
                a_hook(0)
                proj(k_s, 0, 0, tq)
                a_hook(1)
            with sc("s_qk"):
                parts = qk(0)
            ctx_prev = None
            for i in range(nq):
                r0 = i * tq
                with sc("s_mid"):
                    a_hook(10 * (i + 1))
                    if ctx_prev is not None:
                        oproj(i - 1, ctx_prev)
                    a_hook(10 * (i + 1) + 1)
                    if i + 1 < nq:
                        proj(k_s, 0, r0 + tq, tq)
                    a_hook(10 * (i + 1) + 2)
                    proj(v_s, 1, r0, tq)
                    a_hook(10 * (i + 1) + 3)
                    ls = softmax(i, parts)
                with sc("s_pv"):
                    ctx_prev = pv(i, ls)
                    a_hook(10 * (i + 1) + 4)
                if i + 1 < nq:
                    with sc("s_qk"):
                        parts = qk(i + 1)
            with sc("s_o"):
                oproj(nq - 1, ctx_prev)
            return carry

        with jax.named_scope("loop_a"):
            lax.fori_loop(cfg["h0"], H, head_step, 0)
        with jax.named_scope("tail"):
            if cfg["a_out"] == 1:
                a_out()
            for i in range(S // D):
                cols = slice(i * D, (i + 1) * D)
                full = _rowcat([ra_t[AT * LANE:, cols], rb_t[:, cols]])
                out_v[cols, AT * LANE:] = full.T.astype(BF16)
                out_copy(i).start()
            for i in range(S // D + 1):
                out_copy(i).wait()

    scratch = [
        pltpu.VMEM((2, 4, AR // 2, S), U32),
        pltpu.VMEM((KS, M), BF16),
        pltpu.VMEM((M,), BF16),
        pltpu.VMEM((KS + 1, M, LANE), F32),
        pltpu.VMEM((LANE // 2, 2 * LANE), U32),
        pltpu.VMEM((M // 2, S), U32),
        pltpu.VMEM((S // 2, MP), U32),
        pltpu.VMEM((S // 2, C), U32),
        pltpu.VMEM((KT, 4 * TP * 8, LANE), U32),
        pltpu.VMEM((H // 2, MP // 2, 2 * D), U32),
        pltpu.VMEM((H // 2, x_cols, 2 * D), F32),
        pltpu.VMEM((2, 8 * WP * 8, LANE), U32),
        pltpu.VMEM((H, C // 2, 2 * D), U32),
        pltpu.VMEM((2, M // 2, D), U32),
        pltpu.VMEM((H, S // 2, D), U32),
        pltpu.VMEM((S, D), BF16),
        pltpu.VMEM((S, D), BF16),
        pltpu.VMEM((2, tq, S), BF16),
        pltpu.VMEM((M, S), F32),
        pltpu.VMEM((M, S), F32),
        pltpu.VMEM((S, 2 * M), BF16),
        pltpu.SemaphoreType.DMA((XC,)),
        pltpu.SemaphoreType.DMA((4 * KT,)),
        pltpu.SemaphoreType.DMA((16,)),
        pltpu.SemaphoreType.DMA((QIT,)),
        pltpu.SemaphoreType.DMA((2,)),
        pltpu.SemaphoreType.DMA((4,)),
        pltpu.SemaphoreType.DMA((S // D + 1,)),
    ]
    return kernel, scratch


_DEFAULT = dict(tq=512, a_fwd_at=13, a_inv_at=44, pf_at=0, a_gate=1, a_chains=1, a_width=4, a_out=0, dbg=0,
                link_back=176, link_part=32, use_a=1, h0=0)


def _build(**kw):
    cfg = dict(_DEFAULT)
    cfg.update(kw)
    kernel, scratch = _make_kernel(cfg)

    def run(A_q, A_k, A_v, A_shift_k, A_ssm_k, A_ssm_D, B_x, B_c_kv, B_w_q, B_w_uk,
            B_w_uv, B_w_o):
        tr = lambda a: jnp.swapaxes(a, 1, 2).reshape(M, S)
        args = (
            tr(A_q), tr(A_k), tr(A_v), A_shift_k.T, A_ssm_k, A_ssm_D, tr(B_x),
            B_c_kv.reshape(S, C),
            B_w_q.reshape(M // 2, 2 * H, D), B_w_uk.reshape(C // 2, 2 * H, D),
            B_w_uv.reshape(C // 2, 2 * H, D),
            jnp.swapaxes(B_w_o, 1, 2),
        )
        out = pl.pallas_call(
            kernel,
            in_specs=[pl.BlockSpec(memory_space=pl.ANY)] * len(args),
            out_specs=pl.BlockSpec(memory_space=pl.ANY),
            out_shape=jax.ShapeDtypeStruct((S, 2 * M), BF16),
            scratch_shapes=scratch,
            compiler_params=pltpu.CompilerParams(
                vmem_limit_bytes=120 * 1024 * 1024,
                disable_bounds_checks=True),
        )(*args)
        return out.reshape(1, S, 2 * M)

    return run


_run = _build()


@jax.jit
def pallas_concat_heads__ssm_conv_h3__compressed_kv_cla__prompt_kernel(
    A_q: jax.Array,
    A_k: jax.Array,
    A_v: jax.Array,
    A_shift_k: jax.Array,
    A_ssm_k: jax.Array,
    A_ssm_D: jax.Array,
    B_x: jax.Array,
    B_c_kv: jax.Array,
    B_w_q: jax.Array,
    B_w_uk: jax.Array,
    B_w_uv: jax.Array,
    B_w_o: jax.Array,
):
    return _run(A_q, A_k, A_v, A_shift_k, A_ssm_k, A_ssm_D, B_x, B_c_kv, B_w_q,
                B_w_uk, B_w_uv, B_w_o)
```

```python
import functools

import jax
import jax.numpy as jnp
from jax import lax
import jax.experimental.pallas as pl
import jax.experimental.pallas.tpu as pltpu

F32 = jnp.float32
BF16 = jnp.bfloat16
U32 = jnp.uint32

S = 2048
M = 448
MP = 512
C = 1024
H = 16
D = 256
KS = 4
LANE = 128
NB = S // LANE
AR = 32
A_STEPS = M // AR
LOG2E = 1.4426950408889634
NEG = -1e30

NT = (((1,), (1,)), ((), ()))


def _dot(a, b):
    return jnp.dot(a, b, preferred_element_type=F32)


def _dot_nt(a, b):
    return lax.dot_general(a, b, NT, preferred_element_type=F32)


def _bf(x):
    return pltpu.bitcast(x, BF16)


def _u32(x):
    return pltpu.bitcast(x, U32)


def _h(r0, n):
    return pl.ds(r0 // 2, n // 2)


def _repack(ev, od):
    lo = (ev & jnp.uint32(0xFFFF)) | (od << 16)
    hi = (ev >> 16) | (od & jnp.uint32(0xFFFF0000))
    return lo, hi


def _opaque_zero(vals):
    acc = None
    for v in vals:
        b = v if v.dtype == U32 else pltpu.bitcast(v, U32)
        for r in range(0, b.shape[0], 8):
            for c in range(0, b.shape[1], LANE):
                t = b[r:r + 8, c:c + LANE]
                acc = t if acc is None else acc | t
    return jnp.minimum((acc >> 1).astype(jnp.int32), 0)


def _pin(x, zero, r=0, c=0):
    t = pltpu.bitcast(pltpu.bitcast(x[r:r + 8, c:c + LANE], jnp.int32) + zero, x.dtype)
    row = ([x[r:r + 8, :c]] if c > 0 else []) + [t] + (
        [x[r:r + 8, c + LANE:]] if c + LANE < x.shape[1] else [])
    row = jnp.concatenate(row, axis=1) if len(row) > 1 else row[0]
    col = ([x[:r, :]] if r > 0 else []) + [row] + ([x[r + 8:, :]] if r + 8 < x.shape[0] else [])
    return jnp.concatenate(col, axis=0) if len(col) > 1 else col[0]


def _rowcat(xs):
    return jnp.concatenate(xs, axis=0) if len(xs) > 1 else xs[0]


def _lanecat(xs):
    return jnp.concatenate(xs, axis=1) if len(xs) > 1 else xs[0]


def _make_kernel(cfg):
    tq = cfg["tq"]
    nq = S // tq
    nsub = tq // LANE
    KT = MP // LANE
    TP = LANE // 2
    XC = 4
    x_cols = S // XC
    WP = 64
    WS = 3
    QIT = 8
    AT = 3

    def kernel(aq_hbm, ak_hbm, av_hbm, sh_hbm, ssm_hbm, dd_hbm, x_hbm, c_hbm,
               wq_hbm, wk_hbm, wv_hbm, wo_hbm,
               out_hbm,
               a_v, sh_v, dd_v, par_v, f_v,
               xt_v, x_v, c_v, wqs_v, wq_v, qacc, ws_v, wkv_v, wo_v,
               q_all, k_s, v_s, p_s, ra_t, rb_t, out_v,
               sem_x, sem_wq, sem_w, sem_c, sem_s, sem_a, sem_out):
        x32, c32, wq32, wk32, wv32, wo32 = (
            r.bitcast(U32) for r in (x_hbm, c_hbm, wq_hbm, wk_hbm, wv_hbm, wo_hbm))
        a32 = [r.bitcast(U32) for r in (ak_hbm, av_hbm, ssm_hbm, aq_hbm)]

        def x_copy(i):
            cs = pl.ds(i * x_cols, x_cols)
            return pltpu.make_async_copy(x32.at[:, cs], xt_v.at[:, cs], sem_x.at[i])

        def wq_copies(kt):
            dst = wqs_v.reshape(4 * KT, TP, 8, LANE)
            rs = pl.ds(min(kt * TP, M // 2 - TP), TP)
            return [pltpu.make_async_copy(
                wq32.at[rs, pl.ds(8 * (k // 2), 8), pl.ds((k % 2) * LANE, LANE)],
                dst.at[4 * kt + k], sem_wq.at[kt]) for k in range(4)]

        def wq_wait(kt):
            pltpu.make_async_copy(wqs_v.at[kt], wqs_v.at[kt], sem_wq.at[kt]).wait()

        def w_rows(chunk):
            r0 = chunk * WP
            return pl.ds(r0 if isinstance(r0, int) else pl.multiple_of(r0, WP), WP)

        def w_copies(chunk, slot):
            dst = ws_v.reshape(8 * WS, WP, 8, LANE)
            rs = w_rows(chunk)
            out = []
            for which, src in enumerate((wk32, wv32)):
                for par in range(2):
                    for half in range(2):
                        k = 8 * slot + 4 * which + 2 * par + half
                        out.append(pltpu.make_async_copy(
                            src.at[rs, pl.ds(8 * par, 8), pl.ds(half * LANE, LANE)],
                            dst.at[k], sem_w.at[slot]))
            return out

        def w_wait(slot):
            pltpu.make_async_copy(ws_v.at[slot], ws_v.at[slot], sem_w.at[slot]).wait()

        def c_copy(it):
            n = S // 2 // QIT
            rs = pl.ds(pl.multiple_of(it * n, n), n)
            return pltpu.make_async_copy(c32.at[rs], c_v.at[rs], sem_c.at[it])

        wo_copy = pltpu.make_async_copy(wo32, wo_v, sem_a.at[0])
        a_parts = [pl.ds(0, AR // 2), pl.ds(AR // 2, M // 2 - AR // 2)]

        def a_start(part):
            rs = a_parts[part]
            for k in range(4):
                pltpu.make_async_copy(a32[k].at[rs], a_v.at[k, rs], sem_a.at[1 + part]).start()

        def a_wait(part):
            view = a_v.at[:, a_parts[part]]
            pltpu.make_async_copy(view, view, sem_a.at[1 + part]).wait()

        small = [pltpu.make_async_copy(sh_hbm, sh_v, sem_s.at[0]),
                 pltpu.make_async_copy(dd_hbm, dd_v, sem_s.at[1])]

        link = [None]

        def set_link(res, row=None):
            if row is None:
                row = res.shape[0] - cfg["link_back"]
            link[0] = _opaque_zero([res[row:row + 8, res.shape[1] - LANE:]])

        def linked(x):
            return x if link[0] is None or cfg["dbg"] & 2 else _pin(x, link[0])

        with jax.named_scope("first_starts"):
            for cp in small:
                cp.start()
        x_copy(0).start()
        for kt in range(cfg["wq_first"]):
            for cp in wq_copies(kt):
                cp.start()

        bi = lax.broadcasted_iota(jnp.int32, (LANE, LANE), 0)
        mi = lax.broadcasted_iota(jnp.int32, (LANE, LANE), 1)
        ph = ((4 * mi + 1) * bi) & 511
        ang = ph.astype(F32) * (2.0 * 3.141592653589793 / 512.0)
        f_v[:, 0:LANE] = _u32(jnp.cos(ang).astype(BF16))
        f_v[:, LANE:] = _u32((-jnp.sin(ang)).astype(BF16))

        rb_t[...] = jnp.zeros((M, S), F32)

        for kt in range(cfg["wq_first"], KT):
            for cp in wq_copies(kt):
                cp.start()
        with jax.named_scope("small_wait"):
            for cp in small:
                cp.wait()
        sh = sh_v[...].astype(F32)
        for j in range(KS):
            par_v[j] = jnp.broadcast_to(sh[j:j + 1, :], (LANE, M)).T
        dd = dd_v[...].astype(F32).reshape(1, M)
        par_v[KS] = jnp.broadcast_to(dd, (LANE, M)).T

        def x_transpose(i):
            xt = xt_v[:, pl.ds(i * x_cols, x_cols)]
            nfull = (KT - 1) * TP
            xt = _rowcat([xt[:nfull], jnp.zeros((MP // 2 - M // 2, x_cols), U32), xt[nfull:]])
            x_v[_h(i * x_cols, x_cols), :] = _u32(_bf(xt).astype(F32).T.astype(BF16))

        def q_early(kt, first, last):
            r0 = kt * TP
            rows = pl.ds(r0 if isinstance(r0, int) else pl.multiple_of(r0, TP), TP)
            c0 = kt * LANE
            cols = pl.ds(c0 if isinstance(c0, int) else pl.multiple_of(c0, LANE), LANE)
            link[0] = None
            for j in range(H // 2):
                ws = []
                for half in range(2):
                    ev, od = (
                        wqs_v[kt, pl.ds((2 * par + half) * TP * 8 + j, TP, stride=8), :]
                        for par in range(2))
                    ws.append(_repack(ev, od))
                w = _lanecat([ws[0][0], ws[1][0], ws[0][1], ws[1][1]])
                wq_v[j, rows, :] = w
                d = _dot(_bf(linked(x_v[_h(0, x_cols), cols])), _bf(w))
                set_link(d)
                if not first:
                    d = d + qacc[j]
                if last:
                    d = (d * (D ** -0.5 * LOG2E)).astype(BF16)
                    for t in range(2):
                        q_all[2 * j + t, _h(0, x_cols), :] = _u32(d[:, t * D:(t + 1) * D])
                else:
                    qacc[j] = d

        with jax.named_scope("x_wait"):
            x_copy(0).wait()
        x_transpose(0)
        with jax.named_scope("wq_wait"):
            wq_wait(0)
        q_early(0, True, False)
        for i in range(1, XC):
            x_copy(i).start()

        def early_body(kt, carry):
            with jax.named_scope("wq_wait"):
                wq_wait(kt)
            q_early(kt, False, False)
            for cp in w_copies(kt - 1, kt - 1):
                cp.start()
            return carry

        lax.fori_loop(1, KT - 1, early_body, 0)
        with jax.named_scope("wq_wait"):
            wq_wait(KT - 1)
            for i in range(1, XC):
                x_copy(i).wait()
        q_early(KT - 1, False, True)
        for i in range(1, XC):
            x_transpose(i)

        def unpack(chunk, slot, which, half, j):
            ev, od = (
                ws_v[slot, pl.ds((4 * which + 2 * par + half) * WP * 8 + j, WP, stride=8), :]
                for par in range(2))
            lo, hi = _repack(ev, od)
            rows = w_rows(chunk)
            cols = pl.ds(which * D + half * LANE, LANE)
            wkv_v[2 * j, rows, cols] = lo
            wkv_v[2 * j + 1, rows, cols] = hi
            return [lo, hi]

        units = [(w_, h_, j_) for w_ in range(2) for h_ in range(2) for j_ in range(H // 2)]

        def qproj(it, r0, n, t, zeros=(None, None)):
            outs = []
            for u in range(2):
                lhs = _bf(linked(x_v[_h(r0, n), :]))
                d = _dot(lhs, _bf(wq_v[it, :, pl.ds(t * D + u * LANE, LANE)]))
                set_link(d)
                if zeros[u] is not None:
                    for k, z in enumerate(zeros[u]):
                        d = _pin(d, z, 8 * ((k * (n // 8)) // len(zeros[u])))
                outs.append(d)
            q2 = _lanecat(outs)
            q_all[2 * it + t, _h(r0, n), :] = _u32((q2 * (D ** -0.5 * LOG2E)).astype(BF16))

        def q_body(it, carry):
            slot = it % WS

            def q_prefetch():
                c_copy(it).start()

                @pl.when(it + 2 < QIT)
                def _():
                    for cp in w_copies(it + 2, (it + 2) % WS):
                        cp.start()

                @pl.when(it == QIT - 2)
                def _():
                    wo_copy.start()
                    a_start(0)

            if cfg["q_pf"] == -2:
                q_prefetch()
            with jax.named_scope("w_wait"):
                w_wait(slot)
            if cfg["q_pf"] == -1:
                q_prefetch()
            link[0] = None
            pieces = [(pc, t) for pc in range(1, XC) for t in range(2)]
            nd = 2 * len(pieces)
            for k, (pc, t) in enumerate(pieces):
                zeros = []
                for u in range(2):
                    d = 2 * k + u
                    mine = units[d * len(units) // nd:(d + 1) * len(units) // nd]
                    zeros.append([_opaque_zero(unpack(it, slot, *u_)) for u_ in mine])
                qproj(it, pc * x_cols, x_cols, t, zeros)
                if k == cfg["q_pf"]:
                    q_prefetch()
            return carry

        with jax.named_scope("q_loop"):
            lax.fori_loop(0, QIT, q_body, 0)
        a_start(1)
        for it in range(QIT):
            c_copy(it).wait()
        a_wait(0)
        wo_copy.wait()

        tri = (lax.broadcasted_iota(jnp.int32, (LANE, LANE), 1)
               <= lax.broadcasted_iota(jnp.int32, (LANE, LANE), 0))

        def out_copy(i):
            if i == S // D:
                cs = pl.ds(0, AT * LANE)
                return pltpu.make_async_copy(out_v.at[:, cs], out_hbm.at[:, cs], sem_out.at[i])
            rs, cs = pl.ds(i * D, D), pl.ds(AT * LANE, 2 * M - AT * LANE)
            return pltpu.make_async_copy(out_v.at[rs, cs], out_hbm.at[rs, cs], sem_out.at[i])

        def a_out():
            for i in range(S // tq):
                cols = slice(i * tq, (i + 1) * tq)
                out_v[cols, 0:AT * LANE] = ra_t[0:AT * LANE, cols].T.astype(BF16)
            out_copy(S // D).start()

        def head_step(h, carry):
            with jax.named_scope("step"):
                return head_step_(h, carry)

        def head_step_(h, carry):
            with_a = cfg["use_a"]

            if cfg["a_out"] == 0:
                pl.when(h == A_STEPS)(a_out)

            @pl.when(h == cfg["h0"] + 1)
            def _():
                a_wait(1)

            link[0] = None
            n2 = AR // 2
            a_rows2 = pl.ds(pl.multiple_of(jnp.minimum(h, A_STEPS - 1) * n2, n2), n2)
            a_rows = pl.ds(pl.multiple_of(jnp.minimum(h, A_STEPS - 1) * AR, AR), AR)

            def a_fwd():
                kk = _bf(a_v[0, a_rows2, :]).astype(F32)
                lane = lax.broadcasted_iota(jnp.int32, (AR, LANE), 1)
                coef = [par_v[j, a_rows, :] for j in range(KS)]
                rolled = [kk] + [pltpu.roll(kk, j, 1) for j in range(1, KS)]
                vv = _bf(a_v[1, a_rows2, :]).astype(F32)
                kv_blocks = []
                for a in range(NB):
                    cs = slice(a * LANE, (a + 1) * LANE)
                    acc = rolled[0][:, cs] * coef[0]
                    for j in range(1, KS):
                        t = rolled[j][:, cs]
                        if a == 0:
                            t = jnp.where(lane >= j, t, 0.0)
                        acc = acc + t * coef[j]
                    kv_blocks.append(acc * vv[:, cs])
                hk = a_v[2, a_rows2, :]
                hk = _rowcat([hk[:, a * LANE:(a + 1) * LANE] for a in range(NB)])
                fm = _bf(f_v[...])
                hs = _dot(_bf(linked(hk)), fm)
                kv = linked(_rowcat(kv_blocks)).astype(BF16)
                xs = _dot(kv, fm)
                set_link(xs)
                return kv, xs, hs

            def a_conv(xs, hs):
                def tile(v, a, g, part):
                    r = a * AR + 8 * g
                    return v[r:r + 8, part * LANE:(part + 1) * LANE]

                z = {}
                nch = cfg["a_chains"]
                gates = [None] * nch
                width = cfg["a_width"]
                k = 0
                for g in range(AR // 8):
                    hr = [tile(hs, 0, g, 0)] + [
                        tile(hs, j, g, 0) - tile(hs, j - 1, g, 1) for j in range(1, NB)]
                    hi = [tile(hs, 0, g, 1)] + [
                        tile(hs, j, g, 1) + tile(hs, j - 1, g, 0) for j in range(1, NB)]
                    for c0 in range(0, NB, width):
                        ch = k % nch
                        k += 1
                        for a in range(c0 + width):
                            xr, xi = tile(xs, a, g, 0), tile(xs, a, g, 1)
                            if gates[ch] is not None and cfg["a_gate"]:
                                xr, xi = _pin(xr, gates[ch]), _pin(xi, gates[ch])
                            for c in range(max(c0, a), c0 + width):
                                j = c - a
                                tr = xr * hr[j] - xi * hi[j]
                                ti = xr * hi[j] + xi * hr[j]
                                z[c, g] = (tr, ti) if a == 0 else (z[c, g][0] + tr, z[c, g][1] + ti)
                            gates[ch] = _opaque_zero(list(z[c0 + width - 1, g]))
                return z

            def a_inv(kv, z):
                fm = _bf(f_v[...])
                ng = AR // 8
                ys = []
                for u in range(2):
                    rows = [_lanecat(z[c, g]) for g in range(u * ng // 2, (u + 1) * ng // 2)
                            for c in range(NB)]
                    ys.append(_dot_nt(linked(_rowcat(rows)).astype(BF16), fm))
                y = _rowcat(ys)
                dd = par_v[KS, a_rows, :]
                for c in range(NB):
                    cs = slice(c * LANE, (c + 1) * LANE)
                    yc = _rowcat([y[(g * NB + c) * 8:(g * NB + c + 1) * 8, :] for g in range(ng)])
                    qq = _bf(a_v[3, a_rows2, cs]).astype(F32)
                    kvf = kv[c * AR:(c + 1) * AR, :].astype(F32)
                    ra_t[a_rows, cs] = qq * (yc * (1.0 / LANE) + kvf * dd)

            def proj(dst, which, r0, n):
                outs = []
                kw = C // 2
                for t in range(2):
                    acc = None
                    for u in range(2):
                        lhs = linked(c_v[_h(r0, n), pl.ds(u * kw, kw)])
                        w = wkv_v[h, _h(u * kw, kw), pl.ds(which * D + t * LANE, LANE)]
                        d = _dot(_bf(lhs), _bf(w))
                        set_link(d)
                        acc = d if acc is None else acc + d
                    outs.append(acc)
                dst[r0:r0 + n, :] = _lanecat(outs).astype(BF16)

            def qk(i):
                r0 = i * tq
                parts = [_dot_nt(_bf(linked(q_all[h, _h(r0, tq), :])), k_s[0:r0 + LANE, :])]
                if i > 0:
                    link[0] = _opaque_zero([parts[0][0:8, r0 - LANE:r0]])
                for j in range(1, nsub):
                    q = linked(q_all[h, _h(r0 + LANE * j, tq - LANE * j), :])
                    parts.append(_dot_nt(_bf(q), k_s[r0 + LANE * j:r0 + LANE * (j + 1), :]))
                set_link(parts[2], cfg["link_part"])
                return parts

            def softmax(i, parts):
                pb = p_s.at[i % 2]
                chain = _opaque_zero([b[b.shape[0] - 8:, b.shape[1] - LANE:] for b in parts])
                ls = []
                for a in range(nsub):
                    blocks = [parts[j][LANE * (a - j):LANE * (a - j + 1), :] for j in range(a + 1)]
                    last = blocks[-1]
                    w = last.shape[1]
                    dg = jnp.where(tri, last[:, w - LANE:], NEG)
                    blocks[-1] = dg if w == LANE else _lanecat([last[:, :w - LANE], dg])
                    sa = _lanecat(blocks)
                    if cfg["dbg"] & 4:
                        ls.append(jnp.ones((LANE, 1), F32))
                        p = _pin(sa, link[0], 0, 0 if a == 0 else sa.shape[1] - LANE)
                        pb[LANE * a:LANE * (a + 1), 0:sa.shape[1]] = p.astype(BF16)
                        continue
                    mb = jnp.broadcast_to(jnp.max(sa, axis=1, keepdims=True), (LANE, LANE))
                    nt = sa.shape[1] // LANE
                    ptiles, psums = [], []
                    for g in range(0, LANE, 8):
                        mg = _pin(mb[g:g + 8, :], chain)
                        pg = [jnp.exp2(sa[g:g + 8, t * LANE:(t + 1) * LANE] - mg) for t in range(nt)]
                        ps = functools.reduce(jnp.add, pg)
                        chain = _opaque_zero([ps])
                        psums.append(ps)
                        ptiles.append(_lanecat(pg))
                    ls.append(jnp.sum(_rowcat(psums), axis=1, keepdims=True))
                    p = _pin(_rowcat(ptiles), link[0], 0, 0 if a == 0 else sa.shape[1] - LANE)
                    pb[LANE * a:LANE * (a + 1), 0:sa.shape[1]] = p.astype(BF16)
                return ls

            def pv(i, ls):
                r0 = i * tq
                pb = p_s.at[i % 2]
                ctx = [_dot(pb[:, 0:r0 + LANE], v_s[0:r0 + LANE, :])]
                for j in range(1, nsub):
                    ctx.append(_dot(pb[LANE * j:, r0 + LANE * j:r0 + LANE * (j + 1)],
                                    v_s[r0 + LANE * j:r0 + LANE * (j + 1), :]))
                set_link(ctx[2], cfg["link_part"])
                cs = []
                for a in range(nsub):
                    sl = lambda j: slice(LANE * (a - j), LANE * (a - j + 1))
                    r = pl.reciprocal(ls[a], approx=True)
                    r = r * (2.0 - ls[a] * r)
                    cs.append(functools.reduce(jnp.add, [ctx[j][sl(j)] for j in range(a + 1)]) * r)
                return _rowcat(cs).astype(BF16)

            def oproj(i, ctx):
                for u in range(tq // D):
                    res = _dot_nt(_bf(linked(wo_v[h])), ctx[u * D:(u + 1) * D, :])
                    set_link(res)
                    c0 = i * tq + u * D
                    rb_t[:, c0:c0 + D] += res

            a_state = {}

            def a_hook(tag):
                if with_a and tag == cfg["a_fwd_at"]:
                    a_state["kv"], xs, hs = a_fwd()
                    a_state["z"] = a_conv(xs, hs)
                if with_a and tag == cfg["a_inv_at"]:
                    a_inv(a_state["kv"], a_state["z"])

            import contextlib
            sc = (lambda n: jax.named_scope(n)) if cfg["dbg"] & 8 else (lambda n: contextlib.nullcontext())
            with sc("s_kp0"):
                a_hook(0)
                proj(k_s, 0, 0, tq)
                a_hook(1)
            with sc("s_qk"):
                parts = qk(0)
            ctx_prev = None
            for i in range(nq):
                r0 = i * tq
                with sc("s_mid"):
                    a_hook(10 * (i + 1))
                    if ctx_prev is not None:
                        oproj(i - 1, ctx_prev)
                    a_hook(10 * (i + 1) + 1)
                    if i + 1 < nq:
                        proj(k_s, 0, r0 + tq, tq)
                    a_hook(10 * (i + 1) + 2)
                    proj(v_s, 1, r0, tq)
                    a_hook(10 * (i + 1) + 3)
                    ls = softmax(i, parts)
                with sc("s_pv"):
                    ctx_prev = pv(i, ls)
                    a_hook(10 * (i + 1) + 4)
                if i + 1 < nq:
                    with sc("s_qk"):
                        parts = qk(i + 1)
            with sc("s_o"):
                oproj(nq - 1, ctx_prev)
                a_hook(99)
            return carry

        with jax.named_scope("loop_a"):
            lax.fori_loop(cfg["h0"], H, head_step, 0)
        with jax.named_scope("tail"):
            if cfg["a_out"] == 1:
                a_out()
            for i in range(S // D):
                cols = slice(i * D, (i + 1) * D)
                full = _rowcat([ra_t[AT * LANE:, cols], rb_t[:, cols]])
                out_v[cols, AT * LANE:] = full.T.astype(BF16)
                out_copy(i).start()
            for i in range(S // D + 1):
                out_copy(i).wait()

    scratch = [
        pltpu.VMEM((4, M // 2, S), U32),
        pltpu.VMEM((KS, M), BF16),
        pltpu.VMEM((M,), BF16),
        pltpu.VMEM((KS + 1, M, LANE), F32),
        pltpu.VMEM((LANE // 2, 2 * LANE), U32),
        pltpu.VMEM((M // 2, S), U32),
        pltpu.VMEM((S // 2, MP), U32),
        pltpu.VMEM((S // 2, C), U32),
        pltpu.VMEM((KT, 4 * TP * 8, LANE), U32),
        pltpu.VMEM((H // 2, MP // 2, 2 * D), U32),
        pltpu.VMEM((H // 2, x_cols, 2 * D), F32),
        pltpu.VMEM((WS, 8 * WP * 8, LANE), U32),
        pltpu.VMEM((H, C // 2, 2 * D), U32),
        pltpu.VMEM((H, M // 2, D), U32),
        pltpu.VMEM((H, S // 2, D), U32),
        pltpu.VMEM((S, D), BF16),
        pltpu.VMEM((S, D), BF16),
        pltpu.VMEM((2, tq, S), BF16),
        pltpu.VMEM((M, S), F32),
        pltpu.VMEM((M, S), F32),
        pltpu.VMEM((S, 2 * M), BF16),
        pltpu.SemaphoreType.DMA((XC,)),
        pltpu.SemaphoreType.DMA((KT,)),
        pltpu.SemaphoreType.DMA((WS,)),
        pltpu.SemaphoreType.DMA((QIT,)),
        pltpu.SemaphoreType.DMA((2,)),
        pltpu.SemaphoreType.DMA((3,)),
        pltpu.SemaphoreType.DMA((S // D + 1,)),
    ]
    return kernel, scratch


_DEFAULT = dict(tq=512, a_fwd_at=13, a_inv_at=44, a_gate=1, a_chains=1, a_width=4, a_out=0, dbg=0, q_pf=-1, wq_first=1,
                link_back=176, link_part=32, use_a=1, h0=0)


def _build(**kw):
    cfg = dict(_DEFAULT)
    cfg.update(kw)
    kernel, scratch = _make_kernel(cfg)

    def run(A_q, A_k, A_v, A_shift_k, A_ssm_k, A_ssm_D, B_x, B_c_kv, B_w_q, B_w_uk,
            B_w_uv, B_w_o):
        tr = lambda a: jnp.swapaxes(a, 1, 2).reshape(M, S)
        args = (
            tr(A_q), tr(A_k), tr(A_v), A_shift_k.T, A_ssm_k, A_ssm_D, tr(B_x),
            B_c_kv.reshape(S, C),
            B_w_q.reshape(M // 2, 2 * H, D), B_w_uk.reshape(C // 2, 2 * H, D),
            B_w_uv.reshape(C // 2, 2 * H, D),
            jnp.swapaxes(B_w_o, 1, 2),
        )
        out = pl.pallas_call(
            kernel,
            in_specs=[pl.BlockSpec(memory_space=pl.ANY)] * len(args),
            out_specs=pl.BlockSpec(memory_space=pl.ANY),
            out_shape=jax.ShapeDtypeStruct((S, 2 * M), BF16),
            scratch_shapes=scratch,
            compiler_params=pltpu.CompilerParams(
                vmem_limit_bytes=120 * 1024 * 1024,
                disable_bounds_checks=True),
        )(*args)
        return out.reshape(1, S, 2 * M)

    return run


_run = _build()


@jax.jit
def pallas_concat_heads__ssm_conv_h3__compressed_kv_cla__prompt_kernel(
    A_q: jax.Array,
    A_k: jax.Array,
    A_v: jax.Array,
    A_shift_k: jax.Array,
    A_ssm_k: jax.Array,
    A_ssm_D: jax.Array,
    B_x: jax.Array,
    B_c_kv: jax.Array,
    B_w_q: jax.Array,
    B_w_uk: jax.Array,
    B_w_uv: jax.Array,
    B_w_o: jax.Array,
):
    return _run(A_q, A_k, A_v, A_shift_k, A_ssm_k, A_ssm_D, B_x, B_c_kv, B_w_q,
                B_w_uk, B_w_uv, B_w_o)
```

```python
import functools

import jax
import jax.numpy as jnp
from jax import lax
import jax.experimental.pallas as pl
import jax.experimental.pallas.tpu as pltpu

F32 = jnp.float32
BF16 = jnp.bfloat16
U32 = jnp.uint32

S = 2048
M = 448
MP = 512
C = 1024
H = 16
D = 256
KS = 4
LANE = 128
NB = S // LANE
AR = 32
A_STEPS = M // AR
LOG2E = 1.4426950408889634
NEG = -1e30

NT = (((1,), (1,)), ((), ()))


def _dot(a, b):
    return jnp.dot(a, b, preferred_element_type=F32)


def _dot_nt(a, b):
    return lax.dot_general(a, b, NT, preferred_element_type=F32)


def _bf(x):
    return pltpu.bitcast(x, BF16)


def _u32(x):
    return pltpu.bitcast(x, U32)


def _h(r0, n):
    return pl.ds(r0 // 2, n // 2)


def _repack(ev, od):
    lo = (ev & jnp.uint32(0xFFFF)) | (od << 16)
    hi = (ev >> 16) | (od & jnp.uint32(0xFFFF0000))
    return lo, hi


def _opaque_zero(vals):
    acc = None
    for v in vals:
        b = v if v.dtype == U32 else pltpu.bitcast(v, U32)
        for r in range(0, b.shape[0], 8):
            for c in range(0, b.shape[1], LANE):
                t = b[r:r + 8, c:c + LANE]
                acc = t if acc is None else acc | t
    return jnp.minimum((acc >> 1).astype(jnp.int32), 0)


def _pin(x, zero, r=0, c=0):
    t = pltpu.bitcast(pltpu.bitcast(x[r:r + 8, c:c + LANE], jnp.int32) + zero, x.dtype)
    row = ([x[r:r + 8, :c]] if c > 0 else []) + [t] + (
        [x[r:r + 8, c + LANE:]] if c + LANE < x.shape[1] else [])
    row = jnp.concatenate(row, axis=1) if len(row) > 1 else row[0]
    col = ([x[:r, :]] if r > 0 else []) + [row] + ([x[r + 8:, :]] if r + 8 < x.shape[0] else [])
    return jnp.concatenate(col, axis=0) if len(col) > 1 else col[0]


def _rowcat(xs):
    return jnp.concatenate(xs, axis=0) if len(xs) > 1 else xs[0]


def _lanecat(xs):
    return jnp.concatenate(xs, axis=1) if len(xs) > 1 else xs[0]


def _make_kernel(cfg):
    tq = cfg["tq"]
    nq = S // tq
    nsub = tq // LANE
    KT = MP // LANE
    TP = LANE // 2
    XC = 4
    x_cols = S // XC
    WP = 64
    WS = 3
    QIT = 8
    AT = 3

    def kernel(aq_hbm, ak_hbm, av_hbm, sh_hbm, ssm_hbm, dd_hbm, x_hbm, c_hbm,
               wq_hbm, wk_hbm, wv_hbm, wo_hbm,
               out_hbm,
               a_v, sh_v, dd_v, par_v, f_v,
               xt_v, x_v, c_v, wqs_v, wq_v, qacc, ws_v, wkv_v, wo_v,
               q_all, k_s, v_s, p_s, ra_t, rb_t, out_v,
               sem_x, sem_wq, sem_w, sem_c, sem_s, sem_a, sem_out):
        x32, c32, wq32, wk32, wv32, wo32 = (
            r.bitcast(U32) for r in (x_hbm, c_hbm, wq_hbm, wk_hbm, wv_hbm, wo_hbm))
        a32 = [r.bitcast(U32) for r in (ak_hbm, av_hbm, ssm_hbm, aq_hbm)]

        def x_copy(i):
            cs = pl.ds(i * x_cols, x_cols)
            return pltpu.make_async_copy(x32.at[:, cs], xt_v.at[:, cs], sem_x.at[i])

        def wq_copies(kt):
            dst = wqs_v.reshape(4 * KT, TP, 8, LANE)
            rs = pl.ds(min(kt * TP, M // 2 - TP), TP)
            return [pltpu.make_async_copy(
                wq32.at[rs, pl.ds(8 * (k // 2), 8), pl.ds((k % 2) * LANE, LANE)],
                dst.at[4 * kt + k], sem_wq.at[kt]) for k in range(4)]

        def wq_wait(kt):
            pltpu.make_async_copy(wqs_v.at[kt], wqs_v.at[kt], sem_wq.at[kt]).wait()

        def w_rows(chunk):
            r0 = chunk * WP
            return pl.ds(r0 if isinstance(r0, int) else pl.multiple_of(r0, WP), WP)

        def w_copies(chunk, slot):
            dst = ws_v.reshape(8 * WS, WP, 8, LANE)
            rs = w_rows(chunk)
            out = []
            for which, src in enumerate((wk32, wv32)):
                for par in range(2):
                    for half in range(2):
                        k = 8 * slot + 4 * which + 2 * par + half
                        out.append(pltpu.make_async_copy(
                            src.at[rs, pl.ds(8 * par, 8), pl.ds(half * LANE, LANE)],
                            dst.at[k], sem_w.at[slot]))
            return out

        def w_wait(slot):
            pltpu.make_async_copy(ws_v.at[slot], ws_v.at[slot], sem_w.at[slot]).wait()

        def c_copy(it):
            n = S // 2 // QIT
            rs = pl.ds(pl.multiple_of(it * n, n), n)
            return pltpu.make_async_copy(c32.at[rs], c_v.at[rs], sem_c.at[it])

        wo_copy = pltpu.make_async_copy(wo32, wo_v, sem_a.at[0])
        a_parts = [pl.ds(0, AR // 2), pl.ds(AR // 2, M // 2 - AR // 2)]

        def a_start(part):
            rs = a_parts[part]
            for k in range(4):
                pltpu.make_async_copy(a32[k].at[rs], a_v.at[k, rs], sem_a.at[1 + part]).start()

        def a_wait(part):
            view = a_v.at[:, a_parts[part]]
            pltpu.make_async_copy(view, view, sem_a.at[1 + part]).wait()

        small = [pltpu.make_async_copy(sh_hbm, sh_v, sem_s.at[0]),
                 pltpu.make_async_copy(dd_hbm, dd_v, sem_s.at[1])]

        link = [None]

        pace = [None]

        def set_link(res, row=None, pacer=None):
            if row is None:
                row = res.shape[0] - cfg["link_back"]
            link[0] = _opaque_zero([res[row:row + 8, res.shape[1] - LANE:]])
            pace[0] = res if pacer is None else pacer

        def linked(x):
            return x if link[0] is None else _pin(x, link[0])

        def paced(w):
            res = pace[0]
            if res is None or link[0] is None or not cfg["pace_step"]:
                return w
            rows = []
            zs = [_opaque_zero([res[r:r + 8, res.shape[1] - LANE:]])
                  for r in range(cfg["pace_row"], cfg["pace_row"] + 8 * cfg["pace_step"],
                                 cfg["pace_step"])]
            for r in range(0, w.shape[0], 8):
                z = zs[7 - (r // 8) % 8]
                t = pltpu.bitcast(w[r:r + 8, :], jnp.int32)
                rows.append(pltpu.bitcast(t + _lanecat([z] * (w.shape[1] // LANE)), U32))
            return _rowcat(rows)

        with jax.named_scope("first_starts"):
            for cp in small:
                cp.start()
        x_copy(0).start()
        for kt in range(cfg["wq_first"]):
            for cp in wq_copies(kt):
                cp.start()

        bi = lax.broadcasted_iota(jnp.int32, (LANE, LANE), 0)
        mi = lax.broadcasted_iota(jnp.int32, (LANE, LANE), 1)
        ph = ((4 * mi + 1) * bi) & 511
        ang = ph.astype(F32) * (2.0 * 3.141592653589793 / 512.0)
        f_v[:, 0:LANE] = _u32(jnp.cos(ang).astype(BF16))
        f_v[:, LANE:] = _u32((-jnp.sin(ang)).astype(BF16))

        rb_t[...] = jnp.zeros((S // D, M, D), F32)

        for kt in range(cfg["wq_first"], KT):
            for cp in wq_copies(kt):
                cp.start()
        with jax.named_scope("small_wait"):
            for cp in small:
                cp.wait()
        sh = sh_v[...].astype(F32)
        for j in range(KS):
            par_v[j] = jnp.broadcast_to(sh[j:j + 1, :], (LANE, M)).T
        dd = dd_v[...].astype(F32).reshape(1, M)
        par_v[KS] = jnp.broadcast_to(dd, (LANE, M)).T

        def x_transpose(i):
            xt = xt_v[:, pl.ds(i * x_cols, x_cols)]
            nfull = (KT - 1) * TP
            xt = _rowcat([xt[:nfull], jnp.zeros((MP // 2 - M // 2, x_cols), U32), xt[nfull:]])
            x_v[_h(i * x_cols, x_cols), :] = _u32(_bf(xt).astype(F32).T.astype(BF16))

        def q_early(kt, first, last):
            r0 = kt * TP
            rows = pl.ds(r0 if isinstance(r0, int) else pl.multiple_of(r0, TP), TP)
            c0 = kt * LANE
            cols = pl.ds(c0 if isinstance(c0, int) else pl.multiple_of(c0, LANE), LANE)
            link[0] = None
            for j in range(H // 2):
                ws = []
                for half in range(2):
                    ev, od = (
                        wqs_v[kt, pl.ds((2 * par + half) * TP * 8 + j, TP, stride=8), :]
                        for par in range(2))
                    ws.append(_repack(ev, od))
                w = _lanecat([ws[0][0], ws[1][0], ws[0][1], ws[1][1]])
                wq_v[j, rows, :] = w
                d = _dot(_bf(linked(x_v[_h(0, x_cols), cols])), _bf(w))
                set_link(d)
                if not first:
                    d = d + qacc[j]
                if last:
                    d = (d * (D ** -0.5 * LOG2E)).astype(BF16)
                    for t in range(2):
                        q_all[2 * j + t, _h(0, x_cols), :] = _u32(d[:, t * D:(t + 1) * D])
                else:
                    qacc[j] = d

        with jax.named_scope("x_wait"):
            x_copy(0).wait()
        x_transpose(0)
        with jax.named_scope("wq_wait"):
            wq_wait(0)
        q_early(0, True, False)
        for i in range(1, XC):
            x_copy(i).start()

        def early_body(kt, carry):
            with jax.named_scope("wq_wait"):
                wq_wait(kt)
            q_early(kt, False, False)
            for cp in w_copies(kt - 1, kt - 1):
                cp.start()
            return carry

        lax.fori_loop(1, KT - 1, early_body, 0)
        with jax.named_scope("wq_wait"):
            wq_wait(KT - 1)
            for i in range(1, XC):
                x_copy(i).wait()
        q_early(KT - 1, False, True)
        for i in range(1, XC):
            x_transpose(i)

        def unpack(chunk, slot, which, half, j):
            ev, od = (
                ws_v[slot, pl.ds((4 * which + 2 * par + half) * WP * 8 + j, WP, stride=8), :]
                for par in range(2))
            lo, hi = _repack(ev, od)
            rows = w_rows(chunk)
            cols = pl.ds(which * D + half * LANE, LANE)
            wkv_v[2 * j, rows, cols] = lo
            wkv_v[2 * j + 1, rows, cols] = hi
            return [lo, hi]

        units = [(w_, h_, j_) for w_ in range(2) for h_ in range(2) for j_ in range(H // 2)]

        def qproj(it, r0, n, t, zeros=(None, None)):
            outs = []
            for u in range(2):
                lhs = _bf(linked(x_v[_h(r0, n), :]))
                d = _dot(lhs, _bf(wq_v[it, :, pl.ds(t * D + u * LANE, LANE)]))
                set_link(d)
                if zeros[u] is not None:
                    for k, z in enumerate(zeros[u]):
                        d = _pin(d, z, 8 * ((k * (n // 8)) // len(zeros[u])))
                outs.append(d)
            q2 = _lanecat(outs)
            q_all[2 * it + t, _h(r0, n), :] = _u32((q2 * (D ** -0.5 * LOG2E)).astype(BF16))

        def q_body(it, carry):
            slot = it % WS

            def q_prefetch():
                c_copy(it).start()

                @pl.when(it + 2 < QIT)
                def _():
                    for cp in w_copies(it + 2, (it + 2) % WS):
                        cp.start()

                @pl.when(it == QIT - 2)
                def _():
                    wo_copy.start()
                    a_start(0)

            if cfg["q_pf"] == -2:
                q_prefetch()
            with jax.named_scope("w_wait"):
                w_wait(slot)
            if cfg["q_pf"] == -1:
                q_prefetch()
            link[0] = None
            pieces = [(pc, t) for pc in range(1, XC) for t in range(2)]
            nd = 2 * len(pieces)
            for k, (pc, t) in enumerate(pieces):
                zeros = []
                for u in range(2):
                    d = 2 * k + u
                    mine = units[d * len(units) // nd:(d + 1) * len(units) // nd]
                    zeros.append([_opaque_zero(unpack(it, slot, *u_)) for u_ in mine])
                qproj(it, pc * x_cols, x_cols, t, zeros)
                if k == cfg["q_pf"]:
                    q_prefetch()
            return carry

        with jax.named_scope("q_loop"):
            lax.fori_loop(0, QIT, q_body, 0)
        a_start(1)
        for it in range(QIT):
            c_copy(it).wait()
        a_wait(0)
        wo_copy.wait()

        tri = (lax.broadcasted_iota(jnp.int32, (LANE, LANE), 1)
               <= lax.broadcasted_iota(jnp.int32, (LANE, LANE), 0))

        def out_copy(i):
            if i == S // D:
                cs = pl.ds(0, AT * LANE)
                return pltpu.make_async_copy(out_v.at[:, cs], out_hbm.at[:, cs], sem_out.at[i])
            rs, cs = pl.ds(i * D, D), pl.ds(AT * LANE, 2 * M - AT * LANE)
            return pltpu.make_async_copy(out_v.at[rs, cs], out_hbm.at[rs, cs], sem_out.at[i])

        def a_out():
            for i in range(S // tq):
                cols = slice(i * tq, (i + 1) * tq)
                out_v[cols, 0:AT * LANE] = ra_t[0:AT * LANE, cols].T.astype(BF16)
            out_copy(S // D).start()

        def head_step(h, carry):
            with jax.named_scope("step"):
                return head_step_(h, carry)

        def head_step_(h, carry):
            with_a = cfg["use_a"]

            if cfg["a_out"] == 0:
                pl.when(h == A_STEPS)(a_out)

            @pl.when(h == cfg["h0"] + 1)
            def _():
                a_wait(1)

            link[0] = None
            n2 = AR // 2
            a_rows2 = pl.ds(pl.multiple_of(jnp.minimum(h, A_STEPS - 1) * n2, n2), n2)
            a_rows = pl.ds(pl.multiple_of(jnp.minimum(h, A_STEPS - 1) * AR, AR), AR)

            def a_fwd():
                kk = _bf(a_v[0, a_rows2, :]).astype(F32)
                lane = lax.broadcasted_iota(jnp.int32, (AR, LANE), 1)
                coef = [par_v[j, a_rows, :] for j in range(KS)]
                rolled = [kk] + [pltpu.roll(kk, j, 1) for j in range(1, KS)]
                vv = _bf(a_v[1, a_rows2, :]).astype(F32)
                kv_blocks = []
                for a in range(NB):
                    cs = slice(a * LANE, (a + 1) * LANE)
                    acc = rolled[0][:, cs] * coef[0]
                    for j in range(1, KS):
                        t = rolled[j][:, cs]
                        if a == 0:
                            t = jnp.where(lane >= j, t, 0.0)
                        acc = acc + t * coef[j]
                    kv_blocks.append(acc * vv[:, cs])
                hk = a_v[2, a_rows2, :]
                hk = _rowcat([hk[:, a * LANE:(a + 1) * LANE] for a in range(NB)])
                fm = _bf(f_v[...])
                hs = _dot(_bf(linked(hk)), fm)
                kv = linked(_rowcat(kv_blocks)).astype(BF16)
                xs = _dot(kv, fm)
                set_link(xs)
                return kv, xs, hs

            def a_conv(xs, hs):
                def tile(v, a, g, part):
                    r = a * AR + 8 * g
                    return v[r:r + 8, part * LANE:(part + 1) * LANE]

                z = {}
                nch = cfg["a_chains"]
                gates = [None] * nch
                width = cfg["a_width"]
                k = 0
                for g in range(AR // 8):
                    hr = [tile(hs, 0, g, 0)] + [
                        tile(hs, j, g, 0) - tile(hs, j - 1, g, 1) for j in range(1, NB)]
                    hi = [tile(hs, 0, g, 1)] + [
                        tile(hs, j, g, 1) + tile(hs, j - 1, g, 0) for j in range(1, NB)]
                    for c0 in range(0, NB, width):
                        ch = k % nch
                        k += 1
                        for a in range(c0 + width):
                            xr, xi = tile(xs, a, g, 0), tile(xs, a, g, 1)
                            if gates[ch] is not None and cfg["a_gate"]:
                                xr, xi = _pin(xr, gates[ch]), _pin(xi, gates[ch])
                            for c in range(max(c0, a), c0 + width):
                                j = c - a
                                tr = xr * hr[j] - xi * hi[j]
                                ti = xr * hi[j] + xi * hr[j]
                                z[c, g] = (tr, ti) if a == 0 else (z[c, g][0] + tr, z[c, g][1] + ti)
                            gates[ch] = _opaque_zero(list(z[c0 + width - 1, g]))
                return z

            def a_inv(kv, z):
                fm = _bf(f_v[...])
                ng = AR // 8
                ys = []
                for u in range(2):
                    rows = [_lanecat(z[c, g]) for g in range(u * ng // 2, (u + 1) * ng // 2)
                            for c in range(NB)]
                    ys.append(_dot_nt(linked(_rowcat(rows)).astype(BF16), fm))
                y = _rowcat(ys)
                dd = par_v[KS, a_rows, :]
                for c in range(NB):
                    cs = slice(c * LANE, (c + 1) * LANE)
                    yc = _rowcat([y[(g * NB + c) * 8:(g * NB + c + 1) * 8, :] for g in range(ng)])
                    qq = _bf(a_v[3, a_rows2, cs]).astype(F32)
                    kvf = kv[c * AR:(c + 1) * AR, :].astype(F32)
                    ra_t[a_rows, cs] = qq * (yc * (1.0 / LANE) + kvf * dd)

            kw = C // 2

            def proj_w(which, k):
                return wkv_v[h, _h((k % 2) * kw, kw), pl.ds(which * D + (k // 2) * LANE, LANE)]

            def proj(dst, which, r0, n):
                ds = []
                for k in range(4):
                    lhs = linked(c_v[_h(r0, n), pl.ds((k % 2) * kw, kw)])
                    ds.append(_dot(_bf(lhs), _bf(paced(proj_w(which, k)))))
                    set_link(ds[-1])
                dst[r0:r0 + n, :] = _lanecat([ds[0] + ds[1], ds[2] + ds[3]]).astype(BF16)

            def qk(i):
                r0 = i * tq
                parts = [_dot_nt(_bf(linked(q_all[h, _h(r0, tq), :])), k_s[0:r0 + LANE, :])]
                if i > 0:
                    link[0] = _opaque_zero([parts[0][0:8, r0 - LANE:r0]])
                for j in range(1, nsub):
                    q = linked(q_all[h, _h(r0 + LANE * j, tq - LANE * j), :])
                    parts.append(_dot_nt(_bf(q), k_s[r0 + LANE * j:r0 + LANE * (j + 1), :]))
                set_link(parts[2], cfg["link_part"], parts[0])
                return parts

            def softmax(i, parts):
                pb = p_s.at[i % 2]
                chain = _opaque_zero([b[b.shape[0] - 8:, b.shape[1] - LANE:] for b in parts])
                ls = []
                for a in range(nsub):
                    blocks = [parts[j][LANE * (a - j):LANE * (a - j + 1), :] for j in range(a + 1)]
                    last = blocks[-1]
                    w = last.shape[1]
                    dg = jnp.where(tri, last[:, w - LANE:], NEG)
                    blocks[-1] = dg if w == LANE else _lanecat([last[:, :w - LANE], dg])
                    sa = _lanecat(blocks)
                    if cfg["dbg"] & 4:
                        ls.append(jnp.ones((LANE, 1), F32))
                        p = _pin(sa, link[0], 0, 0 if a == 0 else sa.shape[1] - LANE)
                        pb[LANE * a:LANE * (a + 1), 0:sa.shape[1]] = p.astype(BF16)
                        continue
                    mb = jnp.broadcast_to(jnp.max(sa, axis=1, keepdims=True), (LANE, LANE))
                    nt = sa.shape[1] // LANE
                    ptiles, psums = [], []
                    for g in range(0, LANE, 8):
                        mg = _pin(mb[g:g + 8, :], chain)
                        pg = [jnp.exp2(sa[g:g + 8, t * LANE:(t + 1) * LANE] - mg) for t in range(nt)]
                        ps = functools.reduce(jnp.add, pg)
                        chain = _opaque_zero([ps])
                        psums.append(ps)
                        ptiles.append(_lanecat(pg))
                    ls.append(jnp.sum(_rowcat(psums), axis=1, keepdims=True))
                    p = _pin(_rowcat(ptiles), link[0], 0, 0 if a == 0 else sa.shape[1] - LANE)
                    pb[LANE * a:LANE * (a + 1), 0:sa.shape[1]] = p.astype(BF16)
                return ls

            def pv(i, ls):
                r0 = i * tq
                pb = p_s.at[i % 2]
                ctx = [_dot(pb[:, 0:r0 + LANE], v_s[0:r0 + LANE, :])]
                for j in range(1, nsub):
                    ctx.append(_dot(pb[LANE * j:, r0 + LANE * j:r0 + LANE * (j + 1)],
                                    v_s[r0 + LANE * j:r0 + LANE * (j + 1), :]))
                set_link(ctx[2], cfg["link_part"])
                cs = []
                for a in range(nsub):
                    sl = lambda j: slice(LANE * (a - j), LANE * (a - j + 1))
                    r = pl.reciprocal(ls[a], approx=True)
                    r = r * (2.0 - ls[a] * r)
                    cs.append(functools.reduce(jnp.add, [ctx[j][sl(j)] for j in range(a + 1)]) * r)
                return _rowcat(cs).astype(BF16)

            def oproj(i, ctx):
                for u in range(tq // D):
                    res = _dot_nt(_bf(linked(wo_v[h])), ctx[u * D:(u + 1) * D, :])
                    set_link(res)
                    rb_t[i * (tq // D) + u] += res

            a_state = {}

            def a_hook(tag):
                if with_a and tag == cfg["a_fwd_at"]:
                    a_state["kv"], xs, hs = a_fwd()
                    a_state["z"] = a_conv(xs, hs)
                if with_a and tag == cfg["a_inv_at"]:
                    a_inv(a_state["kv"], a_state["z"])

            a_hook(0)
            proj(k_s, 0, 0, tq)
            a_hook(1)
            parts = qk(0)
            ctx_prev = None
            for i in range(nq):
                r0 = i * tq
                a_hook(10 * (i + 1))
                if ctx_prev is not None:
                    oproj(i - 1, ctx_prev)
                a_hook(10 * (i + 1) + 1)
                if i + 1 < nq:
                    proj(k_s, 0, r0 + tq, tq)
                a_hook(10 * (i + 1) + 2)
                proj(v_s, 1, r0, tq)
                a_hook(10 * (i + 1) + 3)
                ls = softmax(i, parts)
                ctx_prev = pv(i, ls)
                a_hook(10 * (i + 1) + 4)
                if i + 1 < nq:
                    parts = qk(i + 1)
            oproj(nq - 1, ctx_prev)
            return carry

        with jax.named_scope("loop_a"):
            lax.fori_loop(cfg["h0"], H, head_step, 0)
        with jax.named_scope("tail"):
            if cfg["a_out"] == 1:
                a_out()
            for i in range(S // D):
                cols = slice(i * D, (i + 1) * D)
                full = _rowcat([ra_t[AT * LANE:, cols], rb_t[i]])
                out_v[cols, AT * LANE:] = full.T.astype(BF16)
                out_copy(i).start()
            for i in range(S // D + 1):
                out_copy(i).wait()

    scratch = [
        pltpu.VMEM((4, M // 2, S), U32),
        pltpu.VMEM((KS, M), BF16),
        pltpu.VMEM((M,), BF16),
        pltpu.VMEM((KS + 1, M, LANE), F32),
        pltpu.VMEM((LANE // 2, 2 * LANE), U32),
        pltpu.VMEM((M // 2, S), U32),
        pltpu.VMEM((S // 2, MP), U32),
        pltpu.VMEM((S // 2, C), U32),
        pltpu.VMEM((KT, 4 * TP * 8, LANE), U32),
        pltpu.VMEM((H // 2, MP // 2, 2 * D), U32),
        pltpu.VMEM((H // 2, x_cols, 2 * D), F32),
        pltpu.VMEM((WS, 8 * WP * 8, LANE), U32),
        pltpu.VMEM((H, C // 2, 2 * D), U32),
        pltpu.VMEM((H, M // 2, D), U32),
        pltpu.VMEM((H, S // 2, D), U32),
        pltpu.VMEM((S, D), BF16),
        pltpu.VMEM((S, D), BF16),
        pltpu.VMEM((2, tq, S), BF16),
        pltpu.VMEM((M, S), F32),
        pltpu.VMEM((S // D, M, D), F32),
        pltpu.VMEM((S, 2 * M), BF16),
        pltpu.SemaphoreType.DMA((XC,)),
        pltpu.SemaphoreType.DMA((KT,)),
        pltpu.SemaphoreType.DMA((WS,)),
        pltpu.SemaphoreType.DMA((QIT,)),
        pltpu.SemaphoreType.DMA((2,)),
        pltpu.SemaphoreType.DMA((3,)),
        pltpu.SemaphoreType.DMA((S // D + 1,)),
    ]
    return kernel, scratch


_DEFAULT = dict(tq=512, a_fwd_at=13, a_inv_at=44, a_gate=1, a_chains=1, a_width=4, a_out=0, dbg=0, q_pf=-1, wq_first=1,
                link_back=176, pace_row=32, pace_step=24, link_part=32, use_a=1, h0=0)


def _build(**kw):
    cfg = dict(_DEFAULT)
    cfg.update(kw)
    kernel, scratch = _make_kernel(cfg)

    def run(A_q, A_k, A_v, A_shift_k, A_ssm_k, A_ssm_D, B_x, B_c_kv, B_w_q, B_w_uk,
            B_w_uv, B_w_o):
        tr = lambda a: jnp.swapaxes(a, 1, 2).reshape(M, S)
        args = (
            tr(A_q), tr(A_k), tr(A_v), A_shift_k.T, A_ssm_k, A_ssm_D, tr(B_x),
            B_c_kv.reshape(S, C),
            B_w_q.reshape(M // 2, 2 * H, D), B_w_uk.reshape(C // 2, 2 * H, D),
            B_w_uv.reshape(C // 2, 2 * H, D),
            jnp.swapaxes(B_w_o, 1, 2),
        )
        out = pl.pallas_call(
            kernel,
            in_specs=[pl.BlockSpec(memory_space=pl.ANY)] * len(args),
            out_specs=pl.BlockSpec(memory_space=pl.ANY),
            out_shape=jax.ShapeDtypeStruct((S, 2 * M), BF16),
            scratch_shapes=scratch,
            compiler_params=pltpu.CompilerParams(
                vmem_limit_bytes=120 * 1024 * 1024,
                disable_bounds_checks=True),
        )(*args)
        return out.reshape(1, S, 2 * M)

    return run


_run = _build()


@jax.jit
def pallas_concat_heads__ssm_conv_h3__compressed_kv_cla__prompt_kernel(
    A_q: jax.Array,
    A_k: jax.Array,
    A_v: jax.Array,
    A_shift_k: jax.Array,
    A_ssm_k: jax.Array,
    A_ssm_D: jax.Array,
    B_x: jax.Array,
    B_c_kv: jax.Array,
    B_w_q: jax.Array,
    B_w_uk: jax.Array,
    B_w_uv: jax.Array,
    B_w_o: jax.Array,
):
    return _run(A_q, A_k, A_v, A_shift_k, A_ssm_k, A_ssm_D, B_x, B_c_kv, B_w_q,
                B_w_uk, B_w_uv, B_w_o)
```

```python
import functools

import jax
import jax.numpy as jnp
from jax import lax
import jax.experimental.pallas as pl
import jax.experimental.pallas.tpu as pltpu

F32 = jnp.float32
BF16 = jnp.bfloat16
U32 = jnp.uint32

S = 2048
M = 448
MP = 512
C = 1024
H = 16
D = 256
KS = 4
LANE = 128
NB = S // LANE
AR = 32
A_STEPS = M // AR
LOG2E = 1.4426950408889634
NEG = -1e30

NT = (((1,), (1,)), ((), ()))


def _dot(a, b):
    return jnp.dot(a, b, preferred_element_type=F32)


def _dot_nt(a, b):
    return lax.dot_general(a, b, NT, preferred_element_type=F32)


def _bf(x):
    return pltpu.bitcast(x, BF16)


def _u32(x):
    return pltpu.bitcast(x, U32)


def _h(r0, n):
    return pl.ds(r0 // 2, n // 2)


def _repack(ev, od):
    lo = (ev & jnp.uint32(0xFFFF)) | (od << 16)
    hi = (ev >> 16) | (od & jnp.uint32(0xFFFF0000))
    return lo, hi


def _opaque_zero(vals):
    acc = None
    for v in vals:
        b = v if v.dtype == U32 else pltpu.bitcast(v, U32)
        for r in range(0, b.shape[0], 8):
            for c in range(0, b.shape[1], LANE):
                t = b[r:r + 8, c:c + LANE]
                acc = t if acc is None else acc | t
    return jnp.minimum((acc >> 1).astype(jnp.int32), 0)


def _pin(x, zero, r=0, c=0):
    t = pltpu.bitcast(pltpu.bitcast(x[r:r + 8, c:c + LANE], jnp.int32) + zero, x.dtype)
    row = ([x[r:r + 8, :c]] if c > 0 else []) + [t] + (
        [x[r:r + 8, c + LANE:]] if c + LANE < x.shape[1] else [])
    row = jnp.concatenate(row, axis=1) if len(row) > 1 else row[0]
    col = ([x[:r, :]] if r > 0 else []) + [row] + ([x[r + 8:, :]] if r + 8 < x.shape[0] else [])
    return jnp.concatenate(col, axis=0) if len(col) > 1 else col[0]


def _rowcat(xs):
    return jnp.concatenate(xs, axis=0) if len(xs) > 1 else xs[0]


def _lanecat(xs):
    return jnp.concatenate(xs, axis=1) if len(xs) > 1 else xs[0]


def _make_kernel(cfg):
    tq = cfg["tq"]
    nq = S // tq
    nsub = tq // LANE
    KT = MP // LANE
    TP = LANE // 2
    XC = 4
    x_cols = S // XC
    WP = 64
    WS = 3
    QIT = 8
    AT = 3

    def kernel(aq_hbm, ak_hbm, av_hbm, sh_hbm, ssm_hbm, dd_hbm, x_hbm, c_hbm,
               wq_hbm, wk_hbm, wv_hbm, wo_hbm,
               out_hbm,
               a_v, sh_v, dd_v, par_v, f_v,
               xt_v, x_v, c_v, wqs_v, wq_v, qacc, ws_v, wkv_v, wo_v,
               q_all, k_s, v_s, p_s, ra_t, rb_t, oa_v, out_v,
               sem_x, sem_wq, sem_w, sem_c, sem_s, sem_a, sem_out):
        x32, c32, wq32, wk32, wv32, wo32 = (
            r.bitcast(U32) for r in (x_hbm, c_hbm, wq_hbm, wk_hbm, wv_hbm, wo_hbm))
        a32 = [r.bitcast(U32) for r in (ak_hbm, av_hbm, ssm_hbm, aq_hbm)]

        def x_copy(i):
            cs = pl.ds(i * x_cols, x_cols)
            return pltpu.make_async_copy(x32.at[:, cs], xt_v.at[:, cs], sem_x.at[i])

        def wq_copies(kt):
            dst = wqs_v.reshape(4 * KT, TP, 8, LANE)
            rs = pl.ds(min(kt * TP, M // 2 - TP), TP)
            return [pltpu.make_async_copy(
                wq32.at[rs, pl.ds(8 * (k // 2), 8), pl.ds((k % 2) * LANE, LANE)],
                dst.at[4 * kt + k], sem_wq.at[kt]) for k in range(4)]

        def wq_wait(kt):
            pltpu.make_async_copy(wqs_v.at[kt], wqs_v.at[kt], sem_wq.at[kt]).wait()

        def w_rows(chunk):
            r0 = chunk * WP
            return pl.ds(r0 if isinstance(r0, int) else pl.multiple_of(r0, WP), WP)

        def w_copies(chunk, slot):
            dst = ws_v.reshape(8 * WS, WP, 8, LANE)
            rs = w_rows(chunk)
            out = []
            for which, src in enumerate((wk32, wv32)):
                for par in range(2):
                    for half in range(2):
                        k = 8 * slot + 4 * which + 2 * par + half
                        out.append(pltpu.make_async_copy(
                            src.at[rs, pl.ds(8 * par, 8), pl.ds(half * LANE, LANE)],
                            dst.at[k], sem_w.at[slot]))
            return out

        def w_wait(slot):
            pltpu.make_async_copy(ws_v.at[slot], ws_v.at[slot], sem_w.at[slot]).wait()

        def c_copy(it):
            n = S // 2 // QIT
            rs = pl.ds(pl.multiple_of(it * n, n), n)
            return pltpu.make_async_copy(c32.at[rs], c_v.at[rs], sem_c.at[it])

        wo_copy = pltpu.make_async_copy(wo32, wo_v, sem_a.at[0])
        a_parts = [pl.ds(0, AR // 2), pl.ds(AR // 2, M // 2 - AR // 2)]

        def a_start(part):
            rs = a_parts[part]
            for k in range(4):
                pltpu.make_async_copy(a32[k].at[rs], a_v.at[k, rs], sem_a.at[1 + part]).start()

        def a_wait(part):
            view = a_v.at[:, a_parts[part]]
            pltpu.make_async_copy(view, view, sem_a.at[1 + part]).wait()

        small = [pltpu.make_async_copy(sh_hbm, sh_v, sem_s.at[0]),
                 pltpu.make_async_copy(dd_hbm, dd_v, sem_s.at[1])]

        link = [None]

        pace = [None]

        def set_link(res, row=None, pacer=None):
            if row is None:
                row = res.shape[0] - cfg["link_back"]
            link[0] = _opaque_zero([res[row:row + 8, res.shape[1] - LANE:]])
            pace[0] = res if pacer is None else pacer

        def linked(x):
            return x if link[0] is None else _pin(x, link[0])

        def paced(w):
            res = pace[0]
            if res is None or link[0] is None or not cfg["pace_step"]:
                return w
            rows = []
            zs = [_opaque_zero([res[r:r + 8, res.shape[1] - LANE:]])
                  for r in range(cfg["pace_row"], cfg["pace_row"] + 8 * cfg["pace_step"],
                                 cfg["pace_step"])]
            for r in range(0, w.shape[0], 8):
                z = zs[7 - (r // 8) % 8]
                t = pltpu.bitcast(w[r:r + 8, :], jnp.int32)
                rows.append(pltpu.bitcast(t + _lanecat([z] * (w.shape[1] // LANE)), U32))
            return _rowcat(rows)

        with jax.named_scope("first_starts"):
            for cp in small:
                cp.start()
        x_copy(0).start()
        for kt in range(cfg["wq_first"]):
            for cp in wq_copies(kt):
                cp.start()

        bi = lax.broadcasted_iota(jnp.int32, (LANE, LANE), 0)
        mi = lax.broadcasted_iota(jnp.int32, (LANE, LANE), 1)
        ph = ((4 * mi + 1) * bi) & 511
        ang = ph.astype(F32) * (2.0 * 3.141592653589793 / 512.0)
        f_v[:, 0:LANE] = _u32(jnp.cos(ang).astype(BF16))
        f_v[:, LANE:] = _u32((-jnp.sin(ang)).astype(BF16))

        rb_t[...] = jnp.zeros((S // D, M, D), F32)
        ra_t[:, 0:LANE, :] = jnp.zeros((2, LANE, S // 2), F32)

        for kt in range(cfg["wq_first"], KT):
            for cp in wq_copies(kt):
                cp.start()
        with jax.named_scope("small_wait"):
            for cp in small:
                cp.wait()
        sh = sh_v[...].astype(F32)
        for j in range(KS):
            par_v[j] = jnp.broadcast_to(sh[j:j + 1, :], (LANE, M)).T
        dd = dd_v[...].astype(F32).reshape(1, M)
        par_v[KS] = jnp.broadcast_to(dd, (LANE, M)).T

        def x_transpose(i):
            xt = xt_v[:, pl.ds(i * x_cols, x_cols)]
            nfull = (KT - 1) * TP
            xt = _rowcat([xt[:nfull], jnp.zeros((MP // 2 - M // 2, x_cols), U32), xt[nfull:]])
            x_v[_h(i * x_cols, x_cols), :] = _u32(_bf(xt).astype(F32).T.astype(BF16))

        def q_early(kt, first, last):
            r0 = kt * TP
            rows = pl.ds(r0 if isinstance(r0, int) else pl.multiple_of(r0, TP), TP)
            c0 = kt * LANE
            cols = pl.ds(c0 if isinstance(c0, int) else pl.multiple_of(c0, LANE), LANE)
            link[0] = None
            for j in range(H // 2):
                ws = []
                for half in range(2):
                    ev, od = (
                        wqs_v[kt, pl.ds((2 * par + half) * TP * 8 + j, TP, stride=8), :]
                        for par in range(2))
                    ws.append(_repack(ev, od))
                w = _lanecat([ws[0][0], ws[1][0], ws[0][1], ws[1][1]])
                wq_v[j, rows, :] = w
                d = _dot(_bf(linked(x_v[_h(0, x_cols), cols])), _bf(w))
                set_link(d)
                if not first:
                    d = d + qacc[j]
                if last:
                    d = (d * (D ** -0.5 * LOG2E)).astype(BF16)
                    for t in range(2):
                        q_all[2 * j + t, _h(0, x_cols), :] = _u32(d[:, t * D:(t + 1) * D])
                else:
                    qacc[j] = d

        with jax.named_scope("x_wait"):
            x_copy(0).wait()
        x_transpose(0)
        with jax.named_scope("wq_wait"):
            wq_wait(0)
        q_early(0, True, False)
        for i in range(1, XC):
            x_copy(i).start()

        def early_body(kt, carry):
            with jax.named_scope("wq_wait"):
                wq_wait(kt)
            q_early(kt, False, False)
            for cp in w_copies(kt - 1, kt - 1):
                cp.start()
            return carry

        lax.fori_loop(1, KT - 1, early_body, 0)
        with jax.named_scope("wq_wait"):
            wq_wait(KT - 1)
            for i in range(1, XC):
                x_copy(i).wait()
        q_early(KT - 1, False, True)
        for i in range(1, XC):
            x_transpose(i)

        def unpack(chunk, slot, which, half, j):
            ev, od = (
                ws_v[slot, pl.ds((4 * which + 2 * par + half) * WP * 8 + j, WP, stride=8), :]
                for par in range(2))
            lo, hi = _repack(ev, od)
            rows = w_rows(chunk)
            cols = pl.ds(which * D + half * LANE, LANE)
            wkv_v[2 * j, rows, cols] = lo
            wkv_v[2 * j + 1, rows, cols] = hi
            return [lo, hi]

        units = [(w_, h_, j_) for w_ in range(2) for h_ in range(2) for j_ in range(H // 2)]

        def qproj(it, r0, n, t, zeros=(None, None)):
            outs = []
            for u in range(2):
                lhs = _bf(linked(x_v[_h(r0, n), :]))
                d = _dot(lhs, _bf(wq_v[it, :, pl.ds(t * D + u * LANE, LANE)]))
                set_link(d)
                if zeros[u] is not None:
                    for k, z in enumerate(zeros[u]):
                        d = _pin(d, z, 8 * ((k * (n // 8)) // len(zeros[u])))
                outs.append(d)
            q2 = _lanecat(outs)
            q_all[2 * it + t, _h(r0, n), :] = _u32((q2 * (D ** -0.5 * LOG2E)).astype(BF16))

        def q_body(it, carry):
            slot = it % WS

            def q_prefetch():
                c_copy(it).start()

                @pl.when(it + 2 < QIT)
                def _():
                    for cp in w_copies(it + 2, (it + 2) % WS):
                        cp.start()

                @pl.when(it == QIT - 2)
                def _():
                    wo_copy.start()
                    a_start(0)

            if cfg["q_pf"] == -2:
                q_prefetch()
            with jax.named_scope("w_wait"):
                w_wait(slot)
            if cfg["q_pf"] == -1:
                q_prefetch()
            link[0] = None
            pieces = [(pc, t) for pc in range(1, XC) for t in range(2)]
            nd = 2 * len(pieces)
            for k, (pc, t) in enumerate(pieces):
                zeros = []
                for u in range(2):
                    d = 2 * k + u
                    mine = units[d * len(units) // nd:(d + 1) * len(units) // nd]
                    zeros.append([_opaque_zero(unpack(it, slot, *u_)) for u_ in mine])
                qproj(it, pc * x_cols, x_cols, t, zeros)
                if k == cfg["q_pf"]:
                    q_prefetch()
            return carry

        with jax.named_scope("q_loop"):
            lax.fori_loop(0, QIT, q_body, 0)
        a_start(1)
        for it in range(QIT):
            c_copy(it).wait()
        a_wait(0)
        wo_copy.wait()

        tri = (lax.broadcasted_iota(jnp.int32, (LANE, LANE), 1)
               <= lax.broadcasted_iota(jnp.int32, (LANE, LANE), 0))

        NOUT = S // D

        def out_copy(i):
            if i >= NOUT:
                t = i - NOUT
                return pltpu.make_async_copy(
                    oa_v.at[t], out_hbm.at[:, pl.ds(t * LANE, LANE)], sem_out.at[i])
            rs = pl.ds(i * D, D)
            return pltpu.make_async_copy(
                out_v.at[rs], out_hbm.at[rs, pl.ds(AT * LANE, 2 * M - AT * LANE)], sem_out.at[i])

        def head_step(h, carry):
            with jax.named_scope("step"):
                return head_step_(h, carry)

        def head_step_(h, carry):
            with_a = cfg["use_a"]

            @pl.when(h == H - 1)
            def _():
                for t in range(AT):
                    out_copy(NOUT + t).start()

            @pl.when(h == cfg["h0"] + 1)
            def _():
                a_wait(1)

            link[0] = None
            n2 = AR // 2
            a_rows2 = pl.ds(pl.multiple_of(jnp.minimum(h, A_STEPS - 1) * n2, n2), n2)
            a_rows = pl.ds(pl.multiple_of(jnp.minimum(h, A_STEPS - 1) * AR, AR), AR)

            def a_fwd():
                kk = _bf(a_v[0, a_rows2, :]).astype(F32)
                lane = lax.broadcasted_iota(jnp.int32, (AR, LANE), 1)
                coef = [par_v[j, a_rows, :] for j in range(KS)]
                rolled = [kk] + [pltpu.roll(kk, j, 1) for j in range(1, KS)]
                vv = _bf(a_v[1, a_rows2, :]).astype(F32)
                kv_blocks = []
                for a in range(NB):
                    cs = slice(a * LANE, (a + 1) * LANE)
                    acc = rolled[0][:, cs] * coef[0]
                    for j in range(1, KS):
                        t = rolled[j][:, cs]
                        if a == 0:
                            t = jnp.where(lane >= j, t, 0.0)
                        acc = acc + t * coef[j]
                    kv_blocks.append(acc * vv[:, cs])
                hk = a_v[2, a_rows2, :]
                hk = _rowcat([hk[:, a * LANE:(a + 1) * LANE] for a in range(NB)])
                fm = _bf(f_v[...])
                hs = _dot(_bf(linked(hk)), fm)
                kv = linked(_rowcat(kv_blocks)).astype(BF16)
                xs = _dot(kv, fm)
                set_link(xs)
                return kv, xs, hs

            def a_conv(xs, hs):
                def tile(v, a, g, part):
                    r = a * AR + 8 * g
                    return v[r:r + 8, part * LANE:(part + 1) * LANE]

                z = {}
                nch = cfg["a_chains"]
                gates = [None] * nch
                width = cfg["a_width"]
                k = 0
                for g in range(AR // 8):
                    hr = [tile(hs, 0, g, 0)] + [
                        tile(hs, j, g, 0) - tile(hs, j - 1, g, 1) for j in range(1, NB)]
                    hi = [tile(hs, 0, g, 1)] + [
                        tile(hs, j, g, 1) + tile(hs, j - 1, g, 0) for j in range(1, NB)]
                    for c0 in range(0, NB, width):
                        ch = k % nch
                        k += 1
                        for a in range(c0 + width):
                            xr, xi = tile(xs, a, g, 0), tile(xs, a, g, 1)
                            if gates[ch] is not None and cfg["a_gate"]:
                                xr, xi = _pin(xr, gates[ch]), _pin(xi, gates[ch])
                            for c in range(max(c0, a), c0 + width):
                                j = c - a
                                tr = xr * hr[j] - xi * hi[j]
                                ti = xr * hi[j] + xi * hr[j]
                                z[c, g] = (tr, ti) if a == 0 else (z[c, g][0] + tr, z[c, g][1] + ti)
                            gates[ch] = _opaque_zero(list(z[c0 + width - 1, g]))
                return z

            def a_inv(kv, z):
                fm = _bf(f_v[...])
                ng = AR // 8
                ys = []
                for u in range(2):
                    rows = [_lanecat(z[c, g]) for g in range(u * ng // 2, (u + 1) * ng // 2)
                            for c in range(NB)]
                    ys.append(_dot_nt(linked(_rowcat(rows)).astype(BF16), fm))
                y = _rowcat(ys)
                dd = par_v[KS, a_rows, :]
                for c in range(NB):
                    cs = slice(c * LANE, (c + 1) * LANE)
                    yc = _rowcat([y[(g * NB + c) * 8:(g * NB + c + 1) * 8, :] for g in range(ng)])
                    qq = _bf(a_v[3, a_rows2, cs]).astype(F32)
                    kvf = kv[c * AR:(c + 1) * AR, :].astype(F32)
                    c2 = (c % (NB // 2)) * LANE
                    ra_t[c // (NB // 2), a_rows, c2:c2 + LANE] = qq * (yc * (1.0 / LANE) + kvf * dd)

            def a_out():
                slab = jnp.clip(h // 4 - 1, 0, AT - 1)
                half = h % 2
                x = ra_t[half, pl.ds(pl.multiple_of(slab * LANE, LANE), LANE), :]
                xt = x.T
                oa_v[slab, pl.ds(pl.multiple_of(half * (S // 2), S // 2), S // 2), :] = xt.astype(BF16)
                return xt

            kw = C // 2

            def proj_w(which, k):
                return wkv_v[h, _h((k % 2) * kw, kw), pl.ds(which * D + (k // 2) * LANE, LANE)]

            def proj(dst, which, r0, n):
                ds = []
                for k in range(4):
                    lhs = linked(c_v[_h(r0, n), pl.ds((k % 2) * kw, kw)])
                    ds.append(_dot(_bf(lhs), _bf(paced(proj_w(which, k)))))
                    set_link(ds[-1])
                dst[r0:r0 + n, :] = _lanecat([ds[0] + ds[1], ds[2] + ds[3]]).astype(BF16)

            def qk(i, dep=None):
                r0 = i * tq
                q = linked(q_all[h, _h(r0, tq), :])
                if dep is not None:
                    q = _pin(q, _opaque_zero([dep]), cfg["ao_row"])
                parts = [_dot_nt(_bf(q), k_s[0:r0 + LANE, :])]
                if i > 0:
                    link[0] = _opaque_zero([parts[0][0:8, r0 - LANE:r0]])
                for j in range(1, nsub):
                    q = linked(q_all[h, _h(r0 + LANE * j, tq - LANE * j), :])
                    parts.append(_dot_nt(_bf(q), k_s[r0 + LANE * j:r0 + LANE * (j + 1), :]))
                set_link(parts[2], cfg["link_part"], parts[0])
                return parts

            def softmax(i, parts):
                pb = p_s.at[i % 2]
                chain = _opaque_zero([b[b.shape[0] - 8:, b.shape[1] - LANE:] for b in parts])
                ls = []
                for a in range(nsub):
                    blocks = [parts[j][LANE * (a - j):LANE * (a - j + 1), :] for j in range(a + 1)]
                    last = blocks[-1]
                    w = last.shape[1]
                    dg = jnp.where(tri, last[:, w - LANE:], NEG)
                    blocks[-1] = dg if w == LANE else _lanecat([last[:, :w - LANE], dg])
                    sa = _lanecat(blocks)
                    if cfg["dbg"] & 4:
                        ls.append(jnp.ones((LANE, 1), F32))
                        p = _pin(sa, link[0], 0, 0 if a == 0 else sa.shape[1] - LANE)
                        pb[LANE * a:LANE * (a + 1), 0:sa.shape[1]] = p.astype(BF16)
                        continue
                    mb = jnp.broadcast_to(jnp.max(sa, axis=1, keepdims=True), (LANE, LANE))
                    nt = sa.shape[1] // LANE
                    ptiles, psums = [], []
                    for g in range(0, LANE, 8):
                        mg = _pin(mb[g:g + 8, :], chain)
                        pg = [jnp.exp2(sa[g:g + 8, t * LANE:(t + 1) * LANE] - mg) for t in range(nt)]
                        ps = functools.reduce(jnp.add, pg)
                        chain = _opaque_zero([ps])
                        psums.append(ps)
                        ptiles.append(_lanecat(pg))
                    ls.append(jnp.sum(_rowcat(psums), axis=1, keepdims=True))
                    p = _pin(_rowcat(ptiles), link[0], 0, 0 if a == 0 else sa.shape[1] - LANE)
                    pb[LANE * a:LANE * (a + 1), 0:sa.shape[1]] = p.astype(BF16)
                return ls

            def pv(i, ls):
                r0 = i * tq
                pb = p_s.at[i % 2]
                ctx = [_dot(pb[:, 0:r0 + LANE], v_s[0:r0 + LANE, :])]
                for j in range(1, nsub):
                    ctx.append(_dot(pb[LANE * j:, r0 + LANE * j:r0 + LANE * (j + 1)],
                                    v_s[r0 + LANE * j:r0 + LANE * (j + 1), :]))
                set_link(ctx[2], cfg["link_part"])
                cs = []
                for a in range(nsub):
                    sl = lambda j: slice(LANE * (a - j), LANE * (a - j + 1))
                    r = pl.reciprocal(ls[a], approx=True)
                    r = r * (2.0 - ls[a] * r)
                    cs.append(functools.reduce(jnp.add, [ctx[j][sl(j)] for j in range(a + 1)]) * r)
                return _rowcat(cs).astype(BF16)

            def oproj(i, ctx):
                for u in range(tq // D):
                    res = _dot_nt(_bf(linked(wo_v[h])), ctx[u * D:(u + 1) * D, :])
                    set_link(res)
                    rb_t[i * (tq // D) + u] += res

            a_state = {}

            def a_hook(tag):
                if with_a and tag == cfg["a_fwd_at"]:
                    a_state["kv"], xs, hs = a_fwd()
                    a_state["z"] = a_conv(xs, hs)
                if with_a and tag == cfg["a_inv_at"]:
                    a_inv(a_state["kv"], a_state["z"])

            a_hook(0)
            proj(k_s, 0, 0, tq)
            a_hook(1)
            parts = qk(0)
            ctx_prev = None
            for i in range(nq):
                r0 = i * tq
                a_hook(10 * (i + 1))
                if ctx_prev is not None:
                    oproj(i - 1, ctx_prev)
                a_hook(10 * (i + 1) + 1)
                if i + 1 < nq:
                    proj(k_s, 0, r0 + tq, tq)
                a_hook(10 * (i + 1) + 2)
                proj(v_s, 1, r0, tq)
                a_hook(10 * (i + 1) + 3)
                ls = softmax(i, parts)
                ctx_prev = pv(i, ls)
                a_hook(10 * (i + 1) + 4)
                if i + 1 < nq:
                    parts = qk(i + 1, a_out() if i + 1 == cfg["ao_at"] else None)
            oproj(nq - 1, ctx_prev)
            return carry

        with jax.named_scope("loop_a"):
            lax.fori_loop(cfg["h0"], H, head_step, 0)
        with jax.named_scope("tail"):
            for i in range(NOUT):
                c0 = (i * D) % (S // 2)
                full = _rowcat([ra_t[i * D // (S // 2), AT * LANE:, c0:c0 + D], rb_t[i]])
                out_v[i * D:(i + 1) * D, :] = full.T.astype(BF16)
                out_copy(i).start()
            for i in range(NOUT + AT):
                out_copy(i).wait()

    scratch = [
        pltpu.VMEM((4, M // 2, S), U32),
        pltpu.VMEM((KS, M), BF16),
        pltpu.VMEM((M,), BF16),
        pltpu.VMEM((KS + 1, M, LANE), F32),
        pltpu.VMEM((LANE // 2, 2 * LANE), U32),
        pltpu.VMEM((M // 2, S), U32),
        pltpu.VMEM((S // 2, MP), U32),
        pltpu.VMEM((S // 2, C), U32),
        pltpu.VMEM((KT, 4 * TP * 8, LANE), U32),
        pltpu.VMEM((H // 2, MP // 2, 2 * D), U32),
        pltpu.VMEM((H // 2, x_cols, 2 * D), F32),
        pltpu.VMEM((WS, 8 * WP * 8, LANE), U32),
        pltpu.VMEM((H, C // 2, 2 * D), U32),
        pltpu.VMEM((H, M // 2, D), U32),
        pltpu.VMEM((H, S // 2, D), U32),
        pltpu.VMEM((S, D), BF16),
        pltpu.VMEM((S, D), BF16),
        pltpu.VMEM((2, tq, S), BF16),
        pltpu.VMEM((2, M, S // 2), F32),
        pltpu.VMEM((S // D, M, D), F32),
        pltpu.VMEM((AT, S, LANE), BF16),
        pltpu.VMEM((S, 2 * M - AT * LANE), BF16),
        pltpu.SemaphoreType.DMA((XC,)),
        pltpu.SemaphoreType.DMA((KT,)),
        pltpu.SemaphoreType.DMA((WS,)),
        pltpu.SemaphoreType.DMA((QIT,)),
        pltpu.SemaphoreType.DMA((2,)),
        pltpu.SemaphoreType.DMA((3,)),
        pltpu.SemaphoreType.DMA((S // D + AT,)),
    ]
    return kernel, scratch


_DEFAULT = dict(tq=512, a_fwd_at=13, a_inv_at=44, a_gate=1, a_chains=1, a_width=4, ao_at=1, ao_row=128, dbg=0, q_pf=-1, wq_first=1,
                link_back=176, pace_row=32, pace_step=24, link_part=32, use_a=1, h0=0)


def _build(**kw):
    cfg = dict(_DEFAULT)
    cfg.update(kw)
    kernel, scratch = _make_kernel(cfg)

    def run(A_q, A_k, A_v, A_shift_k, A_ssm_k, A_ssm_D, B_x, B_c_kv, B_w_q, B_w_uk,
            B_w_uv, B_w_o):
        tr = lambda a: jnp.swapaxes(a, 1, 2).reshape(M, S)
        args = (
            tr(A_q), tr(A_k), tr(A_v), A_shift_k.T, A_ssm_k, A_ssm_D, tr(B_x),
            B_c_kv.reshape(S, C),
            B_w_q.reshape(M // 2, 2 * H, D), B_w_uk.reshape(C // 2, 2 * H, D),
            B_w_uv.reshape(C // 2, 2 * H, D),
            jnp.swapaxes(B_w_o, 1, 2),
        )
        out = pl.pallas_call(
            kernel,
            in_specs=[pl.BlockSpec(memory_space=pl.ANY)] * len(args),
            out_specs=pl.BlockSpec(memory_space=pl.ANY),
            out_shape=jax.ShapeDtypeStruct((S, 2 * M), BF16),
            scratch_shapes=scratch,
            compiler_params=pltpu.CompilerParams(
                vmem_limit_bytes=120 * 1024 * 1024,
                disable_bounds_checks=True),
        )(*args)
        return out.reshape(1, S, 2 * M)

    return run


_run = _build()


@jax.jit
def pallas_concat_heads__ssm_conv_h3__compressed_kv_cla__prompt_kernel(
    A_q: jax.Array,
    A_k: jax.Array,
    A_v: jax.Array,
    A_shift_k: jax.Array,
    A_ssm_k: jax.Array,
    A_ssm_D: jax.Array,
    B_x: jax.Array,
    B_c_kv: jax.Array,
    B_w_q: jax.Array,
    B_w_uk: jax.Array,
    B_w_uv: jax.Array,
    B_w_o: jax.Array,
):
    return _run(A_q, A_k, A_v, A_shift_k, A_ssm_k, A_ssm_D, B_x, B_c_kv, B_w_q,
                B_w_uk, B_w_uv, B_w_o)
```

```python
import functools

import jax
import jax.numpy as jnp
from jax import lax
import jax.experimental.pallas as pl
import jax.experimental.pallas.tpu as pltpu

F32 = jnp.float32
BF16 = jnp.bfloat16
U32 = jnp.uint32

S = 2048
M = 448
MP = 512
C = 1024
H = 16
D = 256
KS = 4
LANE = 128
NB = S // LANE
AR = 32
A_STEPS = M // AR
LOG2E = 1.4426950408889634
NEG = -1e30

NT = (((1,), (1,)), ((), ()))


def _dot(a, b):
    return jnp.dot(a, b, preferred_element_type=F32)


def _dot_nt(a, b):
    return lax.dot_general(a, b, NT, preferred_element_type=F32)


def _bf(x):
    return pltpu.bitcast(x, BF16)


def _u32(x):
    return pltpu.bitcast(x, U32)


def _h(r0, n):
    return pl.ds(r0 // 2, n // 2)


def _repack(ev, od):
    lo = (ev & jnp.uint32(0xFFFF)) | (od << 16)
    hi = (ev >> 16) | (od & jnp.uint32(0xFFFF0000))
    return lo, hi


def _opaque_zero(vals):
    acc = None
    for v in vals:
        b = v if v.dtype == U32 else pltpu.bitcast(v, U32)
        for r in range(0, b.shape[0], 8):
            for c in range(0, b.shape[1], LANE):
                t = b[r:r + 8, c:c + LANE]
                acc = t if acc is None else acc | t
    return jnp.minimum((acc >> 1).astype(jnp.int32), 0)


def _pin(x, zero, r=0, c=0):
    t = pltpu.bitcast(pltpu.bitcast(x[r:r + 8, c:c + LANE], jnp.int32) + zero, x.dtype)
    row = ([x[r:r + 8, :c]] if c > 0 else []) + [t] + (
        [x[r:r + 8, c + LANE:]] if c + LANE < x.shape[1] else [])
    row = jnp.concatenate(row, axis=1) if len(row) > 1 else row[0]
    col = ([x[:r, :]] if r > 0 else []) + [row] + ([x[r + 8:, :]] if r + 8 < x.shape[0] else [])
    return jnp.concatenate(col, axis=0) if len(col) > 1 else col[0]


def _rowcat(xs):
    return jnp.concatenate(xs, axis=0) if len(xs) > 1 else xs[0]


def _lanecat(xs):
    return jnp.concatenate(xs, axis=1) if len(xs) > 1 else xs[0]


def _make_kernel(cfg):
    tq = cfg["tq"]
    nq = S // tq
    nsub = tq // LANE
    KT = MP // LANE
    TP = LANE // 2
    XC = 4
    x_cols = S // XC
    WP = 64
    WS = 3
    QIT = 8
    AT = 3

    def kernel(aq_hbm, ak_hbm, av_hbm, sh_hbm, ssm_hbm, dd_hbm, x_hbm, c_hbm,
               wq_hbm, wk_hbm, wv_hbm, wo_hbm,
               out_hbm,
               a_v, sh_v, dd_v, par_v, f_v,
               xt_v, x_v, c_v, wqs_v, wq_v, qacc, ws_v, wkv_v, wo_v,
               q_all, k_s, v_s, p_s, ra_t, rb_t, oa_v, out_v,
               sem_x, sem_wq, sem_w, sem_c, sem_s, sem_a, sem_out):
        x32, c32, wq32, wk32, wv32, wo32 = (
            r.bitcast(U32) for r in (x_hbm, c_hbm, wq_hbm, wk_hbm, wv_hbm, wo_hbm))
        a32 = [r.bitcast(U32) for r in (ak_hbm, av_hbm, ssm_hbm, aq_hbm)]

        def x_copy(i):
            cs = pl.ds(i * x_cols, x_cols)
            return pltpu.make_async_copy(x32.at[:, cs], xt_v.at[:, cs], sem_x.at[i])

        def wq_copies(kt):
            dst = wqs_v.reshape(4 * KT, TP, 8, LANE)
            rs = pl.ds(min(kt * TP, M // 2 - TP), TP)
            return [pltpu.make_async_copy(
                wq32.at[rs, pl.ds(8 * (k // 2), 8), pl.ds((k % 2) * LANE, LANE)],
                dst.at[4 * kt + k], sem_wq.at[kt]) for k in range(4)]

        def wq_wait(kt):
            pltpu.make_async_copy(wqs_v.at[kt], wqs_v.at[kt], sem_wq.at[kt]).wait()

        def w_rows(chunk):
            r0 = chunk * WP
            return pl.ds(r0 if isinstance(r0, int) else pl.multiple_of(r0, WP), WP)

        def w_copies(chunk, slot):
            dst = ws_v.reshape(8 * WS, WP, 8, LANE)
            rs = w_rows(chunk)
            out = []
            for which, src in enumerate((wk32, wv32)):
                for par in range(2):
                    for half in range(2):
                        k = 8 * slot + 4 * which + 2 * par + half
                        out.append(pltpu.make_async_copy(
                            src.at[rs, pl.ds(8 * par, 8), pl.ds(half * LANE, LANE)],
                            dst.at[k], sem_w.at[slot]))
            return out

        def w_wait(slot):
            pltpu.make_async_copy(ws_v.at[slot], ws_v.at[slot], sem_w.at[slot]).wait()

        def c_copy(it):
            n = S // 2 // QIT
            rs = pl.ds(pl.multiple_of(it * n, n), n)
            return pltpu.make_async_copy(c32.at[rs], c_v.at[rs], sem_c.at[it])

        wo_copy = pltpu.make_async_copy(wo32, wo_v, sem_a.at[0])
        a_parts = [pl.ds(0, AR // 2), pl.ds(AR // 2, M // 2 - AR // 2)]

        def a_start(part):
            rs = a_parts[part]
            for k in range(4):
                pltpu.make_async_copy(a32[k].at[rs], a_v.at[k, rs], sem_a.at[1 + part]).start()

        def a_wait(part):
            view = a_v.at[:, a_parts[part]]
            pltpu.make_async_copy(view, view, sem_a.at[1 + part]).wait()

        small = [pltpu.make_async_copy(sh_hbm, sh_v, sem_s.at[0]),
                 pltpu.make_async_copy(dd_hbm, dd_v, sem_s.at[1])]

        link = [None]

        pace = [None]

        def set_link(res, row=None, pacer=None):
            if row is None:
                row = res.shape[0] - cfg["link_back"]
            link[0] = _opaque_zero([res[row:row + 8, res.shape[1] - LANE:]])
            pace[0] = res if pacer is None else pacer

        def linked(x):
            return x if link[0] is None else _pin(x, link[0])

        def paced(w):
            res = pace[0]
            if res is None or link[0] is None or not cfg["pace_step"]:
                return w
            rows = []
            zs = [_opaque_zero([res[r:r + 8, res.shape[1] - LANE:]])
                  for r in range(cfg["pace_row"], cfg["pace_row"] + 8 * cfg["pace_step"],
                                 cfg["pace_step"])]
            for r in range(0, w.shape[0], 8):
                z = zs[7 - (r // 8) % 8]
                t = pltpu.bitcast(w[r:r + 8, :], jnp.int32)
                rows.append(pltpu.bitcast(t + _lanecat([z] * (w.shape[1] // LANE)), U32))
            return _rowcat(rows)

        with jax.named_scope("first_starts"):
            for cp in small:
                cp.start()
        x_copy(0).start()
        for kt in range(cfg["wq_first"]):
            for cp in wq_copies(kt):
                cp.start()

        bi = lax.broadcasted_iota(jnp.int32, (LANE, LANE), 0)
        mi = lax.broadcasted_iota(jnp.int32, (LANE, LANE), 1)
        ph = ((4 * mi + 1) * bi) & 511
        ang = ph.astype(F32) * (2.0 * 3.141592653589793 / 512.0)
        f_v[:, 0:LANE] = _u32(jnp.cos(ang).astype(BF16))
        f_v[:, LANE:] = _u32((-jnp.sin(ang)).astype(BF16))

        rb_t[...] = jnp.zeros((S // D, M, D), F32)
        ra_t[:, 0:LANE, :] = jnp.zeros((2, LANE, S // 2), F32)

        for kt in range(cfg["wq_first"], KT):
            for cp in wq_copies(kt):
                cp.start()
        with jax.named_scope("small_wait"):
            for cp in small:
                cp.wait()
        sh = sh_v[...].astype(F32)
        for j in range(KS):
            par_v[j] = jnp.broadcast_to(sh[j:j + 1, :], (LANE, M)).T
        dd = dd_v[...].astype(F32).reshape(1, M)
        par_v[KS] = jnp.broadcast_to(dd, (LANE, M)).T

        def x_transpose(i):
            xt = xt_v[:, pl.ds(i * x_cols, x_cols)]
            nfull = (KT - 1) * TP
            xt = _rowcat([xt[:nfull], jnp.zeros((MP // 2 - M // 2, x_cols), U32), xt[nfull:]])
            x_v[_h(i * x_cols, x_cols), :] = _u32(_bf(xt).astype(F32).T.astype(BF16))

        def q_early(kt, first, last):
            r0 = kt * TP
            rows = pl.ds(r0 if isinstance(r0, int) else pl.multiple_of(r0, TP), TP)
            c0 = kt * LANE
            cols = pl.ds(c0 if isinstance(c0, int) else pl.multiple_of(c0, LANE), LANE)
            link[0] = None
            for j in range(H // 2):
                ws = []
                for half in range(2):
                    ev, od = (
                        wqs_v[kt, pl.ds((2 * par + half) * TP * 8 + j, TP, stride=8), :]
                        for par in range(2))
                    ws.append(_repack(ev, od))
                w = _lanecat([ws[0][0], ws[1][0], ws[0][1], ws[1][1]])
                wq_v[j, rows, :] = w
                d = _dot(_bf(linked(x_v[_h(0, x_cols), cols])), _bf(w))
                set_link(d)
                if not first:
                    d = d + qacc[j]
                if last:
                    d = (d * (D ** -0.5 * LOG2E)).astype(BF16)
                    for t in range(2):
                        q_all[2 * j + t, _h(0, x_cols), :] = _u32(d[:, t * D:(t + 1) * D])
                else:
                    qacc[j] = d

        with jax.named_scope("x_wait"):
            x_copy(0).wait()
        x_transpose(0)
        with jax.named_scope("wq_wait"):
            wq_wait(0)
        q_early(0, True, False)
        for i in range(1, XC):
            x_copy(i).start()

        def early_body(kt, carry):
            with jax.named_scope("wq_wait"):
                wq_wait(kt)
            q_early(kt, False, False)
            for cp in w_copies(kt - 1, kt - 1):
                cp.start()
            return carry

        lax.fori_loop(1, KT - 1, early_body, 0)
        with jax.named_scope("wq_wait"):
            wq_wait(KT - 1)
            for i in range(1, XC):
                x_copy(i).wait()
        q_early(KT - 1, False, True)
        for i in range(1, XC):
            x_transpose(i)

        def unpack(chunk, slot, which, half, j):
            ev, od = (
                ws_v[slot, pl.ds((4 * which + 2 * par + half) * WP * 8 + j, WP, stride=8), :]
                for par in range(2))
            lo, hi = _repack(ev, od)
            rows = w_rows(chunk)
            cols = pl.ds(which * D + half * LANE, LANE)
            wkv_v[2 * j, rows, cols] = lo
            wkv_v[2 * j + 1, rows, cols] = hi
            return [lo, hi]

        units = [(w_, h_, j_) for w_ in range(2) for h_ in range(2) for j_ in range(H // 2)]

        def qproj(it, r0, n, t, zeros=(None, None)):
            outs = []
            for u in range(2):
                lhs = _bf(linked(x_v[_h(r0, n), :]))
                d = _dot(lhs, _bf(wq_v[it, :, pl.ds(t * D + u * LANE, LANE)]))
                set_link(d)
                if zeros[u] is not None:
                    for k, z in enumerate(zeros[u]):
                        d = _pin(d, z, 8 * ((k * (n // 8)) // len(zeros[u])))
                outs.append(d)
            q2 = _lanecat(outs)
            q_all[2 * it + t, _h(r0, n), :] = _u32((q2 * (D ** -0.5 * LOG2E)).astype(BF16))

        def q_body(it, carry):
            slot = it % WS

            def q_prefetch():
                c_copy(it).start()

                @pl.when(it + 2 < QIT)
                def _():
                    for cp in w_copies(it + 2, (it + 2) % WS):
                        cp.start()

                @pl.when(it == QIT - 2)
                def _():
                    wo_copy.start()
                    a_start(0)

            if cfg["q_pf"] == -2:
                q_prefetch()
            with jax.named_scope("w_wait"):
                w_wait(slot)
            if cfg["q_pf"] == -1:
                q_prefetch()
            link[0] = None
            pieces = [(pc, t) for pc in range(1, XC) for t in range(2)]
            nd = 2 * len(pieces)
            for k, (pc, t) in enumerate(pieces):
                zeros = []
                for u in range(2):
                    d = 2 * k + u
                    mine = units[d * len(units) // nd:(d + 1) * len(units) // nd]
                    zeros.append([_opaque_zero(unpack(it, slot, *u_)) for u_ in mine])
                qproj(it, pc * x_cols, x_cols, t, zeros)
                if k == cfg["q_pf"]:
                    q_prefetch()
            return carry

        with jax.named_scope("q_loop"):
            lax.fori_loop(0, QIT, q_body, 0)
        a_start(1)
        for it in range(QIT):
            c_copy(it).wait()
        a_wait(0)
        wo_copy.wait()

        tri = (lax.broadcasted_iota(jnp.int32, (LANE, LANE), 1)
               <= lax.broadcasted_iota(jnp.int32, (LANE, LANE), 0))

        NOUT = S // D

        def out_copy(i):
            if i >= NOUT:
                t = i - NOUT
                return pltpu.make_async_copy(
                    oa_v.at[t], out_hbm.at[:, pl.ds(t * LANE, LANE)], sem_out.at[i])
            rs = pl.ds(i * D, D)
            return pltpu.make_async_copy(
                out_v.at[rs], out_hbm.at[rs, pl.ds(AT * LANE, 2 * M - AT * LANE)], sem_out.at[i])

        def b_out(k, tot):
            c0 = (k * D) % (S // 2)
            full = _rowcat([ra_t[k * D // (S // 2), AT * LANE:, c0:c0 + D], tot]).T
            out_v[k * D:(k + 1) * D, :] = full.astype(BF16)
            return full

        def head_step(h, carry):
            with jax.named_scope("step"):
                return head_step_(h, carry)

        def head_step_(h, carry):
            with_a = cfg["use_a"]

            @pl.when(h == H - 1)
            def _():
                for t in range(AT):
                    out_copy(NOUT + t).start()

            @pl.when(h == cfg["h0"] + 1)
            def _():
                a_wait(1)

            link[0] = None
            n2 = AR // 2
            a_rows2 = pl.ds(pl.multiple_of(jnp.minimum(h, A_STEPS - 1) * n2, n2), n2)
            a_rows = pl.ds(pl.multiple_of(jnp.minimum(h, A_STEPS - 1) * AR, AR), AR)

            def a_fwd():
                kk = _bf(a_v[0, a_rows2, :]).astype(F32)
                lane = lax.broadcasted_iota(jnp.int32, (AR, LANE), 1)
                coef = [par_v[j, a_rows, :] for j in range(KS)]
                rolled = [kk] + [pltpu.roll(kk, j, 1) for j in range(1, KS)]
                vv = _bf(a_v[1, a_rows2, :]).astype(F32)
                kv_blocks = []
                for a in range(NB):
                    cs = slice(a * LANE, (a + 1) * LANE)
                    acc = rolled[0][:, cs] * coef[0]
                    for j in range(1, KS):
                        t = rolled[j][:, cs]
                        if a == 0:
                            t = jnp.where(lane >= j, t, 0.0)
                        acc = acc + t * coef[j]
                    kv_blocks.append(acc * vv[:, cs])
                hk = a_v[2, a_rows2, :]
                hk = _rowcat([hk[:, a * LANE:(a + 1) * LANE] for a in range(NB)])
                fm = _bf(f_v[...])
                hs = _dot(_bf(linked(hk)), fm)
                kv = linked(_rowcat(kv_blocks)).astype(BF16)
                xs = _dot(kv, fm)
                set_link(xs)
                return kv, xs, hs

            def a_conv(xs, hs):
                def tile(v, a, g, part):
                    r = a * AR + 8 * g
                    return v[r:r + 8, part * LANE:(part + 1) * LANE]

                z = {}
                nch = cfg["a_chains"]
                gates = [None] * nch
                width = cfg["a_width"]
                k = 0
                for g in range(AR // 8):
                    hr = [tile(hs, 0, g, 0)] + [
                        tile(hs, j, g, 0) - tile(hs, j - 1, g, 1) for j in range(1, NB)]
                    hi = [tile(hs, 0, g, 1)] + [
                        tile(hs, j, g, 1) + tile(hs, j - 1, g, 0) for j in range(1, NB)]
                    for c0 in range(0, NB, width):
                        ch = k % nch
                        k += 1
                        for a in range(c0 + width):
                            xr, xi = tile(xs, a, g, 0), tile(xs, a, g, 1)
                            if gates[ch] is not None and cfg["a_gate"]:
                                xr, xi = _pin(xr, gates[ch]), _pin(xi, gates[ch])
                            for c in range(max(c0, a), c0 + width):
                                j = c - a
                                tr = xr * hr[j] - xi * hi[j]
                                ti = xr * hi[j] + xi * hr[j]
                                z[c, g] = (tr, ti) if a == 0 else (z[c, g][0] + tr, z[c, g][1] + ti)
                            gates[ch] = _opaque_zero(list(z[c0 + width - 1, g]))
                return z

            def a_inv(kv, z):
                fm = _bf(f_v[...])
                ng = AR // 8
                ys = []
                for u in range(2):
                    rows = [_lanecat(z[c, g]) for g in range(u * ng // 2, (u + 1) * ng // 2)
                            for c in range(NB)]
                    ys.append(_dot_nt(linked(_rowcat(rows)).astype(BF16), fm))
                y = _rowcat(ys)
                dd = par_v[KS, a_rows, :]
                for c in range(NB):
                    cs = slice(c * LANE, (c + 1) * LANE)
                    yc = _rowcat([y[(g * NB + c) * 8:(g * NB + c + 1) * 8, :] for g in range(ng)])
                    qq = _bf(a_v[3, a_rows2, cs]).astype(F32)
                    kvf = kv[c * AR:(c + 1) * AR, :].astype(F32)
                    c2 = (c % (NB // 2)) * LANE
                    ra_t[c // (NB // 2), a_rows, c2:c2 + LANE] = qq * (yc * (1.0 / LANE) + kvf * dd)

            def a_out():
                slab = jnp.clip(h // 4 - 1, 0, AT - 1)
                half = h % 2
                x = ra_t[half, pl.ds(pl.multiple_of(slab * LANE, LANE), LANE), :]
                xt = x.T
                oa_v[slab, pl.ds(pl.multiple_of(half * (S // 2), S // 2), S // 2), :] = xt.astype(BF16)
                return xt

            kw = C // 2
            pending = []

            def flush_pending(x, row):
                done = list(pending)
                del pending[:]
                if not done:
                    return x
                x = _pin(x, _opaque_zero([f for _, f in done]), row)

                @pl.when(h == H - 1)
                def _():
                    for k, _f in done:
                        out_copy(k).start()
                return x

            def proj_w(which, k):
                return wkv_v[h, _h((k % 2) * kw, kw), pl.ds(which * D + (k // 2) * LANE, LANE)]

            def proj(dst, which, r0, n):
                ds = []
                for k in range(4):
                    lhs = linked(c_v[_h(r0, n), pl.ds((k % 2) * kw, kw)])
                    if which == 1 and k == cfg["bo_pass"]:
                        lhs = flush_pending(lhs, cfg["ao_row"])
                    ds.append(_dot(_bf(lhs), _bf(paced(proj_w(which, k)))))
                    set_link(ds[-1])
                dst[r0:r0 + n, :] = _lanecat([ds[0] + ds[1], ds[2] + ds[3]]).astype(BF16)

            def qk(i, dep=None):
                r0 = i * tq
                q = linked(q_all[h, _h(r0, tq), :])
                if dep is not None:
                    q = _pin(q, _opaque_zero([dep]), cfg["ao_row"])
                parts = [_dot_nt(_bf(q), k_s[0:r0 + LANE, :])]
                if i > 0:
                    link[0] = _opaque_zero([parts[0][0:8, r0 - LANE:r0]])
                for j in range(1, nsub):
                    q = linked(q_all[h, _h(r0 + LANE * j, tq - LANE * j), :])
                    parts.append(_dot_nt(_bf(q), k_s[r0 + LANE * j:r0 + LANE * (j + 1), :]))
                set_link(parts[2], cfg["link_part"], parts[0])
                return parts

            def softmax(i, parts):
                pb = p_s.at[i % 2]
                chain = _opaque_zero([b[b.shape[0] - 8:, b.shape[1] - LANE:] for b in parts])
                ls = []
                for a in range(nsub):
                    blocks = [parts[j][LANE * (a - j):LANE * (a - j + 1), :] for j in range(a + 1)]
                    last = blocks[-1]
                    w = last.shape[1]
                    dg = jnp.where(tri, last[:, w - LANE:], NEG)
                    blocks[-1] = dg if w == LANE else _lanecat([last[:, :w - LANE], dg])
                    sa = _lanecat(blocks)
                    if cfg["dbg"] & 4:
                        ls.append(jnp.ones((LANE, 1), F32))
                        p = _pin(sa, link[0], 0, 0 if a == 0 else sa.shape[1] - LANE)
                        pb[LANE * a:LANE * (a + 1), 0:sa.shape[1]] = p.astype(BF16)
                        continue
                    mb = jnp.broadcast_to(jnp.max(sa, axis=1, keepdims=True), (LANE, LANE))
                    nt = sa.shape[1] // LANE
                    ptiles, psums = [], []
                    for g in range(0, LANE, 8):
                        mg = _pin(mb[g:g + 8, :], chain)
                        pg = [jnp.exp2(sa[g:g + 8, t * LANE:(t + 1) * LANE] - mg) for t in range(nt)]
                        ps = functools.reduce(jnp.add, pg)
                        chain = _opaque_zero([ps])
                        psums.append(ps)
                        ptiles.append(_lanecat(pg))
                    ls.append(jnp.sum(_rowcat(psums), axis=1, keepdims=True))
                    p = _pin(_rowcat(ptiles), link[0], 0, 0 if a == 0 else sa.shape[1] - LANE)
                    pb[LANE * a:LANE * (a + 1), 0:sa.shape[1]] = p.astype(BF16)
                return ls

            def pv(i, ls):
                r0 = i * tq
                pb = p_s.at[i % 2]
                ctx = [_dot(pb[:, 0:r0 + LANE], v_s[0:r0 + LANE, :])]
                for j in range(1, nsub):
                    ctx.append(_dot(pb[LANE * j:, r0 + LANE * j:r0 + LANE * (j + 1)],
                                    v_s[r0 + LANE * j:r0 + LANE * (j + 1), :]))
                set_link(ctx[2], cfg["link_part"])
                cs = []
                for a in range(nsub):
                    sl = lambda j: slice(LANE * (a - j), LANE * (a - j + 1))
                    r = pl.reciprocal(ls[a], approx=True)
                    r = r * (2.0 - ls[a] * r)
                    cs.append(functools.reduce(jnp.add, [ctx[j][sl(j)] for j in range(a + 1)]) * r)
                return _rowcat(cs).astype(BF16)

            def oproj(i, ctx):
                for u in range(tq // D):
                    res = _dot_nt(_bf(linked(wo_v[h])), ctx[u * D:(u + 1) * D, :])
                    set_link(res)
                    k = i * (tq // D) + u
                    tot = rb_t[k] + res
                    rb_t[k] = tot
                    if cfg["b_out"] and i < nq - 1:
                        pending.append((k, b_out(k, tot)))

            a_state = {}

            def a_hook(tag):
                if with_a and tag == cfg["a_fwd_at"]:
                    a_state["kv"], xs, hs = a_fwd()
                    a_state["z"] = a_conv(xs, hs)
                if with_a and tag == cfg["a_inv_at"]:
                    a_inv(a_state["kv"], a_state["z"])

            a_hook(0)
            proj(k_s, 0, 0, tq)
            a_hook(1)
            parts = qk(0)
            ctx_prev = None
            for i in range(nq):
                r0 = i * tq
                a_hook(10 * (i + 1))
                if ctx_prev is not None:
                    oproj(i - 1, ctx_prev)
                a_hook(10 * (i + 1) + 1)
                if i + 1 < nq:
                    proj(k_s, 0, r0 + tq, tq)
                a_hook(10 * (i + 1) + 2)
                proj(v_s, 1, r0, tq)
                a_hook(10 * (i + 1) + 3)
                ls = softmax(i, parts)
                ctx_prev = pv(i, ls)
                a_hook(10 * (i + 1) + 4)
                if i + 1 < nq:
                    parts = qk(i + 1, a_out() if i + 1 == cfg["ao_at"] else None)
            oproj(nq - 1, ctx_prev)
            return carry

        with jax.named_scope("loop_a"):
            lax.fori_loop(cfg["h0"], H, head_step, 0)
        with jax.named_scope("tail"):
            for i in range((nq - 1) * (tq // D) if cfg["b_out"] else 0, NOUT):
                b_out(i, rb_t[i])
                out_copy(i).start()
            for i in range(NOUT + AT):
                out_copy(i).wait()

    scratch = [
        pltpu.VMEM((4, M // 2, S), U32),
        pltpu.VMEM((KS, M), BF16),
        pltpu.VMEM((M,), BF16),
        pltpu.VMEM((KS + 1, M, LANE), F32),
        pltpu.VMEM((LANE // 2, 2 * LANE), U32),
        pltpu.VMEM((M // 2, S), U32),
        pltpu.VMEM((S // 2, MP), U32),
        pltpu.VMEM((S // 2, C), U32),
        pltpu.VMEM((KT, 4 * TP * 8, LANE), U32),
        pltpu.VMEM((H // 2, MP // 2, 2 * D), U32),
        pltpu.VMEM((H // 2, x_cols, 2 * D), F32),
        pltpu.VMEM((WS, 8 * WP * 8, LANE), U32),
        pltpu.VMEM((H, C // 2, 2 * D), U32),
        pltpu.VMEM((H, M // 2, D), U32),
        pltpu.VMEM((H, S // 2, D), U32),
        pltpu.VMEM((S, D), BF16),
        pltpu.VMEM((S, D), BF16),
        pltpu.VMEM((2, tq, S), BF16),
        pltpu.VMEM((2, M, S // 2), F32),
        pltpu.VMEM((S // D, M, D), F32),
        pltpu.VMEM((AT, S, LANE), BF16),
        pltpu.VMEM((S, 2 * M - AT * LANE), BF16),
        pltpu.SemaphoreType.DMA((XC,)),
        pltpu.SemaphoreType.DMA((KT,)),
        pltpu.SemaphoreType.DMA((WS,)),
        pltpu.SemaphoreType.DMA((QIT,)),
        pltpu.SemaphoreType.DMA((2,)),
        pltpu.SemaphoreType.DMA((3,)),
        pltpu.SemaphoreType.DMA((S // D + AT,)),
    ]
    return kernel, scratch


_DEFAULT = dict(tq=512, a_fwd_at=13, a_inv_at=44, a_gate=1, a_chains=1, a_width=4, ao_at=1, ao_row=240, b_out=1, bo_pass=3, dbg=0, q_pf=-1, wq_first=1,
                link_back=176, pace_row=32, pace_step=24, link_part=32, use_a=1, h0=0)


def _build(**kw):
    cfg = dict(_DEFAULT)
    cfg.update(kw)
    kernel, scratch = _make_kernel(cfg)

    def run(A_q, A_k, A_v, A_shift_k, A_ssm_k, A_ssm_D, B_x, B_c_kv, B_w_q, B_w_uk,
            B_w_uv, B_w_o):
        tr = lambda a: jnp.swapaxes(a, 1, 2).reshape(M, S)
        args = (
            tr(A_q), tr(A_k), tr(A_v), A_shift_k.T, A_ssm_k, A_ssm_D, tr(B_x),
            B_c_kv.reshape(S, C),
            B_w_q.reshape(M // 2, 2 * H, D), B_w_uk.reshape(C // 2, 2 * H, D),
            B_w_uv.reshape(C // 2, 2 * H, D),
            jnp.swapaxes(B_w_o, 1, 2),
        )
        out = pl.pallas_call(
            kernel,
            in_specs=[pl.BlockSpec(memory_space=pl.ANY)] * len(args),
            out_specs=pl.BlockSpec(memory_space=pl.ANY),
            out_shape=jax.ShapeDtypeStruct((S, 2 * M), BF16),
            scratch_shapes=scratch,
            compiler_params=pltpu.CompilerParams(
                vmem_limit_bytes=120 * 1024 * 1024,
                disable_bounds_checks=True),
        )(*args)
        return out.reshape(1, S, 2 * M)

    return run


_run = _build()


@jax.jit
def pallas_concat_heads__ssm_conv_h3__compressed_kv_cla__prompt_kernel(
    A_q: jax.Array,
    A_k: jax.Array,
    A_v: jax.Array,
    A_shift_k: jax.Array,
    A_ssm_k: jax.Array,
    A_ssm_D: jax.Array,
    B_x: jax.Array,
    B_c_kv: jax.Array,
    B_w_q: jax.Array,
    B_w_uk: jax.Array,
    B_w_uv: jax.Array,
    B_w_o: jax.Array,
):
    return _run(A_q, A_k, A_v, A_shift_k, A_ssm_k, A_ssm_D, B_x, B_c_kv, B_w_q,
                B_w_uk, B_w_uv, B_w_o)
```

```python
import functools

import jax
import jax.numpy as jnp
from jax import lax
import jax.experimental.pallas as pl
import jax.experimental.pallas.tpu as pltpu

F32 = jnp.float32
BF16 = jnp.bfloat16
U32 = jnp.uint32

S = 2048
M = 448
MP = 512
C = 1024
H = 16
D = 256
KS = 4
LANE = 128
NB = S // LANE
AR = 32
A_STEPS = M // AR
LOG2E = 1.4426950408889634
NEG = -1e30

NT = (((1,), (1,)), ((), ()))


def _dot(a, b):
    return jnp.dot(a, b, preferred_element_type=F32)


def _dot_nt(a, b):
    return lax.dot_general(a, b, NT, preferred_element_type=F32)


def _bf(x):
    return pltpu.bitcast(x, BF16)


def _u32(x):
    return pltpu.bitcast(x, U32)


def _h(r0, n):
    return pl.ds(r0 // 2, n // 2)


def _repack(ev, od):
    lo = (ev & jnp.uint32(0xFFFF)) | (od << 16)
    hi = (ev >> 16) | (od & jnp.uint32(0xFFFF0000))
    return lo, hi


def _opaque_zero(vals):
    acc = None
    for v in vals:
        b = v if v.dtype == U32 else pltpu.bitcast(v, U32)
        for r in range(0, b.shape[0], 8):
            for c in range(0, b.shape[1], LANE):
                t = b[r:r + 8, c:c + LANE]
                acc = t if acc is None else acc | t
    return jnp.minimum((acc >> 1).astype(jnp.int32), 0)


def _pin(x, zero, r=0, c=0):
    t = pltpu.bitcast(pltpu.bitcast(x[r:r + 8, c:c + LANE], jnp.int32) + zero, x.dtype)
    row = ([x[r:r + 8, :c]] if c > 0 else []) + [t] + (
        [x[r:r + 8, c + LANE:]] if c + LANE < x.shape[1] else [])
    row = jnp.concatenate(row, axis=1) if len(row) > 1 else row[0]
    col = ([x[:r, :]] if r > 0 else []) + [row] + ([x[r + 8:, :]] if r + 8 < x.shape[0] else [])
    return jnp.concatenate(col, axis=0) if len(col) > 1 else col[0]


def _rowcat(xs):
    return jnp.concatenate(xs, axis=0) if len(xs) > 1 else xs[0]


def _lanecat(xs):
    return jnp.concatenate(xs, axis=1) if len(xs) > 1 else xs[0]


def _make_kernel(cfg):
    tq = cfg["tq"]
    nq = S // tq
    nsub = tq // LANE
    KT = MP // LANE
    TP = LANE // 2
    XC = 4
    x_cols = S // XC
    WP = 64
    WS = 3
    QIT = 8
    AT = 3

    def kernel(aq_hbm, ak_hbm, av_hbm, sh_hbm, ssm_hbm, dd_hbm, x_hbm, c_hbm,
               wq_hbm, wk_hbm, wv_hbm, wo_hbm,
               out_hbm,
               a_v, sh_v, dd_v, par_v, f_v,
               xt_v, x_v, c_v, wqs_v, wq_v, qacc, ws_v, wkv_v, wo_v,
               q_all, k_s, v_s, p_s, ra_t, rb_t, oa_v, out_v,
               sem_x, sem_wq, sem_w, sem_c, sem_s, sem_a, sem_out):
        x32, c32, wq32, wk32, wv32, wo32 = (
            r.bitcast(U32) for r in (x_hbm, c_hbm, wq_hbm, wk_hbm, wv_hbm, wo_hbm))
        a32 = [r.bitcast(U32) for r in (ak_hbm, av_hbm, ssm_hbm, aq_hbm)]

        def x_copy(i):
            cs = pl.ds(i * x_cols, x_cols)
            return pltpu.make_async_copy(x32.at[:, cs], xt_v.at[:, cs], sem_x.at[i])

        def wq_copies(kt):
            dst = wqs_v.reshape(4 * KT, TP, 8, LANE)
            rs = pl.ds(min(kt * TP, M // 2 - TP), TP)
            return [pltpu.make_async_copy(
                wq32.at[rs, pl.ds(8 * (k // 2), 8), pl.ds((k % 2) * LANE, LANE)],
                dst.at[4 * kt + k], sem_wq.at[kt]) for k in range(4)]

        def wq_wait(kt):
            pltpu.make_async_copy(wqs_v.at[kt], wqs_v.at[kt], sem_wq.at[kt]).wait()

        def w_rows(chunk):
            r0 = chunk * WP
            return pl.ds(r0 if isinstance(r0, int) else pl.multiple_of(r0, WP), WP)

        def w_copies(chunk, slot):
            dst = ws_v.reshape(8 * WS, WP, 8, LANE)
            rs = w_rows(chunk)
            out = []
            for which, src in enumerate((wk32, wv32)):
                for par in range(2):
                    for half in range(2):
                        k = 8 * slot + 4 * which + 2 * par + half
                        out.append(pltpu.make_async_copy(
                            src.at[rs, pl.ds(8 * par, 8), pl.ds(half * LANE, LANE)],
                            dst.at[k], sem_w.at[slot]))
            return out

        def w_wait(slot):
            pltpu.make_async_copy(ws_v.at[slot], ws_v.at[slot], sem_w.at[slot]).wait()

        def piece_start(it):
            n = S // 2 // QIT
            rs = pl.ds(pl.multiple_of(it * n, n), n)
            pltpu.make_async_copy(c32.at[rs], c_v.at[rs], sem_c.at[0]).start()
            hs = pl.ds(it * (H // QIT), H // QIT)
            pltpu.make_async_copy(wo32.at[hs], wo_v.at[hs], sem_a.at[0]).start()

        a_parts = [pl.ds(0, AR // 2), pl.ds(AR // 2, M // 2 - AR // 2)]

        def a_start(part):
            rs = a_parts[part]
            for k in range(4):
                pltpu.make_async_copy(
                    a32[k].at[rs], a_v.at[k, rs], sem_a.at[1 + part]).start()

        def a_wait(part):
            view = a_v.at[:, a_parts[part]]
            pltpu.make_async_copy(view, view, sem_a.at[1 + part]).wait()

        small = [pltpu.make_async_copy(sh_hbm, sh_v, sem_s.at[0]),
                 pltpu.make_async_copy(dd_hbm, dd_v, sem_s.at[1])]

        link = [None]

        pace = [None]

        def set_link(res, row=None, pacer=None):
            if row is None:
                row = res.shape[0] - cfg["link_back"]
            link[0] = _opaque_zero([res[row:row + 8, res.shape[1] - LANE:]])
            pace[0] = res if pacer is None else pacer

        def linked(x):
            return x if link[0] is None else _pin(x, link[0])

        def paced(w):
            res = pace[0]
            if res is None or link[0] is None or not cfg["pace_step"]:
                return w
            rows = []
            zs = [_opaque_zero([res[r:r + 8, res.shape[1] - LANE:]])
                  for r in range(cfg["pace_row"], cfg["pace_row"] + 8 * cfg["pace_step"],
                                 cfg["pace_step"])]
            for r in range(0, w.shape[0], 8):
                z = zs[7 - (r // 8) % 8]
                t = pltpu.bitcast(w[r:r + 8, :], jnp.int32)
                rows.append(pltpu.bitcast(t + _lanecat([z] * (w.shape[1] // LANE)), U32))
            return _rowcat(rows)

        with jax.named_scope("first_starts"):
            for cp in small:
                cp.start()
        x_copy(0).start()
        for kt in range(cfg["wq_first"]):
            for cp in wq_copies(kt):
                cp.start()

        bi = lax.broadcasted_iota(jnp.int32, (LANE, LANE), 0)
        mi = lax.broadcasted_iota(jnp.int32, (LANE, LANE), 1)
        ph = ((4 * mi + 1) * bi) & 511
        ang = ph.astype(F32) * (2.0 * 3.141592653589793 / 512.0)
        f_v[:, 0:LANE] = _u32(jnp.cos(ang).astype(BF16))
        f_v[:, LANE:] = _u32((-jnp.sin(ang)).astype(BF16))

        rb_t[...] = jnp.zeros((S // D, M, D), F32)
        ra_t[:, 0:LANE, :] = jnp.zeros((2, LANE, S // 2), F32)

        for kt in range(cfg["wq_first"], KT):
            for cp in wq_copies(kt):
                cp.start()
        with jax.named_scope("small_wait"):
            for cp in small:
                cp.wait()
        sh = sh_v[...].astype(F32)
        for j in range(KS):
            par_v[j] = jnp.broadcast_to(sh[j:j + 1, :], (LANE, M)).T
        dd = dd_v[...].astype(F32).reshape(1, M)
        par_v[KS] = jnp.broadcast_to(dd, (LANE, M)).T

        def x_transpose(i):
            xt = xt_v[:, pl.ds(i * x_cols, x_cols)]
            nfull = (KT - 1) * TP
            xt = _rowcat([xt[:nfull], jnp.zeros((MP // 2 - M // 2, x_cols), U32), xt[nfull:]])
            x_v[_h(i * x_cols, x_cols), :] = _u32(_bf(xt).astype(F32).T.astype(BF16))

        def q_early(kt, first, last):
            r0 = kt * TP
            rows = pl.ds(r0 if isinstance(r0, int) else pl.multiple_of(r0, TP), TP)
            c0 = kt * LANE
            cols = pl.ds(c0 if isinstance(c0, int) else pl.multiple_of(c0, LANE), LANE)
            link[0] = None
            for j in range(H // 2):
                ws = []
                for half in range(2):
                    ev, od = (
                        wqs_v[kt, pl.ds((2 * par + half) * TP * 8 + j, TP, stride=8), :]
                        for par in range(2))
                    ws.append(_repack(ev, od))
                w = _lanecat([ws[0][0], ws[1][0], ws[0][1], ws[1][1]])
                wq_v[j, rows, :] = w
                d = _dot(_bf(linked(x_v[_h(0, x_cols), cols])), _bf(w))
                set_link(d)
                if not first:
                    d = d + qacc[j]
                if last:
                    d = (d * (D ** -0.5 * LOG2E)).astype(BF16)
                    for t in range(2):
                        q_all[2 * j + t, _h(0, x_cols), :] = _u32(d[:, t * D:(t + 1) * D])
                else:
                    qacc[j] = d

        with jax.named_scope("x_wait"):
            x_copy(0).wait()
        x_transpose(0)
        with jax.named_scope("wq_wait"):
            wq_wait(0)
        q_early(0, True, False)
        for i in range(1, XC):
            x_copy(i).start()

        def early_body(kt, carry):
            with jax.named_scope("wq_wait"):
                wq_wait(kt)
            q_early(kt, False, False)
            for cp in w_copies(kt - 1, kt - 1):
                cp.start()
            return carry

        lax.fori_loop(1, KT - 1, early_body, 0)
        with jax.named_scope("wq_wait"):
            wq_wait(KT - 1)
            for i in range(1, XC):
                x_copy(i).wait()
        q_early(KT - 1, False, True)
        for i in range(1, XC):
            x_transpose(i)

        def unpack(chunk, slot, which, half, j):
            ev, od = (
                ws_v[slot, pl.ds((4 * which + 2 * par + half) * WP * 8 + j, WP, stride=8), :]
                for par in range(2))
            lo, hi = _repack(ev, od)
            rows = w_rows(chunk)
            cols = pl.ds(which * D + half * LANE, LANE)
            wkv_v[2 * j, rows, cols] = lo
            wkv_v[2 * j + 1, rows, cols] = hi
            return [lo, hi]

        units = [(w_, h_, j_) for w_ in range(2) for h_ in range(2) for j_ in range(H // 2)]

        def qproj(it, r0, n, t, zeros=(None, None)):
            outs = []
            for u in range(2):
                lhs = _bf(linked(x_v[_h(r0, n), :]))
                d = _dot(lhs, _bf(wq_v[it, :, pl.ds(t * D + u * LANE, LANE)]))
                set_link(d)
                if zeros[u] is not None:
                    for k, z in enumerate(zeros[u]):
                        d = _pin(d, z, 8 * ((k * (n // 8)) // len(zeros[u])))
                outs.append(d)
            q2 = _lanecat(outs)
            q_all[2 * it + t, _h(r0, n), :] = _u32((q2 * (D ** -0.5 * LOG2E)).astype(BF16))

        def q_body(it, carry):
            slot = it % WS

            def q_prefetch():
                @pl.when(it + 2 < QIT)
                def _():
                    for cp in w_copies(it + 2, (it + 2) % WS):
                        cp.start()

                piece_start(it)

            if cfg["q_pf"] == -2:
                q_prefetch()
            with jax.named_scope("w_wait"):
                w_wait(slot)
            if cfg["q_pf"] == -1:
                q_prefetch()
            link[0] = None
            pieces = [(pc, t) for pc in range(1, XC) for t in range(2)]
            nd = 2 * len(pieces)
            for k, (pc, t) in enumerate(pieces):
                zeros = []
                for u in range(2):
                    d = 2 * k + u
                    mine = units[d * len(units) // nd:(d + 1) * len(units) // nd]
                    zeros.append([_opaque_zero(unpack(it, slot, *u_)) for u_ in mine])
                qproj(it, pc * x_cols, x_cols, t, zeros)
                if k == cfg["q_pf"]:
                    q_prefetch()
            return carry

        a_start(0)
        with jax.named_scope("q_loop"):
            lax.fori_loop(0, QIT, q_body, 0)
        a_start(1)
        pltpu.make_async_copy(c_v, c_v, sem_c.at[0]).wait()
        a_wait(0)
        pltpu.make_async_copy(wo_v, wo_v, sem_a.at[0]).wait()

        tri = (lax.broadcasted_iota(jnp.int32, (LANE, LANE), 1)
               <= lax.broadcasted_iota(jnp.int32, (LANE, LANE), 0))

        NOUT = S // D

        def out_copy(i):
            if i >= NOUT:
                t = i - NOUT
                return pltpu.make_async_copy(
                    oa_v.at[t], out_hbm.at[:, pl.ds(t * LANE, LANE)], sem_out.at[i])
            rs = pl.ds(i * D, D)
            return pltpu.make_async_copy(
                out_v.at[rs], out_hbm.at[rs, pl.ds(AT * LANE, 2 * M - AT * LANE)], sem_out.at[i])

        def b_out(k, tot):
            c0 = (k * D) % (S // 2)
            full = _rowcat([ra_t[k * D // (S // 2), AT * LANE:, c0:c0 + D], tot]).T
            out_v[k * D:(k + 1) * D, :] = full.astype(BF16)
            return full

        def head_step(h, carry):
            with jax.named_scope("step"):
                return head_step_(h, carry)

        def head_step_(h, carry):
            with_a = cfg["use_a"]

            @pl.when(h == H - 1)
            def _():
                for t in range(AT):
                    out_copy(NOUT + t).start()

            @pl.when(h == cfg["h0"] + 1)
            def _():
                a_wait(1)

            link[0] = None
            n2 = AR // 2
            a_rows2 = pl.ds(pl.multiple_of(jnp.minimum(h, A_STEPS - 1) * n2, n2), n2)
            a_rows = pl.ds(pl.multiple_of(jnp.minimum(h, A_STEPS - 1) * AR, AR), AR)

            def a_fwd():
                kk = _bf(a_v[0, a_rows2, :]).astype(F32)
                lane = lax.broadcasted_iota(jnp.int32, (AR, LANE), 1)
                coef = [par_v[j, a_rows, :] for j in range(KS)]
                rolled = [kk] + [pltpu.roll(kk, j, 1) for j in range(1, KS)]
                vv = _bf(a_v[1, a_rows2, :]).astype(F32)
                kv_blocks = []
                for a in range(NB):
                    cs = slice(a * LANE, (a + 1) * LANE)
                    acc = rolled[0][:, cs] * coef[0]
                    for j in range(1, KS):
                        t = rolled[j][:, cs]
                        if a == 0:
                            t = jnp.where(lane >= j, t, 0.0)
                        acc = acc + t * coef[j]
                    kv_blocks.append(acc * vv[:, cs])
                hk = a_v[2, a_rows2, :]
                hk = _rowcat([hk[:, a * LANE:(a + 1) * LANE] for a in range(NB)])
                fm = _bf(f_v[...])
                hs = _dot(_bf(linked(hk)), fm)
                kv = linked(_rowcat(kv_blocks)).astype(BF16)
                xs = _dot(kv, fm)
                set_link(xs)
                return kv, xs, hs

            def a_conv(xs, hs):
                def tile(v, a, g, part):
                    r = a * AR + 8 * g
                    return v[r:r + 8, part * LANE:(part + 1) * LANE]

                z = {}
                nch = cfg["a_chains"]
                gates = [None] * nch
                width = cfg["a_width"]
                k = 0
                for g in range(AR // 8):
                    hr = [tile(hs, 0, g, 0)] + [
                        tile(hs, j, g, 0) - tile(hs, j - 1, g, 1) for j in range(1, NB)]
                    hi = [tile(hs, 0, g, 1)] + [
                        tile(hs, j, g, 1) + tile(hs, j - 1, g, 0) for j in range(1, NB)]
                    for c0 in range(0, NB, width):
                        ch = k % nch
                        k += 1
                        for a in range(c0 + width):
                            xr, xi = tile(xs, a, g, 0), tile(xs, a, g, 1)
                            if gates[ch] is not None and cfg["a_gate"]:
                                xr, xi = _pin(xr, gates[ch]), _pin(xi, gates[ch])
                            for c in range(max(c0, a), c0 + width):
                                j = c - a
                                tr = xr * hr[j] - xi * hi[j]
                                ti = xr * hi[j] + xi * hr[j]
                                z[c, g] = (tr, ti) if a == 0 else (z[c, g][0] + tr, z[c, g][1] + ti)
                            gates[ch] = _opaque_zero(list(z[c0 + width - 1, g]))
                return z

            def a_inv(kv, z):
                fm = _bf(f_v[...])
                ng = AR // 8
                ys = []
                for u in range(2):
                    rows = [_lanecat(z[c, g]) for g in range(u * ng // 2, (u + 1) * ng // 2)
                            for c in range(NB)]
                    ys.append(_dot_nt(linked(_rowcat(rows)).astype(BF16), fm))
                y = _rowcat(ys)
                dd = par_v[KS, a_rows, :]
                for c in range(NB):
                    cs = slice(c * LANE, (c + 1) * LANE)
                    yc = _rowcat([y[(g * NB + c) * 8:(g * NB + c + 1) * 8, :] for g in range(ng)])
                    qq = _bf(a_v[3, a_rows2, cs]).astype(F32)
                    kvf = kv[c * AR:(c + 1) * AR, :].astype(F32)
                    c2 = (c % (NB // 2)) * LANE
                    ra_t[c // (NB // 2), a_rows, c2:c2 + LANE] = qq * (yc * (1.0 / LANE) + kvf * dd)

            def a_out():
                slab = jnp.clip(h // 4 - 1, 0, AT - 1)
                half = h % 2
                x = ra_t[half, pl.ds(pl.multiple_of(slab * LANE, LANE), LANE), :]
                xt = x.T
                oa_v[slab, pl.ds(pl.multiple_of(half * (S // 2), S // 2), S // 2), :] = xt.astype(BF16)
                return xt

            kw = C // 2
            pending = []

            def flush_pending(x, row):
                done = list(pending)
                del pending[:]
                if not done:
                    return x
                x = _pin(x, _opaque_zero([f for _, f in done]), row)

                @pl.when(h == H - 1)
                def _():
                    for k, _f in done:
                        out_copy(k).start()
                return x

            def proj_w(which, k):
                return wkv_v[h, _h((k % 2) * kw, kw), pl.ds(which * D + (k // 2) * LANE, LANE)]

            def proj(dst, which, r0, n):
                ds = []
                for k in range(4):
                    lhs = linked(c_v[_h(r0, n), pl.ds((k % 2) * kw, kw)])
                    if which == 1 and k == cfg["bo_pass"]:
                        lhs = flush_pending(lhs, cfg["ao_row"])
                    ds.append(_dot(_bf(lhs), _bf(paced(proj_w(which, k)))))
                    set_link(ds[-1])
                dst[r0:r0 + n, :] = _lanecat([ds[0] + ds[1], ds[2] + ds[3]]).astype(BF16)

            def qk(i, dep=None):
                r0 = i * tq
                q = linked(q_all[h, _h(r0, tq), :])
                if dep is not None:
                    q = _pin(q, _opaque_zero([dep]), cfg["ao_row"])
                parts = [_dot_nt(_bf(q), k_s[0:r0 + LANE, :])]
                if i > 0:
                    link[0] = _opaque_zero([parts[0][0:8, r0 - LANE:r0]])
                for j in range(1, nsub):
                    q = linked(q_all[h, _h(r0 + LANE * j, tq - LANE * j), :])
                    parts.append(_dot_nt(_bf(q), k_s[r0 + LANE * j:r0 + LANE * (j + 1), :]))
                set_link(parts[2], cfg["link_part"], parts[0])
                return parts

            def softmax(i, parts):
                pb = p_s.at[i % 2]
                chain = _opaque_zero([b[b.shape[0] - 8:, b.shape[1] - LANE:] for b in parts])
                ls = []
                for a in range(nsub):
                    blocks = [parts[j][LANE * (a - j):LANE * (a - j + 1), :] for j in range(a + 1)]
                    last = blocks[-1]
                    w = last.shape[1]
                    dg = jnp.where(tri, last[:, w - LANE:], NEG)
                    blocks[-1] = dg if w == LANE else _lanecat([last[:, :w - LANE], dg])
                    sa = _lanecat(blocks)
                    if cfg["dbg"] & 4:
                        ls.append(jnp.ones((LANE, 1), F32))
                        p = _pin(sa, link[0], 0, 0 if a == 0 else sa.shape[1] - LANE)
                        pb[LANE * a:LANE * (a + 1), 0:sa.shape[1]] = p.astype(BF16)
                        continue
                    mb = jnp.broadcast_to(jnp.max(sa, axis=1, keepdims=True), (LANE, LANE))
                    nt = sa.shape[1] // LANE
                    ptiles, psums = [], []
                    for g in range(0, LANE, 8):
                        mg = _pin(mb[g:g + 8, :], chain)
                        pg = [jnp.exp2(sa[g:g + 8, t * LANE:(t + 1) * LANE] - mg) for t in range(nt)]
                        ps = functools.reduce(jnp.add, pg)
                        chain = _opaque_zero([ps])
                        psums.append(ps)
                        ptiles.append(_lanecat(pg))
                    ls.append(jnp.sum(_rowcat(psums), axis=1, keepdims=True))
                    p = _pin(_rowcat(ptiles), link[0], 0, 0 if a == 0 else sa.shape[1] - LANE)
                    pb[LANE * a:LANE * (a + 1), 0:sa.shape[1]] = p.astype(BF16)
                return ls

            def pv(i, ls):
                r0 = i * tq
                pb = p_s.at[i % 2]
                ctx = [_dot(pb[:, 0:r0 + LANE], v_s[0:r0 + LANE, :])]
                for j in range(1, nsub):
                    ctx.append(_dot(pb[LANE * j:, r0 + LANE * j:r0 + LANE * (j + 1)],
                                    v_s[r0 + LANE * j:r0 + LANE * (j + 1), :]))
                set_link(ctx[2], cfg["link_part"])
                cs = []
                for a in range(nsub):
                    sl = lambda j: slice(LANE * (a - j), LANE * (a - j + 1))
                    r = pl.reciprocal(ls[a], approx=True)
                    r = r * (2.0 - ls[a] * r)
                    cs.append(functools.reduce(jnp.add, [ctx[j][sl(j)] for j in range(a + 1)]) * r)
                return _rowcat(cs).astype(BF16)

            def oproj(i, ctx):
                for u in range(tq // D):
                    res = _dot_nt(_bf(linked(wo_v[h])), ctx[u * D:(u + 1) * D, :])
                    set_link(res)
                    k = i * (tq // D) + u
                    tot = rb_t[k] + res
                    rb_t[k] = tot
                    if cfg["b_out"] and i < nq - 1:
                        pending.append((k, b_out(k, tot)))

            a_state = {}

            def a_hook(tag):
                if with_a and tag == cfg["a_fwd_at"]:
                    a_state["kv"], xs, hs = a_fwd()
                    a_state["z"] = a_conv(xs, hs)
                if with_a and tag == cfg["a_inv_at"]:
                    a_inv(a_state["kv"], a_state["z"])

            a_hook(0)
            proj(k_s, 0, 0, tq)
            a_hook(1)
            parts = qk(0)
            ctx_prev = None
            for i in range(nq):
                r0 = i * tq
                a_hook(10 * (i + 1))
                if ctx_prev is not None:
                    oproj(i - 1, ctx_prev)
                a_hook(10 * (i + 1) + 1)
                if i + 1 < nq:
                    proj(k_s, 0, r0 + tq, tq)
                a_hook(10 * (i + 1) + 2)
                proj(v_s, 1, r0, tq)
                a_hook(10 * (i + 1) + 3)
                ls = softmax(i, parts)
                ctx_prev = pv(i, ls)
                a_hook(10 * (i + 1) + 4)
                if i + 1 < nq:
                    parts = qk(i + 1, a_out() if i + 1 == cfg["ao_at"] else None)
            oproj(nq - 1, ctx_prev)
            return carry

        with jax.named_scope("loop_a"):
            lax.fori_loop(cfg["h0"], H, head_step, 0)
        with jax.named_scope("tail"):
            for i in range((nq - 1) * (tq // D) if cfg["b_out"] else 0, NOUT):
                b_out(i, rb_t[i])
                out_copy(i).start()
            for i in range(NOUT + AT):
                out_copy(i).wait()

    scratch = [
        pltpu.VMEM((4, M // 2, S), U32),
        pltpu.VMEM((KS, M), BF16),
        pltpu.VMEM((M,), BF16),
        pltpu.VMEM((KS + 1, M, LANE), F32),
        pltpu.VMEM((LANE // 2, 2 * LANE), U32),
        pltpu.VMEM((M // 2, S), U32),
        pltpu.VMEM((S // 2, MP), U32),
        pltpu.VMEM((S // 2, C), U32),
        pltpu.VMEM((KT, 4 * TP * 8, LANE), U32),
        pltpu.VMEM((H // 2, MP // 2, 2 * D), U32),
        pltpu.VMEM((H // 2, x_cols, 2 * D), F32),
        pltpu.VMEM((WS, 8 * WP * 8, LANE), U32),
        pltpu.VMEM((H, C // 2, 2 * D), U32),
        pltpu.VMEM((H, M // 2, D), U32),
        pltpu.VMEM((H, S // 2, D), U32),
        pltpu.VMEM((S, D), BF16),
        pltpu.VMEM((S, D), BF16),
        pltpu.VMEM((2, tq, S), BF16),
        pltpu.VMEM((2, M, S // 2), F32),
        pltpu.VMEM((S // D, M, D), F32),
        pltpu.VMEM((AT, S, LANE), BF16),
        pltpu.VMEM((S, 2 * M - AT * LANE), BF16),
        pltpu.SemaphoreType.DMA((XC,)),
        pltpu.SemaphoreType.DMA((KT,)),
        pltpu.SemaphoreType.DMA((WS,)),
        pltpu.SemaphoreType.DMA((1,)),
        pltpu.SemaphoreType.DMA((2,)),
        pltpu.SemaphoreType.DMA((3,)),
        pltpu.SemaphoreType.DMA((S // D + AT,)),
    ]
    return kernel, scratch


_DEFAULT = dict(tq=512, a_fwd_at=13, a_inv_at=44, a_gate=1, a_chains=1, a_width=4, ao_at=1, ao_row=240, b_out=1, bo_pass=3, dbg=0, q_pf=-1, wq_first=1,
                link_back=176, pace_row=32, pace_step=24, link_part=32, use_a=1, h0=0)


def _build(**kw):
    cfg = dict(_DEFAULT)
    cfg.update(kw)
    kernel, scratch = _make_kernel(cfg)

    def run(A_q, A_k, A_v, A_shift_k, A_ssm_k, A_ssm_D, B_x, B_c_kv, B_w_q, B_w_uk,
            B_w_uv, B_w_o):
        tr = lambda a: jnp.swapaxes(a, 1, 2).reshape(M, S)
        args = (
            tr(A_q), tr(A_k), tr(A_v), A_shift_k.T, A_ssm_k, A_ssm_D, tr(B_x),
            B_c_kv.reshape(S, C),
            B_w_q.reshape(M // 2, 2 * H, D), B_w_uk.reshape(C // 2, 2 * H, D),
            B_w_uv.reshape(C // 2, 2 * H, D),
            jnp.swapaxes(B_w_o, 1, 2),
        )
        out = pl.pallas_call(
            kernel,
            in_specs=[pl.BlockSpec(memory_space=pl.ANY)] * len(args),
            out_specs=pl.BlockSpec(memory_space=pl.ANY),
            out_shape=jax.ShapeDtypeStruct((S, 2 * M), BF16),
            scratch_shapes=scratch,
            compiler_params=pltpu.CompilerParams(
                vmem_limit_bytes=120 * 1024 * 1024,
                disable_bounds_checks=True),
        )(*args)
        return out.reshape(1, S, 2 * M)

    return run


_run = _build()


@jax.jit
def pallas_concat_heads__ssm_conv_h3__compressed_kv_cla__prompt_kernel(
    A_q: jax.Array,
    A_k: jax.Array,
    A_v: jax.Array,
    A_shift_k: jax.Array,
    A_ssm_k: jax.Array,
    A_ssm_D: jax.Array,
    B_x: jax.Array,
    B_c_kv: jax.Array,
    B_w_q: jax.Array,
    B_w_uk: jax.Array,
    B_w_uv: jax.Array,
    B_w_o: jax.Array,
):
    return _run(A_q, A_k, A_v, A_shift_k, A_ssm_k, A_ssm_D, B_x, B_c_kv, B_w_q,
                B_w_uk, B_w_uv, B_w_o)
```

```python
import functools

import jax
import jax.numpy as jnp
from jax import lax
import jax.experimental.pallas as pl
import jax.experimental.pallas.tpu as pltpu

F32 = jnp.float32
BF16 = jnp.bfloat16
U32 = jnp.uint32

S = 2048
M = 448
MP = 512
C = 1024
H = 16
D = 256
KS = 4
LANE = 128
NB = S // LANE
AR = 32
A_STEPS = M // AR
LOG2E = 1.4426950408889634
NEG = -1e30

NT = (((1,), (1,)), ((), ()))


def _dot(a, b):
    return jnp.dot(a, b, preferred_element_type=F32)


def _dot_nt(a, b):
    return lax.dot_general(a, b, NT, preferred_element_type=F32)


def _bf(x):
    return pltpu.bitcast(x, BF16)


def _u32(x):
    return pltpu.bitcast(x, U32)


def _h(r0, n):
    return pl.ds(r0 // 2, n // 2)


def _repack(ev, od):
    lo = (ev & jnp.uint32(0xFFFF)) | (od << 16)
    hi = (ev >> 16) | (od & jnp.uint32(0xFFFF0000))
    return lo, hi


def _opaque_zero(vals):
    acc = None
    for v in vals:
        b = v if v.dtype == U32 else pltpu.bitcast(v, U32)
        for r in range(0, b.shape[0], 8):
            for c in range(0, b.shape[1], LANE):
                t = b[r:r + 8, c:c + LANE]
                acc = t if acc is None else acc | t
    return jnp.minimum((acc >> 1).astype(jnp.int32), 0)


def _pin(x, zero, r=0, c=0):
    t = pltpu.bitcast(pltpu.bitcast(x[r:r + 8, c:c + LANE], jnp.int32) + zero, x.dtype)
    row = ([x[r:r + 8, :c]] if c > 0 else []) + [t] + (
        [x[r:r + 8, c + LANE:]] if c + LANE < x.shape[1] else [])
    row = jnp.concatenate(row, axis=1) if len(row) > 1 else row[0]
    col = ([x[:r, :]] if r > 0 else []) + [row] + ([x[r + 8:, :]] if r + 8 < x.shape[0] else [])
    return jnp.concatenate(col, axis=0) if len(col) > 1 else col[0]


def _rowcat(xs):
    return jnp.concatenate(xs, axis=0) if len(xs) > 1 else xs[0]


def _lanecat(xs):
    return jnp.concatenate(xs, axis=1) if len(xs) > 1 else xs[0]


def _make_kernel(cfg):
    tq = cfg["tq"]
    nq = S // tq
    nsub = tq // LANE
    KT = MP // LANE
    TP = LANE // 2
    XC = 4
    x_cols = S // XC
    QP = cfg["q_pairs"]
    WP = 64 * QP
    WS = 2
    QIT = 8 // QP
    AT = 3

    def kernel(aq_hbm, ak_hbm, av_hbm, sh_hbm, ssm_hbm, dd_hbm, x_hbm, c_hbm,
               wq_hbm, wk_hbm, wv_hbm, wo_hbm,
               out_hbm,
               a_v, sh_v, dd_v, par_v, f_v,
               xt_v, x_v, c_v, wqs_v, wq_v, qacc, ws_v, wkv_v, wo_v,
               q_all, k_s, v_s, p_s, ra_t, rb_t, oa_v, out_v,
               sem_x, sem_wq, sem_w, sem_c, sem_s, sem_a, sem_out):
        x32, c32, wq32, wk32, wv32, wo32 = (
            r.bitcast(U32) for r in (x_hbm, c_hbm, wq_hbm, wk_hbm, wv_hbm, wo_hbm))
        a32 = [r.bitcast(U32) for r in (ak_hbm, av_hbm, ssm_hbm, aq_hbm)]

        def x_copy(i):
            cs = pl.ds(i * x_cols, x_cols)
            return pltpu.make_async_copy(x32.at[:, cs], xt_v.at[:, cs], sem_x.at[i])

        def wq_copies(kt):
            dst = wqs_v.reshape(4 * KT, TP, 8, LANE)
            rs = pl.ds(min(kt * TP, M // 2 - TP), TP)
            return [pltpu.make_async_copy(
                wq32.at[rs, pl.ds(8 * (k // 2), 8), pl.ds((k % 2) * LANE, LANE)],
                dst.at[4 * kt + k], sem_wq.at[kt]) for k in range(4)]

        def wq_wait(kt):
            pltpu.make_async_copy(wqs_v.at[kt], wqs_v.at[kt], sem_wq.at[kt]).wait()

        def w_rows(chunk):
            r0 = chunk * WP
            return pl.ds(r0 if isinstance(r0, int) else pl.multiple_of(r0, WP), WP)

        def w_copies(chunk, slot):
            dst = ws_v.reshape(8 * WS, WP, 8, LANE)
            rs = w_rows(chunk)
            out = []
            for which, src in enumerate((wk32, wv32)):
                for par in range(2):
                    for half in range(2):
                        k = 8 * slot + 4 * which + 2 * par + half
                        out.append(pltpu.make_async_copy(
                            src.at[rs, pl.ds(8 * par, 8), pl.ds(half * LANE, LANE)],
                            dst.at[k], sem_w.at[slot]))
            return out

        def w_wait(slot):
            pltpu.make_async_copy(ws_v.at[slot], ws_v.at[slot], sem_w.at[slot]).wait()

        def piece_start(it):
            n = S // 2 // QIT
            rs = pl.ds(pl.multiple_of(it * n, n), n)
            pltpu.make_async_copy(c32.at[rs], c_v.at[rs], sem_c.at[0]).start()
            hs = pl.ds(it * (H // QIT), H // QIT)
            pltpu.make_async_copy(wo32.at[hs], wo_v.at[hs], sem_a.at[0]).start()

        a_parts = [pl.ds(0, AR // 2), pl.ds(AR // 2, M // 2 - AR // 2)]

        def a_start(part):
            rs = a_parts[part]
            for k in range(4):
                pltpu.make_async_copy(
                    a32[k].at[rs], a_v.at[k, rs], sem_a.at[1 + part]).start()

        def a_wait(part):
            view = a_v.at[:, a_parts[part]]
            pltpu.make_async_copy(view, view, sem_a.at[1 + part]).wait()

        small = [pltpu.make_async_copy(sh_hbm, sh_v, sem_s.at[0]),
                 pltpu.make_async_copy(dd_hbm, dd_v, sem_s.at[1])]

        link = [None]

        pace = [None]

        def set_link(res, row=None, pacer=None):
            if row is None:
                row = res.shape[0] - cfg["link_back"]
            link[0] = _opaque_zero([res[row:row + 8, res.shape[1] - LANE:]])
            pace[0] = res if pacer is None else pacer

        def linked(x):
            return x if link[0] is None else _pin(x, link[0])

        def paced(w):
            res = pace[0]
            if res is None or link[0] is None or not cfg["pace_step"]:
                return w
            rows = []
            zs = [_opaque_zero([res[r:r + 8, res.shape[1] - LANE:]])
                  for r in range(cfg["pace_row"], cfg["pace_row"] + 8 * cfg["pace_step"],
                                 cfg["pace_step"])]
            for r in range(0, w.shape[0], 8):
                z = zs[7 - (r // 8) % 8]
                t = pltpu.bitcast(w[r:r + 8, :], jnp.int32)
                rows.append(pltpu.bitcast(t + _lanecat([z] * (w.shape[1] // LANE)), U32))
            return _rowcat(rows)

        with jax.named_scope("first_starts"):
            for cp in small:
                cp.start()
        x_copy(0).start()
        for kt in range(cfg["wq_first"]):
            for cp in wq_copies(kt):
                cp.start()

        bi = lax.broadcasted_iota(jnp.int32, (LANE, LANE), 0)
        mi = lax.broadcasted_iota(jnp.int32, (LANE, LANE), 1)
        ph = ((4 * mi + 1) * bi) & 511
        ang = ph.astype(F32) * (2.0 * 3.141592653589793 / 512.0)
        f_v[:, 0:LANE] = _u32(jnp.cos(ang).astype(BF16))
        f_v[:, LANE:] = _u32((-jnp.sin(ang)).astype(BF16))

        rb_t[...] = jnp.zeros((S // D, M, D), F32)
        ra_t[:, 0:LANE, :] = jnp.zeros((2, LANE, S // 2), F32)

        for kt in range(cfg["wq_first"], KT):
            for cp in wq_copies(kt):
                cp.start()
        with jax.named_scope("small_wait"):
            for cp in small:
                cp.wait()
        sh = sh_v[...].astype(F32)
        for j in range(KS):
            par_v[j] = jnp.broadcast_to(sh[j:j + 1, :], (LANE, M)).T
        dd = dd_v[...].astype(F32).reshape(1, M)
        par_v[KS] = jnp.broadcast_to(dd, (LANE, M)).T

        def x_transpose(i):
            xt = xt_v[:, pl.ds(i * x_cols, x_cols)]
            nfull = (KT - 1) * TP
            xt = _rowcat([xt[:nfull], jnp.zeros((MP // 2 - M // 2, x_cols), U32), xt[nfull:]])
            x_v[_h(i * x_cols, x_cols), :] = _u32(_bf(xt).astype(F32).T.astype(BF16))

        def q_early(kt, first, last):
            r0 = kt * TP
            rows = pl.ds(r0 if isinstance(r0, int) else pl.multiple_of(r0, TP), TP)
            c0 = kt * LANE
            cols = pl.ds(c0 if isinstance(c0, int) else pl.multiple_of(c0, LANE), LANE)
            link[0] = None
            for j in range(H // 2):
                ws = []
                for half in range(2):
                    ev, od = (
                        wqs_v[kt, pl.ds((2 * par + half) * TP * 8 + j, TP, stride=8), :]
                        for par in range(2))
                    ws.append(_repack(ev, od))
                w = _lanecat([ws[0][0], ws[1][0], ws[0][1], ws[1][1]])
                wq_v[j, rows, :] = w
                d = _dot(_bf(linked(x_v[_h(0, x_cols), cols])), _bf(w))
                set_link(d)
                if not first:
                    d = d + qacc[j]
                if last:
                    d = (d * (D ** -0.5 * LOG2E)).astype(BF16)
                    for t in range(2):
                        q_all[2 * j + t, _h(0, x_cols), :] = _u32(d[:, t * D:(t + 1) * D])
                else:
                    qacc[j] = d

        with jax.named_scope("x_wait"):
            x_copy(0).wait()
        x_transpose(0)
        with jax.named_scope("wq_wait"):
            wq_wait(0)
        q_early(0, True, False)
        for i in range(1, XC):
            x_copy(i).start()
        for cp in w_copies(0, 0):
            cp.start()

        def early_body(kt, carry):
            with jax.named_scope("wq_wait"):
                wq_wait(kt)
            q_early(kt, False, False)
            return carry

        lax.fori_loop(1, KT - 1, early_body, 0)
        with jax.named_scope("wq_wait"):
            wq_wait(KT - 1)
            for i in range(1, XC):
                x_copy(i).wait()
        q_early(KT - 1, False, True)
        for i in range(1, XC):
            x_transpose(i)

        def unpack(chunk, slot, sub, which, half, j):
            ev, od = (
                ws_v[slot, pl.ds(((4 * which + 2 * par + half) * WP + sub * TP) * 8 + j, TP,
                                 stride=8), :]
                for par in range(2))
            lo, hi = _repack(ev, od)
            rows = pl.ds(pl.multiple_of(chunk * WP + sub * TP, TP), TP)
            cols = pl.ds(which * D + half * LANE, LANE)
            wkv_v[2 * j, rows, cols] = lo
            wkv_v[2 * j + 1, rows, cols] = hi
            return [lo, hi]

        units = [(s_, w_, h_, j_) for s_ in range(QP) for w_ in range(2) for h_ in range(2)
                 for j_ in range(H // 2)]

        def qproj(it, r0, n, t, zeros=(None, None)):
            outs = []
            for u in range(2):
                lhs = _bf(linked(x_v[_h(r0, n), :]))
                d = _dot(lhs, _bf(wq_v[it, :, pl.ds(t * D + u * LANE, LANE)]))
                set_link(d)
                if zeros[u] is not None:
                    for k, z in enumerate(zeros[u]):
                        d = _pin(d, z, 8 * ((k * (n // 8)) // len(zeros[u])))
                outs.append(d)
            q2 = _lanecat(outs)
            q_all[2 * it + t, _h(r0, n), :] = _u32((q2 * (D ** -0.5 * LOG2E)).astype(BF16))

        def q_body(it, carry):
            slot = it % WS
            with jax.named_scope("w_wait"):
                w_wait(slot)

            @pl.when(it + 1 < QIT)
            def _():
                for cp in w_copies(it + 1, 1 - slot):
                    cp.start()

            piece_start(it)
            link[0] = None
            pieces = [(p, pc, t) for p in range(QP) for pc in range(1, XC) for t in range(2)]
            nd = 2 * len(pieces)
            for k, (p, pc, t) in enumerate(pieces):
                zeros = []
                for u in range(2):
                    d = 2 * k + u
                    mine = units[d * len(units) // nd:(d + 1) * len(units) // nd]
                    zeros.append([_opaque_zero(unpack(it, slot, *u_)) for u_ in mine])
                qproj(QP * it + p, pc * x_cols, x_cols, t, zeros)
            return carry

        a_start(0)
        with jax.named_scope("q_loop"):
            lax.fori_loop(0, QIT, q_body, 0)
        a_start(1)
        pltpu.make_async_copy(c_v, c_v, sem_c.at[0]).wait()
        a_wait(0)
        pltpu.make_async_copy(wo_v, wo_v, sem_a.at[0]).wait()

        tri = (lax.broadcasted_iota(jnp.int32, (LANE, LANE), 1)
               <= lax.broadcasted_iota(jnp.int32, (LANE, LANE), 0))

        NOUT = S // D

        def out_copy(i):
            if i >= NOUT:
                t = i - NOUT
                return pltpu.make_async_copy(
                    oa_v.at[t], out_hbm.at[:, pl.ds(t * LANE, LANE)], sem_out.at[i])
            rs = pl.ds(i * D, D)
            return pltpu.make_async_copy(
                out_v.at[rs], out_hbm.at[rs, pl.ds(AT * LANE, 2 * M - AT * LANE)], sem_out.at[i])

        def b_out(k, tot):
            c0 = (k * D) % (S // 2)
            full = _rowcat([ra_t[k * D // (S // 2), AT * LANE:, c0:c0 + D], tot]).T
            out_v[k * D:(k + 1) * D, :] = full.astype(BF16)
            return full

        def head_step(h, carry):
            with jax.named_scope("step"):
                return head_step_(h, carry)

        def head_step_(h, carry):
            with_a = cfg["use_a"]

            @pl.when(h == H - 1)
            def _():
                for t in range(AT):
                    out_copy(NOUT + t).start()

            @pl.when(h == cfg["h0"] + 1)
            def _():
                a_wait(1)

            link[0] = None
            n2 = AR // 2
            a_rows2 = pl.ds(pl.multiple_of(jnp.minimum(h, A_STEPS - 1) * n2, n2), n2)
            a_rows = pl.ds(pl.multiple_of(jnp.minimum(h, A_STEPS - 1) * AR, AR), AR)

            def a_fwd():
                kk = _bf(a_v[0, a_rows2, :]).astype(F32)
                lane = lax.broadcasted_iota(jnp.int32, (AR, LANE), 1)
                coef = [par_v[j, a_rows, :] for j in range(KS)]
                rolled = [kk] + [pltpu.roll(kk, j, 1) for j in range(1, KS)]
                vv = _bf(a_v[1, a_rows2, :]).astype(F32)
                kv_blocks = []
                for a in range(NB):
                    cs = slice(a * LANE, (a + 1) * LANE)
                    acc = rolled[0][:, cs] * coef[0]
                    for j in range(1, KS):
                        t = rolled[j][:, cs]
                        if a == 0:
                            t = jnp.where(lane >= j, t, 0.0)
                        acc = acc + t * coef[j]
                    kv_blocks.append(acc * vv[:, cs])
                hk = a_v[2, a_rows2, :]
                hk = _rowcat([hk[:, a * LANE:(a + 1) * LANE] for a in range(NB)])
                fm = _bf(f_v[...])
                hs = _dot(_bf(linked(hk)), fm)
                kv = linked(_rowcat(kv_blocks)).astype(BF16)
                xs = _dot(kv, fm)
                set_link(xs)
                return kv, xs, hs

            def a_conv(xs, hs):
                def tile(v, a, g, part):
                    r = a * AR + 8 * g
                    return v[r:r + 8, part * LANE:(part + 1) * LANE]

                z = {}
                nch = cfg["a_chains"]
                gates = [None] * nch
                width = cfg["a_width"]
                k = 0
                for g in range(AR // 8):
                    hr = [tile(hs, 0, g, 0)] + [
                        tile(hs, j, g, 0) - tile(hs, j - 1, g, 1) for j in range(1, NB)]
                    hi = [tile(hs, 0, g, 1)] + [
                        tile(hs, j, g, 1) + tile(hs, j - 1, g, 0) for j in range(1, NB)]
                    for c0 in range(0, NB, width):
                        ch = k % nch
                        k += 1
                        for a in range(c0 + width):
                            xr, xi = tile(xs, a, g, 0), tile(xs, a, g, 1)
                            if gates[ch] is not None and cfg["a_gate"]:
                                xr, xi = _pin(xr, gates[ch]), _pin(xi, gates[ch])
                            for c in range(max(c0, a), c0 + width):
                                j = c - a
                                tr = xr * hr[j] - xi * hi[j]
                                ti = xr * hi[j] + xi * hr[j]
                                z[c, g] = (tr, ti) if a == 0 else (z[c, g][0] + tr, z[c, g][1] + ti)
                            gates[ch] = _opaque_zero(list(z[c0 + width - 1, g]))
                return z

            def a_inv(kv, z):
                fm = _bf(f_v[...])
                ng = AR // 8
                ys = []
                for u in range(2):
                    rows = [_lanecat(z[c, g]) for g in range(u * ng // 2, (u + 1) * ng // 2)
                            for c in range(NB)]
                    ys.append(_dot_nt(linked(_rowcat(rows)).astype(BF16), fm))
                y = _rowcat(ys)
                dd = par_v[KS, a_rows, :]
                for c in range(NB):
                    cs = slice(c * LANE, (c + 1) * LANE)
                    yc = _rowcat([y[(g * NB + c) * 8:(g * NB + c + 1) * 8, :] for g in range(ng)])
                    qq = _bf(a_v[3, a_rows2, cs]).astype(F32)
                    kvf = kv[c * AR:(c + 1) * AR, :].astype(F32)
                    c2 = (c % (NB // 2)) * LANE
                    ra_t[c // (NB // 2), a_rows, c2:c2 + LANE] = qq * (yc * (1.0 / LANE) + kvf * dd)

            def a_out():
                slab = jnp.clip(h // 4 - 1, 0, AT - 1)
                half = h % 2
                x = ra_t[half, pl.ds(pl.multiple_of(slab * LANE, LANE), LANE), :]
                xt = x.T
                oa_v[slab, pl.ds(pl.multiple_of(half * (S // 2), S // 2), S // 2), :] = xt.astype(BF16)
                return xt

            kw = C // 2
            pending = []

            def flush_pending(x, row):
                done = list(pending)
                del pending[:]
                if not done:
                    return x
                x = _pin(x, _opaque_zero([f for _, f in done]), row)

                @pl.when(h == H - 1)
                def _():
                    for k, _f in done:
                        out_copy(k).start()
                return x

            def proj_w(which, k):
                return wkv_v[h, _h((k % 2) * kw, kw), pl.ds(which * D + (k // 2) * LANE, LANE)]

            def proj(dst, which, r0, n):
                ds = []
                for k in range(4):
                    lhs = linked(c_v[_h(r0, n), pl.ds((k % 2) * kw, kw)])
                    if which == 1 and k == cfg["bo_pass"]:
                        lhs = flush_pending(lhs, cfg["ao_row"])
                    ds.append(_dot(_bf(lhs), _bf(paced(proj_w(which, k)))))
                    set_link(ds[-1])
                dst[r0:r0 + n, :] = _lanecat([ds[0] + ds[1], ds[2] + ds[3]]).astype(BF16)

            def qk(i, dep=None):
                r0 = i * tq
                q = linked(q_all[h, _h(r0, tq), :])
                if dep is not None:
                    q = _pin(q, _opaque_zero([dep]), cfg["ao_row"])
                parts = [_dot_nt(_bf(q), k_s[0:r0 + LANE, :])]
                if i > 0:
                    link[0] = _opaque_zero([parts[0][0:8, r0 - LANE:r0]])
                for j in range(1, nsub):
                    q = linked(q_all[h, _h(r0 + LANE * j, tq - LANE * j), :])
                    parts.append(_dot_nt(_bf(q), k_s[r0 + LANE * j:r0 + LANE * (j + 1), :]))
                set_link(parts[2], cfg["link_part"], parts[0])
                return parts

            def softmax(i, parts):
                pb = p_s.at[i % 2]
                chain = _opaque_zero([b[b.shape[0] - 8:, b.shape[1] - LANE:] for b in parts])
                ls = []
                for a in range(nsub):
                    blocks = [parts[j][LANE * (a - j):LANE * (a - j + 1), :] for j in range(a + 1)]
                    last = blocks[-1]
                    w = last.shape[1]
                    dg = jnp.where(tri, last[:, w - LANE:], NEG)
                    blocks[-1] = dg if w == LANE else _lanecat([last[:, :w - LANE], dg])
                    sa = _lanecat(blocks)
                    if cfg["dbg"] & 4:
                        ls.append(jnp.ones((LANE, 1), F32))
                        p = _pin(sa, link[0], 0, 0 if a == 0 else sa.shape[1] - LANE)
                        pb[LANE * a:LANE * (a + 1), 0:sa.shape[1]] = p.astype(BF16)
                        continue
                    mb = jnp.broadcast_to(jnp.max(sa, axis=1, keepdims=True), (LANE, LANE))
                    nt = sa.shape[1] // LANE
                    ptiles, psums = [], []
                    for g in range(0, LANE, 8):
                        mg = _pin(mb[g:g + 8, :], chain)
                        pg = [jnp.exp2(sa[g:g + 8, t * LANE:(t + 1) * LANE] - mg) for t in range(nt)]
                        ps = functools.reduce(jnp.add, pg)
                        chain = _opaque_zero([ps])
                        psums.append(ps)
                        ptiles.append(_lanecat(pg))
                    ls.append(jnp.sum(_rowcat(psums), axis=1, keepdims=True))
                    p = _pin(_rowcat(ptiles), link[0], 0, 0 if a == 0 else sa.shape[1] - LANE)
                    pb[LANE * a:LANE * (a + 1), 0:sa.shape[1]] = p.astype(BF16)
                return ls

            def pv(i, ls):
                r0 = i * tq
                pb = p_s.at[i % 2]
                ctx = [_dot(pb[:, 0:r0 + LANE], v_s[0:r0 + LANE, :])]
                for j in range(1, nsub):
                    ctx.append(_dot(pb[LANE * j:, r0 + LANE * j:r0 + LANE * (j + 1)],
                                    v_s[r0 + LANE * j:r0 + LANE * (j + 1), :]))
                set_link(ctx[2], cfg["link_part"])
                cs = []
                for a in range(nsub):
                    sl = lambda j: slice(LANE * (a - j), LANE * (a - j + 1))
                    r = pl.reciprocal(ls[a], approx=True)
                    r = r * (2.0 - ls[a] * r)
                    cs.append(functools.reduce(jnp.add, [ctx[j][sl(j)] for j in range(a + 1)]) * r)
                return _rowcat(cs).astype(BF16)

            def oproj(i, ctx):
                for u in range(tq // D):
                    res = _dot_nt(_bf(linked(wo_v[h])), ctx[u * D:(u + 1) * D, :])
                    set_link(res)
                    k = i * (tq // D) + u
                    tot = rb_t[k] + res
                    rb_t[k] = tot
                    if cfg["b_out"] and i < nq - 1:
                        pending.append((k, b_out(k, tot)))

            a_state = {}

            def a_hook(tag):
                if with_a and tag == cfg["a_fwd_at"]:
                    a_state["kv"], xs, hs = a_fwd()
                    a_state["z"] = a_conv(xs, hs)
                if with_a and tag == cfg["a_inv_at"]:
                    a_inv(a_state["kv"], a_state["z"])

            a_hook(0)
            proj(k_s, 0, 0, tq)
            a_hook(1)
            parts = qk(0)
            ctx_prev = None
            for i in range(nq):
                r0 = i * tq
                a_hook(10 * (i + 1))
                if ctx_prev is not None:
                    oproj(i - 1, ctx_prev)
                a_hook(10 * (i + 1) + 1)
                if i + 1 < nq:
                    proj(k_s, 0, r0 + tq, tq)
                a_hook(10 * (i + 1) + 2)
                proj(v_s, 1, r0, tq)
                a_hook(10 * (i + 1) + 3)
                ls = softmax(i, parts)
                ctx_prev = pv(i, ls)
                a_hook(10 * (i + 1) + 4)
                if i + 1 < nq:
                    parts = qk(i + 1, a_out() if i + 1 == cfg["ao_at"] else None)
            oproj(nq - 1, ctx_prev)
            return carry

        with jax.named_scope("loop_a"):
            lax.fori_loop(cfg["h0"], H, head_step, 0)
        with jax.named_scope("tail"):
            for i in range((nq - 1) * (tq // D) if cfg["b_out"] else 0, NOUT):
                b_out(i, rb_t[i])
                out_copy(i).start()
            for i in range(NOUT + AT):
                out_copy(i).wait()

    scratch = [
        pltpu.VMEM((4, M // 2, S), U32),
        pltpu.VMEM((KS, M), BF16),
        pltpu.VMEM((M,), BF16),
        pltpu.VMEM((KS + 1, M, LANE), F32),
        pltpu.VMEM((LANE // 2, 2 * LANE), U32),
        pltpu.VMEM((M // 2, S), U32),
        pltpu.VMEM((S // 2, MP), U32),
        pltpu.VMEM((S // 2, C), U32),
        pltpu.VMEM((KT, 4 * TP * 8, LANE), U32),
        pltpu.VMEM((H // 2, MP // 2, 2 * D), U32),
        pltpu.VMEM((H // 2, x_cols, 2 * D), F32),
        pltpu.VMEM((WS, 8 * WP * 8, LANE), U32),
        pltpu.VMEM((H, C // 2, 2 * D), U32),
        pltpu.VMEM((H, M // 2, D), U32),
        pltpu.VMEM((H, S // 2, D), U32),
        pltpu.VMEM((S, D), BF16),
        pltpu.VMEM((S, D), BF16),
        pltpu.VMEM((2, tq, S), BF16),
        pltpu.VMEM((2, M, S // 2), F32),
        pltpu.VMEM((S // D, M, D), F32),
        pltpu.VMEM((AT, S, LANE), BF16),
        pltpu.VMEM((S, 2 * M - AT * LANE), BF16),
        pltpu.SemaphoreType.DMA((XC,)),
        pltpu.SemaphoreType.DMA((KT,)),
        pltpu.SemaphoreType.DMA((WS,)),
        pltpu.SemaphoreType.DMA((1,)),
        pltpu.SemaphoreType.DMA((2,)),
        pltpu.SemaphoreType.DMA((3,)),
        pltpu.SemaphoreType.DMA((S // D + AT,)),
    ]
    return kernel, scratch


_DEFAULT = dict(tq=512, a_fwd_at=13, a_inv_at=44, a_gate=1, a_chains=1, a_width=4, ao_at=1, ao_row=240, b_out=1, bo_pass=3, dbg=0, q_pairs=2, wq_first=1,
                link_back=176, pace_row=32, pace_step=24, link_part=32, use_a=1, h0=0)


def _build(**kw):
    cfg = dict(_DEFAULT)
    cfg.update(kw)
    kernel, scratch = _make_kernel(cfg)

    def run(A_q, A_k, A_v, A_shift_k, A_ssm_k, A_ssm_D, B_x, B_c_kv, B_w_q, B_w_uk,
            B_w_uv, B_w_o):
        tr = lambda a: jnp.swapaxes(a, 1, 2).reshape(M, S)
        args = (
            tr(A_q), tr(A_k), tr(A_v), A_shift_k.T, A_ssm_k, A_ssm_D, tr(B_x),
            B_c_kv.reshape(S, C),
            B_w_q.reshape(M // 2, 2 * H, D), B_w_uk.reshape(C // 2, 2 * H, D),
            B_w_uv.reshape(C // 2, 2 * H, D),
            jnp.swapaxes(B_w_o, 1, 2),
        )
        out = pl.pallas_call(
            kernel,
            in_specs=[pl.BlockSpec(memory_space=pl.ANY)] * len(args),
            out_specs=pl.BlockSpec(memory_space=pl.ANY),
            out_shape=jax.ShapeDtypeStruct((S, 2 * M), BF16),
            scratch_shapes=scratch,
            compiler_params=pltpu.CompilerParams(
                vmem_limit_bytes=120 * 1024 * 1024,
                disable_bounds_checks=True),
        )(*args)
        return out.reshape(1, S, 2 * M)

    return run


_run = _build()


@jax.jit
def pallas_concat_heads__ssm_conv_h3__compressed_kv_cla__prompt_kernel(
    A_q: jax.Array,
    A_k: jax.Array,
    A_v: jax.Array,
    A_shift_k: jax.Array,
    A_ssm_k: jax.Array,
    A_ssm_D: jax.Array,
    B_x: jax.Array,
    B_c_kv: jax.Array,
    B_w_q: jax.Array,
    B_w_uk: jax.Array,
    B_w_uv: jax.Array,
    B_w_o: jax.Array,
):
    return _run(A_q, A_k, A_v, A_shift_k, A_ssm_k, A_ssm_D, B_x, B_c_kv, B_w_q,
                B_w_uk, B_w_uv, B_w_o)
```

```python
import functools

import jax
import jax.numpy as jnp
from jax import lax
import jax.experimental.pallas as pl
import jax.experimental.pallas.tpu as pltpu

F32 = jnp.float32
BF16 = jnp.bfloat16
U32 = jnp.uint32

S = 2048
M = 448
MP = 512
C = 1024
H = 16
D = 256
KS = 4
LANE = 128
NB = S // LANE
AR = 32
A_STEPS = M // AR
LOG2E = 1.4426950408889634
NEG = -1e30

NT = (((1,), (1,)), ((), ()))


def _dot(a, b):
    return jnp.dot(a, b, preferred_element_type=F32)


def _dot_nt(a, b):
    return lax.dot_general(a, b, NT, preferred_element_type=F32)


def _bf(x):
    return pltpu.bitcast(x, BF16)


def _u32(x):
    return pltpu.bitcast(x, U32)


def _h(r0, n):
    return pl.ds(r0 // 2, n // 2)


def _repack(ev, od):
    lo = (ev & jnp.uint32(0xFFFF)) | (od << 16)
    hi = (ev >> 16) | (od & jnp.uint32(0xFFFF0000))
    return lo, hi


def _opaque_zero(vals):
    acc = None
    for v in vals:
        b = v if v.dtype == U32 else pltpu.bitcast(v, U32)
        for r in range(0, b.shape[0], 8):
            for c in range(0, b.shape[1], LANE):
                t = b[r:r + 8, c:c + LANE]
                acc = t if acc is None else acc | t
    return jnp.minimum((acc >> 1).astype(jnp.int32), 0)


def _pin(x, zero, r=0, c=0):
    t = pltpu.bitcast(pltpu.bitcast(x[r:r + 8, c:c + LANE], jnp.int32) + zero, x.dtype)
    row = ([x[r:r + 8, :c]] if c > 0 else []) + [t] + (
        [x[r:r + 8, c + LANE:]] if c + LANE < x.shape[1] else [])
    row = jnp.concatenate(row, axis=1) if len(row) > 1 else row[0]
    col = ([x[:r, :]] if r > 0 else []) + [row] + ([x[r + 8:, :]] if r + 8 < x.shape[0] else [])
    return jnp.concatenate(col, axis=0) if len(col) > 1 else col[0]


def _rowcat(xs):
    return jnp.concatenate(xs, axis=0) if len(xs) > 1 else xs[0]


def _lanecat(xs):
    return jnp.concatenate(xs, axis=1) if len(xs) > 1 else xs[0]


def _make_kernel(cfg):
    tq = cfg["tq"]
    nq = S // tq
    nsub = tq // LANE
    KT = MP // LANE
    TP = LANE // 2
    XC = 4
    x_cols = S // XC
    QP = cfg["q_pairs"]
    WP = 64 * QP
    WS = 2
    QIT = 8 // QP
    AT = 3

    def kernel(aq_hbm, ak_hbm, av_hbm, sh_hbm, ssm_hbm, dd_hbm, x_hbm, c_hbm,
               wq_hbm, wk_hbm, wv_hbm, wo_hbm,
               out_hbm,
               a_v, sh_v, dd_v, par_v, f_v,
               xt_v, x_v, c_v, wqs_v, wq_v, qacc, ws_v, wkv_v, wo_v,
               q_all, k_s, v_s, p_s, ra_t, rb_t, oa_v, out_v,
               sem_x, sem_wq, sem_w, sem_c, sem_s, sem_a, sem_out):
        x32, c32, wq32, wk32, wv32, wo32 = (
            r.bitcast(U32) for r in (x_hbm, c_hbm, wq_hbm, wk_hbm, wv_hbm, wo_hbm))
        a32 = [r.bitcast(U32) for r in (ak_hbm, av_hbm, ssm_hbm, aq_hbm)]

        def x_copy(i):
            cs = pl.ds(i * x_cols, x_cols)
            return pltpu.make_async_copy(x32.at[:, cs], xt_v.at[:, cs], sem_x.at[i])

        def wq_copies(kt):
            dst = wqs_v.reshape(4 * KT, TP, 8, LANE)
            rs = pl.ds(min(kt * TP, M // 2 - TP), TP)
            return [pltpu.make_async_copy(
                wq32.at[rs, pl.ds(8 * (k // 2), 8), pl.ds((k % 2) * LANE, LANE)],
                dst.at[4 * kt + k], sem_wq.at[kt]) for k in range(4)]

        def wq_wait(kt):
            pltpu.make_async_copy(wqs_v.at[kt], wqs_v.at[kt], sem_wq.at[kt]).wait()

        def w_rows(chunk):
            r0 = chunk * WP
            return pl.ds(r0 if isinstance(r0, int) else pl.multiple_of(r0, WP), WP)

        def w_copies(chunk, slot):
            dst = ws_v.reshape(8 * WS, WP, 8, LANE)
            rs = w_rows(chunk)
            out = []
            for which, src in enumerate((wk32, wv32)):
                for par in range(2):
                    for half in range(2):
                        k = 8 * slot + 4 * which + 2 * par + half
                        out.append(pltpu.make_async_copy(
                            src.at[rs, pl.ds(8 * par, 8), pl.ds(half * LANE, LANE)],
                            dst.at[k], sem_w.at[slot]))
            return out

        def w_wait(slot):
            pltpu.make_async_copy(ws_v.at[slot], ws_v.at[slot], sem_w.at[slot]).wait()

        def piece_start(it):
            n = S // 2 // QIT
            rs = pl.ds(pl.multiple_of(it * n, n), n)
            pltpu.make_async_copy(c32.at[rs], c_v.at[rs], sem_c.at[0]).start()
            hs = pl.ds(it * (H // QIT), H // QIT)
            pltpu.make_async_copy(wo32.at[hs], wo_v.at[hs], sem_a.at[0]).start()

        a_parts = [pl.ds(0, AR // 2), pl.ds(AR // 2, M // 2 - AR // 2)]

        def a_start(part):
            rs = a_parts[part]
            for k in range(4):
                pltpu.make_async_copy(
                    a32[k].at[rs], a_v.at[k, rs], sem_a.at[1 + part]).start()

        def a_wait(part):
            view = a_v.at[:, a_parts[part]]
            pltpu.make_async_copy(view, view, sem_a.at[1 + part]).wait()

        small = [pltpu.make_async_copy(sh_hbm, sh_v, sem_s.at[0]),
                 pltpu.make_async_copy(dd_hbm, dd_v, sem_s.at[1])]

        link = [None]

        pace = [None]

        def set_link(res, row=None, pacer=None):
            if row is None:
                row = res.shape[0] - cfg["link_back"]
            link[0] = _opaque_zero([res[row:row + 8, res.shape[1] - LANE:]])
            pace[0] = res if pacer is None else pacer

        def linked(x):
            return x if link[0] is None else _pin(x, link[0])

        def paced(w):
            res = pace[0]
            if res is None or link[0] is None or not cfg["pace_step"]:
                return w
            rows = []
            zs = [_opaque_zero([res[r:r + 8, res.shape[1] - LANE:]])
                  for r in range(cfg["pace_row"], cfg["pace_row"] + 8 * cfg["pace_step"],
                                 cfg["pace_step"])]
            for r in range(0, w.shape[0], 8):
                z = zs[7 - (r // 8) % 8]
                t = pltpu.bitcast(w[r:r + 8, :], jnp.int32)
                rows.append(pltpu.bitcast(t + _lanecat([z] * (w.shape[1] // LANE)), U32))
            return _rowcat(rows)

        with jax.named_scope("first_starts"):
            for cp in small:
                cp.start()
        x_copy(0).start()
        for kt in range(cfg["wq_first"]):
            for cp in wq_copies(kt):
                cp.start()

        bi = lax.broadcasted_iota(jnp.int32, (LANE, LANE), 0)
        mi = lax.broadcasted_iota(jnp.int32, (LANE, LANE), 1)
        ph = ((4 * mi + 1) * bi) & 511
        ang = ph.astype(F32) * (2.0 * 3.141592653589793 / 512.0)
        f_v[:, 0:LANE] = _u32(jnp.cos(ang).astype(BF16))
        f_v[:, LANE:] = _u32((-jnp.sin(ang)).astype(BF16))

        rb_t[...] = jnp.zeros((S // D, M, D), F32)
        ra_t[:, 0:LANE, :] = jnp.zeros((2, LANE, S // 2), F32)
        ra_t[:, AT * LANE:, :] = jnp.zeros((2, M - AT * LANE, S // 2), F32)

        for kt in range(cfg["wq_first"], KT):
            for cp in wq_copies(kt):
                cp.start()
        with jax.named_scope("small_wait"):
            for cp in small:
                cp.wait()
        sh = sh_v[...].astype(F32)
        for j in range(KS):
            par_v[j] = jnp.broadcast_to(sh[j:j + 1, :], (LANE, M)).T
        dd = dd_v[...].astype(F32).reshape(1, M)
        par_v[KS] = jnp.broadcast_to(dd, (LANE, M)).T

        def x_transpose(i):
            xt = xt_v[:, pl.ds(i * x_cols, x_cols)]
            nfull = (KT - 1) * TP
            xt = _rowcat([xt[:nfull], jnp.zeros((MP // 2 - M // 2, x_cols), U32), xt[nfull:]])
            x_v[_h(i * x_cols, x_cols), :] = _u32(_bf(xt).astype(F32).T.astype(BF16))

        def q_early(kt, first, last):
            r0 = kt * TP
            rows = pl.ds(r0 if isinstance(r0, int) else pl.multiple_of(r0, TP), TP)
            c0 = kt * LANE
            cols = pl.ds(c0 if isinstance(c0, int) else pl.multiple_of(c0, LANE), LANE)
            link[0] = None
            for j in range(H // 2):
                ws = []
                for half in range(2):
                    ev, od = (
                        wqs_v[kt, pl.ds((2 * par + half) * TP * 8 + j, TP, stride=8), :]
                        for par in range(2))
                    ws.append(_repack(ev, od))
                w = _lanecat([ws[0][0], ws[1][0], ws[0][1], ws[1][1]])
                wq_v[j, rows, :] = w
                d = _dot(_bf(linked(x_v[_h(0, x_cols), cols])), _bf(w))
                set_link(d)
                if not first:
                    d = d + qacc[j]
                if last:
                    d = (d * (D ** -0.5 * LOG2E)).astype(BF16)
                    for t in range(2):
                        q_all[2 * j + t, _h(0, x_cols), :] = _u32(d[:, t * D:(t + 1) * D])
                else:
                    qacc[j] = d

        with jax.named_scope("x_wait"):
            x_copy(0).wait()
        x_transpose(0)
        with jax.named_scope("wq_wait"):
            wq_wait(0)
        q_early(0, True, False)
        for i in range(1, XC):
            x_copy(i).start()
        for cp in w_copies(0, 0):
            cp.start()

        def early_body(kt, carry):
            with jax.named_scope("wq_wait"):
                wq_wait(kt)
            q_early(kt, False, False)
            return carry

        lax.fori_loop(1, KT - 1, early_body, 0)
        with jax.named_scope("wq_wait"):
            wq_wait(KT - 1)
            for i in range(1, XC):
                x_copy(i).wait()
        q_early(KT - 1, False, True)
        for i in range(1, XC):
            x_transpose(i)

        def unpack(chunk, slot, sub, which, half, j):
            ev, od = (
                ws_v[slot, pl.ds(((4 * which + 2 * par + half) * WP + sub * TP) * 8 + j, TP,
                                 stride=8), :]
                for par in range(2))
            lo, hi = _repack(ev, od)
            rows = pl.ds(pl.multiple_of(chunk * WP + sub * TP, TP), TP)
            cols = pl.ds(which * D + half * LANE, LANE)
            wkv_v[2 * j, rows, cols] = lo
            wkv_v[2 * j + 1, rows, cols] = hi
            return [lo, hi]

        units = [(s_, w_, h_, j_) for s_ in range(QP) for w_ in range(2) for h_ in range(2)
                 for j_ in range(H // 2)]

        def qproj(it, r0, n, t, zeros=(None, None)):
            outs = []
            for u in range(2):
                lhs = _bf(linked(x_v[_h(r0, n), :]))
                d = _dot(lhs, _bf(wq_v[it, :, pl.ds(t * D + u * LANE, LANE)]))
                set_link(d)
                if zeros[u] is not None:
                    for k, z in enumerate(zeros[u]):
                        d = _pin(d, z, 8 * ((k * (n // 8)) // len(zeros[u])))
                outs.append(d)
            q2 = _lanecat(outs)
            q_all[2 * it + t, _h(r0, n), :] = _u32((q2 * (D ** -0.5 * LOG2E)).astype(BF16))

        def q_body(it, carry):
            slot = it % WS
            with jax.named_scope("w_wait"):
                w_wait(slot)

            @pl.when(it + 1 < QIT)
            def _():
                for cp in w_copies(it + 1, 1 - slot):
                    cp.start()

            piece_start(it)
            link[0] = None
            pieces = [(p, pc, t) for p in range(QP) for pc in range(1, XC) for t in range(2)]
            nd = 2 * len(pieces)
            for k, (p, pc, t) in enumerate(pieces):
                zeros = []
                for u in range(2):
                    d = 2 * k + u
                    mine = units[d * len(units) // nd:(d + 1) * len(units) // nd]
                    zeros.append([_opaque_zero(unpack(it, slot, *u_)) for u_ in mine])
                qproj(QP * it + p, pc * x_cols, x_cols, t, zeros)
            return carry

        a_start(0)
        with jax.named_scope("q_loop"):
            lax.fori_loop(0, QIT, q_body, 0)
        a_start(1)
        pltpu.make_async_copy(c_v, c_v, sem_c.at[0]).wait()
        a_wait(0)
        pltpu.make_async_copy(wo_v, wo_v, sem_a.at[0]).wait()

        tri = (lax.broadcasted_iota(jnp.int32, (LANE, LANE), 1)
               <= lax.broadcasted_iota(jnp.int32, (LANE, LANE), 0))

        NOUT = S // D

        def out_copy(i):
            if i >= NOUT:
                t = i - NOUT
                return pltpu.make_async_copy(
                    oa_v.at[t], out_hbm.at[:, pl.ds(t * LANE, LANE)], sem_out.at[i])
            rs = pl.ds(i * D, D)
            return pltpu.make_async_copy(
                out_v.at[rs], out_hbm.at[rs, pl.ds(AT * LANE, 2 * M - AT * LANE)], sem_out.at[i])

        def b_out(k, tot):
            c0 = (k * D) % (S // 2)
            full = _rowcat([ra_t[k * D // (S // 2), AT * LANE:, c0:c0 + D], tot]).T
            out_v[k * D:(k + 1) * D, :] = full.astype(BF16)
            return full

        def head_step(h, carry):
            with jax.named_scope("step"):
                return head_step_(h, carry)

        def head_step_(h, carry):
            with_a = cfg["use_a"]

            @pl.when(h == A_STEPS)
            def _():
                for t in range(AT):
                    out_copy(NOUT + t).start()

            @pl.when(h == cfg["h0"] + 1)
            def _():
                a_wait(1)

            link[0] = None
            n2 = AR // 2
            a_rows2 = pl.ds(pl.multiple_of(jnp.minimum(h, A_STEPS - 1) * n2, n2), n2)
            a_rows = pl.ds(pl.multiple_of(jnp.minimum(h, A_STEPS - 1) * AR, AR), AR)

            def a_fwd():
                kk = _bf(a_v[0, a_rows2, :]).astype(F32)
                lane = lax.broadcasted_iota(jnp.int32, (AR, LANE), 1)
                coef = [par_v[j, a_rows, :] for j in range(KS)]
                rolled = [kk] + [pltpu.roll(kk, j, 1) for j in range(1, KS)]
                vv = _bf(a_v[1, a_rows2, :]).astype(F32)
                kv_blocks = []
                for a in range(NB):
                    cs = slice(a * LANE, (a + 1) * LANE)
                    acc = rolled[0][:, cs] * coef[0]
                    for j in range(1, KS):
                        t = rolled[j][:, cs]
                        if a == 0:
                            t = jnp.where(lane >= j, t, 0.0)
                        acc = acc + t * coef[j]
                    kv_blocks.append(acc * vv[:, cs])
                hk = a_v[2, a_rows2, :]
                hk = _rowcat([hk[:, a * LANE:(a + 1) * LANE] for a in range(NB)])
                fm = _bf(f_v[...])
                hs = _dot(_bf(linked(hk)), fm)
                kv = linked(_rowcat(kv_blocks)).astype(BF16)
                xs = _dot(kv, fm)
                set_link(xs)
                return kv, xs, hs

            def a_conv(xs, hs):
                def tile(v, a, g, part):
                    r = a * AR + 8 * g
                    return v[r:r + 8, part * LANE:(part + 1) * LANE]

                z = {}
                nch = cfg["a_chains"]
                gates = [None] * nch
                width = cfg["a_width"]
                k = 0
                for g in range(AR // 8):
                    hr = [tile(hs, 0, g, 0)] + [
                        tile(hs, j, g, 0) - tile(hs, j - 1, g, 1) for j in range(1, NB)]
                    hi = [tile(hs, 0, g, 1)] + [
                        tile(hs, j, g, 1) + tile(hs, j - 1, g, 0) for j in range(1, NB)]
                    for c0 in range(0, NB, width):
                        ch = k % nch
                        k += 1
                        for a in range(c0 + width):
                            xr, xi = tile(xs, a, g, 0), tile(xs, a, g, 1)
                            if gates[ch] is not None and cfg["a_gate"]:
                                xr, xi = _pin(xr, gates[ch]), _pin(xi, gates[ch])
                            for c in range(max(c0, a), c0 + width):
                                j = c - a
                                tr = xr * hr[j] - xi * hi[j]
                                ti = xr * hi[j] + xi * hr[j]
                                z[c, g] = (tr, ti) if a == 0 else (z[c, g][0] + tr, z[c, g][1] + ti)
                            gates[ch] = _opaque_zero(list(z[c0 + width - 1, g]))
                return z

            def a_inv(kv, z):
                fm = _bf(f_v[...])
                ng = AR // 8
                ys = []
                for u in range(2):
                    rows = [_lanecat(z[c, g]) for g in range(u * ng // 2, (u + 1) * ng // 2)
                            for c in range(NB)]
                    ys.append(_dot_nt(linked(_rowcat(rows)).astype(BF16), fm))
                y = _rowcat(ys)
                dd = par_v[KS, a_rows, :]
                for c in range(NB):
                    cs = slice(c * LANE, (c + 1) * LANE)
                    yc = _rowcat([y[(g * NB + c) * 8:(g * NB + c + 1) * 8, :] for g in range(ng)])
                    qq = _bf(a_v[3, a_rows2, cs]).astype(F32)
                    kvf = kv[c * AR:(c + 1) * AR, :].astype(F32)
                    c2 = (c % (NB // 2)) * LANE
                    ra_t[c // (NB // 2), a_rows, c2:c2 + LANE] = qq * (yc * (1.0 / LANE) + kvf * dd)

            def a_out():
                slab = jnp.clip(h // 4 - 1, 0, AT - 1)
                half = h % 2
                x = ra_t[half, pl.ds(pl.multiple_of(slab * LANE, LANE), LANE), :]
                xt = x.T
                dst = jnp.where(h >= A_STEPS, AT, slab)
                oa_v[dst, pl.ds(pl.multiple_of(half * (S // 2), S // 2), S // 2), :] = xt.astype(BF16)
                return xt

            kw = C // 2
            pending = []

            def flush_pending(x, row):
                done = list(pending)
                del pending[:]
                if not done:
                    return x
                x = _pin(x, _opaque_zero([f for _, f in done]), row)

                @pl.when(h == H - 1)
                def _():
                    for k, _f in done:
                        out_copy(k).start()
                return x

            def proj_w(which, k):
                return wkv_v[h, _h((k % 2) * kw, kw), pl.ds(which * D + (k // 2) * LANE, LANE)]

            def proj(dst, which, r0, n):
                ds = []
                for k in range(4):
                    lhs = linked(c_v[_h(r0, n), pl.ds((k % 2) * kw, kw)])
                    if which == 1 and k == cfg["bo_pass"]:
                        lhs = flush_pending(lhs, cfg["ao_row"])
                    ds.append(_dot(_bf(lhs), _bf(paced(proj_w(which, k)))))
                    set_link(ds[-1])
                dst[r0:r0 + n, :] = _lanecat([ds[0] + ds[1], ds[2] + ds[3]]).astype(BF16)

            def qk(i, dep=None):
                r0 = i * tq
                q = linked(q_all[h, _h(r0, tq), :])
                if dep is not None:
                    q = _pin(q, _opaque_zero([dep]), cfg["ao_row"])
                parts = [_dot_nt(_bf(q), k_s[0:r0 + LANE, :])]
                if i > 0:
                    link[0] = _opaque_zero([parts[0][0:8, r0 - LANE:r0]])
                for j in range(1, nsub):
                    q = linked(q_all[h, _h(r0 + LANE * j, tq - LANE * j), :])
                    parts.append(_dot_nt(_bf(q), k_s[r0 + LANE * j:r0 + LANE * (j + 1), :]))
                set_link(parts[2], cfg["link_part"], parts[0])
                return parts

            def softmax(i, parts):
                pb = p_s.at[i % 2]
                chain = _opaque_zero([b[b.shape[0] - 8:, b.shape[1] - LANE:] for b in parts])
                ls = []
                for a in range(nsub):
                    blocks = [parts[j][LANE * (a - j):LANE * (a - j + 1), :] for j in range(a + 1)]
                    last = blocks[-1]
                    w = last.shape[1]
                    dg = jnp.where(tri, last[:, w - LANE:], NEG)
                    blocks[-1] = dg if w == LANE else _lanecat([last[:, :w - LANE], dg])
                    sa = _lanecat(blocks)
                    mb = jnp.broadcast_to(jnp.max(sa, axis=1, keepdims=True), (LANE, LANE))
                    nt = sa.shape[1] // LANE
                    ptiles, psums = [], []
                    for g in range(0, LANE, 8):
                        mg = _pin(mb[g:g + 8, :], chain)
                        pg = [jnp.exp2(sa[g:g + 8, t * LANE:(t + 1) * LANE] - mg) for t in range(nt)]
                        ps = functools.reduce(jnp.add, pg)
                        chain = _opaque_zero([ps])
                        psums.append(ps)
                        ptiles.append(_lanecat(pg))
                    ls.append(jnp.sum(_rowcat(psums), axis=1, keepdims=True))
                    p = _pin(_rowcat(ptiles), link[0], 0, 0 if a == 0 else sa.shape[1] - LANE)
                    pb[LANE * a:LANE * (a + 1), 0:sa.shape[1]] = p.astype(BF16)
                return ls

            def pv(i, ls):
                r0 = i * tq
                pb = p_s.at[i % 2]
                ctx = [_dot(pb[:, 0:r0 + LANE], v_s[0:r0 + LANE, :])]
                for j in range(1, nsub):
                    ctx.append(_dot(pb[LANE * j:, r0 + LANE * j:r0 + LANE * (j + 1)],
                                    v_s[r0 + LANE * j:r0 + LANE * (j + 1), :]))
                set_link(ctx[2], cfg["link_part"])
                cs = []
                for a in range(nsub):
                    sl = lambda j: slice(LANE * (a - j), LANE * (a - j + 1))
                    r = pl.reciprocal(ls[a], approx=True)
                    r = r * (2.0 - ls[a] * r)
                    cs.append(functools.reduce(jnp.add, [ctx[j][sl(j)] for j in range(a + 1)]) * r)
                return _rowcat(cs).astype(BF16)

            def oproj(i, ctx):
                for u in range(tq // D):
                    res = _dot_nt(_bf(linked(wo_v[h])), ctx[u * D:(u + 1) * D, :])
                    set_link(res)
                    k = i * (tq // D) + u
                    tot = rb_t[k] + res
                    rb_t[k] = tot
                    if cfg["b_out"] and i < nq - 1:
                        pending.append((k, b_out(k, tot)))

            a_state = {}

            def a_hook(tag):
                if with_a and tag == cfg["a_fwd_at"]:
                    a_state["kv"], xs, hs = a_fwd()
                    a_state["z"] = a_conv(xs, hs)
                if with_a and tag == cfg["a_inv_at"]:
                    a_inv(a_state["kv"], a_state["z"])

            a_hook(0)
            proj(k_s, 0, 0, tq)
            a_hook(1)
            parts = qk(0)
            ctx_prev = None
            for i in range(nq):
                r0 = i * tq
                a_hook(10 * (i + 1))
                if ctx_prev is not None:
                    oproj(i - 1, ctx_prev)
                a_hook(10 * (i + 1) + 1)
                if i + 1 < nq:
                    proj(k_s, 0, r0 + tq, tq)
                a_hook(10 * (i + 1) + 2)
                proj(v_s, 1, r0, tq)
                a_hook(10 * (i + 1) + 3)
                ls = softmax(i, parts)
                ctx_prev = pv(i, ls)
                a_hook(10 * (i + 1) + 4)
                if i + 1 < nq:
                    parts = qk(i + 1, a_out() if i + 1 == cfg["ao_at"] else None)
            oproj(nq - 1, ctx_prev)
            assert not pending
            return carry

        with jax.named_scope("loop_a"):
            lax.fori_loop(cfg["h0"], H, head_step, 0)
        with jax.named_scope("tail"):
            for i in range((nq - 1) * (tq // D) if cfg["b_out"] else 0, NOUT):
                b_out(i, rb_t[i])
                out_copy(i).start()
            for i in range(NOUT + AT):
                out_copy(i).wait()

    scratch = [
        pltpu.VMEM((4, M // 2, S), U32),
        pltpu.VMEM((KS, M), BF16),
        pltpu.VMEM((M,), BF16),
        pltpu.VMEM((KS + 1, M, LANE), F32),
        pltpu.VMEM((LANE // 2, 2 * LANE), U32),
        pltpu.VMEM((M // 2, S), U32),
        pltpu.VMEM((S // 2, MP), U32),
        pltpu.VMEM((S // 2, C), U32),
        pltpu.VMEM((KT, 4 * TP * 8, LANE), U32),
        pltpu.VMEM((H // 2, MP // 2, 2 * D), U32),
        pltpu.VMEM((H // 2, x_cols, 2 * D), F32),
        pltpu.VMEM((WS, 8 * WP * 8, LANE), U32),
        pltpu.VMEM((H, C // 2, 2 * D), U32),
        pltpu.VMEM((H, M // 2, D), U32),
        pltpu.VMEM((H, S // 2, D), U32),
        pltpu.VMEM((S, D), BF16),
        pltpu.VMEM((S, D), BF16),
        pltpu.VMEM((2, tq, S), BF16),
        pltpu.VMEM((2, M, S // 2), F32),
        pltpu.VMEM((S // D, M, D), F32),
        pltpu.VMEM((AT + 1, S, LANE), BF16),
        pltpu.VMEM((S, 2 * M - AT * LANE), BF16),
        pltpu.SemaphoreType.DMA((XC,)),
        pltpu.SemaphoreType.DMA((KT,)),
        pltpu.SemaphoreType.DMA((WS,)),
        pltpu.SemaphoreType.DMA((1,)),
        pltpu.SemaphoreType.DMA((2,)),
        pltpu.SemaphoreType.DMA((3,)),
        pltpu.SemaphoreType.DMA((S // D + AT,)),
    ]
    return kernel, scratch


_DEFAULT = dict(tq=512, a_fwd_at=13, a_inv_at=44, a_gate=1, a_chains=1, a_width=4, ao_at=1, ao_row=240, b_out=1, bo_pass=3, q_pairs=2, wq_first=1,
                link_back=176, pace_row=32, pace_step=24, link_part=32, use_a=1, h0=0)


def _build(**kw):
    cfg = dict(_DEFAULT)
    cfg.update(kw)
    kernel, scratch = _make_kernel(cfg)

    def run(A_q, A_k, A_v, A_shift_k, A_ssm_k, A_ssm_D, B_x, B_c_kv, B_w_q, B_w_uk,
            B_w_uv, B_w_o):
        tr = lambda a: jnp.swapaxes(a, 1, 2).reshape(M, S)
        args = (
            tr(A_q), tr(A_k), tr(A_v), A_shift_k.T, A_ssm_k, A_ssm_D, tr(B_x),
            B_c_kv.reshape(S, C),
            B_w_q.reshape(M // 2, 2 * H, D), B_w_uk.reshape(C // 2, 2 * H, D),
            B_w_uv.reshape(C // 2, 2 * H, D),
            jnp.swapaxes(B_w_o, 1, 2),
        )
        out = pl.pallas_call(
            kernel,
            in_specs=[pl.BlockSpec(memory_space=pl.ANY)] * len(args),
            out_specs=pl.BlockSpec(memory_space=pl.ANY),
            out_shape=jax.ShapeDtypeStruct((S, 2 * M), BF16),
            scratch_shapes=scratch,
            compiler_params=pltpu.CompilerParams(
                vmem_limit_bytes=120 * 1024 * 1024,
                disable_bounds_checks=True),
        )(*args)
        return out.reshape(1, S, 2 * M)

    return run


_run = _build()


@jax.jit
def pallas_concat_heads__ssm_conv_h3__compressed_kv_cla__prompt_kernel(
    A_q: jax.Array,
    A_k: jax.Array,
    A_v: jax.Array,
    A_shift_k: jax.Array,
    A_ssm_k: jax.Array,
    A_ssm_D: jax.Array,
    B_x: jax.Array,
    B_c_kv: jax.Array,
    B_w_q: jax.Array,
    B_w_uk: jax.Array,
    B_w_uv: jax.Array,
    B_w_o: jax.Array,
):
    return _run(A_q, A_k, A_v, A_shift_k, A_ssm_k, A_ssm_D, B_x, B_c_kv, B_w_q,
                B_w_uk, B_w_uv, B_w_o)
```

```python
import functools

import jax
import jax.numpy as jnp
from jax import lax
import jax.experimental.pallas as pl
import jax.experimental.pallas.tpu as pltpu

F32 = jnp.float32
BF16 = jnp.bfloat16
U32 = jnp.uint32

S = 2048
M = 448
MP = 512
C = 1024
H = 16
D = 256
KS = 4
LANE = 128
NB = S // LANE
AR = 32
A_STEPS = M // AR
LOG2E = 1.4426950408889634
NEG = -1e30

NT = (((1,), (1,)), ((), ()))


def _dot(a, b):
    return jnp.dot(a, b, preferred_element_type=F32)


def _dot_nt(a, b):
    return lax.dot_general(a, b, NT, preferred_element_type=F32)


def _bf(x):
    return pltpu.bitcast(x, BF16)


def _u32(x):
    return pltpu.bitcast(x, U32)


def _h(r0, n):
    return pl.ds(r0 // 2, n // 2)


def _repack(ev, od):
    lo = (ev & jnp.uint32(0xFFFF)) | (od << 16)
    hi = (ev >> 16) | (od & jnp.uint32(0xFFFF0000))
    return lo, hi


def _opaque_zero(vals):
    acc = None
    for v in vals:
        b = v if v.dtype == U32 else pltpu.bitcast(v, U32)
        for r in range(0, b.shape[0], 8):
            for c in range(0, b.shape[1], LANE):
                t = b[r:r + 8, c:c + LANE]
                acc = t if acc is None else acc | t
    return jnp.minimum((acc >> 1).astype(jnp.int32), 0)


def _pin(x, zero, r=0, c=0):
    t = pltpu.bitcast(pltpu.bitcast(x[r:r + 8, c:c + LANE], jnp.int32) + zero, x.dtype)
    row = ([x[r:r + 8, :c]] if c > 0 else []) + [t] + (
        [x[r:r + 8, c + LANE:]] if c + LANE < x.shape[1] else [])
    row = jnp.concatenate(row, axis=1) if len(row) > 1 else row[0]
    col = ([x[:r, :]] if r > 0 else []) + [row] + ([x[r + 8:, :]] if r + 8 < x.shape[0] else [])
    return jnp.concatenate(col, axis=0) if len(col) > 1 else col[0]


def _rowcat(xs):
    return jnp.concatenate(xs, axis=0) if len(xs) > 1 else xs[0]


def _lanecat(xs):
    return jnp.concatenate(xs, axis=1) if len(xs) > 1 else xs[0]


def _make_kernel(cfg):
    tq = cfg["tq"]
    nq = S // tq
    nsub = tq // LANE
    KT = MP // LANE
    TP = LANE // 2
    XC = 4
    x_cols = S // XC
    QP = cfg["q_pairs"]
    WP = 64 * QP
    WS = 2
    QIT = 8 // QP
    AT = 3

    def kernel(aq_hbm, ak_hbm, av_hbm, sh_hbm, ssm_hbm, dd_hbm, x_hbm, c_hbm,
               wq_hbm, wk_hbm, wv_hbm, wo_hbm,
               out_hbm,
               a_v, sh_v, dd_v, par_v, f_v,
               xt_v, x_v, c_v, wqs_v, wq_v, qacc, ws_v, wkv_v, wo_v,
               q_all, k_s, v_s, p_s, ra_t, rb_t, oa_v, out_v,
               sem_x, sem_wq, sem_w, sem_c, sem_s, sem_a, sem_out):
        x32, c32, wq32, wk32, wv32, wo32 = (
            r.bitcast(U32) for r in (x_hbm, c_hbm, wq_hbm, wk_hbm, wv_hbm, wo_hbm))
        a32 = [r.bitcast(U32) for r in (ak_hbm, av_hbm, ssm_hbm, aq_hbm)]

        def x_copy(i):
            cs = pl.ds(i * x_cols, x_cols)
            return pltpu.make_async_copy(x32.at[:, cs], xt_v.at[:, cs], sem_x.at[i])

        def wq_copies(kt):
            dst = wqs_v.reshape(4 * KT, TP, 8, LANE)
            rs = pl.ds(min(kt * TP, M // 2 - TP), TP)
            return [pltpu.make_async_copy(
                wq32.at[rs, pl.ds(8 * (k // 2), 8), pl.ds((k % 2) * LANE, LANE)],
                dst.at[4 * kt + k], sem_wq.at[kt]) for k in range(4)]

        def wq_wait(kt):
            pltpu.make_async_copy(wqs_v.at[kt], wqs_v.at[kt], sem_wq.at[kt]).wait()

        def w_rows(chunk):
            r0 = chunk * WP
            return pl.ds(r0 if isinstance(r0, int) else pl.multiple_of(r0, WP), WP)

        def w_copies(chunk, slot):
            dst = ws_v.reshape(8 * WS, WP, 8, LANE)
            rs = w_rows(chunk)
            out = []
            for which, src in enumerate((wk32, wv32)):
                for par in range(2):
                    for half in range(2):
                        k = 8 * slot + 4 * which + 2 * par + half
                        out.append(pltpu.make_async_copy(
                            src.at[rs, pl.ds(8 * par, 8), pl.ds(half * LANE, LANE)],
                            dst.at[k], sem_w.at[slot]))
            return out

        def w_wait(slot):
            pltpu.make_async_copy(ws_v.at[slot], ws_v.at[slot], sem_w.at[slot]).wait()

        def piece_start(it):
            n = S // 2 // QIT
            rs = pl.ds(pl.multiple_of(it * n, n), n)
            pltpu.make_async_copy(c32.at[rs], c_v.at[rs], sem_c.at[0]).start()
            hs = pl.ds(it * (H // QIT), H // QIT)
            pltpu.make_async_copy(wo32.at[hs], wo_v.at[hs], sem_a.at[0]).start()

        a_parts = [pl.ds(0, AR // 2), pl.ds(AR // 2, M // 2 - AR // 2)]

        def a_start(part):
            rs = a_parts[part]
            for k in range(4):
                pltpu.make_async_copy(
                    a32[k].at[rs], a_v.at[k, rs], sem_a.at[1 + part]).start()

        def a_wait(part):
            view = a_v.at[:, a_parts[part]]
            pltpu.make_async_copy(view, view, sem_a.at[1 + part]).wait()

        small = [pltpu.make_async_copy(sh_hbm, sh_v, sem_s.at[0]),
                 pltpu.make_async_copy(dd_hbm, dd_v, sem_s.at[1])]

        link = [None]

        pace = [None]

        def set_link(res, row=None, pacer=None):
            if row is None:
                row = res.shape[0] - cfg["link_back"]
            link[0] = _opaque_zero([res[row:row + 8, res.shape[1] - LANE:]])
            pace[0] = res if pacer is None else pacer

        def linked(x):
            return x if link[0] is None else _pin(x, link[0])

        def paced(w):
            res = pace[0]
            if res is None or link[0] is None or not cfg["pace_step"]:
                return w
            rows = []
            zs = [_opaque_zero([res[r:r + 8, res.shape[1] - LANE:]])
                  for r in range(cfg["pace_row"], cfg["pace_row"] + 8 * cfg["pace_step"],
                                 cfg["pace_step"])]
            for r in range(0, w.shape[0], 8):
                z = zs[7 - (r // 8) % 8]
                t = pltpu.bitcast(w[r:r + 8, :], jnp.int32)
                rows.append(pltpu.bitcast(t + _lanecat([z] * (w.shape[1] // LANE)), U32))
            return _rowcat(rows)

        with jax.named_scope("first_starts"):
            for cp in small:
                cp.start()
        x_copy(0).start()
        for kt in range(cfg["wq_first"]):
            for cp in wq_copies(kt):
                cp.start()

        bi = lax.broadcasted_iota(jnp.int32, (LANE, LANE), 0)
        mi = lax.broadcasted_iota(jnp.int32, (LANE, LANE), 1)
        ph = ((4 * mi + 1) * bi) & 511
        ang = ph.astype(F32) * (2.0 * 3.141592653589793 / 512.0)
        f_v[:, 0:LANE] = _u32(jnp.cos(ang).astype(BF16))
        f_v[:, LANE:] = _u32((-jnp.sin(ang)).astype(BF16))

        rb_t[...] = jnp.zeros((S // D, M, D), F32)
        ra_t[:, 0:LANE, :] = jnp.zeros((2, LANE, S // 2), F32)
        ra_t[:, AT * LANE:, :] = jnp.zeros((2, M - AT * LANE, S // 2), F32)

        for kt in range(cfg["wq_first"], KT):
            for cp in wq_copies(kt):
                cp.start()
        with jax.named_scope("small_wait"):
            for cp in small:
                cp.wait()
        sh = sh_v[...].astype(F32)
        for j in range(KS):
            par_v[j] = jnp.broadcast_to(sh[j:j + 1, :], (LANE, M)).T
        dd = dd_v[...].astype(F32).reshape(1, M)
        par_v[KS] = jnp.broadcast_to(dd, (LANE, M)).T

        def x_transpose(i):
            xt = xt_v[:, pl.ds(i * x_cols, x_cols)]
            nfull = (KT - 1) * TP
            xt = _rowcat([xt[:nfull], jnp.zeros((MP // 2 - M // 2, x_cols), U32), xt[nfull:]])
            x_v[_h(i * x_cols, x_cols), :] = _u32(_bf(xt).astype(F32).T.astype(BF16))

        def q_early(kt, first, last):
            r0 = kt * TP
            rows = pl.ds(r0 if isinstance(r0, int) else pl.multiple_of(r0, TP), TP)
            c0 = kt * LANE
            cols = pl.ds(c0 if isinstance(c0, int) else pl.multiple_of(c0, LANE), LANE)
            link[0] = None
            for j in range(H // 2):
                ws = []
                for half in range(2):
                    ev, od = (
                        wqs_v[kt, pl.ds((2 * par + half) * TP * 8 + j, TP, stride=8), :]
                        for par in range(2))
                    ws.append(_repack(ev, od))
                w = _lanecat([ws[0][0], ws[1][0], ws[0][1], ws[1][1]])
                wq_v[j, rows, :] = w
                d = _dot(_bf(linked(x_v[_h(0, x_cols), cols])), _bf(w))
                set_link(d)
                if not first:
                    d = d + qacc[j]
                if last:
                    d = (d * (D ** -0.5 * LOG2E)).astype(BF16)
                    for t in range(2):
                        q_all[2 * j + t, _h(0, x_cols), :] = _u32(d[:, t * D:(t + 1) * D])
                else:
                    qacc[j] = d

        with jax.named_scope("x_wait"):
            x_copy(0).wait()
        x_transpose(0)
        with jax.named_scope("wq_wait"):
            wq_wait(0)
        q_early(0, True, False)
        for i in range(1, XC):
            x_copy(i).start()
        for cp in w_copies(0, 0):
            cp.start()

        def early_body(kt, carry):
            with jax.named_scope("wq_wait"):
                wq_wait(kt)
            q_early(kt, False, False)
            return carry

        lax.fori_loop(1, KT - 1, early_body, 0)
        with jax.named_scope("wq_wait"):
            wq_wait(KT - 1)
            for i in range(1, XC):
                x_copy(i).wait()
        q_early(KT - 1, False, True)
        for i in range(1, XC):
            x_transpose(i)

        def unpack(chunk, slot, sub, which, half, j):
            ev, od = (
                ws_v[slot, pl.ds(((4 * which + 2 * par + half) * WP + sub * TP) * 8 + j, TP,
                                 stride=8), :]
                for par in range(2))
            lo, hi = _repack(ev, od)
            rows = pl.ds(pl.multiple_of(chunk * WP + sub * TP, TP), TP)
            cols = pl.ds(which * D + half * LANE, LANE)
            wkv_v[2 * j, rows, cols] = lo
            wkv_v[2 * j + 1, rows, cols] = hi
            return [lo, hi]

        units = [(s_, w_, h_, j_) for s_ in range(QP) for w_ in range(2) for h_ in range(2)
                 for j_ in range(H // 2)]

        def qproj(it, r0, n, t, zeros=(None, None)):
            outs = []
            for u in range(2):
                lhs = _bf(linked(x_v[_h(r0, n), :]))
                d = _dot(lhs, _bf(wq_v[it, :, pl.ds(t * D + u * LANE, LANE)]))
                set_link(d)
                if zeros[u] is not None:
                    for k, z in enumerate(zeros[u]):
                        d = _pin(d, z, 8 * ((k * (n // 8)) // len(zeros[u])))
                outs.append(d)
            q2 = _lanecat(outs)
            q_all[2 * it + t, _h(r0, n), :] = _u32((q2 * (D ** -0.5 * LOG2E)).astype(BF16))

        def q_body(it, carry):
            slot = it % WS
            with jax.named_scope("w_wait"):
                w_wait(slot)

            @pl.when(it + 1 < QIT)
            def _():
                for cp in w_copies(it + 1, 1 - slot):
                    cp.start()

            piece_start(it)
            link[0] = None
            pieces = [(p, pc, t) for p in range(QP) for pc in range(1, XC) for t in range(2)]
            nd = 2 * len(pieces)
            for k, (p, pc, t) in enumerate(pieces):
                zeros = []
                for u in range(2):
                    d = 2 * k + u
                    mine = units[d * len(units) // nd:(d + 1) * len(units) // nd]
                    zeros.append([_opaque_zero(unpack(it, slot, *u_)) for u_ in mine])
                qproj(QP * it + p, pc * x_cols, x_cols, t, zeros)
            return carry

        a_start(0)
        with jax.named_scope("q_loop"):
            lax.fori_loop(0, QIT, q_body, 0)
        a_start(1)
        pltpu.make_async_copy(c_v, c_v, sem_c.at[0]).wait()
        a_wait(0)
        pltpu.make_async_copy(wo_v, wo_v, sem_a.at[0]).wait()

        tri = (lax.broadcasted_iota(jnp.int32, (LANE, LANE), 1)
               <= lax.broadcasted_iota(jnp.int32, (LANE, LANE), 0))

        NOUT = S // D

        def out_copy(i):
            if i >= NOUT:
                t = i - NOUT
                return pltpu.make_async_copy(
                    oa_v.at[t], out_hbm.at[:, pl.ds(t * LANE, LANE)], sem_out.at[i])
            rs = pl.ds(i * D, D)
            return pltpu.make_async_copy(
                out_v.at[rs], out_hbm.at[rs, pl.ds(AT * LANE, 2 * M - AT * LANE)], sem_out.at[i])

        def b_out(k, tot):
            c0 = (k * D) % (S // 2)
            full = _rowcat([ra_t[k * D // (S // 2), AT * LANE:, c0:c0 + D], tot]).T
            out_v[k * D:(k + 1) * D, :] = full.astype(BF16)
            return full

        def head_step(h, carry):
            with jax.named_scope("step"):
                return head_step_(h, carry)

        def head_step_(h, carry):
            with_a = cfg["use_a"]

            @pl.when(h == A_STEPS)
            def _():
                for t in range(AT):
                    out_copy(NOUT + t).start()

            @pl.when(h == cfg["h0"] + 1)
            def _():
                a_wait(1)

            link[0] = None
            n2 = AR // 2
            a_rows2 = pl.ds(pl.multiple_of(jnp.minimum(h, A_STEPS - 1) * n2, n2), n2)
            a_rows = pl.ds(pl.multiple_of(jnp.minimum(h, A_STEPS - 1) * AR, AR), AR)

            def a_fwd():
                kk = _bf(a_v[0, a_rows2, :]).astype(F32)
                lane = lax.broadcasted_iota(jnp.int32, (AR, LANE), 1)
                coef = [par_v[j, a_rows, :] for j in range(KS)]
                rolled = [kk] + [pltpu.roll(kk, j, 1) for j in range(1, KS)]
                vv = _bf(a_v[1, a_rows2, :]).astype(F32)
                kv_blocks = []
                for a in range(NB):
                    cs = slice(a * LANE, (a + 1) * LANE)
                    acc = rolled[0][:, cs] * coef[0]
                    for j in range(1, KS):
                        t = rolled[j][:, cs]
                        if a == 0:
                            t = jnp.where(lane >= j, t, 0.0)
                        acc = acc + t * coef[j]
                    kv_blocks.append(acc * vv[:, cs])
                hk = a_v[2, a_rows2, :]
                hk = _rowcat([hk[:, a * LANE:(a + 1) * LANE] for a in range(NB)])
                fm = _bf(f_v[...])
                hs = _dot(_bf(linked(hk)), fm)
                kv = linked(_rowcat(kv_blocks)).astype(BF16)
                xs = _dot(kv, fm)
                set_link(xs)
                return kv, xs, hs

            def a_conv(xs, hs):
                def tile(v, a, g, part):
                    r = a * AR + 8 * g
                    return v[r:r + 8, part * LANE:(part + 1) * LANE]

                z = {}
                nch = cfg["a_chains"]
                gates = [None] * nch
                width = cfg["a_width"]
                k = 0
                for g in range(AR // 8):
                    hr = [tile(hs, 0, g, 0)] + [
                        tile(hs, j, g, 0) - tile(hs, j - 1, g, 1) for j in range(1, NB)]
                    hi = [tile(hs, 0, g, 1)] + [
                        tile(hs, j, g, 1) + tile(hs, j - 1, g, 0) for j in range(1, NB)]
                    for c0 in range(0, NB, width):
                        ch = k % nch
                        k += 1
                        for a in range(c0 + width):
                            xr, xi = tile(xs, a, g, 0), tile(xs, a, g, 1)
                            if gates[ch] is not None and cfg["a_gate"]:
                                xr, xi = _pin(xr, gates[ch]), _pin(xi, gates[ch])
                            for c in range(max(c0, a), c0 + width):
                                j = c - a
                                tr = xr * hr[j] - xi * hi[j]
                                ti = xr * hi[j] + xi * hr[j]
                                z[c, g] = (tr, ti) if a == 0 else (z[c, g][0] + tr, z[c, g][1] + ti)
                            gates[ch] = _opaque_zero(list(z[c0 + width - 1, g]))
                return z

            def a_inv(kv, z):
                fm = _bf(f_v[...])
                ng = AR // 8
                ys = []
                for u in range(2):
                    rows = [_lanecat(z[c, g]) for g in range(u * ng // 2, (u + 1) * ng // 2)
                            for c in range(NB)]
                    ys.append(_dot_nt(linked(_rowcat(rows)).astype(BF16), fm))
                y = _rowcat(ys)
                dd = par_v[KS, a_rows, :]
                for c in range(NB):
                    cs = slice(c * LANE, (c + 1) * LANE)
                    yc = _rowcat([y[(g * NB + c) * 8:(g * NB + c + 1) * 8, :] for g in range(ng)])
                    qq = _bf(a_v[3, a_rows2, cs]).astype(F32)
                    kvf = kv[c * AR:(c + 1) * AR, :].astype(F32)
                    c2 = (c % (NB // 2)) * LANE
                    ra_t[c // (NB // 2), a_rows, c2:c2 + LANE] = qq * (yc * (1.0 / LANE) + kvf * dd)

            def a_out():
                slab = jnp.clip(h // 4 - 1, 0, AT - 1)
                half = h % 2
                x = ra_t[half, pl.ds(pl.multiple_of(slab * LANE, LANE), LANE), :]
                xt = x.T
                dst = jnp.where(h >= A_STEPS, AT, slab)
                oa_v[dst, pl.ds(pl.multiple_of(half * (S // 2), S // 2), S // 2), :] = xt.astype(BF16)
                return xt

            kw = C // 2
            pending = []

            def flush_pending(x, row):
                done = list(pending)
                del pending[:]
                if not done:
                    return x
                x = _pin(x, _opaque_zero([f for _, f in done]), row)

                @pl.when(h == H - 1)
                def _():
                    for k, _f in done:
                        out_copy(k).start()
                return x

            def proj_w(which, k):
                return wkv_v[h, _h((k % 2) * kw, kw), pl.ds(which * D + (k // 2) * LANE, LANE)]

            def proj(dst, which, r0, n):
                ds = []
                for k in range(4):
                    lhs = linked(c_v[_h(r0, n), pl.ds((k % 2) * kw, kw)])
                    if which == 1 and k == cfg["bo_pass"]:
                        lhs = flush_pending(lhs, cfg["ao_row"])
                    ds.append(_dot(_bf(lhs), _bf(paced(proj_w(which, k)))))
                    set_link(ds[-1])
                dst[_h(r0, n), :] = _u32(_lanecat([ds[0] + ds[1], ds[2] + ds[3]]).astype(BF16))

            def qk(i, dep=None):
                r0 = i * tq
                q = linked(q_all[h, _h(r0, tq), :])
                if dep is not None:
                    q = _pin(q, _opaque_zero([dep]), cfg["ao_row"])
                parts = [_dot_nt(_bf(q), _bf(k_s[_h(0, r0 + LANE), :]))]
                if i > 0:
                    link[0] = _opaque_zero([parts[0][0:8, r0 - LANE:r0]])
                for j in range(1, nsub):
                    q = linked(q_all[h, _h(r0 + LANE * j, tq - LANE * j), :])
                    parts.append(_dot_nt(_bf(q), _bf(k_s[_h(r0 + LANE * j, LANE), :])))
                set_link(parts[2], cfg["link_part"], parts[0])
                return parts

            def softmax(i, parts):
                pb = p_s.at[i % 2]
                chain = _opaque_zero([b[b.shape[0] - 8:, b.shape[1] - LANE:] for b in parts])
                ls = []
                for a in range(nsub):
                    blocks = [parts[j][LANE * (a - j):LANE * (a - j + 1), :] for j in range(a + 1)]
                    last = blocks[-1]
                    w = last.shape[1]
                    dg = jnp.where(tri, last[:, w - LANE:], NEG)
                    blocks[-1] = dg if w == LANE else _lanecat([last[:, :w - LANE], dg])
                    sa = _lanecat(blocks)
                    mb = jnp.broadcast_to(jnp.max(sa, axis=1, keepdims=True), (LANE, LANE))
                    nt = sa.shape[1] // LANE
                    ptiles, psums = [], []
                    for g in range(0, LANE, 8):
                        mg = _pin(mb[g:g + 8, :], chain)
                        pg = [jnp.exp2(sa[g:g + 8, t * LANE:(t + 1) * LANE] - mg) for t in range(nt)]
                        ps = functools.reduce(jnp.add, pg)
                        chain = _opaque_zero([ps])
                        psums.append(ps)
                        ptiles.append(_lanecat(pg))
                    ls.append(jnp.sum(_rowcat(psums), axis=1, keepdims=True))
                    p = _pin(_rowcat(ptiles), link[0], 0, 0 if a == 0 else sa.shape[1] - LANE)
                    if cfg["p32"]:
                        pb[_h(LANE * a, LANE), 0:sa.shape[1]] = _u32(p.astype(BF16))
                    else:
                        pb[LANE * a:LANE * (a + 1), 0:sa.shape[1]] = p.astype(BF16)
                return ls

            def pv(i, ls):
                r0 = i * tq
                pb = p_s.at[i % 2]
                def p_of(rows0, c0, n):
                    if cfg["p32"]:
                        return _bf(pb[_h(rows0, tq - rows0), c0:c0 + n])
                    return pb[rows0:, c0:c0 + n]

                ctx = [_dot(p_of(0, 0, r0 + LANE), _bf(v_s[_h(0, r0 + LANE), :]))]
                for j in range(1, nsub):
                    ctx.append(_dot(p_of(LANE * j, r0 + LANE * j, LANE),
                                    _bf(v_s[_h(r0 + LANE * j, LANE), :])))
                set_link(ctx[2], cfg["link_part"])
                cs = []
                for a in range(nsub):
                    sl = lambda j: slice(LANE * (a - j), LANE * (a - j + 1))
                    r = pl.reciprocal(ls[a], approx=True)
                    r = r * (2.0 - ls[a] * r)
                    cs.append(functools.reduce(jnp.add, [ctx[j][sl(j)] for j in range(a + 1)]) * r)
                return _rowcat(cs).astype(BF16)

            def oproj(i, ctx):
                for u in range(tq // D):
                    res = _dot_nt(_bf(linked(wo_v[h])), ctx[u * D:(u + 1) * D, :])
                    set_link(res)
                    k = i * (tq // D) + u
                    tot = rb_t[k] + res
                    rb_t[k] = tot
                    if cfg["b_out"] and i < nq - 1:
                        pending.append((k, b_out(k, tot)))

            a_state = {}

            def a_hook(tag):
                if with_a and tag == cfg["a_fwd_at"]:
                    a_state["kv"], xs, hs = a_fwd()
                    a_state["z"] = a_conv(xs, hs)
                if with_a and tag == cfg["a_inv_at"]:
                    a_inv(a_state["kv"], a_state["z"])

            a_hook(0)
            proj(k_s, 0, 0, tq)
            a_hook(1)
            parts = qk(0)
            ctx_prev = None
            for i in range(nq):
                r0 = i * tq
                a_hook(10 * (i + 1))
                if ctx_prev is not None:
                    oproj(i - 1, ctx_prev)
                a_hook(10 * (i + 1) + 1)
                if i + 1 < nq:
                    proj(k_s, 0, r0 + tq, tq)
                a_hook(10 * (i + 1) + 2)
                proj(v_s, 1, r0, tq)
                a_hook(10 * (i + 1) + 3)
                ls = softmax(i, parts)
                ctx_prev = pv(i, ls)
                a_hook(10 * (i + 1) + 4)
                if i + 1 < nq:
                    parts = qk(i + 1, a_out() if i + 1 == cfg["ao_at"] else None)
            oproj(nq - 1, ctx_prev)
            assert not pending
            return carry

        with jax.named_scope("loop_a"):
            lax.fori_loop(cfg["h0"], H, head_step, 0)
        with jax.named_scope("tail"):
            for i in range((nq - 1) * (tq // D) if cfg["b_out"] else 0, NOUT):
                b_out(i, rb_t[i])
                out_copy(i).start()
            for i in range(NOUT + AT):
                out_copy(i).wait()

    scratch = [
        pltpu.VMEM((4, M // 2, S), U32),
        pltpu.VMEM((KS, M), BF16),
        pltpu.VMEM((M,), BF16),
        pltpu.VMEM((KS + 1, M, LANE), F32),
        pltpu.VMEM((LANE // 2, 2 * LANE), U32),
        pltpu.VMEM((M // 2, S), U32),
        pltpu.VMEM((S // 2, MP), U32),
        pltpu.VMEM((S // 2, C), U32),
        pltpu.VMEM((KT, 4 * TP * 8, LANE), U32),
        pltpu.VMEM((H // 2, MP // 2, 2 * D), U32),
        pltpu.VMEM((H // 2, x_cols, 2 * D), F32),
        pltpu.VMEM((WS, 8 * WP * 8, LANE), U32),
        pltpu.VMEM((H, C // 2, 2 * D), U32),
        pltpu.VMEM((H, M // 2, D), U32),
        pltpu.VMEM((H, S // 2, D), U32),
        pltpu.VMEM((S // 2, D), U32),
        pltpu.VMEM((S // 2, D), U32),
        pltpu.VMEM((2, tq // 2, S), U32) if cfg["p32"] else pltpu.VMEM((2, tq, S), BF16),
        pltpu.VMEM((2, M, S // 2), F32),
        pltpu.VMEM((S // D, M, D), F32),
        pltpu.VMEM((AT + 1, S, LANE), BF16),
        pltpu.VMEM((S, 2 * M - AT * LANE), BF16),
        pltpu.SemaphoreType.DMA((XC,)),
        pltpu.SemaphoreType.DMA((KT,)),
        pltpu.SemaphoreType.DMA((WS,)),
        pltpu.SemaphoreType.DMA((1,)),
        pltpu.SemaphoreType.DMA((2,)),
        pltpu.SemaphoreType.DMA((3,)),
        pltpu.SemaphoreType.DMA((S // D + AT,)),
    ]
    return kernel, scratch


_DEFAULT = dict(tq=512, a_fwd_at=13, a_inv_at=44, a_gate=1, a_chains=1, a_width=4, ao_at=1, ao_row=240, b_out=1, bo_pass=3, q_pairs=2, p32=0, wq_first=1,
                link_back=176, pace_row=32, pace_step=24, link_part=32, use_a=1, h0=0)


def _build(**kw):
    cfg = dict(_DEFAULT)
    cfg.update(kw)
    kernel, scratch = _make_kernel(cfg)

    def run(A_q, A_k, A_v, A_shift_k, A_ssm_k, A_ssm_D, B_x, B_c_kv, B_w_q, B_w_uk,
            B_w_uv, B_w_o):
        tr = lambda a: jnp.swapaxes(a, 1, 2).reshape(M, S)
        args = (
            tr(A_q), tr(A_k), tr(A_v), A_shift_k.T, A_ssm_k, A_ssm_D, tr(B_x),
            B_c_kv.reshape(S, C),
            B_w_q.reshape(M // 2, 2 * H, D), B_w_uk.reshape(C // 2, 2 * H, D),
            B_w_uv.reshape(C // 2, 2 * H, D),
            jnp.swapaxes(B_w_o, 1, 2),
        )
        out = pl.pallas_call(
            kernel,
            in_specs=[pl.BlockSpec(memory_space=pl.ANY)] * len(args),
            out_specs=pl.BlockSpec(memory_space=pl.ANY),
            out_shape=jax.ShapeDtypeStruct((S, 2 * M), BF16),
            scratch_shapes=scratch,
            compiler_params=pltpu.CompilerParams(
                vmem_limit_bytes=120 * 1024 * 1024,
                disable_bounds_checks=True),
        )(*args)
        return out.reshape(1, S, 2 * M)

    return run


_run = _build()


@jax.jit
def pallas_concat_heads__ssm_conv_h3__compressed_kv_cla__prompt_kernel(
    A_q: jax.Array,
    A_k: jax.Array,
    A_v: jax.Array,
    A_shift_k: jax.Array,
    A_ssm_k: jax.Array,
    A_ssm_D: jax.Array,
    B_x: jax.Array,
    B_c_kv: jax.Array,
    B_w_q: jax.Array,
    B_w_uk: jax.Array,
    B_w_uv: jax.Array,
    B_w_o: jax.Array,
):
    return _run(A_q, A_k, A_v, A_shift_k, A_ssm_k, A_ssm_D, B_x, B_c_kv, B_w_q,
                B_w_uk, B_w_uv, B_w_o)
```

```python
import functools

import jax
import jax.numpy as jnp
from jax import lax
import jax.experimental.pallas as pl
import jax.experimental.pallas.tpu as pltpu

F32 = jnp.float32
BF16 = jnp.bfloat16
U32 = jnp.uint32

S = 2048
M = 448
MP = 512
C = 1024
H = 16
D = 256
KS = 4
LANE = 128
NB = S // LANE
AR = 32
A_STEPS = M // AR
LOG2E = 1.4426950408889634
NEG = -1e30

NT = (((1,), (1,)), ((), ()))


def _dot(a, b):
    return jnp.dot(a, b, preferred_element_type=F32)


def _dot_nt(a, b):
    return lax.dot_general(a, b, NT, preferred_element_type=F32)


def _bf(x):
    return pltpu.bitcast(x, BF16)


def _u32(x):
    return pltpu.bitcast(x, U32)


def _h(r0, n):
    return pl.ds(r0 // 2, n // 2)


def _repack(ev, od):
    lo = (ev & jnp.uint32(0xFFFF)) | (od << 16)
    hi = (ev >> 16) | (od & jnp.uint32(0xFFFF0000))
    return lo, hi


def _opaque_zero(vals):
    acc = None
    for v in vals:
        b = v if v.dtype == U32 else pltpu.bitcast(v, U32)
        for r in range(0, b.shape[0], 8):
            for c in range(0, b.shape[1], LANE):
                t = b[r:r + 8, c:c + LANE]
                acc = t if acc is None else acc | t
    return jnp.minimum((acc >> 1).astype(jnp.int32), 0)


def _pin(x, zero, r=0, c=0):
    t = pltpu.bitcast(pltpu.bitcast(x[r:r + 8, c:c + LANE], jnp.int32) + zero, x.dtype)
    row = ([x[r:r + 8, :c]] if c > 0 else []) + [t] + (
        [x[r:r + 8, c + LANE:]] if c + LANE < x.shape[1] else [])
    row = jnp.concatenate(row, axis=1) if len(row) > 1 else row[0]
    col = ([x[:r, :]] if r > 0 else []) + [row] + ([x[r + 8:, :]] if r + 8 < x.shape[0] else [])
    return jnp.concatenate(col, axis=0) if len(col) > 1 else col[0]


def _rowcat(xs):
    return jnp.concatenate(xs, axis=0) if len(xs) > 1 else xs[0]


def _lanecat(xs):
    return jnp.concatenate(xs, axis=1) if len(xs) > 1 else xs[0]


def _make_kernel(cfg):
    tq = cfg["tq"]
    nq = S // tq
    nsub = tq // LANE
    KT = MP // LANE
    TP = LANE // 2
    XC = 4
    x_cols = S // XC
    QP = cfg["q_pairs"]
    WP = 64 * QP
    WS = 2
    QIT = H // 2 // QP
    AT = 3

    def kernel(aq_hbm, ak_hbm, av_hbm, sh_hbm, ssm_hbm, dd_hbm, x_hbm, c_hbm,
               wq_hbm, wk_hbm, wv_hbm, wo_hbm,
               out_hbm,
               a_v, sh_v, dd_v, par_v, f_v,
               xt_v, x_v, c_v, wqs_v, wq_v, qacc, ws_v, wkv_v, wo_v,
               q_all, k_s, v_s, p_s, ra_t, rb_t, oa_v, out_v,
               sem_x, sem_wq, sem_w, sem_c, sem_s, sem_a, sem_out):
        x32, c32, wq32, wk32, wv32, wo32 = (
            r.bitcast(U32) for r in (x_hbm, c_hbm, wq_hbm, wk_hbm, wv_hbm, wo_hbm))
        a32 = [r.bitcast(U32) for r in (ak_hbm, av_hbm, ssm_hbm, aq_hbm)]

        def x_copy(i):
            cs = pl.ds(i * x_cols, x_cols)
            return pltpu.make_async_copy(x32.at[:, cs], xt_v.at[:, cs], sem_x.at[i])

        def wq_copies(kt):
            dst = wqs_v.reshape(4 * KT, TP, 8, LANE)
            rs = pl.ds(min(kt * TP, M // 2 - TP), TP)
            return [pltpu.make_async_copy(
                wq32.at[rs, pl.ds(8 * (k // 2), 8), pl.ds((k % 2) * LANE, LANE)],
                dst.at[4 * kt + k], sem_wq.at[kt]) for k in range(4)]

        def wq_wait(kt):
            pltpu.make_async_copy(wqs_v.at[kt], wqs_v.at[kt], sem_wq.at[kt]).wait()

        def w_rows(chunk):
            r0 = chunk * WP
            return pl.ds(r0 if isinstance(r0, int) else pl.multiple_of(r0, WP), WP)

        def w_copies(chunk, slot):
            dst = ws_v.reshape(8 * WS, WP, 8, LANE)
            rs = w_rows(chunk)
            out = []
            for which, src in enumerate((wk32, wv32)):
                for par in range(2):
                    for half in range(2):
                        k = 8 * slot + 4 * which + 2 * par + half
                        out.append(pltpu.make_async_copy(
                            src.at[rs, pl.ds(8 * par, 8), pl.ds(half * LANE, LANE)],
                            dst.at[k], sem_w.at[slot]))
            return out

        def w_wait(slot):
            pltpu.make_async_copy(ws_v.at[slot], ws_v.at[slot], sem_w.at[slot]).wait()

        def piece_start(it):
            n = S // 2 // QIT
            rs = pl.ds(pl.multiple_of(it * n, n), n)
            pltpu.make_async_copy(c32.at[rs], c_v.at[rs], sem_c.at[0]).start()
            hs = pl.ds(it * (H // QIT), H // QIT)
            pltpu.make_async_copy(wo32.at[hs], wo_v.at[hs], sem_a.at[0]).start()

        a_parts = [pl.ds(0, AR // 2), pl.ds(AR // 2, M // 2 - AR // 2)]

        def a_start(part):
            rs = a_parts[part]
            for k in range(4):
                pltpu.make_async_copy(
                    a32[k].at[rs], a_v.at[k, rs], sem_a.at[1 + part]).start()

        def a_wait(part):
            view = a_v.at[:, a_parts[part]]
            pltpu.make_async_copy(view, view, sem_a.at[1 + part]).wait()

        small = [pltpu.make_async_copy(sh_hbm, sh_v, sem_s.at[0]),
                 pltpu.make_async_copy(dd_hbm, dd_v, sem_s.at[1])]

        link = [None]
        pace = [None]

        def set_link(res, row=None, pacer=None):
            if row is None:
                row = res.shape[0] - cfg["link_back"]
            link[0] = _opaque_zero([res[row:row + 8, res.shape[1] - LANE:]])
            pace[0] = res if pacer is None else pacer

        def linked(x):
            return x if link[0] is None else _pin(x, link[0])

        def paced(w):
            res = pace[0]
            if res is None or link[0] is None or not cfg["pace_step"]:
                return w
            rows = []
            zs = [_opaque_zero([res[r:r + 8, res.shape[1] - LANE:]])
                  for r in range(cfg["pace_row"], cfg["pace_row"] + 8 * cfg["pace_step"],
                                 cfg["pace_step"])]
            for r in range(0, w.shape[0], 8):
                z = zs[7 - (r // 8) % 8]
                t = pltpu.bitcast(w[r:r + 8, :], jnp.int32)
                rows.append(pltpu.bitcast(t + _lanecat([z] * (w.shape[1] // LANE)), U32))
            return _rowcat(rows)

        for cp in small:
            cp.start()
        x_copy(0).start()
        for cp in wq_copies(0):
            cp.start()

        bi = lax.broadcasted_iota(jnp.int32, (LANE, LANE), 0)
        mi = lax.broadcasted_iota(jnp.int32, (LANE, LANE), 1)
        ph = ((4 * mi + 1) * bi) & 511
        ang = ph.astype(F32) * (2.0 * 3.141592653589793 / 512.0)
        f_v[:, 0:LANE] = _u32(jnp.cos(ang).astype(BF16))
        f_v[:, LANE:] = _u32((-jnp.sin(ang)).astype(BF16))

        rb_t[...] = jnp.zeros((S // D, M, D), F32)
        ra_t[:, 0:LANE, :] = jnp.zeros((2, LANE, S // 2), F32)
        ra_t[:, AT * LANE:, :] = jnp.zeros((2, M - AT * LANE, S // 2), F32)

        for kt in range(1, KT):
            for cp in wq_copies(kt):
                cp.start()
        with jax.named_scope("small_wait"):
            for cp in small:
                cp.wait()
        sh = sh_v[...].astype(F32)
        for j in range(KS):
            par_v[j] = jnp.broadcast_to(sh[j:j + 1, :], (LANE, M)).T
        dd = dd_v[...].astype(F32).reshape(1, M)
        par_v[KS] = jnp.broadcast_to(dd, (LANE, M)).T

        def x_transpose(i):
            xt = xt_v[:, pl.ds(i * x_cols, x_cols)]
            nfull = (KT - 1) * TP
            xt = _rowcat([xt[:nfull], jnp.zeros((MP // 2 - M // 2, x_cols), U32), xt[nfull:]])
            x_v[_h(i * x_cols, x_cols), :] = _u32(_bf(xt).astype(F32).T.astype(BF16))

        def q_early(kt, first, last):
            r0 = kt * TP
            rows = pl.ds(r0 if isinstance(r0, int) else pl.multiple_of(r0, TP), TP)
            c0 = kt * LANE
            cols = pl.ds(c0 if isinstance(c0, int) else pl.multiple_of(c0, LANE), LANE)
            link[0] = None
            for j in range(H // 2):
                ws = []
                for half in range(2):
                    ev, od = (
                        wqs_v[kt, pl.ds((2 * par + half) * TP * 8 + j, TP, stride=8), :]
                        for par in range(2))
                    ws.append(_repack(ev, od))
                w = _lanecat([ws[0][0], ws[1][0], ws[0][1], ws[1][1]])
                wq_v[j, rows, :] = w
                d = _dot(_bf(linked(x_v[_h(0, x_cols), cols])), _bf(w))
                set_link(d)
                if not first:
                    d = d + qacc[j]
                if last:
                    d = (d * (D ** -0.5 * LOG2E)).astype(BF16)
                    for t in range(2):
                        q_all[2 * j + t, _h(0, x_cols), :] = _u32(d[:, t * D:(t + 1) * D])
                else:
                    qacc[j] = d

        with jax.named_scope("x_wait"):
            x_copy(0).wait()
        x_transpose(0)
        with jax.named_scope("wq_wait"):
            wq_wait(0)
        q_early(0, True, False)
        for i in range(1, XC):
            x_copy(i).start()
        for cp in w_copies(0, 0):
            cp.start()

        def early_body(kt, carry):
            with jax.named_scope("wq_wait"):
                wq_wait(kt)
            q_early(kt, False, False)
            return carry

        lax.fori_loop(1, KT - 1, early_body, 0)
        with jax.named_scope("wq_wait"):
            wq_wait(KT - 1)
            for i in range(1, XC):
                x_copy(i).wait()
        q_early(KT - 1, False, True)
        for i in range(1, XC):
            x_transpose(i)

        def unpack(chunk, slot, sub, which, half, j):
            ev, od = (
                ws_v[slot, pl.ds(((4 * which + 2 * par + half) * WP + sub * TP) * 8 + j, TP,
                                 stride=8), :]
                for par in range(2))
            lo, hi = _repack(ev, od)
            rows = pl.ds(pl.multiple_of(chunk * WP + sub * TP, TP), TP)
            cols = pl.ds(which * D + half * LANE, LANE)
            wkv_v[2 * j, rows, cols] = lo
            wkv_v[2 * j + 1, rows, cols] = hi
            return [lo, hi]

        units = [(s_, w_, h_, j_) for s_ in range(QP) for w_ in range(2) for h_ in range(2)
                 for j_ in range(H // 2)]

        def qproj(it, r0, n, t, zeros=(None, None)):
            outs = []
            for u in range(2):
                lhs = _bf(linked(x_v[_h(r0, n), :]))
                d = _dot(lhs, _bf(wq_v[it, :, pl.ds(t * D + u * LANE, LANE)]))
                set_link(d)
                if zeros[u] is not None:
                    for k, z in enumerate(zeros[u]):
                        d = _pin(d, z, 8 * ((k * (n // 8)) // len(zeros[u])))
                outs.append(d)
            q2 = _lanecat(outs)
            q_all[2 * it + t, _h(r0, n), :] = _u32((q2 * (D ** -0.5 * LOG2E)).astype(BF16))

        def q_body(it, carry):
            slot = it % WS
            with jax.named_scope("w_wait"):
                w_wait(slot)

            @pl.when(it + 1 < QIT)
            def _():
                for cp in w_copies(it + 1, 1 - slot):
                    cp.start()

            piece_start(it)
            link[0] = None
            pieces = [(p, pc, t) for p in range(QP) for pc in range(1, XC) for t in range(2)]
            nd = 2 * len(pieces)
            for k, (p, pc, t) in enumerate(pieces):
                zeros = []
                for u in range(2):
                    d = 2 * k + u
                    mine = units[d * len(units) // nd:(d + 1) * len(units) // nd]
                    zeros.append([_opaque_zero(unpack(it, slot, *u_)) for u_ in mine])
                qproj(QP * it + p, pc * x_cols, x_cols, t, zeros)
            return carry

        a_start(0)
        with jax.named_scope("q_loop"):
            lax.fori_loop(0, QIT, q_body, 0)
        a_start(1)
        pltpu.make_async_copy(c_v, c_v, sem_c.at[0]).wait()
        a_wait(0)
        pltpu.make_async_copy(wo_v, wo_v, sem_a.at[0]).wait()

        tri = (lax.broadcasted_iota(jnp.int32, (LANE, LANE), 1)
               <= lax.broadcasted_iota(jnp.int32, (LANE, LANE), 0))

        NOUT = S // D

        def out_copy(i):
            if i >= NOUT:
                t = i - NOUT
                return pltpu.make_async_copy(
                    oa_v.at[t], out_hbm.at[:, pl.ds(t * LANE, LANE)], sem_out.at[i])
            rs = pl.ds(i * D, D)
            return pltpu.make_async_copy(
                out_v.at[rs], out_hbm.at[rs, pl.ds(AT * LANE, 2 * M - AT * LANE)], sem_out.at[i])

        def b_out(k, tot):
            c0 = (k * D) % (S // 2)
            full = _rowcat([ra_t[k * D // (S // 2), AT * LANE:, c0:c0 + D], tot]).T
            out_v[k * D:(k + 1) * D, :] = full.astype(BF16)
            return full

        def head_step(h, carry):
            with jax.named_scope("step"):
                return head_step_(h, carry)

        def head_step_(h, carry):
            with_a = cfg["use_a"]

            @pl.when(h == A_STEPS)
            def _():
                for t in range(AT):
                    out_copy(NOUT + t).start()

            @pl.when(h == cfg["h0"] + 1)
            def _():
                a_wait(1)

            link[0] = None
            n2 = AR // 2
            a_rows2 = pl.ds(pl.multiple_of(jnp.minimum(h, A_STEPS - 1) * n2, n2), n2)
            a_rows = pl.ds(pl.multiple_of(jnp.minimum(h, A_STEPS - 1) * AR, AR), AR)

            def a_fwd():
                kk = _bf(a_v[0, a_rows2, :]).astype(F32)
                lane = lax.broadcasted_iota(jnp.int32, (AR, LANE), 1)
                coef = [par_v[j, a_rows, :] for j in range(KS)]
                rolled = [kk] + [pltpu.roll(kk, j, 1) for j in range(1, KS)]
                vv = _bf(a_v[1, a_rows2, :]).astype(F32)
                kv_blocks = []
                for a in range(NB):
                    cs = slice(a * LANE, (a + 1) * LANE)
                    acc = rolled[0][:, cs] * coef[0]
                    for j in range(1, KS):
                        t = rolled[j][:, cs]
                        if a == 0:
                            t = jnp.where(lane >= j, t, 0.0)
                        acc = acc + t * coef[j]
                    kv_blocks.append(acc * vv[:, cs])
                hk = a_v[2, a_rows2, :]
                hk = _rowcat([hk[:, a * LANE:(a + 1) * LANE] for a in range(NB)])
                fm = _bf(f_v[...])
                hs = _dot(_bf(linked(hk)), fm)
                kv = linked(_rowcat(kv_blocks)).astype(BF16)
                xs = _dot(kv, fm)
                set_link(xs)
                return kv, xs, hs

            def a_conv(xs, hs):
                def tile(v, a, g, part):
                    r = a * AR + 8 * g
                    return v[r:r + 8, part * LANE:(part + 1) * LANE]

                z = {}
                gate = None
                width = cfg["a_width"]
                for g in range(AR // 8):
                    hr = [tile(hs, 0, g, 0)] + [
                        tile(hs, j, g, 0) - tile(hs, j - 1, g, 1) for j in range(1, NB)]
                    hi = [tile(hs, 0, g, 1)] + [
                        tile(hs, j, g, 1) + tile(hs, j - 1, g, 0) for j in range(1, NB)]
                    for c0 in range(0, NB, width):
                        for a in range(c0 + width):
                            xr, xi = tile(xs, a, g, 0), tile(xs, a, g, 1)
                            if gate is not None:
                                xr, xi = _pin(xr, gate), _pin(xi, gate)
                            for c in range(max(c0, a), c0 + width):
                                j = c - a
                                tr = xr * hr[j] - xi * hi[j]
                                ti = xr * hi[j] + xi * hr[j]
                                z[c, g] = (tr, ti) if a == 0 else (z[c, g][0] + tr, z[c, g][1] + ti)
                            gate = _opaque_zero(list(z[c0 + width - 1, g]))
                return z

            def a_inv(kv, z):
                fm = _bf(f_v[...])
                ng = AR // 8
                ys = []
                for u in range(2):
                    rows = [_lanecat(z[c, g]) for g in range(u * ng // 2, (u + 1) * ng // 2)
                            for c in range(NB)]
                    ys.append(_dot_nt(linked(_rowcat(rows)).astype(BF16), fm))
                y = _rowcat(ys)
                dd = par_v[KS, a_rows, :]
                for c in range(NB):
                    cs = slice(c * LANE, (c + 1) * LANE)
                    yc = _rowcat([y[(g * NB + c) * 8:(g * NB + c + 1) * 8, :] for g in range(ng)])
                    qq = _bf(a_v[3, a_rows2, cs]).astype(F32)
                    kvf = kv[c * AR:(c + 1) * AR, :].astype(F32)
                    c2 = (c % (NB // 2)) * LANE
                    ra_t[c // (NB // 2), a_rows, c2:c2 + LANE] = qq * (yc * (1.0 / LANE) + kvf * dd)

            def a_out():
                slab = jnp.clip(h // 4 - 1, 0, AT - 1)
                half = h % 2
                x = ra_t[half, pl.ds(pl.multiple_of(slab * LANE, LANE), LANE), :]
                xt = x.T
                dst = jnp.where(h >= A_STEPS, AT, slab)
                oa_v[dst, pl.ds(pl.multiple_of(half * (S // 2), S // 2), S // 2), :] = xt.astype(BF16)
                return xt

            kw = C // 2
            pending = []

            def flush_pending(x, row):
                done = list(pending)
                del pending[:]
                if not done:
                    return x
                x = _pin(x, _opaque_zero([f for _, f in done]), row)

                @pl.when(h == H - 1)
                def _():
                    for k, _f in done:
                        out_copy(k).start()
                return x

            def proj_w(which, k):
                return wkv_v[h, _h((k % 2) * kw, kw), pl.ds(which * D + (k // 2) * LANE, LANE)]

            def proj(dst, which, r0, n):
                ds = []
                for k in range(4):
                    lhs = linked(c_v[_h(r0, n), pl.ds((k % 2) * kw, kw)])
                    if which == 1 and k == cfg["bo_pass"]:
                        lhs = flush_pending(lhs, cfg["ao_row"])
                    ds.append(_dot(_bf(lhs), _bf(paced(proj_w(which, k)))))
                    set_link(ds[-1])
                dst[_h(r0, n), :] = _u32(_lanecat([ds[0] + ds[1], ds[2] + ds[3]]).astype(BF16))

            def qk(i, dep=None):
                r0 = i * tq
                q = linked(q_all[h, _h(r0, tq), :])
                if dep is not None:
                    q = _pin(q, _opaque_zero([dep]), cfg["ao_row"])
                parts = [_dot_nt(_bf(q), _bf(k_s[_h(0, r0 + LANE), :]))]
                if i > 0:
                    link[0] = _opaque_zero([parts[0][0:8, r0 - LANE:r0]])
                for j in range(1, nsub):
                    q = linked(q_all[h, _h(r0 + LANE * j, tq - LANE * j), :])
                    parts.append(_dot_nt(_bf(q), _bf(k_s[_h(r0 + LANE * j, LANE), :])))
                set_link(parts[2], cfg["link_part"], parts[0])
                return parts

            def softmax(i, parts):
                pb = p_s.at[i % 2]
                chain = _opaque_zero([b[b.shape[0] - 8:, b.shape[1] - LANE:] for b in parts])
                ls = []
                for a in range(nsub):
                    blocks = [parts[j][LANE * (a - j):LANE * (a - j + 1), :] for j in range(a + 1)]
                    last = blocks[-1]
                    w = last.shape[1]
                    dg = jnp.where(tri, last[:, w - LANE:], NEG)
                    blocks[-1] = dg if w == LANE else _lanecat([last[:, :w - LANE], dg])
                    sa = _lanecat(blocks)
                    mb = jnp.broadcast_to(jnp.max(sa, axis=1, keepdims=True), (LANE, LANE))
                    nt = sa.shape[1] // LANE
                    ptiles, psums = [], []
                    for g in range(0, LANE, 8):
                        mg = _pin(mb[g:g + 8, :], chain)
                        pg = [jnp.exp2(sa[g:g + 8, t * LANE:(t + 1) * LANE] - mg) for t in range(nt)]
                        ps = functools.reduce(jnp.add, pg)
                        chain = _opaque_zero([ps])
                        psums.append(ps)
                        ptiles.append(_lanecat(pg))
                    ls.append(jnp.sum(_rowcat(psums), axis=1, keepdims=True))
                    p = _pin(_rowcat(ptiles), link[0], 0, 0 if a == 0 else sa.shape[1] - LANE)
                    pb[LANE * a:LANE * (a + 1), 0:sa.shape[1]] = p.astype(BF16)
                return ls

            def pv(i, ls):
                r0 = i * tq
                pb = p_s.at[i % 2]
                ctx = [_dot(pb[:, 0:r0 + LANE], _bf(v_s[_h(0, r0 + LANE), :]))]
                for j in range(1, nsub):
                    c0 = r0 + LANE * j
                    ctx.append(_dot(pb[LANE * j:, c0:c0 + LANE], _bf(v_s[_h(c0, LANE), :])))
                set_link(ctx[2], cfg["link_part"])
                cs = []
                for a in range(nsub):
                    sl = lambda j: slice(LANE * (a - j), LANE * (a - j + 1))
                    r = pl.reciprocal(ls[a], approx=True)
                    r = r * (2.0 - ls[a] * r)
                    cs.append(functools.reduce(jnp.add, [ctx[j][sl(j)] for j in range(a + 1)]) * r)
                return _rowcat(cs).astype(BF16)

            def oproj(i, ctx):
                for u in range(tq // D):
                    res = _dot_nt(_bf(linked(wo_v[h])), ctx[u * D:(u + 1) * D, :])
                    set_link(res)
                    k = i * (tq // D) + u
                    tot = rb_t[k] + res
                    rb_t[k] = tot
                    if i < nq - 1:
                        pending.append((k, b_out(k, tot)))

            a_state = {}

            def a_hook(tag):
                if with_a and tag == cfg["a_fwd_at"]:
                    a_state["kv"], xs, hs = a_fwd()
                    a_state["z"] = a_conv(xs, hs)
                if with_a and tag == cfg["a_inv_at"]:
                    a_inv(a_state["kv"], a_state["z"])

            a_hook(0)
            proj(k_s, 0, 0, tq)
            a_hook(1)
            parts = qk(0)
            ctx_prev = None
            for i in range(nq):
                r0 = i * tq
                a_hook(10 * (i + 1))
                if ctx_prev is not None:
                    oproj(i - 1, ctx_prev)
                a_hook(10 * (i + 1) + 1)
                if i + 1 < nq:
                    proj(k_s, 0, r0 + tq, tq)
                a_hook(10 * (i + 1) + 2)
                proj(v_s, 1, r0, tq)
                a_hook(10 * (i + 1) + 3)
                ls = softmax(i, parts)
                ctx_prev = pv(i, ls)
                a_hook(10 * (i + 1) + 4)
                if i + 1 < nq:
                    parts = qk(i + 1, a_out() if i + 1 == cfg["ao_at"] else None)
            oproj(nq - 1, ctx_prev)
            assert not pending
            return carry

        with jax.named_scope("loop_a"):
            lax.fori_loop(cfg["h0"], H, head_step, 0)
        with jax.named_scope("tail"):
            for i in range((nq - 1) * (tq // D), NOUT):
                b_out(i, rb_t[i])
                out_copy(i).start()
            for i in range(NOUT + AT):
                out_copy(i).wait()

    scratch = [
        pltpu.VMEM((4, M // 2, S), U32),
        pltpu.VMEM((KS, M), BF16),
        pltpu.VMEM((M,), BF16),
        pltpu.VMEM((KS + 1, M, LANE), F32),
        pltpu.VMEM((LANE // 2, 2 * LANE), U32),
        pltpu.VMEM((M // 2, S), U32),
        pltpu.VMEM((S // 2, MP), U32),
        pltpu.VMEM((S // 2, C), U32),
        pltpu.VMEM((KT, 4 * TP * 8, LANE), U32),
        pltpu.VMEM((H // 2, MP // 2, 2 * D), U32),
        pltpu.VMEM((H // 2, x_cols, 2 * D), F32),
        pltpu.VMEM((WS, 8 * WP * 8, LANE), U32),
        pltpu.VMEM((H, C // 2, 2 * D), U32),
        pltpu.VMEM((H, M // 2, D), U32),
        pltpu.VMEM((H, S // 2, D), U32),
        pltpu.VMEM((S // 2, D), U32),
        pltpu.VMEM((S // 2, D), U32),
        pltpu.VMEM((2, tq, S), BF16),
        pltpu.VMEM((2, M, S // 2), F32),
        pltpu.VMEM((S // D, M, D), F32),
        pltpu.VMEM((AT + 1, S, LANE), BF16),
        pltpu.VMEM((S, 2 * M - AT * LANE), BF16),
        pltpu.SemaphoreType.DMA((XC,)),
        pltpu.SemaphoreType.DMA((KT,)),
        pltpu.SemaphoreType.DMA((WS,)),
        pltpu.SemaphoreType.DMA((1,)),
        pltpu.SemaphoreType.DMA((2,)),
        pltpu.SemaphoreType.DMA((3,)),
        pltpu.SemaphoreType.DMA((S // D + AT,)),
    ]
    return kernel, scratch


_DEFAULT = dict(tq=512, q_pairs=2, a_fwd_at=13, a_inv_at=44, a_width=4, ao_at=1, ao_row=240,
                bo_pass=2, link_back=176, link_part=32, pace_row=32, pace_step=24,
                use_a=1, h0=0)


def _build(**kw):
    cfg = dict(_DEFAULT)
    cfg.update(kw)
    kernel, scratch = _make_kernel(cfg)

    def run(A_q, A_k, A_v, A_shift_k, A_ssm_k, A_ssm_D, B_x, B_c_kv, B_w_q, B_w_uk,
            B_w_uv, B_w_o):
        tr = lambda a: jnp.swapaxes(a, 1, 2).reshape(M, S)
        args = (
            tr(A_q), tr(A_k), tr(A_v), A_shift_k.T, A_ssm_k, A_ssm_D, tr(B_x),
            B_c_kv.reshape(S, C),
            B_w_q.reshape(M // 2, 2 * H, D), B_w_uk.reshape(C // 2, 2 * H, D),
            B_w_uv.reshape(C // 2, 2 * H, D),
            jnp.swapaxes(B_w_o, 1, 2),
        )
        out = pl.pallas_call(
            kernel,
            in_specs=[pl.BlockSpec(memory_space=pl.ANY)] * len(args),
            out_specs=pl.BlockSpec(memory_space=pl.ANY),
            out_shape=jax.ShapeDtypeStruct((S, 2 * M), BF16),
            scratch_shapes=scratch,
            compiler_params=pltpu.CompilerParams(
                vmem_limit_bytes=120 * 1024 * 1024,
                disable_bounds_checks=True),
        )(*args)
        return out.reshape(1, S, 2 * M)

    return run


_run = _build()


@jax.jit
def pallas_concat_heads__ssm_conv_h3__compressed_kv_cla__prompt_kernel(
    A_q: jax.Array,
    A_k: jax.Array,
    A_v: jax.Array,
    A_shift_k: jax.Array,
    A_ssm_k: jax.Array,
    A_ssm_D: jax.Array,
    B_x: jax.Array,
    B_c_kv: jax.Array,
    B_w_q: jax.Array,
    B_w_uk: jax.Array,
    B_w_uv: jax.Array,
    B_w_o: jax.Array,
):
    return _run(A_q, A_k, A_v, A_shift_k, A_ssm_k, A_ssm_D, B_x, B_c_kv, B_w_q,
                B_w_uk, B_w_uv, B_w_o)
```

```python
import functools

import jax
import jax.numpy as jnp
from jax import lax
import jax.experimental.pallas as pl
import jax.experimental.pallas.tpu as pltpu

F32 = jnp.float32
BF16 = jnp.bfloat16
U32 = jnp.uint32

S = 2048
M = 448
MP = 512
C = 1024
H = 16
D = 256
KS = 4
LANE = 128
NB = S // LANE
AR = 32
A_STEPS = M // AR
LOG2E = 1.4426950408889634
NEG = -1e30

NT = (((1,), (1,)), ((), ()))


def _dot(a, b):
    return jnp.dot(a, b, preferred_element_type=F32)


def _dot_nt(a, b):
    return lax.dot_general(a, b, NT, preferred_element_type=F32)


def _bf(x):
    return pltpu.bitcast(x, BF16)


def _u32(x):
    return pltpu.bitcast(x, U32)


def _h(r0, n):
    return pl.ds(r0 // 2, n // 2)


def _repack(ev, od):
    lo = (ev & jnp.uint32(0xFFFF)) | (od << 16)
    hi = (ev >> 16) | (od & jnp.uint32(0xFFFF0000))
    return lo, hi


def _opaque_zero(vals):
    acc = None
    for v in vals:
        b = v if v.dtype == U32 else pltpu.bitcast(v, U32)
        for r in range(0, b.shape[0], 8):
            for c in range(0, b.shape[1], LANE):
                t = b[r:r + 8, c:c + LANE]
                acc = t if acc is None else acc | t
    return jnp.minimum((acc >> 1).astype(jnp.int32), 0)


def _pin(x, zero, r=0, c=0):
    t = pltpu.bitcast(pltpu.bitcast(x[r:r + 8, c:c + LANE], jnp.int32) + zero, x.dtype)
    row = ([x[r:r + 8, :c]] if c > 0 else []) + [t] + (
        [x[r:r + 8, c + LANE:]] if c + LANE < x.shape[1] else [])
    row = jnp.concatenate(row, axis=1) if len(row) > 1 else row[0]
    col = ([x[:r, :]] if r > 0 else []) + [row] + ([x[r + 8:, :]] if r + 8 < x.shape[0] else [])
    return jnp.concatenate(col, axis=0) if len(col) > 1 else col[0]


def _rowcat(xs):
    return jnp.concatenate(xs, axis=0) if len(xs) > 1 else xs[0]


def _lanecat(xs):
    return jnp.concatenate(xs, axis=1) if len(xs) > 1 else xs[0]


def _make_kernel(cfg):
    tq = cfg["tq"]
    nq = S // tq
    nsub = tq // LANE
    KT = MP // LANE
    TP = LANE // 2
    XC = 4
    x_cols = S // XC
    QP = cfg["q_pairs"]
    WP = 64 * QP
    QIT = H // 2 // QP
    WS = QIT
    AT = 3

    def kernel(aq_hbm, ak_hbm, av_hbm, sh_hbm, ssm_hbm, dd_hbm, x_hbm, c_hbm,
               wq_hbm, wk_hbm, wv_hbm, wo_hbm,
               out_hbm,
               a_v, sh_v, dd_v, par_v, f_v,
               xt_v, x_v, c_v, wqs_v, wq_v, qacc, ws_v, wkv_v, wo_v,
               q_all, k_s, v_s, p_s, ra_t, rb_t, oa_v, out_v,
               sem_x, sem_wq, sem_w, sem_c, sem_s, sem_a, sem_out):
        x32, c32, wq32, wk32, wv32, wo32 = (
            r.bitcast(U32) for r in (x_hbm, c_hbm, wq_hbm, wk_hbm, wv_hbm, wo_hbm))
        a32 = [r.bitcast(U32) for r in (ak_hbm, av_hbm, ssm_hbm, aq_hbm)]

        def x_copy(i):
            cs = pl.ds(i * x_cols, x_cols)
            return pltpu.make_async_copy(x32.at[:, cs], xt_v.at[:, cs], sem_x.at[i])

        def wq_copies(kt):
            dst = wqs_v.reshape(4 * KT, TP, 8, LANE)
            rs = pl.ds(min(kt * TP, M // 2 - TP), TP)
            return [pltpu.make_async_copy(
                wq32.at[rs, pl.ds(8 * (k // 2), 8), pl.ds((k % 2) * LANE, LANE)],
                dst.at[4 * kt + k], sem_wq.at[kt]) for k in range(4)]

        def wq_wait(kt):
            pltpu.make_async_copy(wqs_v.at[kt], wqs_v.at[kt], sem_wq.at[kt]).wait()

        def w_rows(chunk):
            r0 = chunk * WP
            return pl.ds(r0 if isinstance(r0, int) else pl.multiple_of(r0, WP), WP)

        def w_copies(chunk, slot):
            dst = ws_v.reshape(8 * WS, WP, 8, LANE)
            rs = w_rows(chunk)
            out = []
            for which, src in enumerate((wk32, wv32)):
                for par in range(2):
                    for half in range(2):
                        k = 8 * slot + 4 * which + 2 * par + half
                        out.append(pltpu.make_async_copy(
                            src.at[rs, pl.ds(8 * par, 8), pl.ds(half * LANE, LANE)],
                            dst.at[k], sem_w.at[slot]))
            return out

        def w_wait(slot):
            pltpu.make_async_copy(ws_v.at[slot], ws_v.at[slot], sem_w.at[slot]).wait()

        c_copy = pltpu.make_async_copy(c32, c_v, sem_c.at[0])
        wo_copy = pltpu.make_async_copy(wo32, wo_v, sem_a.at[0])

        a_parts = [pl.ds(0, AR // 2), pl.ds(AR // 2, M // 2 - AR // 2)]

        def a_start(part):
            rs = a_parts[part]
            for k in range(4):
                pltpu.make_async_copy(
                    a32[k].at[rs], a_v.at[k, rs], sem_a.at[1 + part]).start()

        def a_wait(part):
            view = a_v.at[:, a_parts[part]]
            pltpu.make_async_copy(view, view, sem_a.at[1 + part]).wait()

        small = [pltpu.make_async_copy(sh_hbm, sh_v, sem_s.at[0]),
                 pltpu.make_async_copy(dd_hbm, dd_v, sem_s.at[1])]

        link = [None]
        pace = [None]

        def set_link(res, row=None, pacer=None):
            if row is None:
                row = res.shape[0] - cfg["link_back"]
            link[0] = _opaque_zero([res[row:row + 8, res.shape[1] - LANE:]])
            pace[0] = res if pacer is None else pacer

        def linked(x):
            return x if link[0] is None else _pin(x, link[0])

        def paced(w):
            res = pace[0]
            if res is None or link[0] is None or not cfg["pace_step"]:
                return w
            rows = []
            zs = [_opaque_zero([res[r:r + 8, res.shape[1] - LANE:]])
                  for r in range(cfg["pace_row"], cfg["pace_row"] + 8 * cfg["pace_step"],
                                 cfg["pace_step"])]
            for r in range(0, w.shape[0], 8):
                z = zs[7 - (r // 8) % 8]
                t = pltpu.bitcast(w[r:r + 8, :], jnp.int32)
                rows.append(pltpu.bitcast(t + _lanecat([z] * (w.shape[1] // LANE)), U32))
            return _rowcat(rows)

        for cp in small:
            cp.start()
        x_copy(0).start()
        for cp in wq_copies(0):
            cp.start()

        bi = lax.broadcasted_iota(jnp.int32, (LANE, LANE), 0)
        mi = lax.broadcasted_iota(jnp.int32, (LANE, LANE), 1)
        ph = ((4 * mi + 1) * bi) & 511
        ang = ph.astype(F32) * (2.0 * 3.141592653589793 / 512.0)
        f_v[:, 0:LANE] = _u32(jnp.cos(ang).astype(BF16))
        f_v[:, LANE:] = _u32((-jnp.sin(ang)).astype(BF16))

        rb_t[...] = jnp.zeros((S // D, M, D), F32)
        ra_t[:, 0:LANE, :] = jnp.zeros((2, LANE, S // 2), F32)
        ra_t[:, AT * LANE:, :] = jnp.zeros((2, M - AT * LANE, S // 2), F32)

        for kt in range(1, KT):
            for cp in wq_copies(kt):
                cp.start()
        with jax.named_scope("small_wait"):
            for cp in small:
                cp.wait()
        sh = sh_v[...].astype(F32)
        for j in range(KS):
            par_v[j] = jnp.broadcast_to(sh[j:j + 1, :], (LANE, M)).T
        dd = dd_v[...].astype(F32).reshape(1, M)
        par_v[KS] = jnp.broadcast_to(dd, (LANE, M)).T

        def x_transpose(i):
            xt = xt_v[:, pl.ds(i * x_cols, x_cols)]
            nfull = (KT - 1) * TP
            xt = _rowcat([xt[:nfull], jnp.zeros((MP // 2 - M // 2, x_cols), U32), xt[nfull:]])
            x_v[_h(i * x_cols, x_cols), :] = _u32(_bf(xt).astype(F32).T.astype(BF16))

        def q_early(kt, first, last):
            r0 = kt * TP
            rows = pl.ds(r0 if isinstance(r0, int) else pl.multiple_of(r0, TP), TP)
            c0 = kt * LANE
            cols = pl.ds(c0 if isinstance(c0, int) else pl.multiple_of(c0, LANE), LANE)
            link[0] = None
            for j in range(H // 2):
                ws = []
                for half in range(2):
                    ev, od = (
                        wqs_v[kt, pl.ds((2 * par + half) * TP * 8 + j, TP, stride=8), :]
                        for par in range(2))
                    ws.append(_repack(ev, od))
                w = _lanecat([ws[0][0], ws[1][0], ws[0][1], ws[1][1]])
                wq_v[j, rows, :] = w
                d = _dot(_bf(linked(x_v[_h(0, x_cols), cols])), _bf(w))
                set_link(d)
                if not first:
                    d = d + qacc[j]
                if last:
                    d = (d * (D ** -0.5 * LOG2E)).astype(BF16)
                    for t in range(2):
                        q_all[2 * j + t, _h(0, x_cols), :] = _u32(d[:, t * D:(t + 1) * D])
                else:
                    qacc[j] = d

        with jax.named_scope("x_wait"):
            x_copy(0).wait()
        x_transpose(0)
        for i in range(1, XC):
            x_copy(i).start()
        for chunk in range(QIT):
            for cp in w_copies(chunk, chunk):
                cp.start()
        c_copy.start()
        wo_copy.start()
        a_start(0)
        a_start(1)
        with jax.named_scope("wq_wait"):
            wq_wait(0)
        q_early(0, True, False)

        def early_body(kt, carry):
            with jax.named_scope("wq_wait"):
                wq_wait(kt)
            q_early(kt, False, False)
            return carry

        lax.fori_loop(1, KT - 1, early_body, 0)
        with jax.named_scope("wq_wait"):
            wq_wait(KT - 1)
            for i in range(1, XC):
                x_copy(i).wait()
        q_early(KT - 1, False, True)
        for i in range(1, XC):
            x_transpose(i)

        def unpack(chunk, slot, sub, which, half, j):
            ev, od = (
                ws_v[slot, pl.ds(((4 * which + 2 * par + half) * WP + sub * TP) * 8 + j, TP,
                                 stride=8), :]
                for par in range(2))
            lo, hi = _repack(ev, od)
            rows = pl.ds(pl.multiple_of(chunk * WP + sub * TP, TP), TP)
            cols = pl.ds(which * D + half * LANE, LANE)
            wkv_v[2 * j, rows, cols] = lo
            wkv_v[2 * j + 1, rows, cols] = hi
            return [lo, hi]

        units = [(s_, w_, h_, j_) for s_ in range(QP) for w_ in range(2) for h_ in range(2)
                 for j_ in range(H // 2)]

        def qproj(it, r0, n, t, zeros=(None, None)):
            outs = []
            for u in range(2):
                lhs = _bf(linked(x_v[_h(r0, n), :]))
                d = _dot(lhs, _bf(wq_v[it, :, pl.ds(t * D + u * LANE, LANE)]))
                set_link(d)
                if zeros[u] is not None:
                    for k, z in enumerate(zeros[u]):
                        d = _pin(d, z, 8 * ((k * (n // 8)) // len(zeros[u])))
                outs.append(d)
            q2 = _lanecat(outs)
            q_all[2 * it + t, _h(r0, n), :] = _u32((q2 * (D ** -0.5 * LOG2E)).astype(BF16))

        def q_body(it, carry):
            slot = it
            with jax.named_scope("w_wait"):
                w_wait(slot)
            link[0] = None
            pieces = [(p, pc, t) for p in range(QP) for pc in range(1, XC) for t in range(2)]
            nd = 2 * len(pieces)
            for k, (p, pc, t) in enumerate(pieces):
                zeros = []
                for u in range(2):
                    d = 2 * k + u
                    mine = units[d * len(units) // nd:(d + 1) * len(units) // nd]
                    zeros.append([_opaque_zero(unpack(it, slot, *u_)) for u_ in mine])
                qproj(QP * it + p, pc * x_cols, x_cols, t, zeros)
            return carry

        with jax.named_scope("q_loop"):
            lax.fori_loop(0, QIT, q_body, 0)
        c_copy.wait()
        wo_copy.wait()
        a_wait(0)

        tri = (lax.broadcasted_iota(jnp.int32, (LANE, LANE), 1)
               <= lax.broadcasted_iota(jnp.int32, (LANE, LANE), 0))

        NOUT = S // D

        def out_copy(i):
            if i >= NOUT:
                t = i - NOUT
                return pltpu.make_async_copy(
                    oa_v.at[t], out_hbm.at[:, pl.ds(t * LANE, LANE)], sem_out.at[i])
            rs = pl.ds(i * D, D)
            return pltpu.make_async_copy(
                out_v.at[rs], out_hbm.at[rs, pl.ds(AT * LANE, 2 * M - AT * LANE)], sem_out.at[i])

        def b_out(k, tot):
            c0 = (k * D) % (S // 2)
            full = _rowcat([ra_t[k * D // (S // 2), AT * LANE:, c0:c0 + D], tot]).T
            out_v[k * D:(k + 1) * D, :] = full.astype(BF16)
            return full

        def head_step(h, carry):
            with jax.named_scope("step"):
                return head_step_(h, carry)

        def head_step_(h, carry):
            with_a = cfg["use_a"]

            @pl.when(h == A_STEPS)
            def _():
                for t in range(AT):
                    out_copy(NOUT + t).start()

            @pl.when(h == cfg["h0"] + 1)
            def _():
                a_wait(1)

            link[0] = None
            n2 = AR // 2
            a_rows2 = pl.ds(pl.multiple_of(jnp.minimum(h, A_STEPS - 1) * n2, n2), n2)
            a_rows = pl.ds(pl.multiple_of(jnp.minimum(h, A_STEPS - 1) * AR, AR), AR)

            def a_fwd():
                kk = _bf(a_v[0, a_rows2, :]).astype(F32)
                lane = lax.broadcasted_iota(jnp.int32, (AR, LANE), 1)
                coef = [par_v[j, a_rows, :] for j in range(KS)]
                rolled = [kk] + [pltpu.roll(kk, j, 1) for j in range(1, KS)]
                vv = _bf(a_v[1, a_rows2, :]).astype(F32)
                kv_blocks = []
                for a in range(NB):
                    cs = slice(a * LANE, (a + 1) * LANE)
                    acc = rolled[0][:, cs] * coef[0]
                    for j in range(1, KS):
                        t = rolled[j][:, cs]
                        if a == 0:
                            t = jnp.where(lane >= j, t, 0.0)
                        acc = acc + t * coef[j]
                    kv_blocks.append(acc * vv[:, cs])
                hk = a_v[2, a_rows2, :]
                hk = _rowcat([hk[:, a * LANE:(a + 1) * LANE] for a in range(NB)])
                fm = _bf(f_v[...])
                hs = _dot(_bf(linked(hk)), fm)
                kv = linked(_rowcat(kv_blocks)).astype(BF16)
                xs = _dot(kv, fm)
                set_link(xs)
                return kv, xs, hs

            def a_conv(xs, hs):
                def tile(v, a, g, part):
                    r = a * AR + 8 * g
                    return v[r:r + 8, part * LANE:(part + 1) * LANE]

                z = {}
                gate = None
                width = cfg["a_width"]
                for g in range(AR // 8):
                    hr = [tile(hs, 0, g, 0)] + [
                        tile(hs, j, g, 0) - tile(hs, j - 1, g, 1) for j in range(1, NB)]
                    hi = [tile(hs, 0, g, 1)] + [
                        tile(hs, j, g, 1) + tile(hs, j - 1, g, 0) for j in range(1, NB)]
                    for c0 in range(0, NB, width):
                        for a in range(c0 + width):
                            xr, xi = tile(xs, a, g, 0), tile(xs, a, g, 1)
                            if gate is not None:
                                xr, xi = _pin(xr, gate), _pin(xi, gate)
                            for c in range(max(c0, a), c0 + width):
                                j = c - a
                                tr = xr * hr[j] - xi * hi[j]
                                ti = xr * hi[j] + xi * hr[j]
                                z[c, g] = (tr, ti) if a == 0 else (z[c, g][0] + tr, z[c, g][1] + ti)
                            gate = _opaque_zero(list(z[c0 + width - 1, g]))
                return z

            def a_inv(kv, z):
                fm = _bf(f_v[...])
                ng = AR // 8
                ys = []
                for u in range(2):
                    rows = [_lanecat(z[c, g]) for g in range(u * ng // 2, (u + 1) * ng // 2)
                            for c in range(NB)]
                    ys.append(_dot_nt(linked(_rowcat(rows)).astype(BF16), fm))
                y = _rowcat(ys)
                dd = par_v[KS, a_rows, :]
                for c in range(NB):
                    cs = slice(c * LANE, (c + 1) * LANE)
                    yc = _rowcat([y[(g * NB + c) * 8:(g * NB + c + 1) * 8, :] for g in range(ng)])
                    qq = _bf(a_v[3, a_rows2, cs]).astype(F32)
                    kvf = kv[c * AR:(c + 1) * AR, :].astype(F32)
                    c2 = (c % (NB // 2)) * LANE
                    ra_t[c // (NB // 2), a_rows, c2:c2 + LANE] = qq * (yc * (1.0 / LANE) + kvf * dd)

            def a_out():
                slab = jnp.clip(h // 4 - 1, 0, AT - 1)
                half = h % 2
                x = ra_t[half, pl.ds(pl.multiple_of(slab * LANE, LANE), LANE), :]
                xt = x.T
                dst = jnp.where(h >= A_STEPS, AT, slab)
                oa_v[dst, pl.ds(pl.multiple_of(half * (S // 2), S // 2), S // 2), :] = xt.astype(BF16)
                return xt

            kw = C // 2
            pending = []

            def flush_pending(x, row):
                done = list(pending)
                del pending[:]
                if not done:
                    return x
                x = _pin(x, _opaque_zero([f for _, f in done]), row)

                @pl.when(h == H - 1)
                def _():
                    for k, _f in done:
                        out_copy(k).start()
                return x

            def proj_w(which, k):
                return wkv_v[h, _h((k % 2) * kw, kw), pl.ds(which * D + (k // 2) * LANE, LANE)]

            def proj(dst, which, r0, n):
                ds = []
                for k in range(4):
                    lhs = linked(c_v[_h(r0, n), pl.ds((k % 2) * kw, kw)])
                    if which == 1 and k == cfg["bo_pass"]:
                        lhs = flush_pending(lhs, cfg["ao_row"])
                    ds.append(_dot(_bf(lhs), _bf(paced(proj_w(which, k)))))
                    set_link(ds[-1])
                dst[_h(r0, n), :] = _u32(_lanecat([ds[0] + ds[1], ds[2] + ds[3]]).astype(BF16))

            def qk(i, dep=None):
                r0 = i * tq
                q = linked(q_all[h, _h(r0, tq), :])
                if dep is not None:
                    q = _pin(q, _opaque_zero([dep]), cfg["ao_row"])
                parts = [_dot_nt(_bf(q), _bf(k_s[_h(0, r0 + LANE), :]))]
                if i > 0:
                    link[0] = _opaque_zero([parts[0][0:8, r0 - LANE:r0]])
                for j in range(1, nsub):
                    q = linked(q_all[h, _h(r0 + LANE * j, tq - LANE * j), :])
                    parts.append(_dot_nt(_bf(q), _bf(k_s[_h(r0 + LANE * j, LANE), :])))
                set_link(parts[2], cfg["link_part"], parts[0])
                return parts

            def softmax(i, parts):
                pb = p_s.at[i % 2]
                chain = _opaque_zero([b[b.shape[0] - 8:, b.shape[1] - LANE:] for b in parts])
                ls = []
                for a in range(nsub):
                    blocks = [parts[j][LANE * (a - j):LANE * (a - j + 1), :] for j in range(a + 1)]
                    last = blocks[-1]
                    w = last.shape[1]
                    dg = jnp.where(tri, last[:, w - LANE:], NEG)
                    blocks[-1] = dg if w == LANE else _lanecat([last[:, :w - LANE], dg])
                    sa = _lanecat(blocks)
                    mb = jnp.broadcast_to(jnp.max(sa, axis=1, keepdims=True), (LANE, LANE))
                    nt = sa.shape[1] // LANE
                    ptiles, psums = [], []
                    for g in range(0, LANE, 8):
                        mg = _pin(mb[g:g + 8, :], chain)
                        pg = [jnp.exp2(sa[g:g + 8, t * LANE:(t + 1) * LANE] - mg) for t in range(nt)]
                        ps = functools.reduce(jnp.add, pg)
                        chain = _opaque_zero([ps])
                        psums.append(ps)
                        ptiles.append(_lanecat(pg))
                    ls.append(jnp.sum(_rowcat(psums), axis=1, keepdims=True))
                    p = _pin(_rowcat(ptiles), link[0], 0, 0 if a == 0 else sa.shape[1] - LANE)
                    pb[LANE * a:LANE * (a + 1), 0:sa.shape[1]] = p.astype(BF16)
                return ls

            def pv(i, ls):
                r0 = i * tq
                pb = p_s.at[i % 2]
                ctx = [_dot(pb[:, 0:r0 + LANE], _bf(v_s[_h(0, r0 + LANE), :]))]
                for j in range(1, nsub):
                    c0 = r0 + LANE * j
                    ctx.append(_dot(pb[LANE * j:, c0:c0 + LANE], _bf(v_s[_h(c0, LANE), :])))
                set_link(ctx[2], cfg["link_part"])
                cs = []
                for a in range(nsub):
                    sl = lambda j: slice(LANE * (a - j), LANE * (a - j + 1))
                    r = pl.reciprocal(ls[a], approx=True)
                    r = r * (2.0 - ls[a] * r)
                    cs.append(functools.reduce(jnp.add, [ctx[j][sl(j)] for j in range(a + 1)]) * r)
                return _rowcat(cs).astype(BF16)

            def oproj(i, ctx):
                for u in range(tq // D):
                    res = _dot_nt(_bf(linked(wo_v[h])), ctx[u * D:(u + 1) * D, :])
                    set_link(res)
                    k = i * (tq // D) + u
                    tot = rb_t[k] + res
                    rb_t[k] = tot
                    if i < nq - 1:
                        pending.append((k, b_out(k, tot)))

            a_state = {}

            def a_hook(tag):
                if with_a and tag == cfg["a_fwd_at"]:
                    a_state["kv"], xs, hs = a_fwd()
                    a_state["z"] = a_conv(xs, hs)
                if with_a and tag == cfg["a_inv_at"]:
                    a_inv(a_state["kv"], a_state["z"])

            a_hook(0)
            proj(k_s, 0, 0, tq)
            a_hook(1)
            parts = qk(0)
            ctx_prev = None
            for i in range(nq):
                r0 = i * tq
                a_hook(10 * (i + 1))
                if ctx_prev is not None:
                    oproj(i - 1, ctx_prev)
                a_hook(10 * (i + 1) + 1)
                if i + 1 < nq:
                    proj(k_s, 0, r0 + tq, tq)
                a_hook(10 * (i + 1) + 2)
                proj(v_s, 1, r0, tq)
                a_hook(10 * (i + 1) + 3)
                ls = softmax(i, parts)
                ctx_prev = pv(i, ls)
                a_hook(10 * (i + 1) + 4)
                if i + 1 < nq:
                    parts = qk(i + 1, a_out() if i + 1 == cfg["ao_at"] else None)
            oproj(nq - 1, ctx_prev)
            assert not pending
            return carry

        with jax.named_scope("loop_a"):
            lax.fori_loop(cfg["h0"], H, head_step, 0)
        with jax.named_scope("tail"):
            for i in range((nq - 1) * (tq // D), NOUT):
                b_out(i, rb_t[i])
                out_copy(i).start()
            for i in range(NOUT + AT):
                out_copy(i).wait()

    scratch = [
        pltpu.VMEM((4, M // 2, S), U32),
        pltpu.VMEM((KS, M), BF16),
        pltpu.VMEM((M,), BF16),
        pltpu.VMEM((KS + 1, M, LANE), F32),
        pltpu.VMEM((LANE // 2, 2 * LANE), U32),
        pltpu.VMEM((M // 2, S), U32),
        pltpu.VMEM((S // 2, MP), U32),
        pltpu.VMEM((S // 2, C), U32),
        pltpu.VMEM((KT, 4 * TP * 8, LANE), U32),
        pltpu.VMEM((H // 2, MP // 2, 2 * D), U32),
        pltpu.VMEM((H // 2, x_cols, 2 * D), F32),
        pltpu.VMEM((WS, 8 * WP * 8, LANE), U32),
        pltpu.VMEM((H, C // 2, 2 * D), U32),
        pltpu.VMEM((H, M // 2, D), U32),
        pltpu.VMEM((H, S // 2, D), U32),
        pltpu.VMEM((S // 2, D), U32),
        pltpu.VMEM((S // 2, D), U32),
        pltpu.VMEM((2, tq, S), BF16),
        pltpu.VMEM((2, M, S // 2), F32),
        pltpu.VMEM((S // D, M, D), F32),
        pltpu.VMEM((AT + 1, S, LANE), BF16),
        pltpu.VMEM((S, 2 * M - AT * LANE), BF16),
        pltpu.SemaphoreType.DMA((XC,)),
        pltpu.SemaphoreType.DMA((KT,)),
        pltpu.SemaphoreType.DMA((WS,)),
        pltpu.SemaphoreType.DMA((1,)),
        pltpu.SemaphoreType.DMA((2,)),
        pltpu.SemaphoreType.DMA((3,)),
        pltpu.SemaphoreType.DMA((S // D + AT,)),
    ]
    return kernel, scratch


_DEFAULT = dict(tq=512, q_pairs=2, a_fwd_at=13, a_inv_at=44, a_width=4, ao_at=1, ao_row=240,
                bo_pass=2, link_back=176, link_part=32, pace_row=32, pace_step=24,
                use_a=1, h0=0)


def _build(**kw):
    cfg = dict(_DEFAULT)
    cfg.update(kw)
    kernel, scratch = _make_kernel(cfg)

    def run(A_q, A_k, A_v, A_shift_k, A_ssm_k, A_ssm_D, B_x, B_c_kv, B_w_q, B_w_uk,
            B_w_uv, B_w_o):
        tr = lambda a: jnp.swapaxes(a, 1, 2).reshape(M, S)
        args = (
            tr(A_q), tr(A_k), tr(A_v), A_shift_k.T, A_ssm_k, A_ssm_D, tr(B_x),
            B_c_kv.reshape(S, C),
            B_w_q.reshape(M // 2, 2 * H, D), B_w_uk.reshape(C // 2, 2 * H, D),
            B_w_uv.reshape(C // 2, 2 * H, D),
            jnp.swapaxes(B_w_o, 1, 2),
        )
        out = pl.pallas_call(
            kernel,
            in_specs=[pl.BlockSpec(memory_space=pl.ANY)] * len(args),
            out_specs=pl.BlockSpec(memory_space=pl.ANY),
            out_shape=jax.ShapeDtypeStruct((S, 2 * M), BF16),
            scratch_shapes=scratch,
            compiler_params=pltpu.CompilerParams(
                vmem_limit_bytes=120 * 1024 * 1024,
                disable_bounds_checks=True),
        )(*args)
        return out.reshape(1, S, 2 * M)

    return run


_run = _build()


@jax.jit
def pallas_concat_heads__ssm_conv_h3__compressed_kv_cla__prompt_kernel(
    A_q: jax.Array,
    A_k: jax.Array,
    A_v: jax.Array,
    A_shift_k: jax.Array,
    A_ssm_k: jax.Array,
    A_ssm_D: jax.Array,
    B_x: jax.Array,
    B_c_kv: jax.Array,
    B_w_q: jax.Array,
    B_w_uk: jax.Array,
    B_w_uv: jax.Array,
    B_w_o: jax.Array,
):
    return _run(A_q, A_k, A_v, A_shift_k, A_ssm_k, A_ssm_D, B_x, B_c_kv, B_w_q,
                B_w_uk, B_w_uv, B_w_o)
```

```python
import functools

import jax
import jax.numpy as jnp
from jax import lax
import jax.experimental.pallas as pl
import jax.experimental.pallas.tpu as pltpu

F32 = jnp.float32
BF16 = jnp.bfloat16
U32 = jnp.uint32

S = 2048
M = 448
MP = 512
C = 1024
H = 16
D = 256
KS = 4
LANE = 128
NB = S // LANE
AR = 32
A_STEPS = M // AR
LOG2E = 1.4426950408889634
NEG = -1e30

NT = (((1,), (1,)), ((), ()))


def _dot(a, b):
    return jnp.dot(a, b, preferred_element_type=F32)


def _dot_nt(a, b):
    return lax.dot_general(a, b, NT, preferred_element_type=F32)


def _bf(x):
    return pltpu.bitcast(x, BF16)


def _u32(x):
    return pltpu.bitcast(x, U32)


def _h(r0, n):
    return pl.ds(r0 // 2, n // 2)


def _repack(ev, od):
    lo = (ev & jnp.uint32(0xFFFF)) | (od << 16)
    hi = (ev >> 16) | (od & jnp.uint32(0xFFFF0000))
    return lo, hi


def _opaque_zero(vals):
    acc = None
    for v in vals:
        b = v if v.dtype == U32 else pltpu.bitcast(v, U32)
        for r in range(0, b.shape[0], 8):
            for c in range(0, b.shape[1], LANE):
                t = b[r:r + 8, c:c + LANE]
                acc = t if acc is None else acc | t
    return jnp.minimum((acc >> 1).astype(jnp.int32), 0)


def _pin(x, zero, r=0, c=0):
    t = pltpu.bitcast(pltpu.bitcast(x[r:r + 8, c:c + LANE], jnp.int32) + zero, x.dtype)
    row = ([x[r:r + 8, :c]] if c > 0 else []) + [t] + (
        [x[r:r + 8, c + LANE:]] if c + LANE < x.shape[1] else [])
    row = jnp.concatenate(row, axis=1) if len(row) > 1 else row[0]
    col = ([x[:r, :]] if r > 0 else []) + [row] + ([x[r + 8:, :]] if r + 8 < x.shape[0] else [])
    return jnp.concatenate(col, axis=0) if len(col) > 1 else col[0]


def _rowcat(xs):
    return jnp.concatenate(xs, axis=0) if len(xs) > 1 else xs[0]


def _lanecat(xs):
    return jnp.concatenate(xs, axis=1) if len(xs) > 1 else xs[0]


def _make_kernel(cfg):
    tq = cfg["tq"]
    nq = S // tq
    nsub = tq // LANE
    KT = MP // LANE
    TP = LANE // 2
    XC = 4
    x_cols = S // XC
    QP = 2
    QIT = H // 2 // QP
    AT = 3

    def kernel(aq_hbm, ak_hbm, av_hbm, sh_hbm, ssm_hbm, dd_hbm, x_hbm, c_hbm,
               wq_hbm, wk_hbm, wv_hbm, wo_hbm,
               out_hbm,
               a_v, sh_v, dd_v, par_v, f_v,
               xt_v, x_v, c_v, wqs_v, wq_v, qacc, ws_v, wkv_v, wo_v,
               q_all, k_s, v_s, p_s, ra_t, rb_t, oa_v, out_v,
               sem_x, sem_wq, sem_w, sem_c, sem_s, sem_a, sem_out):
        x32, c32, wq32, wk32, wv32, wo32 = (
            r.bitcast(U32) for r in (x_hbm, c_hbm, wq_hbm, wk_hbm, wv_hbm, wo_hbm))
        a32 = [r.bitcast(U32) for r in (ak_hbm, av_hbm, ssm_hbm, aq_hbm)]

        def x_copy(i):
            cs = pl.ds(i * x_cols, x_cols)
            return pltpu.make_async_copy(x32.at[:, cs], xt_v.at[:, cs], sem_x.at[i])

        def wq_copies(kt):
            dst = wqs_v.reshape(4 * KT, TP, 8, LANE)
            rs = pl.ds(min(kt * TP, M // 2 - TP), TP)
            return [pltpu.make_async_copy(
                wq32.at[rs, pl.ds(8 * (k // 2), 8), pl.ds((k % 2) * LANE, LANE)],
                dst.at[4 * kt + k], sem_wq.at[kt]) for k in range(4)]

        def wq_wait(kt):
            pltpu.make_async_copy(wqs_v.at[kt], wqs_v.at[kt], sem_wq.at[kt]).wait()

        def w_copies(g):
            dst = ws_v.reshape(8, C // 2, 8, LANE)
            src = (wk32, wv32)[g // 2]
            return [pltpu.make_async_copy(
                src.at[:, pl.ds(8 * par, 8), pl.ds((g % 2) * LANE, LANE)],
                dst.at[2 * g + par], sem_w.at[g]) for par in range(2)]

        def w_wait(g):
            pltpu.make_async_copy(ws_v.at[g], ws_v.at[g], sem_w.at[g]).wait()

        c_copy = pltpu.make_async_copy(c32, c_v, sem_c.at[0])
        wo_copy = pltpu.make_async_copy(wo32, wo_v, sem_a.at[0])

        a_parts = [pl.ds(0, AR // 2), pl.ds(AR // 2, M // 2 - AR // 2)]

        def a_start(part):
            rs = a_parts[part]
            for k in range(4):
                pltpu.make_async_copy(
                    a32[k].at[rs], a_v.at[k, rs], sem_a.at[1 + part]).start()

        def a_wait(part):
            view = a_v.at[:, a_parts[part]]
            pltpu.make_async_copy(view, view, sem_a.at[1 + part]).wait()

        small = [pltpu.make_async_copy(sh_hbm, sh_v, sem_s.at[0]),
                 pltpu.make_async_copy(dd_hbm, dd_v, sem_s.at[1])]

        link = [None]
        pace = [None]

        def set_link(res, row=None, pacer=None):
            if row is None:
                row = res.shape[0] - cfg["link_back"]
            link[0] = _opaque_zero([res[row:row + 8, res.shape[1] - LANE:]])
            pace[0] = res if pacer is None else pacer

        def linked(x):
            return x if link[0] is None else _pin(x, link[0])

        def paced(w):
            res = pace[0]
            if res is None or link[0] is None or not cfg["pace_step"]:
                return w
            rows = []
            zs = [_opaque_zero([res[r:r + 8, res.shape[1] - LANE:]])
                  for r in range(cfg["pace_row"], cfg["pace_row"] + 8 * cfg["pace_step"],
                                 cfg["pace_step"])]
            for r in range(0, w.shape[0], 8):
                z = zs[7 - (r // 8) % 8]
                t = pltpu.bitcast(w[r:r + 8, :], jnp.int32)
                rows.append(pltpu.bitcast(t + _lanecat([z] * (w.shape[1] // LANE)), U32))
            return _rowcat(rows)

        for cp in small:
            cp.start()
        x_copy(0).start()
        for cp in wq_copies(0):
            cp.start()

        bi = lax.broadcasted_iota(jnp.int32, (LANE, LANE), 0)
        mi = lax.broadcasted_iota(jnp.int32, (LANE, LANE), 1)
        ph = ((4 * mi + 1) * bi) & 511
        ang = ph.astype(F32) * (2.0 * 3.141592653589793 / 512.0)
        f_v[:, 0:LANE] = _u32(jnp.cos(ang).astype(BF16))
        f_v[:, LANE:] = _u32((-jnp.sin(ang)).astype(BF16))

        rb_t[...] = jnp.zeros((S // D, M, D), F32)
        ra_t[:, 0:LANE, :] = jnp.zeros((2, LANE, S // 2), F32)
        ra_t[:, AT * LANE:, :] = jnp.zeros((2, M - AT * LANE, S // 2), F32)

        for kt in range(1, KT):
            for cp in wq_copies(kt):
                cp.start()
        with jax.named_scope("small_wait"):
            for cp in small:
                cp.wait()
        sh = sh_v[...].astype(F32)
        for j in range(KS):
            par_v[j] = jnp.broadcast_to(sh[j:j + 1, :], (LANE, M)).T
        dd = dd_v[...].astype(F32).reshape(1, M)
        par_v[KS] = jnp.broadcast_to(dd, (LANE, M)).T

        def x_transpose(i):
            xt = xt_v[:, pl.ds(i * x_cols, x_cols)]
            nfull = (KT - 1) * TP
            xt = _rowcat([xt[:nfull], jnp.zeros((MP // 2 - M // 2, x_cols), U32), xt[nfull:]])
            x_v[_h(i * x_cols, x_cols), :] = _u32(_bf(xt).astype(F32).T.astype(BF16))

        def q_early(kt, first, last):
            r0 = kt * TP
            rows = pl.ds(r0 if isinstance(r0, int) else pl.multiple_of(r0, TP), TP)
            c0 = kt * LANE
            cols = pl.ds(c0 if isinstance(c0, int) else pl.multiple_of(c0, LANE), LANE)
            link[0] = None
            for j in range(H // 2):
                ws = []
                for half in range(2):
                    ev, od = (
                        wqs_v[kt, pl.ds((2 * par + half) * TP * 8 + j, TP, stride=8), :]
                        for par in range(2))
                    ws.append(_repack(ev, od))
                w = _lanecat([ws[0][0], ws[1][0], ws[0][1], ws[1][1]])
                wq_v[j, rows, :] = w
                d = _dot(_bf(linked(x_v[_h(0, x_cols), cols])), _bf(w))
                set_link(d)
                if not first:
                    d = d + qacc[j]
                if last:
                    d = (d * (D ** -0.5 * LOG2E)).astype(BF16)
                    for t in range(2):
                        q_all[2 * j + t, _h(0, x_cols), :] = _u32(d[:, t * D:(t + 1) * D])
                else:
                    qacc[j] = d

        with jax.named_scope("x_wait"):
            x_copy(0).wait()
        x_transpose(0)
        for i in range(1, XC):
            x_copy(i).start()
        for g in range(QIT):
            for cp in w_copies(g):
                cp.start()
        c_copy.start()
        wo_copy.start()
        a_start(0)
        a_start(1)
        with jax.named_scope("wq_wait"):
            wq_wait(0)
        q_early(0, True, False)

        def early_body(kt, carry):
            with jax.named_scope("wq_wait"):
                wq_wait(kt)
            q_early(kt, False, False)
            return carry

        lax.fori_loop(1, KT - 1, early_body, 0)
        with jax.named_scope("wq_wait"):
            wq_wait(KT - 1)
            for i in range(1, XC):
                x_copy(i).wait()
        q_early(KT - 1, False, True)
        for i in range(1, XC):
            x_transpose(i)

        def unpack(g, sub, j):
            ev, od = (ws_v[g, pl.ds((par * (C // 2) + sub * TP) * 8 + j, TP, stride=8), :]
                      for par in range(2))
            lo, hi = _repack(ev, od)
            rows = pl.ds(sub * TP, TP)
            cols = pl.ds(pl.multiple_of(g * LANE, LANE), LANE)
            wkv_v[2 * j, rows, cols] = lo
            wkv_v[2 * j + 1, rows, cols] = hi
            return [lo, hi]

        units = [(s_, j_) for s_ in range(C // 2 // TP) for j_ in range(H // 2)]

        def qproj(it, r0, n, t, zeros=(None, None)):
            outs = []
            for u in range(2):
                lhs = _bf(linked(x_v[_h(r0, n), :]))
                d = _dot(lhs, _bf(wq_v[it, :, pl.ds(t * D + u * LANE, LANE)]))
                set_link(d)
                if zeros[u] is not None:
                    for k, z in enumerate(zeros[u]):
                        d = _pin(d, z, 8 * ((k * (n // 8)) // len(zeros[u])))
                outs.append(d)
            q2 = _lanecat(outs)
            q_all[2 * it + t, _h(r0, n), :] = _u32((q2 * (D ** -0.5 * LOG2E)).astype(BF16))

        def q_body(it, carry):
            with jax.named_scope("w_wait"):
                w_wait(it)
            link[0] = None
            pieces = [(p, pc, t) for p in range(QP) for pc in range(1, XC) for t in range(2)]
            nd = 2 * len(pieces)
            for k, (p, pc, t) in enumerate(pieces):
                zeros = []
                for u in range(2):
                    d = 2 * k + u
                    mine = units[d * len(units) // nd:(d + 1) * len(units) // nd]
                    zeros.append([_opaque_zero(unpack(it, *u_)) for u_ in mine])
                qproj(QP * it + p, pc * x_cols, x_cols, t, zeros)
            return carry

        with jax.named_scope("q_loop"):
            lax.fori_loop(0, QIT, q_body, 0)
        c_copy.wait()
        wo_copy.wait()
        a_wait(0)

        tri = (lax.broadcasted_iota(jnp.int32, (LANE, LANE), 1)
               <= lax.broadcasted_iota(jnp.int32, (LANE, LANE), 0))

        NOUT = S // D

        def out_copy(i):
            if i >= NOUT:
                t = i - NOUT
                return pltpu.make_async_copy(
                    oa_v.at[t], out_hbm.at[:, pl.ds(t * LANE, LANE)], sem_out.at[i])
            rs = pl.ds(i * D, D)
            return pltpu.make_async_copy(
                out_v.at[rs], out_hbm.at[rs, pl.ds(AT * LANE, 2 * M - AT * LANE)], sem_out.at[i])

        def b_out(k, tot):
            c0 = (k * D) % (S // 2)
            full = _rowcat([ra_t[k * D // (S // 2), AT * LANE:, c0:c0 + D], tot]).T
            out_v[k * D:(k + 1) * D, :] = full.astype(BF16)
            return full

        def head_step(h, carry):
            with jax.named_scope("step"):
                return head_step_(h, carry)

        def head_step_(h, carry):
            with_a = cfg["use_a"]

            @pl.when(h == A_STEPS)
            def _():
                for t in range(AT):
                    out_copy(NOUT + t).start()

            @pl.when(h == cfg["h0"] + 1)
            def _():
                a_wait(1)

            link[0] = None
            n2 = AR // 2
            a_rows2 = pl.ds(pl.multiple_of(jnp.minimum(h, A_STEPS - 1) * n2, n2), n2)
            a_rows = pl.ds(pl.multiple_of(jnp.minimum(h, A_STEPS - 1) * AR, AR), AR)

            def a_fwd():
                kk = _bf(a_v[0, a_rows2, :]).astype(F32)
                lane = lax.broadcasted_iota(jnp.int32, (AR, LANE), 1)
                coef = [par_v[j, a_rows, :] for j in range(KS)]
                rolled = [kk] + [pltpu.roll(kk, j, 1) for j in range(1, KS)]
                vv = _bf(a_v[1, a_rows2, :]).astype(F32)
                kv_blocks = []
                for a in range(NB):
                    cs = slice(a * LANE, (a + 1) * LANE)
                    acc = rolled[0][:, cs] * coef[0]
                    for j in range(1, KS):
                        t = rolled[j][:, cs]
                        if a == 0:
                            t = jnp.where(lane >= j, t, 0.0)
                        acc = acc + t * coef[j]
                    kv_blocks.append(acc * vv[:, cs])
                hk = a_v[2, a_rows2, :]
                hk = _rowcat([hk[:, a * LANE:(a + 1) * LANE] for a in range(NB)])
                fm = _bf(f_v[...])
                hs = _dot(_bf(linked(hk)), fm)
                kv = linked(_rowcat(kv_blocks)).astype(BF16)
                xs = _dot(kv, fm)
                set_link(xs)
                return kv, xs, hs

            def a_conv(xs, hs):
                def tile(v, a, g, part):
                    r = a * AR + 8 * g
                    return v[r:r + 8, part * LANE:(part + 1) * LANE]

                z = {}
                gate = None
                width = cfg["a_width"]
                for g in range(AR // 8):
                    hr = [tile(hs, 0, g, 0)] + [
                        tile(hs, j, g, 0) - tile(hs, j - 1, g, 1) for j in range(1, NB)]
                    hi = [tile(hs, 0, g, 1)] + [
                        tile(hs, j, g, 1) + tile(hs, j - 1, g, 0) for j in range(1, NB)]
                    for c0 in range(0, NB, width):
                        for a in range(c0 + width):
                            xr, xi = tile(xs, a, g, 0), tile(xs, a, g, 1)
                            if gate is not None:
                                xr, xi = _pin(xr, gate), _pin(xi, gate)
                            for c in range(max(c0, a), c0 + width):
                                j = c - a
                                tr = xr * hr[j] - xi * hi[j]
                                ti = xr * hi[j] + xi * hr[j]
                                z[c, g] = (tr, ti) if a == 0 else (z[c, g][0] + tr, z[c, g][1] + ti)
                            gate = _opaque_zero(list(z[c0 + width - 1, g]))
                return z

            def a_inv(kv, z):
                fm = _bf(f_v[...])
                ng = AR // 8
                ys = []
                for u in range(2):
                    rows = [_lanecat(z[c, g]) for g in range(u * ng // 2, (u + 1) * ng // 2)
                            for c in range(NB)]
                    ys.append(_dot_nt(linked(_rowcat(rows)).astype(BF16), fm))
                y = _rowcat(ys)
                dd = par_v[KS, a_rows, :]
                for c in range(NB):
                    cs = slice(c * LANE, (c + 1) * LANE)
                    yc = _rowcat([y[(g * NB + c) * 8:(g * NB + c + 1) * 8, :] for g in range(ng)])
                    qq = _bf(a_v[3, a_rows2, cs]).astype(F32)
                    kvf = kv[c * AR:(c + 1) * AR, :].astype(F32)
                    c2 = (c % (NB // 2)) * LANE
                    ra_t[c // (NB // 2), a_rows, c2:c2 + LANE] = qq * (yc * (1.0 / LANE) + kvf * dd)

            def a_out():
                slab = jnp.clip(h // 4 - 1, 0, AT - 1)
                half = h % 2
                x = ra_t[half, pl.ds(pl.multiple_of(slab * LANE, LANE), LANE), :]
                xt = x.T
                dst = jnp.where(h >= A_STEPS, AT, slab)
                oa_v[dst, pl.ds(pl.multiple_of(half * (S // 2), S // 2), S // 2), :] = xt.astype(BF16)
                return xt

            kw = C // 2
            pending = []

            def flush_pending(x, row):
                done = list(pending)
                del pending[:]
                if not done:
                    return x
                x = _pin(x, _opaque_zero([f for _, f in done]), row)

                @pl.when(h == H - 1)
                def _():
                    for k, _f in done:
                        out_copy(k).start()
                return x

            def proj_w(which, k):
                return wkv_v[h, _h((k % 2) * kw, kw), pl.ds(which * D + (k // 2) * LANE, LANE)]

            def proj(dst, which, r0, n):
                ds = []
                for k in range(4):
                    lhs = linked(c_v[_h(r0, n), pl.ds((k % 2) * kw, kw)])
                    if which == 1 and k == cfg["bo_pass"]:
                        lhs = flush_pending(lhs, cfg["ao_row"])
                    ds.append(_dot(_bf(lhs), _bf(paced(proj_w(which, k)))))
                    set_link(ds[-1])
                dst[_h(r0, n), :] = _u32(_lanecat([ds[0] + ds[1], ds[2] + ds[3]]).astype(BF16))

            def qk(i, dep=None):
                r0 = i * tq
                q = linked(q_all[h, _h(r0, tq), :])
                if dep is not None:
                    q = _pin(q, _opaque_zero([dep]), cfg["ao_row"])
                parts = [_dot_nt(_bf(q), _bf(k_s[_h(0, r0 + LANE), :]))]
                if i > 0:
                    link[0] = _opaque_zero([parts[0][0:8, r0 - LANE:r0]])
                for j in range(1, nsub):
                    q = linked(q_all[h, _h(r0 + LANE * j, tq - LANE * j), :])
                    parts.append(_dot_nt(_bf(q), _bf(k_s[_h(r0 + LANE * j, LANE), :])))
                set_link(parts[2], cfg["link_part"], parts[0])
                return parts

            def softmax(i, parts):
                pb = p_s.at[i % 2]
                chain = _opaque_zero([b[b.shape[0] - 8:, b.shape[1] - LANE:] for b in parts])
                ls = []
                for a in range(nsub):
                    blocks = [parts[j][LANE * (a - j):LANE * (a - j + 1), :] for j in range(a + 1)]
                    last = blocks[-1]
                    w = last.shape[1]
                    dg = jnp.where(tri, last[:, w - LANE:], NEG)
                    blocks[-1] = dg if w == LANE else _lanecat([last[:, :w - LANE], dg])
                    sa = _lanecat(blocks)
                    mb = jnp.broadcast_to(jnp.max(sa, axis=1, keepdims=True), (LANE, LANE))
                    nt = sa.shape[1] // LANE
                    ptiles, psums = [], []
                    for g in range(0, LANE, 8):
                        mg = _pin(mb[g:g + 8, :], chain)
                        pg = [jnp.exp2(sa[g:g + 8, t * LANE:(t + 1) * LANE] - mg) for t in range(nt)]
                        ps = functools.reduce(jnp.add, pg)
                        chain = _opaque_zero([ps])
                        psums.append(ps)
                        ptiles.append(_lanecat(pg))
                    ls.append(jnp.sum(_rowcat(psums), axis=1, keepdims=True))
                    p = _pin(_rowcat(ptiles), link[0], 0, 0 if a == 0 else sa.shape[1] - LANE)
                    pb[LANE * a:LANE * (a + 1), 0:sa.shape[1]] = p.astype(BF16)
                return ls

            def pv(i, ls):
                r0 = i * tq
                pb = p_s.at[i % 2]
                ctx = [_dot(pb[:, 0:r0 + LANE], _bf(v_s[_h(0, r0 + LANE), :]))]
                for j in range(1, nsub):
                    c0 = r0 + LANE * j
                    ctx.append(_dot(pb[LANE * j:, c0:c0 + LANE], _bf(v_s[_h(c0, LANE), :])))
                set_link(ctx[2], cfg["link_part"])
                cs = []
                for a in range(nsub):
                    sl = lambda j: slice(LANE * (a - j), LANE * (a - j + 1))
                    r = pl.reciprocal(ls[a], approx=True)
                    r = r * (2.0 - ls[a] * r)
                    cs.append(functools.reduce(jnp.add, [ctx[j][sl(j)] for j in range(a + 1)]) * r)
                return _rowcat(cs).astype(BF16)

            def oproj(i, ctx):
                for u in range(tq // D):
                    res = _dot_nt(_bf(linked(wo_v[h])), ctx[u * D:(u + 1) * D, :])
                    set_link(res)
                    k = i * (tq // D) + u
                    tot = rb_t[k] + res
                    rb_t[k] = tot
                    if i < nq - 1:
                        pending.append((k, b_out(k, tot)))

            a_state = {}

            def a_hook(tag):
                if with_a and tag == cfg["a_fwd_at"]:
                    a_state["kv"], xs, hs = a_fwd()
                    a_state["z"] = a_conv(xs, hs)
                if with_a and tag == cfg["a_inv_at"]:
                    a_inv(a_state["kv"], a_state["z"])

            a_hook(0)
            proj(k_s, 0, 0, tq)
            a_hook(1)
            parts = qk(0)
            ctx_prev = None
            for i in range(nq):
                r0 = i * tq
                a_hook(10 * (i + 1))
                if ctx_prev is not None:
                    oproj(i - 1, ctx_prev)
                a_hook(10 * (i + 1) + 1)
                if i + 1 < nq:
                    proj(k_s, 0, r0 + tq, tq)
                a_hook(10 * (i + 1) + 2)
                proj(v_s, 1, r0, tq)
                a_hook(10 * (i + 1) + 3)
                ls = softmax(i, parts)
                ctx_prev = pv(i, ls)
                a_hook(10 * (i + 1) + 4)
                if i + 1 < nq:
                    parts = qk(i + 1, a_out() if i + 1 == cfg["ao_at"] else None)
            oproj(nq - 1, ctx_prev)
            assert not pending
            return carry

        with jax.named_scope("loop_a"):
            lax.fori_loop(cfg["h0"], H, head_step, 0)
        with jax.named_scope("tail"):
            for i in range((nq - 1) * (tq // D), NOUT):
                b_out(i, rb_t[i])
                out_copy(i).start()
            for i in range(NOUT + AT):
                out_copy(i).wait()

    scratch = [
        pltpu.VMEM((4, M // 2, S), U32),
        pltpu.VMEM((KS, M), BF16),
        pltpu.VMEM((M,), BF16),
        pltpu.VMEM((KS + 1, M, LANE), F32),
        pltpu.VMEM((LANE // 2, 2 * LANE), U32),
        pltpu.VMEM((M // 2, S), U32),
        pltpu.VMEM((S // 2, MP), U32),
        pltpu.VMEM((S // 2, C), U32),
        pltpu.VMEM((KT, 4 * TP * 8, LANE), U32),
        pltpu.VMEM((H // 2, MP // 2, 2 * D), U32),
        pltpu.VMEM((H // 2, x_cols, 2 * D), F32),
        pltpu.VMEM((QIT, C * 8, LANE), U32),
        pltpu.VMEM((H, C // 2, 2 * D), U32),
        pltpu.VMEM((H, M // 2, D), U32),
        pltpu.VMEM((H, S // 2, D), U32),
        pltpu.VMEM((S // 2, D), U32),
        pltpu.VMEM((S // 2, D), U32),
        pltpu.VMEM((2, tq, S), BF16),
        pltpu.VMEM((2, M, S // 2), F32),
        pltpu.VMEM((S // D, M, D), F32),
        pltpu.VMEM((AT + 1, S, LANE), BF16),
        pltpu.VMEM((S, 2 * M - AT * LANE), BF16),
        pltpu.SemaphoreType.DMA((XC,)),
        pltpu.SemaphoreType.DMA((KT,)),
        pltpu.SemaphoreType.DMA((QIT,)),
        pltpu.SemaphoreType.DMA((1,)),
        pltpu.SemaphoreType.DMA((2,)),
        pltpu.SemaphoreType.DMA((3,)),
        pltpu.SemaphoreType.DMA((S // D + AT,)),
    ]
    return kernel, scratch


_DEFAULT = dict(tq=512, a_fwd_at=13, a_inv_at=44, a_width=4, ao_at=1, ao_row=240,
                bo_pass=2, link_back=176, link_part=32, pace_row=32, pace_step=24,
                use_a=1, h0=0)


def _build(**kw):
    cfg = dict(_DEFAULT)
    cfg.update(kw)
    kernel, scratch = _make_kernel(cfg)

    def run(A_q, A_k, A_v, A_shift_k, A_ssm_k, A_ssm_D, B_x, B_c_kv, B_w_q, B_w_uk,
            B_w_uv, B_w_o):
        tr = lambda a: jnp.swapaxes(a, 1, 2).reshape(M, S)
        args = (
            tr(A_q), tr(A_k), tr(A_v), A_shift_k.T, A_ssm_k, A_ssm_D, tr(B_x),
            B_c_kv.reshape(S, C),
            B_w_q.reshape(M // 2, 2 * H, D), B_w_uk.reshape(C // 2, 2 * H, D),
            B_w_uv.reshape(C // 2, 2 * H, D),
            jnp.swapaxes(B_w_o, 1, 2),
        )
        out = pl.pallas_call(
            kernel,
            in_specs=[pl.BlockSpec(memory_space=pl.ANY)] * len(args),
            out_specs=pl.BlockSpec(memory_space=pl.ANY),
            out_shape=jax.ShapeDtypeStruct((S, 2 * M), BF16),
            scratch_shapes=scratch,
            compiler_params=pltpu.CompilerParams(
                vmem_limit_bytes=120 * 1024 * 1024,
                disable_bounds_checks=True),
        )(*args)
        return out.reshape(1, S, 2 * M)

    return run


_run = _build()


@jax.jit
def pallas_concat_heads__ssm_conv_h3__compressed_kv_cla__prompt_kernel(
    A_q: jax.Array,
    A_k: jax.Array,
    A_v: jax.Array,
    A_shift_k: jax.Array,
    A_ssm_k: jax.Array,
    A_ssm_D: jax.Array,
    B_x: jax.Array,
    B_c_kv: jax.Array,
    B_w_q: jax.Array,
    B_w_uk: jax.Array,
    B_w_uv: jax.Array,
    B_w_o: jax.Array,
):
    return _run(A_q, A_k, A_v, A_shift_k, A_ssm_k, A_ssm_D, B_x, B_c_kv, B_w_q,
                B_w_uk, B_w_uv, B_w_o)
```

```python
import functools

import jax
import jax.numpy as jnp
from jax import lax
import jax.experimental.pallas as pl
import jax.experimental.pallas.tpu as pltpu

F32 = jnp.float32
BF16 = jnp.bfloat16
U32 = jnp.uint32

S = 2048
M = 448
MP = 512
C = 1024
H = 16
D = 256
KS = 4
LANE = 128
NB = S // LANE
AR = 32
A_STEPS = M // AR
LOG2E = 1.4426950408889634
NEG = -1e30

NT = (((1,), (1,)), ((), ()))


def _dot(a, b):
    return jnp.dot(a, b, preferred_element_type=F32)


def _dot_nt(a, b):
    return lax.dot_general(a, b, NT, preferred_element_type=F32)


def _bf(x):
    return pltpu.bitcast(x, BF16)


def _u32(x):
    return pltpu.bitcast(x, U32)


def _h(r0, n):
    return pl.ds(r0 // 2, n // 2)


def _repack(ev, od):
    lo = (ev & jnp.uint32(0xFFFF)) | (od << 16)
    hi = (ev >> 16) | (od & jnp.uint32(0xFFFF0000))
    return lo, hi


def _opaque_zero(vals):
    acc = None
    for v in vals:
        b = v if v.dtype == U32 else pltpu.bitcast(v, U32)
        for r in range(0, b.shape[0], 8):
            for c in range(0, b.shape[1], LANE):
                t = b[r:r + 8, c:c + LANE]
                acc = t if acc is None else acc | t
    return jnp.minimum((acc >> 1).astype(jnp.int32), 0)


def _pin(x, zero, r=0, c=0):
    t = pltpu.bitcast(pltpu.bitcast(x[r:r + 8, c:c + LANE], jnp.int32) + zero, x.dtype)
    row = ([x[r:r + 8, :c]] if c > 0 else []) + [t] + (
        [x[r:r + 8, c + LANE:]] if c + LANE < x.shape[1] else [])
    row = jnp.concatenate(row, axis=1) if len(row) > 1 else row[0]
    col = ([x[:r, :]] if r > 0 else []) + [row] + ([x[r + 8:, :]] if r + 8 < x.shape[0] else [])
    return jnp.concatenate(col, axis=0) if len(col) > 1 else col[0]


def _rowcat(xs):
    return jnp.concatenate(xs, axis=0) if len(xs) > 1 else xs[0]


def _lanecat(xs):
    return jnp.concatenate(xs, axis=1) if len(xs) > 1 else xs[0]


def _make_kernel(cfg):
    tq = cfg["tq"]
    nq = S // tq
    nsub = tq // LANE
    KT = MP // LANE
    TP = LANE // 2
    XC = 4
    x_cols = S // XC
    QP = 2
    QIT = H // 2 // QP
    AT = 3

    def kernel(aq_hbm, ak_hbm, av_hbm, sh_hbm, ssm_hbm, dd_hbm, x_hbm, c_hbm,
               wq_hbm, wk_hbm, wv_hbm, wo_hbm,
               out_hbm,
               a_v, sh_v, dd_v, par_v, f_v,
               xt_v, x_v, c_v, wqs_v, wq_v, qacc, ws_v, wkv_v, wo_v,
               q_all, k_s, v_s, p_s, ra_t, rb_t, oa_v, out_v,
               sem_x, sem_wq, sem_w, sem_c, sem_s, sem_a, sem_out):
        x32, c32, wq32, wk32, wv32, wo32 = (
            r.bitcast(U32) for r in (x_hbm, c_hbm, wq_hbm, wk_hbm, wv_hbm, wo_hbm))
        a32 = [r.bitcast(U32) for r in (ak_hbm, av_hbm, ssm_hbm, aq_hbm)]

        def x_copy(i):
            cs = pl.ds(i * x_cols, x_cols)
            return pltpu.make_async_copy(x32.at[:, cs], xt_v.at[:, cs], sem_x.at[i])

        def wq_copies(kt):
            dst = wqs_v.reshape(4 * KT, TP, 8, LANE)
            rs = pl.ds(min(kt * TP, M // 2 - TP), TP)
            return [pltpu.make_async_copy(
                wq32.at[rs, pl.ds(8 * (k // 2), 8), pl.ds((k % 2) * LANE, LANE)],
                dst.at[4 * kt + k], sem_wq.at[kt]) for k in range(4)]

        def wq_wait(kt):
            pltpu.make_async_copy(wqs_v.at[kt], wqs_v.at[kt], sem_wq.at[kt]).wait()

        def w_copies(g):
            dst = ws_v.reshape(8, C // 2, 8, LANE)
            src = (wk32, wv32)[g // 2]
            return [pltpu.make_async_copy(
                src.at[:, pl.ds(8 * par, 8), pl.ds((g % 2) * LANE, LANE)],
                dst.at[2 * g + par], sem_w.at[g]) for par in range(2)]

        def w_wait(g):
            pltpu.make_async_copy(ws_v.at[g], ws_v.at[g], sem_w.at[g]).wait()

        c_copy = pltpu.make_async_copy(c32, c_v, sem_c.at[0])
        wo_copy = pltpu.make_async_copy(wo32, wo_v, sem_a.at[0])

        a_parts = [pl.ds(0, AR // 2), pl.ds(AR // 2, M // 2 - AR // 2)]

        def a_start(part):
            rs = a_parts[part]
            for k in range(4):
                pltpu.make_async_copy(
                    a32[k].at[rs], a_v.at[k, rs], sem_a.at[1 + part]).start()

        def a_wait(part):
            view = a_v.at[:, a_parts[part]]
            pltpu.make_async_copy(view, view, sem_a.at[1 + part]).wait()

        small = [pltpu.make_async_copy(sh_hbm, sh_v, sem_s.at[0]),
                 pltpu.make_async_copy(dd_hbm, dd_v, sem_s.at[1])]

        link = [None]
        pace = [None]

        def set_link(res, row=None, pacer=None):
            if row is None:
                row = res.shape[0] - cfg["link_back"]
            link[0] = _opaque_zero([res[row:row + 8, res.shape[1] - LANE:]])
            pace[0] = res if pacer is None else pacer

        def linked(x):
            return x if link[0] is None else _pin(x, link[0])

        def paced(w):
            res = pace[0]
            if res is None or link[0] is None or not cfg["pace_step"]:
                return w
            rows = []
            zs = [_opaque_zero([res[r:r + 8, res.shape[1] - LANE:]])
                  for r in range(cfg["pace_row"], cfg["pace_row"] + 8 * cfg["pace_step"],
                                 cfg["pace_step"])]
            for r in range(0, w.shape[0], 8):
                z = zs[7 - (r // 8) % 8]
                t = pltpu.bitcast(w[r:r + 8, :], jnp.int32)
                rows.append(pltpu.bitcast(t + _lanecat([z] * (w.shape[1] // LANE)), U32))
            return _rowcat(rows)

        for cp in small:
            cp.start()
        x_copy(0).start()
        for cp in wq_copies(0):
            cp.start()

        bi = lax.broadcasted_iota(jnp.int32, (LANE, LANE), 0)
        mi = lax.broadcasted_iota(jnp.int32, (LANE, LANE), 1)
        ph = ((4 * mi + 1) * bi) & 511
        ang = ph.astype(F32) * (2.0 * 3.141592653589793 / 512.0)
        f_v[:, 0:LANE] = _u32(jnp.cos(ang).astype(BF16))
        f_v[:, LANE:] = _u32((-jnp.sin(ang)).astype(BF16))

        rb_t[...] = jnp.zeros((S // D, M, D), F32)
        ra_t[:, 0:LANE, :] = jnp.zeros((2, LANE, S // 2), F32)
        ra_t[:, AT * LANE:, :] = jnp.zeros((2, M - AT * LANE, S // 2), F32)

        for kt in range(1, KT):
            for cp in wq_copies(kt):
                cp.start()
        with jax.named_scope("small_wait"):
            for cp in small:
                cp.wait()
        sh = sh_v[...].astype(F32)
        for j in range(KS):
            par_v[j] = jnp.broadcast_to(sh[j:j + 1, :], (LANE, M)).T
        dd = dd_v[...].astype(F32).reshape(1, M)
        par_v[KS] = jnp.broadcast_to(dd, (LANE, M)).T

        def x_transpose(i):
            xt = xt_v[:, pl.ds(i * x_cols, x_cols)]
            nfull = (KT - 1) * TP
            xt = _rowcat([xt[:nfull], jnp.zeros((MP // 2 - M // 2, x_cols), U32), xt[nfull:]])
            x_v[_h(i * x_cols, x_cols), :] = _u32(_bf(xt).astype(F32).T.astype(BF16))

        def q_early(kt, first, last):
            r0 = kt * TP
            rows = pl.ds(r0 if isinstance(r0, int) else pl.multiple_of(r0, TP), TP)
            c0 = kt * LANE
            cols = pl.ds(c0 if isinstance(c0, int) else pl.multiple_of(c0, LANE), LANE)
            link[0] = None
            for j in range(H // 2):
                ws = []
                for half in range(2):
                    ev, od = (
                        wqs_v[kt, pl.ds((2 * par + half) * TP * 8 + j, TP, stride=8), :]
                        for par in range(2))
                    ws.append(_repack(ev, od))
                w = _lanecat([ws[0][0], ws[1][0], ws[0][1], ws[1][1]])
                wq_v[j, rows, :] = w
                d = _dot(_bf(linked(x_v[_h(0, x_cols), cols])), _bf(w))
                set_link(d)
                if not first:
                    d = d + qacc[j]
                if last:
                    d = (d * (D ** -0.5 * LOG2E)).astype(BF16)
                    for t in range(2):
                        q_all[2 * j + t, _h(0, x_cols), :] = _u32(d[:, t * D:(t + 1) * D])
                else:
                    qacc[j] = d

        with jax.named_scope("x_wait"):
            x_copy(0).wait()
        x_transpose(0)
        for i in range(1, XC):
            x_copy(i).start()
        for g in range(QIT):
            for cp in w_copies(g):
                cp.start()
        c_copy.start()
        wo_copy.start()
        a_start(0)
        a_start(1)
        with jax.named_scope("wq_wait"):
            wq_wait(0)
        q_early(0, True, False)

        def early_body(kt, carry):
            with jax.named_scope("wq_wait"):
                wq_wait(kt)
            q_early(kt, False, False)
            return carry

        lax.fori_loop(1, KT - 1, early_body, 0)
        with jax.named_scope("wq_wait"):
            wq_wait(KT - 1)
            for i in range(1, XC):
                x_copy(i).wait()
        q_early(KT - 1, False, True)
        for i in range(1, XC):
            x_transpose(i)

        def unpack(g, sub, j):
            ev, od = (ws_v[g, pl.ds((par * (C // 2) + sub * TP) * 8 + j, TP, stride=8), :]
                      for par in range(2))
            lo, hi = _repack(ev, od)
            rows = pl.ds(sub * TP, TP)
            cols = pl.ds(pl.multiple_of(g * LANE, LANE), LANE)
            wkv_v[2 * j, rows, cols] = lo
            wkv_v[2 * j + 1, rows, cols] = hi
            return [lo, hi]

        units = [(s_, j_) for s_ in range(C // 2 // TP) for j_ in range(H // 2)]

        def qproj(it, r0, n, t, zeros=(None, None)):
            outs = []
            for u in range(2):
                lhs = _bf(linked(x_v[_h(r0, n), :]))
                d = _dot(lhs, _bf(wq_v[it, :, pl.ds(t * D + u * LANE, LANE)]))
                set_link(d)
                if zeros[u] is not None:
                    for k, z in enumerate(zeros[u]):
                        d = _pin(d, z, 8 * ((k * (n // 8)) // len(zeros[u])))
                outs.append(d)
            q2 = _lanecat(outs)
            q_all[2 * it + t, _h(r0, n), :] = _u32((q2 * (D ** -0.5 * LOG2E)).astype(BF16))

        def q_body(it, carry):
            with jax.named_scope("w_wait"):
                w_wait(it)
            link[0] = None
            pieces = [(p, pc, t) for p in range(QP) for pc in range(1, XC) for t in range(2)]
            nd = 2 * len(pieces)
            for k, (p, pc, t) in enumerate(pieces):
                zeros = []
                for u in range(2):
                    d = 2 * k + u
                    mine = units[d * len(units) // nd:(d + 1) * len(units) // nd]
                    zeros.append([_opaque_zero(unpack(it, *u_)) for u_ in mine])
                qproj(QP * it + p, pc * x_cols, x_cols, t, zeros)
            return carry

        with jax.named_scope("q_loop"):
            lax.fori_loop(0, QIT, q_body, 0)
        c_copy.wait()
        wo_copy.wait()
        a_wait(0)

        tri = (lax.broadcasted_iota(jnp.int32, (LANE, LANE), 1)
               <= lax.broadcasted_iota(jnp.int32, (LANE, LANE), 0))

        NOUT = S // D

        def out_copy(i):
            if i >= NOUT:
                t = i - NOUT
                return pltpu.make_async_copy(
                    oa_v.at[t], out_hbm.at[:, pl.ds(t * LANE, LANE)], sem_out.at[i])
            rs = pl.ds(i * D, D)
            return pltpu.make_async_copy(
                out_v.at[rs], out_hbm.at[rs, pl.ds(AT * LANE, 2 * M - AT * LANE)], sem_out.at[i])

        n_body = NOUT - (1 if cfg["last_row"] else tq // D)

        def b_out(k, tot):
            c0 = (k * D) % (S // 2)
            full = _rowcat([ra_t[k * D // (S // 2), AT * LANE:, c0:c0 + D], tot]).T
            out_v[k * D:(k + 1) * D, :] = full.astype(BF16)
            return full

        def head_step(h, carry):
            with jax.named_scope("step"):
                return head_step_(h, carry)

        def head_step_(h, carry):
            with_a = cfg["use_a"]

            @pl.when(h == A_STEPS)
            def _():
                for t in range(AT):
                    out_copy(NOUT + t).start()

            @pl.when(h == cfg["h0"] + 1)
            def _():
                a_wait(1)

            link[0] = None
            n2 = AR // 2
            a_rows2 = pl.ds(pl.multiple_of(jnp.minimum(h, A_STEPS - 1) * n2, n2), n2)
            a_rows = pl.ds(pl.multiple_of(jnp.minimum(h, A_STEPS - 1) * AR, AR), AR)

            def a_fwd():
                kk = _bf(a_v[0, a_rows2, :]).astype(F32)
                lane = lax.broadcasted_iota(jnp.int32, (AR, LANE), 1)
                coef = [par_v[j, a_rows, :] for j in range(KS)]
                rolled = [kk] + [pltpu.roll(kk, j, 1) for j in range(1, KS)]
                vv = _bf(a_v[1, a_rows2, :]).astype(F32)
                kv_blocks = []
                for a in range(NB):
                    cs = slice(a * LANE, (a + 1) * LANE)
                    acc = rolled[0][:, cs] * coef[0]
                    for j in range(1, KS):
                        t = rolled[j][:, cs]
                        if a == 0:
                            t = jnp.where(lane >= j, t, 0.0)
                        acc = acc + t * coef[j]
                    kv_blocks.append(acc * vv[:, cs])
                hk = a_v[2, a_rows2, :]
                hk = _rowcat([hk[:, a * LANE:(a + 1) * LANE] for a in range(NB)])
                fm = _bf(f_v[...])
                hs = _dot(_bf(linked(hk)), fm)
                kv = linked(_rowcat(kv_blocks)).astype(BF16)
                xs = _dot(kv, fm)
                set_link(xs)
                return kv, xs, hs

            def a_conv(xs, hs):
                def tile(v, a, g, part):
                    r = a * AR + 8 * g
                    return v[r:r + 8, part * LANE:(part + 1) * LANE]

                z = {}
                gate = None
                width = cfg["a_width"]
                for g in range(AR // 8):
                    hr = [tile(hs, 0, g, 0)] + [
                        tile(hs, j, g, 0) - tile(hs, j - 1, g, 1) for j in range(1, NB)]
                    hi = [tile(hs, 0, g, 1)] + [
                        tile(hs, j, g, 1) + tile(hs, j - 1, g, 0) for j in range(1, NB)]
                    for c0 in range(0, NB, width):
                        for a in range(c0 + width):
                            xr, xi = tile(xs, a, g, 0), tile(xs, a, g, 1)
                            if gate is not None:
                                xr, xi = _pin(xr, gate), _pin(xi, gate)
                            for c in range(max(c0, a), c0 + width):
                                j = c - a
                                tr = xr * hr[j] - xi * hi[j]
                                ti = xr * hi[j] + xi * hr[j]
                                z[c, g] = (tr, ti) if a == 0 else (z[c, g][0] + tr, z[c, g][1] + ti)
                            gate = _opaque_zero(list(z[c0 + width - 1, g]))
                return z

            def a_inv(kv, z):
                fm = _bf(f_v[...])
                ng = AR // 8
                ys = []
                for u in range(2):
                    rows = [_lanecat(z[c, g]) for g in range(u * ng // 2, (u + 1) * ng // 2)
                            for c in range(NB)]
                    ys.append(_dot_nt(linked(_rowcat(rows)).astype(BF16), fm))
                y = _rowcat(ys)
                dd = par_v[KS, a_rows, :]
                for c in range(NB):
                    cs = slice(c * LANE, (c + 1) * LANE)
                    yc = _rowcat([y[(g * NB + c) * 8:(g * NB + c + 1) * 8, :] for g in range(ng)])
                    qq = _bf(a_v[3, a_rows2, cs]).astype(F32)
                    kvf = kv[c * AR:(c + 1) * AR, :].astype(F32)
                    c2 = (c % (NB // 2)) * LANE
                    ra_t[c // (NB // 2), a_rows, c2:c2 + LANE] = qq * (yc * (1.0 / LANE) + kvf * dd)

            def a_out():
                slab = jnp.clip(h // 4 - 1, 0, AT - 1)
                half = h % 2
                x = ra_t[half, pl.ds(pl.multiple_of(slab * LANE, LANE), LANE), :]
                xt = x.T
                dst = jnp.where(h >= A_STEPS, AT, slab)
                oa_v[dst, pl.ds(pl.multiple_of(half * (S // 2), S // 2), S // 2), :] = xt.astype(BF16)
                return xt

            kw = C // 2
            pending = []

            def flush_pending(x, row):
                done = list(pending)
                del pending[:]
                if not done:
                    return x
                x = _pin(x, _opaque_zero([f for _, f in done]), row)

                @pl.when(h == H - 1)
                def _():
                    for k, _f in done:
                        out_copy(k).start()
                return x

            def proj_w(which, k):
                return wkv_v[h, _h((k % 2) * kw, kw), pl.ds(which * D + (k // 2) * LANE, LANE)]

            def proj(dst, which, r0, n):
                ds = []
                for k in range(4):
                    lhs = linked(c_v[_h(r0, n), pl.ds((k % 2) * kw, kw)])
                    if which == 1 and k == cfg["bo_pass"]:
                        lhs = flush_pending(lhs, cfg["ao_row"])
                    ds.append(_dot(_bf(lhs), _bf(paced(proj_w(which, k)))))
                    set_link(ds[-1])
                dst[_h(r0, n), :] = _u32(_lanecat([ds[0] + ds[1], ds[2] + ds[3]]).astype(BF16))

            def qk(i, dep=None):
                r0 = i * tq
                q = linked(q_all[h, _h(r0, tq), :])
                if dep is not None:
                    q = _pin(q, _opaque_zero([dep]), cfg["ao_row"])
                parts = [_dot_nt(_bf(q), _bf(k_s[_h(0, r0 + LANE), :]))]
                if i > 0:
                    link[0] = _opaque_zero([parts[0][0:8, r0 - LANE:r0]])
                for j in range(1, nsub):
                    q = linked(q_all[h, _h(r0 + LANE * j, tq - LANE * j), :])
                    parts.append(_dot_nt(_bf(q), _bf(k_s[_h(r0 + LANE * j, LANE), :])))
                set_link(parts[2], cfg["link_part"], parts[0])
                return parts

            def softmax(i, parts):
                pb = p_s.at[i % 2]
                chain = _opaque_zero([b[b.shape[0] - 8:, b.shape[1] - LANE:] for b in parts])
                ls = []
                for a in range(nsub):
                    blocks = [parts[j][LANE * (a - j):LANE * (a - j + 1), :] for j in range(a + 1)]
                    last = blocks[-1]
                    w = last.shape[1]
                    dg = jnp.where(tri, last[:, w - LANE:], NEG)
                    blocks[-1] = dg if w == LANE else _lanecat([last[:, :w - LANE], dg])
                    sa = _lanecat(blocks)
                    mb = jnp.broadcast_to(jnp.max(sa, axis=1, keepdims=True), (LANE, LANE))
                    nt = sa.shape[1] // LANE
                    ptiles, psums = [], []
                    for g in range(0, LANE, 8):
                        mg = _pin(mb[g:g + 8, :], chain)
                        pg = [jnp.exp2(sa[g:g + 8, t * LANE:(t + 1) * LANE] - mg) for t in range(nt)]
                        ps = functools.reduce(jnp.add, pg)
                        chain = _opaque_zero([ps])
                        psums.append(ps)
                        ptiles.append(_lanecat(pg))
                    ls.append(jnp.sum(_rowcat(psums), axis=1, keepdims=True))
                    p = _pin(_rowcat(ptiles), link[0], 0, 0 if a == 0 else sa.shape[1] - LANE)
                    pb[LANE * a:LANE * (a + 1), 0:sa.shape[1]] = p.astype(BF16)
                return ls

            def pv(i, ls):
                r0 = i * tq
                pb = p_s.at[i % 2]
                ctx = [_dot(pb[:, 0:r0 + LANE], _bf(v_s[_h(0, r0 + LANE), :]))]
                for j in range(1, nsub):
                    c0 = r0 + LANE * j
                    ctx.append(_dot(pb[LANE * j:, c0:c0 + LANE], _bf(v_s[_h(c0, LANE), :])))
                set_link(ctx[2], cfg["link_part"])
                cs = []
                for a in range(nsub):
                    sl = lambda j: slice(LANE * (a - j), LANE * (a - j + 1))
                    r = pl.reciprocal(ls[a], approx=True)
                    r = r * (2.0 - ls[a] * r)
                    cs.append(functools.reduce(jnp.add, [ctx[j][sl(j)] for j in range(a + 1)]) * r)
                return _rowcat(cs).astype(BF16)

            def oproj(i, ctx):
                for u in range(tq // D):
                    lhs = linked(wo_v[h])
                    if i == nq - 1 and cfg["last_row"]:
                        lhs = flush_pending(lhs, cfg["last_row"])
                    res = _dot_nt(_bf(lhs), ctx[u * D:(u + 1) * D, :])
                    set_link(res)
                    k = i * (tq // D) + u
                    tot = rb_t[k] + res
                    rb_t[k] = tot
                    if k < n_body:
                        pending.append((k, b_out(k, tot)))

            a_state = {}

            def a_hook(tag):
                if with_a and tag == cfg["a_fwd_at"]:
                    a_state["kv"], xs, hs = a_fwd()
                    a_state["z"] = a_conv(xs, hs)
                if with_a and tag == cfg["a_inv_at"]:
                    a_inv(a_state["kv"], a_state["z"])

            a_hook(0)
            proj(k_s, 0, 0, tq)
            a_hook(1)
            parts = qk(0)
            ctx_prev = None
            for i in range(nq):
                r0 = i * tq
                a_hook(10 * (i + 1))
                if ctx_prev is not None:
                    oproj(i - 1, ctx_prev)
                a_hook(10 * (i + 1) + 1)
                if i + 1 < nq:
                    proj(k_s, 0, r0 + tq, tq)
                a_hook(10 * (i + 1) + 2)
                proj(v_s, 1, r0, tq)
                a_hook(10 * (i + 1) + 3)
                ls = softmax(i, parts)
                ctx_prev = pv(i, ls)
                a_hook(10 * (i + 1) + 4)
                if i + 1 < nq:
                    parts = qk(i + 1, a_out() if i + 1 == cfg["ao_at"] else None)
            oproj(nq - 1, ctx_prev)
            assert not pending
            return carry

        with jax.named_scope("loop_a"):
            lax.fori_loop(cfg["h0"], H, head_step, 0)
        with jax.named_scope("tail"):
            for i in range(n_body, NOUT):
                b_out(i, rb_t[i])
                out_copy(i).start()
            for i in range(NOUT + AT):
                out_copy(i).wait()

    scratch = [
        pltpu.VMEM((4, M // 2, S), U32),
        pltpu.VMEM((KS, M), BF16),
        pltpu.VMEM((M,), BF16),
        pltpu.VMEM((KS + 1, M, LANE), F32),
        pltpu.VMEM((LANE // 2, 2 * LANE), U32),
        pltpu.VMEM((M // 2, S), U32),
        pltpu.VMEM((S // 2, MP), U32),
        pltpu.VMEM((S // 2, C), U32),
        pltpu.VMEM((KT, 4 * TP * 8, LANE), U32),
        pltpu.VMEM((H // 2, MP // 2, 2 * D), U32),
        pltpu.VMEM((H // 2, x_cols, 2 * D), F32),
        pltpu.VMEM((QIT, C * 8, LANE), U32),
        pltpu.VMEM((H, C // 2, 2 * D), U32),
        pltpu.VMEM((H, M // 2, D), U32),
        pltpu.VMEM((H, S // 2, D), U32),
        pltpu.VMEM((S // 2, D), U32),
        pltpu.VMEM((S // 2, D), U32),
        pltpu.VMEM((2, tq, S), BF16),
        pltpu.VMEM((2, M, S // 2), F32),
        pltpu.VMEM((S // D, M, D), F32),
        pltpu.VMEM((AT + 1, S, LANE), BF16),
        pltpu.VMEM((S, 2 * M - AT * LANE), BF16),
        pltpu.SemaphoreType.DMA((XC,)),
        pltpu.SemaphoreType.DMA((KT,)),
        pltpu.SemaphoreType.DMA((QIT,)),
        pltpu.SemaphoreType.DMA((1,)),
        pltpu.SemaphoreType.DMA((2,)),
        pltpu.SemaphoreType.DMA((3,)),
        pltpu.SemaphoreType.DMA((S // D + AT,)),
    ]
    return kernel, scratch


_DEFAULT = dict(tq=512, a_fwd_at=13, a_inv_at=44, a_width=4, ao_at=1, ao_row=240,
                bo_pass=2, link_back=176, link_part=32, pace_row=32, pace_step=24,
                use_a=1, h0=0, last_row=216)


def _build(**kw):
    cfg = dict(_DEFAULT)
    cfg.update(kw)
    kernel, scratch = _make_kernel(cfg)

    def run(A_q, A_k, A_v, A_shift_k, A_ssm_k, A_ssm_D, B_x, B_c_kv, B_w_q, B_w_uk,
            B_w_uv, B_w_o):
        tr = lambda a: jnp.swapaxes(a, 1, 2).reshape(M, S)
        args = (
            tr(A_q), tr(A_k), tr(A_v), A_shift_k.T, A_ssm_k, A_ssm_D, tr(B_x),
            B_c_kv.reshape(S, C),
            B_w_q.reshape(M // 2, 2 * H, D), B_w_uk.reshape(C // 2, 2 * H, D),
            B_w_uv.reshape(C // 2, 2 * H, D),
            jnp.swapaxes(B_w_o, 1, 2),
        )
        out = pl.pallas_call(
            kernel,
            in_specs=[pl.BlockSpec(memory_space=pl.ANY)] * len(args),
            out_specs=pl.BlockSpec(memory_space=pl.ANY),
            out_shape=jax.ShapeDtypeStruct((S, 2 * M), BF16),
            scratch_shapes=scratch,
            compiler_params=pltpu.CompilerParams(
                vmem_limit_bytes=120 * 1024 * 1024,
                disable_bounds_checks=True),
        )(*args)
        return out.reshape(1, S, 2 * M)

    return run


_run = _build()


@jax.jit
def pallas_concat_heads__ssm_conv_h3__compressed_kv_cla__prompt_kernel(
    A_q: jax.Array,
    A_k: jax.Array,
    A_v: jax.Array,
    A_shift_k: jax.Array,
    A_ssm_k: jax.Array,
    A_ssm_D: jax.Array,
    B_x: jax.Array,
    B_c_kv: jax.Array,
    B_w_q: jax.Array,
    B_w_uk: jax.Array,
    B_w_uv: jax.Array,
    B_w_o: jax.Array,
):
    return _run(A_q, A_k, A_v, A_shift_k, A_ssm_k, A_ssm_D, B_x, B_c_kv, B_w_q,
                B_w_uk, B_w_uv, B_w_o)
```

```python
import functools

import jax
import jax.numpy as jnp
from jax import lax
import jax.experimental.pallas as pl
import jax.experimental.pallas.tpu as pltpu

F32 = jnp.float32
BF16 = jnp.bfloat16
U32 = jnp.uint32

S = 2048
M = 448
MP = 512
C = 1024
H = 16
D = 256
KS = 4
LANE = 128
NB = S // LANE
AR = 32
A_STEPS = M // AR
LOG2E = 1.4426950408889634
NEG = -1e30

NT = (((1,), (1,)), ((), ()))


def _dot(a, b):
    return jnp.dot(a, b, preferred_element_type=F32)


def _dot_nt(a, b):
    return lax.dot_general(a, b, NT, preferred_element_type=F32)


def _bf(x):
    return pltpu.bitcast(x, BF16)


def _u32(x):
    return pltpu.bitcast(x, U32)


def _h(r0, n):
    return pl.ds(r0 // 2, n // 2)


def _repack(ev, od):
    lo = (ev & jnp.uint32(0xFFFF)) | (od << 16)
    hi = (ev >> 16) | (od & jnp.uint32(0xFFFF0000))
    return lo, hi


def _opaque_zero(vals):
    acc = None
    for v in vals:
        b = v if v.dtype == U32 else pltpu.bitcast(v, U32)
        for r in range(0, b.shape[0], 8):
            for c in range(0, b.shape[1], LANE):
                t = b[r:r + 8, c:c + LANE]
                acc = t if acc is None else acc | t
    return jnp.minimum((acc >> 1).astype(jnp.int32), 0)


def _pin(x, zero, r=0, c=0):
    t = pltpu.bitcast(pltpu.bitcast(x[r:r + 8, c:c + LANE], jnp.int32) + zero, x.dtype)
    row = ([x[r:r + 8, :c]] if c > 0 else []) + [t] + (
        [x[r:r + 8, c + LANE:]] if c + LANE < x.shape[1] else [])
    row = jnp.concatenate(row, axis=1) if len(row) > 1 else row[0]
    col = ([x[:r, :]] if r > 0 else []) + [row] + ([x[r + 8:, :]] if r + 8 < x.shape[0] else [])
    return jnp.concatenate(col, axis=0) if len(col) > 1 else col[0]


def _rowcat(xs):
    return jnp.concatenate(xs, axis=0) if len(xs) > 1 else xs[0]


def _lanecat(xs):
    return jnp.concatenate(xs, axis=1) if len(xs) > 1 else xs[0]


def _make_kernel(cfg):
    tq = cfg["tq"]
    nq = S // tq
    nsub = tq // LANE
    KT = MP // LANE
    TP = LANE // 2
    XC = 4
    x_cols = S // XC
    QP = 2
    QIT = H // 2 // QP
    AT = 3

    def kernel(aq_hbm, ak_hbm, av_hbm, sh_hbm, ssm_hbm, dd_hbm, x_hbm, c_hbm,
               wq_hbm, wk_hbm, wv_hbm, wo_hbm,
               out_hbm,
               a_v, sh_v, dd_v, par_v, f_v,
               xt_v, x_v, c_v, wqs_v, wq_v, qacc, ws_v, wkv_v, wo_v,
               q_all, k_s, v_s, p_s, ra_t, rb_t, oa_v, out_v,
               sem_x, sem_wq, sem_w, sem_c, sem_s, sem_a, sem_out):
        x32, c32, wq32, wk32, wv32, wo32 = (
            r.bitcast(U32) for r in (x_hbm, c_hbm, wq_hbm, wk_hbm, wv_hbm, wo_hbm))
        a32 = [r.bitcast(U32) for r in (ak_hbm, av_hbm, ssm_hbm, aq_hbm)]

        def x_copy(i):
            cs = pl.ds(i * x_cols, x_cols)
            return pltpu.make_async_copy(x32.at[:, cs], xt_v.at[:, cs], sem_x.at[i])

        def wq_copies(kt):
            dst = wqs_v.reshape(4 * KT, TP, 8, LANE)
            rs = pl.ds(min(kt * TP, M // 2 - TP), TP)
            return [pltpu.make_async_copy(
                wq32.at[rs, pl.ds(8 * (k // 2), 8), pl.ds((k % 2) * LANE, LANE)],
                dst.at[4 * kt + k], sem_wq.at[kt]) for k in range(4)]

        def wq_wait(kt):
            pltpu.make_async_copy(wqs_v.at[kt], wqs_v.at[kt], sem_wq.at[kt]).wait()

        def w_copies(g):
            dst = ws_v.reshape(8, C // 2, 8, LANE)
            src = (wk32, wv32)[g // 2]
            return [pltpu.make_async_copy(
                src.at[:, pl.ds(8 * par, 8), pl.ds((g % 2) * LANE, LANE)],
                dst.at[2 * g + par], sem_w.at[g]) for par in range(2)]

        def w_wait(g):
            pltpu.make_async_copy(ws_v.at[g], ws_v.at[g], sem_w.at[g]).wait()

        c_copy = pltpu.make_async_copy(c32, c_v, sem_c.at[0])
        wo_copy = pltpu.make_async_copy(wo32, wo_v, sem_a.at[0])

        a_parts = [pl.ds(0, AR // 2), pl.ds(AR // 2, M // 2 - AR // 2)]

        def a_start(part):
            rs = a_parts[part]
            for k in range(4):
                pltpu.make_async_copy(
                    a32[k].at[rs], a_v.at[k, rs], sem_a.at[1 + part]).start()

        def a_wait(part):
            view = a_v.at[:, a_parts[part]]
            pltpu.make_async_copy(view, view, sem_a.at[1 + part]).wait()

        small = [pltpu.make_async_copy(sh_hbm, sh_v, sem_s.at[0]),
                 pltpu.make_async_copy(dd_hbm, dd_v, sem_s.at[1])]

        link = [None]
        pace = [None]

        def set_link(res, row=None, pacer=None):
            if row is None:
                row = res.shape[0] - cfg["link_back"]
            link[0] = _opaque_zero([res[row:row + 8, res.shape[1] - LANE:]])
            pace[0] = res if pacer is None else pacer

        def linked(x):
            return x if link[0] is None else _pin(x, link[0])

        def paced(w):
            res = pace[0]
            if res is None or link[0] is None or not cfg["pace_step"]:
                return w
            rows = []
            zs = [_opaque_zero([res[r:r + 8, res.shape[1] - LANE:]])
                  for r in range(cfg["pace_row"], cfg["pace_row"] + 8 * cfg["pace_step"],
                                 cfg["pace_step"])]
            for r in range(0, w.shape[0], 8):
                z = zs[7 - (r // 8) % 8]
                t = pltpu.bitcast(w[r:r + 8, :], jnp.int32)
                rows.append(pltpu.bitcast(t + _lanecat([z] * (w.shape[1] // LANE)), U32))
            return _rowcat(rows)

        for cp in small:
            cp.start()
        x_copy(0).start()
        for cp in wq_copies(0):
            cp.start()

        bi = lax.broadcasted_iota(jnp.int32, (LANE, LANE), 0)
        mi = lax.broadcasted_iota(jnp.int32, (LANE, LANE), 1)
        ph = ((4 * mi + 1) * bi) & 511
        ang = ph.astype(F32) * (2.0 * 3.141592653589793 / 512.0)
        f_v[:, 0:LANE] = _u32(jnp.cos(ang).astype(BF16))
        f_v[:, LANE:] = _u32((-jnp.sin(ang)).astype(BF16))

        rb_t[...] = jnp.zeros((S // D, M, D), F32)
        ra_t[:, 0:LANE, :] = jnp.zeros((2, LANE, S // 2), F32)
        ra_t[:, AT * LANE:, :] = jnp.zeros((2, M - AT * LANE, S // 2), F32)

        for kt in range(1, KT):
            for cp in wq_copies(kt):
                cp.start()
        with jax.named_scope("small_wait"):
            for cp in small:
                cp.wait()
        sh = sh_v[...].astype(F32)
        for j in range(KS):
            par_v[j] = jnp.broadcast_to(sh[j:j + 1, :], (LANE, M)).T
        dd = dd_v[...].astype(F32).reshape(1, M)
        par_v[KS] = jnp.broadcast_to(dd, (LANE, M)).T

        def x_transpose(i):
            xt = xt_v[:, pl.ds(i * x_cols, x_cols)]
            nfull = (KT - 1) * TP
            xt = _rowcat([xt[:nfull], jnp.zeros((MP // 2 - M // 2, x_cols), U32), xt[nfull:]])
            x_v[_h(i * x_cols, x_cols), :] = _u32(_bf(xt).astype(F32).T.astype(BF16))

        def q_early(kt, first, last, keep=False):
            r0 = kt * TP
            rows = pl.ds(r0 if isinstance(r0, int) else pl.multiple_of(r0, TP), TP)
            c0 = kt * LANE
            cols = pl.ds(c0 if isinstance(c0, int) else pl.multiple_of(c0, LANE), LANE)
            if not keep:
                link[0] = None
            for j in range(H // 2):
                ws = []
                for half in range(2):
                    ev, od = (
                        wqs_v[kt, pl.ds((2 * par + half) * TP * 8 + j, TP, stride=8), :]
                        for par in range(2))
                    ws.append(_repack(ev, od))
                w = _lanecat([ws[0][0], ws[1][0], ws[0][1], ws[1][1]])
                wq_v[j, rows, :] = w
                d = _dot(_bf(linked(x_v[_h(0, x_cols), cols])), _bf(w))
                set_link(d)
                if not first:
                    d = d + qacc[j]
                if last:
                    d = (d * (D ** -0.5 * LOG2E)).astype(BF16)
                    for t in range(2):
                        q_all[2 * j + t, _h(0, x_cols), :] = _u32(d[:, t * D:(t + 1) * D])
                else:
                    qacc[j] = d

        with jax.named_scope("x_wait"):
            x_copy(0).wait()
        x_transpose(0)
        for i in range(1, XC):
            x_copy(i).start()
        for g in range(QIT):
            for cp in w_copies(g):
                cp.start()
        c_copy.start()
        wo_copy.start()
        a_start(0)
        a_start(1)
        with jax.named_scope("wq_wait"):
            wq_wait(0)
        q_early(0, True, False)

        def early_body(kt, carry):
            with jax.named_scope("wq_wait"):
                wq_wait(kt)
            q_early(kt, False, False)
            return carry

        if cfg["merge12"]:
            with jax.named_scope("wq_wait"):
                wq_wait(1)
                wq_wait(2)
            q_early(1, False, False)
            q_early(2, False, False, keep=True)
        else:
            lax.fori_loop(1, KT - 1, early_body, 0)
        with jax.named_scope("wq_wait"):
            wq_wait(KT - 1)
            for i in range(1, XC):
                x_copy(i).wait()
        q_early(KT - 1, False, True)
        for i in range(1, XC):
            x_transpose(i)

        def unpack(g, sub, j):
            ev, od = (ws_v[g, pl.ds((par * (C // 2) + sub * TP) * 8 + j, TP, stride=8), :]
                      for par in range(2))
            lo, hi = _repack(ev, od)
            rows = pl.ds(sub * TP, TP)
            cols = pl.ds(pl.multiple_of(g * LANE, LANE), LANE)
            wkv_v[2 * j, rows, cols] = lo
            wkv_v[2 * j + 1, rows, cols] = hi
            return [lo, hi]

        units = [(s_, j_) for s_ in range(C // 2 // TP) for j_ in range(H // 2)]

        def qproj(it, r0, n, t, zeros=(None, None)):
            outs = []
            for u in range(2):
                lhs = _bf(linked(x_v[_h(r0, n), :]))
                d = _dot(lhs, _bf(wq_v[it, :, pl.ds(t * D + u * LANE, LANE)]))
                set_link(d)
                if zeros[u] is not None:
                    for k, z in enumerate(zeros[u]):
                        d = _pin(d, z, 8 * ((k * (n // 8)) // len(zeros[u])))
                outs.append(d)
            q2 = _lanecat(outs)
            q_all[2 * it + t, _h(r0, n), :] = _u32((q2 * (D ** -0.5 * LOG2E)).astype(BF16))

        def q_body(it, carry):
            with jax.named_scope("w_wait"):
                w_wait(it)
            link[0] = None
            pieces = [(p, pc, t) for p in range(QP) for pc in range(1, XC) for t in range(2)]
            nd = 2 * len(pieces)
            for k, (p, pc, t) in enumerate(pieces):
                zeros = []
                for u in range(2):
                    d = 2 * k + u
                    mine = units[d * len(units) // nd:(d + 1) * len(units) // nd]
                    zeros.append([_opaque_zero(unpack(it, *u_)) for u_ in mine])
                qproj(QP * it + p, pc * x_cols, x_cols, t, zeros)
            return carry

        with jax.named_scope("q_loop"):
            lax.fori_loop(0, QIT, q_body, 0)
        c_copy.wait()
        wo_copy.wait()
        a_wait(0)

        tri = (lax.broadcasted_iota(jnp.int32, (LANE, LANE), 1)
               <= lax.broadcasted_iota(jnp.int32, (LANE, LANE), 0))

        NOUT = S // D

        def out_copy(i):
            if i >= NOUT:
                t = i - NOUT
                return pltpu.make_async_copy(
                    oa_v.at[t], out_hbm.at[:, pl.ds(t * LANE, LANE)], sem_out.at[i])
            rs = pl.ds(i * D, D)
            return pltpu.make_async_copy(
                out_v.at[rs], out_hbm.at[rs, pl.ds(AT * LANE, 2 * M - AT * LANE)], sem_out.at[i])

        n_body = NOUT - (1 if cfg["last_row"] else tq // D)

        def b_out(k, tot):
            c0 = (k * D) % (S // 2)
            full = _rowcat([ra_t[k * D // (S // 2), AT * LANE:, c0:c0 + D], tot]).T
            out_v[k * D:(k + 1) * D, :] = full.astype(BF16)
            return full

        def head_step(h, carry):
            with jax.named_scope("step"):
                return head_step_(h, carry)

        def head_step_(h, carry):
            with_a = cfg["use_a"]

            @pl.when(h == A_STEPS)
            def _():
                for t in range(AT):
                    out_copy(NOUT + t).start()

            @pl.when(h == cfg["h0"] + 1)
            def _():
                a_wait(1)

            link[0] = None
            n2 = AR // 2
            a_rows2 = pl.ds(pl.multiple_of(jnp.minimum(h, A_STEPS - 1) * n2, n2), n2)
            a_rows = pl.ds(pl.multiple_of(jnp.minimum(h, A_STEPS - 1) * AR, AR), AR)

            def a_fwd():
                kk = _bf(a_v[0, a_rows2, :]).astype(F32)
                lane = lax.broadcasted_iota(jnp.int32, (AR, LANE), 1)
                coef = [par_v[j, a_rows, :] for j in range(KS)]
                rolled = [kk] + [pltpu.roll(kk, j, 1) for j in range(1, KS)]
                vv = _bf(a_v[1, a_rows2, :]).astype(F32)
                kv_blocks = []
                for a in range(NB):
                    cs = slice(a * LANE, (a + 1) * LANE)
                    acc = rolled[0][:, cs] * coef[0]
                    for j in range(1, KS):
                        t = rolled[j][:, cs]
                        if a == 0:
                            t = jnp.where(lane >= j, t, 0.0)
                        acc = acc + t * coef[j]
                    kv_blocks.append(acc * vv[:, cs])
                hk = a_v[2, a_rows2, :]
                hk = _rowcat([hk[:, a * LANE:(a + 1) * LANE] for a in range(NB)])
                fm = _bf(f_v[...])
                hs = _dot(_bf(linked(hk)), fm)
                kv = linked(_rowcat(kv_blocks)).astype(BF16)
                xs = _dot(kv, fm)
                set_link(xs)
                return kv, xs, hs

            def a_conv(xs, hs):
                def tile(v, a, g, part):
                    r = a * AR + 8 * g
                    return v[r:r + 8, part * LANE:(part + 1) * LANE]

                z = {}
                gate = None
                width = cfg["a_width"]
                for g in range(AR // 8):
                    hr = [tile(hs, 0, g, 0)] + [
                        tile(hs, j, g, 0) - tile(hs, j - 1, g, 1) for j in range(1, NB)]
                    hi = [tile(hs, 0, g, 1)] + [
                        tile(hs, j, g, 1) + tile(hs, j - 1, g, 0) for j in range(1, NB)]
                    for c0 in range(0, NB, width):
                        for a in range(c0 + width):
                            xr, xi = tile(xs, a, g, 0), tile(xs, a, g, 1)
                            if gate is not None:
                                xr, xi = _pin(xr, gate), _pin(xi, gate)
                            for c in range(max(c0, a), c0 + width):
                                j = c - a
                                tr = xr * hr[j] - xi * hi[j]
                                ti = xr * hi[j] + xi * hr[j]
                                z[c, g] = (tr, ti) if a == 0 else (z[c, g][0] + tr, z[c, g][1] + ti)
                            gate = _opaque_zero(list(z[c0 + width - 1, g]))
                return z

            def a_inv(kv, z):
                fm = _bf(f_v[...])
                ng = AR // 8
                ys = []
                for u in range(2):
                    rows = [_lanecat(z[c, g]) for g in range(u * ng // 2, (u + 1) * ng // 2)
                            for c in range(NB)]
                    ys.append(_dot_nt(linked(_rowcat(rows)).astype(BF16), fm))
                y = _rowcat(ys)
                dd = par_v[KS, a_rows, :]
                for c in range(NB):
                    cs = slice(c * LANE, (c + 1) * LANE)
                    yc = _rowcat([y[(g * NB + c) * 8:(g * NB + c + 1) * 8, :] for g in range(ng)])
                    qq = _bf(a_v[3, a_rows2, cs]).astype(F32)
                    kvf = kv[c * AR:(c + 1) * AR, :].astype(F32)
                    c2 = (c % (NB // 2)) * LANE
                    ra_t[c // (NB // 2), a_rows, c2:c2 + LANE] = qq * (yc * (1.0 / LANE) + kvf * dd)

            def a_out():
                slab = jnp.clip(h // 4 - 1, 0, AT - 1)
                half = h % 2
                x = ra_t[half, pl.ds(pl.multiple_of(slab * LANE, LANE), LANE), :]
                xt = x.T
                dst = jnp.where(h >= A_STEPS, AT, slab)
                oa_v[dst, pl.ds(pl.multiple_of(half * (S // 2), S // 2), S // 2), :] = xt.astype(BF16)
                return xt

            kw = C // 2
            pending = []

            def flush_pending(x, row):
                done = list(pending)
                del pending[:]
                if not done:
                    return x
                x = _pin(x, _opaque_zero([f for _, f in done]), row)

                @pl.when(h == H - 1)
                def _():
                    for k, _f in done:
                        out_copy(k).start()
                return x

            def proj_w(which, k):
                return wkv_v[h, _h((k % 2) * kw, kw), pl.ds(which * D + (k // 2) * LANE, LANE)]

            def proj(dst, which, r0, n):
                ds = []
                for k in range(4):
                    lhs = linked(c_v[_h(r0, n), pl.ds((k % 2) * kw, kw)])
                    if which == 1 and k == cfg["bo_pass"]:
                        lhs = flush_pending(lhs, cfg["ao_row"])
                    ds.append(_dot(_bf(lhs), _bf(paced(proj_w(which, k)))))
                    set_link(ds[-1])
                dst[_h(r0, n), :] = _u32(_lanecat([ds[0] + ds[1], ds[2] + ds[3]]).astype(BF16))

            def qk(i, dep=None):
                r0 = i * tq
                q = linked(q_all[h, _h(r0, tq), :])
                if dep is not None:
                    q = _pin(q, _opaque_zero([dep]), cfg["ao_row"])
                parts = [_dot_nt(_bf(q), _bf(k_s[_h(0, r0 + LANE), :]))]
                if i > 0:
                    link[0] = _opaque_zero([parts[0][0:8, r0 - LANE:r0]])
                for j in range(1, nsub):
                    q = linked(q_all[h, _h(r0 + LANE * j, tq - LANE * j), :])
                    parts.append(_dot_nt(_bf(q), _bf(k_s[_h(r0 + LANE * j, LANE), :])))
                set_link(parts[2], cfg["link_part"], parts[0])
                return parts

            def softmax(i, parts):
                pb = p_s.at[i % 2]
                chain = _opaque_zero([b[b.shape[0] - 8:, b.shape[1] - LANE:] for b in parts])
                ls = []
                for a in range(nsub):
                    blocks = [parts[j][LANE * (a - j):LANE * (a - j + 1), :] for j in range(a + 1)]
                    last = blocks[-1]
                    w = last.shape[1]
                    dg = jnp.where(tri, last[:, w - LANE:], NEG)
                    blocks[-1] = dg if w == LANE else _lanecat([last[:, :w - LANE], dg])
                    sa = _lanecat(blocks)
                    mb = jnp.broadcast_to(jnp.max(sa, axis=1, keepdims=True), (LANE, LANE))
                    nt = sa.shape[1] // LANE
                    ptiles, psums = [], []
                    for g in range(0, LANE, 8):
                        mg = _pin(mb[g:g + 8, :], chain)
                        pg = [jnp.exp2(sa[g:g + 8, t * LANE:(t + 1) * LANE] - mg) for t in range(nt)]
                        ps = functools.reduce(jnp.add, pg)
                        chain = _opaque_zero([ps])
                        psums.append(ps)
                        ptiles.append(_lanecat(pg))
                    ls.append(jnp.sum(_rowcat(psums), axis=1, keepdims=True))
                    p = _pin(_rowcat(ptiles), link[0], 0, 0 if a == 0 else sa.shape[1] - LANE)
                    pb[LANE * a:LANE * (a + 1), 0:sa.shape[1]] = p.astype(BF16)
                return ls

            def pv(i, ls):
                r0 = i * tq
                pb = p_s.at[i % 2]
                ctx = [_dot(pb[:, 0:r0 + LANE], _bf(v_s[_h(0, r0 + LANE), :]))]
                for j in range(1, nsub):
                    c0 = r0 + LANE * j
                    ctx.append(_dot(pb[LANE * j:, c0:c0 + LANE], _bf(v_s[_h(c0, LANE), :])))
                set_link(ctx[2], cfg["link_part"])
                cs = []
                for a in range(nsub):
                    sl = lambda j: slice(LANE * (a - j), LANE * (a - j + 1))
                    r = pl.reciprocal(ls[a], approx=True)
                    r = r * (2.0 - ls[a] * r)
                    cs.append(functools.reduce(jnp.add, [ctx[j][sl(j)] for j in range(a + 1)]) * r)
                return _rowcat(cs).astype(BF16)

            def oproj(i, ctx):
                for u in range(tq // D):
                    lhs = linked(wo_v[h])
                    if i == nq - 1 and cfg["last_row"]:
                        lhs = flush_pending(lhs, cfg["last_row"])
                    res = _dot_nt(_bf(lhs), ctx[u * D:(u + 1) * D, :])
                    set_link(res)
                    k = i * (tq // D) + u
                    tot = rb_t[k] + res
                    rb_t[k] = tot
                    if k < n_body:
                        pending.append((k, b_out(k, tot)))

            a_state = {}

            def a_hook(tag):
                if with_a and tag == cfg["a_fwd_at"]:
                    a_state["kv"], xs, hs = a_fwd()
                    a_state["z"] = a_conv(xs, hs)
                if with_a and tag == cfg["a_inv_at"]:
                    a_inv(a_state["kv"], a_state["z"])

            a_hook(0)
            proj(k_s, 0, 0, tq)
            a_hook(1)
            parts = qk(0)
            ctx_prev = None
            for i in range(nq):
                r0 = i * tq
                a_hook(10 * (i + 1))
                if ctx_prev is not None:
                    oproj(i - 1, ctx_prev)
                a_hook(10 * (i + 1) + 1)
                if i + 1 < nq:
                    proj(k_s, 0, r0 + tq, tq)
                a_hook(10 * (i + 1) + 2)
                proj(v_s, 1, r0, tq)
                a_hook(10 * (i + 1) + 3)
                ls = softmax(i, parts)
                ctx_prev = pv(i, ls)
                a_hook(10 * (i + 1) + 4)
                if i + 1 < nq:
                    parts = qk(i + 1, a_out() if i + 1 == cfg["ao_at"] else None)
            oproj(nq - 1, ctx_prev)
            assert not pending
            return carry

        with jax.named_scope("loop_a"):
            lax.fori_loop(cfg["h0"], H, head_step, 0)
        with jax.named_scope("tail"):
            for i in range(n_body, NOUT):
                b_out(i, rb_t[i])
                out_copy(i).start()
            for i in range(NOUT + AT):
                out_copy(i).wait()

    scratch = [
        pltpu.VMEM((4, M // 2, S), U32),
        pltpu.VMEM((KS, M), BF16),
        pltpu.VMEM((M,), BF16),
        pltpu.VMEM((KS + 1, M, LANE), F32),
        pltpu.VMEM((LANE // 2, 2 * LANE), U32),
        pltpu.VMEM((M // 2, S), U32),
        pltpu.VMEM((S // 2, MP), U32),
        pltpu.VMEM((S // 2, C), U32),
        pltpu.VMEM((KT, 4 * TP * 8, LANE), U32),
        pltpu.VMEM((H // 2, MP // 2, 2 * D), U32),
        pltpu.VMEM((H // 2, x_cols, 2 * D), F32),
        pltpu.VMEM((QIT, C * 8, LANE), U32),
        pltpu.VMEM((H, C // 2, 2 * D), U32),
        pltpu.VMEM((H, M // 2, D), U32),
        pltpu.VMEM((H, S // 2, D), U32),
        pltpu.VMEM((S // 2, D), U32),
        pltpu.VMEM((S // 2, D), U32),
        pltpu.VMEM((2, tq, S), BF16),
        pltpu.VMEM((2, M, S // 2), F32),
        pltpu.VMEM((S // D, M, D), F32),
        pltpu.VMEM((AT + 1, S, LANE), BF16),
        pltpu.VMEM((S, 2 * M - AT * LANE), BF16),
        pltpu.SemaphoreType.DMA((XC,)),
        pltpu.SemaphoreType.DMA((KT,)),
        pltpu.SemaphoreType.DMA((QIT,)),
        pltpu.SemaphoreType.DMA((1,)),
        pltpu.SemaphoreType.DMA((2,)),
        pltpu.SemaphoreType.DMA((3,)),
        pltpu.SemaphoreType.DMA((S // D + AT,)),
    ]
    return kernel, scratch


_DEFAULT = dict(tq=512, a_fwd_at=13, a_inv_at=44, a_width=4, ao_at=1, ao_row=240,
                bo_pass=2, link_back=176, link_part=32, pace_row=32, pace_step=24,
                use_a=1, h0=0, last_row=216, merge12=1)


def _build(**kw):
    cfg = dict(_DEFAULT)
    cfg.update(kw)
    kernel, scratch = _make_kernel(cfg)

    def run(A_q, A_k, A_v, A_shift_k, A_ssm_k, A_ssm_D, B_x, B_c_kv, B_w_q, B_w_uk,
            B_w_uv, B_w_o):
        tr = lambda a: jnp.swapaxes(a, 1, 2).reshape(M, S)
        args = (
            tr(A_q), tr(A_k), tr(A_v), A_shift_k.T, A_ssm_k, A_ssm_D, tr(B_x),
            B_c_kv.reshape(S, C),
            B_w_q.reshape(M // 2, 2 * H, D), B_w_uk.reshape(C // 2, 2 * H, D),
            B_w_uv.reshape(C // 2, 2 * H, D),
            jnp.swapaxes(B_w_o, 1, 2),
        )
        out = pl.pallas_call(
            kernel,
            in_specs=[pl.BlockSpec(memory_space=pl.ANY)] * len(args),
            out_specs=pl.BlockSpec(memory_space=pl.ANY),
            out_shape=jax.ShapeDtypeStruct((S, 2 * M), BF16),
            scratch_shapes=scratch,
            compiler_params=pltpu.CompilerParams(
                vmem_limit_bytes=120 * 1024 * 1024,
                disable_bounds_checks=True),
        )(*args)
        return out.reshape(1, S, 2 * M)

    return run


_run = _build()


@jax.jit
def pallas_concat_heads__ssm_conv_h3__compressed_kv_cla__prompt_kernel(
    A_q: jax.Array,
    A_k: jax.Array,
    A_v: jax.Array,
    A_shift_k: jax.Array,
    A_ssm_k: jax.Array,
    A_ssm_D: jax.Array,
    B_x: jax.Array,
    B_c_kv: jax.Array,
    B_w_q: jax.Array,
    B_w_uk: jax.Array,
    B_w_uv: jax.Array,
    B_w_o: jax.Array,
):
    return _run(A_q, A_k, A_v, A_shift_k, A_ssm_k, A_ssm_D, B_x, B_c_kv, B_w_q,
                B_w_uk, B_w_uv, B_w_o)
```

```python
import functools

import jax
import jax.numpy as jnp
from jax import lax
import jax.experimental.pallas as pl
import jax.experimental.pallas.tpu as pltpu

F32 = jnp.float32
BF16 = jnp.bfloat16
U32 = jnp.uint32

S = 2048
M = 448
MP = 512
C = 1024
H = 16
D = 256
KS = 4
LANE = 128
NB = S // LANE
AR = 32
A_STEPS = M // AR
LOG2E = 1.4426950408889634
NEG = -1e30

NT = (((1,), (1,)), ((), ()))


def _dot(a, b):
    return jnp.dot(a, b, preferred_element_type=F32)


def _dot_nt(a, b):
    return lax.dot_general(a, b, NT, preferred_element_type=F32)


def _bf(x):
    return pltpu.bitcast(x, BF16)


def _u32(x):
    return pltpu.bitcast(x, U32)


def _h(r0, n):
    return pl.ds(r0 // 2, n // 2)


def _repack(ev, od):
    lo = (ev & jnp.uint32(0xFFFF)) | (od << 16)
    hi = (ev >> 16) | (od & jnp.uint32(0xFFFF0000))
    return lo, hi


def _opaque_zero(vals):
    acc = None
    for v in vals:
        b = v if v.dtype == U32 else pltpu.bitcast(v, U32)
        for r in range(0, b.shape[0], 8):
            for c in range(0, b.shape[1], LANE):
                t = b[r:r + 8, c:c + LANE]
                acc = t if acc is None else acc | t
    return jnp.minimum((acc >> 1).astype(jnp.int32), 0)


def _pin(x, zero, r=0, c=0):
    t = pltpu.bitcast(pltpu.bitcast(x[r:r + 8, c:c + LANE], jnp.int32) + zero, x.dtype)
    row = ([x[r:r + 8, :c]] if c > 0 else []) + [t] + (
        [x[r:r + 8, c + LANE:]] if c + LANE < x.shape[1] else [])
    row = jnp.concatenate(row, axis=1) if len(row) > 1 else row[0]
    col = ([x[:r, :]] if r > 0 else []) + [row] + ([x[r + 8:, :]] if r + 8 < x.shape[0] else [])
    return jnp.concatenate(col, axis=0) if len(col) > 1 else col[0]


def _rowcat(xs):
    return jnp.concatenate(xs, axis=0) if len(xs) > 1 else xs[0]


def _lanecat(xs):
    return jnp.concatenate(xs, axis=1) if len(xs) > 1 else xs[0]


def _make_kernel(cfg):
    tq = cfg["tq"]
    nq = S // tq
    nsub = tq // LANE
    KT = MP // LANE
    TP = LANE // 2
    XC = 4
    x_cols = S // XC
    QP = 2
    QIT = H // 2 // QP
    AT = 3

    def kernel(aq_hbm, ak_hbm, av_hbm, sh_hbm, ssm_hbm, dd_hbm, x_hbm, c_hbm,
               wq_hbm, wk_hbm, wv_hbm, wo_hbm,
               out_hbm,
               a_v, sh_v, dd_v, par_v, f_v,
               xt_v, x_v, c_v, wqs_v, wq_v, qacc, ws_v, wkv_v, wo_v,
               q_all, k_s, v_s, p_s, ra_t, rb_t, oa_v, out_v,
               sem_x, sem_wq, sem_w, sem_c, sem_s, sem_a, sem_out):
        x32, c32, wq32, wk32, wv32, wo32 = (
            r.bitcast(U32) for r in (x_hbm, c_hbm, wq_hbm, wk_hbm, wv_hbm, wo_hbm))
        a32 = [r.bitcast(U32) for r in (ak_hbm, av_hbm, ssm_hbm, aq_hbm)]

        def x_copy(i):
            cs = pl.ds(i * x_cols, x_cols)
            return pltpu.make_async_copy(x32.at[:, cs], xt_v.at[:, cs], sem_x.at[i])

        def wq_pairs(kt):
            return min(TP, M // 2 - kt * TP)

        def wq_copies(kt):
            n = wq_pairs(kt)
            dst = wqs_v[kt].reshape(4, n, 8, LANE)
            return [pltpu.make_async_copy(
                wq32.at[pl.ds(kt * TP, n), pl.ds(8 * (k // 2), 8), pl.ds((k % 2) * LANE, LANE)],
                dst.at[k], sem_wq.at[kt]) for k in range(4)]

        def wq_wait(kt):
            pltpu.make_async_copy(wqs_v[kt], wqs_v[kt], sem_wq.at[kt]).wait()

        def w_copies(g):
            dst = ws_v.reshape(8, C // 2, 8, LANE)
            src = (wk32, wv32)[g // 2]
            return [pltpu.make_async_copy(
                src.at[:, pl.ds(8 * par, 8), pl.ds((g % 2) * LANE, LANE)],
                dst.at[2 * g + par], sem_w.at[g]) for par in range(2)]

        def w_wait(g):
            pltpu.make_async_copy(ws_v.at[g], ws_v.at[g], sem_w.at[g]).wait()

        c_copy = pltpu.make_async_copy(c32, c_v, sem_c.at[0])
        wo_copy = pltpu.make_async_copy(wo32, wo_v, sem_a.at[0])

        a_parts = [pl.ds(0, AR // 2), pl.ds(AR // 2, M // 2 - AR // 2)]

        def a_start(part):
            rs = a_parts[part]
            for k in range(4):
                pltpu.make_async_copy(
                    a32[k].at[rs], a_v.at[k, rs], sem_a.at[1 + part]).start()

        def a_wait(part):
            view = a_v.at[:, a_parts[part]]
            pltpu.make_async_copy(view, view, sem_a.at[1 + part]).wait()

        small = [pltpu.make_async_copy(sh_hbm, sh_v, sem_s.at[0]),
                 pltpu.make_async_copy(dd_hbm, dd_v, sem_s.at[1])]

        link = [None]
        pace = [None]

        def set_link(res, row=None, pacer=None):
            if row is None:
                row = res.shape[0] - cfg["link_back"]
            link[0] = _opaque_zero([res[row:row + 8, res.shape[1] - LANE:]])
            pace[0] = res if pacer is None else pacer

        def linked(x):
            return x if link[0] is None else _pin(x, link[0])

        def paced(w):
            res = pace[0]
            if res is None or link[0] is None or not cfg["pace_step"]:
                return w
            rows = []
            zs = [_opaque_zero([res[r:r + 8, res.shape[1] - LANE:]])
                  for r in range(cfg["pace_row"], cfg["pace_row"] + 8 * cfg["pace_step"],
                                 cfg["pace_step"])]
            for r in range(0, w.shape[0], 8):
                z = zs[7 - (r // 8) % 8]
                t = pltpu.bitcast(w[r:r + 8, :], jnp.int32)
                rows.append(pltpu.bitcast(t + _lanecat([z] * (w.shape[1] // LANE)), U32))
            return _rowcat(rows)

        for cp in small:
            cp.start()
        x_copy(0).start()
        for cp in wq_copies(0):
            cp.start()

        bi = lax.broadcasted_iota(jnp.int32, (LANE, LANE), 0)
        mi = lax.broadcasted_iota(jnp.int32, (LANE, LANE), 1)
        ph = ((4 * mi + 1) * bi) & 511
        ang = ph.astype(F32) * (2.0 * 3.141592653589793 / 512.0)
        f_v[:, 0:LANE] = _u32(jnp.cos(ang).astype(BF16))
        f_v[:, LANE:] = _u32((-jnp.sin(ang)).astype(BF16))

        rb_t[...] = jnp.zeros((S // D, M, D), F32)
        ra_t[:, 0:LANE, :] = jnp.zeros((2, LANE, S // 2), F32)
        ra_t[:, AT * LANE:, :] = jnp.zeros((2, M - AT * LANE, S // 2), F32)

        for kt in range(1, KT):
            for cp in wq_copies(kt):
                cp.start()
        with jax.named_scope("small_wait"):
            for cp in small:
                cp.wait()
        sh = sh_v[...].astype(F32)
        for j in range(KS):
            par_v[j] = jnp.broadcast_to(sh[j:j + 1, :], (LANE, M)).T
        dd = dd_v[...].astype(F32).reshape(1, M)
        par_v[KS] = jnp.broadcast_to(dd, (LANE, M)).T

        def x_transpose(i):
            xt = xt_v[:, pl.ds(i * x_cols, x_cols)]
            xt = _rowcat([xt, jnp.zeros((MP // 2 - M // 2, x_cols), U32)])
            x_v[_h(i * x_cols, x_cols), :] = _u32(_bf(xt).astype(F32).T.astype(BF16))

        def q_early(kt, keep=False):
            first, last = kt == 0, kt == KT - 1
            n = wq_pairs(kt)
            cols = pl.ds(kt * LANE, LANE)
            if not keep:
                link[0] = None
            for j in range(H // 2):
                ws = []
                for half in range(2):
                    ev, od = (wqs_v[kt][pl.ds((2 * par + half) * n * 8 + j, n, stride=8), :]
                              for par in range(2))
                    ws.append(_repack(ev, od))
                w = _lanecat([ws[0][0], ws[1][0], ws[0][1], ws[1][1]])
                if n < TP:
                    w = _rowcat([w, jnp.zeros((TP - n, 2 * D), U32)])
                wq_v[j, pl.ds(kt * TP, TP), :] = w
                d = _dot(_bf(linked(x_v[_h(0, x_cols), cols])), _bf(w))
                set_link(d)
                if not first:
                    d = d + qacc[j]
                if last:
                    d = (d * (D ** -0.5 * LOG2E)).astype(BF16)
                    for t in range(2):
                        q_all[2 * j + t, _h(0, x_cols), :] = _u32(d[:, t * D:(t + 1) * D])
                else:
                    qacc[j] = d

        with jax.named_scope("x_wait"):
            x_copy(0).wait()
        x_transpose(0)
        for i in range(1, XC):
            x_copy(i).start()
        for g in range(QIT):
            for cp in w_copies(g):
                cp.start()
        c_copy.start()
        wo_copy.start()
        a_start(0)
        a_start(1)
        with jax.named_scope("wq_wait"):
            wq_wait(0)
        q_early(0)
        with jax.named_scope("wq_wait"):
            wq_wait(1)
            wq_wait(2)
        q_early(1)
        q_early(2, keep=True)
        with jax.named_scope("wq_wait"):
            wq_wait(3)
            for i in range(1, XC):
                x_copy(i).wait()
        q_early(3)
        for i in range(1, XC):
            x_transpose(i)

        def unpack(g, sub, j):
            ev, od = (ws_v[g, pl.ds((par * (C // 2) + sub * TP) * 8 + j, TP, stride=8), :]
                      for par in range(2))
            lo, hi = _repack(ev, od)
            rows = pl.ds(sub * TP, TP)
            cols = pl.ds(pl.multiple_of(g * LANE, LANE), LANE)
            wkv_v[2 * j, rows, cols] = lo
            wkv_v[2 * j + 1, rows, cols] = hi
            return [lo, hi]

        units = [(s_, j_) for s_ in range(C // 2 // TP) for j_ in range(H // 2)]

        def qproj(it, r0, n, t, zeros=(None, None)):
            outs = []
            for u in range(2):
                lhs = _bf(linked(x_v[_h(r0, n), :]))
                d = _dot(lhs, _bf(wq_v[it, :, pl.ds(t * D + u * LANE, LANE)]))
                set_link(d)
                if zeros[u] is not None:
                    for k, z in enumerate(zeros[u]):
                        d = _pin(d, z, 8 * ((k * (n // 8)) // len(zeros[u])))
                outs.append(d)
            q2 = _lanecat(outs)
            q_all[2 * it + t, _h(r0, n), :] = _u32((q2 * (D ** -0.5 * LOG2E)).astype(BF16))

        def q_body(it, carry):
            with jax.named_scope("w_wait"):
                w_wait(it)
            link[0] = None
            pieces = [(p, pc, t) for p in range(QP) for pc in range(1, XC) for t in range(2)]
            nd = 2 * len(pieces)
            for k, (p, pc, t) in enumerate(pieces):
                zeros = []
                for u in range(2):
                    d = 2 * k + u
                    mine = units[d * len(units) // nd:(d + 1) * len(units) // nd]
                    zeros.append([_opaque_zero(unpack(it, *u_)) for u_ in mine])
                qproj(QP * it + p, pc * x_cols, x_cols, t, zeros)
            return carry

        with jax.named_scope("q_loop"):
            lax.fori_loop(0, QIT, q_body, 0)
        c_copy.wait()
        wo_copy.wait()
        a_wait(0)

        tri = (lax.broadcasted_iota(jnp.int32, (LANE, LANE), 1)
               <= lax.broadcasted_iota(jnp.int32, (LANE, LANE), 0))

        NOUT = S // D

        def out_copy(i):
            if i >= NOUT:
                t = i - NOUT
                return pltpu.make_async_copy(
                    oa_v.at[t], out_hbm.at[:, pl.ds(t * LANE, LANE)], sem_out.at[i])
            rs = pl.ds(i * D, D)
            return pltpu.make_async_copy(
                out_v.at[rs], out_hbm.at[rs, pl.ds(AT * LANE, 2 * M - AT * LANE)], sem_out.at[i])

        n_body = NOUT - (1 if cfg["last_row"] else tq // D)

        def b_out(k, tot):
            c0 = (k * D) % (S // 2)
            full = _rowcat([ra_t[k * D // (S // 2), AT * LANE:, c0:c0 + D], tot]).T
            out_v[k * D:(k + 1) * D, :] = full.astype(BF16)
            return full

        def head_step(h, carry):
            with jax.named_scope("step"):
                return head_step_(h, carry)

        def head_step_(h, carry):
            with_a = cfg["use_a"]

            @pl.when(h == A_STEPS)
            def _():
                for t in range(AT):
                    out_copy(NOUT + t).start()

            @pl.when(h == cfg["h0"] + 1)
            def _():
                a_wait(1)

            link[0] = None
            n2 = AR // 2
            a_rows2 = pl.ds(pl.multiple_of(jnp.minimum(h, A_STEPS - 1) * n2, n2), n2)
            a_rows = pl.ds(pl.multiple_of(jnp.minimum(h, A_STEPS - 1) * AR, AR), AR)

            def a_fwd():
                kk = _bf(a_v[0, a_rows2, :]).astype(F32)
                lane = lax.broadcasted_iota(jnp.int32, (AR, LANE), 1)
                coef = [par_v[j, a_rows, :] for j in range(KS)]
                rolled = [kk] + [pltpu.roll(kk, j, 1) for j in range(1, KS)]
                vv = _bf(a_v[1, a_rows2, :]).astype(F32)
                kv_blocks = []
                for a in range(NB):
                    cs = slice(a * LANE, (a + 1) * LANE)
                    acc = rolled[0][:, cs] * coef[0]
                    for j in range(1, KS):
                        t = rolled[j][:, cs]
                        if a == 0:
                            t = jnp.where(lane >= j, t, 0.0)
                        acc = acc + t * coef[j]
                    kv_blocks.append(acc * vv[:, cs])
                hk = a_v[2, a_rows2, :]
                hk = _rowcat([hk[:, a * LANE:(a + 1) * LANE] for a in range(NB)])
                fm = _bf(f_v[...])
                hs = _dot(_bf(linked(hk)), fm)
                kv = linked(_rowcat(kv_blocks)).astype(BF16)
                xs = _dot(kv, fm)
                set_link(xs)
                return kv, xs, hs

            def a_conv(xs, hs):
                def tile(v, a, g, part):
                    r = a * AR + 8 * g
                    return v[r:r + 8, part * LANE:(part + 1) * LANE]

                z = {}
                gate = None
                width = cfg["a_width"]
                for g in range(AR // 8):
                    hr = [tile(hs, 0, g, 0)] + [
                        tile(hs, j, g, 0) - tile(hs, j - 1, g, 1) for j in range(1, NB)]
                    hi = [tile(hs, 0, g, 1)] + [
                        tile(hs, j, g, 1) + tile(hs, j - 1, g, 0) for j in range(1, NB)]
                    for c0 in range(0, NB, width):
                        for a in range(c0 + width):
                            xr, xi = tile(xs, a, g, 0), tile(xs, a, g, 1)
                            if gate is not None:
                                xr, xi = _pin(xr, gate), _pin(xi, gate)
                            for c in range(max(c0, a), c0 + width):
                                j = c - a
                                tr = xr * hr[j] - xi * hi[j]
                                ti = xr * hi[j] + xi * hr[j]
                                z[c, g] = (tr, ti) if a == 0 else (z[c, g][0] + tr, z[c, g][1] + ti)
                            gate = _opaque_zero(list(z[c0 + width - 1, g]))
                return z

            def a_inv(kv, z):
                fm = _bf(f_v[...])
                ng = AR // 8
                ys = []
                for u in range(2):
                    rows = [_lanecat(z[c, g]) for g in range(u * ng // 2, (u + 1) * ng // 2)
                            for c in range(NB)]
                    ys.append(_dot_nt(linked(_rowcat(rows)).astype(BF16), fm))
                y = _rowcat(ys)
                dd = par_v[KS, a_rows, :]
                for c in range(NB):
                    cs = slice(c * LANE, (c + 1) * LANE)
                    yc = _rowcat([y[(g * NB + c) * 8:(g * NB + c + 1) * 8, :] for g in range(ng)])
                    qq = _bf(a_v[3, a_rows2, cs]).astype(F32)
                    kvf = kv[c * AR:(c + 1) * AR, :].astype(F32)
                    c2 = (c % (NB // 2)) * LANE
                    ra_t[c // (NB // 2), a_rows, c2:c2 + LANE] = qq * (yc * (1.0 / LANE) + kvf * dd)

            def a_out():
                slab = jnp.clip(h // 4 - 1, 0, AT - 1)
                half = h % 2
                x = ra_t[half, pl.ds(pl.multiple_of(slab * LANE, LANE), LANE), :]
                xt = x.T
                dst = jnp.where(h >= A_STEPS, AT, slab)
                oa_v[dst, pl.ds(pl.multiple_of(half * (S // 2), S // 2), S // 2), :] = xt.astype(BF16)
                return xt

            kw = C // 2
            pending = []

            def flush_pending(x, row):
                done = list(pending)
                del pending[:]
                if not done:
                    return x
                x = _pin(x, _opaque_zero([f for _, f in done]), row)

                @pl.when(h == H - 1)
                def _():
                    for k, _f in done:
                        out_copy(k).start()
                return x

            def proj_w(which, k):
                return wkv_v[h, _h((k % 2) * kw, kw), pl.ds(which * D + (k // 2) * LANE, LANE)]

            def proj(dst, which, r0, n):
                ds = []
                for k in range(4):
                    lhs = linked(c_v[_h(r0, n), pl.ds((k % 2) * kw, kw)])
                    if which == 1 and k == cfg["bo_pass"]:
                        lhs = flush_pending(lhs, cfg["ao_row"])
                    ds.append(_dot(_bf(lhs), _bf(paced(proj_w(which, k)))))
                    set_link(ds[-1])
                dst[_h(r0, n), :] = _u32(_lanecat([ds[0] + ds[1], ds[2] + ds[3]]).astype(BF16))

            def qk(i, dep=None):
                r0 = i * tq
                q = linked(q_all[h, _h(r0, tq), :])
                if dep is not None:
                    q = _pin(q, _opaque_zero([dep]), cfg["ao_row"])
                parts = [_dot_nt(_bf(q), _bf(k_s[_h(0, r0 + LANE), :]))]
                if i > 0:
                    link[0] = _opaque_zero([parts[0][0:8, r0 - LANE:r0]])
                for j in range(1, nsub):
                    q = linked(q_all[h, _h(r0 + LANE * j, tq - LANE * j), :])
                    parts.append(_dot_nt(_bf(q), _bf(k_s[_h(r0 + LANE * j, LANE), :])))
                set_link(parts[2], cfg["link_part"], parts[0])
                return parts

            def softmax(i, parts):
                pb = p_s.at[i % 2]
                chain = _opaque_zero([b[b.shape[0] - 8:, b.shape[1] - LANE:] for b in parts])
                ls = []
                for a in range(nsub):
                    blocks = [parts[j][LANE * (a - j):LANE * (a - j + 1), :] for j in range(a + 1)]
                    last = blocks[-1]
                    w = last.shape[1]
                    dg = jnp.where(tri, last[:, w - LANE:], NEG)
                    blocks[-1] = dg if w == LANE else _lanecat([last[:, :w - LANE], dg])
                    sa = _lanecat(blocks)
                    mb = jnp.broadcast_to(jnp.max(sa, axis=1, keepdims=True), (LANE, LANE))
                    nt = sa.shape[1] // LANE
                    ptiles, psums = [], []
                    for g in range(0, LANE, 8):
                        mg = _pin(mb[g:g + 8, :], chain)
                        pg = [jnp.exp2(sa[g:g + 8, t * LANE:(t + 1) * LANE] - mg) for t in range(nt)]
                        ps = functools.reduce(jnp.add, pg)
                        chain = _opaque_zero([ps])
                        psums.append(ps)
                        ptiles.append(_lanecat(pg))
                    ls.append(jnp.sum(_rowcat(psums), axis=1, keepdims=True))
                    p = _pin(_rowcat(ptiles), link[0], 0, 0 if a == 0 else sa.shape[1] - LANE)
                    pb[LANE * a:LANE * (a + 1), 0:sa.shape[1]] = p.astype(BF16)
                return ls

            def pv(i, ls):
                r0 = i * tq
                pb = p_s.at[i % 2]
                ctx = [_dot(pb[:, 0:r0 + LANE], _bf(v_s[_h(0, r0 + LANE), :]))]
                for j in range(1, nsub):
                    c0 = r0 + LANE * j
                    ctx.append(_dot(pb[LANE * j:, c0:c0 + LANE], _bf(v_s[_h(c0, LANE), :])))
                set_link(ctx[2], cfg["link_part"])
                cs = []
                for a in range(nsub):
                    sl = lambda j: slice(LANE * (a - j), LANE * (a - j + 1))
                    r = pl.reciprocal(ls[a], approx=True)
                    r = r * (2.0 - ls[a] * r)
                    cs.append(functools.reduce(jnp.add, [ctx[j][sl(j)] for j in range(a + 1)]) * r)
                return _rowcat(cs).astype(BF16)

            def oproj(i, ctx):
                for u in range(tq // D):
                    lhs = linked(wo_v[h])
                    if i == nq - 1 and cfg["last_row"]:
                        lhs = flush_pending(lhs, cfg["last_row"])
                    res = _dot_nt(_bf(lhs), ctx[u * D:(u + 1) * D, :])
                    set_link(res)
                    k = i * (tq // D) + u
                    tot = rb_t[k] + res
                    rb_t[k] = tot
                    if k < n_body:
                        pending.append((k, b_out(k, tot)))

            a_state = {}

            def a_hook(tag):
                if with_a and tag == cfg["a_fwd_at"]:
                    a_state["kv"], xs, hs = a_fwd()
                    a_state["z"] = a_conv(xs, hs)
                if with_a and tag == cfg["a_inv_at"]:
                    a_inv(a_state["kv"], a_state["z"])

            a_hook(0)
            proj(k_s, 0, 0, tq)
            a_hook(1)
            parts = qk(0)
            ctx_prev = None
            for i in range(nq):
                r0 = i * tq
                a_hook(10 * (i + 1))
                if ctx_prev is not None:
                    oproj(i - 1, ctx_prev)
                a_hook(10 * (i + 1) + 1)
                if i + 1 < nq:
                    proj(k_s, 0, r0 + tq, tq)
                a_hook(10 * (i + 1) + 2)
                proj(v_s, 1, r0, tq)
                a_hook(10 * (i + 1) + 3)
                ls = softmax(i, parts)
                ctx_prev = pv(i, ls)
                a_hook(10 * (i + 1) + 4)
                if i + 1 < nq:
                    parts = qk(i + 1, a_out() if i + 1 == cfg["ao_at"] else None)
            oproj(nq - 1, ctx_prev)
            assert not pending
            return carry

        with jax.named_scope("loop_a"):
            lax.fori_loop(cfg["h0"], H, head_step, 0)
        with jax.named_scope("tail"):
            for i in range(n_body, NOUT):
                b_out(i, rb_t[i])
                out_copy(i).start()
            for i in range(NOUT + AT):
                out_copy(i).wait()

    scratch = [
        pltpu.VMEM((4, M // 2, S), U32),
        pltpu.VMEM((KS, M), BF16),
        pltpu.VMEM((M,), BF16),
        pltpu.VMEM((KS + 1, M, LANE), F32),
        pltpu.VMEM((LANE // 2, 2 * LANE), U32),
        pltpu.VMEM((M // 2, S), U32),
        pltpu.VMEM((S // 2, MP), U32),
        pltpu.VMEM((S // 2, C), U32),
        [pltpu.VMEM((4 * min(TP, M // 2 - kt * TP) * 8, LANE), U32)
         for kt in range(KT)],
        pltpu.VMEM((H // 2, MP // 2, 2 * D), U32),
        pltpu.VMEM((H // 2, x_cols, 2 * D), F32),
        pltpu.VMEM((QIT, C * 8, LANE), U32),
        pltpu.VMEM((H, C // 2, 2 * D), U32),
        pltpu.VMEM((H, M // 2, D), U32),
        pltpu.VMEM((H, S // 2, D), U32),
        pltpu.VMEM((S // 2, D), U32),
        pltpu.VMEM((S // 2, D), U32),
        pltpu.VMEM((2, tq, S), BF16),
        pltpu.VMEM((2, M, S // 2), F32),
        pltpu.VMEM((S // D, M, D), F32),
        pltpu.VMEM((AT + 1, S, LANE), BF16),
        pltpu.VMEM((S, 2 * M - AT * LANE), BF16),
        pltpu.SemaphoreType.DMA((XC,)),
        pltpu.SemaphoreType.DMA((KT,)),
        pltpu.SemaphoreType.DMA((QIT,)),
        pltpu.SemaphoreType.DMA((1,)),
        pltpu.SemaphoreType.DMA((2,)),
        pltpu.SemaphoreType.DMA((3,)),
        pltpu.SemaphoreType.DMA((S // D + AT,)),
    ]
    return kernel, scratch


_DEFAULT = dict(tq=512, a_fwd_at=13, a_inv_at=44, a_width=4, ao_at=1, ao_row=240,
                bo_pass=2, link_back=176, link_part=32, pace_row=32, pace_step=24,
                use_a=1, h0=0, last_row=216)


def _build(**kw):
    cfg = dict(_DEFAULT)
    cfg.update(kw)
    kernel, scratch = _make_kernel(cfg)

    def run(A_q, A_k, A_v, A_shift_k, A_ssm_k, A_ssm_D, B_x, B_c_kv, B_w_q, B_w_uk,
            B_w_uv, B_w_o):
        tr = lambda a: jnp.swapaxes(a, 1, 2).reshape(M, S)
        args = (
            tr(A_q), tr(A_k), tr(A_v), A_shift_k.T, A_ssm_k, A_ssm_D, tr(B_x),
            B_c_kv.reshape(S, C),
            B_w_q.reshape(M // 2, 2 * H, D), B_w_uk.reshape(C // 2, 2 * H, D),
            B_w_uv.reshape(C // 2, 2 * H, D),
            jnp.swapaxes(B_w_o, 1, 2),
        )
        out = pl.pallas_call(
            kernel,
            in_specs=[pl.BlockSpec(memory_space=pl.ANY)] * len(args),
            out_specs=pl.BlockSpec(memory_space=pl.ANY),
            out_shape=jax.ShapeDtypeStruct((S, 2 * M), BF16),
            scratch_shapes=scratch,
            compiler_params=pltpu.CompilerParams(
                vmem_limit_bytes=120 * 1024 * 1024,
                disable_bounds_checks=True),
        )(*args)
        return out.reshape(1, S, 2 * M)

    return run


_run = _build()


@jax.jit
def pallas_concat_heads__ssm_conv_h3__compressed_kv_cla__prompt_kernel(
    A_q: jax.Array,
    A_k: jax.Array,
    A_v: jax.Array,
    A_shift_k: jax.Array,
    A_ssm_k: jax.Array,
    A_ssm_D: jax.Array,
    B_x: jax.Array,
    B_c_kv: jax.Array,
    B_w_q: jax.Array,
    B_w_uk: jax.Array,
    B_w_uv: jax.Array,
    B_w_o: jax.Array,
):
    return _run(A_q, A_k, A_v, A_shift_k, A_ssm_k, A_ssm_D, B_x, B_c_kv, B_w_q,
                B_w_uk, B_w_uv, B_w_o)
```

```python
import functools

import jax
import jax.numpy as jnp
from jax import lax
import jax.experimental.pallas as pl
import jax.experimental.pallas.tpu as pltpu

F32 = jnp.float32
BF16 = jnp.bfloat16
U32 = jnp.uint32

S = 2048
M = 448
MP = 512
C = 1024
H = 16
D = 256
KS = 4
LANE = 128
NB = S // LANE
AR = 32
A_STEPS = M // AR
LOG2E = 1.4426950408889634
NEG = -1e30

NT = (((1,), (1,)), ((), ()))


def _dot(a, b):
    return jnp.dot(a, b, preferred_element_type=F32)


def _dot_nt(a, b):
    return lax.dot_general(a, b, NT, preferred_element_type=F32)


def _bf(x):
    return pltpu.bitcast(x, BF16)


def _u32(x):
    return pltpu.bitcast(x, U32)


def _h(r0, n):
    return pl.ds(r0 // 2, n // 2)


def _repack(ev, od):
    lo = (ev & jnp.uint32(0xFFFF)) | (od << 16)
    hi = (ev >> 16) | (od & jnp.uint32(0xFFFF0000))
    return lo, hi


def _split(w):
    return (pltpu.bitcast(w << 16, F32), pltpu.bitcast(w & jnp.uint32(0xFFFF0000), F32))


def _join(lo, hi):
    half = jnp.uint32(0x8000)
    lo = (pltpu.bitcast(lo, U32) + half) >> 16
    hi = (pltpu.bitcast(hi, U32) + half) & jnp.uint32(0xFFFF0000)
    return lo | hi


def _add(a, b):
    return _join(a[0] + b[0], a[1] + b[1])


def _sub(a, b):
    return _join(a[0] - b[0], a[1] - b[1])


def _opaque_zero(vals):
    acc = None
    for v in vals:
        b = v if v.dtype == U32 else pltpu.bitcast(v, U32)
        for r in range(0, b.shape[0], 8):
            for c in range(0, b.shape[1], LANE):
                t = b[r:r + 8, c:c + LANE]
                acc = t if acc is None else acc | t
    return jnp.minimum((acc >> 1).astype(jnp.int32), 0)


def _pin(x, zero, r=0, c=0):
    t = pltpu.bitcast(pltpu.bitcast(x[r:r + 8, c:c + LANE], jnp.int32) + zero, x.dtype)
    row = ([x[r:r + 8, :c]] if c > 0 else []) + [t] + (
        [x[r:r + 8, c + LANE:]] if c + LANE < x.shape[1] else [])
    row = jnp.concatenate(row, axis=1) if len(row) > 1 else row[0]
    col = ([x[:r, :]] if r > 0 else []) + [row] + ([x[r + 8:, :]] if r + 8 < x.shape[0] else [])
    return jnp.concatenate(col, axis=0) if len(col) > 1 else col[0]


def _rowcat(xs):
    return jnp.concatenate(xs, axis=0) if len(xs) > 1 else xs[0]


def _lanecat(xs):
    return jnp.concatenate(xs, axis=1) if len(xs) > 1 else xs[0]


def _make_kernel(cfg):
    tq = cfg["tq"]
    nq = S // tq
    nsub = tq // LANE
    KT = MP // LANE
    TP = LANE // 2
    XC = 4
    x_cols = S // XC
    QP = 2
    QIT = H // 2 // QP
    AT = 3

    def kernel(aq_hbm, ak_hbm, av_hbm, sh_hbm, ssm_hbm, dd_hbm, x_hbm, c_hbm,
               wq_hbm, wk_hbm, wv_hbm, wo_hbm,
               out_hbm,
               a_v, sh_v, dd_v, par_v, f_v,
               xt_v, x_v, c_v, wqs_v, wq_v, qacc, ws_v, wkv_v, wo_v,
               q_all, k_s, v_s, p_s, ra_t, rb_t, oa_v, out_v,
               sem_x, sem_wq, sem_w, sem_c, sem_s, sem_a, sem_out):
        x32, c32, wq32, wk32, wv32, wo32 = (
            r.bitcast(U32) for r in (x_hbm, c_hbm, wq_hbm, wk_hbm, wv_hbm, wo_hbm))
        a32 = [r.bitcast(U32) for r in (ak_hbm, av_hbm, ssm_hbm, aq_hbm)]

        sa_v = qacc

        def x_copy(i):
            cs = pl.ds(i * x_cols, x_cols)
            return pltpu.make_async_copy(x32.at[:, cs], xt_v.at[:, cs], sem_x.at[i])

        def wq_pairs(kt):
            return min(TP, M // 2 - kt * TP)

        def wq_copies(kt):
            n = wq_pairs(kt)
            dst = wqs_v[kt].reshape(4, n, 8, LANE)
            return [pltpu.make_async_copy(
                wq32.at[pl.ds(kt * TP, n), pl.ds(8 * (k // 2), 8), pl.ds((k % 2) * LANE, LANE)],
                dst.at[k], sem_wq.at[kt]) for k in range(4)]

        def wq_wait(kt):
            pltpu.make_async_copy(wqs_v[kt], wqs_v[kt], sem_wq.at[kt]).wait()

        def w_copies(g):
            dst = ws_v.reshape(8, C // 2, 8, LANE)
            src = (wk32, wv32)[g // 2]
            return [pltpu.make_async_copy(
                src.at[:, pl.ds(8 * par, 8), pl.ds((g % 2) * LANE, LANE)],
                dst.at[2 * g + par], sem_w.at[g]) for par in range(2)]

        def w_wait(g):
            pltpu.make_async_copy(ws_v.at[g], ws_v.at[g], sem_w.at[g]).wait()

        CP = S // 4 // QIT

        def c_copies(p):
            r0 = p * CP
            return [pltpu.make_async_copy(c32.at[rs], c_v.at[rs], sem_c.at[p])
                    for rs in (pl.ds(r0, CP), pl.ds(S // 4 + r0, CP))]

        wo_copy = pltpu.make_async_copy(wo32, wo_v, sem_a.at[0])

        a_parts = [pl.ds(0, AR // 2), pl.ds(AR // 2, M // 2 - AR // 2)]

        def a_start(part):
            rs = a_parts[part]
            for k in range(4):
                pltpu.make_async_copy(
                    a32[k].at[rs], a_v.at[k, rs], sem_a.at[1 + part]).start()

        def a_wait(part):
            view = a_v.at[:, a_parts[part]]
            pltpu.make_async_copy(view, view, sem_a.at[1 + part]).wait()

        small = [pltpu.make_async_copy(sh_hbm, sh_v, sem_s.at[0]),
                 pltpu.make_async_copy(dd_hbm, dd_v, sem_s.at[1])]

        link = [None]
        pace = [None]

        def set_link(res, row=None, pacer=None):
            if row is None:
                row = res.shape[0] - cfg["link_back"]
            link[0] = _opaque_zero([res[row:row + 8, res.shape[1] - LANE:]])
            pace[0] = res if pacer is None else pacer

        def linked(x):
            return x if link[0] is None else _pin(x, link[0])

        def paced(w):
            res = pace[0]
            if res is None or link[0] is None or not cfg["pace_step"]:
                return w
            rows = []
            zs = [_opaque_zero([res[r:r + 8, res.shape[1] - LANE:]])
                  for r in range(cfg["pace_row"], cfg["pace_row"] + 8 * cfg["pace_step"],
                                 cfg["pace_step"])]
            for r in range(0, w.shape[0], 8):
                z = zs[7 - (r // 8) % 8]
                t = pltpu.bitcast(w[r:r + 8, :], jnp.int32)
                rows.append(pltpu.bitcast(t + _lanecat([z] * (w.shape[1] // LANE)), U32))
            return _rowcat(rows)

        for cp in small:
            cp.start()
        x_copy(0).start()
        for cp in wq_copies(0):
            cp.start()

        bi = lax.broadcasted_iota(jnp.int32, (LANE, LANE), 0)
        mi = lax.broadcasted_iota(jnp.int32, (LANE, LANE), 1)
        ph = ((4 * mi + 1) * bi) & 511
        ang = ph.astype(F32) * (2.0 * 3.141592653589793 / 512.0)
        f_v[:, 0:LANE] = _u32(jnp.cos(ang).astype(BF16))
        f_v[:, LANE:] = _u32((-jnp.sin(ang)).astype(BF16))

        rb_t[...] = jnp.zeros((S // D, M, D), F32)
        ra_t[:, 0:LANE, :] = jnp.zeros((2, LANE, S // 2), F32)
        ra_t[:, AT * LANE:, :] = jnp.zeros((2, M - AT * LANE, S // 2), F32)

        for kt in range(1, KT):
            for cp in wq_copies(kt):
                cp.start()
        with jax.named_scope("small_wait"):
            for cp in small:
                cp.wait()
        sh = sh_v[...].astype(F32)
        for j in range(KS):
            par_v[j] = jnp.broadcast_to(sh[j:j + 1, :], (LANE, M)).T
        dd = dd_v[...].astype(F32).reshape(1, M)
        par_v[KS] = jnp.broadcast_to(dd, (LANE, M)).T

        def x_transpose(i):
            xt = xt_v[:, pl.ds(i * x_cols, x_cols)]
            xt = _rowcat([xt, jnp.zeros((MP // 2 - M // 2, x_cols), U32)])
            x_v[_h(i * x_cols, x_cols), :] = _u32(_bf(xt).astype(F32).T.astype(BF16))

        def q_early(kt, keep=False):
            first, last = kt == 0, kt == KT - 1
            n = wq_pairs(kt)
            cols = pl.ds(kt * LANE, LANE)
            if not keep:
                link[0] = None
            for j in range(H // 2):
                ws = []
                for half in range(2):
                    ev, od = (wqs_v[kt][pl.ds((2 * par + half) * n * 8 + j, n, stride=8), :]
                              for par in range(2))
                    ws.append(_repack(ev, od))
                w = _lanecat([ws[0][0], ws[1][0], ws[0][1], ws[1][1]])
                if n < TP:
                    w = _rowcat([w, jnp.zeros((TP - n, 2 * D), U32)])
                wq_v[j, pl.ds(kt * TP, TP), :] = w
                d = _dot(_bf(linked(x_v[_h(0, x_cols), cols])), _bf(w))
                set_link(d)
                if not first:
                    d = d + pltpu.bitcast(qacc[j], F32)
                if last:
                    d = (d * (D ** -0.5 * LOG2E)).astype(BF16)
                    for t in range(2):
                        q_all[2 * j + t, _h(0, x_cols), :] = _u32(d[:, t * D:(t + 1) * D])
                else:
                    qacc[j] = pltpu.bitcast(d, U32)

        with jax.named_scope("x_wait"):
            x_copy(0).wait()
        x_transpose(0)
        for i in range(1, XC):
            x_copy(i).start()
        for g in range(QIT):
            for cp in c_copies(g) + w_copies(g):
                cp.start()
        wo_copy.start()
        a_start(0)
        a_start(1)
        with jax.named_scope("wq_wait"):
            wq_wait(0)
        q_early(0)
        with jax.named_scope("wq_wait"):
            wq_wait(1)
            wq_wait(2)
        q_early(1)
        q_early(2, keep=True)
        with jax.named_scope("wq_wait"):
            wq_wait(3)
            for i in range(1, XC):
                x_copy(i).wait()
        q_early(3)
        for i in range(1, XC):
            x_transpose(i)

        def unpack(g, sub, j):
            ev, od = (ws_v[g, pl.ds((par * (C // 2) + sub * TP) * 8 + j, TP, stride=8), :]
                      for par in range(2))
            lo, hi = _repack(ev, od)
            rows = pl.ds(sub * TP, TP)
            cols = pl.ds(pl.multiple_of(g * LANE, LANE), LANE)
            wkv_v[2 * j, rows, cols] = lo
            wkv_v[2 * j + 1, rows, cols] = hi
            return [lo, hi]

        def a_sums(it, u):
            r0 = pl.multiple_of(it * CP + 8 * u, 8)
            kw = C // 2
            a11, a12, a21, a22 = (
                _split(c_v[pl.ds(r0 + rb * (S // 4), 8), pl.ds(cb * kw, kw)])
                for rb in range(2) for cb in range(2))
            outs = [_add(a11, a22), _add(a21, a22), _add(a11, a12), _sub(a21, a11),
                    _sub(a12, a22)]
            for k, o in enumerate(outs):
                sa_v[k, pl.ds(r0, 8), :] = o
            return outs

        units = [functools.partial(unpack, sub=s_, j=j_)
                 for s_ in range(C // 2 // TP) for j_ in range(H // 2)]
        for u_ in range(CP // 8):
            units.insert(5 * u_ + 4, functools.partial(a_sums, u=u_))

        def qproj(it, r0, n, t, zeros=(None, None)):
            outs = []
            for u in range(2):
                lhs = _bf(linked(x_v[_h(r0, n), :]))
                d = _dot(lhs, _bf(wq_v[it, :, pl.ds(t * D + u * LANE, LANE)]))
                set_link(d)
                if zeros[u] is not None:
                    for k, z in enumerate(zeros[u]):
                        d = _pin(d, z, 8 * ((k * (n // 8)) // len(zeros[u])))
                outs.append(d)
            q2 = _lanecat(outs)
            q_all[2 * it + t, _h(r0, n), :] = _u32((q2 * (D ** -0.5 * LOG2E)).astype(BF16))

        def q_body(it, carry):
            with jax.named_scope("w_wait"):
                w_wait(it)
                r0 = pl.multiple_of(it * CP, CP)
                for rs in (pl.ds(r0, CP), pl.ds(S // 4 + r0, CP)):
                    pltpu.make_async_copy(c_v.at[rs], c_v.at[rs], sem_c.at[it]).wait()
            link[0] = None
            pieces = [(p, pc, t) for p in range(QP) for pc in range(1, XC) for t in range(2)]
            nd = 2 * len(pieces)
            for k, (p, pc, t) in enumerate(pieces):
                zeros = []
                for u in range(2):
                    d = 2 * k + u
                    mine = units[d * len(units) // nd:(d + 1) * len(units) // nd]
                    zeros.append([_opaque_zero(u_(it)) for u_ in mine])
                qproj(QP * it + p, pc * x_cols, x_cols, t, zeros)
            return carry

        with jax.named_scope("q_loop"):
            lax.fori_loop(0, QIT, q_body, 0)
        wo_copy.wait()
        a_wait(0)

        tri = (lax.broadcasted_iota(jnp.int32, (LANE, LANE), 1)
               <= lax.broadcasted_iota(jnp.int32, (LANE, LANE), 0))

        NOUT = S // D

        def out_copy(i):
            if i >= NOUT:
                t = i - NOUT
                return pltpu.make_async_copy(
                    oa_v.at[t], out_hbm.at[:, pl.ds(t * LANE, LANE)], sem_out.at[i])
            rs = pl.ds(i * D, D)
            return pltpu.make_async_copy(
                out_v.at[rs], out_hbm.at[rs, pl.ds(AT * LANE, 2 * M - AT * LANE)], sem_out.at[i])

        n_body = NOUT - (1 if cfg["last_row"] else tq // D)

        def b_out(k, tot):
            c0 = (k * D) % (S // 2)
            full = _rowcat([ra_t[k * D // (S // 2), AT * LANE:, c0:c0 + D], tot]).T
            out_v[k * D:(k + 1) * D, :] = full.astype(BF16)
            return full

        def head_step(h, carry):
            with jax.named_scope("step"):
                return head_step_(h, carry)

        def head_step_(h, carry):
            with_a = cfg["use_a"]

            @pl.when(h == A_STEPS)
            def _():
                for t in range(AT):
                    out_copy(NOUT + t).start()

            @pl.when(h == cfg["h0"] + 1)
            def _():
                a_wait(1)

            link[0] = None
            n2 = AR // 2
            a_rows2 = pl.ds(pl.multiple_of(jnp.minimum(h, A_STEPS - 1) * n2, n2), n2)
            a_rows = pl.ds(pl.multiple_of(jnp.minimum(h, A_STEPS - 1) * AR, AR), AR)

            def a_fwd():
                kk = _bf(a_v[0, a_rows2, :]).astype(F32)
                lane = lax.broadcasted_iota(jnp.int32, (AR, LANE), 1)
                coef = [par_v[j, a_rows, :] for j in range(KS)]
                rolled = [kk] + [pltpu.roll(kk, j, 1) for j in range(1, KS)]
                vv = _bf(a_v[1, a_rows2, :]).astype(F32)
                kv_blocks = []
                for a in range(NB):
                    cs = slice(a * LANE, (a + 1) * LANE)
                    acc = rolled[0][:, cs] * coef[0]
                    for j in range(1, KS):
                        t = rolled[j][:, cs]
                        if a == 0:
                            t = jnp.where(lane >= j, t, 0.0)
                        acc = acc + t * coef[j]
                    kv_blocks.append(acc * vv[:, cs])
                hk = a_v[2, a_rows2, :]
                hk = _rowcat([hk[:, a * LANE:(a + 1) * LANE] for a in range(NB)])
                fm = _bf(f_v[...])
                hs = _dot(_bf(linked(hk)), fm)
                kv = linked(_rowcat(kv_blocks)).astype(BF16)
                xs = _dot(kv, fm)
                set_link(xs)
                return kv, xs, hs

            def a_conv(xs, hs):
                def tile(v, a, g, part):
                    r = a * AR + 8 * g
                    return v[r:r + 8, part * LANE:(part + 1) * LANE]

                z = {}
                gate = None
                width = cfg["a_width"]
                for g in range(AR // 8):
                    hr = [tile(hs, 0, g, 0)] + [
                        tile(hs, j, g, 0) - tile(hs, j - 1, g, 1) for j in range(1, NB)]
                    hi = [tile(hs, 0, g, 1)] + [
                        tile(hs, j, g, 1) + tile(hs, j - 1, g, 0) for j in range(1, NB)]
                    for c0 in range(0, NB, width):
                        for a in range(c0 + width):
                            xr, xi = tile(xs, a, g, 0), tile(xs, a, g, 1)
                            if gate is not None:
                                xr, xi = _pin(xr, gate), _pin(xi, gate)
                            for c in range(max(c0, a), c0 + width):
                                j = c - a
                                tr = xr * hr[j] - xi * hi[j]
                                ti = xr * hi[j] + xi * hr[j]
                                z[c, g] = (tr, ti) if a == 0 else (z[c, g][0] + tr, z[c, g][1] + ti)
                            gate = _opaque_zero(list(z[c0 + width - 1, g]))
                return z

            def a_inv(kv, z):
                fm = _bf(f_v[...])
                ng = AR // 8
                ys = []
                for u in range(2):
                    rows = [_lanecat(z[c, g]) for g in range(u * ng // 2, (u + 1) * ng // 2)
                            for c in range(NB)]
                    ys.append(_dot_nt(linked(_rowcat(rows)).astype(BF16), fm))
                y = _rowcat(ys)
                dd = par_v[KS, a_rows, :]
                for c in range(NB):
                    cs = slice(c * LANE, (c + 1) * LANE)
                    yc = _rowcat([y[(g * NB + c) * 8:(g * NB + c + 1) * 8, :] for g in range(ng)])
                    qq = _bf(a_v[3, a_rows2, cs]).astype(F32)
                    kvf = kv[c * AR:(c + 1) * AR, :].astype(F32)
                    c2 = (c % (NB // 2)) * LANE
                    ra_t[c // (NB // 2), a_rows, c2:c2 + LANE] = qq * (yc * (1.0 / LANE) + kvf * dd)

            def a_out():
                slab = jnp.clip(h // 4 - 1, 0, AT - 1)
                half = h % 2
                x = ra_t[half, pl.ds(pl.multiple_of(slab * LANE, LANE), LANE), :]
                xt = x.T
                dst = jnp.where(h >= A_STEPS, AT, slab)
                oa_v[dst, pl.ds(pl.multiple_of(half * (S // 2), S // 2), S // 2), :] = xt.astype(BF16)
                return xt

            kw = C // 2
            pending = []

            def flush_pending(x, row):
                done = list(pending)
                del pending[:]
                if not done:
                    return x
                x = _pin(x, _opaque_zero([f for _, f in done]), row)

                @pl.when(h == H - 1)
                def _():
                    for k, _f in done:
                        out_copy(k).start()
                return x

            def w_blk(r, c):
                return wkv_v[h, _h(r * kw, kw), pl.ds(c * LANE, LANE)]

            def one_pass(lhs, w, flush):
                lhs = linked(lhs)
                if flush:
                    lhs = flush_pending(lhs, cfg["ao_row"])
                d = _dot(_bf(lhs), _bf(paced(w)))
                set_link(d)
                return d

            def k_proj(blk, flush=-1):
                ds = [one_pass(c_v[_h(blk * tq, tq), pl.ds((k % 2) * kw, kw)],
                               w_blk(k % 2, k // 2), k == flush) for k in range(4)]
                k_s[_h(blk * tq, tq), :] = _u32(
                    _lanecat([ds[0] + ds[1], ds[2] + ds[3]]).astype(BF16))

            def b_op(m):
                blk = lambda r, c: _split(w_blk(r, 2 + c))
                return {1: lambda: _add(blk(0, 0), blk(1, 1)),
                        2: lambda: w_blk(0, 2),
                        3: lambda: _sub(blk(0, 1), blk(1, 1)),
                        4: lambda: _sub(blk(1, 0), blk(0, 0)),
                        5: lambda: w_blk(1, 3),
                        6: lambda: _add(blk(0, 0), blk(0, 1)),
                        7: lambda: _add(blk(1, 0), blk(1, 1))}[m]()

            def a_op(m, rho):
                rs = _h(rho * tq, tq)
                if m == 3:
                    return c_v[rs, 0:kw]
                if m == 4:
                    return c_v[_h(S // 2 + rho * tq, tq), kw:]
                return sa_v[{1: 0, 2: 1, 5: 2, 6: 3, 7: 4}[m], rs, :]

            b_cache, prod = {}, {}

            def v_proj(blk, flush=-1):
                rho = blk % 2
                for k, m in enumerate((5, 1, 4, 7, 3) if blk < 2 else (2, 6)):
                    if m not in b_cache:
                        b_cache[m] = b_op(m)
                    prod[m, rho] = one_pass(a_op(m, rho), b_cache[m], k == flush)
                p = lambda m: prod[m, rho]
                if blk < 2:
                    v = [(p(1) + p(4)) + (p(7) - p(5)), p(3) + p(5)]
                else:
                    v = [p(2) + p(4), (p(1) + p(3)) + (p(6) - p(2))]
                v_s[_h(blk * tq, tq), :] = _u32(_lanecat(v).astype(BF16))

            def qk(i, dep=None, flush=False):
                r0 = i * tq
                q = linked(q_all[h, _h(r0, tq), :])
                if dep is not None:
                    q = _pin(q, _opaque_zero([dep]), cfg["ao_row"])
                if flush:
                    q = flush_pending(q, cfg["ao_row"] - 8)
                parts = [_dot_nt(_bf(q), _bf(k_s[_h(0, r0 + LANE), :]))]
                if i > 0:
                    link[0] = _opaque_zero([parts[0][0:8, r0 - LANE:r0]])
                for j in range(1, nsub):
                    q = linked(q_all[h, _h(r0 + LANE * j, tq - LANE * j), :])
                    parts.append(_dot_nt(_bf(q), _bf(k_s[_h(r0 + LANE * j, LANE), :])))
                set_link(parts[2], cfg["link_part"], parts[0])
                return parts

            def softmax(i, parts):
                pb = p_s.at[i % 2]
                chain = _opaque_zero([b[b.shape[0] - 8:, b.shape[1] - LANE:] for b in parts])
                ls = []
                for a in range(nsub):
                    blocks = [parts[j][LANE * (a - j):LANE * (a - j + 1), :] for j in range(a + 1)]
                    last = blocks[-1]
                    w = last.shape[1]
                    dg = jnp.where(tri, last[:, w - LANE:], NEG)
                    blocks[-1] = dg if w == LANE else _lanecat([last[:, :w - LANE], dg])
                    sa = _lanecat(blocks)
                    mb = jnp.broadcast_to(jnp.max(sa, axis=1, keepdims=True), (LANE, LANE))
                    nt = sa.shape[1] // LANE
                    ptiles, psums = [], []
                    for g in range(0, LANE, 8):
                        mg = _pin(mb[g:g + 8, :], chain)
                        pg = [jnp.exp2(sa[g:g + 8, t * LANE:(t + 1) * LANE] - mg) for t in range(nt)]
                        ps = functools.reduce(jnp.add, pg)
                        chain = _opaque_zero([ps])
                        psums.append(ps)
                        ptiles.append(_lanecat(pg))
                    ls.append(jnp.sum(_rowcat(psums), axis=1, keepdims=True))
                    p = _pin(_rowcat(ptiles), link[0], 0, 0 if a == 0 else sa.shape[1] - LANE)
                    pb[LANE * a:LANE * (a + 1), 0:sa.shape[1]] = p.astype(BF16)
                return ls

            def pv(i, ls):
                r0 = i * tq
                pb = p_s.at[i % 2]
                ctx = [_dot(pb[:, 0:r0 + LANE], _bf(v_s[_h(0, r0 + LANE), :]))]
                for j in range(1, nsub):
                    c0 = r0 + LANE * j
                    ctx.append(_dot(pb[LANE * j:, c0:c0 + LANE], _bf(v_s[_h(c0, LANE), :])))
                set_link(ctx[2], cfg["link_part"], ctx[0])
                cs = []
                for a in range(nsub):
                    sl = lambda j: slice(LANE * (a - j), LANE * (a - j + 1))
                    r = pl.reciprocal(ls[a], approx=True)
                    r = r * (2.0 - ls[a] * r)
                    cs.append(functools.reduce(jnp.add, [ctx[j][sl(j)] for j in range(a + 1)]) * r)
                return _rowcat(cs).astype(BF16)

            def oproj(i, ctx):
                for u in range(tq // D):
                    lhs = linked(wo_v[h])
                    if i == nq - 1 and cfg["last_row"]:
                        lhs = flush_pending(lhs, cfg["last_row"])
                    res = _dot_nt(_bf(lhs), ctx[u * D:(u + 1) * D, :])
                    set_link(res)
                    k = i * (tq // D) + u
                    tot = rb_t[k] + res
                    rb_t[k] = tot
                    if k < n_body:
                        pending.append((k, b_out(k, tot)))

            st = {}
            for op in cfg["seq"].split():
                op, _, fl = op.partition("!")
                fl = int(fl) if fl else -1
                kind, i = op[0], int(op[1:] or 0)
                if kind == "K":
                    k_proj(i, fl)
                elif kind == "V":
                    v_proj(i, fl)
                elif kind == "Q":
                    st["s", i] = qk(i, a_out() if i == cfg["ao_at"] else None, fl >= 0)
                elif kind == "P":
                    st["ctx", i] = pv(i, softmax(i, st["s", i]))
                elif kind == "O":
                    oproj(i, st["ctx", i])
                elif kind == "F" and with_a:
                    st["kv"], xs, hs = a_fwd()
                    st["z"] = a_conv(xs, hs)
                elif kind == "I" and with_a:
                    a_inv(st["kv"], st["z"])
            assert not pending
            return carry

        with jax.named_scope("loop_a"):
            lax.fori_loop(cfg["h0"], H, head_step, 0)
        with jax.named_scope("tail"):
            for i in range(n_body, NOUT):
                b_out(i, rb_t[i])
                out_copy(i).start()
            for i in range(NOUT + AT):
                out_copy(i).wait()

    scratch = [
        pltpu.VMEM((4, M // 2, S), U32),
        pltpu.VMEM((KS, M), BF16),
        pltpu.VMEM((M,), BF16),
        pltpu.VMEM((KS + 1, M, LANE), F32),
        pltpu.VMEM((LANE // 2, 2 * LANE), U32),
        pltpu.VMEM((M // 2, S), U32),
        pltpu.VMEM((S // 2, MP), U32),
        pltpu.VMEM((S // 2, C), U32),
        [pltpu.VMEM((4 * min(TP, M // 2 - kt * TP) * 8, LANE), U32)
         for kt in range(KT)],
        pltpu.VMEM((H // 2, MP // 2, 2 * D), U32),
        pltpu.VMEM((H // 2, x_cols, 2 * D), U32),
        pltpu.VMEM((QIT, C * 8, LANE), U32),
        pltpu.VMEM((H, C // 2, 2 * D), U32),
        pltpu.VMEM((H, M // 2, D), U32),
        pltpu.VMEM((H, S // 2, D), U32),
        pltpu.VMEM((S // 2, D), U32),
        pltpu.VMEM((S // 2, D), U32),
        pltpu.VMEM((2, tq, S), BF16),
        pltpu.VMEM((2, M, S // 2), F32),
        pltpu.VMEM((S // D, M, D), F32),
        pltpu.VMEM((AT + 1, S, LANE), BF16),
        pltpu.VMEM((S, 2 * M - AT * LANE), BF16),
        pltpu.SemaphoreType.DMA((XC,)),
        pltpu.SemaphoreType.DMA((KT,)),
        pltpu.SemaphoreType.DMA((QIT,)),
        pltpu.SemaphoreType.DMA((QIT,)),
        pltpu.SemaphoreType.DMA((2,)),
        pltpu.SemaphoreType.DMA((3,)),
        pltpu.SemaphoreType.DMA((S // D + AT,)),
    ]
    return kernel, scratch


_DEFAULT = dict(
    tq=512, a_width=4, ao_at=1, ao_row=240, link_back=176, link_part=32, pace_row=32,
    pace_step=24, use_a=1, h0=0, last_row=216,
    seq="K0 Q0 K1 Q1 V0 F P0 K2 Q2 O0 V1!2 P1 K3 Q3 O1 V2!1 P2 O2 V3!1 P3 I O3")


def _build(**kw):
    cfg = dict(_DEFAULT)
    cfg.update(kw)
    kernel, scratch = _make_kernel(cfg)

    def run(A_q, A_k, A_v, A_shift_k, A_ssm_k, A_ssm_D, B_x, B_c_kv, B_w_q, B_w_uk,
            B_w_uv, B_w_o):
        tr = lambda a: jnp.swapaxes(a, 1, 2).reshape(M, S)
        args = (
            tr(A_q), tr(A_k), tr(A_v), A_shift_k.T, A_ssm_k, A_ssm_D, tr(B_x),
            B_c_kv.reshape(S, C),
            B_w_q.reshape(M // 2, 2 * H, D), B_w_uk.reshape(C // 2, 2 * H, D),
            B_w_uv.reshape(C // 2, 2 * H, D),
            jnp.swapaxes(B_w_o, 1, 2),
        )
        out = pl.pallas_call(
            kernel,
            in_specs=[pl.BlockSpec(memory_space=pl.ANY)] * len(args),
            out_specs=pl.BlockSpec(memory_space=pl.ANY),
            out_shape=jax.ShapeDtypeStruct((S, 2 * M), BF16),
            scratch_shapes=scratch,
            compiler_params=pltpu.CompilerParams(
                vmem_limit_bytes=120 * 1024 * 1024,
                disable_bounds_checks=True),
        )(*args)
        return out.reshape(1, S, 2 * M)

    return run


_run = _build()


@jax.jit
def pallas_concat_heads__ssm_conv_h3__compressed_kv_cla__prompt_kernel(
    A_q: jax.Array,
    A_k: jax.Array,
    A_v: jax.Array,
    A_shift_k: jax.Array,
    A_ssm_k: jax.Array,
    A_ssm_D: jax.Array,
    B_x: jax.Array,
    B_c_kv: jax.Array,
    B_w_q: jax.Array,
    B_w_uk: jax.Array,
    B_w_uv: jax.Array,
    B_w_o: jax.Array,
):
    return _run(A_q, A_k, A_v, A_shift_k, A_ssm_k, A_ssm_D, B_x, B_c_kv, B_w_q,
                B_w_uk, B_w_uv, B_w_o)
```

```python
import functools

import jax
import jax.numpy as jnp
from jax import lax
import jax.experimental.pallas as pl
import jax.experimental.pallas.tpu as pltpu

F32 = jnp.float32
BF16 = jnp.bfloat16
U32 = jnp.uint32

S = 2048
M = 448
MP = 512
C = 1024
H = 16
D = 256
KS = 4
LANE = 128
NB = S // LANE
AR = 32
A_STEPS = M // AR
LOG2E = 1.4426950408889634
NEG = -1e30

NT = (((1,), (1,)), ((), ()))


def _dot(a, b):
    return jnp.dot(a, b, preferred_element_type=F32)


def _dot_nt(a, b):
    return lax.dot_general(a, b, NT, preferred_element_type=F32)


def _bf(x):
    return pltpu.bitcast(x, BF16)


def _u32(x):
    return pltpu.bitcast(x, U32)


def _h(r0, n):
    return pl.ds(r0 // 2, n // 2)


def _repack(ev, od):
    lo = (ev & jnp.uint32(0xFFFF)) | (od << 16)
    hi = (ev >> 16) | (od & jnp.uint32(0xFFFF0000))
    return lo, hi


def _split(w):
    return (pltpu.bitcast(w << 16, F32), pltpu.bitcast(w & jnp.uint32(0xFFFF0000), F32))


def _join(lo, hi):
    half = jnp.uint32(0x8000)
    lo = (pltpu.bitcast(lo, U32) + half) >> 16
    hi = (pltpu.bitcast(hi, U32) + half) & jnp.uint32(0xFFFF0000)
    return lo | hi


def _add(a, b):
    return _join(a[0] + b[0], a[1] + b[1])


def _sub(a, b):
    return _join(a[0] - b[0], a[1] - b[1])


def _opaque_zero(vals):
    acc = None
    for v in vals:
        b = v if v.dtype == U32 else pltpu.bitcast(v, U32)
        for r in range(0, b.shape[0], 8):
            for c in range(0, b.shape[1], LANE):
                t = b[r:r + 8, c:c + LANE]
                acc = t if acc is None else acc | t
    return jnp.minimum((acc >> 1).astype(jnp.int32), 0)


def _pin(x, zero, r=0, c=0):
    t = pltpu.bitcast(pltpu.bitcast(x[r:r + 8, c:c + LANE], jnp.int32) + zero, x.dtype)
    row = ([x[r:r + 8, :c]] if c > 0 else []) + [t] + (
        [x[r:r + 8, c + LANE:]] if c + LANE < x.shape[1] else [])
    row = jnp.concatenate(row, axis=1) if len(row) > 1 else row[0]
    col = ([x[:r, :]] if r > 0 else []) + [row] + ([x[r + 8:, :]] if r + 8 < x.shape[0] else [])
    return jnp.concatenate(col, axis=0) if len(col) > 1 else col[0]


def _rowcat(xs):
    return jnp.concatenate(xs, axis=0) if len(xs) > 1 else xs[0]


def _lanecat(xs):
    return jnp.concatenate(xs, axis=1) if len(xs) > 1 else xs[0]


def _make_kernel(cfg):
    tq = cfg["tq"]
    nq = S // tq
    nsub = tq // LANE
    KT = MP // LANE
    TP = LANE // 2
    XC = 4
    x_cols = S // XC
    QP = 2
    QIT = H // 2 // QP
    AT = 3

    def kernel(aq_hbm, ak_hbm, av_hbm, sh_hbm, ssm_hbm, dd_hbm, x_hbm, c_hbm,
               wq_hbm, wk_hbm, wv_hbm, wo_hbm,
               out_hbm,
               a_v, sh_v, dd_v, par_v, f_v,
               xt_v, x_v, c_v, wqs_v, wq_v, qacc, ws_v, wkv_v, wo_v,
               q_all, k_s, v_s, p_s, ra_t, rb_t, oa_v, out_v,
               sem_x, sem_wq, sem_w, sem_c, sem_s, sem_a, sem_out):
        x32, c32, wq32, wk32, wv32, wo32 = (
            r.bitcast(U32) for r in (x_hbm, c_hbm, wq_hbm, wk_hbm, wv_hbm, wo_hbm))
        a32 = [r.bitcast(U32) for r in (ak_hbm, av_hbm, ssm_hbm, aq_hbm)]

        sa_v = qacc

        def x_copy(i):
            cs = pl.ds(i * x_cols, x_cols)
            return pltpu.make_async_copy(x32.at[:, cs], xt_v.at[:, cs], sem_x.at[i])

        def wq_pairs(kt):
            return min(TP, M // 2 - kt * TP)

        def wq_copies(kt):
            n = wq_pairs(kt)
            dst = wqs_v[kt].reshape(4, n, 8, LANE)
            return [pltpu.make_async_copy(
                wq32.at[pl.ds(kt * TP, n), pl.ds(8 * (k // 2), 8), pl.ds((k % 2) * LANE, LANE)],
                dst.at[k], sem_wq.at[kt]) for k in range(4)]

        def wq_wait(kt):
            pltpu.make_async_copy(wqs_v[kt], wqs_v[kt], sem_wq.at[kt]).wait()

        def w_copies(g):
            dst = ws_v.reshape(8, C // 2, 8, LANE)
            src = (wk32, wv32)[g // 2]
            return [pltpu.make_async_copy(
                src.at[:, pl.ds(8 * par, 8), pl.ds((g % 2) * LANE, LANE)],
                dst.at[2 * g + par], sem_w.at[g]) for par in range(2)]

        def w_wait(g):
            pltpu.make_async_copy(ws_v.at[g], ws_v.at[g], sem_w.at[g]).wait()

        CP = S // 4 // QIT

        def c_copies(p):
            r0 = p * CP
            return [pltpu.make_async_copy(c32.at[rs], c_v.at[rs], sem_c.at[p])
                    for rs in (pl.ds(r0, CP), pl.ds(S // 4 + r0, CP))]

        wo_copy = pltpu.make_async_copy(wo32, wo_v, sem_a.at[0])

        a_parts = [pl.ds(0, AR // 2), pl.ds(AR // 2, M // 2 - AR // 2)]

        def a_start(part):
            rs = a_parts[part]
            for k in range(4):
                pltpu.make_async_copy(
                    a32[k].at[rs], a_v.at[k, rs], sem_a.at[1 + part]).start()

        def a_wait(part):
            view = a_v.at[:, a_parts[part]]
            pltpu.make_async_copy(view, view, sem_a.at[1 + part]).wait()

        small = [pltpu.make_async_copy(sh_hbm, sh_v, sem_s.at[0]),
                 pltpu.make_async_copy(dd_hbm, dd_v, sem_s.at[1])]

        link = [None]
        pace = [None]

        def set_link(res, row=None, pacer=None):
            if row is None:
                row = res.shape[0] - cfg["link_back"]
            link[0] = _opaque_zero([res[row:row + 8, res.shape[1] - LANE:]])
            pace[0] = res if pacer is None else pacer

        def linked(x):
            return x if link[0] is None else _pin(x, link[0])

        def paced(w):
            res = pace[0]
            if res is None or link[0] is None or not cfg["pace_step"]:
                return w
            rows = []
            r0, step = cfg["pace_row"], cfg["pace_step"]
            if res.shape[0] < 400:
                r0, step = 0, 8
            if res.shape[0] < 200:
                return w
            zs = [_opaque_zero([res[r:r + 8, res.shape[1] - LANE:]])
                  for r in range(r0, r0 + 8 * step, step)]
            for r in range(0, w.shape[0], 8):
                z = zs[7 - (r // 8) % 8]
                t = pltpu.bitcast(w[r:r + 8, :], jnp.int32)
                rows.append(pltpu.bitcast(t + _lanecat([z] * (w.shape[1] // LANE)), U32))
            return _rowcat(rows)

        for cp in small:
            cp.start()
        x_copy(0).start()
        for cp in wq_copies(0):
            cp.start()

        bi = lax.broadcasted_iota(jnp.int32, (LANE, LANE), 0)
        mi = lax.broadcasted_iota(jnp.int32, (LANE, LANE), 1)
        ph = ((4 * mi + 1) * bi) & 511
        ang = ph.astype(F32) * (2.0 * 3.141592653589793 / 512.0)
        f_v[:, 0:LANE] = _u32(jnp.cos(ang).astype(BF16))
        f_v[:, LANE:] = _u32((-jnp.sin(ang)).astype(BF16))

        rb_t[...] = jnp.zeros((S // D, M, D), F32)
        ra_t[:, 0:LANE, :] = jnp.zeros((2, LANE, S // 2), F32)
        ra_t[:, AT * LANE:, :] = jnp.zeros((2, M - AT * LANE, S // 2), F32)

        for kt in range(1, KT):
            for cp in wq_copies(kt):
                cp.start()
        with jax.named_scope("small_wait"):
            for cp in small:
                cp.wait()
        sh = sh_v[...].astype(F32)
        for j in range(KS):
            par_v[j] = jnp.broadcast_to(sh[j:j + 1, :], (LANE, M)).T
        dd = dd_v[...].astype(F32).reshape(1, M)
        par_v[KS] = jnp.broadcast_to(dd, (LANE, M)).T

        def x_transpose(i):
            xt = xt_v[:, pl.ds(i * x_cols, x_cols)]
            xt = _rowcat([xt, jnp.zeros((MP // 2 - M // 2, x_cols), U32)])
            x_v[_h(i * x_cols, x_cols), :] = _u32(_bf(xt).astype(F32).T.astype(BF16))

        def q_early(kt, keep=False):
            first, last = kt == 0, kt == KT - 1
            n = wq_pairs(kt)
            cols = pl.ds(kt * LANE, LANE)
            if not keep:
                link[0] = None
            for j in range(H // 2):
                ws = []
                for half in range(2):
                    ev, od = (wqs_v[kt][pl.ds((2 * par + half) * n * 8 + j, n, stride=8), :]
                              for par in range(2))
                    ws.append(_repack(ev, od))
                w = _lanecat([ws[0][0], ws[1][0], ws[0][1], ws[1][1]])
                if n < TP:
                    w = _rowcat([w, jnp.zeros((TP - n, 2 * D), U32)])
                wq_v[j, pl.ds(kt * TP, TP), :] = w
                d = _dot(_bf(linked(x_v[_h(0, x_cols), cols])), _bf(w))
                set_link(d)
                if not first:
                    d = d + pltpu.bitcast(qacc[j], F32)
                if last:
                    d = (d * (D ** -0.5 * LOG2E)).astype(BF16)
                    for t in range(2):
                        q_all[2 * j + t, _h(0, x_cols), :] = _u32(d[:, t * D:(t + 1) * D])
                else:
                    qacc[j] = pltpu.bitcast(d, U32)

        with jax.named_scope("x_wait"):
            x_copy(0).wait()
        x_transpose(0)
        for i in range(1, XC):
            x_copy(i).start()
        for g in range(QIT):
            for cp in c_copies(g) + w_copies(g):
                cp.start()
        wo_copy.start()
        a_start(0)
        a_start(1)
        with jax.named_scope("wq_wait"):
            wq_wait(0)
        q_early(0)
        with jax.named_scope("wq_wait"):
            wq_wait(1)
            wq_wait(2)
        q_early(1)
        q_early(2, keep=True)
        with jax.named_scope("wq_wait"):
            wq_wait(3)
            for i in range(1, XC):
                x_copy(i).wait()
        q_early(3)
        for i in range(1, XC):
            x_transpose(i)

        def unpack(g, sub, j):
            ev, od = (ws_v[g, pl.ds((par * (C // 2) + sub * TP) * 8 + j, TP, stride=8), :]
                      for par in range(2))
            lo, hi = _repack(ev, od)
            rows = pl.ds(sub * TP, TP)
            cols = pl.ds(pl.multiple_of(g * LANE, LANE), LANE)
            wkv_v[2 * j, rows, cols] = lo
            wkv_v[2 * j + 1, rows, cols] = hi
            return [lo, hi]

        def a_sums(it, u):
            r0 = pl.multiple_of(it * CP + 8 * u, 8)
            kw = C // 2
            a11, a12, a21, a22 = (
                _split(c_v[pl.ds(r0 + rb * (S // 4), 8), pl.ds(cb * kw, kw)])
                for rb in range(2) for cb in range(2))
            outs = [_add(a11, a22), _add(a21, a22), _add(a11, a12), _sub(a21, a11),
                    _sub(a12, a22)]
            for k, o in enumerate(outs):
                sa_v[k, pl.ds(r0, 8), :] = o
            return outs

        units = [functools.partial(unpack, sub=s_, j=j_)
                 for s_ in range(C // 2 // TP) for j_ in range(H // 2)]
        for u_ in range(CP // 8):
            units.insert(5 * u_ + 4, functools.partial(a_sums, u=u_))

        def qproj(it, r0, n, t, zeros=(None, None)):
            outs = []
            for u in range(2):
                lhs = _bf(linked(x_v[_h(r0, n), :]))
                d = _dot(lhs, _bf(wq_v[it, :, pl.ds(t * D + u * LANE, LANE)]))
                set_link(d)
                if zeros[u] is not None:
                    for k, z in enumerate(zeros[u]):
                        d = _pin(d, z, 8 * ((k * (n // 8)) // len(zeros[u])))
                outs.append(d)
            q2 = _lanecat(outs)
            q_all[2 * it + t, _h(r0, n), :] = _u32((q2 * (D ** -0.5 * LOG2E)).astype(BF16))

        def q_body(it, carry):
            with jax.named_scope("w_wait"):
                w_wait(it)
                r0 = pl.multiple_of(it * CP, CP)
                for rs in (pl.ds(r0, CP), pl.ds(S // 4 + r0, CP)):
                    pltpu.make_async_copy(c_v.at[rs], c_v.at[rs], sem_c.at[it]).wait()
            link[0] = None
            pieces = [(p, pc, t) for p in range(QP) for pc in range(1, XC) for t in range(2)]
            nd = 2 * len(pieces)
            for k, (p, pc, t) in enumerate(pieces):
                zeros = []
                for u in range(2):
                    d = 2 * k + u
                    mine = units[d * len(units) // nd:(d + 1) * len(units) // nd]
                    zeros.append([_opaque_zero(u_(it)) for u_ in mine])
                qproj(QP * it + p, pc * x_cols, x_cols, t, zeros)
            return carry

        with jax.named_scope("q_loop"):
            lax.fori_loop(0, QIT, q_body, 0)
        wo_copy.wait()
        a_wait(0)

        tri = (lax.broadcasted_iota(jnp.int32, (LANE, LANE), 1)
               <= lax.broadcasted_iota(jnp.int32, (LANE, LANE), 0))

        NOUT = S // D

        def out_copy(i):
            if i >= NOUT:
                t = i - NOUT
                return pltpu.make_async_copy(
                    oa_v.at[t], out_hbm.at[:, pl.ds(t * LANE, LANE)], sem_out.at[i])
            rs = pl.ds(i * D, D)
            return pltpu.make_async_copy(
                out_v.at[rs], out_hbm.at[rs, pl.ds(AT * LANE, 2 * M - AT * LANE)], sem_out.at[i])

        n_body = NOUT - (tq // D if nq - 1 in cfg["o_str"] else 1)

        def b_out(k, tot):
            c0 = (k * D) % (S // 2)
            full = _rowcat([ra_t[k * D // (S // 2), AT * LANE:, c0:c0 + D], tot]).T
            out_v[k * D:(k + 1) * D, :] = full.astype(BF16)
            return full

        def head_step(h, carry):
            with jax.named_scope("step"):
                return head_step_(h, carry)

        def head_step_(h, carry):
            with_a = cfg["use_a"]

            @pl.when(h == A_STEPS)
            def _():
                for t in range(AT):
                    out_copy(NOUT + t).start()

            @pl.when(h == cfg["h0"] + 1)
            def _():
                a_wait(1)

            link[0] = None
            n2 = AR // 2
            a_rows2 = pl.ds(pl.multiple_of(jnp.minimum(h, A_STEPS - 1) * n2, n2), n2)
            a_rows = pl.ds(pl.multiple_of(jnp.minimum(h, A_STEPS - 1) * AR, AR), AR)

            kw = C // 2
            pending = []

            def flush_pending(x, row):
                done = list(pending)
                del pending[:]
                if not done:
                    return x
                x = _pin(x, _opaque_zero([f for _, f in done]), row)

                @pl.when(h == H - 1)
                def _():
                    for k, _f in done:
                        out_copy(k).start()
                return x

            def a_fwd():
                kk = _bf(a_v[0, a_rows2, :]).astype(F32)
                lane = lax.broadcasted_iota(jnp.int32, (AR, LANE), 1)
                coef = [par_v[j, a_rows, :] for j in range(KS)]
                rolled = [kk] + [pltpu.roll(kk, j, 1) for j in range(1, KS)]
                vv = _bf(a_v[1, a_rows2, :]).astype(F32)
                kv_blocks = []
                for a in range(NB):
                    cs = slice(a * LANE, (a + 1) * LANE)
                    acc = rolled[0][:, cs] * coef[0]
                    for j in range(1, KS):
                        t = rolled[j][:, cs]
                        if a == 0:
                            t = jnp.where(lane >= j, t, 0.0)
                        acc = acc + t * coef[j]
                    kv_blocks.append(acc * vv[:, cs])
                hk = a_v[2, a_rows2, :]
                hk = _rowcat([hk[:, a * LANE:(a + 1) * LANE] for a in range(NB)])
                fm = _bf(f_v[...])
                hs = _dot(_bf(linked(hk)), fm)
                kv = linked(_rowcat(kv_blocks)).astype(BF16)
                xs = _dot(kv, fm)
                set_link(xs)
                return kv, xs, hs

            def a_conv(xs, hs):
                def tile(v, a, g, part):
                    r = a * AR + 8 * g
                    return v[r:r + 8, part * LANE:(part + 1) * LANE]

                z = {}
                gate = None
                width = cfg["a_width"]
                for g in range(AR // 8):
                    hr = [tile(hs, 0, g, 0)] + [
                        tile(hs, j, g, 0) - tile(hs, j - 1, g, 1) for j in range(1, NB)]
                    hi = [tile(hs, 0, g, 1)] + [
                        tile(hs, j, g, 1) + tile(hs, j - 1, g, 0) for j in range(1, NB)]
                    for c0 in range(0, NB, width):
                        for a in range(c0 + width):
                            xr, xi = tile(xs, a, g, 0), tile(xs, a, g, 1)
                            if gate is not None:
                                xr, xi = _pin(xr, gate), _pin(xi, gate)
                            for c in range(max(c0, a), c0 + width):
                                j = c - a
                                tr = xr * hr[j] - xi * hi[j]
                                ti = xr * hi[j] + xi * hr[j]
                                z[c, g] = (tr, ti) if a == 0 else (z[c, g][0] + tr, z[c, g][1] + ti)
                            gate = _opaque_zero(list(z[c0 + width - 1, g]))
                return z

            def a_inv(kv, z, flush=False):
                fm = _bf(f_v[...])
                ng = AR // 8
                ys = []
                for u in range(2):
                    rows = [_lanecat(z[c, g]) for g in range(u * ng // 2, (u + 1) * ng // 2)
                            for c in range(NB)]
                    lhs = linked(_rowcat(rows))
                    if flush:
                        lhs = flush_pending(lhs, 8)
                    ys.append(_dot_nt(lhs.astype(BF16), fm))
                y = _rowcat(ys)
                dd = par_v[KS, a_rows, :]
                for c in range(NB):
                    cs = slice(c * LANE, (c + 1) * LANE)
                    yc = _rowcat([y[(g * NB + c) * 8:(g * NB + c + 1) * 8, :] for g in range(ng)])
                    qq = _bf(a_v[3, a_rows2, cs]).astype(F32)
                    kvf = kv[c * AR:(c + 1) * AR, :].astype(F32)
                    c2 = (c % (NB // 2)) * LANE
                    ra_t[c // (NB // 2), a_rows, c2:c2 + LANE] = qq * (yc * (1.0 / LANE) + kvf * dd)

            def a_out():
                slab = jnp.clip(h // 4 - 1, 0, AT - 1)
                half = h % 2
                x = ra_t[half, pl.ds(pl.multiple_of(slab * LANE, LANE), LANE), :]
                xt = x.T
                dst = jnp.where(h >= A_STEPS, AT, slab)
                oa_v[dst, pl.ds(pl.multiple_of(half * (S // 2), S // 2), S // 2), :] = xt.astype(BF16)
                return xt

            def w_blk(r, c):
                return wkv_v[h, _h(r * kw, kw), pl.ds(c * LANE, LANE)]

            def one_pass(lhs, w, flush):
                lhs = linked(lhs)
                if flush:
                    lhs = flush_pending(lhs, cfg["ao_row"])
                d = _dot(_bf(lhs), _bf(paced(w)))
                set_link(d)
                return d

            def k_proj(blk, flush=-1):
                ds = [one_pass(c_v[_h(blk * tq, tq), pl.ds((k % 2) * kw, kw)],
                               w_blk(k % 2, k // 2), k == flush) for k in range(4)]
                k_s[_h(blk * tq, tq), :] = _u32(
                    _lanecat([ds[0] + ds[1], ds[2] + ds[3]]).astype(BF16))

            def b_op(m):
                blk = lambda r, c: _split(w_blk(r, 2 + c))
                return {1: lambda: _add(blk(0, 0), blk(1, 1)),
                        2: lambda: w_blk(0, 2),
                        3: lambda: _sub(blk(0, 1), blk(1, 1)),
                        4: lambda: _sub(blk(1, 0), blk(0, 0)),
                        5: lambda: w_blk(1, 3),
                        6: lambda: _add(blk(0, 0), blk(0, 1)),
                        7: lambda: _add(blk(1, 0), blk(1, 1))}[m]()

            def a_op(m, rho):
                rs = _h(rho * tq, tq)
                if m == 3:
                    return c_v[rs, 0:kw]
                if m == 4:
                    return c_v[_h(S // 2 + rho * tq, tq), kw:]
                return sa_v[{1: 0, 2: 1, 5: 2, 6: 3, 7: 4}[m], rs, :]

            b_cache, prod = {}, {}

            def v_proj(blk, flush=-1):
                rho = blk % 2
                for k, m in enumerate((5, 1, 4, 7, 3) if blk < 2 else (2, 6)):
                    if m not in b_cache:
                        b_cache[m] = b_op(m)
                    prod[m, rho] = one_pass(a_op(m, rho), b_cache[m], k == flush)
                p = lambda m: prod[m, rho]
                if blk < 2:
                    v = [(p(1) + p(4)) + (p(7) - p(5)), p(3) + p(5)]
                else:
                    v = [p(2) + p(4), (p(1) + p(3)) + (p(6) - p(2))]
                v_s[_h(blk * tq, tq), :] = _u32(_lanecat(v).astype(BF16))

            def qk(i, dep=None, flush=False):
                r0 = i * tq
                q = linked(q_all[h, _h(r0, tq), :])
                if dep is not None:
                    q = _pin(q, _opaque_zero([dep]), cfg["ao_row"])
                if flush:
                    q = flush_pending(q, cfg["ao_row"] - 8)
                parts = [_dot_nt(_bf(q), _bf(k_s[_h(0, r0 + LANE), :]))]
                if i > 0:
                    link[0] = _opaque_zero([parts[0][0:8, r0 - LANE:r0]])
                for j in range(1, nsub):
                    q = linked(q_all[h, _h(r0 + LANE * j, tq - LANE * j), :])
                    parts.append(_dot_nt(_bf(q), _bf(k_s[_h(r0 + LANE * j, LANE), :])))
                set_link(parts[2], cfg["link_part"], parts[0])
                return parts

            def softmax(i, parts):
                pb = p_s.at[i % 2]
                chain = _opaque_zero([b[b.shape[0] - 8:, b.shape[1] - LANE:] for b in parts])
                ls = []
                for a in range(nsub):
                    blocks = [parts[j][LANE * (a - j):LANE * (a - j + 1), :] for j in range(a + 1)]
                    last = blocks[-1]
                    w = last.shape[1]
                    dg = jnp.where(tri, last[:, w - LANE:], NEG)
                    blocks[-1] = dg if w == LANE else _lanecat([last[:, :w - LANE], dg])
                    sa = _lanecat(blocks)
                    mb = jnp.broadcast_to(jnp.max(sa, axis=1, keepdims=True), (LANE, LANE))
                    nt = sa.shape[1] // LANE
                    ptiles, psums = [], []
                    for g in range(0, LANE, 8):
                        mg = _pin(mb[g:g + 8, :], chain)
                        pg = [jnp.exp2(sa[g:g + 8, t * LANE:(t + 1) * LANE] - mg) for t in range(nt)]
                        ps = functools.reduce(jnp.add, pg)
                        chain = _opaque_zero([ps])
                        psums.append(ps)
                        ptiles.append(_lanecat(pg))
                    ls.append(jnp.sum(_rowcat(psums), axis=1, keepdims=True))
                    p = _pin(_rowcat(ptiles), link[0], 0, 0 if a == 0 else sa.shape[1] - LANE)
                    pb[LANE * a:LANE * (a + 1), 0:sa.shape[1]] = p.astype(BF16)
                return ls

            def pv(i, ls):
                r0 = i * tq
                pb = p_s.at[i % 2]
                ctx = [_dot(pb[:, 0:r0 + LANE], _bf(v_s[_h(0, r0 + LANE), :]))]
                for j in range(1, nsub):
                    c0 = r0 + LANE * j
                    ctx.append(_dot(pb[LANE * j:, c0:c0 + LANE], _bf(v_s[_h(c0, LANE), :])))
                set_link(ctx[2], cfg["link_part"], ctx[0])
                cs = []
                for a in range(nsub):
                    sl = lambda j: slice(LANE * (a - j), LANE * (a - j + 1))
                    r = pl.reciprocal(ls[a], approx=True)
                    r = r * (2.0 - ls[a] * r)
                    cs.append(functools.reduce(jnp.add, [ctx[j][sl(j)] for j in range(a + 1)]) * r)
                return _rowcat(cs)

            def accumulate(k, res):
                tot = rb_t[k] + res
                rb_t[k] = tot
                if k < n_body:
                    pending.append((k, b_out(k, tot)))

            def oproj_plain(i, ctx):
                ctx = ctx.astype(BF16)
                for u in range(tq // D):
                    lhs = linked(wo_v[h])
                    if i == nq - 1:
                        lhs = flush_pending(lhs, cfg["last_row"])
                    res = _dot_nt(_bf(lhs), ctx[u * D:(u + 1) * D, :])
                    set_link(res)
                    accumulate(i * (tq // D) + u, res)

            wo_cache = {}

            def oproj(i, ctx):
                if i not in cfg["o_str"]:
                    return oproj_plain(i, ctx)
                mh = M // 4
                raw = lambda r, c: wo_v[h, r * mh:(r + 1) * mh, c * LANE:(c + 1) * LANE]
                a = lambda r, c: _split(raw(r, c))
                a_ops = {1: lambda: _add(a(0, 0), a(1, 1)), 2: lambda: _add(a(1, 0), a(1, 1)),
                         3: lambda: raw(0, 0), 4: lambda: raw(1, 1),
                         5: lambda: _add(a(0, 0), a(0, 1)), 6: lambda: _sub(a(1, 0), a(0, 0)),
                         7: lambda: _sub(a(0, 1), a(1, 1))}
                b = lambda r, c: ctx[c * D:(c + 1) * D, r * LANE:(r + 1) * LANE]
                b_ops = {1: lambda: b(0, 0) + b(1, 1), 2: lambda: b(0, 0),
                         3: lambda: b(0, 1) - b(1, 1), 4: lambda: b(1, 0) - b(0, 0),
                         5: lambda: b(1, 1), 6: lambda: b(0, 0) + b(0, 1),
                         7: lambda: b(1, 0) + b(1, 1)}
                p = {}
                for n, m in enumerate((5, 2, 4, 1, 7, 3, 6)):
                    if m not in wo_cache:
                        wo_cache[m] = a_ops[m]()
                    rhs = b_ops[m]().astype(BF16)
                    if n == cfg["o_half"]:
                        halves = [_dot_nt(_bf(linked(wo_cache[m][r:r + mh // 2])), rhs)
                                  for r in (0, mh // 2)]
                        p[m] = _rowcat(halves)
                        set_link(halves[1], 0)
                    else:
                        p[m] = _dot_nt(_bf(linked(wo_cache[m])), rhs)
                        if (n - (n > cfg["o_half"])) % 2 == 1:
                            set_link(p[m], cfg["o_link"])
                accumulate(2 * i, _rowcat([(p[1] + p[4]) + (p[7] - p[5]), p[2] + p[4]]))
                accumulate(2 * i + 1, _rowcat([p[3] + p[5], (p[1] + p[3]) + (p[6] - p[2])]))

            st = {}
            for op in cfg["seq"].split():
                op, _, fl = op.partition("!")
                fl = int(fl) if fl else -1
                kind, i = op[0], int(op[1:] or 0)
                if kind == "K":
                    k_proj(i, fl)
                elif kind == "V":
                    v_proj(i, fl)
                elif kind == "Q":
                    st["s", i] = qk(i, a_out() if i == cfg["ao_at"] else None, fl >= 0)
                elif kind == "P":
                    st["ctx", i] = pv(i, softmax(i, st["s", i]))
                elif kind == "O":
                    oproj(i, st["ctx", i])
                elif kind == "F" and with_a:
                    st["kv"], xs, hs = a_fwd()
                    st["z"] = a_conv(xs, hs)
                elif kind == "I" and with_a:
                    a_inv(st["kv"], st["z"], fl >= 0)
            assert not pending
            return carry

        with jax.named_scope("loop_a"):
            lax.fori_loop(cfg["h0"], H, head_step, 0)
        with jax.named_scope("tail"):
            for i in range(n_body, NOUT):
                b_out(i, rb_t[i])
                out_copy(i).start()
            for i in range(NOUT + AT):
                out_copy(i).wait()

    scratch = [
        pltpu.VMEM((4, M // 2, S), U32),
        pltpu.VMEM((KS, M), BF16),
        pltpu.VMEM((M,), BF16),
        pltpu.VMEM((KS + 1, M, LANE), F32),
        pltpu.VMEM((LANE // 2, 2 * LANE), U32),
        pltpu.VMEM((M // 2, S), U32),
        pltpu.VMEM((S // 2, MP), U32),
        pltpu.VMEM((S // 2, C), U32),
        [pltpu.VMEM((4 * min(TP, M // 2 - kt * TP) * 8, LANE), U32)
         for kt in range(KT)],
        pltpu.VMEM((H // 2, MP // 2, 2 * D), U32),
        pltpu.VMEM((H // 2, x_cols, 2 * D), U32),
        pltpu.VMEM((QIT, C * 8, LANE), U32),
        pltpu.VMEM((H, C // 2, 2 * D), U32),
        pltpu.VMEM((H, M // 2, D), U32),
        pltpu.VMEM((H, S // 2, D), U32),
        pltpu.VMEM((S // 2, D), U32),
        pltpu.VMEM((S // 2, D), U32),
        pltpu.VMEM((2, tq, S), BF16),
        pltpu.VMEM((2, M, S // 2), F32),
        pltpu.VMEM((S // D, M, D), F32),
        pltpu.VMEM((AT + 1, S, LANE), BF16),
        pltpu.VMEM((S, 2 * M - AT * LANE), BF16),
        pltpu.SemaphoreType.DMA((XC,)),
        pltpu.SemaphoreType.DMA((KT,)),
        pltpu.SemaphoreType.DMA((QIT,)),
        pltpu.SemaphoreType.DMA((QIT,)),
        pltpu.SemaphoreType.DMA((2,)),
        pltpu.SemaphoreType.DMA((3,)),
        pltpu.SemaphoreType.DMA((S // D + AT,)),
    ]
    return kernel, scratch


_DEFAULT = dict(
    tq=512, a_width=4, ao_at=1, ao_row=240, link_back=176, link_part=32, pace_row=32,
    pace_step=24, use_a=1, h0=0, last_row=216, o_str=(0, 1, 2, 3), o_link=48, o_half=6,
    seq="K0 Q0 K1 Q1 V0 F P0 K2 Q2 O0 V1!2 P1 K3 Q3 O1 V2!1 P2 V3 O2 P3 I!0 O3")


def _build(**kw):
    cfg = dict(_DEFAULT)
    cfg.update(kw)
    kernel, scratch = _make_kernel(cfg)

    def run(A_q, A_k, A_v, A_shift_k, A_ssm_k, A_ssm_D, B_x, B_c_kv, B_w_q, B_w_uk,
            B_w_uv, B_w_o):
        tr = lambda a: jnp.swapaxes(a, 1, 2).reshape(M, S)
        args = (
            tr(A_q), tr(A_k), tr(A_v), A_shift_k.T, A_ssm_k, A_ssm_D, tr(B_x),
            B_c_kv.reshape(S, C),
            B_w_q.reshape(M // 2, 2 * H, D), B_w_uk.reshape(C // 2, 2 * H, D),
            B_w_uv.reshape(C // 2, 2 * H, D),
            jnp.swapaxes(B_w_o, 1, 2),
        )
        out = pl.pallas_call(
            kernel,
            in_specs=[pl.BlockSpec(memory_space=pl.ANY)] * len(args),
            out_specs=pl.BlockSpec(memory_space=pl.ANY),
            out_shape=jax.ShapeDtypeStruct((S, 2 * M), BF16),
            scratch_shapes=scratch,
            compiler_params=pltpu.CompilerParams(
                vmem_limit_bytes=120 * 1024 * 1024,
                disable_bounds_checks=True),
        )(*args)
        return out.reshape(1, S, 2 * M)

    return run


_run = _build()


@jax.jit
def pallas_concat_heads__ssm_conv_h3__compressed_kv_cla__prompt_kernel(
    A_q: jax.Array,
    A_k: jax.Array,
    A_v: jax.Array,
    A_shift_k: jax.Array,
    A_ssm_k: jax.Array,
    A_ssm_D: jax.Array,
    B_x: jax.Array,
    B_c_kv: jax.Array,
    B_w_q: jax.Array,
    B_w_uk: jax.Array,
    B_w_uv: jax.Array,
    B_w_o: jax.Array,
):
    return _run(A_q, A_k, A_v, A_shift_k, A_ssm_k, A_ssm_D, B_x, B_c_kv, B_w_q,
                B_w_uk, B_w_uv, B_w_o)
```

```python
import functools

import jax
import jax.numpy as jnp
from jax import lax
import jax.experimental.pallas as pl
import jax.experimental.pallas.tpu as pltpu

F32 = jnp.float32
BF16 = jnp.bfloat16
U32 = jnp.uint32

S = 2048
M = 448
MP = 512
C = 1024
H = 16
D = 256
KS = 4
LANE = 128
NB = S // LANE
AR = 32
A_STEPS = M // AR
LOG2E = 1.4426950408889634
NEG = -1e30

NT = (((1,), (1,)), ((), ()))


def _dot(a, b):
    return jnp.dot(a, b, preferred_element_type=F32)


def _dot_nt(a, b):
    return lax.dot_general(a, b, NT, preferred_element_type=F32)


def _bf(x):
    return pltpu.bitcast(x, BF16)


def _u32(x):
    return pltpu.bitcast(x, U32)


def _h(r0, n):
    return pl.ds(r0 // 2, n // 2)


def _repack(ev, od):
    lo = (ev & jnp.uint32(0xFFFF)) | (od << 16)
    hi = (ev >> 16) | (od & jnp.uint32(0xFFFF0000))
    return lo, hi


def _split(w):
    return (pltpu.bitcast(w << 16, F32), pltpu.bitcast(w & jnp.uint32(0xFFFF0000), F32))


def _join(lo, hi):
    half = jnp.uint32(0x8000)
    lo = (pltpu.bitcast(lo, U32) + half) >> 16
    hi = (pltpu.bitcast(hi, U32) + half) & jnp.uint32(0xFFFF0000)
    return lo | hi


def _add(a, b):
    return _join(a[0] + b[0], a[1] + b[1])


def _sub(a, b):
    return _join(a[0] - b[0], a[1] - b[1])


def _opaque_zero(vals):
    acc = None
    for v in vals:
        b = v if v.dtype == U32 else pltpu.bitcast(v, U32)
        for r in range(0, b.shape[0], 8):
            for c in range(0, b.shape[1], LANE):
                t = b[r:r + 8, c:c + LANE]
                acc = t if acc is None else acc | t
    return jnp.minimum((acc >> 1).astype(jnp.int32), 0)


def _pin(x, zero, r=0, c=0):
    t = pltpu.bitcast(pltpu.bitcast(x[r:r + 8, c:c + LANE], jnp.int32) + zero, x.dtype)
    row = ([x[r:r + 8, :c]] if c > 0 else []) + [t] + (
        [x[r:r + 8, c + LANE:]] if c + LANE < x.shape[1] else [])
    row = jnp.concatenate(row, axis=1) if len(row) > 1 else row[0]
    col = ([x[:r, :]] if r > 0 else []) + [row] + ([x[r + 8:, :]] if r + 8 < x.shape[0] else [])
    return jnp.concatenate(col, axis=0) if len(col) > 1 else col[0]


def _rowcat(xs):
    return jnp.concatenate(xs, axis=0) if len(xs) > 1 else xs[0]


def _lanecat(xs):
    return jnp.concatenate(xs, axis=1) if len(xs) > 1 else xs[0]


def _make_kernel(cfg):
    tq = cfg["tq"]
    nq = S // tq
    nsub = tq // LANE
    KT = MP // LANE
    TP = LANE // 2
    XC = 4
    x_cols = S // XC
    QP = 2
    QIT = H // 2 // QP
    AT = 3

    def kernel(aq_hbm, ak_hbm, av_hbm, sh_hbm, ssm_hbm, dd_hbm, x_hbm, c_hbm,
               wq_hbm, wk_hbm, wv_hbm, wo_hbm,
               out_hbm,
               a_v, sh_v, dd_v, par_v, f_v,
               xt_v, x_v, c_v, wqs_v, wq_v, qacc, ws_v, wkv_v, wo_v,
               q_all, k_s, v_s, p_s, ra_t, rb_t, oa_v, out_v,
               sem_x, sem_wq, sem_w, sem_c, sem_s, sem_a, sem_out):
        x32, c32, wq32, wk32, wv32, wo32 = (
            r.bitcast(U32) for r in (x_hbm, c_hbm, wq_hbm, wk_hbm, wv_hbm, wo_hbm))
        a32 = [r.bitcast(U32) for r in (ak_hbm, av_hbm, ssm_hbm, aq_hbm)]

        sa_v = qacc

        def x_copy(i):
            cs = pl.ds(i * x_cols, x_cols)
            return pltpu.make_async_copy(x32.at[:, cs], xt_v.at[:, cs], sem_x.at[i])

        def wq_pairs(kt):
            return min(TP, M // 2 - kt * TP)

        def wq_copies(kt):
            n = wq_pairs(kt)
            dst = wqs_v[kt].reshape(4, n, 8, LANE)
            return [pltpu.make_async_copy(
                wq32.at[pl.ds(kt * TP, n), pl.ds(8 * (k // 2), 8), pl.ds((k % 2) * LANE, LANE)],
                dst.at[k], sem_wq.at[kt]) for k in range(4)]

        def wq_wait(kt):
            pltpu.make_async_copy(wqs_v[kt], wqs_v[kt], sem_wq.at[kt]).wait()

        def w_copies(g):
            dst = ws_v.reshape(8, C // 2, 8, LANE)
            src = (wk32, wv32)[g // 2]
            return [pltpu.make_async_copy(
                src.at[:, pl.ds(8 * par, 8), pl.ds((g % 2) * LANE, LANE)],
                dst.at[2 * g + par], sem_w.at[g]) for par in range(2)]

        def w_wait(g):
            pltpu.make_async_copy(ws_v.at[g], ws_v.at[g], sem_w.at[g]).wait()

        CP = S // 4 // QIT

        def c_copies(p):
            r0 = p * CP
            return [pltpu.make_async_copy(c32.at[rs], c_v.at[rs], sem_c.at[p])
                    for rs in (pl.ds(r0, CP), pl.ds(S // 4 + r0, CP))]

        wo_copy = pltpu.make_async_copy(wo32, wo_v, sem_a.at[0])

        a_parts = [pl.ds(0, AR // 2), pl.ds(AR // 2, M // 2 - AR // 2)]

        def a_start(part):
            rs = a_parts[part]
            for k in range(4):
                pltpu.make_async_copy(
                    a32[k].at[rs], a_v.at[k, rs], sem_a.at[1 + part]).start()

        def a_wait(part):
            view = a_v.at[:, a_parts[part]]
            pltpu.make_async_copy(view, view, sem_a.at[1 + part]).wait()

        small = [pltpu.make_async_copy(sh_hbm, sh_v, sem_s.at[0]),
                 pltpu.make_async_copy(dd_hbm, dd_v, sem_s.at[1])]

        link = [None]
        pace = [None]

        def set_link(res, row=None, pacer=None):
            if row is None:
                row = res.shape[0] - cfg["link_back"]
            link[0] = _opaque_zero([res[row:row + 8, res.shape[1] - LANE:]])
            pace[0] = res if pacer is None else pacer

        def linked(x):
            return x if link[0] is None else _pin(x, link[0])

        def paced(w):
            res = pace[0]
            if res is None or link[0] is None or not cfg["pace_step"]:
                return w
            rows = []
            r0, step = cfg["pace_row"], cfg["pace_step"]
            if res.shape[0] < 400:
                r0, step = 0, 8
            if res.shape[0] < 200:
                return w
            zs = [_opaque_zero([res[r:r + 8, res.shape[1] - LANE:]])
                  for r in range(r0, r0 + 8 * step, step)]
            for r in range(0, w.shape[0], 8):
                z = zs[7 - (r // 8) % 8]
                t = pltpu.bitcast(w[r:r + 8, :], jnp.int32)
                rows.append(pltpu.bitcast(t + _lanecat([z] * (w.shape[1] // LANE)), U32))
            return _rowcat(rows)

        for cp in small:
            cp.start()
        x_copy(0).start()
        for cp in wq_copies(0):
            cp.start()

        def dft_body(k, carry):
            n = 32
            bi = lax.broadcasted_iota(jnp.int32, (n, LANE), 0) + k * n
            mi = lax.broadcasted_iota(jnp.int32, (n, LANE), 1)
            ph = ((4 * mi + 1) * bi) & 511
            ang = ph.astype(F32) * (2.0 * 3.141592653589793 / 512.0)
            rs = pl.ds(pl.multiple_of(k * (n // 2), n // 2), n // 2)
            f_v[rs, 0:LANE] = _u32(jnp.cos(ang).astype(BF16))
            f_v[rs, LANE:] = _u32((-jnp.sin(ang)).astype(BF16))
            return carry

        lax.fori_loop(0, 4, dft_body, 0)

        def zero_body(k, carry):
            rb_t[k] = jnp.zeros((M, D), F32)
            cs = pl.ds(pl.multiple_of((k % 4) * D, D), D)
            ra_t[k // 4, 0:LANE, cs] = jnp.zeros((LANE, D), F32)
            ra_t[k // 4, AT * LANE:, cs] = jnp.zeros((M - AT * LANE, D), F32)
            return carry

        lax.fori_loop(0, S // D, zero_body, 0)

        for kt in range(1, KT):
            for cp in wq_copies(kt):
                cp.start()
        with jax.named_scope("small_wait"):
            for cp in small:
                cp.wait()
        sh = sh_v[...].astype(F32)
        for j in range(KS):
            par_v[j] = jnp.broadcast_to(sh[j:j + 1, :], (LANE, M)).T
        dd = dd_v[...].astype(F32).reshape(1, M)
        par_v[KS] = jnp.broadcast_to(dd, (LANE, M)).T

        def x_transpose(i):
            xt = xt_v[:, pl.ds(i * x_cols, x_cols)]
            xt = _rowcat([xt, jnp.zeros((MP // 2 - M // 2, x_cols), U32)])
            x_v[_h(i * x_cols, x_cols), :] = _u32(_bf(xt).astype(F32).T.astype(BF16))

        def q_early(kt, keep=False):
            first, last = kt == 0, kt == KT - 1
            n = wq_pairs(kt)
            cols = pl.ds(kt * LANE, LANE)
            if not keep:
                link[0] = None
            for j in range(H // 2):
                ws = []
                for half in range(2):
                    ev, od = (wqs_v[kt][pl.ds((2 * par + half) * n * 8 + j, n, stride=8), :]
                              for par in range(2))
                    ws.append(_repack(ev, od))
                w = _lanecat([ws[0][0], ws[1][0], ws[0][1], ws[1][1]])
                if n < TP:
                    w = _rowcat([w, jnp.zeros((TP - n, 2 * D), U32)])
                wq_v[j, pl.ds(kt * TP, TP), :] = w
                d = _dot(_bf(linked(x_v[_h(0, x_cols), cols])), _bf(w))
                set_link(d)
                if not first:
                    d = d + pltpu.bitcast(qacc[j], F32)
                if last:
                    d = (d * (D ** -0.5 * LOG2E)).astype(BF16)
                    for t in range(2):
                        q_all[2 * j + t, _h(0, x_cols), :] = _u32(d[:, t * D:(t + 1) * D])
                else:
                    qacc[j] = pltpu.bitcast(d, U32)

        with jax.named_scope("x_wait"):
            x_copy(0).wait()
        x_transpose(0)
        for i in range(1, XC):
            x_copy(i).start()
        for g in range(QIT):
            for cp in c_copies(g) + w_copies(g):
                cp.start()
        wo_copy.start()
        a_start(0)
        a_start(1)
        with jax.named_scope("wq_wait"):
            wq_wait(0)
        q_early(0)
        with jax.named_scope("wq_wait"):
            wq_wait(1)
            wq_wait(2)
        q_early(1)
        q_early(2, keep=True)
        with jax.named_scope("wq_wait"):
            wq_wait(3)
            for i in range(1, XC):
                x_copy(i).wait()
        q_early(3)
        for i in range(1, XC):
            x_transpose(i)

        def unpack(g, sub, j):
            ev, od = (ws_v[g, pl.ds((par * (C // 2) + sub * TP) * 8 + j, TP, stride=8), :]
                      for par in range(2))
            lo, hi = _repack(ev, od)
            rows = pl.ds(sub * TP, TP)
            cols = pl.ds(pl.multiple_of(g * LANE, LANE), LANE)
            wkv_v[2 * j, rows, cols] = lo
            wkv_v[2 * j + 1, rows, cols] = hi
            return [lo, hi]

        def a_sums(it, u):
            r0 = pl.multiple_of(it * CP + 8 * u, 8)
            kw = C // 2
            a11, a12, a21, a22 = (
                _split(c_v[pl.ds(r0 + rb * (S // 4), 8), pl.ds(cb * kw, kw)])
                for rb in range(2) for cb in range(2))
            outs = [_add(a11, a22), _add(a21, a22), _add(a11, a12), _sub(a21, a11),
                    _sub(a12, a22)]
            for k, o in enumerate(outs):
                sa_v[k, pl.ds(r0, 8), :] = o
            return outs

        units = [functools.partial(unpack, sub=s_, j=j_)
                 for s_ in range(C // 2 // TP) for j_ in range(H // 2)]
        for u_ in range(CP // 8):
            units.insert(5 * u_ + 4, functools.partial(a_sums, u=u_))

        def qproj(it, r0, n, t, zeros=(None, None)):
            outs = []
            for u in range(2):
                lhs = _bf(linked(x_v[_h(r0, n), :]))
                d = _dot(lhs, _bf(wq_v[it, :, pl.ds(t * D + u * LANE, LANE)]))
                set_link(d)
                if zeros[u] is not None:
                    for k, z in enumerate(zeros[u]):
                        d = _pin(d, z, 8 * ((k * (n // 8)) // len(zeros[u])))
                outs.append(d)
            q2 = _lanecat(outs)
            q_all[2 * it + t, _h(r0, n), :] = _u32((q2 * (D ** -0.5 * LOG2E)).astype(BF16))

        def q_body(it, carry):
            with jax.named_scope("w_wait"):
                w_wait(it)
                r0 = pl.multiple_of(it * CP, CP)
                for rs in (pl.ds(r0, CP), pl.ds(S // 4 + r0, CP)):
                    pltpu.make_async_copy(c_v.at[rs], c_v.at[rs], sem_c.at[it]).wait()
            link[0] = None
            pieces = [(p, pc, t) for p in range(QP) for pc in range(1, XC) for t in range(2)]
            nd = 2 * len(pieces)
            for k, (p, pc, t) in enumerate(pieces):
                zeros = []
                for u in range(2):
                    d = 2 * k + u
                    mine = units[d * len(units) // nd:(d + 1) * len(units) // nd]
                    zeros.append([_opaque_zero(u_(it)) for u_ in mine])
                qproj(QP * it + p, pc * x_cols, x_cols, t, zeros)
            return carry

        with jax.named_scope("q_loop"):
            lax.fori_loop(0, QIT, q_body, 0)
        wo_copy.wait()
        a_wait(0)

        tri = (lax.broadcasted_iota(jnp.int32, (LANE, LANE), 1)
               <= lax.broadcasted_iota(jnp.int32, (LANE, LANE), 0))

        NOUT = S // D

        def out_copy(i):
            if i >= NOUT:
                t = i - NOUT
                return pltpu.make_async_copy(
                    oa_v.at[t], out_hbm.at[:, pl.ds(t * LANE, LANE)], sem_out.at[i])
            rs = pl.ds(i * D, D)
            return pltpu.make_async_copy(
                out_v.at[rs], out_hbm.at[rs, pl.ds(AT * LANE, 2 * M - AT * LANE)], sem_out.at[i])

        n_body = NOUT - (tq // D if nq - 1 in cfg["o_str"] else 1)

        def b_out(k, tot):
            c0 = (k * D) % (S // 2)
            full = _rowcat([ra_t[k * D // (S // 2), AT * LANE:, c0:c0 + D], tot]).T
            out_v[k * D:(k + 1) * D, :] = full.astype(BF16)
            return full

        def head_step(h, carry):
            with jax.named_scope("step"):
                return head_step_(h, carry)

        def head_step_(h, carry):
            with_a = cfg["use_a"]

            @pl.when(h == A_STEPS)
            def _():
                for t in range(AT):
                    out_copy(NOUT + t).start()

            @pl.when(h == cfg["h0"] + 1)
            def _():
                a_wait(1)

            link[0] = None
            n2 = AR // 2
            a_rows2 = pl.ds(pl.multiple_of(jnp.minimum(h, A_STEPS - 1) * n2, n2), n2)
            a_rows = pl.ds(pl.multiple_of(jnp.minimum(h, A_STEPS - 1) * AR, AR), AR)

            kw = C // 2
            pending = []

            def flush_pending(x, row):
                done = list(pending)
                del pending[:]
                if not done:
                    return x
                x = _pin(x, _opaque_zero([f for _, f in done]), row)

                @pl.when(h == H - 1)
                def _():
                    for k, _f in done:
                        out_copy(k).start()
                return x

            def a_fwd():
                kk = _bf(a_v[0, a_rows2, :]).astype(F32)
                lane = lax.broadcasted_iota(jnp.int32, (AR, LANE), 1)
                coef = [par_v[j, a_rows, :] for j in range(KS)]
                rolled = [kk] + [pltpu.roll(kk, j, 1) for j in range(1, KS)]
                vv = _bf(a_v[1, a_rows2, :]).astype(F32)
                kv_blocks = []
                for a in range(NB):
                    cs = slice(a * LANE, (a + 1) * LANE)
                    acc = rolled[0][:, cs] * coef[0]
                    for j in range(1, KS):
                        t = rolled[j][:, cs]
                        if a == 0:
                            t = jnp.where(lane >= j, t, 0.0)
                        acc = acc + t * coef[j]
                    kv_blocks.append(acc * vv[:, cs])
                hk = a_v[2, a_rows2, :]
                hk = _rowcat([hk[:, a * LANE:(a + 1) * LANE] for a in range(NB)])
                fm = _bf(f_v[...])
                hs = _dot(_bf(linked(hk)), fm)
                kv = linked(_rowcat(kv_blocks)).astype(BF16)
                xs = _dot(kv, fm)
                set_link(xs)
                return kv, xs, hs

            def a_conv(xs, hs):
                def tile(v, a, g, part):
                    r = a * AR + 8 * g
                    return v[r:r + 8, part * LANE:(part + 1) * LANE]

                z = {}
                gate = None
                width = cfg["a_width"]
                for g in range(AR // 8):
                    hr = [tile(hs, 0, g, 0)] + [
                        tile(hs, j, g, 0) - tile(hs, j - 1, g, 1) for j in range(1, NB)]
                    hi = [tile(hs, 0, g, 1)] + [
                        tile(hs, j, g, 1) + tile(hs, j - 1, g, 0) for j in range(1, NB)]
                    for c0 in range(0, NB, width):
                        for a in range(c0 + width):
                            xr, xi = tile(xs, a, g, 0), tile(xs, a, g, 1)
                            if gate is not None:
                                xr, xi = _pin(xr, gate), _pin(xi, gate)
                            for c in range(max(c0, a), c0 + width):
                                j = c - a
                                tr = xr * hr[j] - xi * hi[j]
                                ti = xr * hi[j] + xi * hr[j]
                                z[c, g] = (tr, ti) if a == 0 else (z[c, g][0] + tr, z[c, g][1] + ti)
                            gate = _opaque_zero(list(z[c0 + width - 1, g]))
                return z

            def a_inv(kv, z, flush=False):
                fm = _bf(f_v[...])
                ng = AR // 8
                ys = []
                for u in range(2):
                    rows = [_lanecat(z[c, g]) for g in range(u * ng // 2, (u + 1) * ng // 2)
                            for c in range(NB)]
                    lhs = linked(_rowcat(rows))
                    if flush:
                        lhs = flush_pending(lhs, 8)
                    ys.append(_dot_nt(lhs.astype(BF16), fm))
                y = _rowcat(ys)
                dd = par_v[KS, a_rows, :]
                for c in range(NB):
                    cs = slice(c * LANE, (c + 1) * LANE)
                    yc = _rowcat([y[(g * NB + c) * 8:(g * NB + c + 1) * 8, :] for g in range(ng)])
                    qq = _bf(a_v[3, a_rows2, cs]).astype(F32)
                    kvf = kv[c * AR:(c + 1) * AR, :].astype(F32)
                    c2 = (c % (NB // 2)) * LANE
                    ra_t[c // (NB // 2), a_rows, c2:c2 + LANE] = qq * (yc * (1.0 / LANE) + kvf * dd)

            def a_out():
                slab = jnp.clip(h // 4 - 1, 0, AT - 1)
                half = h % 2
                x = ra_t[half, pl.ds(pl.multiple_of(slab * LANE, LANE), LANE), :]
                xt = x.T
                dst = jnp.where(h >= A_STEPS, AT, slab)
                oa_v[dst, pl.ds(pl.multiple_of(half * (S // 2), S // 2), S // 2), :] = xt.astype(BF16)
                return xt

            def w_blk(r, c):
                return wkv_v[h, _h(r * kw, kw), pl.ds(c * LANE, LANE)]

            def one_pass(lhs, w, flush):
                lhs = linked(lhs)
                if flush:
                    lhs = flush_pending(lhs, cfg["ao_row"])
                d = _dot(_bf(lhs), _bf(paced(w)))
                set_link(d)
                return d

            def k_proj(blk, flush=-1):
                ds = [one_pass(c_v[_h(blk * tq, tq), pl.ds((k % 2) * kw, kw)],
                               w_blk(k % 2, k // 2), k == flush) for k in range(4)]
                k_s[_h(blk * tq, tq), :] = _u32(
                    _lanecat([ds[0] + ds[1], ds[2] + ds[3]]).astype(BF16))

            def b_op(m):
                blk = lambda r, c: _split(w_blk(r, 2 + c))
                return {1: lambda: _add(blk(0, 0), blk(1, 1)),
                        2: lambda: w_blk(0, 2),
                        3: lambda: _sub(blk(0, 1), blk(1, 1)),
                        4: lambda: _sub(blk(1, 0), blk(0, 0)),
                        5: lambda: w_blk(1, 3),
                        6: lambda: _add(blk(0, 0), blk(0, 1)),
                        7: lambda: _add(blk(1, 0), blk(1, 1))}[m]()

            def a_op(m, rho):
                rs = _h(rho * tq, tq)
                if m == 3:
                    return c_v[rs, 0:kw]
                if m == 4:
                    return c_v[_h(S // 2 + rho * tq, tq), kw:]
                return sa_v[{1: 0, 2: 1, 5: 2, 6: 3, 7: 4}[m], rs, :]

            b_cache, prod = {}, {}

            def v_proj(blk, flush=-1):
                rho = blk % 2
                for k, m in enumerate((5, 1, 4, 7, 3) if blk < 2 else (2, 6)):
                    if m not in b_cache:
                        b_cache[m] = b_op(m)
                    prod[m, rho] = one_pass(a_op(m, rho), b_cache[m], k == flush)
                p = lambda m: prod[m, rho]
                if blk < 2:
                    v = [(p(1) + p(4)) + (p(7) - p(5)), p(3) + p(5)]
                else:
                    v = [p(2) + p(4), (p(1) + p(3)) + (p(6) - p(2))]
                v_s[_h(blk * tq, tq), :] = _u32(_lanecat(v).astype(BF16))

            def qk(i, dep=None, flush=False):
                r0 = i * tq
                q = linked(q_all[h, _h(r0, tq), :])
                if dep is not None:
                    q = _pin(q, _opaque_zero([dep]), cfg["ao_row"])
                if flush:
                    q = flush_pending(q, cfg["ao_row"] - 8)
                parts = [_dot_nt(_bf(q), _bf(k_s[_h(0, r0 + LANE), :]))]
                if i > 0:
                    link[0] = _opaque_zero([parts[0][0:8, r0 - LANE:r0]])
                for j in range(1, nsub):
                    q = linked(q_all[h, _h(r0 + LANE * j, tq - LANE * j), :])
                    parts.append(_dot_nt(_bf(q), _bf(k_s[_h(r0 + LANE * j, LANE), :])))
                set_link(parts[2], cfg["link_part"], parts[0])
                return parts

            def softmax(i, parts):
                pb = p_s.at[i % 2]
                chain = _opaque_zero([b[b.shape[0] - 8:, b.shape[1] - LANE:] for b in parts])
                ls = []
                for a in range(nsub):
                    blocks = [parts[j][LANE * (a - j):LANE * (a - j + 1), :] for j in range(a + 1)]
                    last = blocks[-1]
                    w = last.shape[1]
                    dg = jnp.where(tri, last[:, w - LANE:], NEG)
                    blocks[-1] = dg if w == LANE else _lanecat([last[:, :w - LANE], dg])
                    sa = _lanecat(blocks)
                    mb = jnp.broadcast_to(jnp.max(sa, axis=1, keepdims=True), (LANE, LANE))
                    nt = sa.shape[1] // LANE
                    ptiles, psums = [], []
                    for g in range(0, LANE, 8):
                        mg = _pin(mb[g:g + 8, :], chain)
                        pg = [jnp.exp2(sa[g:g + 8, t * LANE:(t + 1) * LANE] - mg) for t in range(nt)]
                        ps = functools.reduce(jnp.add, pg)
                        chain = _opaque_zero([ps])
                        psums.append(ps)
                        ptiles.append(_lanecat(pg))
                    ls.append(jnp.sum(_rowcat(psums), axis=1, keepdims=True))
                    p = _pin(_rowcat(ptiles), link[0], 0, 0 if a == 0 else sa.shape[1] - LANE)
                    pb[LANE * a:LANE * (a + 1), 0:sa.shape[1]] = p.astype(BF16)
                return ls

            def pv(i, ls):
                r0 = i * tq
                pb = p_s.at[i % 2]
                ctx = [_dot(pb[:, 0:r0 + LANE], _bf(v_s[_h(0, r0 + LANE), :]))]
                for j in range(1, nsub):
                    c0 = r0 + LANE * j
                    ctx.append(_dot(pb[LANE * j:, c0:c0 + LANE], _bf(v_s[_h(c0, LANE), :])))
                set_link(ctx[2], cfg["link_part"], ctx[0])
                cs = []
                for a in range(nsub):
                    sl = lambda j: slice(LANE * (a - j), LANE * (a - j + 1))
                    r = pl.reciprocal(ls[a], approx=True)
                    r = r * (2.0 - ls[a] * r)
                    cs.append(functools.reduce(jnp.add, [ctx[j][sl(j)] for j in range(a + 1)]) * r)
                return _rowcat(cs)

            def accumulate(k, res):
                tot = rb_t[k] + res
                rb_t[k] = tot
                if k < n_body:
                    pending.append((k, b_out(k, tot)))

            def oproj_plain(i, ctx):
                ctx = ctx.astype(BF16)
                for u in range(tq // D):
                    lhs = linked(wo_v[h])
                    if i == nq - 1:
                        lhs = flush_pending(lhs, cfg["last_row"])
                    res = _dot_nt(_bf(lhs), ctx[u * D:(u + 1) * D, :])
                    set_link(res)
                    accumulate(i * (tq // D) + u, res)

            wo_cache = {}

            def oproj(i, ctx):
                if i not in cfg["o_str"]:
                    return oproj_plain(i, ctx)
                mh = M // 4
                raw = lambda r, c: wo_v[h, r * mh:(r + 1) * mh, c * LANE:(c + 1) * LANE]
                a = lambda r, c: _split(raw(r, c))
                a_ops = {1: lambda: _add(a(0, 0), a(1, 1)), 2: lambda: _add(a(1, 0), a(1, 1)),
                         3: lambda: raw(0, 0), 4: lambda: raw(1, 1),
                         5: lambda: _add(a(0, 0), a(0, 1)), 6: lambda: _sub(a(1, 0), a(0, 0)),
                         7: lambda: _sub(a(0, 1), a(1, 1))}
                b = lambda r, c: ctx[c * D:(c + 1) * D, r * LANE:(r + 1) * LANE]
                b_ops = {1: lambda: b(0, 0) + b(1, 1), 2: lambda: b(0, 0),
                         3: lambda: b(0, 1) - b(1, 1), 4: lambda: b(1, 0) - b(0, 0),
                         5: lambda: b(1, 1), 6: lambda: b(0, 0) + b(0, 1),
                         7: lambda: b(1, 0) + b(1, 1)}
                p = {}
                for n, m in enumerate((5, 2, 4, 1, 7, 3, 6)):
                    if m not in wo_cache:
                        wo_cache[m] = a_ops[m]()
                    rhs = b_ops[m]().astype(BF16)
                    if n == cfg["o_half"]:
                        halves = [_dot_nt(_bf(linked(wo_cache[m][r:r + mh // 2])), rhs)
                                  for r in (0, mh // 2)]
                        p[m] = _rowcat(halves)
                        set_link(halves[1], 0)
                    else:
                        p[m] = _dot_nt(_bf(linked(wo_cache[m])), rhs)
                        if (n - (n > cfg["o_half"])) % 2 == 1:
                            set_link(p[m], cfg["o_link"])
                accumulate(2 * i, _rowcat([(p[1] + p[4]) + (p[7] - p[5]), p[2] + p[4]]))
                accumulate(2 * i + 1, _rowcat([p[3] + p[5], (p[1] + p[3]) + (p[6] - p[2])]))

            st = {}
            for op in cfg["seq"].split():
                op, _, fl = op.partition("!")
                fl = int(fl) if fl else -1
                kind, i = op[0], int(op[1:] or 0)
                if kind == "K":
                    k_proj(i, fl)
                elif kind == "V":
                    v_proj(i, fl)
                elif kind == "Q":
                    st["s", i] = qk(i, a_out() if i == cfg["ao_at"] else None, fl >= 0)
                elif kind == "P":
                    st["ctx", i] = pv(i, softmax(i, st["s", i]))
                elif kind == "O":
                    oproj(i, st["ctx", i])
                elif kind == "F" and with_a:
                    st["kv"], xs, hs = a_fwd()
                    st["z"] = a_conv(xs, hs)
                elif kind == "I" and with_a:
                    a_inv(st["kv"], st["z"], fl >= 0)
            assert not pending
            return carry

        with jax.named_scope("loop_a"):
            lax.fori_loop(cfg["h0"], H, head_step, 0)
        with jax.named_scope("tail"):
            for i in range(n_body, NOUT):
                b_out(i, rb_t[i])
                out_copy(i).start()
            for i in range(NOUT + AT):
                out_copy(i).wait()

    scratch = [
        pltpu.VMEM((4, M // 2, S), U32),
        pltpu.VMEM((KS, M), BF16),
        pltpu.VMEM((M,), BF16),
        pltpu.VMEM((KS + 1, M, LANE), F32),
        pltpu.VMEM((LANE // 2, 2 * LANE), U32),
        pltpu.VMEM((M // 2, S), U32),
        pltpu.VMEM((S // 2, MP), U32),
        pltpu.VMEM((S // 2, C), U32),
        [pltpu.VMEM((4 * min(TP, M // 2 - kt * TP) * 8, LANE), U32)
         for kt in range(KT)],
        pltpu.VMEM((H // 2, MP // 2, 2 * D), U32),
        pltpu.VMEM((H // 2, x_cols, 2 * D), U32),
        pltpu.VMEM((QIT, C * 8, LANE), U32),
        pltpu.VMEM((H, C // 2, 2 * D), U32),
        pltpu.VMEM((H, M // 2, D), U32),
        pltpu.VMEM((H, S // 2, D), U32),
        pltpu.VMEM((S // 2, D), U32),
        pltpu.VMEM((S // 2, D), U32),
        pltpu.VMEM((2, tq, S), BF16),
        pltpu.VMEM((2, M, S // 2), F32),
        pltpu.VMEM((S // D, M, D), F32),
        pltpu.VMEM((AT + 1, S, LANE), BF16),
        pltpu.VMEM((S, 2 * M - AT * LANE), BF16),
        pltpu.SemaphoreType.DMA((XC,)),
        pltpu.SemaphoreType.DMA((KT,)),
        pltpu.SemaphoreType.DMA((QIT,)),
        pltpu.SemaphoreType.DMA((QIT,)),
        pltpu.SemaphoreType.DMA((2,)),
        pltpu.SemaphoreType.DMA((3,)),
        pltpu.SemaphoreType.DMA((S // D + AT,)),
    ]
    return kernel, scratch


_DEFAULT = dict(
    tq=512, a_width=4, ao_at=1, ao_row=240, link_back=176, link_part=32, pace_row=32,
    pace_step=24, use_a=1, h0=0, last_row=216, o_str=(0, 1, 2, 3), o_link=48, o_half=6,
    seq="K0 Q0 K1 Q1 V0 F P0 K2 Q2 O0 V1!2 P1 K3 Q3 O1 V2!1 P2 V3 O2 P3 I!0 O3")


def _build(**kw):
    cfg = dict(_DEFAULT)
    cfg.update(kw)
    kernel, scratch = _make_kernel(cfg)

    def run(A_q, A_k, A_v, A_shift_k, A_ssm_k, A_ssm_D, B_x, B_c_kv, B_w_q, B_w_uk,
            B_w_uv, B_w_o):
        tr = lambda a: jnp.swapaxes(a, 1, 2).reshape(M, S)
        args = (
            tr(A_q), tr(A_k), tr(A_v), A_shift_k.T, A_ssm_k, A_ssm_D, tr(B_x),
            B_c_kv.reshape(S, C),
            B_w_q.reshape(M // 2, 2 * H, D), B_w_uk.reshape(C // 2, 2 * H, D),
            B_w_uv.reshape(C // 2, 2 * H, D),
            jnp.swapaxes(B_w_o, 1, 2),
        )
        out = pl.pallas_call(
            kernel,
            in_specs=[pl.BlockSpec(memory_space=pl.ANY)] * len(args),
            out_specs=pl.BlockSpec(memory_space=pl.ANY),
            out_shape=jax.ShapeDtypeStruct((S, 2 * M), BF16),
            scratch_shapes=scratch,
            compiler_params=pltpu.CompilerParams(
                vmem_limit_bytes=120 * 1024 * 1024,
                disable_bounds_checks=True),
        )(*args)
        return out.reshape(1, S, 2 * M)

    return run


_run = _build()


@jax.jit
def pallas_concat_heads__ssm_conv_h3__compressed_kv_cla__prompt_kernel(
    A_q: jax.Array,
    A_k: jax.Array,
    A_v: jax.Array,
    A_shift_k: jax.Array,
    A_ssm_k: jax.Array,
    A_ssm_D: jax.Array,
    B_x: jax.Array,
    B_c_kv: jax.Array,
    B_w_q: jax.Array,
    B_w_uk: jax.Array,
    B_w_uv: jax.Array,
    B_w_o: jax.Array,
):
    return _run(A_q, A_k, A_v, A_shift_k, A_ssm_k, A_ssm_D, B_x, B_c_kv, B_w_q,
                B_w_uk, B_w_uv, B_w_o)
```

```python
import functools

import jax
import jax.numpy as jnp
from jax import lax
import jax.experimental.pallas as pl
import jax.experimental.pallas.tpu as pltpu

F32 = jnp.float32
BF16 = jnp.bfloat16
U32 = jnp.uint32

S = 2048
M = 448
MP = 512
C = 1024
H = 16
D = 256
KS = 4
LANE = 128
NB = S // LANE
AR = 32
A_STEPS = M // AR
LOG2E = 1.4426950408889634
NEG = -1e30

NT = (((1,), (1,)), ((), ()))


def _dot(a, b):
    return jnp.dot(a, b, preferred_element_type=F32)


def _dot_nt(a, b):
    return lax.dot_general(a, b, NT, preferred_element_type=F32)


def _bf(x):
    return pltpu.bitcast(x, BF16)


def _u32(x):
    return pltpu.bitcast(x, U32)


def _h(r0, n):
    return pl.ds(r0 // 2, n // 2)


def _repack(ev, od):
    lo = (ev & jnp.uint32(0xFFFF)) | (od << 16)
    hi = (ev >> 16) | (od & jnp.uint32(0xFFFF0000))
    return lo, hi


def _split(w):
    return (pltpu.bitcast(w << 16, F32), pltpu.bitcast(w & jnp.uint32(0xFFFF0000), F32))


def _join(lo, hi):
    half = jnp.uint32(0x8000)
    lo = (pltpu.bitcast(lo, U32) + half) >> 16
    hi = (pltpu.bitcast(hi, U32) + half) & jnp.uint32(0xFFFF0000)
    return lo | hi


def _add(a, b):
    return _join(a[0] + b[0], a[1] + b[1])


def _sub(a, b):
    return _join(a[0] - b[0], a[1] - b[1])


def _opaque_zero(vals):
    acc = None
    for v in vals:
        b = v if v.dtype == U32 else pltpu.bitcast(v, U32)
        for r in range(0, b.shape[0], 8):
            for c in range(0, b.shape[1], LANE):
                t = b[r:r + 8, c:c + LANE]
                acc = t if acc is None else acc | t
    return jnp.minimum((acc >> 1).astype(jnp.int32), 0)


def _pin(x, zero, r=0, c=0):
    t = pltpu.bitcast(pltpu.bitcast(x[r:r + 8, c:c + LANE], jnp.int32) + zero, x.dtype)
    row = ([x[r:r + 8, :c]] if c > 0 else []) + [t] + (
        [x[r:r + 8, c + LANE:]] if c + LANE < x.shape[1] else [])
    row = jnp.concatenate(row, axis=1) if len(row) > 1 else row[0]
    col = ([x[:r, :]] if r > 0 else []) + [row] + ([x[r + 8:, :]] if r + 8 < x.shape[0] else [])
    return jnp.concatenate(col, axis=0) if len(col) > 1 else col[0]


def _rowcat(xs):
    return jnp.concatenate(xs, axis=0) if len(xs) > 1 else xs[0]


def _lanecat(xs):
    return jnp.concatenate(xs, axis=1) if len(xs) > 1 else xs[0]


def _make_kernel(cfg):
    tq = cfg["tq"]
    nq = S // tq
    nsub = tq // LANE
    KT = MP // LANE
    TP = LANE // 2
    XC = 4
    x_cols = S // XC
    QP = 2
    QIT = H // 2 // QP
    CP = 176
    AT = 3

    def kernel(aq_hbm, ak_hbm, av_hbm, sh_hbm, ssm_hbm, dd_hbm, x_hbm, c_hbm,
               wq_hbm, wk_hbm, wv_hbm, wo_hbm,
               out_hbm,
               a_v, sh_v, dd_v, par_v, f_v,
               xt_v, x_v, c_v, wqs_v, wq_v, qacc, ws_v, wkv_v, wo_v,
               q_all, k_s, v_s, p_s, ra_t, rb_t, oa_v, out_v,
               sem_x, sem_wq, sem_w, sem_c, sem_s, sem_a, sem_out):
        x32, c32, wq32, wk32, wv32, wo32 = (
            r.bitcast(U32) for r in (x_hbm, c_hbm, wq_hbm, wk_hbm, wv_hbm, wo_hbm))
        a32 = [r.bitcast(U32) for r in (ak_hbm, av_hbm, ssm_hbm, aq_hbm)]

        sa_v = qacc

        def x_copy(i):
            cs = pl.ds(i * x_cols, x_cols)
            return pltpu.make_async_copy(x32.at[:, cs], xt_v.at[:, cs], sem_x.at[i])

        def wq_pairs(kt):
            return min(TP, M // 2 - kt * TP)

        def wq_copies(kt):
            n = wq_pairs(kt)
            dst = wqs_v[kt].reshape(4, n, 8, LANE)
            return [pltpu.make_async_copy(
                wq32.at[pl.ds(kt * TP, n), pl.ds(8 * (k // 2), 8), pl.ds((k % 2) * LANE, LANE)],
                dst.at[k], sem_wq.at[kt]) for k in range(4)]

        def wq_wait(kt):
            pltpu.make_async_copy(wqs_v[kt], wqs_v[kt], sem_wq.at[kt]).wait()

        def w_copies(g):
            dst = ws_v.reshape(8, C // 2, 8, LANE)
            src = (wk32, wv32)[g // 2]
            return [pltpu.make_async_copy(
                src.at[:, pl.ds(8 * par, 8), pl.ds((g % 2) * LANE, LANE)],
                dst.at[2 * g + par], sem_w.at[g]) for par in range(2)]

        def w_wait(g):
            pltpu.make_async_copy(ws_v.at[g], ws_v.at[g], sem_w.at[g]).wait()

        c_bounds = [0, CP, 2 * CP, S // 4]

        def c_copies(p):
            r0, n = c_bounds[p], c_bounds[p + 1] - c_bounds[p]
            return [pltpu.make_async_copy(c32.at[rs], c_v.at[rs], sem_c.at[p])
                    for rs in (pl.ds(r0, n), pl.ds(S // 4 + r0, n))]

        wo_copy = pltpu.make_async_copy(wo32, wo_v, sem_a.at[0])

        a_parts = [pl.ds(0, AR // 2), pl.ds(AR // 2, M // 2 - AR // 2)]

        def a_start(part):
            rs = a_parts[part]
            for k in range(4):
                pltpu.make_async_copy(
                    a32[k].at[rs], a_v.at[k, rs], sem_a.at[1 + part]).start()

        def a_wait(part):
            view = a_v.at[:, a_parts[part]]
            pltpu.make_async_copy(view, view, sem_a.at[1 + part]).wait()

        small = [pltpu.make_async_copy(sh_hbm, sh_v, sem_s.at[0]),
                 pltpu.make_async_copy(dd_hbm, dd_v, sem_s.at[1])]

        link = [None]
        pace = [None]

        def set_link(res, row=None, pacer=None):
            if row is None:
                row = res.shape[0] - cfg["link_back"]
            link[0] = _opaque_zero([res[row:row + 8, res.shape[1] - LANE:]])
            pace[0] = res if pacer is None else pacer

        def linked(x):
            return x if link[0] is None else _pin(x, link[0])

        def paced(w):
            res = pace[0]
            if res is None or link[0] is None or not cfg["pace_step"]:
                return w
            rows = []
            r0, step = cfg["pace_row"], cfg["pace_step"]
            if res.shape[0] < 400:
                r0, step = 0, 8
            if res.shape[0] < 200:
                return w
            zs = [_opaque_zero([res[r:r + 8, res.shape[1] - LANE:]])
                  for r in range(r0, r0 + 8 * step, step)]
            for r in range(0, w.shape[0], 8):
                z = zs[7 - (r // 8) % 8]
                t = pltpu.bitcast(w[r:r + 8, :], jnp.int32)
                rows.append(pltpu.bitcast(t + _lanecat([z] * (w.shape[1] // LANE)), U32))
            return _rowcat(rows)

        for cp in small:
            cp.start()
        x_copy(0).start()
        for cp in wq_copies(0):
            cp.start()

        def zero_body(k, carry):
            n = LANE // (S // D)
            bi = lax.broadcasted_iota(jnp.int32, (n, LANE), 0) + k * n
            mi = lax.broadcasted_iota(jnp.int32, (n, LANE), 1)
            ph = ((4 * mi + 1) * bi) & 511
            ang = ph.astype(F32) * (2.0 * 3.141592653589793 / 512.0)
            rs = pl.ds(pl.multiple_of(k * (n // 2), n // 2), n // 2)
            f_v[rs, 0:LANE] = _u32(jnp.cos(ang).astype(BF16))
            f_v[rs, LANE:] = _u32((-jnp.sin(ang)).astype(BF16))

            rb_t[k] = jnp.zeros((M, D), F32)
            cs = pl.ds(pl.multiple_of((k % 4) * D, D), D)
            ra_t[k // 4, 0:LANE, cs] = jnp.zeros((LANE, D), F32)
            ra_t[k // 4, AT * LANE:, cs] = jnp.zeros((M - AT * LANE, D), F32)
            return carry

        lax.fori_loop(0, S // D, zero_body, 0)
        c_v[S // 2:, :] = jnp.zeros((8, C), U32)

        for kt in range(1, KT):
            for cp in wq_copies(kt):
                cp.start()
        with jax.named_scope("small_wait"):
            for cp in small:
                cp.wait()
        sh = sh_v[...].astype(F32)
        for j in range(KS):
            par_v[j] = jnp.broadcast_to(sh[j:j + 1, :], (LANE, M)).T
        dd = dd_v[...].astype(F32).reshape(1, M)
        par_v[KS] = jnp.broadcast_to(dd, (LANE, M)).T

        def x_transpose(i):
            xt = xt_v[:, pl.ds(i * x_cols, x_cols)]
            xt = _rowcat([xt, jnp.zeros((MP // 2 - M // 2, x_cols), U32)])
            x_v[_h(i * x_cols, x_cols), :] = _u32(_bf(xt).astype(F32).T.astype(BF16))

        def q_early(kt, keep=False):
            first, last = kt == 0, kt == KT - 1
            n = wq_pairs(kt)
            cols = pl.ds(kt * LANE, LANE)
            if not keep:
                link[0] = None
            for j in range(H // 2):
                ws = []
                for half in range(2):
                    ev, od = (wqs_v[kt][pl.ds((2 * par + half) * n * 8 + j, n, stride=8), :]
                              for par in range(2))
                    ws.append(_repack(ev, od))
                w = _lanecat([ws[0][0], ws[1][0], ws[0][1], ws[1][1]])
                if n < TP:
                    w = _rowcat([w, jnp.zeros((TP - n, 2 * D), U32)])
                wq_v[j, pl.ds(kt * TP, TP), :] = w
                d = _dot(_bf(linked(x_v[_h(0, x_cols), cols])), _bf(w))
                set_link(d)
                if not first:
                    d = d + pltpu.bitcast(qacc[j], F32)
                if last:
                    d = (d * (D ** -0.5 * LOG2E)).astype(BF16)
                    for t in range(2):
                        q_all[2 * j + t, _h(0, x_cols), :] = _u32(d[:, t * D:(t + 1) * D])
                else:
                    qacc[j] = pltpu.bitcast(d, U32)

        with jax.named_scope("x_wait"):
            x_copy(0).wait()
        x_transpose(0)
        for i in range(1, XC):
            x_copy(i).start()
        for g in range(QIT):
            for cp in w_copies(g) + (c_copies(g) if g < QIT - 1 else []):
                cp.start()
        wo_copy.start()
        a_start(0)
        a_start(1)
        with jax.named_scope("wq_wait"):
            wq_wait(0)
        q_early(0)
        with jax.named_scope("wq_wait"):
            wq_wait(1)
            wq_wait(2)
        q_early(1)
        q_early(2, keep=True)
        with jax.named_scope("wq_wait"):
            wq_wait(3)
            for i in range(1, XC):
                x_copy(i).wait()
        q_early(3)
        for i in range(1, XC):
            x_transpose(i)

        def unpack(g, sub, j):
            ev, od = (ws_v[g, pl.ds((par * (C // 2) + sub * TP) * 8 + j, TP, stride=8), :]
                      for par in range(2))
            lo, hi = _repack(ev, od)
            rows = pl.ds(sub * TP, TP)
            cols = pl.ds(pl.multiple_of(g * LANE, LANE), LANE)
            wkv_v[2 * j, rows, cols] = lo
            wkv_v[2 * j + 1, rows, cols] = hi
            return [lo, hi]

        def a_sums(it, u):
            r0 = jnp.clip((it - 1) * CP, 0, S // 4 - CP) + 8 * u
            src = [jnp.where(it == 0, S // 2, r0 + rb * (S // 4)) for rb in range(2)]
            r0 = pl.multiple_of(r0, 8)
            kw = C // 2
            a11, a12, a21, a22 = (
                _split(c_v[pl.ds(pl.multiple_of(src[rb], 8), 8), pl.ds(cb * kw, kw)])
                for rb in range(2) for cb in range(2))
            outs = [_add(a11, a22), _add(a21, a22), _add(a11, a12), _sub(a21, a11),
                    _sub(a12, a22)]
            for k, o in enumerate(outs):
                sa_v[k, pl.ds(r0, 8), :] = o
            return outs

        units = [functools.partial(unpack, sub=s_, j=j_)
                 for s_ in range(C // 2 // TP) for j_ in range(H // 2)]
        for u_ in range(CP // 8):
            units.insert(4 * u_ + 1, functools.partial(a_sums, u=u_))

        def qproj(it, r0, n, t, zeros=(None, None)):
            outs = []
            for u in range(2):
                lhs = _bf(linked(x_v[_h(r0, n), :]))
                d = _dot(lhs, _bf(wq_v[it, :, pl.ds(t * D + u * LANE, LANE)]))
                set_link(d)
                if zeros[u] is not None:
                    for k, z in enumerate(zeros[u]):
                        d = _pin(d, z, 8 * ((k * (n // 8)) // len(zeros[u])))
                outs.append(d)
            q2 = _lanecat(outs)
            q_all[2 * it + t, _h(r0, n), :] = _u32((q2 * (D ** -0.5 * LOG2E)).astype(BF16))

        def q_body(it, carry):
            with jax.named_scope("w_wait"):
                w_wait(it)
                for p in range(QIT - 1):
                    @pl.when(it == p + 1)
                    def _():
                        for cp in c_copies(p):
                            cp.wait()
            link[0] = None
            pieces = [(p, pc, t) for p in range(QP) for pc in range(1, XC) for t in range(2)]
            nd = 2 * len(pieces)
            for k, (p, pc, t) in enumerate(pieces):
                zeros = []
                for u in range(2):
                    d = 2 * k + u
                    mine = units[d * len(units) // nd:(d + 1) * len(units) // nd]
                    zeros.append([_opaque_zero(u_(it)) for u_ in mine])
                qproj(QP * it + p, pc * x_cols, x_cols, t, zeros)
            return carry

        with jax.named_scope("q_loop"):
            lax.fori_loop(0, QIT, q_body, 0)
        wo_copy.wait()
        a_wait(0)

        tri = (lax.broadcasted_iota(jnp.int32, (LANE, LANE), 1)
               <= lax.broadcasted_iota(jnp.int32, (LANE, LANE), 0))

        NOUT = S // D

        def out_copy(i):
            if i >= NOUT:
                t = i - NOUT
                return pltpu.make_async_copy(
                    oa_v.at[t], out_hbm.at[:, pl.ds(t * LANE, LANE)], sem_out.at[i])
            rs = pl.ds(i * D, D)
            return pltpu.make_async_copy(
                out_v.at[rs], out_hbm.at[rs, pl.ds(AT * LANE, 2 * M - AT * LANE)], sem_out.at[i])

        n_body = NOUT - (tq // D if nq - 1 in cfg["o_str"] else 1)

        def b_out(k, tot):
            c0 = (k * D) % (S // 2)
            full = _rowcat([ra_t[k * D // (S // 2), AT * LANE:, c0:c0 + D], tot]).T
            out_v[k * D:(k + 1) * D, :] = full.astype(BF16)
            return full

        def head_step(h, carry):
            with jax.named_scope("step"):
                return head_step_(h, carry)

        def head_step_(h, carry):
            with_a = cfg["use_a"]

            @pl.when(h == A_STEPS)
            def _():
                for t in range(AT):
                    out_copy(NOUT + t).start()

            @pl.when(h == cfg["h0"] + 1)
            def _():
                a_wait(1)

            link[0] = None
            n2 = AR // 2
            a_rows2 = pl.ds(pl.multiple_of(jnp.minimum(h, A_STEPS - 1) * n2, n2), n2)
            a_rows = pl.ds(pl.multiple_of(jnp.minimum(h, A_STEPS - 1) * AR, AR), AR)

            kw = C // 2
            pending = []

            def flush_pending(x, row):
                done = list(pending)
                del pending[:]
                if not done:
                    return x
                x = _pin(x, _opaque_zero([f for _, f in done]), row)

                @pl.when(h == H - 1)
                def _():
                    for k, _f in done:
                        out_copy(k).start()
                return x

            def a_fwd():
                kk = _bf(a_v[0, a_rows2, :]).astype(F32)
                lane = lax.broadcasted_iota(jnp.int32, (AR, LANE), 1)
                coef = [par_v[j, a_rows, :] for j in range(KS)]
                rolled = [kk] + [pltpu.roll(kk, j, 1) for j in range(1, KS)]
                vv = _bf(a_v[1, a_rows2, :]).astype(F32)
                kv_blocks = []
                for a in range(NB):
                    cs = slice(a * LANE, (a + 1) * LANE)
                    acc = rolled[0][:, cs] * coef[0]
                    for j in range(1, KS):
                        t = rolled[j][:, cs]
                        if a == 0:
                            t = jnp.where(lane >= j, t, 0.0)
                        acc = acc + t * coef[j]
                    kv_blocks.append(acc * vv[:, cs])
                hk = a_v[2, a_rows2, :]
                hk = _rowcat([hk[:, a * LANE:(a + 1) * LANE] for a in range(NB)])
                fm = _bf(f_v[...])
                hs = _dot(_bf(linked(hk)), fm)
                kv = linked(_rowcat(kv_blocks)).astype(BF16)
                xs = _dot(kv, fm)
                set_link(xs)
                return kv, xs, hs

            def a_conv(xs, hs):
                def tile(v, a, g, part):
                    r = a * AR + 8 * g
                    return v[r:r + 8, part * LANE:(part + 1) * LANE]

                z = {}
                gate = None
                width = cfg["a_width"]
                for g in range(AR // 8):
                    hr = [tile(hs, 0, g, 0)] + [
                        tile(hs, j, g, 0) - tile(hs, j - 1, g, 1) for j in range(1, NB)]
                    hi = [tile(hs, 0, g, 1)] + [
                        tile(hs, j, g, 1) + tile(hs, j - 1, g, 0) for j in range(1, NB)]
                    for c0 in range(0, NB, width):
                        for a in range(c0 + width):
                            xr, xi = tile(xs, a, g, 0), tile(xs, a, g, 1)
                            if gate is not None:
                                xr, xi = _pin(xr, gate), _pin(xi, gate)
                            for c in range(max(c0, a), c0 + width):
                                j = c - a
                                tr = xr * hr[j] - xi * hi[j]
                                ti = xr * hi[j] + xi * hr[j]
                                z[c, g] = (tr, ti) if a == 0 else (z[c, g][0] + tr, z[c, g][1] + ti)
                            gate = _opaque_zero(list(z[c0 + width - 1, g]))
                return z

            def a_inv(kv, z, flush=False):
                fm = _bf(f_v[...])
                ng = AR // 8
                ys = []
                for u in range(2):
                    rows = [_lanecat(z[c, g]) for g in range(u * ng // 2, (u + 1) * ng // 2)
                            for c in range(NB)]
                    lhs = linked(_rowcat(rows))
                    if flush:
                        lhs = flush_pending(lhs, 8)
                    ys.append(_dot_nt(lhs.astype(BF16), fm))
                y = _rowcat(ys)
                dd = par_v[KS, a_rows, :]
                for c in range(NB):
                    cs = slice(c * LANE, (c + 1) * LANE)
                    yc = _rowcat([y[(g * NB + c) * 8:(g * NB + c + 1) * 8, :] for g in range(ng)])
                    qq = _bf(a_v[3, a_rows2, cs]).astype(F32)
                    kvf = kv[c * AR:(c + 1) * AR, :].astype(F32)
                    c2 = (c % (NB // 2)) * LANE
                    ra_t[c // (NB // 2), a_rows, c2:c2 + LANE] = qq * (yc * (1.0 / LANE) + kvf * dd)

            def a_out():
                slab = jnp.clip(h // 4 - 1, 0, AT - 1)
                half = h % 2
                x = ra_t[half, pl.ds(pl.multiple_of(slab * LANE, LANE), LANE), :]
                xt = x.T
                dst = jnp.where(h >= A_STEPS, AT, slab)
                oa_v[dst, pl.ds(pl.multiple_of(half * (S // 2), S // 2), S // 2), :] = xt.astype(BF16)
                return xt

            def w_blk(r, c):
                return wkv_v[h, _h(r * kw, kw), pl.ds(c * LANE, LANE)]

            def one_pass(lhs, w, flush):
                lhs = linked(lhs)
                if flush:
                    lhs = flush_pending(lhs, cfg["ao_row"])
                d = _dot(_bf(lhs), _bf(paced(w)))
                set_link(d)
                return d

            def k_proj(blk, flush=-1):
                ds = [one_pass(c_v[_h(blk * tq, tq), pl.ds((k % 2) * kw, kw)],
                               w_blk(k % 2, k // 2), k == flush) for k in range(4)]
                k_s[_h(blk * tq, tq), :] = _u32(
                    _lanecat([ds[0] + ds[1], ds[2] + ds[3]]).astype(BF16))

            def b_op(m):
                blk = lambda r, c: _split(w_blk(r, 2 + c))
                return {1: lambda: _add(blk(0, 0), blk(1, 1)),
                        2: lambda: w_blk(0, 2),
                        3: lambda: _sub(blk(0, 1), blk(1, 1)),
                        4: lambda: _sub(blk(1, 0), blk(0, 0)),
                        5: lambda: w_blk(1, 3),
                        6: lambda: _add(blk(0, 0), blk(0, 1)),
                        7: lambda: _add(blk(1, 0), blk(1, 1))}[m]()

            def a_op(m, rho):
                rs = _h(rho * tq, tq)
                if m == 3:
                    return c_v[rs, 0:kw]
                if m == 4:
                    return c_v[_h(S // 2 + rho * tq, tq), kw:]
                return sa_v[{1: 0, 2: 1, 5: 2, 6: 3, 7: 4}[m], rs, :]

            b_cache, prod = {}, {}

            def v_proj(blk, flush=-1):
                rho = blk % 2
                for k, m in enumerate((5, 1, 4, 7, 3) if blk < 2 else (2, 6)):
                    if m not in b_cache:
                        b_cache[m] = b_op(m)
                    prod[m, rho] = one_pass(a_op(m, rho), b_cache[m], k == flush)
                p = lambda m: prod[m, rho]
                if blk < 2:
                    v = [(p(1) + p(4)) + (p(7) - p(5)), p(3) + p(5)]
                else:
                    v = [p(2) + p(4), (p(1) + p(3)) + (p(6) - p(2))]
                v_s[_h(blk * tq, tq), :] = _u32(_lanecat(v).astype(BF16))

            def qk(i, dep=None, flush=False):
                r0 = i * tq
                q = linked(q_all[h, _h(r0, tq), :])
                if dep is not None:
                    q = _pin(q, _opaque_zero([dep]), cfg["ao_row"])
                if flush:
                    q = flush_pending(q, cfg["ao_row"] - 8)
                parts = [_dot_nt(_bf(q), _bf(k_s[_h(0, r0 + LANE), :]))]
                if i > 0:
                    link[0] = _opaque_zero([parts[0][0:8, r0 - LANE:r0]])
                for j in range(1, nsub):
                    q = linked(q_all[h, _h(r0 + LANE * j, tq - LANE * j), :])
                    parts.append(_dot_nt(_bf(q), _bf(k_s[_h(r0 + LANE * j, LANE), :])))
                set_link(parts[2], cfg["link_part"], parts[0])
                return parts

            def softmax(i, parts):
                pb = p_s.at[i % 2]
                chain = _opaque_zero([b[b.shape[0] - 8:, b.shape[1] - LANE:] for b in parts])
                ls = []
                for a in range(nsub):
                    blocks = [parts[j][LANE * (a - j):LANE * (a - j + 1), :] for j in range(a + 1)]
                    last = blocks[-1]
                    w = last.shape[1]
                    dg = jnp.where(tri, last[:, w - LANE:], NEG)
                    blocks[-1] = dg if w == LANE else _lanecat([last[:, :w - LANE], dg])
                    sa = _lanecat(blocks)
                    mb = jnp.broadcast_to(jnp.max(sa, axis=1, keepdims=True), (LANE, LANE))
                    nt = sa.shape[1] // LANE
                    ptiles, psums = [], []
                    for g in range(0, LANE, 8):
                        mg = _pin(mb[g:g + 8, :], chain)
                        pg = [jnp.exp2(sa[g:g + 8, t * LANE:(t + 1) * LANE] - mg) for t in range(nt)]
                        ps = functools.reduce(jnp.add, pg)
                        chain = _opaque_zero([ps])
                        psums.append(ps)
                        ptiles.append(_lanecat(pg))
                    ls.append(jnp.sum(_rowcat(psums), axis=1, keepdims=True))
                    p = _pin(_rowcat(ptiles), link[0], 0, 0 if a == 0 else sa.shape[1] - LANE)
                    pb[LANE * a:LANE * (a + 1), 0:sa.shape[1]] = p.astype(BF16)
                return ls

            def pv(i, ls):
                r0 = i * tq
                pb = p_s.at[i % 2]
                ctx = [_dot(pb[:, 0:r0 + LANE], _bf(v_s[_h(0, r0 + LANE), :]))]
                for j in range(1, nsub):
                    c0 = r0 + LANE * j
                    ctx.append(_dot(pb[LANE * j:, c0:c0 + LANE], _bf(v_s[_h(c0, LANE), :])))
                set_link(ctx[2], cfg["link_part"], ctx[0])
                cs = []
                for a in range(nsub):
                    sl = lambda j: slice(LANE * (a - j), LANE * (a - j + 1))
                    r = pl.reciprocal(ls[a], approx=True)
                    r = r * (2.0 - ls[a] * r)
                    cs.append(functools.reduce(jnp.add, [ctx[j][sl(j)] for j in range(a + 1)]) * r)
                return _rowcat(cs)

            def accumulate(k, res):
                tot = rb_t[k] + res
                rb_t[k] = tot
                if k < n_body:
                    pending.append((k, b_out(k, tot)))

            def oproj_plain(i, ctx):
                ctx = ctx.astype(BF16)
                for u in range(tq // D):
                    lhs = linked(wo_v[h])
                    if i == nq - 1:
                        lhs = flush_pending(lhs, cfg["last_row"])
                    res = _dot_nt(_bf(lhs), ctx[u * D:(u + 1) * D, :])
                    set_link(res)
                    accumulate(i * (tq // D) + u, res)

            wo_cache = {}

            def oproj(i, ctx):
                if i not in cfg["o_str"]:
                    return oproj_plain(i, ctx)
                mh = M // 4
                raw = lambda r, c: wo_v[h, r * mh:(r + 1) * mh, c * LANE:(c + 1) * LANE]
                a = lambda r, c: _split(raw(r, c))
                a_ops = {1: lambda: _add(a(0, 0), a(1, 1)), 2: lambda: _add(a(1, 0), a(1, 1)),
                         3: lambda: raw(0, 0), 4: lambda: raw(1, 1),
                         5: lambda: _add(a(0, 0), a(0, 1)), 6: lambda: _sub(a(1, 0), a(0, 0)),
                         7: lambda: _sub(a(0, 1), a(1, 1))}
                b = lambda r, c: ctx[c * D:(c + 1) * D, r * LANE:(r + 1) * LANE]
                b_ops = {1: lambda: b(0, 0) + b(1, 1), 2: lambda: b(0, 0),
                         3: lambda: b(0, 1) - b(1, 1), 4: lambda: b(1, 0) - b(0, 0),
                         5: lambda: b(1, 1), 6: lambda: b(0, 0) + b(0, 1),
                         7: lambda: b(1, 0) + b(1, 1)}
                p = {}
                for n, m in enumerate((5, 2, 4, 1, 7, 3, 6)):
                    if m not in wo_cache:
                        wo_cache[m] = a_ops[m]()
                    rhs = b_ops[m]().astype(BF16)
                    if n == cfg["o_half"]:
                        halves = [_dot_nt(_bf(linked(wo_cache[m][r:r + mh // 2])), rhs)
                                  for r in (0, mh // 2)]
                        p[m] = _rowcat(halves)
                        set_link(halves[1], 0)
                    else:
                        p[m] = _dot_nt(_bf(linked(wo_cache[m])), rhs)
                        if (n - (n > cfg["o_half"])) % 2 == 1:
                            set_link(p[m], cfg["o_link"])
                accumulate(2 * i, _rowcat([(p[1] + p[4]) + (p[7] - p[5]), p[2] + p[4]]))
                accumulate(2 * i + 1, _rowcat([p[3] + p[5], (p[1] + p[3]) + (p[6] - p[2])]))

            st = {}
            for op in cfg["seq"].split():
                op, _, fl = op.partition("!")
                fl = int(fl) if fl else -1
                kind, i = op[0], int(op[1:] or 0)
                if kind == "K":
                    k_proj(i, fl)
                elif kind == "V":
                    v_proj(i, fl)
                elif kind == "Q":
                    st["s", i] = qk(i, a_out() if i == cfg["ao_at"] else None, fl >= 0)
                elif kind == "P":
                    st["ctx", i] = pv(i, softmax(i, st["s", i]))
                elif kind == "O":
                    oproj(i, st["ctx", i])
                elif kind == "F" and with_a:
                    st["kv"], xs, hs = a_fwd()
                    st["z"] = a_conv(xs, hs)
                elif kind == "I" and with_a:
                    a_inv(st["kv"], st["z"], fl >= 0)
            assert not pending
            return carry

        with jax.named_scope("loop_a"):
            lax.fori_loop(cfg["h0"], H, head_step, 0)
        with jax.named_scope("tail"):
            for i in range(n_body, NOUT):
                b_out(i, rb_t[i])
                out_copy(i).start()
            for i in range(NOUT + AT):
                out_copy(i).wait()

    scratch = [
        pltpu.VMEM((4, M // 2, S), U32),
        pltpu.VMEM((KS, M), BF16),
        pltpu.VMEM((M,), BF16),
        pltpu.VMEM((KS + 1, M, LANE), F32),
        pltpu.VMEM((LANE // 2, 2 * LANE), U32),
        pltpu.VMEM((M // 2, S), U32),
        pltpu.VMEM((S // 2, MP), U32),
        pltpu.VMEM((S // 2 + 8, C), U32),
        [pltpu.VMEM((4 * min(TP, M // 2 - kt * TP) * 8, LANE), U32)
         for kt in range(KT)],
        pltpu.VMEM((H // 2, MP // 2, 2 * D), U32),
        pltpu.VMEM((H // 2, x_cols, 2 * D), U32),
        pltpu.VMEM((QIT, C * 8, LANE), U32),
        pltpu.VMEM((H, C // 2, 2 * D), U32),
        pltpu.VMEM((H, M // 2, D), U32),
        pltpu.VMEM((H, S // 2, D), U32),
        pltpu.VMEM((S // 2, D), U32),
        pltpu.VMEM((S // 2, D), U32),
        pltpu.VMEM((2, tq, S), BF16),
        pltpu.VMEM((2, M, S // 2), F32),
        pltpu.VMEM((S // D, M, D), F32),
        pltpu.VMEM((AT + 1, S, LANE), BF16),
        pltpu.VMEM((S, 2 * M - AT * LANE), BF16),
        pltpu.SemaphoreType.DMA((XC,)),
        pltpu.SemaphoreType.DMA((KT,)),
        pltpu.SemaphoreType.DMA((QIT,)),
        pltpu.SemaphoreType.DMA((QIT,)),
        pltpu.SemaphoreType.DMA((2,)),
        pltpu.SemaphoreType.DMA((3,)),
        pltpu.SemaphoreType.DMA((S // D + AT,)),
    ]
    return kernel, scratch


_DEFAULT = dict(
    tq=512, a_width=4, ao_at=1, ao_row=240, link_back=176, link_part=32, pace_row=32,
    pace_step=24, use_a=1, h0=0, last_row=216, o_str=(0, 1, 2, 3), o_link=48, o_half=6,
    seq="K0 Q0 K1 Q1 V0 F P0 K2 Q2 O0 V1!2 P1 K3 Q3 O1 V2!1 P2 V3 O2 P3 I!0 O3")


def _build(**kw):
    cfg = dict(_DEFAULT)
    cfg.update(kw)
    kernel, scratch = _make_kernel(cfg)

    def run(A_q, A_k, A_v, A_shift_k, A_ssm_k, A_ssm_D, B_x, B_c_kv, B_w_q, B_w_uk,
            B_w_uv, B_w_o):
        tr = lambda a: jnp.swapaxes(a, 1, 2).reshape(M, S)
        args = (
            tr(A_q), tr(A_k), tr(A_v), A_shift_k.T, A_ssm_k, A_ssm_D, tr(B_x),
            B_c_kv.reshape(S, C),
            B_w_q.reshape(M // 2, 2 * H, D), B_w_uk.reshape(C // 2, 2 * H, D),
            B_w_uv.reshape(C // 2, 2 * H, D),
            jnp.swapaxes(B_w_o, 1, 2),
        )
        out = pl.pallas_call(
            kernel,
            in_specs=[pl.BlockSpec(memory_space=pl.ANY)] * len(args),
            out_specs=pl.BlockSpec(memory_space=pl.ANY),
            out_shape=jax.ShapeDtypeStruct((S, 2 * M), BF16),
            scratch_shapes=scratch,
            compiler_params=pltpu.CompilerParams(
                vmem_limit_bytes=120 * 1024 * 1024,
                disable_bounds_checks=True),
        )(*args)
        return out.reshape(1, S, 2 * M)

    return run


_run = _build()


@jax.jit
def pallas_concat_heads__ssm_conv_h3__compressed_kv_cla__prompt_kernel(
    A_q: jax.Array,
    A_k: jax.Array,
    A_v: jax.Array,
    A_shift_k: jax.Array,
    A_ssm_k: jax.Array,
    A_ssm_D: jax.Array,
    B_x: jax.Array,
    B_c_kv: jax.Array,
    B_w_q: jax.Array,
    B_w_uk: jax.Array,
    B_w_uv: jax.Array,
    B_w_o: jax.Array,
):
    return _run(A_q, A_k, A_v, A_shift_k, A_ssm_k, A_ssm_D, B_x, B_c_kv, B_w_q,
                B_w_uk, B_w_uv, B_w_o)
```

```python
import functools

import jax
import jax.numpy as jnp
from jax import lax
import jax.experimental.pallas as pl
import jax.experimental.pallas.tpu as pltpu

F32 = jnp.float32
BF16 = jnp.bfloat16
U32 = jnp.uint32

S = 2048
M = 448
MP = 512
C = 1024
H = 16
D = 256
KS = 4
LANE = 128
NB = S // LANE
AR = 32
A_STEPS = M // AR
LOG2E = 1.4426950408889634
NEG = -1e30

NT = (((1,), (1,)), ((), ()))


def _dot(a, b):
    return jnp.dot(a, b, preferred_element_type=F32)


def _dot_nt(a, b):
    return lax.dot_general(a, b, NT, preferred_element_type=F32)


def _bf(x):
    return pltpu.bitcast(x, BF16)


def _u32(x):
    return pltpu.bitcast(x, U32)


def _h(r0, n):
    return pl.ds(r0 // 2, n // 2)


def _repack(ev, od):
    lo = (ev & jnp.uint32(0xFFFF)) | (od << 16)
    hi = (ev >> 16) | (od & jnp.uint32(0xFFFF0000))
    return lo, hi


def _split(w):
    return (pltpu.bitcast(w << 16, F32), pltpu.bitcast(w & jnp.uint32(0xFFFF0000), F32))


def _join(lo, hi):
    half = jnp.uint32(0x8000)
    lo = (pltpu.bitcast(lo, U32) + half) >> 16
    hi = (pltpu.bitcast(hi, U32) + half) & jnp.uint32(0xFFFF0000)
    return lo | hi


def _add(a, b):
    return _join(a[0] + b[0], a[1] + b[1])


def _sub(a, b):
    return _join(a[0] - b[0], a[1] - b[1])


def _opaque_zero(vals):
    acc = None
    for v in vals:
        b = v if v.dtype == U32 else pltpu.bitcast(v, U32)
        for r in range(0, b.shape[0], 8):
            for c in range(0, b.shape[1], LANE):
                t = b[r:r + 8, c:c + LANE]
                acc = t if acc is None else acc | t
    return jnp.minimum((acc >> 1).astype(jnp.int32), 0)


def _pin(x, zero, r=0, c=0):
    t = pltpu.bitcast(pltpu.bitcast(x[r:r + 8, c:c + LANE], jnp.int32) + zero, x.dtype)
    row = ([x[r:r + 8, :c]] if c > 0 else []) + [t] + (
        [x[r:r + 8, c + LANE:]] if c + LANE < x.shape[1] else [])
    row = jnp.concatenate(row, axis=1) if len(row) > 1 else row[0]
    col = ([x[:r, :]] if r > 0 else []) + [row] + ([x[r + 8:, :]] if r + 8 < x.shape[0] else [])
    return jnp.concatenate(col, axis=0) if len(col) > 1 else col[0]


def _rowcat(xs):
    return jnp.concatenate(xs, axis=0) if len(xs) > 1 else xs[0]


def _lanecat(xs):
    return jnp.concatenate(xs, axis=1) if len(xs) > 1 else xs[0]


def _make_kernel(cfg):
    tq = cfg["tq"]
    nq = S // tq
    nsub = tq // LANE
    KT = MP // LANE
    TP = LANE // 2
    XC = 4
    x_cols = S // XC
    QP = 2
    QIT = H // 2 // QP
    CP = 176
    AT = 3

    def kernel(aq_hbm, ak_hbm, av_hbm, sh_hbm, ssm_hbm, dd_hbm, x_hbm, c_hbm,
               wq_hbm, wk_hbm, wv_hbm, wo_hbm,
               out_hbm,
               a_v, sh_v, dd_v, par_v, f_v,
               xt_v, x_v, c_v, wqs_v, wq_v, qacc, ws_v, wkv_v, wo_v,
               q_all, k_s, v_s, vb_s, pd_s, pa_s, ra_t, rb_t, oa_v, out_v,
               sem_x, sem_wq, sem_w, sem_c, sem_s, sem_a, sem_out):
        x32, c32, wq32, wk32, wv32, wo32 = (
            r.bitcast(U32) for r in (x_hbm, c_hbm, wq_hbm, wk_hbm, wv_hbm, wo_hbm))
        a32 = [r.bitcast(U32) for r in (ak_hbm, av_hbm, ssm_hbm, aq_hbm)]

        sa_v = qacc

        def x_copy(i):
            cs = pl.ds(i * x_cols, x_cols)
            return pltpu.make_async_copy(x32.at[:, cs], xt_v.at[:, cs], sem_x.at[i])

        def wq_pairs(kt):
            return min(TP, M // 2 - kt * TP)

        def wq_copies(kt):
            n = wq_pairs(kt)
            dst = wqs_v[kt].reshape(4, n, 8, LANE)
            return [pltpu.make_async_copy(
                wq32.at[pl.ds(kt * TP, n), pl.ds(8 * (k // 2), 8), pl.ds((k % 2) * LANE, LANE)],
                dst.at[k], sem_wq.at[kt]) for k in range(4)]

        def wq_wait(kt):
            pltpu.make_async_copy(wqs_v[kt], wqs_v[kt], sem_wq.at[kt]).wait()

        def w_copies(g):
            dst = ws_v.reshape(8, C // 2, 8, LANE)
            src = (wk32, wv32)[g // 2]
            return [pltpu.make_async_copy(
                src.at[:, pl.ds(8 * par, 8), pl.ds((g % 2) * LANE, LANE)],
                dst.at[2 * g + par], sem_w.at[g]) for par in range(2)]

        def w_wait(g):
            pltpu.make_async_copy(ws_v.at[g], ws_v.at[g], sem_w.at[g]).wait()

        c_bounds = [0, CP, 2 * CP, S // 4]

        def c_copies(p):
            r0, n = c_bounds[p], c_bounds[p + 1] - c_bounds[p]
            return [pltpu.make_async_copy(c32.at[rs], c_v.at[rs], sem_c.at[p])
                    for rs in (pl.ds(r0, n), pl.ds(S // 4 + r0, n))]

        wo_copy = pltpu.make_async_copy(wo32, wo_v, sem_a.at[0])

        a_parts = [pl.ds(0, AR // 2), pl.ds(AR // 2, M // 2 - AR // 2)]

        def a_start(part):
            rs = a_parts[part]
            for k in range(4):
                pltpu.make_async_copy(
                    a32[k].at[rs], a_v.at[k, rs], sem_a.at[1 + part]).start()

        def a_wait(part):
            view = a_v.at[:, a_parts[part]]
            pltpu.make_async_copy(view, view, sem_a.at[1 + part]).wait()

        small = [pltpu.make_async_copy(sh_hbm, sh_v, sem_s.at[0]),
                 pltpu.make_async_copy(dd_hbm, dd_v, sem_s.at[1])]

        link = [None]
        pace = [None]

        def set_link(res, row=None, pacer=None):
            if row is None:
                row = res.shape[0] - cfg["link_back"]
            link[0] = _opaque_zero([res[row:row + 8, res.shape[1] - LANE:]])
            pace[0] = res if pacer is None else pacer

        def linked(x):
            return x if link[0] is None else _pin(x, link[0])

        def paced(w):
            res = pace[0]
            if res is None or link[0] is None or not cfg["pace_step"]:
                return w
            rows = []
            r0, step = cfg["pace_row"], cfg["pace_step"]
            if res.shape[0] < 400:
                r0, step = 0, 8
            if res.shape[0] < 200:
                return w
            zs = [_opaque_zero([res[r:r + 8, res.shape[1] - LANE:]])
                  for r in range(r0, r0 + 8 * step, step)]
            for r in range(0, w.shape[0], 8):
                z = zs[7 - (r // 8) % 8]
                t = pltpu.bitcast(w[r:r + 8, :], jnp.int32)
                rows.append(pltpu.bitcast(t + _lanecat([z] * (w.shape[1] // LANE)), U32))
            return _rowcat(rows)

        for cp in small:
            cp.start()
        x_copy(0).start()
        for cp in wq_copies(0):
            cp.start()

        def zero_body(k, carry):
            n = LANE // (S // D)
            bi = lax.broadcasted_iota(jnp.int32, (n, LANE), 0) + k * n
            mi = lax.broadcasted_iota(jnp.int32, (n, LANE), 1)
            ph = ((4 * mi + 1) * bi) & 511
            ang = ph.astype(F32) * (2.0 * 3.141592653589793 / 512.0)
            rs = pl.ds(pl.multiple_of(k * (n // 2), n // 2), n // 2)
            f_v[rs, 0:LANE] = _u32(jnp.cos(ang).astype(BF16))
            f_v[rs, LANE:] = _u32((-jnp.sin(ang)).astype(BF16))

            rb_t[k] = jnp.zeros((M, D), F32)
            cs = pl.ds(pl.multiple_of((k % 4) * D, D), D)
            ra_t[k // 4, 0:LANE, cs] = jnp.zeros((LANE, D), F32)
            ra_t[k // 4, AT * LANE:, cs] = jnp.zeros((M - AT * LANE, D), F32)
            return carry

        lax.fori_loop(0, S // D, zero_body, 0)
        c_v[S // 2:, :] = jnp.zeros((8, C), U32)

        for kt in range(1, KT):
            for cp in wq_copies(kt):
                cp.start()
        with jax.named_scope("small_wait"):
            for cp in small:
                cp.wait()
        sh = sh_v[...].astype(F32)
        for j in range(KS):
            par_v[j] = jnp.broadcast_to(sh[j:j + 1, :], (LANE, M)).T
        dd = dd_v[...].astype(F32).reshape(1, M)
        par_v[KS] = jnp.broadcast_to(dd, (LANE, M)).T

        def x_transpose(i):
            xt = xt_v[:, pl.ds(i * x_cols, x_cols)]
            xt = _rowcat([xt, jnp.zeros((MP // 2 - M // 2, x_cols), U32)])
            x_v[_h(i * x_cols, x_cols), :] = _u32(_bf(xt).astype(F32).T.astype(BF16))

        def q_early(kt, keep=False):
            first, last = kt == 0, kt == KT - 1
            n = wq_pairs(kt)
            cols = pl.ds(kt * LANE, LANE)
            if not keep:
                link[0] = None
            for j in range(H // 2):
                ws = []
                for half in range(2):
                    ev, od = (wqs_v[kt][pl.ds((2 * par + half) * n * 8 + j, n, stride=8), :]
                              for par in range(2))
                    ws.append(_repack(ev, od))
                w = _lanecat([ws[0][0], ws[1][0], ws[0][1], ws[1][1]])
                if n < TP:
                    w = _rowcat([w, jnp.zeros((TP - n, 2 * D), U32)])
                wq_v[j, pl.ds(kt * TP, TP), :] = w
                d = _dot(_bf(linked(x_v[_h(0, x_cols), cols])), _bf(w))
                set_link(d)
                if not first:
                    d = d + pltpu.bitcast(qacc[j], F32)
                if last:
                    d = (d * (D ** -0.5 * LOG2E)).astype(BF16)
                    for t in range(2):
                        q_all[2 * j + t, _h(0, x_cols), :] = _u32(d[:, t * D:(t + 1) * D])
                else:
                    qacc[j] = pltpu.bitcast(d, U32)

        with jax.named_scope("x_wait"):
            x_copy(0).wait()
        x_transpose(0)
        for i in range(1, XC):
            x_copy(i).start()
        for g in range(QIT):
            for cp in w_copies(g) + (c_copies(g) if g < QIT - 1 else []):
                cp.start()
        wo_copy.start()
        a_start(0)
        a_start(1)
        with jax.named_scope("wq_wait"):
            wq_wait(0)
        q_early(0)
        with jax.named_scope("wq_wait"):
            wq_wait(1)
            wq_wait(2)
        q_early(1)
        q_early(2, keep=True)
        with jax.named_scope("wq_wait"):
            wq_wait(3)
            for i in range(1, XC):
                x_copy(i).wait()
        q_early(3)
        for i in range(1, XC):
            x_transpose(i)

        def unpack(g, sub, j):
            ev, od = (ws_v[g, pl.ds((par * (C // 2) + sub * TP) * 8 + j, TP, stride=8), :]
                      for par in range(2))
            lo, hi = _repack(ev, od)
            rows = pl.ds(sub * TP, TP)
            cols = pl.ds(pl.multiple_of(g * LANE, LANE), LANE)
            wkv_v[2 * j, rows, cols] = lo
            wkv_v[2 * j + 1, rows, cols] = hi
            return [lo, hi]

        def a_sums(it, u):
            r0 = jnp.clip((it - 1) * CP, 0, S // 4 - CP) + 8 * u
            src = [jnp.where(it == 0, S // 2, r0 + rb * (S // 4)) for rb in range(2)]
            r0 = pl.multiple_of(r0, 8)
            kw = C // 2
            a11, a12, a21, a22 = (
                _split(c_v[pl.ds(pl.multiple_of(src[rb], 8), 8), pl.ds(cb * kw, kw)])
                for rb in range(2) for cb in range(2))
            outs = [_add(a11, a22), _add(a21, a22), _add(a11, a12), _sub(a21, a11),
                    _sub(a12, a22)]
            for k, o in enumerate(outs):
                sa_v[k, pl.ds(r0, 8), :] = o
            return outs

        units = [functools.partial(unpack, sub=s_, j=j_)
                 for s_ in range(C // 2 // TP) for j_ in range(H // 2)]
        for u_ in range(CP // 8):
            units.insert(4 * u_ + 1, functools.partial(a_sums, u=u_))

        def qproj(it, r0, n, t, zeros=(None, None)):
            outs = []
            for u in range(2):
                lhs = _bf(linked(x_v[_h(r0, n), :]))
                d = _dot(lhs, _bf(wq_v[it, :, pl.ds(t * D + u * LANE, LANE)]))
                set_link(d)
                if zeros[u] is not None:
                    for k, z in enumerate(zeros[u]):
                        d = _pin(d, z, 8 * ((k * (n // 8)) // len(zeros[u])))
                outs.append(d)
            q2 = _lanecat(outs)
            q_all[2 * it + t, _h(r0, n), :] = _u32((q2 * (D ** -0.5 * LOG2E)).astype(BF16))

        def q_body(it, carry):
            with jax.named_scope("w_wait"):
                w_wait(it)
                for p in range(QIT - 1):
                    @pl.when(it == p + 1)
                    def _():
                        for cp in c_copies(p):
                            cp.wait()
            link[0] = None
            pieces = [(p, pc, t) for p in range(QP) for pc in range(1, XC) for t in range(2)]
            nd = 2 * len(pieces)
            for k, (p, pc, t) in enumerate(pieces):
                zeros = []
                for u in range(2):
                    d = 2 * k + u
                    mine = units[d * len(units) // nd:(d + 1) * len(units) // nd]
                    zeros.append([_opaque_zero(u_(it)) for u_ in mine])
                qproj(QP * it + p, pc * x_cols, x_cols, t, zeros)
            return carry

        with jax.named_scope("q_loop"):
            lax.fori_loop(0, QIT, q_body, 0)
        wo_copy.wait()
        a_wait(0)

        tri = (lax.broadcasted_iota(jnp.int32, (LANE, LANE), 1)
               <= lax.broadcasted_iota(jnp.int32, (LANE, LANE), 0))

        NOUT = S // D

        def out_copy(i):
            if i >= NOUT:
                t = i - NOUT
                return pltpu.make_async_copy(
                    oa_v.at[t], out_hbm.at[:, pl.ds(t * LANE, LANE)], sem_out.at[i])
            rs = pl.ds(i * D, D)
            return pltpu.make_async_copy(
                out_v.at[rs], out_hbm.at[rs, pl.ds(AT * LANE, 2 * M - AT * LANE)], sem_out.at[i])

        n_body = NOUT - (tq // D if nq - 1 in cfg["o_str"] else 1)

        def b_out(k, tot):
            c0 = (k * D) % (S // 2)
            full = _rowcat([ra_t[k * D // (S // 2), AT * LANE:, c0:c0 + D], tot]).T
            out_v[k * D:(k + 1) * D, :] = full.astype(BF16)
            return full

        def head_step(h, carry):
            with jax.named_scope("step"):
                return head_step_(h, carry)

        def head_step_(h, carry):
            with_a = cfg["use_a"]

            @pl.when(h == A_STEPS)
            def _():
                for t in range(AT):
                    out_copy(NOUT + t).start()

            @pl.when(h == cfg["h0"] + 1)
            def _():
                a_wait(1)

            link[0] = None
            n2 = AR // 2
            a_rows2 = pl.ds(pl.multiple_of(jnp.minimum(h, A_STEPS - 1) * n2, n2), n2)
            a_rows = pl.ds(pl.multiple_of(jnp.minimum(h, A_STEPS - 1) * AR, AR), AR)

            kw = C // 2
            pending = []
            chains = {i: [] for i in range(nq)}
            deadline = [None]

            def flush_pending(x, row):
                done = list(pending)
                del pending[:]
                if not done:
                    return x
                x = _pin(x, _opaque_zero([f for _, f in done]), row)

                @pl.when(h == H - 1)
                def _():
                    for k, _f in done:
                        out_copy(k).start()
                return x

            def a_fwd():
                kk = _bf(a_v[0, a_rows2, :]).astype(F32)
                lane = lax.broadcasted_iota(jnp.int32, (AR, LANE), 1)
                coef = [par_v[j, a_rows, :] for j in range(KS)]
                rolled = [kk] + [pltpu.roll(kk, j, 1) for j in range(1, KS)]
                vv = _bf(a_v[1, a_rows2, :]).astype(F32)
                kv_blocks = []
                for a in range(NB):
                    cs = slice(a * LANE, (a + 1) * LANE)
                    acc = rolled[0][:, cs] * coef[0]
                    for j in range(1, KS):
                        t = rolled[j][:, cs]
                        if a == 0:
                            t = jnp.where(lane >= j, t, 0.0)
                        acc = acc + t * coef[j]
                    kv_blocks.append(acc * vv[:, cs])
                hk = a_v[2, a_rows2, :]
                hk = _rowcat([hk[:, a * LANE:(a + 1) * LANE] for a in range(NB)])
                fm = _bf(f_v[...])
                hs = _dot(_bf(linked(hk)), fm)
                kv = linked(_rowcat(kv_blocks)).astype(BF16)
                xs = _dot(kv, fm)
                set_link(xs)
                return kv, xs, hs

            def a_conv(xs, hs):
                def tile(v, a, g, part):
                    r = a * AR + 8 * g
                    return v[r:r + 8, part * LANE:(part + 1) * LANE]

                z = {}
                gate = None
                width = cfg["a_width"]
                for g in range(AR // 8):
                    hr = [tile(hs, 0, g, 0)] + [
                        tile(hs, j, g, 0) - tile(hs, j - 1, g, 1) for j in range(1, NB)]
                    hi = [tile(hs, 0, g, 1)] + [
                        tile(hs, j, g, 1) + tile(hs, j - 1, g, 0) for j in range(1, NB)]
                    for c0 in range(0, NB, width):
                        for a in range(c0 + width):
                            xr, xi = tile(xs, a, g, 0), tile(xs, a, g, 1)
                            if gate is not None:
                                xr, xi = _pin(xr, gate), _pin(xi, gate)
                            for c in range(max(c0, a), c0 + width):
                                j = c - a
                                tr = xr * hr[j] - xi * hi[j]
                                ti = xr * hi[j] + xi * hr[j]
                                z[c, g] = (tr, ti) if a == 0 else (z[c, g][0] + tr, z[c, g][1] + ti)
                            gate = _opaque_zero(list(z[c0 + width - 1, g]))
                return z

            def a_inv(kv, z, flush=False):
                fm = _bf(f_v[...])
                ng = AR // 8
                ys = []
                for u in range(2):
                    rows = [_lanecat(z[c, g]) for g in range(u * ng // 2, (u + 1) * ng // 2)
                            for c in range(NB)]
                    lhs = linked(_rowcat(rows))
                    if flush:
                        lhs = flush_pending(lhs, 8)
                    ys.append(_dot_nt(lhs.astype(BF16), fm))
                y = _rowcat(ys)
                dd = par_v[KS, a_rows, :]
                for c in range(NB):
                    cs = slice(c * LANE, (c + 1) * LANE)
                    yc = _rowcat([y[(g * NB + c) * 8:(g * NB + c + 1) * 8, :] for g in range(ng)])
                    qq = _bf(a_v[3, a_rows2, cs]).astype(F32)
                    kvf = kv[c * AR:(c + 1) * AR, :].astype(F32)
                    c2 = (c % (NB // 2)) * LANE
                    ra_t[c // (NB // 2), a_rows, c2:c2 + LANE] = qq * (yc * (1.0 / LANE) + kvf * dd)

            def a_out():
                slab = jnp.clip(h // 4 - 1, 0, AT - 1)
                half = h % 2
                x = ra_t[half, pl.ds(pl.multiple_of(slab * LANE, LANE), LANE), :]
                xt = x.T
                dst = jnp.where(h >= A_STEPS, AT, slab)
                oa_v[dst, pl.ds(pl.multiple_of(half * (S // 2), S // 2), S // 2), :] = xt.astype(BF16)
                return xt

            def w_blk(r, c):
                return wkv_v[h, _h(r * kw, kw), pl.ds(c * LANE, LANE)]

            def one_pass(lhs, w, flush):
                lhs = linked(lhs)
                if flush:
                    lhs = flush_pending(lhs, cfg["ao_row"])
                if deadline[0] is not None:
                    if deadline[0][0] == 0:
                        lhs = _pin(lhs, deadline[0][1], cfg["ao_row"] - 8)
                        deadline[0] = None
                    else:
                        deadline[0] = (deadline[0][0] - 1, deadline[0][1])
                d = _dot(_bf(lhs), _bf(paced(w)))
                set_link(d)
                return d

            def k_proj(blk, flush=-1):
                ds = [one_pass(c_v[_h(blk * tq, tq), pl.ds((k % 2) * kw, kw)],
                               w_blk(k % 2, k // 2), k == flush) for k in range(4)]
                k_s[_h(blk * tq, tq), :] = _u32(
                    _lanecat([ds[0] + ds[1], ds[2] + ds[3]]).astype(BF16))

            def b_op(m):
                blk = lambda r, c: _split(w_blk(r, 2 + c))
                return {1: lambda: _add(blk(0, 0), blk(1, 1)),
                        2: lambda: w_blk(0, 2),
                        3: lambda: _sub(blk(0, 1), blk(1, 1)),
                        4: lambda: _sub(blk(1, 0), blk(0, 0)),
                        5: lambda: w_blk(1, 3),
                        6: lambda: _add(blk(0, 0), blk(0, 1)),
                        7: lambda: _add(blk(1, 0), blk(1, 1))}[m]()

            def a_op(m, rho):
                rs = _h(rho * tq, tq)
                if m == 3:
                    return c_v[rs, 0:kw]
                if m == 4:
                    return c_v[_h(S // 2 + rho * tq, tq), kw:]
                return sa_v[{1: 0, 2: 1, 5: 2, 6: 3, 7: 4}[m], rs, :]

            b_cache, prod = {}, {}

            def v_proj(blk, flush=-1):
                rho = blk % 2
                for k, m in enumerate((5, 1, 4, 7, 3) if blk < 2 else (2, 6)):
                    if m not in b_cache:
                        b_cache[m] = b_op(m)
                    prod[m, rho] = one_pass(a_op(m, rho), b_cache[m], k == flush)
                p = lambda m: prod[m, rho]
                if blk < 2:
                    v = [(p(1) + p(4)) + (p(7) - p(5)), p(3) + p(5)]
                else:
                    v = [p(2) + p(4), (p(1) + p(3)) + (p(6) - p(2))]
                v_s[_h(blk * tq, tq), :] = _u32(_lanecat(v).astype(BF16))
                if blk < nq - 1:
                    b = lambda r, c: v[c][r * D:(r + 1) * D, :]
                    sums = [b(0, 0) + b(1, 1), b(0, 1) - b(1, 1), b(1, 0) - b(0, 0),
                            b(0, 0) + b(0, 1), b(1, 0) + b(1, 1)]
                    for k, x in enumerate(sums):
                        vb_s[k, _h(blk * D, D), :] = _u32(x.astype(BF16))

            def qk(i, dep=None, flush=False):
                r0 = i * tq
                q = linked(q_all[h, _h(r0, tq), :])
                if dep is not None:
                    q = _pin(q, _opaque_zero([dep]), cfg["ao_row"])
                parts = [_dot_nt(_bf(q), _bf(k_s[_h(0, r0 + LANE), :]))]
                early = None
                if i > 0:
                    link[0] = _opaque_zero([parts[0][0:8, r0 - LANE:r0]])
                    ne = r0 // LANE - cfg["max_late"]
                    if cfg["max_late"] and ne > 1:
                        early = (ne, functools.reduce(jnp.maximum, [
                            parts[0][:, t * LANE:(t + 1) * LANE] for t in range(ne)]))
                for j in range(1, nsub):
                    q = linked(q_all[h, _h(r0 + LANE * j, tq - LANE * j), :])
                    if j == cfg["q_pin"]:
                        if flush:
                            q = flush_pending(q, 8)
                        if early is not None:
                            q = _pin(q, _opaque_zero([early[1]]), 16)
                    parts.append(_dot_nt(_bf(q), _bf(k_s[_h(r0 + LANE * j, LANE), :])))
                set_link(parts[2], cfg["link_part"], parts[0])
                return parts, early

            def exps(i, parts, early):
                sas, mbs = [], []
                for a in range(nsub):
                    blocks = [parts[j][LANE * (a - j):LANE * (a - j + 1), :] for j in range(a + 1)]
                    last = blocks[-1]
                    w = last.shape[1]
                    dg = jnp.where(tri, last[:, w - LANE:], NEG)
                    blocks[-1] = dg if w == LANE else _lanecat([last[:, :w - LANE], dg])
                    sas.append(_lanecat(blocks))
                    mx = sas[a]
                    if early is not None:
                        mx = _lanecat([early[1][LANE * a:LANE * (a + 1)], mx[:, early[0] * LANE:]])
                    mbs.append(jnp.broadcast_to(jnp.max(mx, axis=1, keepdims=True), (LANE, LANE)))
                chain = _opaque_zero([b[b.shape[0] - 8:, b.shape[1] - LANE:] for b in parts])
                pg, psums = {}, {}
                for r in range(0, tq // 2, 8):
                    for row in (r, r + tq // 2):
                        a, g = divmod(row, LANE)
                        mg = _pin(mbs[a][g:g + 8, :], chain)
                        pg[row] = [jnp.exp2(sas[a][g:g + 8, t:t + LANE] - mg)
                                   for t in range(0, sas[a].shape[1], LANE)]
                        psums[row] = functools.reduce(jnp.add, pg[row])
                        chain = _opaque_zero([psums[row]])
                        chains[i].append(chain)
                return pg, psums

            def softmax(i, pg, psums):
                r0 = i * tq
                pd, pa = pd_s.at[i % 2], pa_s[i % 2]
                first = lambda x, c=0: _pin(x, link[0], 0, c).astype(BF16)
                nt0 = r0 // LANE
                ls = []
                for a in range(nsub):
                    rows = range(LANE * a, LANE * (a + 1), 8)
                    ls.append(jnp.sum(_rowcat([psums[r] for r in rows]), axis=1, keepdims=True))
                    pd[LANE * a:LANE * (a + 1), 0:LANE * (a + 1)] = first(
                        _rowcat([_lanecat(pg[r][nt0:]) for r in rows]), LANE * a)
                if i > 0:
                    quad = lambda rh, ch: _rowcat([
                        _lanecat([pg[rh * (tq // 2) + r][4 * j + 2 * ch + t]
                                  for j in range(i) for t in range(2)])
                        for r in range(0, tq // 2, 8)])
                    a11, a12, a21, a22 = quad(0, 0), quad(0, 1), quad(1, 0), quad(1, 1)
                    ops = [a11 + a22, a21 + a22, a11, a22, a11 + a12, a21 - a11, a12 - a22]
                    for m, x in enumerate(ops):
                        if i == 3:
                            x = _pin(x, link[0], 0, 2 * D)
                        pa[m, :, 0:i * D] = first(x)
                return ls

            def pv(i, ls):
                r0 = i * tq
                pd, pa = pd_s.at[i % 2], pa_s[i % 2]
                off = None
                if i > 0:
                    def b_rows(m, j0, j1):
                        if m in (2, 5):
                            q = 0 if m == 2 else 1
                            return _bf(_rowcat([
                                v_s[_h(j * tq + q * D, D), q * LANE:(q + 1) * LANE]
                                for j in range(j0, j1)]))
                        k = {1: 0, 3: 1, 4: 2, 6: 3, 7: 4}[m]
                        return _bf(vb_s[k, _h(j0 * D, (j1 - j0) * D), :])

                    p = {}
                    for j0, j1 in {1: [(0, 1)], 2: [(0, 2)], 3: [(0, 2), (2, 3)]}[i]:
                        for m in range(1, 8):
                            cols = slice(j0 * D, j1 * D)
                            rhs = b_rows(m, j0, j1)
                            if j1 - j0 == 1 and m == 7:
                                d = _rowcat([_dot(pa[m - 1, r:r + LANE, cols], rhs)
                                             for r in (0, LANE)])
                            else:
                                d = _dot(pa[m - 1, :, cols], rhs)
                            p[m] = d if m not in p else p[m] + d
                    off = _rowcat([
                        _lanecat([(p[1] + p[4]) + (p[7] - p[5]), p[3] + p[5]]),
                        _lanecat([p[2] + p[4], (p[1] + p[3]) + (p[6] - p[2])])])
                ctx = []
                for j in range(nsub):
                    c0 = LANE * j
                    ctx.append(_dot(pd[c0:, c0:c0 + LANE], _bf(v_s[_h(r0 + c0, LANE), :])))
                set_link(ctx[2], cfg["link_part"], ctx[0])
                cs = []
                for a in range(nsub):
                    sl = lambda j: slice(LANE * (a - j), LANE * (a - j + 1))
                    r = pl.reciprocal(ls[a], approx=True)
                    r = r * (2.0 - ls[a] * r)
                    terms = [ctx[j][sl(j)] for j in range(a + 1)]
                    if off is not None:
                        terms.append(off[sl(0)])
                    cs.append(functools.reduce(jnp.add, terms) * r)
                return _rowcat(cs)

            def accumulate(k, res):
                tot = rb_t[k] + res
                rb_t[k] = tot
                if k < n_body:
                    pending.append((k, b_out(k, tot)))

            def oproj_plain(i, ctx):
                ctx = ctx.astype(BF16)
                for u in range(tq // D):
                    lhs = linked(wo_v[h])
                    if i == nq - 1:
                        lhs = flush_pending(lhs, cfg["last_row"])
                    res = _dot_nt(_bf(lhs), ctx[u * D:(u + 1) * D, :])
                    set_link(res)
                    accumulate(i * (tq // D) + u, res)

            wo_cache = {}

            def oproj(i, ctx):
                if i not in cfg["o_str"]:
                    return oproj_plain(i, ctx)
                mh = M // 4
                raw = lambda r, c: wo_v[h, r * mh:(r + 1) * mh, c * LANE:(c + 1) * LANE]
                a = lambda r, c: _split(raw(r, c))
                a_ops = {1: lambda: _add(a(0, 0), a(1, 1)), 2: lambda: _add(a(1, 0), a(1, 1)),
                         3: lambda: raw(0, 0), 4: lambda: raw(1, 1),
                         5: lambda: _add(a(0, 0), a(0, 1)), 6: lambda: _sub(a(1, 0), a(0, 0)),
                         7: lambda: _sub(a(0, 1), a(1, 1))}
                b = lambda r, c: ctx[c * D:(c + 1) * D, r * LANE:(r + 1) * LANE]
                b_ops = {1: lambda: b(0, 0) + b(1, 1), 2: lambda: b(0, 0),
                         3: lambda: b(0, 1) - b(1, 1), 4: lambda: b(1, 0) - b(0, 0),
                         5: lambda: b(1, 1), 6: lambda: b(0, 0) + b(0, 1),
                         7: lambda: b(1, 0) + b(1, 1)}
                p = {}
                for n, m in enumerate((5, 2, 4, 1, 7, 3, 6)):
                    if m not in wo_cache:
                        wo_cache[m] = a_ops[m]()
                    rhs = b_ops[m]().astype(BF16)
                    if n == cfg["o_half"]:
                        halves = [_dot_nt(_bf(linked(wo_cache[m][r:r + mh // 2])), rhs)
                                  for r in (0, mh // 2)]
                        p[m] = _rowcat(halves)
                        set_link(halves[1], 0)
                    else:
                        p[m] = _dot_nt(_bf(linked(wo_cache[m])), rhs)
                        if (n - (n > cfg["o_half"])) % 2 == 1:
                            set_link(p[m], cfg["o_link"])
                accumulate(2 * i, _rowcat([(p[1] + p[4]) + (p[7] - p[5]), p[2] + p[4]]))
                accumulate(2 * i + 1, _rowcat([p[3] + p[5], (p[1] + p[3]) + (p[6] - p[2])]))

            st = {}
            for op in cfg["seq"].split():
                op, _, dl = op.partition("@")
                if dl:
                    ch = chains[int(dl[0])]
                    deadline[0] = (int(dl[1]), ch[int(dl[2:]) * len(ch) // 16 - 1])
                op, _, fl = op.partition("!")
                fl = int(fl) if fl else -1
                kind, i = op[0], int(op[1:] or 0)
                if kind == "K":
                    k_proj(i, fl)
                elif kind == "V":
                    v_proj(i, fl)
                elif kind == "Q":
                    st["e", i] = exps(
                        i, *qk(i, a_out() if i == cfg["ao_at"] else None, fl >= 0))
                elif kind == "P":
                    st["ctx", i] = pv(i, softmax(i, *st["e", i]))
                elif kind == "O":
                    oproj(i, st["ctx", i])
                elif kind == "F" and with_a:
                    st["kv"], xs, hs = a_fwd()
                    st["z"] = a_conv(xs, hs)
                elif kind == "I" and with_a:
                    a_inv(st["kv"], st["z"], fl >= 0)
            assert not pending and deadline[0] is None
            return carry

        with jax.named_scope("loop_a"):
            lax.fori_loop(cfg["h0"], H, head_step, 0)
        with jax.named_scope("tail"):
            for i in range(n_body, NOUT):
                b_out(i, rb_t[i])
                out_copy(i).start()
            for i in range(NOUT + AT):
                out_copy(i).wait()

    scratch = [
        pltpu.VMEM((4, M // 2, S), U32),
        pltpu.VMEM((KS, M), BF16),
        pltpu.VMEM((M,), BF16),
        pltpu.VMEM((KS + 1, M, LANE), F32),
        pltpu.VMEM((LANE // 2, 2 * LANE), U32),
        pltpu.VMEM((M // 2, S), U32),
        pltpu.VMEM((S // 2, MP), U32),
        pltpu.VMEM((S // 2 + 8, C), U32),
        [pltpu.VMEM((4 * min(TP, M // 2 - kt * TP) * 8, LANE), U32)
         for kt in range(KT)],
        pltpu.VMEM((H // 2, MP // 2, 2 * D), U32),
        pltpu.VMEM((H // 2, x_cols, 2 * D), U32),
        pltpu.VMEM((QIT, C * 8, LANE), U32),
        pltpu.VMEM((H, C // 2, 2 * D), U32),
        pltpu.VMEM((H, M // 2, D), U32),
        pltpu.VMEM((H, S // 2, D), U32),
        pltpu.VMEM((S // 2, D), U32),
        pltpu.VMEM((S // 2, D), U32),
        pltpu.VMEM((5, (nq - 1) * D // 2, LANE), U32),
        pltpu.VMEM((2, tq, tq), BF16),
        [pltpu.VMEM((7, tq // 2, n * D), BF16) for n in (2, 3)],
        pltpu.VMEM((2, M, S // 2), F32),
        pltpu.VMEM((S // D, M, D), F32),
        pltpu.VMEM((AT + 1, S, LANE), BF16),
        pltpu.VMEM((S, 2 * M - AT * LANE), BF16),
        pltpu.SemaphoreType.DMA((XC,)),
        pltpu.SemaphoreType.DMA((KT,)),
        pltpu.SemaphoreType.DMA((QIT,)),
        pltpu.SemaphoreType.DMA((QIT,)),
        pltpu.SemaphoreType.DMA((2,)),
        pltpu.SemaphoreType.DMA((3,)),
        pltpu.SemaphoreType.DMA((S // D + AT,)),
    ]
    return kernel, scratch


_DEFAULT = dict(
    tq=512, a_width=4, ao_at=1, ao_row=240, link_back=176, link_part=32, pace_row=32,
    pace_step=24, use_a=1, h0=0, last_row=216, o_str=(0, 1, 2, 3), o_link=48, o_half=6, max_late=0, q_pin=2,
    seq="K0 Q0 K1 Q1 V0 F P0 K2@1316 O0 Q2!0 V1 P1 K3@2316 O1 Q3!0 V2 P2 V3@3116 O2 P3 I!0 O3")


def _build(**kw):
    cfg = dict(_DEFAULT)
    cfg.update(kw)
    kernel, scratch = _make_kernel(cfg)

    def run(A_q, A_k, A_v, A_shift_k, A_ssm_k, A_ssm_D, B_x, B_c_kv, B_w_q, B_w_uk,
            B_w_uv, B_w_o):
        tr = lambda a: jnp.swapaxes(a, 1, 2).reshape(M, S)
        args = (
            tr(A_q), tr(A_k), tr(A_v), A_shift_k.T, A_ssm_k, A_ssm_D, tr(B_x),
            B_c_kv.reshape(S, C),
            B_w_q.reshape(M // 2, 2 * H, D), B_w_uk.reshape(C // 2, 2 * H, D),
            B_w_uv.reshape(C // 2, 2 * H, D),
            jnp.swapaxes(B_w_o, 1, 2),
        )
        out = pl.pallas_call(
            kernel,
            in_specs=[pl.BlockSpec(memory_space=pl.ANY)] * len(args),
            out_specs=pl.BlockSpec(memory_space=pl.ANY),
            out_shape=jax.ShapeDtypeStruct((S, 2 * M), BF16),
            scratch_shapes=scratch,
            compiler_params=pltpu.CompilerParams(
                vmem_limit_bytes=126 * 1024 * 1024,
                disable_bounds_checks=True),
        )(*args)
        return out.reshape(1, S, 2 * M)

    return run


_run = _build()


@jax.jit
def pallas_concat_heads__ssm_conv_h3__compressed_kv_cla__prompt_kernel(
    A_q: jax.Array,
    A_k: jax.Array,
    A_v: jax.Array,
    A_shift_k: jax.Array,
    A_ssm_k: jax.Array,
    A_ssm_D: jax.Array,
    B_x: jax.Array,
    B_c_kv: jax.Array,
    B_w_q: jax.Array,
    B_w_uk: jax.Array,
    B_w_uv: jax.Array,
    B_w_o: jax.Array,
):
    return _run(A_q, A_k, A_v, A_shift_k, A_ssm_k, A_ssm_D, B_x, B_c_kv, B_w_q,
                B_w_uk, B_w_uv, B_w_o)
```

```python
import functools

import jax
import jax.numpy as jnp
from jax import lax
import jax.experimental.pallas as pl
import jax.experimental.pallas.tpu as pltpu

F32 = jnp.float32
BF16 = jnp.bfloat16
U32 = jnp.uint32

S = 2048
M = 448
MP = 512
C = 1024
H = 16
D = 256
KS = 4
LANE = 128
NB = S // LANE
AR = 32
A_STEPS = M // AR
LOG2E = 1.4426950408889634
NEG = -1e30

NT = (((1,), (1,)), ((), ()))


def _dot(a, b):
    return jnp.dot(a, b, preferred_element_type=F32)


def _dot_nt(a, b):
    return lax.dot_general(a, b, NT, preferred_element_type=F32)


def _bf(x):
    return pltpu.bitcast(x, BF16)


def _u32(x):
    return pltpu.bitcast(x, U32)


def _h(r0, n):
    return pl.ds(r0 // 2, n // 2)


def _repack(ev, od):
    lo = (ev & jnp.uint32(0xFFFF)) | (od << 16)
    hi = (ev >> 16) | (od & jnp.uint32(0xFFFF0000))
    return lo, hi


def _split(w):
    return (pltpu.bitcast(w << 16, F32), pltpu.bitcast(w & jnp.uint32(0xFFFF0000), F32))


def _join(lo, hi):
    half = jnp.uint32(0x8000)
    lo = (pltpu.bitcast(lo, U32) + half) >> 16
    hi = (pltpu.bitcast(hi, U32) + half) & jnp.uint32(0xFFFF0000)
    return lo | hi


def _add(a, b):
    return _join(a[0] + b[0], a[1] + b[1])


def _sub(a, b):
    return _join(a[0] - b[0], a[1] - b[1])


def _opaque_zero(vals):
    acc = None
    for v in vals:
        b = v if v.dtype == U32 else pltpu.bitcast(v, U32)
        for r in range(0, b.shape[0], 8):
            for c in range(0, b.shape[1], LANE):
                t = b[r:r + 8, c:c + LANE]
                acc = t if acc is None else acc | t
    return jnp.minimum((acc >> 1).astype(jnp.int32), 0)


def _pin(x, zero, r=0, c=0):
    t = pltpu.bitcast(pltpu.bitcast(x[r:r + 8, c:c + LANE], jnp.int32) + zero, x.dtype)
    row = ([x[r:r + 8, :c]] if c > 0 else []) + [t] + (
        [x[r:r + 8, c + LANE:]] if c + LANE < x.shape[1] else [])
    row = jnp.concatenate(row, axis=1) if len(row) > 1 else row[0]
    col = ([x[:r, :]] if r > 0 else []) + [row] + ([x[r + 8:, :]] if r + 8 < x.shape[0] else [])
    return jnp.concatenate(col, axis=0) if len(col) > 1 else col[0]


def _rowcat(xs):
    return jnp.concatenate(xs, axis=0) if len(xs) > 1 else xs[0]


def _lanecat(xs):
    return jnp.concatenate(xs, axis=1) if len(xs) > 1 else xs[0]


def _make_kernel(cfg):
    tq = cfg["tq"]
    nq = S // tq
    nsub = tq // LANE
    KT = MP // LANE
    TP = LANE // 2
    XC = 4
    x_cols = S // XC
    QP = 2
    QIT = H // 2 // QP
    CP = 176
    AT = 3

    def kernel(aq_hbm, ak_hbm, av_hbm, sh_hbm, ssm_hbm, dd_hbm, x_hbm, c_hbm,
               wq_hbm, wk_hbm, wv_hbm, wo_hbm,
               out_hbm,
               a_v, sh_v, dd_v, par_v, f_v,
               xt_v, x_v, c_v, wqs_v, wq_v, qacc, ws_v, wkv_v, wo_v,
               q_all, k_s, v_s, vb_s, pd_s, pa_s, ra_t, rb_t, oa_v, out_v,
               sem_x, sem_wq, sem_w, sem_c, sem_s, sem_a, sem_out):
        x32, c32, wq32, wk32, wv32, wo32 = (
            r.bitcast(U32) for r in (x_hbm, c_hbm, wq_hbm, wk_hbm, wv_hbm, wo_hbm))
        a32 = [r.bitcast(U32) for r in (ak_hbm, av_hbm, ssm_hbm, aq_hbm)]

        sa_v = qacc

        def x_copy(i):
            cs = pl.ds(i * x_cols, x_cols)
            return pltpu.make_async_copy(x32.at[:, cs], xt_v.at[:, cs], sem_x.at[i])

        def wq_pairs(kt):
            return min(TP, M // 2 - kt * TP)

        def wq_copies(kt):
            n = wq_pairs(kt)
            dst = wqs_v[kt].reshape(4, n, 8, LANE)
            return [pltpu.make_async_copy(
                wq32.at[pl.ds(kt * TP, n), pl.ds(8 * (k // 2), 8), pl.ds((k % 2) * LANE, LANE)],
                dst.at[k], sem_wq.at[kt]) for k in range(4)]

        def wq_wait(kt):
            pltpu.make_async_copy(wqs_v[kt], wqs_v[kt], sem_wq.at[kt]).wait()

        def w_copies(g):
            dst = ws_v.reshape(8, C // 2, 8, LANE)
            src = (wk32, wv32)[g // 2]
            return [pltpu.make_async_copy(
                src.at[:, pl.ds(8 * par, 8), pl.ds((g % 2) * LANE, LANE)],
                dst.at[2 * g + par], sem_w.at[g]) for par in range(2)]

        def w_wait(g):
            pltpu.make_async_copy(ws_v.at[g], ws_v.at[g], sem_w.at[g]).wait()

        c_bounds = [0, CP, 2 * CP, S // 4]

        def c_copies(p):
            r0, n = c_bounds[p], c_bounds[p + 1] - c_bounds[p]
            return [pltpu.make_async_copy(c32.at[rs], c_v.at[rs], sem_c.at[p])
                    for rs in (pl.ds(r0, n), pl.ds(S // 4 + r0, n))]

        wo_copy = pltpu.make_async_copy(wo32, wo_v, sem_a.at[0])

        a_parts = [pl.ds(0, AR // 2), pl.ds(AR // 2, M // 2 - AR // 2)]

        def a_start(part):
            rs = a_parts[part]
            for k in range(4):
                pltpu.make_async_copy(
                    a32[k].at[rs], a_v.at[k, rs], sem_a.at[1 + part]).start()

        def a_wait(part):
            view = a_v.at[:, a_parts[part]]
            pltpu.make_async_copy(view, view, sem_a.at[1 + part]).wait()

        small = [pltpu.make_async_copy(sh_hbm, sh_v, sem_s.at[0]),
                 pltpu.make_async_copy(dd_hbm, dd_v, sem_s.at[1])]

        link = [None]
        pace = [None]

        def set_link(res, row=None, pacer=None):
            if row is None:
                row = res.shape[0] - cfg["link_back"]
            link[0] = _opaque_zero([res[row:row + 8, res.shape[1] - LANE:]])
            pace[0] = res if pacer is None else pacer

        def linked(x):
            return x if link[0] is None else _pin(x, link[0])

        def paced(w):
            res = pace[0]
            if res is None or link[0] is None or not cfg["pace_step"]:
                return w
            rows = []
            r0, step = cfg["pace_row"], cfg["pace_step"]
            if res.shape[0] < 400:
                r0, step = 0, 8
            if res.shape[0] < 200:
                return w
            zs = [_opaque_zero([res[r:r + 8, res.shape[1] - LANE:]])
                  for r in range(r0, r0 + 8 * step, step)]
            for r in range(0, w.shape[0], 8):
                z = zs[7 - (r // 8) % 8]
                t = pltpu.bitcast(w[r:r + 8, :], jnp.int32)
                rows.append(pltpu.bitcast(t + _lanecat([z] * (w.shape[1] // LANE)), U32))
            return _rowcat(rows)

        for cp in small:
            cp.start()
        x_copy(0).start()
        for cp in wq_copies(0):
            cp.start()

        def zero_body(k, carry):
            n = LANE // (S // D)
            bi = lax.broadcasted_iota(jnp.int32, (n, LANE), 0) + k * n
            mi = lax.broadcasted_iota(jnp.int32, (n, LANE), 1)
            ph = ((4 * mi + 1) * bi) & 511
            ang = ph.astype(F32) * (2.0 * 3.141592653589793 / 512.0)
            rs = pl.ds(pl.multiple_of(k * (n // 2), n // 2), n // 2)
            f_v[rs, 0:LANE] = _u32(jnp.cos(ang).astype(BF16))
            f_v[rs, LANE:] = _u32((-jnp.sin(ang)).astype(BF16))

            rb_t[k] = jnp.zeros((M, D), F32)
            cs = pl.ds(pl.multiple_of((k % 4) * D, D), D)
            ra_t[k // 4, 0:LANE, cs] = jnp.zeros((LANE, D), F32)
            ra_t[k // 4, AT * LANE:, cs] = jnp.zeros((M - AT * LANE, D), F32)
            return carry

        lax.fori_loop(0, S // D, zero_body, 0)
        c_v[S // 2:, :] = jnp.zeros((8, C), U32)

        for kt in range(1, KT):
            for cp in wq_copies(kt):
                cp.start()
        with jax.named_scope("small_wait"):
            for cp in small:
                cp.wait()
        sh = sh_v[...].astype(F32)
        for j in range(KS):
            par_v[j] = jnp.broadcast_to(sh[j:j + 1, :], (LANE, M)).T
        dd = dd_v[...].astype(F32).reshape(1, M)
        par_v[KS] = jnp.broadcast_to(dd, (LANE, M)).T

        def x_transpose(i):
            xt = xt_v[:, pl.ds(i * x_cols, x_cols)]
            xt = _rowcat([xt, jnp.zeros((MP // 2 - M // 2, x_cols), U32)])
            x_v[_h(i * x_cols, x_cols), :] = _u32(_bf(xt).astype(F32).T.astype(BF16))

        def q_early(kt, keep=False):
            first, last = kt == 0, kt == KT - 1
            n = wq_pairs(kt)
            cols = pl.ds(kt * LANE, LANE)
            if not keep:
                link[0] = None
            for j in range(H // 2):
                ws = []
                for half in range(2):
                    ev, od = (wqs_v[kt][pl.ds((2 * par + half) * n * 8 + j, n, stride=8), :]
                              for par in range(2))
                    ws.append(_repack(ev, od))
                w = _lanecat([ws[0][0], ws[1][0], ws[0][1], ws[1][1]])
                if n < TP:
                    w = _rowcat([w, jnp.zeros((TP - n, 2 * D), U32)])
                wq_v[j, pl.ds(kt * TP, TP), :] = w
                d = _dot(_bf(linked(x_v[_h(0, x_cols), cols])), _bf(w))
                set_link(d)
                if not first:
                    d = d + pltpu.bitcast(qacc[j], F32)
                if last:
                    d = (d * (D ** -0.5 * LOG2E)).astype(BF16)
                    for t in range(2):
                        q_all[2 * j + t, _h(0, x_cols), :] = _u32(d[:, t * D:(t + 1) * D])
                else:
                    qacc[j] = pltpu.bitcast(d, U32)

        with jax.named_scope("x_wait"):
            x_copy(0).wait()
        x_transpose(0)
        for i in range(1, XC):
            x_copy(i).start()
        for g in range(QIT):
            for cp in w_copies(g) + (c_copies(g) if g < QIT - 1 else []):
                cp.start()
        wo_copy.start()
        a_start(0)
        a_start(1)
        with jax.named_scope("wq_wait"):
            wq_wait(0)
        q_early(0)
        with jax.named_scope("wq_wait"):
            wq_wait(1)
            wq_wait(2)
        q_early(1)
        q_early(2, keep=True)
        with jax.named_scope("wq_wait"):
            wq_wait(3)
            for i in range(1, XC):
                x_copy(i).wait()
        q_early(3)
        for i in range(1, XC):
            x_transpose(i)

        def unpack(g, sub, j):
            ev, od = (ws_v[g, pl.ds((par * (C // 2) + sub * TP) * 8 + j, TP, stride=8), :]
                      for par in range(2))
            lo, hi = _repack(ev, od)
            rows = pl.ds(sub * TP, TP)
            cols = pl.ds(pl.multiple_of(g * LANE, LANE), LANE)
            wkv_v[2 * j, rows, cols] = lo
            wkv_v[2 * j + 1, rows, cols] = hi
            return [lo, hi]

        def a_sums(it, u):
            r0 = jnp.clip((it - 1) * CP, 0, S // 4 - CP) + 8 * u
            src = [jnp.where(it == 0, S // 2, r0 + rb * (S // 4)) for rb in range(2)]
            r0 = pl.multiple_of(r0, 8)
            kw = C // 2
            a11, a12, a21, a22 = (
                _split(c_v[pl.ds(pl.multiple_of(src[rb], 8), 8), pl.ds(cb * kw, kw)])
                for rb in range(2) for cb in range(2))
            outs = [_add(a11, a22), _add(a21, a22), _add(a11, a12), _sub(a21, a11),
                    _sub(a12, a22)]
            for k, o in enumerate(outs):
                sa_v[k, pl.ds(r0, 8), :] = o
            return outs

        units = [functools.partial(unpack, sub=s_, j=j_)
                 for s_ in range(C // 2 // TP) for j_ in range(H // 2)]
        for u_ in range(CP // 8):
            units.insert(4 * u_ + 1, functools.partial(a_sums, u=u_))

        def qproj(it, r0, n, t, zeros=(None, None)):
            outs = []
            for u in range(2):
                lhs = _bf(linked(x_v[_h(r0, n), :]))
                d = _dot(lhs, _bf(wq_v[it, :, pl.ds(t * D + u * LANE, LANE)]))
                set_link(d)
                if zeros[u] is not None:
                    for k, z in enumerate(zeros[u]):
                        d = _pin(d, z, 8 * ((k * (n // 8)) // len(zeros[u])))
                outs.append(d)
            q2 = _lanecat(outs)
            q_all[2 * it + t, _h(r0, n), :] = _u32((q2 * (D ** -0.5 * LOG2E)).astype(BF16))

        def q_body(it, carry):
            with jax.named_scope("w_wait"):
                w_wait(it)
                for p in range(QIT - 1):
                    @pl.when(it == p + 1)
                    def _():
                        for cp in c_copies(p):
                            cp.wait()
            link[0] = None
            pieces = [(p, pc, t) for p in range(QP) for pc in range(1, XC) for t in range(2)]
            nd = 2 * len(pieces)
            for k, (p, pc, t) in enumerate(pieces):
                zeros = []
                for u in range(2):
                    d = 2 * k + u
                    mine = units[d * len(units) // nd:(d + 1) * len(units) // nd]
                    zeros.append([_opaque_zero(u_(it)) for u_ in mine])
                qproj(QP * it + p, pc * x_cols, x_cols, t, zeros)
            return carry

        with jax.named_scope("q_loop"):
            lax.fori_loop(0, QIT, q_body, 0)
        wo_copy.wait()
        a_wait(0)

        tri = (lax.broadcasted_iota(jnp.int32, (LANE, LANE), 1)
               <= lax.broadcasted_iota(jnp.int32, (LANE, LANE), 0))

        NOUT = S // D

        def out_copy(i):
            if i >= NOUT:
                t = i - NOUT
                return pltpu.make_async_copy(
                    oa_v.at[t], out_hbm.at[:, pl.ds(t * LANE, LANE)], sem_out.at[i])
            rs = pl.ds(i * D, D)
            return pltpu.make_async_copy(
                out_v.at[rs], out_hbm.at[rs, pl.ds(AT * LANE, 2 * M - AT * LANE)], sem_out.at[i])

        n_body = NOUT - (tq // D if nq - 1 in cfg["o_str"] else 1)

        def b_out(k, tot):
            c0 = (k * D) % (S // 2)
            full = _rowcat([ra_t[k * D // (S // 2), AT * LANE:, c0:c0 + D], tot]).T
            out_v[k * D:(k + 1) * D, :] = full.astype(BF16)
            return full

        def head_step(h, carry):
            with jax.named_scope("step"):
                return head_step_(h, carry)

        def head_step_(h, carry):
            with_a = cfg["use_a"]

            @pl.when(h == A_STEPS)
            def _():
                for t in range(AT):
                    out_copy(NOUT + t).start()

            @pl.when(h == cfg["h0"] + 1)
            def _():
                a_wait(1)

            link[0] = None
            n2 = AR // 2
            a_rows2 = pl.ds(pl.multiple_of(jnp.minimum(h, A_STEPS - 1) * n2, n2), n2)
            a_rows = pl.ds(pl.multiple_of(jnp.minimum(h, A_STEPS - 1) * AR, AR), AR)

            kw = C // 2
            pending = []
            chains = {i: [] for i in range(nq)}
            deadline = [None]

            def flush_pending(x, row):
                done = list(pending)
                del pending[:]
                if not done:
                    return x
                x = _pin(x, _opaque_zero([f for _, f in done]), row)

                @pl.when(h == H - 1)
                def _():
                    for k, _f in done:
                        out_copy(k).start()
                return x

            def a_fwd():
                kk = _bf(a_v[0, a_rows2, :]).astype(F32)
                lane = lax.broadcasted_iota(jnp.int32, (AR, LANE), 1)
                coef = [par_v[j, a_rows, :] for j in range(KS)]
                rolled = [kk] + [pltpu.roll(kk, j, 1) for j in range(1, KS)]
                vv = _bf(a_v[1, a_rows2, :]).astype(F32)
                kv_blocks = []
                for a in range(NB):
                    cs = slice(a * LANE, (a + 1) * LANE)
                    acc = rolled[0][:, cs] * coef[0]
                    for j in range(1, KS):
                        t = rolled[j][:, cs]
                        if a == 0:
                            t = jnp.where(lane >= j, t, 0.0)
                        acc = acc + t * coef[j]
                    kv_blocks.append(acc * vv[:, cs])
                hk = a_v[2, a_rows2, :]
                hk = _rowcat([hk[:, a * LANE:(a + 1) * LANE] for a in range(NB)])
                fm = _bf(f_v[...])
                hs = _dot(_bf(linked(hk)), fm)
                kv = linked(_rowcat(kv_blocks)).astype(BF16)
                xs = _dot(kv, fm)
                set_link(xs)
                return kv, xs, hs

            def a_conv(xs, hs):
                def tile(v, a, g, part):
                    r = a * AR + 8 * g
                    return v[r:r + 8, part * LANE:(part + 1) * LANE]

                z = {}
                gate = None
                width = cfg["a_width"]
                for g in range(AR // 8):
                    hr = [tile(hs, 0, g, 0)] + [
                        tile(hs, j, g, 0) - tile(hs, j - 1, g, 1) for j in range(1, NB)]
                    hi = [tile(hs, 0, g, 1)] + [
                        tile(hs, j, g, 1) + tile(hs, j - 1, g, 0) for j in range(1, NB)]
                    for c0 in range(0, NB, width):
                        for a in range(c0 + width):
                            xr, xi = tile(xs, a, g, 0), tile(xs, a, g, 1)
                            if gate is not None:
                                xr, xi = _pin(xr, gate), _pin(xi, gate)
                            for c in range(max(c0, a), c0 + width):
                                j = c - a
                                tr = xr * hr[j] - xi * hi[j]
                                ti = xr * hi[j] + xi * hr[j]
                                z[c, g] = (tr, ti) if a == 0 else (z[c, g][0] + tr, z[c, g][1] + ti)
                            gate = _opaque_zero(list(z[c0 + width - 1, g]))
                return z

            def a_inv(kv, z, flush=False):
                fm = _bf(f_v[...])
                ng = AR // 8
                ys = []
                for u in range(2):
                    rows = [_lanecat(z[c, g]) for g in range(u * ng // 2, (u + 1) * ng // 2)
                            for c in range(NB)]
                    lhs = linked(_rowcat(rows))
                    if flush:
                        lhs = flush_pending(lhs, 8)
                    ys.append(_dot_nt(lhs.astype(BF16), fm))
                y = _rowcat(ys)
                dd = par_v[KS, a_rows, :]
                for c in range(NB):
                    cs = slice(c * LANE, (c + 1) * LANE)
                    yc = _rowcat([y[(g * NB + c) * 8:(g * NB + c + 1) * 8, :] for g in range(ng)])
                    qq = _bf(a_v[3, a_rows2, cs]).astype(F32)
                    kvf = kv[c * AR:(c + 1) * AR, :].astype(F32)
                    c2 = (c % (NB // 2)) * LANE
                    ra_t[c // (NB // 2), a_rows, c2:c2 + LANE] = qq * (yc * (1.0 / LANE) + kvf * dd)

            def a_out():
                slab = jnp.clip(h // 4 - 1, 0, AT - 1)
                half = h % 2
                x = ra_t[half, pl.ds(pl.multiple_of(slab * LANE, LANE), LANE), :]
                xt = x.T
                dst = jnp.where(h >= A_STEPS, AT, slab)
                oa_v[dst, pl.ds(pl.multiple_of(half * (S // 2), S // 2), S // 2), :] = xt.astype(BF16)
                return xt

            def w_blk(r, c):
                return wkv_v[h, _h(r * kw, kw), pl.ds(c * LANE, LANE)]

            def one_pass(lhs, w, flush):
                lhs = linked(lhs)
                if flush:
                    lhs = flush_pending(lhs, cfg["ao_row"])
                if deadline[0] is not None:
                    if deadline[0][0] == 0:
                        lhs = _pin(lhs, deadline[0][1], cfg["ao_row"] - 8)
                        deadline[0] = None
                    else:
                        deadline[0] = (deadline[0][0] - 1, deadline[0][1])
                d = _dot(_bf(lhs), _bf(paced(w)))
                set_link(d)
                return d

            def b_op(which, m):
                raw = lambda r, c: w_blk(r, 2 * which + c)
                blk = lambda r, c: _split(raw(r, c))
                return {1: lambda: _add(blk(0, 0), blk(1, 1)),
                        2: lambda: raw(0, 0),
                        3: lambda: _sub(blk(0, 1), blk(1, 1)),
                        4: lambda: _sub(blk(1, 0), blk(0, 0)),
                        5: lambda: raw(1, 1),
                        6: lambda: _add(blk(0, 0), blk(0, 1)),
                        7: lambda: _add(blk(1, 0), blk(1, 1))}[m]()

            def a_op(m, rho):
                rs = _h(rho * tq, tq)
                if m == 3:
                    return c_v[rs, 0:kw]
                if m == 4:
                    return c_v[_h(S // 2 + rho * tq, tq), kw:]
                return sa_v[{1: 0, 2: 1, 5: 2, 6: 3, 7: 4}[m], rs, :]

            b_cache, prod = {}, {}

            def kv_proj(which, blk, flush):
                rho = blk % 2
                for k, m in enumerate((5, 1, 4, 7, 3) if blk < 2 else (2, 6)):
                    if (which, m) not in b_cache:
                        b_cache[which, m] = b_op(which, m)
                    prod[which, m, rho] = one_pass(a_op(m, rho), b_cache[which, m], k == flush)
                p = lambda m: prod[which, m, rho]
                if blk < 2:
                    return [(p(1) + p(4)) + (p(7) - p(5)), p(3) + p(5)]
                return [p(2) + p(4), (p(1) + p(3)) + (p(6) - p(2))]

            def k_proj(blk, flush=-1):
                if cfg["k_str"]:
                    k = kv_proj(0, blk, flush)
                else:
                    ds = [one_pass(c_v[_h(blk * tq, tq), pl.ds((k % 2) * kw, kw)],
                                   w_blk(k % 2, k // 2), k == flush) for k in range(4)]
                    k = [ds[0] + ds[1], ds[2] + ds[3]]
                k_s[_h(blk * tq, tq), :] = _u32(_lanecat(k).astype(BF16))

            def v_proj(blk, flush=-1):
                v = kv_proj(1, blk, flush)
                v_s[_h(blk * tq, tq), :] = _u32(_lanecat(v).astype(BF16))
                if blk < nq - 1:
                    b = lambda r, c: v[c][r * D:(r + 1) * D, :]
                    sums = [b(0, 0) + b(1, 1), b(0, 1) - b(1, 1), b(1, 0) - b(0, 0),
                            b(0, 0) + b(0, 1), b(1, 0) + b(1, 1)]
                    for k, x in enumerate(sums):
                        vb_s[k, _h(blk * D, D), :] = _u32(x.astype(BF16))

            def qk(i, dep=None, flush=False):
                r0 = i * tq
                q = linked(q_all[h, _h(r0, tq), :])
                if dep is not None:
                    q = _pin(q, _opaque_zero([dep]), cfg["ao_row"])
                parts = [_dot_nt(_bf(q), _bf(k_s[_h(0, r0 + LANE), :]))]
                early = None
                if i > 0:
                    link[0] = _opaque_zero([parts[0][0:8, r0 - LANE:r0]])
                    ne = r0 // LANE - cfg["max_late"]
                    if cfg["max_late"] and ne > 1:
                        early = (ne, functools.reduce(jnp.maximum, [
                            parts[0][:, t * LANE:(t + 1) * LANE] for t in range(ne)]))
                for j in range(1, nsub):
                    q = linked(q_all[h, _h(r0 + LANE * j, tq - LANE * j), :])
                    if j == cfg["q_pin"]:
                        if flush:
                            q = flush_pending(q, 8)
                        if early is not None:
                            q = _pin(q, _opaque_zero([early[1]]), 16)
                    parts.append(_dot_nt(_bf(q), _bf(k_s[_h(r0 + LANE * j, LANE), :])))
                set_link(parts[2], cfg["link_part"], parts[0])
                return parts, early

            def exps(i, parts, early):
                sas, mbs = [], []
                for a in range(nsub):
                    blocks = [parts[j][LANE * (a - j):LANE * (a - j + 1), :] for j in range(a + 1)]
                    last = blocks[-1]
                    w = last.shape[1]
                    dg = jnp.where(tri, last[:, w - LANE:], NEG)
                    blocks[-1] = dg if w == LANE else _lanecat([last[:, :w - LANE], dg])
                    sas.append(_lanecat(blocks))
                    mx = sas[a]
                    if early is not None:
                        mx = _lanecat([early[1][LANE * a:LANE * (a + 1)], mx[:, early[0] * LANE:]])
                    mbs.append(jnp.broadcast_to(jnp.max(mx, axis=1, keepdims=True), (LANE, LANE)))
                chain = _opaque_zero([b[b.shape[0] - 8:, b.shape[1] - LANE:] for b in parts])
                pg, psums = {}, {}
                for r in range(0, tq // 2, 8):
                    for row in (r, r + tq // 2):
                        a, g = divmod(row, LANE)
                        mg = _pin(mbs[a][g:g + 8, :], chain)
                        pg[row] = [jnp.exp2(sas[a][g:g + 8, t:t + LANE] - mg)
                                   for t in range(0, sas[a].shape[1], LANE)]
                        psums[row] = functools.reduce(jnp.add, pg[row])
                        chain = _opaque_zero([psums[row]])
                        chains[i].append(chain)
                return pg, psums

            def softmax(i, pg, psums):
                r0 = i * tq
                pd, pa = pd_s.at[i % 2], pa_s[i % 2]
                first = lambda x, c=0: _pin(x, link[0], 0, c).astype(BF16)
                nt0 = r0 // LANE
                ls = []
                for a in range(nsub):
                    rows = range(LANE * a, LANE * (a + 1), 8)
                    ls.append(jnp.sum(_rowcat([psums[r] for r in rows]), axis=1, keepdims=True))
                    pd[LANE * a:LANE * (a + 1), 0:LANE * (a + 1)] = first(
                        _rowcat([_lanecat(pg[r][nt0:]) for r in rows]), LANE * a)
                if i > 0:
                    quad = lambda rh, ch: _rowcat([
                        _lanecat([pg[rh * (tq // 2) + r][4 * j + 2 * ch + t]
                                  for j in range(i) for t in range(2)])
                        for r in range(0, tq // 2, 8)])
                    a11, a12, a21, a22 = quad(0, 0), quad(0, 1), quad(1, 0), quad(1, 1)
                    ops = [a11 + a22, a21 + a22, a11, a22, a11 + a12, a21 - a11, a12 - a22]
                    for m, x in enumerate(ops):
                        if i == 3:
                            x = _pin(x, link[0], 0, 2 * D)
                        pa[m, :, 0:i * D] = first(x)
                return ls

            def pv(i, ls):
                r0 = i * tq
                pd, pa = pd_s.at[i % 2], pa_s[i % 2]
                off = None
                if i > 0:
                    def b_rows(m, j0, j1):
                        if m in (2, 5):
                            q = 0 if m == 2 else 1
                            return _bf(_rowcat([
                                v_s[_h(j * tq + q * D, D), q * LANE:(q + 1) * LANE]
                                for j in range(j0, j1)]))
                        k = {1: 0, 3: 1, 4: 2, 6: 3, 7: 4}[m]
                        return _bf(vb_s[k, _h(j0 * D, (j1 - j0) * D), :])

                    p = {}
                    for j0, j1 in {1: [(0, 1)], 2: [(0, 2)], 3: [(0, 2), (2, 3)]}[i]:
                        for m in range(1, 8):
                            cols = slice(j0 * D, j1 * D)
                            rhs = b_rows(m, j0, j1)
                            if j1 - j0 == 1 and m == 7:
                                d = _rowcat([_dot(pa[m - 1, r:r + LANE, cols], rhs)
                                             for r in (0, LANE)])
                            else:
                                d = _dot(pa[m - 1, :, cols], rhs)
                            p[m] = d if m not in p else p[m] + d
                    off = _rowcat([
                        _lanecat([(p[1] + p[4]) + (p[7] - p[5]), p[3] + p[5]]),
                        _lanecat([p[2] + p[4], (p[1] + p[3]) + (p[6] - p[2])])])
                ctx = []
                for j in range(nsub):
                    c0 = LANE * j
                    ctx.append(_dot(pd[c0:, c0:c0 + LANE], _bf(v_s[_h(r0 + c0, LANE), :])))
                set_link(ctx[2], cfg["link_part"], ctx[0])
                cs = []
                for a in range(nsub):
                    sl = lambda j: slice(LANE * (a - j), LANE * (a - j + 1))
                    r = pl.reciprocal(ls[a], approx=True)
                    r = r * (2.0 - ls[a] * r)
                    terms = [ctx[j][sl(j)] for j in range(a + 1)]
                    if off is not None:
                        terms.append(off[sl(0)])
                    cs.append(functools.reduce(jnp.add, terms) * r)
                return _rowcat(cs)

            def accumulate(k, res):
                tot = rb_t[k] + res
                rb_t[k] = tot
                if k < n_body:
                    pending.append((k, b_out(k, tot)))

            def oproj_plain(i, ctx):
                ctx = ctx.astype(BF16)
                for u in range(tq // D):
                    lhs = linked(wo_v[h])
                    if i == nq - 1:
                        lhs = flush_pending(lhs, cfg["last_row"])
                    res = _dot_nt(_bf(lhs), ctx[u * D:(u + 1) * D, :])
                    set_link(res)
                    accumulate(i * (tq // D) + u, res)

            wo_cache = {}

            def oproj(i, ctx):
                if i not in cfg["o_str"]:
                    return oproj_plain(i, ctx)
                mh = M // 4
                raw = lambda r, c: wo_v[h, r * mh:(r + 1) * mh, c * LANE:(c + 1) * LANE]
                a = lambda r, c: _split(raw(r, c))
                a_ops = {1: lambda: _add(a(0, 0), a(1, 1)), 2: lambda: _add(a(1, 0), a(1, 1)),
                         3: lambda: raw(0, 0), 4: lambda: raw(1, 1),
                         5: lambda: _add(a(0, 0), a(0, 1)), 6: lambda: _sub(a(1, 0), a(0, 0)),
                         7: lambda: _sub(a(0, 1), a(1, 1))}
                b = lambda r, c: ctx[c * D:(c + 1) * D, r * LANE:(r + 1) * LANE]
                b_ops = {1: lambda: b(0, 0) + b(1, 1), 2: lambda: b(0, 0),
                         3: lambda: b(0, 1) - b(1, 1), 4: lambda: b(1, 0) - b(0, 0),
                         5: lambda: b(1, 1), 6: lambda: b(0, 0) + b(0, 1),
                         7: lambda: b(1, 0) + b(1, 1)}
                p = {}
                for n, m in enumerate((5, 2, 4, 1, 7, 3, 6)):
                    if m not in wo_cache:
                        wo_cache[m] = a_ops[m]()
                    rhs = b_ops[m]().astype(BF16)
                    if n == cfg["o_half"]:
                        halves = [_dot_nt(_bf(linked(wo_cache[m][r:r + mh // 2])), rhs)
                                  for r in (0, mh // 2)]
                        p[m] = _rowcat(halves)
                        set_link(halves[1], 0)
                    else:
                        p[m] = _dot_nt(_bf(linked(wo_cache[m])), rhs)
                        if (n - (n > cfg["o_half"])) % 2 == 1:
                            set_link(p[m], cfg["o_link"])
                accumulate(2 * i, _rowcat([(p[1] + p[4]) + (p[7] - p[5]), p[2] + p[4]]))
                accumulate(2 * i + 1, _rowcat([p[3] + p[5], (p[1] + p[3]) + (p[6] - p[2])]))

            st = {}
            for op in cfg["seq"].split():
                op, _, dl = op.partition("@")
                if dl:
                    ch = chains[int(dl[0])]
                    deadline[0] = (int(dl[1]), ch[int(dl[2:]) * len(ch) // 16 - 1])
                op, _, fl = op.partition("!")
                fl = int(fl) if fl else -1
                kind, i = op[0], int(op[1:] or 0)
                if kind == "K":
                    k_proj(i, fl)
                elif kind == "V":
                    v_proj(i, fl)
                elif kind == "Q":
                    st["e", i] = exps(
                        i, *qk(i, a_out() if i == cfg["ao_at"] else None, fl >= 0))
                elif kind == "P":
                    st["ctx", i] = pv(i, softmax(i, *st["e", i]))
                elif kind == "O":
                    oproj(i, st["ctx", i])
                elif kind == "F" and with_a:
                    st["kv"], xs, hs = a_fwd()
                    st["z"] = a_conv(xs, hs)
                elif kind == "I" and with_a:
                    a_inv(st["kv"], st["z"], fl >= 0)
            assert not pending and deadline[0] is None
            return carry

        with jax.named_scope("loop_a"):
            lax.fori_loop(cfg["h0"], H, head_step, 0)
        with jax.named_scope("tail"):
            for i in range(n_body, NOUT):
                b_out(i, rb_t[i])
                out_copy(i).start()
            for i in range(NOUT + AT):
                out_copy(i).wait()

    scratch = [
        pltpu.VMEM((4, M // 2, S), U32),
        pltpu.VMEM((KS, M), BF16),
        pltpu.VMEM((M,), BF16),
        pltpu.VMEM((KS + 1, M, LANE), F32),
        pltpu.VMEM((LANE // 2, 2 * LANE), U32),
        pltpu.VMEM((M // 2, S), U32),
        pltpu.VMEM((S // 2, MP), U32),
        pltpu.VMEM((S // 2 + 8, C), U32),
        [pltpu.VMEM((4 * min(TP, M // 2 - kt * TP) * 8, LANE), U32)
         for kt in range(KT)],
        pltpu.VMEM((H // 2, MP // 2, 2 * D), U32),
        pltpu.VMEM((H // 2, x_cols, 2 * D), U32),
        pltpu.VMEM((QIT, C * 8, LANE), U32),
        pltpu.VMEM((H, C // 2, 2 * D), U32),
        pltpu.VMEM((H, M // 2, D), U32),
        pltpu.VMEM((H, S // 2, D), U32),
        pltpu.VMEM((S // 2, D), U32),
        pltpu.VMEM((S // 2, D), U32),
        pltpu.VMEM((5, (nq - 1) * D // 2, LANE), U32),
        pltpu.VMEM((2, tq, tq), BF16),
        [pltpu.VMEM((7, tq // 2, n * D), BF16) for n in (2, 3)],
        pltpu.VMEM((2, M, S // 2), F32),
        pltpu.VMEM((S // D, M, D), F32),
        pltpu.VMEM((AT + 1, S, LANE), BF16),
        pltpu.VMEM((S, 2 * M - AT * LANE), BF16),
        pltpu.SemaphoreType.DMA((XC,)),
        pltpu.SemaphoreType.DMA((KT,)),
        pltpu.SemaphoreType.DMA((QIT,)),
        pltpu.SemaphoreType.DMA((QIT,)),
        pltpu.SemaphoreType.DMA((2,)),
        pltpu.SemaphoreType.DMA((3,)),
        pltpu.SemaphoreType.DMA((S // D + AT,)),
    ]
    return kernel, scratch


_DEFAULT = dict(
    tq=512, a_width=4, ao_at=1, ao_row=240, link_back=176, link_part=32, pace_row=32,
    pace_step=24, use_a=1, h0=0, last_row=216, o_str=(0, 1, 2, 3), o_link=48, o_half=6, k_str=1, max_late=0, q_pin=2,
    seq="K0 Q0 K1 Q1 V0 F P0 K2@1116 O0 Q2!0 V1 P1 K3@2116 O1 Q3!0 V2 P2 V3@3116 O2 P3 I!0 O3")


def _build(**kw):
    cfg = dict(_DEFAULT)
    cfg.update(kw)
    kernel, scratch = _make_kernel(cfg)

    def run(A_q, A_k, A_v, A_shift_k, A_ssm_k, A_ssm_D, B_x, B_c_kv, B_w_q, B_w_uk,
            B_w_uv, B_w_o):
        tr = lambda a: jnp.swapaxes(a, 1, 2).reshape(M, S)
        args = (
            tr(A_q), tr(A_k), tr(A_v), A_shift_k.T, A_ssm_k, A_ssm_D, tr(B_x),
            B_c_kv.reshape(S, C),
            B_w_q.reshape(M // 2, 2 * H, D), B_w_uk.reshape(C // 2, 2 * H, D),
            B_w_uv.reshape(C // 2, 2 * H, D),
            jnp.swapaxes(B_w_o, 1, 2),
        )
        out = pl.pallas_call(
            kernel,
            in_specs=[pl.BlockSpec(memory_space=pl.ANY)] * len(args),
            out_specs=pl.BlockSpec(memory_space=pl.ANY),
            out_shape=jax.ShapeDtypeStruct((S, 2 * M), BF16),
            scratch_shapes=scratch,
            compiler_params=pltpu.CompilerParams(
                vmem_limit_bytes=126 * 1024 * 1024,
                disable_bounds_checks=True),
        )(*args)
        return out.reshape(1, S, 2 * M)

    return run


_run = _build()


@jax.jit
def pallas_concat_heads__ssm_conv_h3__compressed_kv_cla__prompt_kernel(
    A_q: jax.Array,
    A_k: jax.Array,
    A_v: jax.Array,
    A_shift_k: jax.Array,
    A_ssm_k: jax.Array,
    A_ssm_D: jax.Array,
    B_x: jax.Array,
    B_c_kv: jax.Array,
    B_w_q: jax.Array,
    B_w_uk: jax.Array,
    B_w_uv: jax.Array,
    B_w_o: jax.Array,
):
    return _run(A_q, A_k, A_v, A_shift_k, A_ssm_k, A_ssm_D, B_x, B_c_kv, B_w_q,
                B_w_uk, B_w_uv, B_w_o)
```

```python
import functools

import jax
import jax.numpy as jnp
from jax import lax
import jax.experimental.pallas as pl
import jax.experimental.pallas.tpu as pltpu

F32 = jnp.float32
BF16 = jnp.bfloat16
U32 = jnp.uint32

S = 2048
M = 448
MP = 512
C = 1024
H = 16
D = 256
KS = 4
LANE = 128
NB = S // LANE
AR = 32
A_STEPS = M // AR
LOG2E = 1.4426950408889634
NEG = -1e30

NT = (((1,), (1,)), ((), ()))


def _dot(a, b):
    return jnp.dot(a, b, preferred_element_type=F32)


def _dot_nt(a, b):
    return lax.dot_general(a, b, NT, preferred_element_type=F32)


def _bf(x):
    return pltpu.bitcast(x, BF16)


def _u32(x):
    return pltpu.bitcast(x, U32)


def _h(r0, n):
    return pl.ds(r0 // 2, n // 2)


def _repack(ev, od):
    lo = (ev & jnp.uint32(0xFFFF)) | (od << 16)
    hi = (ev >> 16) | (od & jnp.uint32(0xFFFF0000))
    return lo, hi


def _split(w):
    return (pltpu.bitcast(w << 16, F32), pltpu.bitcast(w & jnp.uint32(0xFFFF0000), F32))


def _join(lo, hi):
    half = jnp.uint32(0x8000)
    lo = (pltpu.bitcast(lo, U32) + half) >> 16
    hi = (pltpu.bitcast(hi, U32) + half) & jnp.uint32(0xFFFF0000)
    return lo | hi


def _add(a, b):
    return _join(a[0] + b[0], a[1] + b[1])


def _sub(a, b):
    return _join(a[0] - b[0], a[1] - b[1])


def _opaque_zero(vals):
    acc = None
    for v in vals:
        b = v if v.dtype == U32 else pltpu.bitcast(v, U32)
        for r in range(0, b.shape[0], 8):
            for c in range(0, b.shape[1], LANE):
                t = b[r:r + 8, c:c + LANE]
                acc = t if acc is None else acc | t
    return jnp.minimum((acc >> 1).astype(jnp.int32), 0)


def _pin(x, zero, r=0, c=0):
    t = pltpu.bitcast(pltpu.bitcast(x[r:r + 8, c:c + LANE], jnp.int32) + zero, x.dtype)
    row = ([x[r:r + 8, :c]] if c > 0 else []) + [t] + (
        [x[r:r + 8, c + LANE:]] if c + LANE < x.shape[1] else [])
    row = jnp.concatenate(row, axis=1) if len(row) > 1 else row[0]
    col = ([x[:r, :]] if r > 0 else []) + [row] + ([x[r + 8:, :]] if r + 8 < x.shape[0] else [])
    return jnp.concatenate(col, axis=0) if len(col) > 1 else col[0]


def _rowcat(xs):
    return jnp.concatenate(xs, axis=0) if len(xs) > 1 else xs[0]


def _lanecat(xs):
    return jnp.concatenate(xs, axis=1) if len(xs) > 1 else xs[0]


def _make_kernel(cfg):
    tq = cfg["tq"]
    nq = S // tq
    nsub = tq // LANE
    KT = MP // LANE
    TP = LANE // 2
    XC = 4
    x_cols = S // XC
    QP = 2
    QIT = H // 2 // QP
    CP = 176
    AT = 3

    def kernel(aq_hbm, ak_hbm, av_hbm, sh_hbm, ssm_hbm, dd_hbm, x_hbm, c_hbm,
               wq_hbm, wk_hbm, wv_hbm, wo_hbm,
               out_hbm,
               a_v, sh_v, dd_v, par_v, f_v,
               xt_v, x_v, c_v, wqs_v, wq_v, qacc, ws_v, wkv_v, wo_v,
               q_all, k_s, v_s, kb_s, vb_s, pd_s, pa_s, ra_t, rb_t, oa_v, out_v,
               sem_x, sem_wq, sem_w, sem_c, sem_s, sem_a, sem_out):
        x32, c32, wq32, wk32, wv32, wo32 = (
            r.bitcast(U32) for r in (x_hbm, c_hbm, wq_hbm, wk_hbm, wv_hbm, wo_hbm))
        a32 = [r.bitcast(U32) for r in (ak_hbm, av_hbm, ssm_hbm, aq_hbm)]

        sa_v = qacc

        def x_copy(i):
            cs = pl.ds(i * x_cols, x_cols)
            return pltpu.make_async_copy(x32.at[:, cs], xt_v.at[:, cs], sem_x.at[i])

        def wq_pairs(kt):
            return min(TP, M // 2 - kt * TP)

        def wq_copies(kt):
            n = wq_pairs(kt)
            dst = wqs_v[kt].reshape(4, n, 8, LANE)
            return [pltpu.make_async_copy(
                wq32.at[pl.ds(kt * TP, n), pl.ds(8 * (k // 2), 8), pl.ds((k % 2) * LANE, LANE)],
                dst.at[k], sem_wq.at[kt]) for k in range(4)]

        def wq_wait(kt):
            pltpu.make_async_copy(wqs_v[kt], wqs_v[kt], sem_wq.at[kt]).wait()

        def w_copies(g):
            dst = ws_v.reshape(8, C // 2, 8, LANE)
            src = (wk32, wv32)[g // 2]
            return [pltpu.make_async_copy(
                src.at[:, pl.ds(8 * par, 8), pl.ds((g % 2) * LANE, LANE)],
                dst.at[2 * g + par], sem_w.at[g]) for par in range(2)]

        def w_wait(g):
            pltpu.make_async_copy(ws_v.at[g], ws_v.at[g], sem_w.at[g]).wait()

        c_bounds = [0, CP, 2 * CP, S // 4]

        def c_copies(p):
            r0, n = c_bounds[p], c_bounds[p + 1] - c_bounds[p]
            return [pltpu.make_async_copy(c32.at[rs], c_v.at[rs], sem_c.at[p])
                    for rs in (pl.ds(r0, n), pl.ds(S // 4 + r0, n))]

        wo_copy = pltpu.make_async_copy(wo32, wo_v, sem_a.at[0])

        a_parts = [pl.ds(0, AR // 2), pl.ds(AR // 2, M // 2 - AR // 2)]

        def a_start(part):
            rs = a_parts[part]
            for k in range(4):
                pltpu.make_async_copy(
                    a32[k].at[rs], a_v.at[k, rs], sem_a.at[1 + part]).start()

        def a_wait(part):
            view = a_v.at[:, a_parts[part]]
            pltpu.make_async_copy(view, view, sem_a.at[1 + part]).wait()

        small = [pltpu.make_async_copy(sh_hbm, sh_v, sem_s.at[0]),
                 pltpu.make_async_copy(dd_hbm, dd_v, sem_s.at[1])]

        link = [None]
        pace = [None]

        def set_link(res, row=None, pacer=None):
            if row is None:
                row = res.shape[0] - cfg["link_back"]
            link[0] = _opaque_zero([res[row:row + 8, res.shape[1] - LANE:]])
            pace[0] = res if pacer is None else pacer

        def linked(x):
            return x if link[0] is None else _pin(x, link[0])

        def paced(w):
            res = pace[0]
            if res is None or link[0] is None or not cfg["pace_step"]:
                return w
            rows = []
            r0, step = cfg["pace_row"], cfg["pace_step"]
            if res.shape[0] < 400:
                r0, step = 0, 8
            if res.shape[0] < 200:
                return w
            zs = [_opaque_zero([res[r:r + 8, res.shape[1] - LANE:]])
                  for r in range(r0, r0 + 8 * step, step)]
            for r in range(0, w.shape[0], 8):
                z = zs[7 - (r // 8) % 8]
                t = pltpu.bitcast(w[r:r + 8, :], jnp.int32)
                rows.append(pltpu.bitcast(t + _lanecat([z] * (w.shape[1] // LANE)), U32))
            return _rowcat(rows)

        for cp in small:
            cp.start()
        x_copy(0).start()
        for cp in wq_copies(0):
            cp.start()

        def zero_body(k, carry):
            n = LANE // (S // D)
            bi = lax.broadcasted_iota(jnp.int32, (n, LANE), 0) + k * n
            mi = lax.broadcasted_iota(jnp.int32, (n, LANE), 1)
            ph = ((4 * mi + 1) * bi) & 511
            ang = ph.astype(F32) * (2.0 * 3.141592653589793 / 512.0)
            rs = pl.ds(pl.multiple_of(k * (n // 2), n // 2), n // 2)
            f_v[rs, 0:LANE] = _u32(jnp.cos(ang).astype(BF16))
            f_v[rs, LANE:] = _u32((-jnp.sin(ang)).astype(BF16))

            rb_t[k] = jnp.zeros((M, D), F32)
            cs = pl.ds(pl.multiple_of((k % 4) * D, D), D)
            ra_t[k // 4, 0:LANE, cs] = jnp.zeros((LANE, D), F32)
            ra_t[k // 4, AT * LANE:, cs] = jnp.zeros((M - AT * LANE, D), F32)
            return carry

        lax.fori_loop(0, S // D, zero_body, 0)
        c_v[S // 2:, :] = jnp.zeros((8, C), U32)

        for kt in range(1, KT):
            for cp in wq_copies(kt):
                cp.start()
        with jax.named_scope("small_wait"):
            for cp in small:
                cp.wait()
        sh = sh_v[...].astype(F32)
        for j in range(KS):
            par_v[j] = jnp.broadcast_to(sh[j:j + 1, :], (LANE, M)).T
        dd = dd_v[...].astype(F32).reshape(1, M)
        par_v[KS] = jnp.broadcast_to(dd, (LANE, M)).T

        def x_transpose(i):
            xt = xt_v[:, pl.ds(i * x_cols, x_cols)]
            xt = _rowcat([xt, jnp.zeros((MP // 2 - M // 2, x_cols), U32)])
            x_v[_h(i * x_cols, x_cols), :] = _u32(_bf(xt).astype(F32).T.astype(BF16))

        def q_early(kt, keep=False):
            first, last = kt == 0, kt == KT - 1
            n = wq_pairs(kt)
            cols = pl.ds(kt * LANE, LANE)
            if not keep:
                link[0] = None
            for j in range(H // 2):
                ws = []
                for half in range(2):
                    ev, od = (wqs_v[kt][pl.ds((2 * par + half) * n * 8 + j, n, stride=8), :]
                              for par in range(2))
                    ws.append(_repack(ev, od))
                w = _lanecat([ws[0][0], ws[1][0], ws[0][1], ws[1][1]])
                if n < TP:
                    w = _rowcat([w, jnp.zeros((TP - n, 2 * D), U32)])
                wq_v[j, pl.ds(kt * TP, TP), :] = w
                d = _dot(_bf(linked(x_v[_h(0, x_cols), cols])), _bf(w))
                set_link(d)
                if not first:
                    d = d + pltpu.bitcast(qacc[j], F32)
                if last:
                    d = (d * (D ** -0.5 * LOG2E)).astype(BF16)
                    for t in range(2):
                        q_all[2 * j + t, _h(0, x_cols), :] = _u32(d[:, t * D:(t + 1) * D])
                else:
                    qacc[j] = pltpu.bitcast(d, U32)

        with jax.named_scope("x_wait"):
            x_copy(0).wait()
        x_transpose(0)
        for i in range(1, XC):
            x_copy(i).start()
        for g in range(QIT):
            for cp in w_copies(g) + (c_copies(g) if g < QIT - 1 else []):
                cp.start()
        wo_copy.start()
        a_start(0)
        a_start(1)
        with jax.named_scope("wq_wait"):
            wq_wait(0)
        q_early(0)
        with jax.named_scope("wq_wait"):
            wq_wait(1)
            wq_wait(2)
        q_early(1)
        q_early(2, keep=True)
        with jax.named_scope("wq_wait"):
            wq_wait(3)
            for i in range(1, XC):
                x_copy(i).wait()
        q_early(3)
        for i in range(1, XC):
            x_transpose(i)

        def unpack(g, sub, j):
            ev, od = (ws_v[g, pl.ds((par * (C // 2) + sub * TP) * 8 + j, TP, stride=8), :]
                      for par in range(2))
            lo, hi = _repack(ev, od)
            rows = pl.ds(sub * TP, TP)
            cols = pl.ds(pl.multiple_of(g * LANE, LANE), LANE)
            wkv_v[2 * j, rows, cols] = lo
            wkv_v[2 * j + 1, rows, cols] = hi
            return [lo, hi]

        def a_sums(it, u):
            r0 = jnp.clip((it - 1) * CP, 0, S // 4 - CP) + 8 * u
            src = [jnp.where(it == 0, S // 2, r0 + rb * (S // 4)) for rb in range(2)]
            r0 = pl.multiple_of(r0, 8)
            kw = C // 2
            a11, a12, a21, a22 = (
                _split(c_v[pl.ds(pl.multiple_of(src[rb], 8), 8), pl.ds(cb * kw, kw)])
                for rb in range(2) for cb in range(2))
            outs = [_add(a11, a22), _add(a21, a22), _add(a11, a12), _sub(a21, a11),
                    _sub(a12, a22)]
            for k, o in enumerate(outs):
                sa_v[k, pl.ds(r0, 8), :] = o
            return outs

        units = [functools.partial(unpack, sub=s_, j=j_)
                 for s_ in range(C // 2 // TP) for j_ in range(H // 2)]
        for u_ in range(CP // 8):
            units.insert(4 * u_ + 1, functools.partial(a_sums, u=u_))

        def qproj(it, r0, n, t, zeros=(None, None)):
            outs = []
            for u in range(2):
                lhs = _bf(linked(x_v[_h(r0, n), :]))
                d = _dot(lhs, _bf(wq_v[it, :, pl.ds(t * D + u * LANE, LANE)]))
                set_link(d)
                if zeros[u] is not None:
                    for k, z in enumerate(zeros[u]):
                        d = _pin(d, z, 8 * ((k * (n // 8)) // len(zeros[u])))
                outs.append(d)
            q2 = _lanecat(outs)
            q_all[2 * it + t, _h(r0, n), :] = _u32((q2 * (D ** -0.5 * LOG2E)).astype(BF16))

        def q_body(it, carry):
            with jax.named_scope("w_wait"):
                w_wait(it)
                for p in range(QIT - 1):
                    @pl.when(it == p + 1)
                    def _():
                        for cp in c_copies(p):
                            cp.wait()
            link[0] = None
            pieces = [(p, pc, t) for p in range(QP) for pc in range(1, XC) for t in range(2)]
            nd = 2 * len(pieces)
            for k, (p, pc, t) in enumerate(pieces):
                zeros = []
                for u in range(2):
                    d = 2 * k + u
                    mine = units[d * len(units) // nd:(d + 1) * len(units) // nd]
                    zeros.append([_opaque_zero(u_(it)) for u_ in mine])
                qproj(QP * it + p, pc * x_cols, x_cols, t, zeros)
            return carry

        with jax.named_scope("q_loop"):
            lax.fori_loop(0, QIT, q_body, 0)
        wo_copy.wait()
        a_wait(0)

        tri = (lax.broadcasted_iota(jnp.int32, (LANE, LANE), 1)
               <= lax.broadcasted_iota(jnp.int32, (LANE, LANE), 0))

        NOUT = S // D

        def out_copy(i):
            if i >= NOUT:
                t = i - NOUT
                return pltpu.make_async_copy(
                    oa_v.at[t], out_hbm.at[:, pl.ds(t * LANE, LANE)], sem_out.at[i])
            rs = pl.ds(i * D, D)
            return pltpu.make_async_copy(
                out_v.at[rs], out_hbm.at[rs, pl.ds(AT * LANE, 2 * M - AT * LANE)], sem_out.at[i])

        n_body = NOUT - (tq // D if nq - 1 in cfg["o_str"] else 1)

        def b_out(k, tot):
            c0 = (k * D) % (S // 2)
            full = _rowcat([ra_t[k * D // (S // 2), AT * LANE:, c0:c0 + D], tot]).T
            out_v[k * D:(k + 1) * D, :] = full.astype(BF16)
            return full

        def head_step(h, carry):
            with jax.named_scope("step"):
                return head_step_(h, carry)

        def head_step_(h, carry):
            with_a = cfg["use_a"]

            @pl.when(h == A_STEPS)
            def _():
                for t in range(AT):
                    out_copy(NOUT + t).start()

            @pl.when(h == cfg["h0"] + 1)
            def _():
                a_wait(1)

            link[0] = None
            n2 = AR // 2
            a_rows2 = pl.ds(pl.multiple_of(jnp.minimum(h, A_STEPS - 1) * n2, n2), n2)
            a_rows = pl.ds(pl.multiple_of(jnp.minimum(h, A_STEPS - 1) * AR, AR), AR)

            kw = C // 2
            pending = []
            chains = {i: [] for i in range(nq)}
            deadline = [None]

            def flush_pending(x, row):
                done = list(pending)
                del pending[:]
                if not done:
                    return x
                x = _pin(x, _opaque_zero([f for _, f in done]), row)

                @pl.when(h == H - 1)
                def _():
                    for k, _f in done:
                        out_copy(k).start()
                return x

            def a_fwd():
                kk = _bf(a_v[0, a_rows2, :]).astype(F32)
                lane = lax.broadcasted_iota(jnp.int32, (AR, LANE), 1)
                coef = [par_v[j, a_rows, :] for j in range(KS)]
                rolled = [kk] + [pltpu.roll(kk, j, 1) for j in range(1, KS)]
                vv = _bf(a_v[1, a_rows2, :]).astype(F32)
                kv_blocks = []
                for a in range(NB):
                    cs = slice(a * LANE, (a + 1) * LANE)
                    acc = rolled[0][:, cs] * coef[0]
                    for j in range(1, KS):
                        t = rolled[j][:, cs]
                        if a == 0:
                            t = jnp.where(lane >= j, t, 0.0)
                        acc = acc + t * coef[j]
                    kv_blocks.append(acc * vv[:, cs])
                hk = a_v[2, a_rows2, :]
                hk = _rowcat([hk[:, a * LANE:(a + 1) * LANE] for a in range(NB)])
                fm = _bf(f_v[...])
                hs = _dot(_bf(linked(hk)), fm)
                kv = linked(_rowcat(kv_blocks)).astype(BF16)
                xs = _dot(kv, fm)
                set_link(xs)
                return kv, xs, hs

            def a_conv(xs, hs):
                def tile(v, a, g, part):
                    r = a * AR + 8 * g
                    return v[r:r + 8, part * LANE:(part + 1) * LANE]

                z = {}
                gate = None
                width = cfg["a_width"]
                for g in range(AR // 8):
                    hr = [tile(hs, 0, g, 0)] + [
                        tile(hs, j, g, 0) - tile(hs, j - 1, g, 1) for j in range(1, NB)]
                    hi = [tile(hs, 0, g, 1)] + [
                        tile(hs, j, g, 1) + tile(hs, j - 1, g, 0) for j in range(1, NB)]
                    for c0 in range(0, NB, width):
                        for a in range(c0 + width):
                            xr, xi = tile(xs, a, g, 0), tile(xs, a, g, 1)
                            if gate is not None:
                                xr, xi = _pin(xr, gate), _pin(xi, gate)
                            for c in range(max(c0, a), c0 + width):
                                j = c - a
                                tr = xr * hr[j] - xi * hi[j]
                                ti = xr * hi[j] + xi * hr[j]
                                z[c, g] = (tr, ti) if a == 0 else (z[c, g][0] + tr, z[c, g][1] + ti)
                            gate = _opaque_zero(list(z[c0 + width - 1, g]))
                return z

            def a_inv(kv, z, flush=False):
                fm = _bf(f_v[...])
                ng = AR // 8
                ys = []
                for u in range(2):
                    rows = [_lanecat(z[c, g]) for g in range(u * ng // 2, (u + 1) * ng // 2)
                            for c in range(NB)]
                    lhs = linked(_rowcat(rows))
                    if flush:
                        lhs = flush_pending(lhs, 8)
                    ys.append(_dot_nt(lhs.astype(BF16), fm))
                y = _rowcat(ys)
                dd = par_v[KS, a_rows, :]
                for c in range(NB):
                    cs = slice(c * LANE, (c + 1) * LANE)
                    yc = _rowcat([y[(g * NB + c) * 8:(g * NB + c + 1) * 8, :] for g in range(ng)])
                    qq = _bf(a_v[3, a_rows2, cs]).astype(F32)
                    kvf = kv[c * AR:(c + 1) * AR, :].astype(F32)
                    c2 = (c % (NB // 2)) * LANE
                    ra_t[c // (NB // 2), a_rows, c2:c2 + LANE] = qq * (yc * (1.0 / LANE) + kvf * dd)

            def a_out():
                slab = jnp.clip(h // 4 - 1, 0, AT - 1)
                half = h % 2
                x = ra_t[half, pl.ds(pl.multiple_of(slab * LANE, LANE), LANE), :]
                xt = x.T
                dst = jnp.where(h >= A_STEPS, AT, slab)
                oa_v[dst, pl.ds(pl.multiple_of(half * (S // 2), S // 2), S // 2), :] = xt.astype(BF16)
                return xt

            def w_blk(r, c):
                return wkv_v[h, _h(r * kw, kw), pl.ds(c * LANE, LANE)]

            def one_pass(lhs, w, flush):
                lhs = linked(lhs)
                if flush:
                    lhs = flush_pending(lhs, cfg["ao_row"])
                if deadline[0] is not None:
                    if deadline[0][0] == 0:
                        lhs = _pin(lhs, deadline[0][1], cfg["ao_row"] - 8)
                        deadline[0] = None
                    else:
                        deadline[0] = (deadline[0][0] - 1, deadline[0][1])
                d = _dot(_bf(lhs), _bf(paced(w)))
                set_link(d)
                return d

            def b_op(which, m):
                raw = lambda r, c: w_blk(r, 2 * which + c)
                blk = lambda r, c: _split(raw(r, c))
                return {1: lambda: _add(blk(0, 0), blk(1, 1)),
                        2: lambda: raw(0, 0),
                        3: lambda: _sub(blk(0, 1), blk(1, 1)),
                        4: lambda: _sub(blk(1, 0), blk(0, 0)),
                        5: lambda: raw(1, 1),
                        6: lambda: _add(blk(0, 0), blk(0, 1)),
                        7: lambda: _add(blk(1, 0), blk(1, 1))}[m]()

            def a_op(m, rho):
                rs = _h(rho * tq, tq)
                if m == 3:
                    return c_v[rs, 0:kw]
                if m == 4:
                    return c_v[_h(S // 2 + rho * tq, tq), kw:]
                return sa_v[{1: 0, 2: 1, 5: 2, 6: 3, 7: 4}[m], rs, :]

            b_cache, prod = {}, {}

            def kv_proj(which, blk, flush):
                rho = blk % 2
                for k, m in enumerate((5, 1, 4, 7, 3) if blk < 2 else (2, 6)):
                    if (which, m) not in b_cache:
                        b_cache[which, m] = b_op(which, m)
                    prod[which, m, rho] = one_pass(a_op(m, rho), b_cache[which, m], k == flush)
                p = lambda m: prod[which, m, rho]
                if blk < 2:
                    return [(p(1) + p(4)) + (p(7) - p(5)), p(3) + p(5)]
                return [p(2) + p(4), (p(1) + p(3)) + (p(6) - p(2))]

            def k_proj(blk, flush=-1):
                if cfg["k_str"]:
                    k = kv_proj(0, blk, flush)
                else:
                    ds = [one_pass(c_v[_h(blk * tq, tq), pl.ds((k % 2) * kw, kw)],
                                   w_blk(k % 2, k // 2), k == flush) for k in range(4)]
                    k = [ds[0] + ds[1], ds[2] + ds[3]]
                k_s[_h(blk * tq, tq), :] = _u32(_lanecat(k).astype(BF16))
                if cfg["s_str"] and blk < nq - 1:
                    b = lambda r, c: k[r][c * D:(c + 1) * D, :]
                    sums = [b(0, 0) + b(1, 1), b(0, 1) - b(1, 1), b(1, 0) - b(0, 0),
                            b(0, 0) + b(0, 1), b(1, 0) + b(1, 1)]
                    for n, x in enumerate(sums):
                        kb_s[n, _h(blk * D, D), :] = _u32(x.astype(BF16))

            def v_proj(blk, flush=-1):
                v = kv_proj(1, blk, flush)
                v_s[_h(blk * tq, tq), :] = _u32(_lanecat(v).astype(BF16))
                if blk < nq - 1:
                    b = lambda r, c: v[c][r * D:(r + 1) * D, :]
                    sums = [b(0, 0) + b(1, 1), b(0, 1) - b(1, 1), b(1, 0) - b(0, 0),
                            b(0, 0) + b(0, 1), b(1, 0) + b(1, 1)]
                    for k, x in enumerate(sums):
                        vb_s[k, _h(blk * D, D), :] = _u32(x.astype(BF16))

            def qk(i, dep=None, flush=False):
                r0 = i * tq
                off = None
                if cfg["s_str"] and i > 0:
                    raw = lambda r, c: q_all[h, _h(r0 + r * D, D), c * LANE:(c + 1) * LANE]
                    a = lambda r, c: _split(raw(r, c))
                    sa = {1: _add(a(0, 0), a(1, 1)), 2: _add(a(1, 0), a(1, 1)), 3: raw(0, 0),
                          4: raw(1, 1), 5: _add(a(0, 0), a(0, 1)), 6: _sub(a(1, 0), a(0, 0)),
                          7: _sub(a(0, 1), a(1, 1))}

                    def sb(m, j, t):
                        if m in (2, 5):
                            c = 0 if m == 2 else 1
                            rows = _h(j * tq + c * D + t * LANE, LANE)
                            return k_s[rows, c * LANE:(c + 1) * LANE]
                        n = {1: 0, 3: 1, 4: 2, 6: 3, 7: 4}[m]
                        return kb_s[n, _h(j * D + t * LANE, LANE), :]

                    top, bot, due = {}, {}, []
                    n_dot = 0
                    for j in range(i):
                        for t in range(2):
                            p = {}
                            for n, m in enumerate((5, 1, 4, 7, 2, 3, 6)):
                                lhs = linked(sa[m])
                                if due and n == cfg["s_due"]:
                                    lhs = _pin(lhs, due.pop(), cfg["s_row"])
                                p[m] = _dot_nt(_bf(lhs), _bf(sb(m, j, t)))
                                n_dot += 1
                                if n_dot % 4 == 0:
                                    set_link(p[m], cfg["s_link"])
                            top[4 * j + t] = (p[1] + p[4]) + (p[7] - p[5])
                            top[4 * j + 2 + t] = p[3] + p[5]
                            bot[4 * j + t] = p[2] + p[4]
                            bot[4 * j + 2 + t] = (p[1] + p[3]) + (p[6] - p[2])
                            due.append(_opaque_zero(
                                [x[4 * j + c + t] for x in (top, bot) for c in (0, 2)]))
                    off = _rowcat([_lanecat([x[c] for c in range(4 * i)]) for x in (top, bot)])
                q = linked(q_all[h, _h(r0, tq), :])
                if off is not None:
                    q = _pin(q, due.pop(), cfg["ao_row"] - 8)
                if dep is not None:
                    q = _pin(q, _opaque_zero([dep]), cfg["ao_row"])
                k0 = 0 if off is None else r0
                main = _dot_nt(_bf(q), _bf(k_s[_h(k0, r0 + LANE - k0), :]))
                parts = [main if off is None else _lanecat([off, main])]
                early = None
                if off is not None and cfg["max_late"]:
                    ne = 4 * i - cfg["max_late"] + 1
                    early = (ne, functools.reduce(jnp.maximum, [
                        off[:, t * LANE:(t + 1) * LANE] for t in range(ne)]))
                if i > 0 and off is None:
                    link[0] = _opaque_zero([parts[0][0:8, r0 - LANE:r0]])
                for j in range(1, nsub):
                    q = linked(q_all[h, _h(r0 + LANE * j, tq - LANE * j), :])
                    if j == cfg["q_pin"]:
                        if flush:
                            q = flush_pending(q, 8)
                        if early is not None:
                            q = _pin(q, _opaque_zero([early[1]]), 16)
                    parts.append(_dot_nt(_bf(q), _bf(k_s[_h(r0 + LANE * j, LANE), :])))
                set_link(parts[2], cfg["link_part"], main)
                return parts, early

            def exps(i, parts, early):
                sas, mbs = [], []
                for a in range(nsub):
                    blocks = [parts[j][LANE * (a - j):LANE * (a - j + 1), :] for j in range(a + 1)]
                    last = blocks[-1]
                    w = last.shape[1]
                    dg = jnp.where(tri, last[:, w - LANE:], NEG)
                    blocks[-1] = dg if w == LANE else _lanecat([last[:, :w - LANE], dg])
                    sas.append(_lanecat(blocks))
                    mx = sas[a]
                    if early is not None:
                        mx = _lanecat([early[1][LANE * a:LANE * (a + 1)], mx[:, early[0] * LANE:]])
                    mbs.append(jnp.broadcast_to(jnp.max(mx, axis=1, keepdims=True), (LANE, LANE)))
                chain = _opaque_zero([b[b.shape[0] - 8:, b.shape[1] - LANE:] for b in parts])
                pg, psums = {}, {}
                for r in range(0, tq // 2, 8):
                    for row in (r, r + tq // 2):
                        a, g = divmod(row, LANE)
                        mg = _pin(mbs[a][g:g + 8, :], chain)
                        pg[row] = [jnp.exp2(sas[a][g:g + 8, t:t + LANE] - mg)
                                   for t in range(0, sas[a].shape[1], LANE)]
                        psums[row] = functools.reduce(jnp.add, pg[row])
                        chain = _opaque_zero([psums[row]])
                        chains[i].append(chain)
                return pg, psums

            def softmax(i, pg, psums):
                r0 = i * tq
                pd, pa = pd_s.at[i % 2], pa_s[i % 2]
                first = lambda x, c=0: _pin(x, link[0], 0, c).astype(BF16)
                nt0 = r0 // LANE
                ls = []
                for a in range(nsub):
                    rows = range(LANE * a, LANE * (a + 1), 8)
                    ls.append(jnp.sum(_rowcat([psums[r] for r in rows]), axis=1, keepdims=True))
                    pd[LANE * a:LANE * (a + 1), 0:LANE * (a + 1)] = first(
                        _rowcat([_lanecat(pg[r][nt0:]) for r in rows]), LANE * a)
                if i > 0:
                    quad = lambda rh, ch: _rowcat([
                        _lanecat([pg[rh * (tq // 2) + r][4 * j + 2 * ch + t]
                                  for j in range(i) for t in range(2)])
                        for r in range(0, tq // 2, 8)])
                    a11, a12, a21, a22 = quad(0, 0), quad(0, 1), quad(1, 0), quad(1, 1)
                    ops = [a11 + a22, a21 + a22, a11, a22, a11 + a12, a21 - a11, a12 - a22]
                    for m, x in enumerate(ops):
                        if i == 3:
                            x = _pin(x, link[0], 0, 2 * D)
                        pa[m, :, 0:i * D] = first(x)
                return ls

            def pv(i, ls):
                r0 = i * tq
                pd, pa = pd_s.at[i % 2], pa_s[i % 2]
                off = None
                if i > 0:
                    def b_rows(m, j0, j1):
                        if m in (2, 5):
                            q = 0 if m == 2 else 1
                            return _bf(_rowcat([
                                v_s[_h(j * tq + q * D, D), q * LANE:(q + 1) * LANE]
                                for j in range(j0, j1)]))
                        k = {1: 0, 3: 1, 4: 2, 6: 3, 7: 4}[m]
                        return _bf(vb_s[k, _h(j0 * D, (j1 - j0) * D), :])

                    p = {}
                    for j0, j1 in {1: [(0, 1)], 2: [(0, 2)], 3: [(0, 2), (2, 3)]}[i]:
                        for m in range(1, 8):
                            cols = slice(j0 * D, j1 * D)
                            rhs = b_rows(m, j0, j1)
                            if j1 - j0 == 1 and m == 7:
                                d = _rowcat([_dot(pa[m - 1, r:r + LANE, cols], rhs)
                                             for r in (0, LANE)])
                            else:
                                d = _dot(pa[m - 1, :, cols], rhs)
                            p[m] = d if m not in p else p[m] + d
                    off = _rowcat([
                        _lanecat([(p[1] + p[4]) + (p[7] - p[5]), p[3] + p[5]]),
                        _lanecat([p[2] + p[4], (p[1] + p[3]) + (p[6] - p[2])])])
                ctx = []
                for j in range(nsub):
                    c0 = LANE * j
                    ctx.append(_dot(pd[c0:, c0:c0 + LANE], _bf(v_s[_h(r0 + c0, LANE), :])))
                set_link(ctx[2], cfg["link_part"], ctx[0])
                cs = []
                for a in range(nsub):
                    sl = lambda j: slice(LANE * (a - j), LANE * (a - j + 1))
                    r = pl.reciprocal(ls[a], approx=True)
                    r = r * (2.0 - ls[a] * r)
                    terms = [ctx[j][sl(j)] for j in range(a + 1)]
                    if off is not None:
                        terms.append(off[sl(0)])
                    cs.append(functools.reduce(jnp.add, terms) * r)
                return _rowcat(cs)

            def accumulate(k, res):
                tot = rb_t[k] + res
                rb_t[k] = tot
                if k < n_body:
                    pending.append((k, b_out(k, tot)))

            def oproj_plain(i, ctx):
                ctx = ctx.astype(BF16)
                for u in range(tq // D):
                    lhs = linked(wo_v[h])
                    if i == nq - 1:
                        lhs = flush_pending(lhs, cfg["last_row"])
                    res = _dot_nt(_bf(lhs), ctx[u * D:(u + 1) * D, :])
                    set_link(res)
                    accumulate(i * (tq // D) + u, res)

            wo_cache = {}

            def oproj(i, ctx):
                if i not in cfg["o_str"]:
                    return oproj_plain(i, ctx)
                mh = M // 4
                raw = lambda r, c: wo_v[h, r * mh:(r + 1) * mh, c * LANE:(c + 1) * LANE]
                a = lambda r, c: _split(raw(r, c))
                a_ops = {1: lambda: _add(a(0, 0), a(1, 1)), 2: lambda: _add(a(1, 0), a(1, 1)),
                         3: lambda: raw(0, 0), 4: lambda: raw(1, 1),
                         5: lambda: _add(a(0, 0), a(0, 1)), 6: lambda: _sub(a(1, 0), a(0, 0)),
                         7: lambda: _sub(a(0, 1), a(1, 1))}
                b = lambda r, c: ctx[c * D:(c + 1) * D, r * LANE:(r + 1) * LANE]
                b_ops = {1: lambda: b(0, 0) + b(1, 1), 2: lambda: b(0, 0),
                         3: lambda: b(0, 1) - b(1, 1), 4: lambda: b(1, 0) - b(0, 0),
                         5: lambda: b(1, 1), 6: lambda: b(0, 0) + b(0, 1),
                         7: lambda: b(1, 0) + b(1, 1)}
                p = {}
                for n, m in enumerate((5, 2, 4, 1, 7, 3, 6)):
                    if m not in wo_cache:
                        wo_cache[m] = a_ops[m]()
                    rhs = b_ops[m]().astype(BF16)
                    if n == cfg["o_half"]:
                        halves = [_dot_nt(_bf(linked(wo_cache[m][r:r + mh // 2])), rhs)
                                  for r in (0, mh // 2)]
                        p[m] = _rowcat(halves)
                        set_link(halves[1], 0)
                    else:
                        p[m] = _dot_nt(_bf(linked(wo_cache[m])), rhs)
                        if (n - (n > cfg["o_half"])) % 2 == 1:
                            set_link(p[m], cfg["o_link"])
                accumulate(2 * i, _rowcat([(p[1] + p[4]) + (p[7] - p[5]), p[2] + p[4]]))
                accumulate(2 * i + 1, _rowcat([p[3] + p[5], (p[1] + p[3]) + (p[6] - p[2])]))

            st = {}
            for op in cfg["seq"].split():
                op, _, dl = op.partition("@")
                if dl:
                    ch = chains[int(dl[0])]
                    deadline[0] = (int(dl[1]), ch[int(dl[2:]) * len(ch) // 16 - 1])
                op, _, fl = op.partition("!")
                fl = int(fl) if fl else -1
                kind, i = op[0], int(op[1:] or 0)
                if kind == "K":
                    k_proj(i, fl)
                elif kind == "V":
                    v_proj(i, fl)
                elif kind == "Q":
                    st["e", i] = exps(
                        i, *qk(i, a_out() if i == cfg["ao_at"] else None, fl >= 0))
                elif kind == "P":
                    st["ctx", i] = pv(i, softmax(i, *st["e", i]))
                elif kind == "O":
                    oproj(i, st["ctx", i])
                elif kind == "F" and with_a:
                    st["kv"], xs, hs = a_fwd()
                    st["z"] = a_conv(xs, hs)
                elif kind == "I" and with_a:
                    a_inv(st["kv"], st["z"], fl >= 0)
            assert not pending and deadline[0] is None
            return carry

        with jax.named_scope("loop_a"):
            lax.fori_loop(cfg["h0"], H, head_step, 0)
        with jax.named_scope("tail"):
            for i in range(n_body, NOUT):
                b_out(i, rb_t[i])
                out_copy(i).start()
            for i in range(NOUT + AT):
                out_copy(i).wait()

    scratch = [
        pltpu.VMEM((4, M // 2, S), U32),
        pltpu.VMEM((KS, M), BF16),
        pltpu.VMEM((M,), BF16),
        pltpu.VMEM((KS + 1, M, LANE), F32),
        pltpu.VMEM((LANE // 2, 2 * LANE), U32),
        pltpu.VMEM((M // 2, S), U32),
        pltpu.VMEM((S // 2, MP), U32),
        pltpu.VMEM((S // 2 + 8, C), U32),
        [pltpu.VMEM((4 * min(TP, M // 2 - kt * TP) * 8, LANE), U32)
         for kt in range(KT)],
        pltpu.VMEM((H // 2, MP // 2, 2 * D), U32),
        pltpu.VMEM((H // 2, x_cols, 2 * D), U32),
        pltpu.VMEM((QIT, C * 8, LANE), U32),
        pltpu.VMEM((H, C // 2, 2 * D), U32),
        pltpu.VMEM((H, M // 2, D), U32),
        pltpu.VMEM((H, S // 2, D), U32),
        pltpu.VMEM((S // 2, D), U32),
        pltpu.VMEM((S // 2, D), U32),
        pltpu.VMEM((5, (nq - 1) * D // 2, LANE), U32),
        pltpu.VMEM((5, (nq - 1) * D // 2, LANE), U32),
        pltpu.VMEM((2, tq, tq), BF16),
        [pltpu.VMEM((7, tq // 2, n * D), BF16) for n in (2, 3)],
        pltpu.VMEM((2, M, S // 2), F32),
        pltpu.VMEM((S // D, M, D), F32),
        pltpu.VMEM((AT + 1, S, LANE), BF16),
        pltpu.VMEM((S, 2 * M - AT * LANE), BF16),
        pltpu.SemaphoreType.DMA((XC,)),
        pltpu.SemaphoreType.DMA((KT,)),
        pltpu.SemaphoreType.DMA((QIT,)),
        pltpu.SemaphoreType.DMA((QIT,)),
        pltpu.SemaphoreType.DMA((2,)),
        pltpu.SemaphoreType.DMA((3,)),
        pltpu.SemaphoreType.DMA((S // D + AT,)),
    ]
    return kernel, scratch


_DEFAULT = dict(
    tq=512, a_width=4, ao_at=1, ao_row=240, link_back=176, link_part=32, pace_row=32,
    pace_step=24, use_a=1, h0=0, last_row=216, o_str=(0, 1, 2, 3), o_link=48, o_half=6, s_str=1, s_link=64, s_due=4, s_row=120, k_str=1, max_late=0, q_pin=2,
    seq="K0 Q0 K1 Q1 V0 F P0 K2@1116 Q2 O0 V1!4 P1 K3@2116 O1 Q3!0 V2 P2 V3@3116 O2 P3 I!0 O3")


def _build(**kw):
    cfg = dict(_DEFAULT)
    cfg.update(kw)
    kernel, scratch = _make_kernel(cfg)

    def run(A_q, A_k, A_v, A_shift_k, A_ssm_k, A_ssm_D, B_x, B_c_kv, B_w_q, B_w_uk,
            B_w_uv, B_w_o):
        tr = lambda a: jnp.swapaxes(a, 1, 2).reshape(M, S)
        args = (
            tr(A_q), tr(A_k), tr(A_v), A_shift_k.T, A_ssm_k, A_ssm_D, tr(B_x),
            B_c_kv.reshape(S, C),
            B_w_q.reshape(M // 2, 2 * H, D), B_w_uk.reshape(C // 2, 2 * H, D),
            B_w_uv.reshape(C // 2, 2 * H, D),
            jnp.swapaxes(B_w_o, 1, 2),
        )
        out = pl.pallas_call(
            kernel,
            in_specs=[pl.BlockSpec(memory_space=pl.ANY)] * len(args),
            out_specs=pl.BlockSpec(memory_space=pl.ANY),
            out_shape=jax.ShapeDtypeStruct((S, 2 * M), BF16),
            scratch_shapes=scratch,
            compiler_params=pltpu.CompilerParams(
                vmem_limit_bytes=126 * 1024 * 1024,
                disable_bounds_checks=True),
        )(*args)
        return out.reshape(1, S, 2 * M)

    return run


_run = _build()


@jax.jit
def pallas_concat_heads__ssm_conv_h3__compressed_kv_cla__prompt_kernel(
    A_q: jax.Array,
    A_k: jax.Array,
    A_v: jax.Array,
    A_shift_k: jax.Array,
    A_ssm_k: jax.Array,
    A_ssm_D: jax.Array,
    B_x: jax.Array,
    B_c_kv: jax.Array,
    B_w_q: jax.Array,
    B_w_uk: jax.Array,
    B_w_uv: jax.Array,
    B_w_o: jax.Array,
):
    return _run(A_q, A_k, A_v, A_shift_k, A_ssm_k, A_ssm_D, B_x, B_c_kv, B_w_q,
                B_w_uk, B_w_uv, B_w_o)
```

```python
import functools

import jax
import jax.numpy as jnp
from jax import lax
import jax.experimental.pallas as pl
import jax.experimental.pallas.tpu as pltpu

F32 = jnp.float32
BF16 = jnp.bfloat16
U32 = jnp.uint32

S = 2048
M = 448
MP = 512
C = 1024
H = 16
D = 256
KS = 4
LANE = 128
NB = S // LANE
AR = 32
A_STEPS = M // AR
LOG2E = 1.4426950408889634
NEG = -1e30

NT = (((1,), (1,)), ((), ()))


def _dot(a, b):
    return jnp.dot(a, b, preferred_element_type=F32)


def _dot_nt(a, b):
    return lax.dot_general(a, b, NT, preferred_element_type=F32)


def _bf(x):
    return pltpu.bitcast(x, BF16)


def _u32(x):
    return pltpu.bitcast(x, U32)


def _h(r0, n):
    return pl.ds(r0 // 2, n // 2)


def _repack(ev, od):
    lo = (ev & jnp.uint32(0xFFFF)) | (od << 16)
    hi = (ev >> 16) | (od & jnp.uint32(0xFFFF0000))
    return lo, hi


def _split(w):
    return (pltpu.bitcast(w << 16, F32), pltpu.bitcast(w & jnp.uint32(0xFFFF0000), F32))


def _join(lo, hi):
    half = jnp.uint32(0x8000)
    lo = (pltpu.bitcast(lo, U32) + half) >> 16
    hi = (pltpu.bitcast(hi, U32) + half) & jnp.uint32(0xFFFF0000)
    return lo | hi


def _add(a, b):
    return _join(a[0] + b[0], a[1] + b[1])


def _sub(a, b):
    return _join(a[0] - b[0], a[1] - b[1])


def _opaque_zero(vals):
    acc = None
    for v in vals:
        b = v if v.dtype == U32 else pltpu.bitcast(v, U32)
        for r in range(0, b.shape[0], 8):
            for c in range(0, b.shape[1], LANE):
                t = b[r:r + 8, c:c + LANE]
                acc = t if acc is None else acc | t
    return jnp.minimum((acc >> 1).astype(jnp.int32), 0)


def _pin(x, zero, r=0, c=0):
    t = pltpu.bitcast(pltpu.bitcast(x[r:r + 8, c:c + LANE], jnp.int32) + zero, x.dtype)
    row = ([x[r:r + 8, :c]] if c > 0 else []) + [t] + (
        [x[r:r + 8, c + LANE:]] if c + LANE < x.shape[1] else [])
    row = jnp.concatenate(row, axis=1) if len(row) > 1 else row[0]
    col = ([x[:r, :]] if r > 0 else []) + [row] + ([x[r + 8:, :]] if r + 8 < x.shape[0] else [])
    return jnp.concatenate(col, axis=0) if len(col) > 1 else col[0]


def _rowcat(xs):
    return jnp.concatenate(xs, axis=0) if len(xs) > 1 else xs[0]


def _lanecat(xs):
    return jnp.concatenate(xs, axis=1) if len(xs) > 1 else xs[0]


def _make_kernel(cfg):
    tq = cfg["tq"]
    nq = S // tq
    nsub = tq // LANE
    KT = MP // LANE
    TP = LANE // 2
    XC = 4
    x_cols = S // XC
    QP = 2
    QIT = H // 2 // QP
    XH = (S - x_cols) // 2
    CP = 176
    AT = 3

    def kernel(aq_hbm, ak_hbm, av_hbm, sh_hbm, ssm_hbm, dd_hbm, x_hbm, c_hbm,
               wq_hbm, wk_hbm, wv_hbm, wo_hbm,
               out_hbm,
               a_v, sh_v, dd_v, par_v, f_v,
               xt_v, x_v, xs_v, c_v, wqs_v, wq_v, qacc, ws_v, wkv_v, wo_v,
               q_all, k_s, v_s, kb_s, vb_s, pd_s, pa_s, ra_t, rb_t, oa_v, out_v,
               sem_x, sem_wq, sem_w, sem_c, sem_s, sem_a, sem_out):
        x32, c32, wq32, wk32, wv32, wo32 = (
            r.bitcast(U32) for r in (x_hbm, c_hbm, wq_hbm, wk_hbm, wv_hbm, wo_hbm))
        a32 = [r.bitcast(U32) for r in (ak_hbm, av_hbm, ssm_hbm, aq_hbm)]

        sa_v = qacc

        def x_copy(i):
            cs = pl.ds(i * x_cols, x_cols)
            return pltpu.make_async_copy(x32.at[:, cs], xt_v.at[:, cs], sem_x.at[i])

        def wq_pairs(kt):
            return min(TP, M // 2 - kt * TP)

        def wq_copies(kt):
            n = wq_pairs(kt)
            dst = wqs_v[kt].reshape(4, n, 8, LANE)
            return [pltpu.make_async_copy(
                wq32.at[pl.ds(kt * TP, n), pl.ds(8 * (k // 2), 8), pl.ds((k % 2) * LANE, LANE)],
                dst.at[k], sem_wq.at[kt]) for k in range(4)]

        def wq_wait(kt):
            pltpu.make_async_copy(wqs_v[kt], wqs_v[kt], sem_wq.at[kt]).wait()

        def w_copies(g):
            dst = ws_v.reshape(8, C // 2, 8, LANE)
            src = (wk32, wv32)[g // 2]
            return [pltpu.make_async_copy(
                src.at[:, pl.ds(8 * par, 8), pl.ds((g % 2) * LANE, LANE)],
                dst.at[2 * g + par], sem_w.at[g]) for par in range(2)]

        def w_wait(g):
            pltpu.make_async_copy(ws_v.at[g], ws_v.at[g], sem_w.at[g]).wait()

        c_bounds = [0, CP, 2 * CP, S // 4]

        def c_copies(p):
            r0, n = c_bounds[p], c_bounds[p + 1] - c_bounds[p]
            return [pltpu.make_async_copy(c32.at[rs], c_v.at[rs], sem_c.at[p])
                    for rs in (pl.ds(r0, n), pl.ds(S // 4 + r0, n))]

        wo_copy = pltpu.make_async_copy(wo32, wo_v, sem_a.at[0])

        a_parts = [pl.ds(0, AR // 2), pl.ds(AR // 2, M // 2 - AR // 2)]

        def a_start(part):
            rs = a_parts[part]
            for k in range(4):
                pltpu.make_async_copy(
                    a32[k].at[rs], a_v.at[k, rs], sem_a.at[1 + part]).start()

        def a_wait(part):
            view = a_v.at[:, a_parts[part]]
            pltpu.make_async_copy(view, view, sem_a.at[1 + part]).wait()

        small = [pltpu.make_async_copy(sh_hbm, sh_v, sem_s.at[0]),
                 pltpu.make_async_copy(dd_hbm, dd_v, sem_s.at[1])]

        link = [None]
        pace = [None]

        def set_link(res, row=None, pacer=None):
            if row is None:
                row = res.shape[0] - cfg["link_back"]
            link[0] = _opaque_zero([res[row:row + 8, res.shape[1] - LANE:]])
            pace[0] = res if pacer is None else pacer

        def linked(x):
            return x if link[0] is None else _pin(x, link[0])

        def paced(w):
            res = pace[0]
            if res is None or link[0] is None or not cfg["pace_step"]:
                return w
            rows = []
            r0, step = cfg["pace_row"], cfg["pace_step"]
            if res.shape[0] < 400:
                r0, step = 0, 8
            if res.shape[0] < 200:
                return w
            zs = [_opaque_zero([res[r:r + 8, res.shape[1] - LANE:]])
                  for r in range(r0, r0 + 8 * step, step)]
            for r in range(0, w.shape[0], 8):
                z = zs[7 - (r // 8) % 8]
                t = pltpu.bitcast(w[r:r + 8, :], jnp.int32)
                rows.append(pltpu.bitcast(t + _lanecat([z] * (w.shape[1] // LANE)), U32))
            return _rowcat(rows)

        for cp in small:
            cp.start()
        x_copy(0).start()
        for cp in wq_copies(0):
            cp.start()

        def zero_body(k, carry):
            n = LANE // (S // D)
            bi = lax.broadcasted_iota(jnp.int32, (n, LANE), 0) + k * n
            mi = lax.broadcasted_iota(jnp.int32, (n, LANE), 1)
            ph = ((4 * mi + 1) * bi) & 511
            ang = ph.astype(F32) * (2.0 * 3.141592653589793 / 512.0)
            rs = pl.ds(pl.multiple_of(k * (n // 2), n // 2), n // 2)
            f_v[rs, 0:LANE] = _u32(jnp.cos(ang).astype(BF16))
            f_v[rs, LANE:] = _u32((-jnp.sin(ang)).astype(BF16))

            rb_t[k] = jnp.zeros((M, D), F32)
            cs = pl.ds(pl.multiple_of((k % 4) * D, D), D)
            ra_t[k // 4, 0:LANE, cs] = jnp.zeros((LANE, D), F32)
            ra_t[k // 4, AT * LANE:, cs] = jnp.zeros((M - AT * LANE, D), F32)
            return carry

        lax.fori_loop(0, S // D, zero_body, 0)
        c_v[S // 2:, :] = jnp.zeros((8, C), U32)

        for kt in range(1, KT):
            for cp in wq_copies(kt):
                cp.start()
        with jax.named_scope("small_wait"):
            for cp in small:
                cp.wait()
        sh = sh_v[...].astype(F32)
        for j in range(KS):
            par_v[j] = jnp.broadcast_to(sh[j:j + 1, :], (LANE, M)).T
        dd = dd_v[...].astype(F32).reshape(1, M)
        par_v[KS] = jnp.broadcast_to(dd, (LANE, M)).T

        def x_transpose(i):
            xt = xt_v[:, pl.ds(i * x_cols, x_cols)]
            xt = _rowcat([xt, jnp.zeros((MP // 2 - M // 2, x_cols), U32)])
            x_v[_h(i * x_cols, x_cols), :] = _u32(_bf(xt).astype(F32).T.astype(BF16))

        def q_early(kt, keep=False, jobs=()):
            first, last = kt == 0, kt == KT - 1
            n = wq_pairs(kt)
            cols = pl.ds(kt * LANE, LANE)
            if not keep:
                link[0] = None
            for j in range(H // 2):
                ws = []
                for half in range(2):
                    ev, od = (wqs_v[kt][pl.ds((2 * par + half) * n * 8 + j, n, stride=8), :]
                              for par in range(2))
                    ws.append(_repack(ev, od))
                w = _lanecat([ws[0][0], ws[1][0], ws[0][1], ws[1][1]])
                if n < TP:
                    w = _rowcat([w, jnp.zeros((TP - n, 2 * D), U32)])
                wq_v[j, pl.ds(kt * TP, TP), :] = w
                lhs = linked(x_v[_h(0, x_cols), cols])
                j0 = cfg["xs_from"]
                if jobs and j >= j0:
                    nj = H // 2 - j0
                    mine = jobs[(j - j0) * len(jobs) // nj:(j - j0 + 1) * len(jobs) // nj]
                    for k, job in enumerate(mine):
                        lhs = _pin(lhs, _opaque_zero(job()), 8 * (1 + k * 30 // len(mine)))
                d = _dot(_bf(lhs), _bf(w))
                set_link(d)
                if not first:
                    d = d + pltpu.bitcast(qacc[j], F32)
                if last:
                    d = (d * (D ** -0.5 * LOG2E)).astype(BF16)
                    for t in range(2):
                        q_all[2 * j + t, _h(0, x_cols), :] = _u32(d[:, t * D:(t + 1) * D])
                else:
                    qacc[j] = pltpu.bitcast(d, U32)

        with jax.named_scope("x_wait"):
            x_copy(0).wait()
        x_transpose(0)
        for i in range(1, XC):
            x_copy(i).start()
        for g in range(QIT):
            for cp in w_copies(g) + (c_copies(g) if g < QIT - 1 else []):
                cp.start()
        wo_copy.start()
        a_start(0)
        a_start(1)
        with jax.named_scope("wq_wait"):
            wq_wait(0)
        q_early(0)
        with jax.named_scope("wq_wait"):
            wq_wait(1)
            wq_wait(2)
        q_early(1)
        q_early(2, keep=True)
        with jax.named_scope("wq_wait"):
            wq_wait(3)
            for i in range(1, XC):
                x_copy(i).wait()
        for i in range(1, XC):
            x_transpose(i)

        def x_sums(u):
            a11, a12, a21, a22 = (
                _split(x_v[pl.ds((x_cols + rb * XH) // 2 + 8 * u, 8), cb * D:(cb + 1) * D])
                for rb in range(2) for cb in range(2))
            outs = [_add(a11, a22), _add(a21, a22), _add(a11, a12), _sub(a21, a11),
                    _sub(a12, a22)]
            for k, o in enumerate(outs):
                xs_v[k, 8 * u:8 * u + 8, :] = o
            return outs

        q_early(3, jobs=[functools.partial(x_sums, u) for u in range(XH // 16)])

        def unpack(it, sub, j):
            g = it
            ev, od = (ws_v[g, pl.ds((par * (C // 2) + sub * TP) * 8 + j, TP, stride=8), :]
                      for par in range(2))
            lo, hi = _repack(ev, od)
            rows = pl.ds(sub * TP, TP)
            cols = pl.ds(pl.multiple_of(g * LANE, LANE), LANE)
            wkv_v[2 * j, rows, cols] = lo
            wkv_v[2 * j + 1, rows, cols] = hi
            return [lo, hi]

        def a_sums(it, u):
            r0 = jnp.clip((it - 1) * CP, 0, S // 4 - CP) + 8 * u
            src = [jnp.where(it == 0, S // 2, r0 + rb * (S // 4)) for rb in range(2)]
            r0 = pl.multiple_of(r0, 8)
            kw = C // 2
            a11, a12, a21, a22 = (
                _split(c_v[pl.ds(pl.multiple_of(src[rb], 8), 8), pl.ds(cb * kw, kw)])
                for rb in range(2) for cb in range(2))
            outs = [_add(a11, a22), _add(a21, a22), _add(a11, a12), _sub(a21, a11),
                    _sub(a12, a22)]
            for k, o in enumerate(outs):
                sa_v[k, pl.ds(r0, 8), :] = o
            return outs

        units = [functools.partial(unpack, sub=s_, j=j_)
                 for s_ in range(C // 2 // TP) for j_ in range(H // 2)]
        for u_ in range(CP // 8):
            units.insert(4 * u_ + 1, functools.partial(a_sums, u=u_))

        def q_pair(pair, todo):
            raw = lambda r, c: _lanecat([
                wq_v[pair, r * LANE:(r + 1) * LANE, pl.ds(t * D + c * LANE, LANE)]
                for t in range(2)])
            b = lambda r, c: _split(raw(r, c))
            sb = {1: _add(b(0, 0), b(1, 1)), 2: raw(0, 0), 3: _sub(b(0, 1), b(1, 1)),
                  4: _sub(b(1, 0), b(0, 0)), 5: raw(1, 1), 6: _add(b(0, 0), b(0, 1)),
                  7: _add(b(1, 0), b(1, 1))}
            n = XH // 2
            for rho in range(2):
                def sa(m):
                    if m == 3:
                        return x_v[_h(x_cols + rho * n, n), 0:D]
                    if m == 4:
                        return x_v[_h(x_cols + XH + rho * n, n), D:]
                    return xs_v[{1: 0, 2: 1, 5: 2, 6: 3, 7: 4}[m], _h(rho * n, n), :]

                def put(half, c0, c1):
                    rows = _h(x_cols + half * XH + rho * n, n)
                    out = []
                    for t in range(2):
                        q = _lanecat([c[:, t * LANE:(t + 1) * LANE] for c in (c0, c1)])
                        out.append(_u32((q * (D ** -0.5 * LOG2E)).astype(BF16)))
                        q_all[2 * pair + t, rows, :] = out[-1]
                    q_due.append(_opaque_zero(out))

                p = {}
                for m in (5, 1, 4, 7, 3, 2, 6):
                    lhs = linked(sa(m))
                    nj = min(len(todo), cfg["q_jobs"][rho])
                    jobs = [todo.pop()(it=pair // QP) for _ in range(nj)]
                    for k, job in enumerate(jobs):
                        lhs = _pin(lhs, _opaque_zero(job), 8 * (1 + k * (n // 16 - 1) // nj))
                    if q_due and m in (1, 6):
                        lhs = _pin(lhs, q_due.pop(), n // 2 - 8, LANE)
                    p[m] = _dot(_bf(lhs), _bf(sb[m]))
                    set_link(p[m])
                    if m == 3:
                        put(0, (p[1] + p[4]) + (p[7] - p[5]), p[3] + p[5])
                put(1, p[2] + p[4], (p[1] + p[3]) + (p[6] - p[2]))

        q_due = []

        def q_body(it, carry):
            with jax.named_scope("w_wait"):
                w_wait(it)
                for p in range(QIT - 1):
                    @pl.when(it == p + 1)
                    def _():
                        for cp in c_copies(p):
                            cp.wait()
            link[0] = None
            todo = units[::-1]
            del q_due[:]
            for p in range(QP):
                q_pair(QP * it + p, todo)
            assert not todo
            return carry

        with jax.named_scope("q_loop"):
            lax.fori_loop(0, QIT, q_body, 0)
        wo_copy.wait()
        a_wait(0)

        tri = (lax.broadcasted_iota(jnp.int32, (LANE, LANE), 1)
               <= lax.broadcasted_iota(jnp.int32, (LANE, LANE), 0))

        NOUT = S // D

        def out_copy(i):
            if i >= NOUT:
                t = i - NOUT
                return pltpu.make_async_copy(
                    oa_v.at[t], out_hbm.at[:, pl.ds(t * LANE, LANE)], sem_out.at[i])
            rs = pl.ds(i * D, D)
            return pltpu.make_async_copy(
                out_v.at[rs], out_hbm.at[rs, pl.ds(AT * LANE, 2 * M - AT * LANE)], sem_out.at[i])

        n_body = NOUT - (tq // D if nq - 1 in cfg["o_str"] else 1)

        def b_out(k, tot):
            c0 = (k * D) % (S // 2)
            full = _rowcat([ra_t[k * D // (S // 2), AT * LANE:, c0:c0 + D], tot]).T
            out_v[k * D:(k + 1) * D, :] = full.astype(BF16)
            return full

        def head_step(h, carry):
            with jax.named_scope("step"):
                return head_step_(h, carry)

        def head_step_(h, carry):
            with_a = cfg["use_a"]

            @pl.when(h == A_STEPS)
            def _():
                for t in range(AT):
                    out_copy(NOUT + t).start()

            @pl.when(h == cfg["h0"] + 1)
            def _():
                a_wait(1)

            link[0] = None
            n2 = AR // 2
            a_rows2 = pl.ds(pl.multiple_of(jnp.minimum(h, A_STEPS - 1) * n2, n2), n2)
            a_rows = pl.ds(pl.multiple_of(jnp.minimum(h, A_STEPS - 1) * AR, AR), AR)

            kw = C // 2
            pending = []
            chains = {i: [] for i in range(nq)}
            deadline = [None]

            def flush_pending(x, row):
                done = list(pending)
                del pending[:]
                if not done:
                    return x
                x = _pin(x, _opaque_zero([f for _, f in done]), row)

                @pl.when(h == H - 1)
                def _():
                    for k, _f in done:
                        out_copy(k).start()
                return x

            def a_fwd():
                kk = _bf(a_v[0, a_rows2, :]).astype(F32)
                lane = lax.broadcasted_iota(jnp.int32, (AR, LANE), 1)
                coef = [par_v[j, a_rows, :] for j in range(KS)]
                rolled = [kk] + [pltpu.roll(kk, j, 1) for j in range(1, KS)]
                vv = _bf(a_v[1, a_rows2, :]).astype(F32)
                kv_blocks = []
                for a in range(NB):
                    cs = slice(a * LANE, (a + 1) * LANE)
                    acc = rolled[0][:, cs] * coef[0]
                    for j in range(1, KS):
                        t = rolled[j][:, cs]
                        if a == 0:
                            t = jnp.where(lane >= j, t, 0.0)
                        acc = acc + t * coef[j]
                    kv_blocks.append(acc * vv[:, cs])
                hk = a_v[2, a_rows2, :]
                hk = _rowcat([hk[:, a * LANE:(a + 1) * LANE] for a in range(NB)])
                fm = _bf(f_v[...])
                hs = _dot(_bf(linked(hk)), fm)
                kv = linked(_rowcat(kv_blocks)).astype(BF16)
                xs = _dot(kv, fm)
                set_link(xs)
                return kv, xs, hs

            def a_conv(xs, hs):
                def tile(v, a, g, part):
                    r = a * AR + 8 * g
                    return v[r:r + 8, part * LANE:(part + 1) * LANE]

                z = {}
                gate = None
                width = cfg["a_width"]
                for g in range(AR // 8):
                    hr = [tile(hs, 0, g, 0)] + [
                        tile(hs, j, g, 0) - tile(hs, j - 1, g, 1) for j in range(1, NB)]
                    hi = [tile(hs, 0, g, 1)] + [
                        tile(hs, j, g, 1) + tile(hs, j - 1, g, 0) for j in range(1, NB)]
                    for c0 in range(0, NB, width):
                        for a in range(c0 + width):
                            xr, xi = tile(xs, a, g, 0), tile(xs, a, g, 1)
                            if gate is not None:
                                xr, xi = _pin(xr, gate), _pin(xi, gate)
                            for c in range(max(c0, a), c0 + width):
                                j = c - a
                                tr = xr * hr[j] - xi * hi[j]
                                ti = xr * hi[j] + xi * hr[j]
                                z[c, g] = (tr, ti) if a == 0 else (z[c, g][0] + tr, z[c, g][1] + ti)
                            gate = _opaque_zero(list(z[c0 + width - 1, g]))
                return z

            def a_inv(kv, z, flush=False):
                fm = _bf(f_v[...])
                ng = AR // 8
                ys = []
                for u in range(2):
                    rows = [_lanecat(z[c, g]) for g in range(u * ng // 2, (u + 1) * ng // 2)
                            for c in range(NB)]
                    lhs = linked(_rowcat(rows))
                    if flush:
                        lhs = flush_pending(lhs, 8)
                    ys.append(_dot_nt(lhs.astype(BF16), fm))
                y = _rowcat(ys)
                dd = par_v[KS, a_rows, :]
                for c in range(NB):
                    cs = slice(c * LANE, (c + 1) * LANE)
                    yc = _rowcat([y[(g * NB + c) * 8:(g * NB + c + 1) * 8, :] for g in range(ng)])
                    qq = _bf(a_v[3, a_rows2, cs]).astype(F32)
                    kvf = kv[c * AR:(c + 1) * AR, :].astype(F32)
                    c2 = (c % (NB // 2)) * LANE
                    ra_t[c // (NB // 2), a_rows, c2:c2 + LANE] = qq * (yc * (1.0 / LANE) + kvf * dd)

            def a_out():
                slab = jnp.clip(h // 4 - 1, 0, AT - 1)
                half = h % 2
                x = ra_t[half, pl.ds(pl.multiple_of(slab * LANE, LANE), LANE), :]
                xt = x.T
                dst = jnp.where(h >= A_STEPS, AT, slab)
                oa_v[dst, pl.ds(pl.multiple_of(half * (S // 2), S // 2), S // 2), :] = xt.astype(BF16)
                return xt

            def w_blk(r, c):
                return wkv_v[h, _h(r * kw, kw), pl.ds(c * LANE, LANE)]

            def one_pass(lhs, w, flush):
                lhs = linked(lhs)
                if flush:
                    lhs = flush_pending(lhs, cfg["ao_row"])
                if deadline[0] is not None:
                    if deadline[0][0] == 0:
                        lhs = _pin(lhs, deadline[0][1], cfg["ao_row"] - 8)
                        deadline[0] = None
                    else:
                        deadline[0] = (deadline[0][0] - 1, deadline[0][1])
                d = _dot(_bf(lhs), _bf(paced(w)))
                set_link(d)
                return d

            def b_op(which, m):
                raw = lambda r, c: w_blk(r, 2 * which + c)
                blk = lambda r, c: _split(raw(r, c))
                return {1: lambda: _add(blk(0, 0), blk(1, 1)),
                        2: lambda: raw(0, 0),
                        3: lambda: _sub(blk(0, 1), blk(1, 1)),
                        4: lambda: _sub(blk(1, 0), blk(0, 0)),
                        5: lambda: raw(1, 1),
                        6: lambda: _add(blk(0, 0), blk(0, 1)),
                        7: lambda: _add(blk(1, 0), blk(1, 1))}[m]()

            def a_op(m, rho):
                rs = _h(rho * tq, tq)
                if m == 3:
                    return c_v[rs, 0:kw]
                if m == 4:
                    return c_v[_h(S // 2 + rho * tq, tq), kw:]
                return sa_v[{1: 0, 2: 1, 5: 2, 6: 3, 7: 4}[m], rs, :]

            b_cache, prod = {}, {}

            def kv_proj(which, blk, flush):
                rho = blk % 2
                for k, m in enumerate((5, 1, 4, 7, 3) if blk < 2 else (2, 6)):
                    if (which, m) not in b_cache:
                        b_cache[which, m] = b_op(which, m)
                    prod[which, m, rho] = one_pass(a_op(m, rho), b_cache[which, m], k == flush)
                p = lambda m: prod[which, m, rho]
                if blk < 2:
                    return [(p(1) + p(4)) + (p(7) - p(5)), p(3) + p(5)]
                return [p(2) + p(4), (p(1) + p(3)) + (p(6) - p(2))]

            def k_proj(blk, flush=-1):
                if cfg["k_str"]:
                    k = kv_proj(0, blk, flush)
                else:
                    ds = [one_pass(c_v[_h(blk * tq, tq), pl.ds((k % 2) * kw, kw)],
                                   w_blk(k % 2, k // 2), k == flush) for k in range(4)]
                    k = [ds[0] + ds[1], ds[2] + ds[3]]
                k_s[_h(blk * tq, tq), :] = _u32(_lanecat(k).astype(BF16))
                if cfg["s_str"] and blk < nq - 1:
                    b = lambda r, c: k[r][c * D:(c + 1) * D, :]
                    sums = [b(0, 0) + b(1, 1), b(0, 1) - b(1, 1), b(1, 0) - b(0, 0),
                            b(0, 0) + b(0, 1), b(1, 0) + b(1, 1)]
                    for n, x in enumerate(sums):
                        kb_s[n, _h(blk * D, D), :] = _u32(x.astype(BF16))

            def v_proj(blk, flush=-1):
                v = kv_proj(1, blk, flush)
                v_s[_h(blk * tq, tq), :] = _u32(_lanecat(v).astype(BF16))
                if blk < nq - 1:
                    b = lambda r, c: v[c][r * D:(r + 1) * D, :]
                    sums = [b(0, 0) + b(1, 1), b(0, 1) - b(1, 1), b(1, 0) - b(0, 0),
                            b(0, 0) + b(0, 1), b(1, 0) + b(1, 1)]
                    for k, x in enumerate(sums):
                        vb_s[k, _h(blk * D, D), :] = _u32(x.astype(BF16))

            def qk(i, dep=None, flush=False):
                r0 = i * tq
                off = None
                if cfg["s_str"] and i > 0:
                    raw = lambda r, c: q_all[h, _h(r0 + r * D, D), c * LANE:(c + 1) * LANE]
                    a = lambda r, c: _split(raw(r, c))
                    sa = {1: _add(a(0, 0), a(1, 1)), 2: _add(a(1, 0), a(1, 1)), 3: raw(0, 0),
                          4: raw(1, 1), 5: _add(a(0, 0), a(0, 1)), 6: _sub(a(1, 0), a(0, 0)),
                          7: _sub(a(0, 1), a(1, 1))}

                    def sb(m, j, t):
                        if m in (2, 5):
                            c = 0 if m == 2 else 1
                            rows = _h(j * tq + c * D + t * LANE, LANE)
                            return k_s[rows, c * LANE:(c + 1) * LANE]
                        n = {1: 0, 3: 1, 4: 2, 6: 3, 7: 4}[m]
                        return kb_s[n, _h(j * D + t * LANE, LANE), :]

                    top, bot, due = {}, {}, []
                    n_dot = 0
                    for j in range(i):
                        for t in range(2):
                            p = {}
                            for n, m in enumerate((5, 1, 4, 7, 2, 3, 6)):
                                lhs = linked(sa[m])
                                if due and n == cfg["s_due"]:
                                    lhs = _pin(lhs, due.pop(), cfg["s_row"])
                                p[m] = _dot_nt(_bf(lhs), _bf(sb(m, j, t)))
                                n_dot += 1
                                if n_dot % 4 == 0:
                                    set_link(p[m], cfg["s_link"])
                            top[4 * j + t] = (p[1] + p[4]) + (p[7] - p[5])
                            top[4 * j + 2 + t] = p[3] + p[5]
                            bot[4 * j + t] = p[2] + p[4]
                            bot[4 * j + 2 + t] = (p[1] + p[3]) + (p[6] - p[2])
                            due.append(_opaque_zero(
                                [x[4 * j + c + t] for x in (top, bot) for c in (0, 2)]))
                    off = _rowcat([_lanecat([x[c] for c in range(4 * i)]) for x in (top, bot)])
                q = linked(q_all[h, _h(r0, tq), :])
                if off is not None:
                    q = _pin(q, due.pop(), cfg["ao_row"] - 8)
                if dep is not None:
                    q = _pin(q, _opaque_zero([dep]), cfg["ao_row"])
                k0 = 0 if off is None else r0
                main = _dot_nt(_bf(q), _bf(k_s[_h(k0, r0 + LANE - k0), :]))
                parts = [main if off is None else _lanecat([off, main])]
                early = None
                if off is not None and cfg["max_late"]:
                    ne = 4 * i - cfg["max_late"] + 1
                    early = (ne, functools.reduce(jnp.maximum, [
                        off[:, t * LANE:(t + 1) * LANE] for t in range(ne)]))
                if i > 0 and off is None:
                    link[0] = _opaque_zero([parts[0][0:8, r0 - LANE:r0]])
                for j in range(1, nsub):
                    q = linked(q_all[h, _h(r0 + LANE * j, tq - LANE * j), :])
                    if j == cfg["q_pin"]:
                        if flush:
                            q = flush_pending(q, 8)
                        if early is not None:
                            q = _pin(q, _opaque_zero([early[1]]), 16)
                    parts.append(_dot_nt(_bf(q), _bf(k_s[_h(r0 + LANE * j, LANE), :])))
                set_link(parts[2], cfg["link_part"], main)
                return parts, early

            def exps(i, parts, early):
                sas, mbs = [], []
                for a in range(nsub):
                    blocks = [parts[j][LANE * (a - j):LANE * (a - j + 1), :] for j in range(a + 1)]
                    last = blocks[-1]
                    w = last.shape[1]
                    dg = jnp.where(tri, last[:, w - LANE:], NEG)
                    blocks[-1] = dg if w == LANE else _lanecat([last[:, :w - LANE], dg])
                    sas.append(_lanecat(blocks))
                    mx = sas[a]
                    if early is not None:
                        mx = _lanecat([early[1][LANE * a:LANE * (a + 1)], mx[:, early[0] * LANE:]])
                    mbs.append(jnp.broadcast_to(jnp.max(mx, axis=1, keepdims=True), (LANE, LANE)))
                chain = _opaque_zero([b[b.shape[0] - 8:, b.shape[1] - LANE:] for b in parts])
                pg, psums = {}, {}
                for r in range(0, tq // 2, 8):
                    for row in (r, r + tq // 2):
                        a, g = divmod(row, LANE)
                        mg = _pin(mbs[a][g:g + 8, :], chain)
                        pg[row] = [jnp.exp2(sas[a][g:g + 8, t:t + LANE] - mg)
                                   for t in range(0, sas[a].shape[1], LANE)]
                        psums[row] = functools.reduce(jnp.add, pg[row])
                        chain = _opaque_zero([psums[row]])
                        chains[i].append(chain)
                return pg, psums

            def softmax(i, pg, psums):
                r0 = i * tq
                pd, pa = pd_s.at[i % 2], pa_s[i % 2]
                first = lambda x, c=0: _pin(x, link[0], 0, c).astype(BF16)
                nt0 = r0 // LANE
                ls = []
                for a in range(nsub):
                    rows = range(LANE * a, LANE * (a + 1), 8)
                    ls.append(jnp.sum(_rowcat([psums[r] for r in rows]), axis=1, keepdims=True))
                    pd[LANE * a:LANE * (a + 1), 0:LANE * (a + 1)] = first(
                        _rowcat([_lanecat(pg[r][nt0:]) for r in rows]), LANE * a)
                if i > 0:
                    quad = lambda rh, ch: _rowcat([
                        _lanecat([pg[rh * (tq // 2) + r][4 * j + 2 * ch + t]
                                  for j in range(i) for t in range(2)])
                        for r in range(0, tq // 2, 8)])
                    a11, a12, a21, a22 = quad(0, 0), quad(0, 1), quad(1, 0), quad(1, 1)
                    ops = [a11 + a22, a21 + a22, a11, a22, a11 + a12, a21 - a11, a12 - a22]
                    for m, x in enumerate(ops):
                        if i == 3:
                            x = _pin(x, link[0], 0, 2 * D)
                        pa[m, :, 0:i * D] = first(x)
                return ls

            def pv(i, ls):
                r0 = i * tq
                pd, pa = pd_s.at[i % 2], pa_s[i % 2]
                off = None
                if i > 0:
                    def b_rows(m, j0, j1):
                        if m in (2, 5):
                            q = 0 if m == 2 else 1
                            return _bf(_rowcat([
                                v_s[_h(j * tq + q * D, D), q * LANE:(q + 1) * LANE]
                                for j in range(j0, j1)]))
                        k = {1: 0, 3: 1, 4: 2, 6: 3, 7: 4}[m]
                        return _bf(vb_s[k, _h(j0 * D, (j1 - j0) * D), :])

                    p = {}
                    for j0, j1 in {1: [(0, 1)], 2: [(0, 2)], 3: [(0, 2), (2, 3)]}[i]:
                        for m in range(1, 8):
                            cols = slice(j0 * D, j1 * D)
                            rhs = b_rows(m, j0, j1)
                            if j1 - j0 == 1 and m == 7:
                                d = _rowcat([_dot(pa[m - 1, r:r + LANE, cols], rhs)
                                             for r in (0, LANE)])
                            else:
                                d = _dot(pa[m - 1, :, cols], rhs)
                            p[m] = d if m not in p else p[m] + d
                    off = _rowcat([
                        _lanecat([(p[1] + p[4]) + (p[7] - p[5]), p[3] + p[5]]),
                        _lanecat([p[2] + p[4], (p[1] + p[3]) + (p[6] - p[2])])])
                ctx = []
                for j in range(nsub):
                    c0 = LANE * j
                    ctx.append(_dot(pd[c0:, c0:c0 + LANE], _bf(v_s[_h(r0 + c0, LANE), :])))
                set_link(ctx[2], cfg["link_part"], ctx[0])
                cs = []
                for a in range(nsub):
                    sl = lambda j: slice(LANE * (a - j), LANE * (a - j + 1))
                    r = pl.reciprocal(ls[a], approx=True)
                    r = r * (2.0 - ls[a] * r)
                    terms = [ctx[j][sl(j)] for j in range(a + 1)]
                    if off is not None:
                        terms.append(off[sl(0)])
                    cs.append(functools.reduce(jnp.add, terms) * r)
                return _rowcat(cs)

            def accumulate(k, res):
                tot = rb_t[k] + res
                rb_t[k] = tot
                if k < n_body:
                    pending.append((k, b_out(k, tot)))

            def oproj_plain(i, ctx):
                ctx = ctx.astype(BF16)
                for u in range(tq // D):
                    lhs = linked(wo_v[h])
                    if i == nq - 1:
                        lhs = flush_pending(lhs, cfg["last_row"])
                    res = _dot_nt(_bf(lhs), ctx[u * D:(u + 1) * D, :])
                    set_link(res)
                    accumulate(i * (tq // D) + u, res)

            wo_cache = {}

            def oproj(i, ctx):
                if i not in cfg["o_str"]:
                    return oproj_plain(i, ctx)
                mh = M // 4
                raw = lambda r, c: wo_v[h, r * mh:(r + 1) * mh, c * LANE:(c + 1) * LANE]
                a = lambda r, c: _split(raw(r, c))
                a_ops = {1: lambda: _add(a(0, 0), a(1, 1)), 2: lambda: _add(a(1, 0), a(1, 1)),
                         3: lambda: raw(0, 0), 4: lambda: raw(1, 1),
                         5: lambda: _add(a(0, 0), a(0, 1)), 6: lambda: _sub(a(1, 0), a(0, 0)),
                         7: lambda: _sub(a(0, 1), a(1, 1))}
                b = lambda r, c: ctx[c * D:(c + 1) * D, r * LANE:(r + 1) * LANE]
                b_ops = {1: lambda: b(0, 0) + b(1, 1), 2: lambda: b(0, 0),
                         3: lambda: b(0, 1) - b(1, 1), 4: lambda: b(1, 0) - b(0, 0),
                         5: lambda: b(1, 1), 6: lambda: b(0, 0) + b(0, 1),
                         7: lambda: b(1, 0) + b(1, 1)}
                p = {}
                for n, m in enumerate((5, 2, 4, 1, 7, 3, 6)):
                    if m not in wo_cache:
                        wo_cache[m] = a_ops[m]()
                    rhs = b_ops[m]().astype(BF16)
                    if n == cfg["o_half"]:
                        halves = [_dot_nt(_bf(linked(wo_cache[m][r:r + mh // 2])), rhs)
                                  for r in (0, mh // 2)]
                        p[m] = _rowcat(halves)
                        set_link(halves[1], 0)
                    else:
                        p[m] = _dot_nt(_bf(linked(wo_cache[m])), rhs)
                        if (n - (n > cfg["o_half"])) % 2 == 1:
                            set_link(p[m], cfg["o_link"])
                accumulate(2 * i, _rowcat([(p[1] + p[4]) + (p[7] - p[5]), p[2] + p[4]]))
                accumulate(2 * i + 1, _rowcat([p[3] + p[5], (p[1] + p[3]) + (p[6] - p[2])]))

            st = {}
            for op in cfg["seq"].split():
                op, _, dl = op.partition("@")
                if dl:
                    ch = chains[int(dl[0])]
                    deadline[0] = (int(dl[1]), ch[int(dl[2:]) * len(ch) // 16 - 1])
                op, _, fl = op.partition("!")
                fl = int(fl) if fl else -1
                kind, i = op[0], int(op[1:] or 0)
                if kind == "K":
                    k_proj(i, fl)
                elif kind == "V":
                    v_proj(i, fl)
                elif kind == "Q":
                    st["e", i] = exps(
                        i, *qk(i, a_out() if i == cfg["ao_at"] else None, fl >= 0))
                elif kind == "P":
                    st["ctx", i] = pv(i, softmax(i, *st["e", i]))
                elif kind == "O":
                    oproj(i, st["ctx", i])
                elif kind == "F" and with_a:
                    st["kv"], xs, hs = a_fwd()
                    st["z"] = a_conv(xs, hs)
                elif kind == "I" and with_a:
                    a_inv(st["kv"], st["z"], fl >= 0)
            assert not pending and deadline[0] is None
            return carry

        with jax.named_scope("loop_a"):
            lax.fori_loop(cfg["h0"], H, head_step, 0)
        with jax.named_scope("tail"):
            for i in range(n_body, NOUT):
                b_out(i, rb_t[i])
                out_copy(i).start()
            for i in range(NOUT + AT):
                out_copy(i).wait()

    scratch = [
        pltpu.VMEM((4, M // 2, S), U32),
        pltpu.VMEM((KS, M), BF16),
        pltpu.VMEM((M,), BF16),
        pltpu.VMEM((KS + 1, M, LANE), F32),
        pltpu.VMEM((LANE // 2, 2 * LANE), U32),
        pltpu.VMEM((M // 2, S), U32),
        pltpu.VMEM((S // 2, MP), U32),
        pltpu.VMEM((5, XH // 2, D), U32),
        pltpu.VMEM((S // 2 + 8, C), U32),
        [pltpu.VMEM((4 * min(TP, M // 2 - kt * TP) * 8, LANE), U32)
         for kt in range(KT)],
        pltpu.VMEM((H // 2, MP // 2, 2 * D), U32),
        pltpu.VMEM((H // 2, x_cols, 2 * D), U32),
        pltpu.VMEM((QIT, C * 8, LANE), U32),
        pltpu.VMEM((H, C // 2, 2 * D), U32),
        pltpu.VMEM((H, M // 2, D), U32),
        pltpu.VMEM((H, S // 2, D), U32),
        pltpu.VMEM((S // 2, D), U32),
        pltpu.VMEM((S // 2, D), U32),
        pltpu.VMEM((5, (nq - 1) * D // 2, LANE), U32),
        pltpu.VMEM((5, (nq - 1) * D // 2, LANE), U32),
        pltpu.VMEM((2, tq, tq), BF16),
        [pltpu.VMEM((7, tq // 2, n * D), BF16) for n in (2, 3)],
        pltpu.VMEM((2, M, S // 2), F32),
        pltpu.VMEM((S // D, M, D), F32),
        pltpu.VMEM((AT + 1, S, LANE), BF16),
        pltpu.VMEM((S, 2 * M - AT * LANE), BF16),
        pltpu.SemaphoreType.DMA((XC,)),
        pltpu.SemaphoreType.DMA((KT,)),
        pltpu.SemaphoreType.DMA((QIT,)),
        pltpu.SemaphoreType.DMA((QIT,)),
        pltpu.SemaphoreType.DMA((2,)),
        pltpu.SemaphoreType.DMA((3,)),
        pltpu.SemaphoreType.DMA((S // D + AT,)),
    ]
    return kernel, scratch


_DEFAULT = dict(
    tq=512, a_width=16, ao_at=1, ao_row=240, link_back=176, link_part=32, pace_row=32,
    pace_step=24, use_a=1, h0=0, last_row=216, o_str=(0, 1, 2, 3), o_link=48, o_half=6, q_jobs=(3, 4), xs_from=3, s_str=1, s_link=64, s_due=4, s_row=120, k_str=1, max_late=0, q_pin=2,
    seq="K0 Q0 K1 Q1 V0 F P0 K2@1116 Q2 O0 V1!4 P1 K3@2116 O1 Q3!0 V2 P2 V3@3116 O2 P3 I!0 O3")


def _build(**kw):
    cfg = dict(_DEFAULT)
    cfg.update(kw)
    kernel, scratch = _make_kernel(cfg)

    def run(A_q, A_k, A_v, A_shift_k, A_ssm_k, A_ssm_D, B_x, B_c_kv, B_w_q, B_w_uk,
            B_w_uv, B_w_o):
        tr = lambda a: jnp.swapaxes(a, 1, 2).reshape(M, S)
        args = (
            tr(A_q), tr(A_k), tr(A_v), A_shift_k.T, A_ssm_k, A_ssm_D, tr(B_x),
            B_c_kv.reshape(S, C),
            B_w_q.reshape(M // 2, 2 * H, D), B_w_uk.reshape(C // 2, 2 * H, D),
            B_w_uv.reshape(C // 2, 2 * H, D),
            jnp.swapaxes(B_w_o, 1, 2),
        )
        out = pl.pallas_call(
            kernel,
            in_specs=[pl.BlockSpec(memory_space=pl.ANY)] * len(args),
            out_specs=pl.BlockSpec(memory_space=pl.ANY),
            out_shape=jax.ShapeDtypeStruct((S, 2 * M), BF16),
            scratch_shapes=scratch,
            compiler_params=pltpu.CompilerParams(
                vmem_limit_bytes=126 * 1024 * 1024,
                disable_bounds_checks=True),
        )(*args)
        return out.reshape(1, S, 2 * M)

    return run


_run = _build()


@jax.jit
def pallas_concat_heads__ssm_conv_h3__compressed_kv_cla__prompt_kernel(
    A_q: jax.Array,
    A_k: jax.Array,
    A_v: jax.Array,
    A_shift_k: jax.Array,
    A_ssm_k: jax.Array,
    A_ssm_D: jax.Array,
    B_x: jax.Array,
    B_c_kv: jax.Array,
    B_w_q: jax.Array,
    B_w_uk: jax.Array,
    B_w_uv: jax.Array,
    B_w_o: jax.Array,
):
    return _run(A_q, A_k, A_v, A_shift_k, A_ssm_k, A_ssm_D, B_x, B_c_kv, B_w_q,
                B_w_uk, B_w_uv, B_w_o)
```

```python
import functools

import jax
import jax.numpy as jnp
from jax import lax
import jax.experimental.pallas as pl
import jax.experimental.pallas.tpu as pltpu

F32 = jnp.float32
BF16 = jnp.bfloat16
U32 = jnp.uint32

S = 2048
M = 448
MP = 512
C = 1024
H = 16
D = 256
KS = 4
LANE = 128
NB = S // LANE
AR = 32
A_STEPS = M // AR
LOG2E = 1.4426950408889634
NEG = -1e30

NT = (((1,), (1,)), ((), ()))


def _dot(a, b):
    return jnp.dot(a, b, preferred_element_type=F32)


def _dot_nt(a, b):
    return lax.dot_general(a, b, NT, preferred_element_type=F32)


def _bf(x):
    return pltpu.bitcast(x, BF16)


def _u32(x):
    return pltpu.bitcast(x, U32)


def _h(r0, n):
    return pl.ds(r0 // 2, n // 2)


def _repack(ev, od):
    lo = (ev & jnp.uint32(0xFFFF)) | (od << 16)
    hi = (ev >> 16) | (od & jnp.uint32(0xFFFF0000))
    return lo, hi


def _split(w):
    return (pltpu.bitcast(w << 16, F32), pltpu.bitcast(w & jnp.uint32(0xFFFF0000), F32))


def _join(lo, hi):
    half = jnp.uint32(0x8000)
    lo = (pltpu.bitcast(lo, U32) + half) >> 16
    hi = (pltpu.bitcast(hi, U32) + half) & jnp.uint32(0xFFFF0000)
    return lo | hi


def _add(a, b):
    return _join(a[0] + b[0], a[1] + b[1])


def _sub(a, b):
    return _join(a[0] - b[0], a[1] - b[1])


def _opaque_zero(vals):
    acc = None
    for v in vals:
        b = v if v.dtype == U32 else pltpu.bitcast(v, U32)
        for r in range(0, b.shape[0], 8):
            for c in range(0, b.shape[1], LANE):
                t = b[r:r + 8, c:c + LANE]
                acc = t if acc is None else acc | t
    return jnp.minimum((acc >> 1).astype(jnp.int32), 0)


def _pin(x, zero, r=0, c=0):
    t = pltpu.bitcast(pltpu.bitcast(x[r:r + 8, c:c + LANE], jnp.int32) + zero, x.dtype)
    row = ([x[r:r + 8, :c]] if c > 0 else []) + [t] + (
        [x[r:r + 8, c + LANE:]] if c + LANE < x.shape[1] else [])
    row = jnp.concatenate(row, axis=1) if len(row) > 1 else row[0]
    col = ([x[:r, :]] if r > 0 else []) + [row] + ([x[r + 8:, :]] if r + 8 < x.shape[0] else [])
    return jnp.concatenate(col, axis=0) if len(col) > 1 else col[0]


def _rowcat(xs):
    return jnp.concatenate(xs, axis=0) if len(xs) > 1 else xs[0]


def _lanecat(xs):
    return jnp.concatenate(xs, axis=1) if len(xs) > 1 else xs[0]


def _make_kernel(cfg):
    tq = cfg["tq"]
    nq = S // tq
    nsub = tq // LANE
    KT = MP // LANE
    TP = LANE // 2
    XC = 4
    x_cols = S // XC
    QP = 2
    QIT = H // 2 // QP
    XH = (S - x_cols) // 2
    CP = 176
    AT = 3

    def kernel(aq_hbm, ak_hbm, av_hbm, sh_hbm, ssm_hbm, dd_hbm, x_hbm, c_hbm,
               wq_hbm, wk_hbm, wv_hbm, wo_hbm,
               out_hbm,
               a_v, sh_v, dd_v, par_v, f_v,
               xt_v, x_v, xs_v, c_v, wqs_v, wq_v, qacc, ws_v, wkv_v, wo_v,
               q_all, k_s, v_s, kb_s, vb_s, pd_s, pa_s, ra_t, rb_t, oa_v, out_v,
               sem_x, sem_wq, sem_w, sem_c, sem_s, sem_a, sem_out):
        x32, c32, wq32, wk32, wv32, wo32 = (
            r.bitcast(U32) for r in (x_hbm, c_hbm, wq_hbm, wk_hbm, wv_hbm, wo_hbm))
        a32 = [r.bitcast(U32) for r in (ak_hbm, av_hbm, ssm_hbm, aq_hbm)]

        sa_v = qacc

        def x_copy(i):
            cs = pl.ds(i * x_cols, x_cols)
            return pltpu.make_async_copy(x32.at[:, cs], xt_v.at[:, cs], sem_x.at[i])

        def wq_pairs(kt):
            return min(TP, M // 2 - kt * TP)

        def wq_copies(kt):
            n = wq_pairs(kt)
            dst = wqs_v[kt].reshape(4, n, 8, LANE)
            return [pltpu.make_async_copy(
                wq32.at[pl.ds(kt * TP, n), pl.ds(8 * (k // 2), 8), pl.ds((k % 2) * LANE, LANE)],
                dst.at[k], sem_wq.at[kt]) for k in range(4)]

        def wq_wait(kt):
            pltpu.make_async_copy(wqs_v[kt], wqs_v[kt], sem_wq.at[kt]).wait()

        def w_copies(g):
            dst = ws_v.reshape(8, C // 2, 8, LANE)
            src = (wk32, wv32)[g // 2]
            return [pltpu.make_async_copy(
                src.at[:, pl.ds(8 * par, 8), pl.ds((g % 2) * LANE, LANE)],
                dst.at[2 * g + par], sem_w.at[g]) for par in range(2)]

        def w_wait(g):
            pltpu.make_async_copy(ws_v.at[g], ws_v.at[g], sem_w.at[g]).wait()

        c_bounds = [0, CP, 2 * CP, S // 4]

        def c_copies(p):
            r0, n = c_bounds[p], c_bounds[p + 1] - c_bounds[p]
            return [pltpu.make_async_copy(c32.at[rs], c_v.at[rs], sem_c.at[p])
                    for rs in (pl.ds(r0, n), pl.ds(S // 4 + r0, n))]

        wo_copy = pltpu.make_async_copy(wo32, wo_v, sem_a.at[0])

        a_parts = [pl.ds(0, AR // 2), pl.ds(AR // 2, M // 2 - AR // 2)]

        def a_start(part):
            rs = a_parts[part]
            for k in range(4):
                pltpu.make_async_copy(
                    a32[k].at[rs], a_v.at[k, rs], sem_a.at[1 + part]).start()

        def a_wait(part):
            view = a_v.at[:, a_parts[part]]
            pltpu.make_async_copy(view, view, sem_a.at[1 + part]).wait()

        small = [pltpu.make_async_copy(sh_hbm, sh_v, sem_s.at[0]),
                 pltpu.make_async_copy(dd_hbm, dd_v, sem_s.at[1])]

        link = [None]
        pace = [None]

        def set_link(res, row=None, pacer=None):
            if row is None:
                row = res.shape[0] - cfg["link_back"]
            link[0] = _opaque_zero([res[row:row + 8, res.shape[1] - LANE:]])
            pace[0] = res if pacer is None else pacer

        def linked(x):
            return x if link[0] is None else _pin(x, link[0])

        def paced(w):
            res = pace[0]
            if res is None or link[0] is None or not cfg["pace_step"]:
                return w
            rows = []
            r0, step = cfg["pace_row"], cfg["pace_step"]
            if res.shape[0] < 400:
                r0, step = 0, 8
            if res.shape[0] < 200:
                return w
            zs = [_opaque_zero([res[r:r + 8, res.shape[1] - LANE:]])
                  for r in range(r0, r0 + 8 * step, step)]
            for r in range(0, w.shape[0], 8):
                z = zs[7 - (r // 8) % 8]
                t = pltpu.bitcast(w[r:r + 8, :], jnp.int32)
                rows.append(pltpu.bitcast(t + _lanecat([z] * (w.shape[1] // LANE)), U32))
            return _rowcat(rows)

        for cp in small:
            cp.start()
        x_copy(0).start()
        for cp in wq_copies(0):
            cp.start()

        def zero_body(k, carry):
            n = LANE // (S // D)
            bi = lax.broadcasted_iota(jnp.int32, (n, LANE), 0) + k * n
            mi = lax.broadcasted_iota(jnp.int32, (n, LANE), 1)
            ph = ((4 * mi + 1) * bi) & 511
            ang = ph.astype(F32) * (2.0 * 3.141592653589793 / 512.0)
            rs = pl.ds(pl.multiple_of(k * (n // 2), n // 2), n // 2)
            f_v[rs, 0:LANE] = _u32(jnp.cos(ang).astype(BF16))
            f_v[rs, LANE:] = _u32((-jnp.sin(ang)).astype(BF16))

            rb_t[k] = jnp.zeros((M, D), F32)
            cs = pl.ds(pl.multiple_of((k % 4) * D, D), D)
            ra_t[k // 4, 0:LANE, cs] = jnp.zeros((LANE, D), F32)
            ra_t[k // 4, AT * LANE:, cs] = jnp.zeros((M - AT * LANE, D), F32)
            return carry

        lax.fori_loop(0, S // D, zero_body, 0)
        c_v[S // 2:, :] = jnp.zeros((8, C), U32)

        for kt in range(1, KT):
            for cp in wq_copies(kt):
                cp.start()
        with jax.named_scope("small_wait"):
            for cp in small:
                cp.wait()
        sh = sh_v[...].astype(F32)
        for j in range(KS):
            par_v[j] = jnp.broadcast_to(sh[j:j + 1, :], (LANE, M)).T
        dd = dd_v[...].astype(F32).reshape(1, M)
        par_v[KS] = jnp.broadcast_to(dd, (LANE, M)).T

        def x_transpose(i):
            xt = xt_v[:, pl.ds(i * x_cols, x_cols)]
            xt = _rowcat([xt, jnp.zeros((MP // 2 - M // 2, x_cols), U32)])
            x_v[_h(i * x_cols, x_cols), :] = _u32(_bf(xt).astype(F32).T.astype(BF16))

        def q_early(kt, keep=False, jobs=()):
            first, last = kt == 0, kt == KT - 1
            n = wq_pairs(kt)
            cols = pl.ds(kt * LANE, LANE)
            if not keep:
                link[0] = None
            for j in range(H // 2):
                ws = []
                for half in range(2):
                    ev, od = (wqs_v[kt][pl.ds((2 * par + half) * n * 8 + j, n, stride=8), :]
                              for par in range(2))
                    ws.append(_repack(ev, od))
                w = _lanecat([ws[0][0], ws[1][0], ws[0][1], ws[1][1]])
                if n < TP:
                    w = _rowcat([w, jnp.zeros((TP - n, 2 * D), U32)])
                wq_v[j, pl.ds(kt * TP, TP), :] = w
                lhs = linked(x_v[_h(0, x_cols), cols])
                j0 = cfg["xs_from"]
                if jobs and j >= j0:
                    nj = H // 2 - j0
                    mine = jobs[(j - j0) * len(jobs) // nj:(j - j0 + 1) * len(jobs) // nj]
                    for k, job in enumerate(mine):
                        lhs = _pin(lhs, _opaque_zero(job()), 8 * (1 + k * 30 // len(mine)))
                d = _dot(_bf(lhs), _bf(w))
                set_link(d)
                if not first:
                    d = d + pltpu.bitcast(qacc[j], F32)
                if last:
                    d = (d * (D ** -0.5 * LOG2E)).astype(BF16)
                    for t in range(2):
                        q_all[2 * j + t, _h(0, x_cols), :] = _u32(d[:, t * D:(t + 1) * D])
                else:
                    qacc[j] = pltpu.bitcast(d, U32)

        with jax.named_scope("x_wait"):
            x_copy(0).wait()
        x_transpose(0)
        for i in range(1, XC):
            x_copy(i).start()
        for g in range(QIT):
            for cp in w_copies(g) + (c_copies(g) if g < QIT - 1 else []):
                cp.start()
        wo_copy.start()
        a_start(0)
        a_start(1)
        with jax.named_scope("wq_wait"):
            wq_wait(0)
        q_early(0)
        with jax.named_scope("wq_wait"):
            wq_wait(1)
            wq_wait(2)
        q_early(1)
        q_early(2, keep=True)
        with jax.named_scope("wq_wait"):
            wq_wait(3)
            for i in range(1, XC):
                x_copy(i).wait()
        for i in range(1, XC):
            x_transpose(i)

        def x_sums(u):
            a11, a12, a21, a22 = (
                _split(x_v[pl.ds((x_cols + rb * XH) // 2 + 8 * u, 8), cb * D:(cb + 1) * D])
                for rb in range(2) for cb in range(2))
            outs = [_add(a11, a22), _add(a21, a22), _add(a11, a12), _sub(a21, a11),
                    _sub(a12, a22)]
            for k, o in enumerate(outs):
                xs_v[k, 8 * u:8 * u + 8, :] = o
            return outs

        q_early(3, jobs=[functools.partial(x_sums, u) for u in range(XH // 16)])

        def unpack(it, sub, j):
            g = it
            ev, od = (ws_v[g, pl.ds((par * (C // 2) + sub * TP) * 8 + j, TP, stride=8), :]
                      for par in range(2))
            lo, hi = _repack(ev, od)
            rows = pl.ds(sub * TP, TP)
            cols = pl.ds(pl.multiple_of(g * LANE, LANE), LANE)
            wkv_v[2 * j, rows, cols] = lo
            wkv_v[2 * j + 1, rows, cols] = hi
            return [lo, hi]

        def a_sums(it, u):
            r0 = jnp.clip((it - 1) * CP, 0, S // 4 - CP) + 8 * u
            src = [jnp.where(it == 0, S // 2, r0 + rb * (S // 4)) for rb in range(2)]
            r0 = pl.multiple_of(r0, 8)
            kw = C // 2
            a11, a12, a21, a22 = (
                _split(c_v[pl.ds(pl.multiple_of(src[rb], 8), 8), pl.ds(cb * kw, kw)])
                for rb in range(2) for cb in range(2))
            outs = [_add(a11, a22), _add(a21, a22), _add(a11, a12), _sub(a21, a11),
                    _sub(a12, a22)]
            for k, o in enumerate(outs):
                sa_v[k, pl.ds(r0, 8), :] = o
            return outs

        units = [functools.partial(unpack, sub=s_, j=j_)
                 for s_ in range(C // 2 // TP) for j_ in range(H // 2)]
        for u_ in range(CP // 8):
            units.insert(4 * u_ + 1, functools.partial(a_sums, u=u_))

        def q_pair(pair, todo):
            raw = lambda r, c: _lanecat([
                wq_v[pair, r * LANE:(r + 1) * LANE, pl.ds(t * D + c * LANE, LANE)]
                for t in range(2)])
            b = lambda r, c: _split(raw(r, c))
            sb = {1: _add(b(0, 0), b(1, 1)), 2: raw(0, 0), 3: _sub(b(0, 1), b(1, 1)),
                  4: _sub(b(1, 0), b(0, 0)), 5: raw(1, 1), 6: _add(b(0, 0), b(0, 1)),
                  7: _add(b(1, 0), b(1, 1))}
            n = XH // 2
            for rho in range(2):
                def sa(m):
                    if m == 3:
                        return x_v[_h(x_cols + rho * n, n), 0:D]
                    if m == 4:
                        return x_v[_h(x_cols + XH + rho * n, n), D:]
                    return xs_v[{1: 0, 2: 1, 5: 2, 6: 3, 7: 4}[m], _h(rho * n, n), :]

                def put(half, c0, c1):
                    rows = _h(x_cols + half * XH + rho * n, n)
                    out = []
                    for t in range(2):
                        q = _lanecat([c[:, t * LANE:(t + 1) * LANE] for c in (c0, c1)])
                        out.append(_u32((q * (D ** -0.5 * LOG2E)).astype(BF16)))
                        q_all[2 * pair + t, rows, :] = out[-1]
                    q_due.append(_opaque_zero(out))

                p = {}
                for m in (5, 1, 4, 7, 3, 2, 6):
                    lhs = linked(sa(m))
                    nj = min(len(todo), cfg["q_jobs"][rho])
                    jobs = [todo.pop()(it=pair // QP) for _ in range(nj)]
                    for k, job in enumerate(jobs):
                        lhs = _pin(lhs, _opaque_zero(job), 8 * (1 + k * (n // 16 - 1) // nj))
                    if q_due and m in (1, 6):
                        lhs = _pin(lhs, q_due.pop(), n // 2 - 8, LANE)
                    p[m] = _dot(_bf(lhs), _bf(sb[m]))
                    set_link(p[m])
                    if m == 3:
                        put(0, (p[1] + p[4]) + (p[7] - p[5]), p[3] + p[5])
                put(1, p[2] + p[4], (p[1] + p[3]) + (p[6] - p[2]))

        q_due = []

        def q_body(it, carry):
            with jax.named_scope("w_wait"):
                w_wait(it)
                for p in range(QIT - 1):
                    @pl.when(it == p + 1)
                    def _():
                        for cp in c_copies(p):
                            cp.wait()
            link[0] = None
            todo = units[::-1]
            del q_due[:]
            for p in range(QP):
                q_pair(QP * it + p, todo)
            assert not todo
            return carry

        with jax.named_scope("q_loop"):
            lax.fori_loop(0, QIT, q_body, 0)
        wo_copy.wait()
        a_wait(0)

        tri = (lax.broadcasted_iota(jnp.int32, (LANE, LANE), 1)
               <= lax.broadcasted_iota(jnp.int32, (LANE, LANE), 0))

        NOUT = S // D

        def out_copy(i):
            if i >= NOUT:
                t = i - NOUT
                return pltpu.make_async_copy(
                    oa_v.at[t], out_hbm.at[:, pl.ds(t * LANE, LANE)], sem_out.at[i])
            rs = pl.ds(i * D, D)
            return pltpu.make_async_copy(
                out_v.at[rs], out_hbm.at[rs, pl.ds(AT * LANE, 2 * M - AT * LANE)], sem_out.at[i])

        n_body = NOUT - (tq // D if nq - 1 in cfg["o_str"] else 1)

        def b_out(k, tot):
            c0 = (k * D) % (S // 2)
            full = _rowcat([ra_t[k * D // (S // 2), AT * LANE:, c0:c0 + D], tot]).T
            out_v[k * D:(k + 1) * D, :] = full.astype(BF16)
            return full

        def head_step(h, carry):
            with jax.named_scope("step"):
                return head_step_(h, carry)

        def head_step_(h, carry):
            with_a = cfg["use_a"]

            @pl.when(h == A_STEPS)
            def _():
                for t in range(AT):
                    out_copy(NOUT + t).start()

            @pl.when(h == cfg["h0"] + 1)
            def _():
                a_wait(1)

            link[0] = None
            n2 = AR // 2
            a_rows2 = pl.ds(pl.multiple_of(jnp.minimum(h, A_STEPS - 1) * n2, n2), n2)
            a_rows = pl.ds(pl.multiple_of(jnp.minimum(h, A_STEPS - 1) * AR, AR), AR)

            kw = C // 2
            pending = []
            chains = {i: [] for i in range(nq + 1)}
            deadline = [None]

            def flush_pending(x, row):
                done = list(pending)
                del pending[:]
                if not done:
                    return x
                x = _pin(x, _opaque_zero([f for _, f in done]), row)

                @pl.when(h == H - 1)
                def _():
                    for k, _f in done:
                        out_copy(k).start()
                return x

            def a_fwd():
                kk = _bf(a_v[0, a_rows2, :]).astype(F32)
                lane = lax.broadcasted_iota(jnp.int32, (AR, LANE), 1)
                coef = [par_v[j, a_rows, :] for j in range(KS)]
                rolled = [kk] + [pltpu.roll(kk, j, 1) for j in range(1, KS)]
                vv = _bf(a_v[1, a_rows2, :]).astype(F32)
                kv_blocks = []
                for a in range(NB):
                    cs = slice(a * LANE, (a + 1) * LANE)
                    acc = rolled[0][:, cs] * coef[0]
                    for j in range(1, KS):
                        t = rolled[j][:, cs]
                        if a == 0:
                            t = jnp.where(lane >= j, t, 0.0)
                        acc = acc + t * coef[j]
                    kv_blocks.append(acc * vv[:, cs])
                hk = a_v[2, a_rows2, :]
                hk = _rowcat([hk[:, a * LANE:(a + 1) * LANE] for a in range(NB)])
                fm = _bf(f_v[...])
                hs = _dot(_bf(linked(hk)), fm)
                kv = linked(_rowcat(kv_blocks)).astype(BF16)
                xs = _dot(kv, fm)
                set_link(xs)
                return kv, xs, hs

            def a_conv(xs, hs):
                def tile(v, a, g, part):
                    r = a * AR + 8 * g
                    return v[r:r + 8, part * LANE:(part + 1) * LANE]

                z = {}
                gate = None
                width = cfg["a_width"]
                for g in range(AR // 8):
                    hr = [tile(hs, 0, g, 0)] + [
                        tile(hs, j, g, 0) - tile(hs, j - 1, g, 1) for j in range(1, NB)]
                    hi = [tile(hs, 0, g, 1)] + [
                        tile(hs, j, g, 1) + tile(hs, j - 1, g, 0) for j in range(1, NB)]
                    for c0 in range(0, NB, width):
                        for a in range(c0 + width):
                            xr, xi = tile(xs, a, g, 0), tile(xs, a, g, 1)
                            if gate is not None:
                                xr, xi = _pin(xr, gate), _pin(xi, gate)
                            for c in range(max(c0, a), c0 + width):
                                j = c - a
                                tr = xr * hr[j] - xi * hi[j]
                                ti = xr * hi[j] + xi * hr[j]
                                z[c, g] = (tr, ti) if a == 0 else (z[c, g][0] + tr, z[c, g][1] + ti)
                            gate = _opaque_zero(list(z[c0 + width - 1, g]))
                            chains[nq].append(gate)
                return z

            def a_inv(kv, z, flush=False):
                fm = _bf(f_v[...])
                ng = AR // 8
                ys = []
                for u in range(2):
                    rows = [_lanecat(z[c, g]) for g in range(u * ng // 2, (u + 1) * ng // 2)
                            for c in range(NB)]
                    lhs = linked(_rowcat(rows))
                    if flush:
                        lhs = flush_pending(lhs, 8)
                    ys.append(_dot_nt(lhs.astype(BF16), fm))
                y = _rowcat(ys)
                dd = par_v[KS, a_rows, :]
                for c in range(NB):
                    cs = slice(c * LANE, (c + 1) * LANE)
                    yc = _rowcat([y[(g * NB + c) * 8:(g * NB + c + 1) * 8, :] for g in range(ng)])
                    qq = _bf(a_v[3, a_rows2, cs]).astype(F32)
                    kvf = kv[c * AR:(c + 1) * AR, :].astype(F32)
                    c2 = (c % (NB // 2)) * LANE
                    ra_t[c // (NB // 2), a_rows, c2:c2 + LANE] = qq * (yc * (1.0 / LANE) + kvf * dd)

            def a_out():
                slab = jnp.clip(h // 4 - 1, 0, AT - 1)
                half = h % 2
                x = ra_t[half, pl.ds(pl.multiple_of(slab * LANE, LANE), LANE), :]
                xt = x.T
                dst = jnp.where(h >= A_STEPS, AT, slab)
                oa_v[dst, pl.ds(pl.multiple_of(half * (S // 2), S // 2), S // 2), :] = xt.astype(BF16)
                return xt

            def w_blk(r, c):
                return wkv_v[h, _h(r * kw, kw), pl.ds(c * LANE, LANE)]

            def one_pass(lhs, w, flush):
                lhs = linked(lhs)
                if flush:
                    lhs = flush_pending(lhs, cfg["ao_row"])
                if deadline[0] is not None:
                    if deadline[0][0] == 0:
                        lhs = _pin(lhs, deadline[0][1], cfg["ao_row"] - 8)
                        deadline[0] = None
                    else:
                        deadline[0] = (deadline[0][0] - 1, deadline[0][1])
                d = _dot(_bf(lhs), _bf(paced(w)))
                set_link(d)
                return d

            def b_op(which, m):
                raw = lambda r, c: w_blk(r, 2 * which + c)
                blk = lambda r, c: _split(raw(r, c))
                return {1: lambda: _add(blk(0, 0), blk(1, 1)),
                        2: lambda: raw(0, 0),
                        3: lambda: _sub(blk(0, 1), blk(1, 1)),
                        4: lambda: _sub(blk(1, 0), blk(0, 0)),
                        5: lambda: raw(1, 1),
                        6: lambda: _add(blk(0, 0), blk(0, 1)),
                        7: lambda: _add(blk(1, 0), blk(1, 1))}[m]()

            def a_op(m, rho):
                rs = _h(rho * tq, tq)
                if m == 3:
                    return c_v[rs, 0:kw]
                if m == 4:
                    return c_v[_h(S // 2 + rho * tq, tq), kw:]
                return sa_v[{1: 0, 2: 1, 5: 2, 6: 3, 7: 4}[m], rs, :]

            b_cache, prod = {}, {}

            def kv_proj(which, blk, flush):
                rho = blk % 2
                for k, m in enumerate((5, 1, 4, 7, 3) if blk < 2 else (2, 6)):
                    if (which, m) not in b_cache:
                        b_cache[which, m] = b_op(which, m)
                    prod[which, m, rho] = one_pass(a_op(m, rho), b_cache[which, m], k == flush)
                p = lambda m: prod[which, m, rho]
                if blk < 2:
                    return [(p(1) + p(4)) + (p(7) - p(5)), p(3) + p(5)]
                return [p(2) + p(4), (p(1) + p(3)) + (p(6) - p(2))]

            def k_proj(blk, flush=-1):
                if cfg["k_str"]:
                    k = kv_proj(0, blk, flush)
                else:
                    ds = [one_pass(c_v[_h(blk * tq, tq), pl.ds((k % 2) * kw, kw)],
                                   w_blk(k % 2, k // 2), k == flush) for k in range(4)]
                    k = [ds[0] + ds[1], ds[2] + ds[3]]
                k_s[_h(blk * tq, tq), :] = _u32(_lanecat(k).astype(BF16))
                if cfg["s_str"] and blk < nq - 1:
                    b = lambda r, c: k[r][c * D:(c + 1) * D, :]
                    sums = [b(0, 0) + b(1, 1), b(0, 1) - b(1, 1), b(1, 0) - b(0, 0),
                            b(0, 0) + b(0, 1), b(1, 0) + b(1, 1)]
                    for n, x in enumerate(sums):
                        kb_s[n, _h(blk * D, D), :] = _u32(x.astype(BF16))

            def v_proj(blk, flush=-1):
                v = kv_proj(1, blk, flush)
                v_s[_h(blk * tq, tq), :] = _u32(_lanecat(v).astype(BF16))
                if blk < nq - 1:
                    b = lambda r, c: v[c][r * D:(r + 1) * D, :]
                    sums = [b(0, 0) + b(1, 1), b(0, 1) - b(1, 1), b(1, 0) - b(0, 0),
                            b(0, 0) + b(0, 1), b(1, 0) + b(1, 1)]
                    for k, x in enumerate(sums):
                        vb_s[k, _h(blk * D, D), :] = _u32(x.astype(BF16))

            def qk(i, dep=None, flush=False):
                r0 = i * tq
                off = None
                if cfg["s_str"] and i > 0:
                    raw = lambda r, c: q_all[h, _h(r0 + r * D, D), c * LANE:(c + 1) * LANE]
                    a = lambda r, c: _split(raw(r, c))
                    sa = {1: _add(a(0, 0), a(1, 1)), 2: _add(a(1, 0), a(1, 1)), 3: raw(0, 0),
                          4: raw(1, 1), 5: _add(a(0, 0), a(0, 1)), 6: _sub(a(1, 0), a(0, 0)),
                          7: _sub(a(0, 1), a(1, 1))}

                    def sb(m, j, t):
                        if m in (2, 5):
                            c = 0 if m == 2 else 1
                            rows = _h(j * tq + c * D + t * LANE, LANE)
                            return k_s[rows, c * LANE:(c + 1) * LANE]
                        n = {1: 0, 3: 1, 4: 2, 6: 3, 7: 4}[m]
                        return kb_s[n, _h(j * D + t * LANE, LANE), :]

                    top, bot, due = {}, {}, []
                    n_dot = 0
                    for j in range(i):
                        for t in range(2):
                            p = {}
                            for n, m in enumerate((5, 1, 4, 7, 2, 3, 6)):
                                lhs = linked(sa[m])
                                if due and n == cfg["s_due"]:
                                    lhs = _pin(lhs, due.pop(), cfg["s_row"])
                                p[m] = _dot_nt(_bf(lhs), _bf(sb(m, j, t)))
                                n_dot += 1
                                if n_dot % 4 == 0:
                                    set_link(p[m], cfg["s_link"])
                            top[4 * j + t] = (p[1] + p[4]) + (p[7] - p[5])
                            top[4 * j + 2 + t] = p[3] + p[5]
                            bot[4 * j + t] = p[2] + p[4]
                            bot[4 * j + 2 + t] = (p[1] + p[3]) + (p[6] - p[2])
                            due.append(_opaque_zero(
                                [x[4 * j + c + t] for x in (top, bot) for c in (0, 2)]))
                    off = _rowcat([_lanecat([x[c] for c in range(4 * i)]) for x in (top, bot)])
                q = linked(q_all[h, _h(r0, tq), :])
                if off is not None:
                    q = _pin(q, due.pop(), cfg["ao_row"] - 8)
                if dep is not None:
                    q = _pin(q, _opaque_zero([dep]), cfg["ao_row"])
                k0 = 0 if off is None else r0
                main = _dot_nt(_bf(q), _bf(k_s[_h(k0, r0 + LANE - k0), :]))
                parts = [main if off is None else _lanecat([off, main])]
                early = None
                if off is not None and cfg["max_late"]:
                    ne = 4 * i - cfg["max_late"] + 1
                    early = (ne, functools.reduce(jnp.maximum, [
                        off[:, t * LANE:(t + 1) * LANE] for t in range(ne)]))
                if i > 0 and off is None:
                    link[0] = _opaque_zero([parts[0][0:8, r0 - LANE:r0]])
                for j in range(1, nsub):
                    q = linked(q_all[h, _h(r0 + LANE * j, tq - LANE * j), :])
                    if j == cfg["q_pin"]:
                        if flush:
                            q = flush_pending(q, 8)
                        if early is not None:
                            q = _pin(q, _opaque_zero([early[1]]), 16)
                    parts.append(_dot_nt(_bf(q), _bf(k_s[_h(r0 + LANE * j, LANE), :])))
                set_link(parts[2], cfg["link_part"], main)
                return parts, early

            def exps(i, parts, early):
                sas, mbs = [], []
                for a in range(nsub):
                    blocks = [parts[j][LANE * (a - j):LANE * (a - j + 1), :] for j in range(a + 1)]
                    last = blocks[-1]
                    w = last.shape[1]
                    dg = jnp.where(tri, last[:, w - LANE:], NEG)
                    blocks[-1] = dg if w == LANE else _lanecat([last[:, :w - LANE], dg])
                    sas.append(_lanecat(blocks))
                    mx = sas[a]
                    if early is not None:
                        mx = _lanecat([early[1][LANE * a:LANE * (a + 1)], mx[:, early[0] * LANE:]])
                    mbs.append(jnp.broadcast_to(jnp.max(mx, axis=1, keepdims=True), (LANE, LANE)))
                chain = _opaque_zero([b[b.shape[0] - 8:, b.shape[1] - LANE:] for b in parts])
                pg, psums = {}, {}
                for r in range(0, tq // 2, 8):
                    for row in (r, r + tq // 2):
                        a, g = divmod(row, LANE)
                        mg = _pin(mbs[a][g:g + 8, :], chain)
                        pg[row] = [jnp.exp2(sas[a][g:g + 8, t:t + LANE] - mg)
                                   for t in range(0, sas[a].shape[1], LANE)]
                        psums[row] = functools.reduce(jnp.add, pg[row])
                        chain = _opaque_zero([psums[row]])
                        chains[i].append(chain)
                return pg, psums

            def softmax(i, pg, psums):
                r0 = i * tq
                pd, pa = pd_s.at[i % 2], pa_s[i % 2]
                first = lambda x, c=0: _pin(x, link[0], 0, c).astype(BF16)
                nt0 = r0 // LANE
                ls = []
                for a in range(nsub):
                    rows = range(LANE * a, LANE * (a + 1), 8)
                    ls.append(jnp.sum(_rowcat([psums[r] for r in rows]), axis=1, keepdims=True))
                    pd[LANE * a:LANE * (a + 1), 0:LANE * (a + 1)] = first(
                        _rowcat([_lanecat(pg[r][nt0:]) for r in rows]), LANE * a)
                if i > 0:
                    quad = lambda rh, ch: _rowcat([
                        _lanecat([pg[rh * (tq // 2) + r][4 * j + 2 * ch + t]
                                  for j in range(i) for t in range(2)])
                        for r in range(0, tq // 2, 8)])
                    a11, a12, a21, a22 = quad(0, 0), quad(0, 1), quad(1, 0), quad(1, 1)
                    ops = [a11 + a22, a21 + a22, a11, a22, a11 + a12, a21 - a11, a12 - a22]
                    for m, x in enumerate(ops):
                        if i == 3:
                            x = _pin(x, link[0], 0, 2 * D)
                        pa[m, :, 0:i * D] = first(x)
                return ls

            def pv(i, ls, flush=-1):
                r0 = i * tq
                pd, pa = pd_s.at[i % 2], pa_s[i % 2]
                off = None
                if i > 0:
                    def b_rows(m, j0, j1):
                        if m in (2, 5):
                            q = 0 if m == 2 else 1
                            return _rowcat([
                                v_s[_h(j * tq + q * D, D), q * LANE:(q + 1) * LANE]
                                for j in range(j0, j1)])
                        k = {1: 0, 3: 1, 4: 2, 6: 3, 7: 4}[m]
                        return vb_s[k, _h(j0 * D, (j1 - j0) * D), :]

                    p, n_dot = {}, 0
                    for j0, j1 in {1: [(0, 1)], 2: [(0, 2)], 3: [(0, 2), (2, 3)]}[i]:
                        for m in range(1, 8):
                            cols = slice(j0 * D, j1 * D)
                            rhs = b_rows(m, j0, j1)
                            if n_dot == flush:
                                rhs = flush_pending(rhs, 0)
                            rhs = _bf(rhs)
                            n_dot += 1
                            if j1 - j0 == 1 and m == 7:
                                d = _rowcat([_dot(pa[m - 1, r:r + LANE, cols], rhs)
                                             for r in (0, LANE)])
                            else:
                                d = _dot(pa[m - 1, :, cols], rhs)
                            p[m] = d if m not in p else p[m] + d
                    off = _rowcat([
                        _lanecat([(p[1] + p[4]) + (p[7] - p[5]), p[3] + p[5]]),
                        _lanecat([p[2] + p[4], (p[1] + p[3]) + (p[6] - p[2])])])
                ctx = []
                for j in range(nsub):
                    c0 = LANE * j
                    ctx.append(_dot(pd[c0:, c0:c0 + LANE], _bf(v_s[_h(r0 + c0, LANE), :])))
                set_link(ctx[2], cfg["link_part"], ctx[0])
                cs = []
                for a in range(nsub):
                    sl = lambda j: slice(LANE * (a - j), LANE * (a - j + 1))
                    r = pl.reciprocal(ls[a], approx=True)
                    r = r * (2.0 - ls[a] * r)
                    terms = [ctx[j][sl(j)] for j in range(a + 1)]
                    if off is not None:
                        terms.append(off[sl(0)])
                    cs.append(functools.reduce(jnp.add, terms) * r)
                return _rowcat(cs)

            def accumulate(k, res):
                tot = rb_t[k] + res
                rb_t[k] = tot
                if k < n_body:
                    pending.append((k, b_out(k, tot)))

            def oproj_plain(i, ctx):
                ctx = ctx.astype(BF16)
                for u in range(tq // D):
                    lhs = linked(wo_v[h])
                    if i == nq - 1:
                        lhs = flush_pending(lhs, cfg["last_row"])
                    res = _dot_nt(_bf(lhs), ctx[u * D:(u + 1) * D, :])
                    set_link(res)
                    accumulate(i * (tq // D) + u, res)

            wo_cache = {}

            def oproj(i, ctx):
                if i not in cfg["o_str"]:
                    return oproj_plain(i, ctx)
                mh = M // 4
                raw = lambda r, c: wo_v[h, r * mh:(r + 1) * mh, c * LANE:(c + 1) * LANE]
                a = lambda r, c: _split(raw(r, c))
                a_ops = {1: lambda: _add(a(0, 0), a(1, 1)), 2: lambda: _add(a(1, 0), a(1, 1)),
                         3: lambda: raw(0, 0), 4: lambda: raw(1, 1),
                         5: lambda: _add(a(0, 0), a(0, 1)), 6: lambda: _sub(a(1, 0), a(0, 0)),
                         7: lambda: _sub(a(0, 1), a(1, 1))}
                b = lambda r, c: ctx[c * D:(c + 1) * D, r * LANE:(r + 1) * LANE]
                b_ops = {1: lambda: b(0, 0) + b(1, 1), 2: lambda: b(0, 0),
                         3: lambda: b(0, 1) - b(1, 1), 4: lambda: b(1, 0) - b(0, 0),
                         5: lambda: b(1, 1), 6: lambda: b(0, 0) + b(0, 1),
                         7: lambda: b(1, 0) + b(1, 1)}
                p = {}
                for n, m in enumerate((5, 2, 4, 1, 7, 3, 6)):
                    if m not in wo_cache:
                        wo_cache[m] = a_ops[m]()
                    rhs = b_ops[m]().astype(BF16)
                    if n == cfg["o_half"]:
                        halves = [_dot_nt(_bf(linked(wo_cache[m][r:r + mh // 2])), rhs)
                                  for r in (0, mh // 2)]
                        p[m] = _rowcat(halves)
                        set_link(halves[1], 0)
                    else:
                        p[m] = _dot_nt(_bf(linked(wo_cache[m])), rhs)
                        if (n - (n > cfg["o_half"])) % 2 == 1:
                            set_link(p[m], cfg["o_link"])
                accumulate(2 * i, _rowcat([(p[1] + p[4]) + (p[7] - p[5]), p[2] + p[4]]))
                accumulate(2 * i + 1, _rowcat([p[3] + p[5], (p[1] + p[3]) + (p[6] - p[2])]))

            st = {}
            for op in cfg["seq"].split():
                op, _, dl = op.partition("@")
                if dl:
                    ch = chains[int(dl[0])]
                    deadline[0] = (int(dl[1]), ch[int(dl[2:]) * len(ch) // 16 - 1])
                op, _, fl = op.partition("!")
                fl = int(fl) if fl else -1
                kind, i = op[0], int(op[1:] or 0)
                if kind == "K":
                    k_proj(i, fl)
                elif kind == "V":
                    v_proj(i, fl)
                elif kind == "Q":
                    st["e", i] = exps(
                        i, *qk(i, a_out() if i == cfg["ao_at"] else None, fl >= 0))
                elif kind == "P":
                    st["ctx", i] = pv(i, softmax(i, *st["e", i]), fl)
                elif kind == "O":
                    oproj(i, st["ctx", i])
                elif kind == "F" and with_a:
                    st["kv"], xs, hs = a_fwd()
                    st["z"] = a_conv(xs, hs)
                elif kind == "I" and with_a:
                    a_inv(st["kv"], st["z"], fl >= 0)
            assert not pending and deadline[0] is None
            return carry

        with jax.named_scope("loop_a"):
            lax.fori_loop(cfg["h0"], H, head_step, 0)
        with jax.named_scope("tail"):
            for i in range(n_body, NOUT):
                b_out(i, rb_t[i])
                out_copy(i).start()
            for i in range(NOUT + AT):
                out_copy(i).wait()

    scratch = [
        pltpu.VMEM((4, M // 2, S), U32),
        pltpu.VMEM((KS, M), BF16),
        pltpu.VMEM((M,), BF16),
        pltpu.VMEM((KS + 1, M, LANE), F32),
        pltpu.VMEM((LANE // 2, 2 * LANE), U32),
        pltpu.VMEM((M // 2, S), U32),
        pltpu.VMEM((S // 2, MP), U32),
        pltpu.VMEM((5, XH // 2, D), U32),
        pltpu.VMEM((S // 2 + 8, C), U32),
        [pltpu.VMEM((4 * min(TP, M // 2 - kt * TP) * 8, LANE), U32)
         for kt in range(KT)],
        pltpu.VMEM((H // 2, MP // 2, 2 * D), U32),
        pltpu.VMEM((H // 2, x_cols, 2 * D), U32),
        pltpu.VMEM((QIT, C * 8, LANE), U32),
        pltpu.VMEM((H, C // 2, 2 * D), U32),
        pltpu.VMEM((H, M // 2, D), U32),
        pltpu.VMEM((H, S // 2, D), U32),
        pltpu.VMEM((S // 2, D), U32),
        pltpu.VMEM((S // 2, D), U32),
        pltpu.VMEM((5, (nq - 1) * D // 2, LANE), U32),
        pltpu.VMEM((5, (nq - 1) * D // 2, LANE), U32),
        pltpu.VMEM((2, tq, tq), BF16),
        [pltpu.VMEM((7, tq // 2, n * D), BF16) for n in (2, 3)],
        pltpu.VMEM((2, M, S // 2), F32),
        pltpu.VMEM((S // D, M, D), F32),
        pltpu.VMEM((AT + 1, S, LANE), BF16),
        pltpu.VMEM((S, 2 * M - AT * LANE), BF16),
        pltpu.SemaphoreType.DMA((XC,)),
        pltpu.SemaphoreType.DMA((KT,)),
        pltpu.SemaphoreType.DMA((QIT,)),
        pltpu.SemaphoreType.DMA((QIT,)),
        pltpu.SemaphoreType.DMA((2,)),
        pltpu.SemaphoreType.DMA((3,)),
        pltpu.SemaphoreType.DMA((S // D + AT,)),
    ]
    return kernel, scratch


_DEFAULT = dict(
    tq=512, a_width=16, ao_at=1, ao_row=240, link_back=176, link_part=32, pace_row=32,
    pace_step=24, use_a=1, h0=0, last_row=216, o_str=(0, 1, 2, 3), o_link=48, o_half=6, q_jobs=(3, 4), xs_from=3, s_str=1, s_link=64, s_due=4, s_row=120, k_str=1, max_late=0, q_pin=2,
    seq="K0 Q0 K1 Q1 V0 F P0 K2@1116 Q2 O0 V1!4 P1 K3@2116 O1 Q3!0 V2@4012 P2 V3@3116 O2 P3!6 I O3")


def _build(**kw):
    cfg = dict(_DEFAULT)
    cfg.update(kw)
    kernel, scratch = _make_kernel(cfg)

    def run(A_q, A_k, A_v, A_shift_k, A_ssm_k, A_ssm_D, B_x, B_c_kv, B_w_q, B_w_uk,
            B_w_uv, B_w_o):
        tr = lambda a: jnp.swapaxes(a, 1, 2).reshape(M, S)
        args = (
            tr(A_q), tr(A_k), tr(A_v), A_shift_k.T, A_ssm_k, A_ssm_D, tr(B_x),
            B_c_kv.reshape(S, C),
            B_w_q.reshape(M // 2, 2 * H, D), B_w_uk.reshape(C // 2, 2 * H, D),
            B_w_uv.reshape(C // 2, 2 * H, D),
            jnp.swapaxes(B_w_o, 1, 2),
        )
        out = pl.pallas_call(
            kernel,
            in_specs=[pl.BlockSpec(memory_space=pl.ANY)] * len(args),
            out_specs=pl.BlockSpec(memory_space=pl.ANY),
            out_shape=jax.ShapeDtypeStruct((S, 2 * M), BF16),
            scratch_shapes=scratch,
            compiler_params=pltpu.CompilerParams(
                vmem_limit_bytes=126 * 1024 * 1024,
                disable_bounds_checks=True),
        )(*args)
        return out.reshape(1, S, 2 * M)

    return run


_run = _build()


@jax.jit
def pallas_concat_heads__ssm_conv_h3__compressed_kv_cla__prompt_kernel(
    A_q: jax.Array,
    A_k: jax.Array,
    A_v: jax.Array,
    A_shift_k: jax.Array,
    A_ssm_k: jax.Array,
    A_ssm_D: jax.Array,
    B_x: jax.Array,
    B_c_kv: jax.Array,
    B_w_q: jax.Array,
    B_w_uk: jax.Array,
    B_w_uv: jax.Array,
    B_w_o: jax.Array,
):
    return _run(A_q, A_k, A_v, A_shift_k, A_ssm_k, A_ssm_D, B_x, B_c_kv, B_w_q,
                B_w_uk, B_w_uv, B_w_o)
```

```python
import functools

import jax
import jax.numpy as jnp
from jax import lax
import jax.experimental.pallas as pl
import jax.experimental.pallas.tpu as pltpu

F32 = jnp.float32
BF16 = jnp.bfloat16
U32 = jnp.uint32

S = 2048
M = 448
MP = 512
C = 1024
H = 16
D = 256
KS = 4
LANE = 128
NB = S // LANE
AR = 32
A_STEPS = M // AR
LOG2E = 1.4426950408889634
QSCALE = D ** -0.5 * LOG2E
NEG = -1e30

NT = (((1,), (1,)), ((), ()))


def _dot(a, b):
    return jnp.dot(a, b, preferred_element_type=F32)


def _dot_nt(a, b):
    return lax.dot_general(a, b, NT, preferred_element_type=F32)


def _bf(x):
    return pltpu.bitcast(x, BF16)


def _u32(x):
    return pltpu.bitcast(x, U32)


def _h(r0, n):
    return pl.ds(r0 // 2, n // 2)


def _repack(ev, od):
    lo = (ev & jnp.uint32(0xFFFF)) | (od << 16)
    hi = (ev >> 16) | (od & jnp.uint32(0xFFFF0000))
    return lo, hi


def _split(w):
    return (pltpu.bitcast(w << 16, F32), pltpu.bitcast(w & jnp.uint32(0xFFFF0000), F32))


def _join(lo, hi):
    half = jnp.uint32(0x8000)
    lo = (pltpu.bitcast(lo, U32) + half) >> 16
    hi = (pltpu.bitcast(hi, U32) + half) & jnp.uint32(0xFFFF0000)
    return lo | hi


def _add(a, b):
    return _join(a[0] + b[0], a[1] + b[1])


def _sub(a, b):
    return _join(a[0] - b[0], a[1] - b[1])


def _opaque_zero(vals):
    acc = None
    for v in vals:
        b = v if v.dtype == U32 else pltpu.bitcast(v, U32)
        for r in range(0, b.shape[0], 8):
            for c in range(0, b.shape[1], LANE):
                t = b[r:r + 8, c:c + LANE]
                acc = t if acc is None else acc | t
    return jnp.minimum((acc >> 1).astype(jnp.int32), 0)


def _pin(x, zero, r=0, c=0):
    t = pltpu.bitcast(pltpu.bitcast(x[r:r + 8, c:c + LANE], jnp.int32) + zero, x.dtype)
    row = ([x[r:r + 8, :c]] if c > 0 else []) + [t] + (
        [x[r:r + 8, c + LANE:]] if c + LANE < x.shape[1] else [])
    row = jnp.concatenate(row, axis=1) if len(row) > 1 else row[0]
    col = ([x[:r, :]] if r > 0 else []) + [row] + ([x[r + 8:, :]] if r + 8 < x.shape[0] else [])
    return jnp.concatenate(col, axis=0) if len(col) > 1 else col[0]


def _rowcat(xs):
    return jnp.concatenate(xs, axis=0) if len(xs) > 1 else xs[0]


def _lanecat(xs):
    return jnp.concatenate(xs, axis=1) if len(xs) > 1 else xs[0]


def _make_kernel(cfg):
    tq = cfg["tq"]
    nq = S // tq
    nsub = tq // LANE
    KT = MP // LANE
    TP = LANE // 2
    XC = 4
    x_cols = S // XC
    QP = 2
    QIT = H // 2 // QP
    XH = (S - x_cols) // 2
    CP = 176
    AT = 3

    def kernel(aq_hbm, ak_hbm, av_hbm, sh_hbm, ssm_hbm, dd_hbm, x_hbm, c_hbm,
               wq_hbm, wk_hbm, wv_hbm, wo_hbm,
               out_hbm,
               a_v, sh_v, dd_v, par_v, f_v,
               xt_v, x_v, xs_v, c_v, wqs_v, wq_v, qacc, ws_v, wkv_v, wo_v,
               q_all, k_s, v_s, kb_s, vb_s, pd_s, pa_s, ra_t, rb_t, oa_v, out_v,
               sem_x, sem_wq, sem_w, sem_c, sem_s, sem_a, sem_out):
        x32, c32, wq32, wk32, wv32, wo32 = (
            r.bitcast(U32) for r in (x_hbm, c_hbm, wq_hbm, wk_hbm, wv_hbm, wo_hbm))
        a32 = [r.bitcast(U32) for r in (ak_hbm, av_hbm, ssm_hbm, aq_hbm)]

        sa_v = qacc

        def x_copy(i):
            cs = pl.ds(i * x_cols, x_cols)
            return pltpu.make_async_copy(x32.at[:, cs], xt_v.at[:, cs], sem_x.at[i])

        def wq_pairs(kt):
            return min(TP, M // 2 - kt * TP)

        def wq_copies(kt):
            n = wq_pairs(kt)
            dst = wqs_v[kt].reshape(4, n, 8, LANE)
            return [pltpu.make_async_copy(
                wq32.at[pl.ds(kt * TP, n), pl.ds(8 * (k // 2), 8), pl.ds((k % 2) * LANE, LANE)],
                dst.at[k], sem_wq.at[kt]) for k in range(4)]

        def wq_wait(kt):
            pltpu.make_async_copy(wqs_v[kt], wqs_v[kt], sem_wq.at[kt]).wait()

        def w_copies(g):
            dst = ws_v.reshape(8, C // 2, 8, LANE)
            src = (wk32, wv32)[g // 2]
            return [pltpu.make_async_copy(
                src.at[:, pl.ds(8 * par, 8), pl.ds((g % 2) * LANE, LANE)],
                dst.at[2 * g + par], sem_w.at[g]) for par in range(2)]

        def w_wait(g):
            pltpu.make_async_copy(ws_v.at[g], ws_v.at[g], sem_w.at[g]).wait()

        c_bounds = [0, CP, 2 * CP, S // 4]

        def c_copies(p):
            r0, n = c_bounds[p], c_bounds[p + 1] - c_bounds[p]
            return [pltpu.make_async_copy(c32.at[rs], c_v.at[rs], sem_c.at[p])
                    for rs in (pl.ds(r0, n), pl.ds(S // 4 + r0, n))]

        wo_copy = pltpu.make_async_copy(wo32, wo_v, sem_a.at[0])

        a_parts = [pl.ds(0, AR // 2), pl.ds(AR // 2, M // 2 - AR // 2)]

        def a_start(part):
            rs = a_parts[part]
            for k in range(4):
                pltpu.make_async_copy(
                    a32[k].at[rs], a_v.at[k, rs], sem_a.at[1 + part]).start()

        def a_wait(part):
            view = a_v.at[:, a_parts[part]]
            pltpu.make_async_copy(view, view, sem_a.at[1 + part]).wait()

        small = [pltpu.make_async_copy(sh_hbm, sh_v, sem_s.at[0]),
                 pltpu.make_async_copy(dd_hbm, dd_v, sem_s.at[1])]

        link = [None]
        pace = [None]

        def set_link(res, row=None, pacer=None):
            if row is None:
                row = res.shape[0] - cfg["link_back"]
            link[0] = _opaque_zero([res[row:row + 8, res.shape[1] - LANE:]])
            pace[0] = res if pacer is None else pacer

        def linked(x):
            return x if link[0] is None else _pin(x, link[0])

        def paced(w):
            res = pace[0]
            if res is None or link[0] is None or not cfg["pace_step"]:
                return w
            rows = []
            r0, step = cfg["pace_row"], cfg["pace_step"]
            if res.shape[0] < 400:
                r0, step = 0, 8
            if res.shape[0] < 200:
                return w
            zs = [_opaque_zero([res[r:r + 8, res.shape[1] - LANE:]])
                  for r in range(r0, r0 + 8 * step, step)]
            for r in range(0, w.shape[0], 8):
                z = zs[7 - (r // 8) % 8]
                t = pltpu.bitcast(w[r:r + 8, :], jnp.int32)
                rows.append(pltpu.bitcast(t + _lanecat([z] * (w.shape[1] // LANE)), U32))
            return _rowcat(rows)

        for cp in small:
            cp.start()
        x_copy(0).start()
        for cp in wq_copies(0):
            cp.start()

        def zero_body(k, carry):
            n = LANE // (S // D)
            bi = lax.broadcasted_iota(jnp.int32, (n, LANE), 0) + k * n
            mi = lax.broadcasted_iota(jnp.int32, (n, LANE), 1)
            ph = ((4 * mi + 1) * bi) & 511
            ang = ph.astype(F32) * (2.0 * 3.141592653589793 / 512.0)
            rs = pl.ds(pl.multiple_of(k * (n // 2), n // 2), n // 2)
            f_v[rs, 0:LANE] = _u32(jnp.cos(ang).astype(BF16))
            f_v[rs, LANE:] = _u32((-jnp.sin(ang)).astype(BF16))

            rb_t[k] = jnp.zeros((M, D), F32)
            cs = pl.ds(pl.multiple_of((k % 4) * D, D), D)
            ra_t[k // 4, 0:LANE, cs] = jnp.zeros((LANE, D), F32)
            ra_t[k // 4, AT * LANE:, cs] = jnp.zeros((M - AT * LANE, D), F32)
            return carry

        lax.fori_loop(0, S // D, zero_body, 0)
        c_v[S // 2:, :] = jnp.zeros((8, C), U32)

        for kt in range(1, KT):
            for cp in wq_copies(kt):
                cp.start()
        with jax.named_scope("small_wait"):
            for cp in small:
                cp.wait()
        sh = sh_v[...].astype(F32)
        for j in range(KS):
            par_v[j] = jnp.broadcast_to(sh[j:j + 1, :], (LANE, M)).T
        dd = dd_v[...].astype(F32).reshape(1, M)
        par_v[KS] = jnp.broadcast_to(dd, (LANE, M)).T

        def x_transpose(i):
            xt = xt_v[:, pl.ds(i * x_cols, x_cols)]
            xt = _rowcat([xt, jnp.zeros((MP // 2 - M // 2, x_cols), U32)])
            x_v[_h(i * x_cols, x_cols), :] = _u32(_bf(xt).astype(F32).T.astype(BF16))

        def q_early(kt, keep=False, jobs=()):
            first, last = kt == 0, kt == KT - 1
            n = wq_pairs(kt)
            cols = pl.ds(kt * LANE, LANE)
            if not keep:
                link[0] = None
            for j in range(H // 2):
                ws = []
                for half in range(2):
                    ev, od = (wqs_v[kt][pl.ds((2 * par + half) * n * 8 + j, n, stride=8), :]
                              for par in range(2))
                    ws.append(_repack(ev, od))
                w = _lanecat([ws[0][0], ws[1][0], ws[0][1], ws[1][1]])
                if cfg["w_scale"]:
                    w = _join(*(x * QSCALE for x in _split(w)))
                if n < TP:
                    w = _rowcat([w, jnp.zeros((TP - n, 2 * D), U32)])
                wq_v[j, pl.ds(kt * TP, TP), :] = w
                lhs = linked(x_v[_h(0, x_cols), cols])
                j0 = cfg["xs_from"]
                if jobs and j >= j0:
                    nj = H // 2 - j0
                    mine = jobs[(j - j0) * len(jobs) // nj:(j - j0 + 1) * len(jobs) // nj]
                    for k, job in enumerate(mine):
                        lhs = _pin(lhs, _opaque_zero(job()), 8 * (1 + k * 30 // len(mine)))
                d = _dot(_bf(lhs), _bf(w))
                set_link(d)
                if not first:
                    d = d + pltpu.bitcast(qacc[j], F32)
                if last:
                    d = (d if cfg["w_scale"] else d * QSCALE).astype(BF16)
                    for t in range(2):
                        q_all[2 * j + t, _h(0, x_cols), :] = _u32(d[:, t * D:(t + 1) * D])
                else:
                    qacc[j] = pltpu.bitcast(d, U32)

        with jax.named_scope("x_wait"):
            x_copy(0).wait()
        x_transpose(0)
        for i in range(1, XC):
            x_copy(i).start()
        for g in range(QIT):
            for cp in w_copies(g) + (c_copies(g) if g < QIT - 1 else []):
                cp.start()
        wo_copy.start()
        a_start(0)
        a_start(1)
        with jax.named_scope("wq_wait"):
            wq_wait(0)
        q_early(0)
        with jax.named_scope("wq_wait"):
            wq_wait(1)
        q_early(1)
        with jax.named_scope("wq_wait"):
            wq_wait(2)
            wq_wait(3)
            for i in range(1, XC):
                x_copy(i).wait()
        for i in range(1, XC):
            x_transpose(i)

        def x_sums(u):
            a11, a12, a21, a22 = (
                _split(x_v[pl.ds((x_cols + rb * XH) // 2 + 8 * u, 8), cb * D:(cb + 1) * D])
                for rb in range(2) for cb in range(2))
            outs = [_add(a11, a22), _add(a21, a22), _add(a11, a12), _sub(a21, a11),
                    _sub(a12, a22)]
            for k, o in enumerate(outs):
                xs_v[k, 8 * u:8 * u + 8, :] = o
            return outs

        q_early(2, jobs=[functools.partial(x_sums, u) for u in range(XH // 16)])
        q_early(3, keep=True)

        def unpack(it, sub, j):
            g = it
            ev, od = (ws_v[g, pl.ds((par * (C // 2) + sub * TP) * 8 + j, TP, stride=8), :]
                      for par in range(2))
            lo, hi = _repack(ev, od)
            rows = pl.ds(sub * TP, TP)
            cols = pl.ds(pl.multiple_of(g * LANE, LANE), LANE)
            wkv_v[2 * j, rows, cols] = lo
            wkv_v[2 * j + 1, rows, cols] = hi
            return [lo, hi]

        def a_sums(it, u):
            r0 = jnp.clip((it - 1) * CP, 0, S // 4 - CP) + 8 * u
            src = [jnp.where(it == 0, S // 2, r0 + rb * (S // 4)) for rb in range(2)]
            r0 = pl.multiple_of(r0, 8)
            kw = C // 2
            a11, a12, a21, a22 = (
                _split(c_v[pl.ds(pl.multiple_of(src[rb], 8), 8), pl.ds(cb * kw, kw)])
                for rb in range(2) for cb in range(2))
            outs = [_add(a11, a22), _add(a21, a22), _add(a11, a12), _sub(a21, a11),
                    _sub(a12, a22)]
            for k, o in enumerate(outs):
                sa_v[k, pl.ds(r0, 8), :] = o
            return outs

        units = [functools.partial(unpack, sub=s_, j=j_)
                 for s_ in range(C // 2 // TP) for j_ in range(H // 2)]
        for u_ in range(CP // 8):
            units.insert(4 * u_ + 1, functools.partial(a_sums, u=u_))

        def q_pair(pair, todo):
            raw = lambda r, c: _lanecat([
                wq_v[pair, r * LANE:(r + 1) * LANE, pl.ds(t * D + c * LANE, LANE)]
                for t in range(2)])
            b = lambda r, c: _split(raw(r, c))
            sb = {1: _add(b(0, 0), b(1, 1)), 2: raw(0, 0), 3: _sub(b(0, 1), b(1, 1)),
                  4: _sub(b(1, 0), b(0, 0)), 5: raw(1, 1), 6: _add(b(0, 0), b(0, 1)),
                  7: _add(b(1, 0), b(1, 1))}
            n = XH // 2
            for rho in range(2):
                def sa(m):
                    if m == 3:
                        return x_v[_h(x_cols + rho * n, n), 0:D]
                    if m == 4:
                        return x_v[_h(x_cols + XH + rho * n, n), D:]
                    return xs_v[{1: 0, 2: 1, 5: 2, 6: 3, 7: 4}[m], _h(rho * n, n), :]

                def put(half, c0, c1):
                    rows = _h(x_cols + half * XH + rho * n, n)
                    out = []
                    for t in range(2):
                        q = _lanecat([c[:, t * LANE:(t + 1) * LANE] for c in (c0, c1)])
                        out.append(_u32((q if cfg["w_scale"] else q * QSCALE).astype(BF16)))
                        q_all[2 * pair + t, rows, :] = out[-1]
                    nd = cfg["q_nd"]
                    step = n // 2 // nd
                    q_due.append([_opaque_zero([o[k * step:(k + 1) * step] for o in out])
                                  for k in range(nd)])

                p = {}
                for pos, m in enumerate((5, 1, 4, 7, 3, 2, 6)):
                    lhs = linked(sa(m))
                    nj = min(len(todo), cfg["q_jobs"][7 * rho + pos])
                    jobs = [todo.pop()(it=pair // QP) for _ in range(nj)]
                    for k, job in enumerate(jobs):
                        lhs = _pin(lhs, _opaque_zero(job), 8 * (1 + k * (n // 16 - 1) // nj))
                    if q_due and m in cfg["q_due_at"]:
                        zs = q_due.pop()
                        for k, z in enumerate(zs):
                            lhs = _pin(lhs, z, 8 * ((k + 1) * (n // 16) // len(zs) - 1), LANE)
                    p[m] = _dot(_bf(lhs), _bf(sb[m]))
                    set_link(p[m])
                    if m == 3:
                        put(0, (p[1] + p[4]) + (p[7] - p[5]), p[3] + p[5])
                put(1, p[2] + p[4], (p[1] + p[3]) + (p[6] - p[2]))

        q_due = []

        def q_body(it, carry):
            with jax.named_scope("w_wait"):
                w_wait(it)
                for p in range(QIT - 1):
                    @pl.when(it == p + 1)
                    def _():
                        for cp in c_copies(p):
                            cp.wait()
            link[0] = None
            todo = units[::-1]
            del q_due[:]
            for p in range(QP):
                q_pair(QP * it + p, todo)
            assert not todo
            return carry

        with jax.named_scope("q_loop"):
            lax.fori_loop(0, QIT, q_body, 0)
        wo_copy.wait()
        a_wait(0)

        tri = (lax.broadcasted_iota(jnp.int32, (LANE, LANE), 1)
               <= lax.broadcasted_iota(jnp.int32, (LANE, LANE), 0))

        NOUT = S // D

        def out_copy(i):
            if i >= NOUT:
                t = i - NOUT
                return pltpu.make_async_copy(
                    oa_v.at[t], out_hbm.at[:, pl.ds(t * LANE, LANE)], sem_out.at[i])
            rs = pl.ds(i * D, D)
            return pltpu.make_async_copy(
                out_v.at[rs], out_hbm.at[rs, pl.ds(AT * LANE, 2 * M - AT * LANE)], sem_out.at[i])

        n_body = NOUT - (tq // D if nq - 1 in cfg["o_str"] else 1)

        def b_out(k, tot):
            c0 = (k * D) % (S // 2)
            full = _rowcat([ra_t[k * D // (S // 2), AT * LANE:, c0:c0 + D], tot]).T
            out_v[k * D:(k + 1) * D, :] = full.astype(BF16)
            return full

        def head_step(h, carry):
            with jax.named_scope("step"):
                return head_step_(h, carry)

        def head_step_(h, carry):
            with_a = cfg["use_a"]

            @pl.when(h == A_STEPS)
            def _():
                for t in range(AT):
                    out_copy(NOUT + t).start()

            @pl.when(h == cfg["h0"] + 1)
            def _():
                a_wait(1)

            link[0] = None
            n2 = AR // 2
            a_rows2 = pl.ds(pl.multiple_of(jnp.minimum(h, A_STEPS - 1) * n2, n2), n2)
            a_rows = pl.ds(pl.multiple_of(jnp.minimum(h, A_STEPS - 1) * AR, AR), AR)

            kw = C // 2
            pending = []
            chains = {i: [] for i in range(nq + 1)}
            deadline = [None]

            def flush_pending(x, row):
                done = list(pending)
                del pending[:]
                if not done:
                    return x
                x = _pin(x, _opaque_zero([f for _, f in done]), row)

                @pl.when(h == H - 1)
                def _():
                    for k, _f in done:
                        out_copy(k).start()
                return x

            def a_fwd():
                kk = _bf(a_v[0, a_rows2, :]).astype(F32)
                lane = lax.broadcasted_iota(jnp.int32, (AR, LANE), 1)
                coef = [par_v[j, a_rows, :] for j in range(KS)]
                rolled = [kk] + [pltpu.roll(kk, j, 1) for j in range(1, KS)]
                vv = _bf(a_v[1, a_rows2, :]).astype(F32)
                kv_blocks = []
                for a in range(NB):
                    cs = slice(a * LANE, (a + 1) * LANE)
                    acc = rolled[0][:, cs] * coef[0]
                    for j in range(1, KS):
                        t = rolled[j][:, cs]
                        if a == 0:
                            t = jnp.where(lane >= j, t, 0.0)
                        acc = acc + t * coef[j]
                    kv_blocks.append(acc * vv[:, cs])
                hk = a_v[2, a_rows2, :]
                hk = _rowcat([hk[:, a * LANE:(a + 1) * LANE] for a in range(NB)])
                fm = _bf(f_v[...])
                hs = _dot(_bf(linked(hk)), fm)
                kv = linked(_rowcat(kv_blocks)).astype(BF16)
                xs = _dot(kv, fm)
                set_link(xs)
                return kv, xs, hs

            def a_conv(xs, hs):
                def tile(v, a, g, part):
                    r = a * AR + 8 * g
                    return v[r:r + 8, part * LANE:(part + 1) * LANE]

                z = {}
                gate = None
                width = cfg["a_width"]
                for g in range(AR // 8):
                    hr = [tile(hs, 0, g, 0)] + [
                        tile(hs, j, g, 0) - tile(hs, j - 1, g, 1) for j in range(1, NB)]
                    hi = [tile(hs, 0, g, 1)] + [
                        tile(hs, j, g, 1) + tile(hs, j - 1, g, 0) for j in range(1, NB)]
                    for c0 in range(0, NB, width):
                        for a in range(c0 + width):
                            xr, xi = tile(xs, a, g, 0), tile(xs, a, g, 1)
                            if gate is not None:
                                xr, xi = _pin(xr, gate), _pin(xi, gate)
                            for c in range(max(c0, a), c0 + width):
                                j = c - a
                                tr = xr * hr[j] - xi * hi[j]
                                ti = xr * hi[j] + xi * hr[j]
                                z[c, g] = (tr, ti) if a == 0 else (z[c, g][0] + tr, z[c, g][1] + ti)
                            gate = _opaque_zero(list(z[c0 + width - 1, g]))
                            chains[nq].append(gate)
                return z

            def a_inv(kv, z, flush=False):
                fm = _bf(f_v[...])
                ng = AR // 8
                ys = []
                for u in range(2):
                    rows = [_lanecat(z[c, g]) for g in range(u * ng // 2, (u + 1) * ng // 2)
                            for c in range(NB)]
                    lhs = linked(_rowcat(rows))
                    if flush:
                        lhs = flush_pending(lhs, 8)
                    ys.append(_dot_nt(lhs.astype(BF16), fm))
                y = _rowcat(ys)
                dd = par_v[KS, a_rows, :]
                for c in range(NB):
                    cs = slice(c * LANE, (c + 1) * LANE)
                    yc = _rowcat([y[(g * NB + c) * 8:(g * NB + c + 1) * 8, :] for g in range(ng)])
                    qq = _bf(a_v[3, a_rows2, cs]).astype(F32)
                    kvf = kv[c * AR:(c + 1) * AR, :].astype(F32)
                    c2 = (c % (NB // 2)) * LANE
                    ra_t[c // (NB // 2), a_rows, c2:c2 + LANE] = qq * (yc * (1.0 / LANE) + kvf * dd)

            def a_out():
                slab = jnp.clip(h // 4 - 1, 0, AT - 1)
                half = h % 2
                x = ra_t[half, pl.ds(pl.multiple_of(slab * LANE, LANE), LANE), :]
                xt = x.T
                dst = jnp.where(h >= A_STEPS, AT, slab)
                oa_v[dst, pl.ds(pl.multiple_of(half * (S // 2), S // 2), S // 2), :] = xt.astype(BF16)
                return xt

            def w_blk(r, c):
                return wkv_v[h, _h(r * kw, kw), pl.ds(c * LANE, LANE)]

            def one_pass(lhs, w, flush):
                lhs = linked(lhs)
                if flush:
                    lhs = flush_pending(lhs, cfg["ao_row"])
                if deadline[0] is not None:
                    if deadline[0][0] == 0:
                        lhs = _pin(lhs, deadline[0][1], cfg["ao_row"] - 8)
                        deadline[0] = None
                    else:
                        deadline[0] = (deadline[0][0] - 1, deadline[0][1])
                d = _dot(_bf(lhs), _bf(paced(w)))
                set_link(d)
                return d

            def b_op(which, m):
                raw = lambda r, c: w_blk(r, 2 * which + c)
                blk = lambda r, c: _split(raw(r, c))
                return {1: lambda: _add(blk(0, 0), blk(1, 1)),
                        2: lambda: raw(0, 0),
                        3: lambda: _sub(blk(0, 1), blk(1, 1)),
                        4: lambda: _sub(blk(1, 0), blk(0, 0)),
                        5: lambda: raw(1, 1),
                        6: lambda: _add(blk(0, 0), blk(0, 1)),
                        7: lambda: _add(blk(1, 0), blk(1, 1))}[m]()

            def a_op(m, rho):
                rs = _h(rho * tq, tq)
                if m == 3:
                    return c_v[rs, 0:kw]
                if m == 4:
                    return c_v[_h(S // 2 + rho * tq, tq), kw:]
                return sa_v[{1: 0, 2: 1, 5: 2, 6: 3, 7: 4}[m], rs, :]

            b_cache, prod = {}, {}

            def kv_proj(which, blk, flush):
                rho = blk % 2
                for k, m in enumerate((5, 1, 4, 7, 3) if blk < 2 else (2, 6)):
                    if (which, m) not in b_cache:
                        b_cache[which, m] = b_op(which, m)
                    prod[which, m, rho] = one_pass(a_op(m, rho), b_cache[which, m], k == flush)
                p = lambda m: prod[which, m, rho]
                if blk < 2:
                    return [(p(1) + p(4)) + (p(7) - p(5)), p(3) + p(5)]
                return [p(2) + p(4), (p(1) + p(3)) + (p(6) - p(2))]

            def k_proj(blk, flush=-1):
                if cfg["k_str"]:
                    k = kv_proj(0, blk, flush)
                else:
                    ds = [one_pass(c_v[_h(blk * tq, tq), pl.ds((k % 2) * kw, kw)],
                                   w_blk(k % 2, k // 2), k == flush) for k in range(4)]
                    k = [ds[0] + ds[1], ds[2] + ds[3]]
                k_s[_h(blk * tq, tq), :] = _u32(_lanecat(k).astype(BF16))
                if cfg["s_str"] and blk < nq - 1:
                    b = lambda r, c: k[r][c * D:(c + 1) * D, :]
                    sums = [b(0, 0) + b(1, 1), b(0, 1) - b(1, 1), b(1, 0) - b(0, 0),
                            b(0, 0) + b(0, 1), b(1, 0) + b(1, 1)]
                    for n, x in enumerate(sums):
                        kb_s[n, _h(blk * D, D), :] = _u32(x.astype(BF16))

            def v_proj(blk, flush=-1):
                v = kv_proj(1, blk, flush)
                v_s[_h(blk * tq, tq), :] = _u32(_lanecat(v).astype(BF16))
                if blk < nq - 1:
                    b = lambda r, c: v[c][r * D:(r + 1) * D, :]
                    sums = [b(0, 0) + b(1, 1), b(0, 1) - b(1, 1), b(1, 0) - b(0, 0),
                            b(0, 0) + b(0, 1), b(1, 0) + b(1, 1)]
                    for k, x in enumerate(sums):
                        vb_s[k, _h(blk * D, D), :] = _u32(x.astype(BF16))

            def qk(i, dep=None, flush=False):
                r0 = i * tq
                off = None
                if cfg["s_str"] and i > 0:
                    raw = lambda r, c: q_all[h, _h(r0 + r * D, D), c * LANE:(c + 1) * LANE]
                    a = lambda r, c: _split(raw(r, c))
                    sa = {1: _add(a(0, 0), a(1, 1)), 2: _add(a(1, 0), a(1, 1)), 3: raw(0, 0),
                          4: raw(1, 1), 5: _add(a(0, 0), a(0, 1)), 6: _sub(a(1, 0), a(0, 0)),
                          7: _sub(a(0, 1), a(1, 1))}

                    def sb(m, j, t):
                        if m in (2, 5):
                            c = 0 if m == 2 else 1
                            rows = _h(j * tq + c * D + t * LANE, LANE)
                            return k_s[rows, c * LANE:(c + 1) * LANE]
                        n = {1: 0, 3: 1, 4: 2, 6: 3, 7: 4}[m]
                        return kb_s[n, _h(j * D + t * LANE, LANE), :]

                    top, bot, due, pmax = {}, {}, [], []
                    n_dot = 0
                    for j in range(i):
                        for t in range(2):
                            p = {}
                            for n, m in enumerate((5, 1, 4, 7, 2, 3, 6)):
                                lhs = linked(sa[m])
                                if due and n == cfg["s_due"]:
                                    lhs = _pin(lhs, due.pop(), cfg["s_row"])
                                p[m] = _dot_nt(_bf(lhs), _bf(sb(m, j, t)))
                                n_dot += 1
                                if n_dot % 4 == 0:
                                    set_link(p[m], cfg["s_link"])
                            top[4 * j + t] = (p[1] + p[4]) + (p[7] - p[5])
                            top[4 * j + 2 + t] = p[3] + p[5]
                            bot[4 * j + t] = p[2] + p[4]
                            bot[4 * j + 2 + t] = (p[1] + p[3]) + (p[6] - p[2])
                            if cfg["s_max"]:
                                mx = _rowcat([jnp.maximum(x[4 * j + t], x[4 * j + 2 + t])
                                              for x in (top, bot)])
                                if cfg["s_max"] == 2 and pmax:
                                    mx = jnp.maximum(mx, pmax.pop())
                                pmax.append(mx)
                                due.append(_opaque_zero([mx]))
                            else:
                                due.append(_opaque_zero(
                                    [x[4 * j + c + t] for x in (top, bot) for c in (0, 2)]))
                    off = _rowcat([_lanecat([x[c] for c in range(4 * i)]) for x in (top, bot)])
                q = linked(q_all[h, _h(r0, tq), :])
                if off is not None:
                    q = _pin(q, due.pop(), cfg["ao_row"] - 8)
                if dep is not None:
                    q = _pin(q, _opaque_zero([dep]), cfg["ao_row"])
                k0 = 0 if off is None else r0
                main = _dot_nt(_bf(q), _bf(k_s[_h(k0, r0 + LANE - k0), :]))
                parts = [main if off is None else _lanecat([off, main])]
                early = None
                if off is not None and cfg["s_max"]:
                    early = (4 * i, _lanecat(pmax))
                if i > 0 and off is None:
                    link[0] = _opaque_zero([parts[0][0:8, r0 - LANE:r0]])
                for j in range(1, nsub):
                    q = linked(q_all[h, _h(r0 + LANE * j, tq - LANE * j), :])
                    if j == cfg["q_pin"]:
                        if flush:
                            q = flush_pending(q, 8)
                    parts.append(_dot_nt(_bf(q), _bf(k_s[_h(r0 + LANE * j, LANE), :])))
                set_link(parts[2], cfg["link_part"], main)
                return parts, early

            def exps(i, parts, early):
                sas, mbs = [], []
                for a in range(nsub):
                    blocks = [parts[j][LANE * (a - j):LANE * (a - j + 1), :] for j in range(a + 1)]
                    last = blocks[-1]
                    w = last.shape[1]
                    dg = jnp.where(tri, last[:, w - LANE:], NEG)
                    blocks[-1] = dg if w == LANE else _lanecat([last[:, :w - LANE], dg])
                    sas.append(_lanecat(blocks))
                    mx = sas[a]
                    if early is not None:
                        mx = _lanecat([early[1][LANE * a:LANE * (a + 1)], mx[:, early[0] * LANE:]])
                    mbs.append(jnp.broadcast_to(jnp.max(mx, axis=1, keepdims=True), (LANE, LANE)))
                chain = _opaque_zero([b[b.shape[0] - 8:, b.shape[1] - LANE:] for b in parts])
                pg, psums = {}, {}
                for r in range(0, tq // 2, 8):
                    for row in (r, r + tq // 2):
                        a, g = divmod(row, LANE)
                        mg = _pin(mbs[a][g:g + 8, :], chain)
                        pg[row] = [jnp.exp2(sas[a][g:g + 8, t:t + LANE] - mg)
                                   for t in range(0, sas[a].shape[1], LANE)]
                        psums[row] = functools.reduce(jnp.add, pg[row])
                        chain = _opaque_zero([psums[row]])
                        chains[i].append(chain)
                return pg, psums

            def softmax(i, pg, psums):
                r0 = i * tq
                pd, pa = pd_s.at[i % 2], pa_s[i % 2]
                first = lambda x, c=0: _pin(x, link[0], 0, c).astype(BF16)
                nt0 = r0 // LANE
                ls = []
                for a in range(nsub):
                    rows = range(LANE * a, LANE * (a + 1), 8)
                    ls.append(jnp.sum(_rowcat([psums[r] for r in rows]), axis=1, keepdims=True))
                    pd[LANE * a:LANE * (a + 1), 0:LANE * (a + 1)] = first(
                        _rowcat([_lanecat(pg[r][nt0:]) for r in rows]), LANE * a)
                if i > 0:
                    quad = lambda rh, ch: _rowcat([
                        _lanecat([pg[rh * (tq // 2) + r][4 * j + 2 * ch + t]
                                  for j in range(i) for t in range(2)])
                        for r in range(0, tq // 2, 8)])
                    a11, a12, a21, a22 = quad(0, 0), quad(0, 1), quad(1, 0), quad(1, 1)
                    ops = [a11 + a22, a21 + a22, a11, a22, a11 + a12, a21 - a11, a12 - a22]
                    for m, x in enumerate(ops):
                        if i == 3:
                            x = _pin(x, link[0], 0, 2 * D)
                        pa[m, :, 0:i * D] = first(x)
                return ls

            def pv(i, ls, flush=-1):
                r0 = i * tq
                pd, pa = pd_s.at[i % 2], pa_s[i % 2]
                off = None
                if i > 0:
                    def b_rows(m, j0, j1):
                        if m in (2, 5):
                            q = 0 if m == 2 else 1
                            return _rowcat([
                                v_s[_h(j * tq + q * D, D), q * LANE:(q + 1) * LANE]
                                for j in range(j0, j1)])
                        k = {1: 0, 3: 1, 4: 2, 6: 3, 7: 4}[m]
                        return vb_s[k, _h(j0 * D, (j1 - j0) * D), :]

                    p, n_dot = {}, 0
                    for j0, j1 in {1: [(0, 1)], 2: [(0, 2)], 3: [(0, 2), (2, 3)]}[i]:
                        for m in range(1, 8):
                            cols = slice(j0 * D, j1 * D)
                            rhs = b_rows(m, j0, j1)
                            if n_dot == flush:
                                rhs = flush_pending(rhs, 0)
                            rhs = _bf(rhs)
                            n_dot += 1
                            if j1 - j0 == 1 and m == 7:
                                d = _rowcat([_dot(pa[m - 1, r:r + LANE, cols], rhs)
                                             for r in (0, LANE)])
                            else:
                                d = _dot(pa[m - 1, :, cols], rhs)
                            p[m] = d if m not in p else p[m] + d
                    off = _rowcat([
                        _lanecat([(p[1] + p[4]) + (p[7] - p[5]), p[3] + p[5]]),
                        _lanecat([p[2] + p[4], (p[1] + p[3]) + (p[6] - p[2])])])
                ctx = []
                for j in range(nsub):
                    c0 = LANE * j
                    ctx.append(_dot(pd[c0:, c0:c0 + LANE], _bf(v_s[_h(r0 + c0, LANE), :])))
                set_link(ctx[2], cfg["link_part"], ctx[0])
                cs = []
                for a in range(nsub):
                    sl = lambda j: slice(LANE * (a - j), LANE * (a - j + 1))
                    r = pl.reciprocal(ls[a], approx=True)
                    r = r * (2.0 - ls[a] * r)
                    terms = [ctx[j][sl(j)] for j in range(a + 1)]
                    if off is not None:
                        terms.append(off[sl(0)])
                    cs.append(functools.reduce(jnp.add, terms) * r)
                return _rowcat(cs)

            def accumulate(k, res):
                tot = rb_t[k] + res
                rb_t[k] = tot
                if k < n_body:
                    pending.append((k, b_out(k, tot)))

            def oproj_plain(i, ctx):
                ctx = ctx.astype(BF16)
                for u in range(tq // D):
                    lhs = linked(wo_v[h])
                    if i == nq - 1:
                        lhs = flush_pending(lhs, cfg["last_row"])
                    res = _dot_nt(_bf(lhs), ctx[u * D:(u + 1) * D, :])
                    set_link(res)
                    accumulate(i * (tq // D) + u, res)

            wo_cache = {}

            def oproj(i, ctx):
                if i not in cfg["o_str"]:
                    return oproj_plain(i, ctx)
                mh = M // 4
                raw = lambda r, c: wo_v[h, r * mh:(r + 1) * mh, c * LANE:(c + 1) * LANE]
                a = lambda r, c: _split(raw(r, c))
                a_ops = {1: lambda: _add(a(0, 0), a(1, 1)), 2: lambda: _add(a(1, 0), a(1, 1)),
                         3: lambda: raw(0, 0), 4: lambda: raw(1, 1),
                         5: lambda: _add(a(0, 0), a(0, 1)), 6: lambda: _sub(a(1, 0), a(0, 0)),
                         7: lambda: _sub(a(0, 1), a(1, 1))}
                b = lambda r, c: ctx[c * D:(c + 1) * D, r * LANE:(r + 1) * LANE]
                b_ops = {1: lambda: b(0, 0) + b(1, 1), 2: lambda: b(0, 0),
                         3: lambda: b(0, 1) - b(1, 1), 4: lambda: b(1, 0) - b(0, 0),
                         5: lambda: b(1, 1), 6: lambda: b(0, 0) + b(0, 1),
                         7: lambda: b(1, 0) + b(1, 1)}
                p = {}
                for n, m in enumerate((5, 2, 4, 1, 7, 3, 6)):
                    if m not in wo_cache:
                        wo_cache[m] = a_ops[m]()
                    rhs = b_ops[m]().astype(BF16)
                    if n == cfg["o_half"]:
                        halves = [_dot_nt(_bf(linked(wo_cache[m][r:r + mh // 2])), rhs)
                                  for r in (0, mh // 2)]
                        p[m] = _rowcat(halves)
                        set_link(halves[1], 0)
                    else:
                        p[m] = _dot_nt(_bf(linked(wo_cache[m])), rhs)
                        if (n - (n > cfg["o_half"])) % 2 == 1:
                            set_link(p[m], cfg["o_link"])
                accumulate(2 * i, _rowcat([(p[1] + p[4]) + (p[7] - p[5]), p[2] + p[4]]))
                accumulate(2 * i + 1, _rowcat([p[3] + p[5], (p[1] + p[3]) + (p[6] - p[2])]))

            st = {}
            for op in cfg["seq"].split():
                op, _, dl = op.partition("@")
                if dl:
                    ch = chains[int(dl[0])]
                    deadline[0] = (int(dl[1]), ch[int(dl[2:]) * len(ch) // 16 - 1])
                op, _, fl = op.partition("!")
                fl = int(fl) if fl else -1
                kind, i = op[0], int(op[1:] or 0)
                if kind == "K":
                    k_proj(i, fl)
                elif kind == "V":
                    v_proj(i, fl)
                elif kind == "Q":
                    st["e", i] = exps(
                        i, *qk(i, a_out() if i == cfg["ao_at"] else None, fl >= 0))
                elif kind == "P":
                    st["ctx", i] = pv(i, softmax(i, *st["e", i]), fl)
                elif kind == "O":
                    oproj(i, st["ctx", i])
                elif kind == "F" and with_a:
                    st["kv"], xs, hs = a_fwd()
                    st["z"] = a_conv(xs, hs)
                elif kind == "I" and with_a:
                    a_inv(st["kv"], st["z"], fl >= 0)
            assert not pending and deadline[0] is None
            return carry

        with jax.named_scope("loop_a"):
            lax.fori_loop(cfg["h0"], H, head_step, 0)
        with jax.named_scope("tail"):
            for i in range(n_body, NOUT):
                b_out(i, rb_t[i])
                out_copy(i).start()
            for i in range(NOUT + AT):
                out_copy(i).wait()

    scratch = [
        pltpu.VMEM((4, M // 2, S), U32),
        pltpu.VMEM((KS, M), BF16),
        pltpu.VMEM((M,), BF16),
        pltpu.VMEM((KS + 1, M, LANE), F32),
        pltpu.VMEM((LANE // 2, 2 * LANE), U32),
        pltpu.VMEM((M // 2, S), U32),
        pltpu.VMEM((S // 2, MP), U32),
        pltpu.VMEM((5, XH // 2, D), U32),
        pltpu.VMEM((S // 2 + 8, C), U32),
        [pltpu.VMEM((4 * min(TP, M // 2 - kt * TP) * 8, LANE), U32)
         for kt in range(KT)],
        pltpu.VMEM((H // 2, MP // 2, 2 * D), U32),
        pltpu.VMEM((H // 2, x_cols, 2 * D), U32),
        pltpu.VMEM((QIT, C * 8, LANE), U32),
        pltpu.VMEM((H, C // 2, 2 * D), U32),
        pltpu.VMEM((H, M // 2, D), U32),
        pltpu.VMEM((H, S // 2, D), U32),
        pltpu.VMEM((S // 2, D), U32),
        pltpu.VMEM((S // 2, D), U32),
        pltpu.VMEM((5, (nq - 1) * D // 2, LANE), U32),
        pltpu.VMEM((5, (nq - 1) * D // 2, LANE), U32),
        pltpu.VMEM((2, tq, tq), BF16),
        [pltpu.VMEM((7, tq // 2, n * D), BF16) for n in (2, 3)],
        pltpu.VMEM((2, M, S // 2), F32),
        pltpu.VMEM((S // D, M, D), F32),
        pltpu.VMEM((AT + 1, S, LANE), BF16),
        pltpu.VMEM((S, 2 * M - AT * LANE), BF16),
        pltpu.SemaphoreType.DMA((XC,)),
        pltpu.SemaphoreType.DMA((KT,)),
        pltpu.SemaphoreType.DMA((QIT,)),
        pltpu.SemaphoreType.DMA((QIT,)),
        pltpu.SemaphoreType.DMA((2,)),
        pltpu.SemaphoreType.DMA((3,)),
        pltpu.SemaphoreType.DMA((S // D + AT,)),
    ]
    return kernel, scratch


_DEFAULT = dict(
    tq=512, a_width=16, ao_at=1, ao_row=240, link_back=176, link_part=32, pace_row=32,
    pace_step=24, use_a=1, h0=0, last_row=216, o_str=(0, 1, 2, 3), o_link=48, o_half=6, q_jobs=(2, 4, 4, 4, 1, 3, 1, 3, 5, 6, 6, 1, 2, 1), w_scale=0, xs_from=3, q_nd=1, q_due_at=(9, 9), s_str=1, s_link=64, s_due=4, s_row=120, k_str=1, s_max=0, q_pin=2,
    seq="K0 Q0 K1 Q1 V0 F P0 K2@1116 Q2 O0 V1!4 P1 K3@2116 O1 Q3!0 V2@4012 P2 V3@3116 O2 P3!6 I O3")


def _build(**kw):
    cfg = dict(_DEFAULT)
    cfg.update(kw)
    kernel, scratch = _make_kernel(cfg)

    def run(A_q, A_k, A_v, A_shift_k, A_ssm_k, A_ssm_D, B_x, B_c_kv, B_w_q, B_w_uk,
            B_w_uv, B_w_o):
        tr = lambda a: jnp.swapaxes(a, 1, 2).reshape(M, S)
        args = (
            tr(A_q), tr(A_k), tr(A_v), A_shift_k.T, A_ssm_k, A_ssm_D, tr(B_x),
            B_c_kv.reshape(S, C),
            B_w_q.reshape(M // 2, 2 * H, D), B_w_uk.reshape(C // 2, 2 * H, D),
            B_w_uv.reshape(C // 2, 2 * H, D),
            jnp.swapaxes(B_w_o, 1, 2),
        )
        out = pl.pallas_call(
            kernel,
            in_specs=[pl.BlockSpec(memory_space=pl.ANY)] * len(args),
            out_specs=pl.BlockSpec(memory_space=pl.ANY),
            out_shape=jax.ShapeDtypeStruct((S, 2 * M), BF16),
            scratch_shapes=scratch,
            compiler_params=pltpu.CompilerParams(
                vmem_limit_bytes=126 * 1024 * 1024,
                disable_bounds_checks=True),
        )(*args)
        return out.reshape(1, S, 2 * M)

    return run


_run = _build()


@jax.jit
def pallas_concat_heads__ssm_conv_h3__compressed_kv_cla__prompt_kernel(
    A_q: jax.Array,
    A_k: jax.Array,
    A_v: jax.Array,
    A_shift_k: jax.Array,
    A_ssm_k: jax.Array,
    A_ssm_D: jax.Array,
    B_x: jax.Array,
    B_c_kv: jax.Array,
    B_w_q: jax.Array,
    B_w_uk: jax.Array,
    B_w_uv: jax.Array,
    B_w_o: jax.Array,
):
    return _run(A_q, A_k, A_v, A_shift_k, A_ssm_k, A_ssm_D, B_x, B_c_kv, B_w_q,
                B_w_uk, B_w_uv, B_w_o)
```

```python
import functools

import jax
import jax.numpy as jnp
from jax import lax
import jax.experimental.pallas as pl
import jax.experimental.pallas.tpu as pltpu

F32 = jnp.float32
BF16 = jnp.bfloat16
U32 = jnp.uint32

S = 2048
M = 448
MP = 512
C = 1024
H = 16
D = 256
KS = 4
LANE = 128
NB = S // LANE
AR = 32
A_STEPS = M // AR
LOG2E = 1.4426950408889634
QSCALE = D ** -0.5 * LOG2E
NEG = -1e30

NT = (((1,), (1,)), ((), ()))


def _dot(a, b):
    return jnp.dot(a, b, preferred_element_type=F32)


def _dot_nt(a, b):
    return lax.dot_general(a, b, NT, preferred_element_type=F32)


def _bf(x):
    return pltpu.bitcast(x, BF16)


def _u32(x):
    return pltpu.bitcast(x, U32)


def _h(r0, n):
    return pl.ds(r0 // 2, n // 2)


def _repack(ev, od):
    lo = (ev & jnp.uint32(0xFFFF)) | (od << 16)
    hi = (ev >> 16) | (od & jnp.uint32(0xFFFF0000))
    return lo, hi


def _split(w):
    return (pltpu.bitcast(w << 16, F32), pltpu.bitcast(w & jnp.uint32(0xFFFF0000), F32))


def _join(lo, hi):
    half = jnp.uint32(0x8000)
    lo = (pltpu.bitcast(lo, U32) + half) >> 16
    hi = (pltpu.bitcast(hi, U32) + half) & jnp.uint32(0xFFFF0000)
    return lo | hi


def _add(a, b):
    return _join(a[0] + b[0], a[1] + b[1])


def _sub(a, b):
    return _join(a[0] - b[0], a[1] - b[1])


def _opaque_zero(vals):
    acc = None
    for v in vals:
        b = v if v.dtype == U32 else pltpu.bitcast(v, U32)
        for r in range(0, b.shape[0], 8):
            for c in range(0, b.shape[1], LANE):
                t = b[r:r + 8, c:c + LANE]
                acc = t if acc is None else acc | t
    return jnp.minimum((acc >> 1).astype(jnp.int32), 0)


def _pin(x, zero, r=0, c=0):
    t = pltpu.bitcast(pltpu.bitcast(x[r:r + 8, c:c + LANE], jnp.int32) + zero, x.dtype)
    row = ([x[r:r + 8, :c]] if c > 0 else []) + [t] + (
        [x[r:r + 8, c + LANE:]] if c + LANE < x.shape[1] else [])
    row = jnp.concatenate(row, axis=1) if len(row) > 1 else row[0]
    col = ([x[:r, :]] if r > 0 else []) + [row] + ([x[r + 8:, :]] if r + 8 < x.shape[0] else [])
    return jnp.concatenate(col, axis=0) if len(col) > 1 else col[0]


def _digits(n):
    return [int(c) for c in str(n)]


def _rowcat(xs):
    return jnp.concatenate(xs, axis=0) if len(xs) > 1 else xs[0]


def _lanecat(xs):
    return jnp.concatenate(xs, axis=1) if len(xs) > 1 else xs[0]


def _make_kernel(cfg):
    tq = cfg["tq"]
    nq = S // tq
    nsub = tq // LANE
    KT = MP // LANE
    TP = LANE // 2
    XC = 4
    x_cols = S // XC
    QP = 2
    QIT = H // 2 // QP
    XH = (S - x_cols) // 2
    CP = 176
    AT = 3

    def kernel(aq_hbm, ak_hbm, av_hbm, sh_hbm, ssm_hbm, dd_hbm, x_hbm, c_hbm,
               wq_hbm, wk_hbm, wv_hbm, wo_hbm,
               out_hbm,
               a_v, sh_v, dd_v, par_v, f_v,
               xt_v, x_v, xs_v, c_v, wqs_v, wq_v, qacc, ws_v, wkv_v, wo_v,
               q_all, k_s, v_s, kb_s, vb_s, pd_s, pa_s, ra_t, rb_t, oa_v, out_v,
               sem_x, sem_wq, sem_w, sem_c, sem_s, sem_a, sem_out):
        x32, c32, wq32, wk32, wv32, wo32 = (
            r.bitcast(U32) for r in (x_hbm, c_hbm, wq_hbm, wk_hbm, wv_hbm, wo_hbm))
        a32 = [r.bitcast(U32) for r in (ak_hbm, av_hbm, ssm_hbm, aq_hbm)]

        sa_v = qacc

        def x_copy(i):
            cs = pl.ds(i * x_cols, x_cols)
            return pltpu.make_async_copy(x32.at[:, cs], xt_v.at[:, cs], sem_x.at[i])

        def wq_pairs(kt):
            return min(TP, M // 2 - kt * TP)

        def wq_copies(kt):
            n = wq_pairs(kt)
            dst = wqs_v[kt].reshape(4, n, 8, LANE)
            return [pltpu.make_async_copy(
                wq32.at[pl.ds(kt * TP, n), pl.ds(8 * (k // 2), 8), pl.ds((k % 2) * LANE, LANE)],
                dst.at[k], sem_wq.at[kt]) for k in range(4)]

        def wq_wait(kt):
            pltpu.make_async_copy(wqs_v[kt], wqs_v[kt], sem_wq.at[kt]).wait()

        def w_copies(g):
            dst = ws_v.reshape(8, C // 2, 8, LANE)
            src = (wk32, wv32)[g // 2]
            return [pltpu.make_async_copy(
                src.at[:, pl.ds(8 * par, 8), pl.ds((g % 2) * LANE, LANE)],
                dst.at[2 * g + par], sem_w.at[g]) for par in range(2)]

        def w_wait(g):
            pltpu.make_async_copy(ws_v.at[g], ws_v.at[g], sem_w.at[g]).wait()

        c_bounds = [0, CP, 2 * CP, S // 4]

        def c_copies(p):
            r0, n = c_bounds[p], c_bounds[p + 1] - c_bounds[p]
            return [pltpu.make_async_copy(c32.at[rs], c_v.at[rs], sem_c.at[p])
                    for rs in (pl.ds(r0, n), pl.ds(S // 4 + r0, n))]

        wo_copy = pltpu.make_async_copy(wo32, wo_v, sem_a.at[0])

        a_parts = [pl.ds(0, AR // 2), pl.ds(AR // 2, M // 2 - AR // 2)]

        def a_start(part):
            rs = a_parts[part]
            for k in range(4):
                pltpu.make_async_copy(
                    a32[k].at[rs], a_v.at[k, rs], sem_a.at[1 + part]).start()

        def a_wait(part):
            view = a_v.at[:, a_parts[part]]
            pltpu.make_async_copy(view, view, sem_a.at[1 + part]).wait()

        small = [pltpu.make_async_copy(sh_hbm, sh_v, sem_s.at[0]),
                 pltpu.make_async_copy(dd_hbm, dd_v, sem_s.at[1])]

        link = [None]
        pace = [None]

        def set_link(res, row=None, pacer=None):
            if row is None:
                row = res.shape[0] - cfg["link_back"]
            link[0] = _opaque_zero([res[row:row + 8, res.shape[1] - LANE:]])
            pace[0] = res if pacer is None else pacer

        def linked(x):
            return x if link[0] is None else _pin(x, link[0])

        def paced(w):
            res = pace[0]
            if res is None or link[0] is None or not cfg["pace_step"]:
                return w
            rows = []
            r0, step = cfg["pace_row"], cfg["pace_step"]
            if res.shape[0] < 400:
                r0, step = 0, 8
            if res.shape[0] < 200:
                return w
            zs = [_opaque_zero([res[r:r + 8, res.shape[1] - LANE:]])
                  for r in range(r0, r0 + 8 * step, step)]
            for r in range(0, w.shape[0], 8):
                z = zs[7 - (r // 8) % 8]
                t = pltpu.bitcast(w[r:r + 8, :], jnp.int32)
                rows.append(pltpu.bitcast(t + _lanecat([z] * (w.shape[1] // LANE)), U32))
            return _rowcat(rows)

        for cp in small:
            cp.start()
        x_copy(0).start()
        for cp in wq_copies(0):
            cp.start()

        def zero_body(k, carry):
            n = LANE // (S // D)
            bi = lax.broadcasted_iota(jnp.int32, (n, LANE), 0) + k * n
            mi = lax.broadcasted_iota(jnp.int32, (n, LANE), 1)
            ph = ((4 * mi + 1) * bi) & 511
            ang = ph.astype(F32) * (2.0 * 3.141592653589793 / 512.0)
            rs = pl.ds(pl.multiple_of(k * (n // 2), n // 2), n // 2)
            f_v[rs, 0:LANE] = _u32(jnp.cos(ang).astype(BF16))
            f_v[rs, LANE:] = _u32((-jnp.sin(ang)).astype(BF16))

            rb_t[k] = jnp.zeros((M, D), F32)
            cs = pl.ds(pl.multiple_of((k % 4) * D, D), D)
            ra_t[k // 4, 0:LANE, cs] = jnp.zeros((LANE, D), F32)
            ra_t[k // 4, AT * LANE:, cs] = jnp.zeros((M - AT * LANE, D), F32)
            return carry

        lax.fori_loop(0, S // D, zero_body, 0)
        c_v[S // 2:, :] = jnp.zeros((8, C), U32)

        for kt in range(1, KT):
            for cp in wq_copies(kt):
                cp.start()
        with jax.named_scope("small_wait"):
            for cp in small:
                cp.wait()
        sh = sh_v[...].astype(F32)
        for j in range(KS):
            par_v[j] = jnp.broadcast_to(sh[j:j + 1, :], (LANE, M)).T
        dd = dd_v[...].astype(F32).reshape(1, M)
        par_v[KS] = jnp.broadcast_to(dd, (LANE, M)).T

        def x_transpose(i):
            xt = xt_v[:, pl.ds(i * x_cols, x_cols)]
            xt = _rowcat([xt, jnp.zeros((MP // 2 - M // 2, x_cols), U32)])
            x_v[_h(i * x_cols, x_cols), :] = _u32(_bf(xt).astype(F32).T.astype(BF16))

        def q_early(kt, keep=False, jobs=()):
            first, last = kt == 0, kt == KT - 1
            n = wq_pairs(kt)
            cols = pl.ds(kt * LANE, LANE)
            if not keep:
                link[0] = None
            for j in range(H // 2):
                ws = []
                for half in range(2):
                    ev, od = (wqs_v[kt][pl.ds((2 * par + half) * n * 8 + j, n, stride=8), :]
                              for par in range(2))
                    ws.append(_repack(ev, od))
                w = _lanecat([ws[0][0], ws[1][0], ws[0][1], ws[1][1]])
                if n < TP:
                    w = _rowcat([w, jnp.zeros((TP - n, 2 * D), U32)])
                wq_v[j, pl.ds(kt * TP, TP), :] = w
                lhs = linked(x_v[_h(0, x_cols), cols])
                j0 = cfg["xs_from"]
                if jobs and j >= j0:
                    nj = H // 2 - j0
                    mine = jobs[(j - j0) * len(jobs) // nj:(j - j0 + 1) * len(jobs) // nj]
                    for k, job in enumerate(mine):
                        lhs = _pin(lhs, _opaque_zero(job()), 8 * (1 + k * 30 // len(mine)))
                d = _dot(_bf(lhs), _bf(w))
                set_link(d)
                if not first:
                    d = d + pltpu.bitcast(qacc[j], F32)
                if last:
                    d = (d * QSCALE).astype(BF16)
                    for t in range(2):
                        q_all[2 * j + t, _h(0, x_cols), :] = _u32(d[:, t * D:(t + 1) * D])
                else:
                    qacc[j] = pltpu.bitcast(d, U32)

        with jax.named_scope("x_wait"):
            x_copy(0).wait()
        x_transpose(0)
        for i in range(1, XC):
            x_copy(i).start()
        for g in range(QIT):
            for cp in w_copies(g) + (c_copies(g) if g < QIT - 1 else []):
                cp.start()
        wo_copy.start()
        a_start(0)
        a_start(1)
        with jax.named_scope("wq_wait"):
            wq_wait(0)
        q_early(0)
        with jax.named_scope("wq_wait"):
            wq_wait(1)
        q_early(1)
        with jax.named_scope("wq_wait"):
            wq_wait(2)
            wq_wait(3)
            for i in range(1, XC):
                x_copy(i).wait()
        for i in range(1, XC):
            x_transpose(i)

        def x_sums(u):
            a11, a12, a21, a22 = (
                _split(x_v[pl.ds((x_cols + rb * XH) // 2 + 8 * u, 8), cb * D:(cb + 1) * D])
                for rb in range(2) for cb in range(2))
            outs = [_add(a11, a22), _add(a21, a22), _add(a11, a12), _sub(a21, a11),
                    _sub(a12, a22)]
            for k, o in enumerate(outs):
                xs_v[k, 8 * u:8 * u + 8, :] = o
            return outs

        q_early(2, jobs=[functools.partial(x_sums, u) for u in range(XH // 16)])
        q_early(3, keep=True)

        def unpack(it, sub, j):
            g = it
            ev, od = (ws_v[g, pl.ds((par * (C // 2) + sub * TP) * 8 + j, TP, stride=8), :]
                      for par in range(2))
            lo, hi = _repack(ev, od)
            rows = pl.ds(sub * TP, TP)
            cols = pl.ds(pl.multiple_of(g * LANE, LANE), LANE)
            wkv_v[2 * j, rows, cols] = lo
            wkv_v[2 * j + 1, rows, cols] = hi
            return [lo, hi]

        def a_sums(it, u):
            r0 = jnp.clip((it - 1) * CP, 0, S // 4 - CP) + 8 * u
            src = [jnp.where(it == 0, S // 2, r0 + rb * (S // 4)) for rb in range(2)]
            r0 = pl.multiple_of(r0, 8)
            kw = C // 2
            a11, a12, a21, a22 = (
                _split(c_v[pl.ds(pl.multiple_of(src[rb], 8), 8), pl.ds(cb * kw, kw)])
                for rb in range(2) for cb in range(2))
            outs = [_add(a11, a22), _add(a21, a22), _add(a11, a12), _sub(a21, a11),
                    _sub(a12, a22)]
            for k, o in enumerate(outs):
                sa_v[k, pl.ds(r0, 8), :] = o
            return outs

        units = [functools.partial(unpack, sub=s_, j=j_)
                 for s_ in range(C // 2 // TP) for j_ in range(H // 2)]
        for u_ in range(CP // 8):
            units.insert(4 * u_ + 1, functools.partial(a_sums, u=u_))

        def q_pair(pair, todo):
            raw = lambda r, c: _lanecat([
                wq_v[pair, r * LANE:(r + 1) * LANE, pl.ds(t * D + c * LANE, LANE)]
                for t in range(2)])
            b = lambda r, c: _split(raw(r, c))
            sb = {1: _add(b(0, 0), b(1, 1)), 2: raw(0, 0), 3: _sub(b(0, 1), b(1, 1)),
                  4: _sub(b(1, 0), b(0, 0)), 5: raw(1, 1), 6: _add(b(0, 0), b(0, 1)),
                  7: _add(b(1, 0), b(1, 1))}
            n = XH // 2
            for rho in range(2):
                def sa(m):
                    if m == 3:
                        return x_v[_h(x_cols + rho * n, n), 0:D]
                    if m == 4:
                        return x_v[_h(x_cols + XH + rho * n, n), D:]
                    return xs_v[{1: 0, 2: 1, 5: 2, 6: 3, 7: 4}[m], _h(rho * n, n), :]

                def put(half, c0, c1):
                    rows = _h(x_cols + half * XH + rho * n, n)
                    for t in range(2):
                        q = _lanecat([c[:, t * LANE:(t + 1) * LANE] for c in (c0, c1)])
                        q_all[2 * pair + t, rows, :] = _u32((q * QSCALE).astype(BF16))

                p = {}
                for pos, m in enumerate((5, 1, 4, 7, 3, 2, 6)):
                    lhs = linked(sa(m))
                    nj = min(len(todo), cfg["q_jobs"][7 * rho + pos])
                    jobs = [todo.pop()(it=pair // QP) for _ in range(nj)]
                    for k, job in enumerate(jobs):
                        lhs = _pin(lhs, _opaque_zero(job), 8 * (1 + k * (n // 16 - 1) // nj))
                    p[m] = _dot(_bf(lhs), _bf(sb[m]))
                    set_link(p[m])
                    if m == 3:
                        put(0, (p[1] + p[4]) + (p[7] - p[5]), p[3] + p[5])
                put(1, p[2] + p[4], (p[1] + p[3]) + (p[6] - p[2]))

        def q_body(it, carry):
            with jax.named_scope("w_wait"):
                w_wait(it)
                for p in range(QIT - 1):
                    @pl.when(it == p + 1)
                    def _():
                        for cp in c_copies(p):
                            cp.wait()
            link[0] = None
            todo = units[::-1]
            for p in range(QP):
                q_pair(QP * it + p, todo)
            assert not todo
            return carry

        with jax.named_scope("q_loop"):
            lax.fori_loop(0, QIT, q_body, 0)
        wo_copy.wait()
        a_wait(0)

        tri = (lax.broadcasted_iota(jnp.int32, (LANE, LANE), 1)
               <= lax.broadcasted_iota(jnp.int32, (LANE, LANE), 0))

        NOUT = S // D

        def out_copy(i):
            if i >= NOUT:
                t = i - NOUT
                return pltpu.make_async_copy(
                    oa_v.at[t], out_hbm.at[:, pl.ds(t * LANE, LANE)], sem_out.at[i])
            rs = pl.ds(i * D, D)
            return pltpu.make_async_copy(
                out_v.at[rs], out_hbm.at[rs, pl.ds(AT * LANE, 2 * M - AT * LANE)], sem_out.at[i])

        body_chunks = _digits(cfg["body_chunks"])

        def b_out(k, tot):
            c0 = (k * D) % (S // 2)
            full = _rowcat([ra_t[k * D // (S // 2), AT * LANE:, c0:c0 + D], tot]).T
            out_v[k * D:(k + 1) * D, :] = full.astype(BF16)
            return full

        def head_step(h, carry):
            with jax.named_scope("step"):
                return head_step_(h, carry)

        def head_step_(h, carry):
            with_a = cfg["use_a"]

            @pl.when(h == A_STEPS)
            def _():
                for t in range(AT):
                    out_copy(NOUT + t).start()

            @pl.when(h == cfg["h0"] + 1)
            def _():
                a_wait(1)

            link[0] = None
            n2 = AR // 2
            a_rows2 = pl.ds(pl.multiple_of(jnp.minimum(h, A_STEPS - 1) * n2, n2), n2)
            a_rows = pl.ds(pl.multiple_of(jnp.minimum(h, A_STEPS - 1) * AR, AR), AR)

            kw = C // 2
            pending = []
            chains = {i: [] for i in range(nq + 1)}
            deadline = [None]

            def flush_pending(x, row):
                done = list(pending)
                del pending[:]
                if not done:
                    return x
                x = _pin(x, _opaque_zero([f for _, f in done]), row)

                @pl.when(h == H - 1)
                def _():
                    for k, _f in done:
                        out_copy(k).start()
                return x

            def a_fwd():
                kk = _bf(a_v[0, a_rows2, :]).astype(F32)
                lane = lax.broadcasted_iota(jnp.int32, (AR, LANE), 1)
                coef = [par_v[j, a_rows, :] for j in range(KS)]
                rolled = [kk] + [pltpu.roll(kk, j, 1) for j in range(1, KS)]
                vv = _bf(a_v[1, a_rows2, :]).astype(F32)
                kv_blocks = []
                for a in range(NB):
                    cs = slice(a * LANE, (a + 1) * LANE)
                    acc = rolled[0][:, cs] * coef[0]
                    for j in range(1, KS):
                        t = rolled[j][:, cs]
                        if a == 0:
                            t = jnp.where(lane >= j, t, 0.0)
                        acc = acc + t * coef[j]
                    kv_blocks.append(acc * vv[:, cs])
                hk = a_v[2, a_rows2, :]
                hk = _rowcat([hk[:, a * LANE:(a + 1) * LANE] for a in range(NB)])
                fm = _bf(f_v[...])
                hs = _dot(_bf(linked(hk)), fm)
                kv = linked(_rowcat(kv_blocks)).astype(BF16)
                xs = _dot(kv, fm)
                set_link(xs)
                return kv, xs, hs

            def a_conv(xs, hs):
                def tile(v, a, g, part):
                    r = a * AR + 8 * g
                    return v[r:r + 8, part * LANE:(part + 1) * LANE]

                z = {}
                gate = None
                width = cfg["a_width"]
                for g in range(AR // 8):
                    hr = [tile(hs, 0, g, 0)] + [
                        tile(hs, j, g, 0) - tile(hs, j - 1, g, 1) for j in range(1, NB)]
                    hi = [tile(hs, 0, g, 1)] + [
                        tile(hs, j, g, 1) + tile(hs, j - 1, g, 0) for j in range(1, NB)]
                    for c0 in range(0, NB, width):
                        for a in range(c0 + width):
                            xr, xi = tile(xs, a, g, 0), tile(xs, a, g, 1)
                            if gate is not None:
                                xr, xi = _pin(xr, gate), _pin(xi, gate)
                            for c in range(max(c0, a), c0 + width):
                                j = c - a
                                tr = xr * hr[j] - xi * hi[j]
                                ti = xr * hi[j] + xi * hr[j]
                                z[c, g] = (tr, ti) if a == 0 else (z[c, g][0] + tr, z[c, g][1] + ti)
                            gate = _opaque_zero(list(z[c0 + width - 1, g]))
                            chains[nq].append(gate)
                return z

            def a_inv(kv, z, flush=False):
                fm = _bf(f_v[...])
                ng = AR // 8
                ys = []
                for u in range(2):
                    rows = [_lanecat(z[c, g]) for g in range(u * ng // 2, (u + 1) * ng // 2)
                            for c in range(NB)]
                    lhs = linked(_rowcat(rows))
                    if flush:
                        lhs = flush_pending(lhs, 8)
                    ys.append(_dot_nt(lhs.astype(BF16), fm))
                y = _rowcat(ys)
                dd = par_v[KS, a_rows, :]
                for c in range(NB):
                    cs = slice(c * LANE, (c + 1) * LANE)
                    yc = _rowcat([y[(g * NB + c) * 8:(g * NB + c + 1) * 8, :] for g in range(ng)])
                    qq = _bf(a_v[3, a_rows2, cs]).astype(F32)
                    kvf = kv[c * AR:(c + 1) * AR, :].astype(F32)
                    c2 = (c % (NB // 2)) * LANE
                    ra_t[c // (NB // 2), a_rows, c2:c2 + LANE] = qq * (yc * (1.0 / LANE) + kvf * dd)

            def a_out():
                slab = jnp.clip(h // 4 - 1, 0, AT - 1)
                half = h % 2
                x = ra_t[half, pl.ds(pl.multiple_of(slab * LANE, LANE), LANE), :]
                xt = x.T
                dst = jnp.where(h >= A_STEPS, AT, slab)
                oa_v[dst, pl.ds(pl.multiple_of(half * (S // 2), S // 2), S // 2), :] = xt.astype(BF16)
                return xt

            def w_blk(r, c):
                return wkv_v[h, _h(r * kw, kw), pl.ds(c * LANE, LANE)]

            def one_pass(lhs, w, flush):
                lhs = linked(lhs)
                if flush:
                    lhs = flush_pending(lhs, cfg["ao_row"])
                if deadline[0] is not None:
                    if deadline[0][0] == 0:
                        lhs = _pin(lhs, deadline[0][1], cfg["ao_row"] - 8)
                        deadline[0] = None
                    else:
                        deadline[0] = (deadline[0][0] - 1, deadline[0][1])
                d = _dot(_bf(lhs), _bf(paced(w)))
                set_link(d)
                return d

            def b_op(which, m):
                raw = lambda r, c: w_blk(r, 2 * which + c)
                blk = lambda r, c: _split(raw(r, c))
                return {1: lambda: _add(blk(0, 0), blk(1, 1)),
                        2: lambda: raw(0, 0),
                        3: lambda: _sub(blk(0, 1), blk(1, 1)),
                        4: lambda: _sub(blk(1, 0), blk(0, 0)),
                        5: lambda: raw(1, 1),
                        6: lambda: _add(blk(0, 0), blk(0, 1)),
                        7: lambda: _add(blk(1, 0), blk(1, 1))}[m]()

            def a_op(m, rho):
                rs = _h(rho * tq, tq)
                if m == 3:
                    return c_v[rs, 0:kw]
                if m == 4:
                    return c_v[_h(S // 2 + rho * tq, tq), kw:]
                return sa_v[{1: 0, 2: 1, 5: 2, 6: 3, 7: 4}[m], rs, :]

            b_cache, prod = {}, {}

            def kv_proj(which, blk, flush):
                rho = blk % 2
                for k, m in enumerate(_digits(cfg["kv_top" if blk < 2 else "kv_bot"])):
                    if (which, m) not in b_cache:
                        b_cache[which, m] = b_op(which, m)
                    prod[which, m, rho] = one_pass(a_op(m, rho), b_cache[which, m], k == flush)
                p = lambda m: prod[which, m, rho]
                if blk < 2:
                    return [(p(1) + p(4)) + (p(7) - p(5)), p(3) + p(5)]
                return [p(2) + p(4), (p(1) + p(3)) + (p(6) - p(2))]

            def k_proj(blk, flush=-1):
                k = kv_proj(0, blk, flush)
                k_s[_h(blk * tq, tq), :] = _u32(_lanecat(k).astype(BF16))
                if blk < nq - 1:
                    b = lambda r, c: k[r][c * D:(c + 1) * D, :]
                    sums = [b(0, 0) + b(1, 1), b(0, 1) - b(1, 1), b(1, 0) - b(0, 0),
                            b(0, 0) + b(0, 1), b(1, 0) + b(1, 1)]
                    for n, x in enumerate(sums):
                        kb_s[n, _h(blk * D, D), :] = _u32(x.astype(BF16))

            def v_proj(blk, flush=-1):
                v = kv_proj(1, blk, flush)
                v_s[_h(blk * tq, tq), :] = _u32(_lanecat(v).astype(BF16))
                if blk < nq - 1:
                    b = lambda r, c: v[c][r * D:(r + 1) * D, :]
                    sums = [b(0, 0) + b(1, 1), b(0, 1) - b(1, 1), b(1, 0) - b(0, 0),
                            b(0, 0) + b(0, 1), b(1, 0) + b(1, 1)]
                    for k, x in enumerate(sums):
                        vb_s[k, _h(blk * D, D), :] = _u32(x.astype(BF16))

            def qk(i, dep=None, flush=False):
                r0 = i * tq
                off = None
                if i > 0:
                    raw = lambda r, c: q_all[h, _h(r0 + r * D, D), c * LANE:(c + 1) * LANE]
                    a = lambda r, c: _split(raw(r, c))
                    sa = {1: _add(a(0, 0), a(1, 1)), 2: _add(a(1, 0), a(1, 1)), 3: raw(0, 0),
                          4: raw(1, 1), 5: _add(a(0, 0), a(0, 1)), 6: _sub(a(1, 0), a(0, 0)),
                          7: _sub(a(0, 1), a(1, 1))}

                    def sb(m, j, t):
                        if m in (2, 5):
                            c = 0 if m == 2 else 1
                            rows = _h(j * tq + c * D + t * LANE, LANE)
                            return k_s[rows, c * LANE:(c + 1) * LANE]
                        n = {1: 0, 3: 1, 4: 2, 6: 3, 7: 4}[m]
                        return kb_s[n, _h(j * D + t * LANE, LANE), :]

                    top, bot, due = {}, {}, []
                    n_dot = 0
                    for j in range(i):
                        for t in range(2):
                            p = {}
                            for n, m in enumerate(_digits(cfg["s_ord"])):
                                lhs = linked(sa[m])
                                if due and n == cfg["s_due"]:
                                    lhs = _pin(lhs, due.pop(), cfg["s_row"])
                                p[m] = _dot_nt(_bf(lhs), _bf(sb(m, j, t)))
                                n_dot += 1
                                if n_dot % 4 == 0:
                                    set_link(p[m], cfg["s_link"])
                            top[4 * j + t] = (p[1] + p[4]) + (p[7] - p[5])
                            top[4 * j + 2 + t] = p[3] + p[5]
                            bot[4 * j + t] = p[2] + p[4]
                            bot[4 * j + 2 + t] = (p[1] + p[3]) + (p[6] - p[2])
                            due.append(_opaque_zero(
                                [x[4 * j + c + t] for x in (top, bot) for c in (0, 2)]))
                    off = _rowcat([_lanecat([x[c] for c in range(4 * i)]) for x in (top, bot)])
                q = linked(q_all[h, _h(r0, tq), :])
                if off is not None:
                    q = _pin(q, due.pop(), cfg["ao_row"] - 8)
                if dep is not None:
                    q = _pin(q, _opaque_zero([dep]), cfg["ao_row"])
                main = _dot_nt(_bf(q), _bf(k_s[_h(r0, LANE), :]))
                parts = [main if off is None else _lanecat([off, main])]
                for j in range(1, nsub):
                    q = linked(q_all[h, _h(r0 + LANE * j, tq - LANE * j), :])
                    if flush and j == cfg["q_pin"]:
                        q = flush_pending(q, 8)
                    parts.append(_dot_nt(_bf(q), _bf(k_s[_h(r0 + LANE * j, LANE), :])))
                set_link(parts[2], cfg["link_part"], main)
                return parts

            def exps(i, parts):
                sas, mbs = [], []
                for a in range(nsub):
                    blocks = [parts[j][LANE * (a - j):LANE * (a - j + 1), :] for j in range(a + 1)]
                    last = blocks[-1]
                    w = last.shape[1]
                    dg = jnp.where(tri, last[:, w - LANE:], NEG)
                    blocks[-1] = dg if w == LANE else _lanecat([last[:, :w - LANE], dg])
                    sas.append(_lanecat(blocks))
                    mx = jnp.max(sas[a], axis=1, keepdims=True)
                    mbs.append(jnp.broadcast_to(mx, (LANE, LANE)))
                chain = _opaque_zero([b[b.shape[0] - 8:, b.shape[1] - LANE:] for b in parts])
                pg, psums = {}, {}
                for r in range(0, tq // 2, 8):
                    for row in (r, r + tq // 2):
                        a, g = divmod(row, LANE)
                        mg = _pin(mbs[a][g:g + 8, :], chain)
                        pg[row] = [jnp.exp2(sas[a][g:g + 8, t:t + LANE] - mg)
                                   for t in range(0, sas[a].shape[1], LANE)]
                        psums[row] = functools.reduce(jnp.add, pg[row])
                        chain = _opaque_zero([psums[row]])
                        chains[i].append(chain)
                return pg, psums

            def softmax(i, pg, psums):
                r0 = i * tq
                pd, pa = pd_s.at[i % 2], pa_s[i % 2]
                first = lambda x, c=0: _pin(x, link[0], 0, c).astype(BF16)
                nt0 = r0 // LANE
                ls = []
                for a in range(nsub):
                    rows = range(LANE * a, LANE * (a + 1), 8)
                    ls.append(jnp.sum(_rowcat([psums[r] for r in rows]), axis=1, keepdims=True))
                    pd[LANE * a:LANE * (a + 1), 0:LANE * (a + 1)] = first(
                        _rowcat([_lanecat(pg[r][nt0:]) for r in rows]), LANE * a)
                if i > 0:
                    quad = lambda rh, ch: _rowcat([
                        _lanecat([pg[rh * (tq // 2) + r][4 * j + 2 * ch + t]
                                  for j in range(i) for t in range(2)])
                        for r in range(0, tq // 2, 8)])
                    a11, a12, a21, a22 = quad(0, 0), quad(0, 1), quad(1, 0), quad(1, 1)
                    ops = [a11 + a22, a21 + a22, a11, a22, a11 + a12, a21 - a11, a12 - a22]
                    for m, x in enumerate(ops):
                        if i == 3:
                            x = _pin(x, link[0], 0, 2 * D)
                        pa[m, :, 0:i * D] = first(x)
                return ls

            def pv(i, ls, flush=-1):
                r0 = i * tq
                pd, pa = pd_s.at[i % 2], pa_s[i % 2]
                off = None
                if i > 0:
                    def b_rows(m, j0, j1):
                        if m in (2, 5):
                            q = 0 if m == 2 else 1
                            return _rowcat([
                                v_s[_h(j * tq + q * D, D), q * LANE:(q + 1) * LANE]
                                for j in range(j0, j1)])
                        k = {1: 0, 3: 1, 4: 2, 6: 3, 7: 4}[m]
                        return vb_s[k, _h(j0 * D, (j1 - j0) * D), :]

                    p, n_dot = {}, 0
                    for j0, j1 in {1: [(0, 1)], 2: [(0, 2)], 3: [(0, 2), (2, 3)]}[i]:
                        for m in _digits(cfg["p_ord"]):
                            cols = slice(j0 * D, j1 * D)
                            rhs = b_rows(m, j0, j1)
                            if n_dot == flush:
                                rhs = flush_pending(rhs, 0)
                            rhs = _bf(rhs)
                            n_dot += 1
                            if j1 - j0 == 1 and m == cfg["p_ord"] % 10:
                                d = _rowcat([_dot(pa[m - 1, r:r + LANE, cols], rhs)
                                             for r in (0, LANE)])
                            else:
                                d = _dot(pa[m - 1, :, cols], rhs)
                            p[m] = d if m not in p else p[m] + d
                    off = _rowcat([
                        _lanecat([(p[1] + p[4]) + (p[7] - p[5]), p[3] + p[5]]),
                        _lanecat([p[2] + p[4], (p[1] + p[3]) + (p[6] - p[2])])])
                ctx = []
                for j in range(nsub):
                    c0 = LANE * j
                    ctx.append(_dot(pd[c0:, c0:c0 + LANE], _bf(v_s[_h(r0 + c0, LANE), :])))
                set_link(ctx[2], cfg["link_part"], ctx[0])
                cs = []
                for a in range(nsub):
                    sl = lambda j: slice(LANE * (a - j), LANE * (a - j + 1))
                    r = pl.reciprocal(ls[a], approx=True)
                    r = r * (2.0 - ls[a] * r)
                    terms = [ctx[j][sl(j)] for j in range(a + 1)]
                    if off is not None:
                        terms.append(off[sl(0)])
                    cs.append(functools.reduce(jnp.add, terms) * r)
                return _rowcat(cs)

            wo_cache = {}

            def oproj(i, ctx):
                mh = M // 4
                raw = lambda r, c: wo_v[h, r * mh:(r + 1) * mh, c * LANE:(c + 1) * LANE]
                a = lambda r, c: _split(raw(r, c))
                a_ops = {1: lambda: _add(a(0, 0), a(1, 1)), 2: lambda: _add(a(1, 0), a(1, 1)),
                         3: lambda: raw(0, 0), 4: lambda: raw(1, 1),
                         5: lambda: _add(a(0, 0), a(0, 1)), 6: lambda: _sub(a(1, 0), a(0, 0)),
                         7: lambda: _sub(a(0, 1), a(1, 1))}
                b = lambda r, c: ctx[c * D:(c + 1) * D, r * LANE:(r + 1) * LANE]
                b_ops = {1: lambda: b(0, 0) + b(1, 1), 2: lambda: b(0, 0),
                         3: lambda: b(0, 1) - b(1, 1), 4: lambda: b(1, 0) - b(0, 0),
                         5: lambda: b(1, 1), 6: lambda: b(0, 0) + b(0, 1),
                         7: lambda: b(1, 0) + b(1, 1)}
                p = {}
                order = _digits(cfg["o_ord"])
                mm = M // 2
                old = lambda r, c: rb_t[2 * i + c, r * mm:(r + 1) * mm, :]
                terms = {(0, 0): (1, 4, -5, 7), (0, 1): (3, 5), (1, 0): (2, 4), (1, 1): (1, -2, 3, 6)}

                def total(q):
                    acc = old(*q)
                    for m in sorted(terms[q], key=lambda m: order.index(abs(m))):
                        acc = acc + p[m] if m > 0 else acc - p[-m]
                    return acc

                for n, m in enumerate(order):
                    if m not in wo_cache:
                        wo_cache[m] = a_ops[m]()
                    rhs = b_ops[m]().astype(BF16)
                    if n == cfg["o_half"]:
                        lhs = [linked(wo_cache[m][r:r + mh // 2]) for r in (0, mh // 2)]
                        halves = [_dot_nt(_bf(x), rhs) for x in lhs]
                        p[m] = _rowcat(halves)
                        set_link(halves[1], 0)
                    else:
                        p[m] = _dot_nt(_bf(linked(wo_cache[m])), rhs)
                        if (n - (n > cfg["o_half"])) % 2 == 1:
                            set_link(p[m], cfg["o_link"])
                for c in range(2):
                    k = 2 * i + c
                    tot = _rowcat([total((r, c)) for r in range(2)])
                    rb_t[k] = tot
                    if k + 1 in body_chunks:
                        pending.append((k, b_out(k, tot)))

            st = {}
            for op in cfg["seq"].split():
                op, _, dl = op.partition("@")
                if dl:
                    ch = chains[int(dl[0])]
                    deadline[0] = (int(dl[1]), ch[int(dl[2:]) * len(ch) // 16 - 1])
                op, _, fl = op.partition("!")
                fl = int(fl) if fl else -1
                kind, i = op[0], int(op[1:] or 0)
                if kind == "K":
                    k_proj(i, fl)
                elif kind == "V":
                    v_proj(i, fl)
                elif kind == "Q":
                    st["e", i] = exps(
                        i, qk(i, a_out() if i == cfg["ao_at"] else None, fl >= 0))
                elif kind == "P":
                    st["ctx", i] = pv(i, softmax(i, *st["e", i]), fl)
                elif kind == "O":
                    oproj(i, st["ctx", i])
                elif kind == "F" and with_a:
                    st["kv"], xs, hs = a_fwd()
                    st["z"] = a_conv(xs, hs)
                elif kind == "I" and with_a:
                    a_inv(st["kv"], st["z"], fl >= 0)
            assert not pending and deadline[0] is None
            return carry

        with jax.named_scope("loop_a"):
            lax.fori_loop(cfg["h0"], H, head_step, 0)
        with jax.named_scope("tail"):
            for i in [k for k in range(NOUT) if k + 1 not in body_chunks]:
                b_out(i, rb_t[i])
                out_copy(i).start()
            for i in range(NOUT + AT):
                out_copy(i).wait()

    scratch = [
        pltpu.VMEM((4, M // 2, S), U32),
        pltpu.VMEM((KS, M), BF16),
        pltpu.VMEM((M,), BF16),
        pltpu.VMEM((KS + 1, M, LANE), F32),
        pltpu.VMEM((LANE // 2, 2 * LANE), U32),
        pltpu.VMEM((M // 2, S), U32),
        pltpu.VMEM((S // 2, MP), U32),
        pltpu.VMEM((5, XH // 2, D), U32),
        pltpu.VMEM((S // 2 + 8, C), U32),
        [pltpu.VMEM((4 * min(TP, M // 2 - kt * TP) * 8, LANE), U32)
         for kt in range(KT)],
        pltpu.VMEM((H // 2, MP // 2, 2 * D), U32),
        pltpu.VMEM((H // 2, x_cols, 2 * D), U32),
        pltpu.VMEM((QIT, C * 8, LANE), U32),
        pltpu.VMEM((H, C // 2, 2 * D), U32),
        pltpu.VMEM((H, M // 2, D), U32),
        pltpu.VMEM((H, S // 2, D), U32),
        pltpu.VMEM((S // 2, D), U32),
        pltpu.VMEM((S // 2, D), U32),
        pltpu.VMEM((5, (nq - 1) * D // 2, LANE), U32),
        pltpu.VMEM((5, (nq - 1) * D // 2, LANE), U32),
        pltpu.VMEM((2, tq, tq), BF16),
        [pltpu.VMEM((7, tq // 2, n * D), BF16) for n in (2, 3)],
        pltpu.VMEM((2, M, S // 2), F32),
        pltpu.VMEM((S // D, M, D), F32),
        pltpu.VMEM((AT + 1, S, LANE), BF16),
        pltpu.VMEM((S, 2 * M - AT * LANE), BF16),
        pltpu.SemaphoreType.DMA((XC,)),
        pltpu.SemaphoreType.DMA((KT,)),
        pltpu.SemaphoreType.DMA((QIT,)),
        pltpu.SemaphoreType.DMA((QIT,)),
        pltpu.SemaphoreType.DMA((2,)),
        pltpu.SemaphoreType.DMA((3,)),
        pltpu.SemaphoreType.DMA((S // D + AT,)),
    ]
    return kernel, scratch


_DEFAULT = dict(
    tq=512, a_width=16, ao_at=1, ao_row=240, link_back=176, link_part=32, pace_row=32,
    pace_step=24, use_a=1, h0=0, body_chunks=123456, kv_top=51473, kv_bot=26, s_ord=5147236,
    o_ord=5241736, p_ord=1234567, o_link=48, o_half=6, q_jobs=(2, 4, 4, 4, 1, 3, 1, 3, 5, 6, 6, 1, 2, 1), xs_from=3, s_link=64, s_due=4, s_row=120, q_pin=2,
    seq="K0 Q0 K1 Q1 V0 F P0 K2@1116 Q2 O0 V1!4 P1 K3@2116 O1 Q3!0 V2@4012 P2 V3@3116 O2 P3!6 I O3")


def _build(**kw):
    cfg = dict(_DEFAULT)
    cfg.update(kw)
    kernel, scratch = _make_kernel(cfg)

    def run(A_q, A_k, A_v, A_shift_k, A_ssm_k, A_ssm_D, B_x, B_c_kv, B_w_q, B_w_uk,
            B_w_uv, B_w_o):
        tr = lambda a: jnp.swapaxes(a, 1, 2).reshape(M, S)
        args = (
            tr(A_q), tr(A_k), tr(A_v), A_shift_k.T, A_ssm_k, A_ssm_D, tr(B_x),
            B_c_kv.reshape(S, C),
            B_w_q.reshape(M // 2, 2 * H, D), B_w_uk.reshape(C // 2, 2 * H, D),
            B_w_uv.reshape(C // 2, 2 * H, D),
            jnp.swapaxes(B_w_o, 1, 2),
        )
        out = pl.pallas_call(
            kernel,
            in_specs=[pl.BlockSpec(memory_space=pl.ANY)] * len(args),
            out_specs=pl.BlockSpec(memory_space=pl.ANY),
            out_shape=jax.ShapeDtypeStruct((S, 2 * M), BF16),
            scratch_shapes=scratch,
            compiler_params=pltpu.CompilerParams(
                vmem_limit_bytes=126 * 1024 * 1024,
                disable_bounds_checks=True),
        )(*args)
        return out.reshape(1, S, 2 * M)

    return run


_run = _build()


@jax.jit
def pallas_concat_heads__ssm_conv_h3__compressed_kv_cla__prompt_kernel(
    A_q: jax.Array,
    A_k: jax.Array,
    A_v: jax.Array,
    A_shift_k: jax.Array,
    A_ssm_k: jax.Array,
    A_ssm_D: jax.Array,
    B_x: jax.Array,
    B_c_kv: jax.Array,
    B_w_q: jax.Array,
    B_w_uk: jax.Array,
    B_w_uv: jax.Array,
    B_w_o: jax.Array,
):
    return _run(A_q, A_k, A_v, A_shift_k, A_ssm_k, A_ssm_D, B_x, B_c_kv, B_w_q,
                B_w_uk, B_w_uv, B_w_o)
```

```python
import functools

import jax
import jax.numpy as jnp
from jax import lax
import jax.experimental.pallas as pl
import jax.experimental.pallas.tpu as pltpu

F32 = jnp.float32
BF16 = jnp.bfloat16
U32 = jnp.uint32

S = 2048
M = 448
MP = 512
C = 1024
H = 16
D = 256
KS = 4
LANE = 128
NB = S // LANE
AR = 32
A_STEPS = M // AR
LOG2E = 1.4426950408889634
QSCALE = D ** -0.5 * LOG2E
NEG = -1e30

NT = (((1,), (1,)), ((), ()))


def _dot(a, b):
    return jnp.dot(a, b, preferred_element_type=F32)


def _dot_nt(a, b):
    return lax.dot_general(a, b, NT, preferred_element_type=F32)


def _bf(x):
    return pltpu.bitcast(x, BF16)


def _u32(x):
    return pltpu.bitcast(x, U32)


def _h(r0, n):
    return pl.ds(r0 // 2, n // 2)


def _repack(ev, od):
    lo = (ev & jnp.uint32(0xFFFF)) | (od << 16)
    hi = (ev >> 16) | (od & jnp.uint32(0xFFFF0000))
    return lo, hi


def _split(w):
    return (pltpu.bitcast(w << 16, F32), pltpu.bitcast(w & jnp.uint32(0xFFFF0000), F32))


def _join(lo, hi):
    half = jnp.uint32(0x8000)
    lo = (pltpu.bitcast(lo, U32) + half) >> 16
    hi = (pltpu.bitcast(hi, U32) + half) & jnp.uint32(0xFFFF0000)
    return lo | hi


def _add(a, b):
    return _join(a[0] + b[0], a[1] + b[1])


def _sub(a, b):
    return _join(a[0] - b[0], a[1] - b[1])


def _opaque_zero(vals):
    acc = None
    for v in vals:
        b = v if v.dtype == U32 else pltpu.bitcast(v, U32)
        for r in range(0, b.shape[0], 8):
            for c in range(0, b.shape[1], LANE):
                t = b[r:r + 8, c:c + LANE]
                acc = t if acc is None else acc | t
    return jnp.minimum((acc >> 1).astype(jnp.int32), 0)


def _pin(x, zero, r=0, c=0):
    t = pltpu.bitcast(pltpu.bitcast(x[r:r + 8, c:c + LANE], jnp.int32) + zero, x.dtype)
    row = ([x[r:r + 8, :c]] if c > 0 else []) + [t] + (
        [x[r:r + 8, c + LANE:]] if c + LANE < x.shape[1] else [])
    row = jnp.concatenate(row, axis=1) if len(row) > 1 else row[0]
    col = ([x[:r, :]] if r > 0 else []) + [row] + ([x[r + 8:, :]] if r + 8 < x.shape[0] else [])
    return jnp.concatenate(col, axis=0) if len(col) > 1 else col[0]


def _digits(n):
    return [int(c) for c in str(n)]


def _rowcat(xs):
    return jnp.concatenate(xs, axis=0) if len(xs) > 1 else xs[0]


def _lanecat(xs):
    return jnp.concatenate(xs, axis=1) if len(xs) > 1 else xs[0]


def _make_kernel(cfg):
    tq = cfg["tq"]
    nq = S // tq
    nsub = tq // LANE
    KT = MP // LANE
    TP = LANE // 2
    XC = 4
    x_cols = S // XC
    QP = 2
    QIT = H // 2 // QP
    XH = (S - x_cols) // 2
    CP = 176
    AT = 3

    def kernel(aq_hbm, ak_hbm, av_hbm, sh_hbm, ssm_hbm, dd_hbm, x_hbm, c_hbm,
               wq_hbm, wk_hbm, wv_hbm, wo_hbm,
               out_hbm,
               a_v, sh_v, dd_v, par_v, f_v,
               xt_v, x_v, xs_v, c_v, wqs_v, wq_v, qacc, ws_v, wkv_v, wo_v,
               q_all, k_s, v_s, kb_s, vb_s, pd_s, pa_s, ra_t, rb_t, oa_v, out_v,
               sem_x, sem_wq, sem_w, sem_c, sem_s, sem_a, sem_out):
        x32, c32, wq32, wk32, wv32, wo32 = (
            r.bitcast(U32) for r in (x_hbm, c_hbm, wq_hbm, wk_hbm, wv_hbm, wo_hbm))
        a32 = [r.bitcast(U32) for r in (ak_hbm, av_hbm, ssm_hbm, aq_hbm)]

        sa_v = qacc

        def x_copy(i):
            cs = pl.ds(i * x_cols, x_cols)
            return pltpu.make_async_copy(x32.at[:, cs], xt_v.at[:, cs], sem_x.at[i])

        def wq_pairs(kt):
            return min(TP, M // 2 - kt * TP)

        def wq_copies(kt):
            n = wq_pairs(kt)
            dst = wqs_v[kt].reshape(4, n, 8, LANE)
            return [pltpu.make_async_copy(
                wq32.at[pl.ds(kt * TP, n), pl.ds(8 * (k // 2), 8), pl.ds((k % 2) * LANE, LANE)],
                dst.at[k], sem_wq.at[kt]) for k in range(4)]

        def wq_wait(kt):
            pltpu.make_async_copy(wqs_v[kt], wqs_v[kt], sem_wq.at[kt]).wait()

        def w_copies(g):
            dst = ws_v.reshape(8, C // 2, 8, LANE)
            src = (wk32, wv32)[g // 2]
            return [pltpu.make_async_copy(
                src.at[:, pl.ds(8 * par, 8), pl.ds((g % 2) * LANE, LANE)],
                dst.at[2 * g + par], sem_w.at[g]) for par in range(2)]

        def w_wait(g):
            pltpu.make_async_copy(ws_v.at[g], ws_v.at[g], sem_w.at[g]).wait()

        c_bounds = [0, CP, 2 * CP, S // 4]

        def c_copies(p):
            r0, n = c_bounds[p], c_bounds[p + 1] - c_bounds[p]
            return [pltpu.make_async_copy(c32.at[rs], c_v.at[rs], sem_c.at[p])
                    for rs in (pl.ds(r0, n), pl.ds(S // 4 + r0, n))]

        wo_copy = pltpu.make_async_copy(wo32, wo_v, sem_a.at[0])

        a_parts = [pl.ds(0, AR // 2), pl.ds(AR // 2, M // 2 - AR // 2)]

        def a_start(part):
            rs = a_parts[part]
            for k in range(4):
                pltpu.make_async_copy(
                    a32[k].at[rs], a_v.at[k, rs], sem_a.at[1 + part]).start()

        def a_wait(part):
            view = a_v.at[:, a_parts[part]]
            pltpu.make_async_copy(view, view, sem_a.at[1 + part]).wait()

        small = [pltpu.make_async_copy(sh_hbm, sh_v, sem_s.at[0]),
                 pltpu.make_async_copy(dd_hbm, dd_v, sem_s.at[1])]

        link = [None]
        pace = [None]

        def set_link(res, row=None, pacer=None):
            if row is None:
                row = res.shape[0] - cfg["link_back"]
            link[0] = _opaque_zero([res[row:row + 8, res.shape[1] - LANE:]])
            pace[0] = res if pacer is None else pacer

        def linked(x):
            return x if link[0] is None else _pin(x, link[0])

        def paced(w):
            res = pace[0]
            if res is None or link[0] is None or not cfg["pace_step"]:
                return w
            rows = []
            r0, step = cfg["pace_row"], cfg["pace_step"]
            if res.shape[0] < 400:
                r0, step = 0, 8
            if res.shape[0] < 200:
                return w
            zs = [_opaque_zero([res[r:r + 8, res.shape[1] - LANE:]])
                  for r in range(r0, r0 + 8 * step, step)]
            for r in range(0, w.shape[0], 8):
                z = zs[7 - (r // 8) % 8]
                t = pltpu.bitcast(w[r:r + 8, :], jnp.int32)
                rows.append(pltpu.bitcast(t + _lanecat([z] * (w.shape[1] // LANE)), U32))
            return _rowcat(rows)

        for cp in small:
            cp.start()
        x_copy(0).start()
        for cp in wq_copies(0):
            cp.start()

        def zero_body(k, carry):
            n = LANE // (S // D)
            bi = lax.broadcasted_iota(jnp.int32, (n, LANE), 0) + k * n
            mi = lax.broadcasted_iota(jnp.int32, (n, LANE), 1)
            ph = ((4 * mi + 1) * bi) & 511
            ang = ph.astype(F32) * (2.0 * 3.141592653589793 / 512.0)
            rs = pl.ds(pl.multiple_of(k * (n // 2), n // 2), n // 2)
            f_v[rs, 0:LANE] = _u32(jnp.cos(ang).astype(BF16))
            f_v[rs, LANE:] = _u32((-jnp.sin(ang)).astype(BF16))

            rb_t[k] = jnp.zeros((M, D), F32)
            cs = pl.ds(pl.multiple_of((k % 4) * D, D), D)
            ra_t[k // 4, 0:LANE, cs] = jnp.zeros((LANE, D), F32)
            ra_t[k // 4, AT * LANE:, cs] = jnp.zeros((M - AT * LANE, D), F32)
            return carry

        lax.fori_loop(0, S // D, zero_body, 0)
        c_v[S // 2:, :] = jnp.zeros((8, C), U32)

        for kt in range(1, KT):
            for cp in wq_copies(kt):
                cp.start()
        with jax.named_scope("small_wait"):
            for cp in small:
                cp.wait()
        sh = sh_v[...].astype(F32)
        for j in range(KS):
            par_v[j] = jnp.broadcast_to(sh[j:j + 1, :], (LANE, M)).T
        dd = dd_v[...].astype(F32).reshape(1, M)
        par_v[KS] = jnp.broadcast_to(dd, (LANE, M)).T

        def x_transpose(i):
            xt = xt_v[:, pl.ds(i * x_cols, x_cols)]
            xt = _rowcat([xt, jnp.zeros((MP // 2 - M // 2, x_cols), U32)])
            x_v[_h(i * x_cols, x_cols), :] = _u32(_bf(xt).astype(F32).T.astype(BF16))

        def q_early(kt, keep=False, jobs=()):
            first, last = kt == 0, kt == KT - 1
            n = wq_pairs(kt)
            cols = pl.ds(kt * LANE, LANE)
            if not keep:
                link[0] = None
            for j in range(H // 2):
                ws = []
                for half in range(2):
                    ev, od = (wqs_v[kt][pl.ds((2 * par + half) * n * 8 + j, n, stride=8), :]
                              for par in range(2))
                    ws.append(_repack(ev, od))
                w = _lanecat([ws[0][0], ws[1][0], ws[0][1], ws[1][1]])
                if n < TP:
                    w = _rowcat([w, jnp.zeros((TP - n, 2 * D), U32)])
                wq_v[j, pl.ds(kt * TP, TP), :] = w
                lhs = linked(x_v[_h(0, x_cols), cols])
                j0 = cfg["xs_from"]
                if jobs and j >= j0:
                    nj = H // 2 - j0
                    mine = jobs[(j - j0) * len(jobs) // nj:(j - j0 + 1) * len(jobs) // nj]
                    for k, job in enumerate(mine):
                        lhs = _pin(lhs, _opaque_zero(job()), 8 * (1 + k * 30 // len(mine)))
                d = _dot(_bf(lhs), _bf(w))
                set_link(d)
                if not first:
                    d = d + pltpu.bitcast(qacc[j], F32)
                if last:
                    d = (d * QSCALE).astype(BF16)
                    for t in range(2):
                        q_all[2 * j + t, _h(0, x_cols), :] = _u32(d[:, t * D:(t + 1) * D])
                else:
                    qacc[j] = pltpu.bitcast(d, U32)

        with jax.named_scope("x_wait"):
            x_copy(0).wait()
        x_transpose(0)
        for i in range(1, XC):
            x_copy(i).start()
        for g in range(QIT):
            for cp in w_copies(g) + (c_copies(g) if g < QIT - 1 else []):
                cp.start()
        wo_copy.start()
        a_start(0)
        a_start(1)
        with jax.named_scope("wq_wait"):
            wq_wait(0)
        q_early(0)
        with jax.named_scope("wq_wait"):
            wq_wait(1)
        q_early(1)
        with jax.named_scope("wq_wait"):
            wq_wait(2)
            wq_wait(3)
            for i in range(1, XC):
                x_copy(i).wait()
        for i in range(1, XC):
            x_transpose(i)

        def x_sums(u):
            a11, a12, a21, a22 = (
                _split(x_v[pl.ds((x_cols + rb * XH) // 2 + 8 * u, 8), cb * D:(cb + 1) * D])
                for rb in range(2) for cb in range(2))
            outs = [_add(a11, a22), _add(a21, a22), _add(a11, a12), _sub(a21, a11),
                    _sub(a12, a22)]
            for k, o in enumerate(outs):
                xs_v[k, 8 * u:8 * u + 8, :] = o
            return outs

        q_early(2, jobs=[functools.partial(x_sums, u) for u in range(XH // 16)])
        q_early(3, keep=True)

        def unpack(it, sub, j):
            g = it
            ev, od = (ws_v[g, pl.ds((par * (C // 2) + sub * TP) * 8 + j, TP, stride=8), :]
                      for par in range(2))
            lo, hi = _repack(ev, od)
            rows = pl.ds(sub * TP, TP)
            cols = pl.ds(pl.multiple_of(g * LANE, LANE), LANE)
            wkv_v[2 * j, rows, cols] = lo
            wkv_v[2 * j + 1, rows, cols] = hi
            return [lo, hi]

        def a_sums(it, u):
            r0 = jnp.clip((it - 1) * CP, 0, S // 4 - CP) + 8 * u
            src = [jnp.where(it == 0, S // 2, r0 + rb * (S // 4)) for rb in range(2)]
            r0 = pl.multiple_of(r0, 8)
            kw = C // 2
            a11, a12, a21, a22 = (
                _split(c_v[pl.ds(pl.multiple_of(src[rb], 8), 8), pl.ds(cb * kw, kw)])
                for rb in range(2) for cb in range(2))
            outs = [_add(a11, a22), _add(a21, a22), _add(a11, a12), _sub(a21, a11),
                    _sub(a12, a22)]
            for k, o in enumerate(outs):
                sa_v[k, pl.ds(r0, 8), :] = o
            return outs

        units = [functools.partial(unpack, sub=s_, j=j_)
                 for s_ in range(C // 2 // TP) for j_ in range(H // 2)]
        for u_ in range(CP // 8):
            units.insert(4 * u_ + 1, functools.partial(a_sums, u=u_))

        def q_pair(pair, todo):
            raw = lambda r, c: _lanecat([
                wq_v[pair, r * LANE:(r + 1) * LANE, pl.ds(t * D + c * LANE, LANE)]
                for t in range(2)])
            b = lambda r, c: _split(raw(r, c))
            sb = {1: _add(b(0, 0), b(1, 1)), 2: raw(0, 0), 3: _sub(b(0, 1), b(1, 1)),
                  4: _sub(b(1, 0), b(0, 0)), 5: raw(1, 1), 6: _add(b(0, 0), b(0, 1)),
                  7: _add(b(1, 0), b(1, 1))}
            n = XH // 2
            for rho in range(2):
                def sa(m):
                    if m == 3:
                        return x_v[_h(x_cols + rho * n, n), 0:D]
                    if m == 4:
                        return x_v[_h(x_cols + XH + rho * n, n), D:]
                    return xs_v[{1: 0, 2: 1, 5: 2, 6: 3, 7: 4}[m], _h(rho * n, n), :]

                def put(half, c0, c1):
                    rows = _h(x_cols + half * XH + rho * n, n)
                    for t in range(2):
                        q = _lanecat([c[:, t * LANE:(t + 1) * LANE] for c in (c0, c1)])
                        q_all[2 * pair + t, rows, :] = _u32((q * QSCALE).astype(BF16))

                p = {}
                for pos, m in enumerate((5, 1, 4, 7, 3, 2, 6)):
                    lhs = linked(sa(m))
                    nj = min(len(todo), cfg["q_jobs"][7 * rho + pos])
                    jobs = [todo.pop()(it=pair // QP) for _ in range(nj)]
                    for k, job in enumerate(jobs):
                        lhs = _pin(lhs, _opaque_zero(job), 8 * (1 + k * (n // 16 - 1) // nj))
                    p[m] = _dot(_bf(lhs), _bf(sb[m]))
                    set_link(p[m])
                    if m == 3:
                        put(0, (p[1] + p[4]) + (p[7] - p[5]), p[3] + p[5])
                put(1, p[2] + p[4], (p[1] + p[3]) + (p[6] - p[2]))

        def q_body(it, carry):
            with jax.named_scope("w_wait"):
                w_wait(it)
                for p in range(QIT - 1):
                    @pl.when(it == p + 1)
                    def _():
                        for cp in c_copies(p):
                            cp.wait()
            link[0] = None
            todo = units[::-1]
            for p in range(QP):
                q_pair(QP * it + p, todo)
            assert not todo
            return carry

        with jax.named_scope("q_loop"):
            lax.fori_loop(0, QIT, q_body, 0)
        wo_copy.wait()
        a_wait(0)

        tri = (lax.broadcasted_iota(jnp.int32, (LANE, LANE), 1)
               <= lax.broadcasted_iota(jnp.int32, (LANE, LANE), 0))

        NOUT = S // D

        def out_copy(i):
            if i >= NOUT:
                t = i - NOUT
                return pltpu.make_async_copy(
                    oa_v.at[t], out_hbm.at[:, pl.ds(t * LANE, LANE)], sem_out.at[i])
            rs = pl.ds(i * D, D)
            return pltpu.make_async_copy(
                out_v.at[rs], out_hbm.at[rs, pl.ds(AT * LANE, 2 * M - AT * LANE)], sem_out.at[i])

        body_chunks = _digits(cfg["body_chunks"])

        def b_out(k, tot):
            c0 = (k * D) % (S // 2)
            full = _rowcat([ra_t[k * D // (S // 2), AT * LANE:, c0:c0 + D], tot]).T
            out_v[k * D:(k + 1) * D, :] = full.astype(BF16)
            return full

        def head_step(h, carry):
            with jax.named_scope("step"):
                return head_step_(h, carry)

        def head_step_(h, carry):
            with_a = cfg["use_a"]

            @pl.when(h == A_STEPS)
            def _():
                for t in range(AT):
                    out_copy(NOUT + t).start()

            @pl.when(h == cfg["h0"] + 1)
            def _():
                a_wait(1)

            link[0] = None
            n2 = AR // 2
            a_rows2 = pl.ds(pl.multiple_of(jnp.minimum(h, A_STEPS - 1) * n2, n2), n2)
            a_rows = pl.ds(pl.multiple_of(jnp.minimum(h, A_STEPS - 1) * AR, AR), AR)

            kw = C // 2
            pending = []
            chains = {i: [] for i in range(nq + 1)}
            deadline = [None]

            def flush_pending(x, row):
                done = list(pending)
                del pending[:]
                if not done:
                    return x
                x = _pin(x, _opaque_zero([f for _, f in done]), row)

                @pl.when(h == H - 1)
                def _():
                    for k, _f in done:
                        out_copy(k).start()
                return x

            def a_fwd():
                kk = _bf(a_v[0, a_rows2, :]).astype(F32)
                lane = lax.broadcasted_iota(jnp.int32, (AR, LANE), 1)
                coef = [par_v[j, a_rows, :] for j in range(KS)]
                rolled = [kk] + [pltpu.roll(kk, j, 1) for j in range(1, KS)]
                vv = _bf(a_v[1, a_rows2, :]).astype(F32)
                kv_blocks = []
                for a in range(NB):
                    cs = slice(a * LANE, (a + 1) * LANE)
                    acc = rolled[0][:, cs] * coef[0]
                    for j in range(1, KS):
                        t = rolled[j][:, cs]
                        if a == 0:
                            t = jnp.where(lane >= j, t, 0.0)
                        acc = acc + t * coef[j]
                    kv_blocks.append(acc * vv[:, cs])
                hk = a_v[2, a_rows2, :]
                hk = _rowcat([hk[:, a * LANE:(a + 1) * LANE] for a in range(NB)])
                fm = _bf(f_v[...])
                hs = _dot(_bf(linked(hk)), fm)
                kv = linked(_rowcat(kv_blocks)).astype(BF16)
                xs = _dot(kv, fm)
                set_link(xs)
                return kv, xs, hs

            def a_conv(xs, hs):
                def tile(v, a, g, part):
                    r = a * AR + 8 * g
                    return v[r:r + 8, part * LANE:(part + 1) * LANE]

                z = {}
                gate = None
                width = cfg["a_width"]
                for g in range(AR // 8):
                    hr = [tile(hs, 0, g, 0)] + [
                        tile(hs, j, g, 0) - tile(hs, j - 1, g, 1) for j in range(1, NB)]
                    hi = [tile(hs, 0, g, 1)] + [
                        tile(hs, j, g, 1) + tile(hs, j - 1, g, 0) for j in range(1, NB)]
                    for c0 in range(0, NB, width):
                        for a in range(c0 + width):
                            xr, xi = tile(xs, a, g, 0), tile(xs, a, g, 1)
                            if gate is not None:
                                xr, xi = _pin(xr, gate), _pin(xi, gate)
                            for c in range(max(c0, a), c0 + width):
                                j = c - a
                                tr = xr * hr[j] - xi * hi[j]
                                ti = xr * hi[j] + xi * hr[j]
                                z[c, g] = (tr, ti) if a == 0 else (z[c, g][0] + tr, z[c, g][1] + ti)
                            gate = _opaque_zero(list(z[c0 + width - 1, g]))
                            chains[nq].append(gate)
                return z

            def a_inv(kv, z, flush=False):
                fm = _bf(f_v[...])
                ng = AR // 8
                ys = []
                for u in range(2):
                    rows = [_lanecat(z[c, g]) for g in range(u * ng // 2, (u + 1) * ng // 2)
                            for c in range(NB)]
                    lhs = linked(_rowcat(rows))
                    if flush:
                        lhs = flush_pending(lhs, 8)
                    ys.append(_dot_nt(lhs.astype(BF16), fm))
                y = _rowcat(ys)
                dd = par_v[KS, a_rows, :]
                for c in range(NB):
                    cs = slice(c * LANE, (c + 1) * LANE)
                    yc = _rowcat([y[(g * NB + c) * 8:(g * NB + c + 1) * 8, :] for g in range(ng)])
                    qq = _bf(a_v[3, a_rows2, cs]).astype(F32)
                    kvf = kv[c * AR:(c + 1) * AR, :].astype(F32)
                    c2 = (c % (NB // 2)) * LANE
                    ra_t[c // (NB // 2), a_rows, c2:c2 + LANE] = qq * (yc * (1.0 / LANE) + kvf * dd)

            def a_out():
                slab = jnp.clip(h // 4 - 1, 0, AT - 1)
                half = h % 2
                x = ra_t[half, pl.ds(pl.multiple_of(slab * LANE, LANE), LANE), :]
                xt = x.T
                dst = jnp.where(h >= A_STEPS, AT, slab)
                oa_v[dst, pl.ds(pl.multiple_of(half * (S // 2), S // 2), S // 2), :] = xt.astype(BF16)
                return xt

            def w_blk(r, c):
                return wkv_v[h, _h(r * kw, kw), pl.ds(c * LANE, LANE)]

            def one_pass(lhs, w, flush):
                lhs = linked(lhs)
                if flush:
                    lhs = flush_pending(lhs, cfg["ao_row"])
                if deadline[0] is not None:
                    if deadline[0][0] == 0:
                        lhs = _pin(lhs, deadline[0][1], cfg["ao_row"] - 8)
                        deadline[0] = None
                    else:
                        deadline[0] = (deadline[0][0] - 1, deadline[0][1])
                d = _dot(_bf(lhs), _bf(paced(w)))
                set_link(d)
                return d

            def b_op(which, m):
                raw = lambda r, c: w_blk(r, 2 * which + c)
                blk = lambda r, c: _split(raw(r, c))
                return {1: lambda: _add(blk(0, 0), blk(1, 1)),
                        2: lambda: raw(0, 0),
                        3: lambda: _sub(blk(0, 1), blk(1, 1)),
                        4: lambda: _sub(blk(1, 0), blk(0, 0)),
                        5: lambda: raw(1, 1),
                        6: lambda: _add(blk(0, 0), blk(0, 1)),
                        7: lambda: _add(blk(1, 0), blk(1, 1))}[m]()

            def a_op(m, rho):
                rs = _h(rho * tq, tq)
                if m == 3:
                    return c_v[rs, 0:kw]
                if m == 4:
                    return c_v[_h(S // 2 + rho * tq, tq), kw:]
                return sa_v[{1: 0, 2: 1, 5: 2, 6: 3, 7: 4}[m], rs, :]

            b_cache, prod = {}, {}

            def kv_proj(which, blk, flush):
                rho = blk % 2
                for k, m in enumerate(_digits(cfg["kv_top" if blk < 2 else "kv_bot"])):
                    if (which, m) not in b_cache:
                        b_cache[which, m] = b_op(which, m)
                    prod[which, m, rho] = one_pass(a_op(m, rho), b_cache[which, m], k == flush)
                p = lambda m: prod[which, m, rho]
                if blk < 2:
                    return [(p(1) + p(4)) + (p(7) - p(5)), p(3) + p(5)]
                return [p(2) + p(4), (p(1) + p(3)) + (p(6) - p(2))]

            def k_proj(blk, flush=-1):
                k = kv_proj(0, blk, flush)
                k_s[_h(blk * tq, tq), :] = _u32(_lanecat(k).astype(BF16))
                if blk < nq - 1:
                    b = lambda r, c: k[r][c * D:(c + 1) * D, :]
                    sums = [b(0, 0) + b(1, 1), b(0, 1) - b(1, 1), b(1, 0) - b(0, 0),
                            b(0, 0) + b(0, 1), b(1, 0) + b(1, 1)]
                    for n, x in enumerate(sums):
                        kb_s[n, _h(blk * D, D), :] = _u32(x.astype(BF16))

            def v_proj(blk, flush=-1):
                v = kv_proj(1, blk, flush)
                v_s[_h(blk * tq, tq), :] = _u32(_lanecat(v).astype(BF16))
                if blk < nq - 1:
                    b = lambda r, c: v[c][r * D:(r + 1) * D, :]
                    sums = [b(0, 0) + b(1, 1), b(0, 1) - b(1, 1), b(1, 0) - b(0, 0),
                            b(0, 0) + b(0, 1), b(1, 0) + b(1, 1)]
                    for k, x in enumerate(sums):
                        vb_s[k, _h(blk * D, D), :] = _u32(x.astype(BF16))

            def qk(i, dep=None, flush=False):
                r0 = i * tq
                off = None
                if i > 0:
                    raw = lambda r, c: q_all[h, _h(r0 + r * D, D), c * LANE:(c + 1) * LANE]
                    a = lambda r, c: _split(raw(r, c))
                    sa = {1: _add(a(0, 0), a(1, 1)), 2: _add(a(1, 0), a(1, 1)), 3: raw(0, 0),
                          4: raw(1, 1), 5: _add(a(0, 0), a(0, 1)), 6: _sub(a(1, 0), a(0, 0)),
                          7: _sub(a(0, 1), a(1, 1))}

                    def sb(m, j, t):
                        if m in (2, 5):
                            c = 0 if m == 2 else 1
                            rows = _h(j * tq + c * D + t * LANE, LANE)
                            return k_s[rows, c * LANE:(c + 1) * LANE]
                        n = {1: 0, 3: 1, 4: 2, 6: 3, 7: 4}[m]
                        return kb_s[n, _h(j * D + t * LANE, LANE), :]

                    top, bot, due = {}, {}, []
                    n_dot = 0
                    for j in range(i):
                        for t in range(2):
                            p = {}
                            for n, m in enumerate(_digits(cfg["s_ord"])):
                                lhs = linked(sa[m])
                                if due and n == cfg["s_due"]:
                                    lhs = _pin(lhs, due.pop(), cfg["s_row"])
                                p[m] = _dot_nt(_bf(lhs), _bf(sb(m, j, t)))
                                n_dot += 1
                                if n_dot % 4 == 0:
                                    set_link(p[m], cfg["s_link"])
                            top[4 * j + t] = (p[1] + p[4]) + (p[7] - p[5])
                            top[4 * j + 2 + t] = p[3] + p[5]
                            bot[4 * j + t] = p[2] + p[4]
                            bot[4 * j + 2 + t] = (p[1] + p[3]) + (p[6] - p[2])
                            due.append(_opaque_zero(
                                [x[4 * j + c + t] for x in (top, bot) for c in (0, 2)]))
                    off = _rowcat([_lanecat([x[c] for c in range(4 * i)]) for x in (top, bot)])
                q = linked(q_all[h, _h(r0, tq), :])
                if off is not None:
                    q = _pin(q, due.pop(), cfg["ao_row"] - 8)
                if dep is not None:
                    q = _pin(q, _opaque_zero([dep]), cfg["ao_row"])
                main = _dot_nt(_bf(q), _bf(k_s[_h(r0, LANE), :]))
                parts = [main if off is None else _lanecat([off, main])]
                for j in range(1, nsub):
                    q = linked(q_all[h, _h(r0 + LANE * j, tq - LANE * j), :])
                    if flush and j == cfg["q_pin"]:
                        q = flush_pending(q, 8)
                    parts.append(_dot_nt(_bf(q), _bf(k_s[_h(r0 + LANE * j, LANE), :])))
                set_link(parts[2], cfg["link_part"], main)
                return parts

            def exps(i, parts):
                sas, mbs = [], []
                for a in range(nsub):
                    blocks = [parts[j][LANE * (a - j):LANE * (a - j + 1), :] for j in range(a + 1)]
                    last = blocks[-1]
                    w = last.shape[1]
                    dg = jnp.where(tri, last[:, w - LANE:], NEG)
                    blocks[-1] = dg if w == LANE else _lanecat([last[:, :w - LANE], dg])
                    sas.append(_lanecat(blocks))
                    lane_max = functools.reduce(jnp.maximum, [
                        sas[a][:, t:t + LANE] for t in range(0, sas[a].shape[1], LANE)])
                    mx = jnp.max(lane_max, axis=1, keepdims=True)
                    if i > 0:
                        mx = mx + jnp.log2(jnp.sum(jnp.exp2(lane_max - mx), axis=1, keepdims=True))
                    mbs.append(jnp.broadcast_to(mx, (LANE, LANE)))
                chain = _opaque_zero([b[b.shape[0] - 8:, b.shape[1] - LANE:] for b in parts])
                pg, psums = {}, {}
                for r in range(0, tq // 2, 8):
                    for row in (r, r + tq // 2):
                        a, g = divmod(row, LANE)
                        mg = _pin(mbs[a][g:g + 8, :], chain)
                        pg[row] = [jnp.exp2(sas[a][g:g + 8, t:t + LANE] - mg)
                                   for t in range(0, sas[a].shape[1], LANE)]
                        psums[row] = functools.reduce(jnp.add, pg[row])
                        chain = _opaque_zero([psums[row]])
                        chains[i].append(chain)
                return pg, psums

            def softmax(i, pg, psums):
                r0 = i * tq
                pd, pa = pd_s.at[i % 2], pa_s[i % 2]
                first = lambda x, c=0: _pin(x, link[0], 0, c).astype(BF16)
                nt0 = r0 // LANE
                ls = []
                for a in range(nsub):
                    rows = range(LANE * a, LANE * (a + 1), 8)
                    ls.append(jnp.sum(_rowcat([psums[r] for r in rows]), axis=1, keepdims=True))
                    pd[LANE * a:LANE * (a + 1), 0:LANE * (a + 1)] = first(
                        _rowcat([_lanecat(pg[r][nt0:]) for r in rows]), LANE * a)
                if i > 0:
                    quad = lambda rh, ch: _rowcat([
                        _lanecat([pg[rh * (tq // 2) + r][4 * j + 2 * ch + t]
                                  for j in range(i) for t in range(2)])
                        for r in range(0, tq // 2, 8)])
                    a11, a12, a21, a22 = quad(0, 0), quad(0, 1), quad(1, 0), quad(1, 1)
                    ops = [a11 + a22, a21 + a22, a11, a22, a11 + a12, a21 - a11, a12 - a22]
                    for m, x in enumerate(ops):
                        if i == 3:
                            x = _pin(x, link[0], 0, 2 * D)
                        pa[m, :, 0:i * D] = first(x)
                return ls

            def pv(i, ls, flush=-1):
                r0 = i * tq
                pd, pa = pd_s.at[i % 2], pa_s[i % 2]
                off = None
                if i > 0:
                    def b_rows(m, j0, j1):
                        if m in (2, 5):
                            q = 0 if m == 2 else 1
                            return _rowcat([
                                v_s[_h(j * tq + q * D, D), q * LANE:(q + 1) * LANE]
                                for j in range(j0, j1)])
                        k = {1: 0, 3: 1, 4: 2, 6: 3, 7: 4}[m]
                        return vb_s[k, _h(j0 * D, (j1 - j0) * D), :]

                    p, n_dot = {}, 0
                    for j0, j1 in {1: [(0, 1)], 2: [(0, 2)], 3: [(0, 2), (2, 3)]}[i]:
                        for m in _digits(cfg["p_ord"]):
                            cols = slice(j0 * D, j1 * D)
                            rhs = b_rows(m, j0, j1)
                            if n_dot == flush:
                                rhs = flush_pending(rhs, 0)
                            rhs = _bf(rhs)
                            n_dot += 1
                            if j1 - j0 == 1 and m == cfg["p_ord"] % 10:
                                d = _rowcat([_dot(pa[m - 1, r:r + LANE, cols], rhs)
                                             for r in (0, LANE)])
                            else:
                                d = _dot(pa[m - 1, :, cols], rhs)
                            p[m] = d if m not in p else p[m] + d
                    off = _rowcat([
                        _lanecat([(p[1] + p[4]) + (p[7] - p[5]), p[3] + p[5]]),
                        _lanecat([p[2] + p[4], (p[1] + p[3]) + (p[6] - p[2])])])
                ctx = []
                for j in range(nsub):
                    c0 = LANE * j
                    ctx.append(_dot(pd[c0:, c0:c0 + LANE], _bf(v_s[_h(r0 + c0, LANE), :])))
                set_link(ctx[2], cfg["link_part"], ctx[0])
                cs = []
                for a in range(nsub):
                    sl = lambda j: slice(LANE * (a - j), LANE * (a - j + 1))
                    r = pl.reciprocal(ls[a], approx=True)
                    r = r * (2.0 - ls[a] * r)
                    terms = [ctx[j][sl(j)] for j in range(a + 1)]
                    if off is not None:
                        terms.append(off[sl(0)])
                    cs.append(functools.reduce(jnp.add, terms) * r)
                return _rowcat(cs)

            wo_cache = {}

            def oproj(i, ctx):
                mh = M // 4
                raw = lambda r, c: wo_v[h, r * mh:(r + 1) * mh, c * LANE:(c + 1) * LANE]
                a = lambda r, c: _split(raw(r, c))
                a_ops = {1: lambda: _add(a(0, 0), a(1, 1)), 2: lambda: _add(a(1, 0), a(1, 1)),
                         3: lambda: raw(0, 0), 4: lambda: raw(1, 1),
                         5: lambda: _add(a(0, 0), a(0, 1)), 6: lambda: _sub(a(1, 0), a(0, 0)),
                         7: lambda: _sub(a(0, 1), a(1, 1))}
                b = lambda r, c: ctx[c * D:(c + 1) * D, r * LANE:(r + 1) * LANE]
                b_ops = {1: lambda: b(0, 0) + b(1, 1), 2: lambda: b(0, 0),
                         3: lambda: b(0, 1) - b(1, 1), 4: lambda: b(1, 0) - b(0, 0),
                         5: lambda: b(1, 1), 6: lambda: b(0, 0) + b(0, 1),
                         7: lambda: b(1, 0) + b(1, 1)}
                p = {}
                order = _digits(cfg["o_ord"])
                mm = M // 2
                old = lambda r, c: rb_t[2 * i + c, r * mm:(r + 1) * mm, :]
                terms = {(0, 0): (1, 4, -5, 7), (0, 1): (3, 5), (1, 0): (2, 4), (1, 1): (1, -2, 3, 6)}

                def total(q):
                    acc = old(*q)
                    for m in sorted(terms[q], key=lambda m: order.index(abs(m))):
                        acc = acc + p[m] if m > 0 else acc - p[-m]
                    return acc

                for n, m in enumerate(order):
                    if m not in wo_cache:
                        wo_cache[m] = a_ops[m]()
                    rhs = b_ops[m]().astype(BF16)
                    if n == cfg["o_half"]:
                        lhs = [linked(wo_cache[m][r:r + mh // 2]) for r in (0, mh // 2)]
                        halves = [_dot_nt(_bf(x), rhs) for x in lhs]
                        p[m] = _rowcat(halves)
                        set_link(halves[1], 0)
                    else:
                        p[m] = _dot_nt(_bf(linked(wo_cache[m])), rhs)
                        if (n - (n > cfg["o_half"])) % 2 == 1:
                            set_link(p[m], cfg["o_link"])
                for c in range(2):
                    k = 2 * i + c
                    tot = _rowcat([total((r, c)) for r in range(2)])
                    rb_t[k] = tot
                    if k + 1 in body_chunks:
                        pending.append((k, b_out(k, tot)))

            st = {}
            for op in cfg["seq"].split():
                op, _, dl = op.partition("@")
                if dl:
                    ch = chains[int(dl[0])]
                    deadline[0] = (int(dl[1]), ch[int(dl[2:]) * len(ch) // 16 - 1])
                op, _, fl = op.partition("!")
                fl = int(fl) if fl else -1
                kind, i = op[0], int(op[1:] or 0)
                if kind == "K":
                    k_proj(i, fl)
                elif kind == "V":
                    v_proj(i, fl)
                elif kind == "Q":
                    st["e", i] = exps(
                        i, qk(i, a_out() if i == cfg["ao_at"] else None, fl >= 0))
                elif kind == "P":
                    st["ctx", i] = pv(i, softmax(i, *st["e", i]), fl)
                elif kind == "O":
                    oproj(i, st["ctx", i])
                elif kind == "F" and with_a:
                    st["kv"], xs, hs = a_fwd()
                    st["z"] = a_conv(xs, hs)
                elif kind == "I" and with_a:
                    a_inv(st["kv"], st["z"], fl >= 0)
            assert not pending and deadline[0] is None
            return carry

        with jax.named_scope("loop_a"):
            lax.fori_loop(cfg["h0"], H, head_step, 0)
        with jax.named_scope("tail"):
            for i in [k for k in range(NOUT) if k + 1 not in body_chunks]:
                b_out(i, rb_t[i])
                out_copy(i).start()
            for i in range(NOUT + AT):
                out_copy(i).wait()

    scratch = [
        pltpu.VMEM((4, M // 2, S), U32),
        pltpu.VMEM((KS, M), BF16),
        pltpu.VMEM((M,), BF16),
        pltpu.VMEM((KS + 1, M, LANE), F32),
        pltpu.VMEM((LANE // 2, 2 * LANE), U32),
        pltpu.VMEM((M // 2, S), U32),
        pltpu.VMEM((S // 2, MP), U32),
        pltpu.VMEM((5, XH // 2, D), U32),
        pltpu.VMEM((S // 2 + 8, C), U32),
        [pltpu.VMEM((4 * min(TP, M // 2 - kt * TP) * 8, LANE), U32)
         for kt in range(KT)],
        pltpu.VMEM((H // 2, MP // 2, 2 * D), U32),
        pltpu.VMEM((H // 2, x_cols, 2 * D), U32),
        pltpu.VMEM((QIT, C * 8, LANE), U32),
        pltpu.VMEM((H, C // 2, 2 * D), U32),
        pltpu.VMEM((H, M // 2, D), U32),
        pltpu.VMEM((H, S // 2, D), U32),
        pltpu.VMEM((S // 2, D), U32),
        pltpu.VMEM((S // 2, D), U32),
        pltpu.VMEM((5, (nq - 1) * D // 2, LANE), U32),
        pltpu.VMEM((5, (nq - 1) * D // 2, LANE), U32),
        pltpu.VMEM((2, tq, tq), BF16),
        [pltpu.VMEM((7, tq // 2, n * D), BF16) for n in (2, 3)],
        pltpu.VMEM((2, M, S // 2), F32),
        pltpu.VMEM((S // D, M, D), F32),
        pltpu.VMEM((AT + 1, S, LANE), BF16),
        pltpu.VMEM((S, 2 * M - AT * LANE), BF16),
        pltpu.SemaphoreType.DMA((XC,)),
        pltpu.SemaphoreType.DMA((KT,)),
        pltpu.SemaphoreType.DMA((QIT,)),
        pltpu.SemaphoreType.DMA((QIT,)),
        pltpu.SemaphoreType.DMA((2,)),
        pltpu.SemaphoreType.DMA((3,)),
        pltpu.SemaphoreType.DMA((S // D + AT,)),
    ]
    return kernel, scratch


_DEFAULT = dict(
    tq=512, a_width=16, ao_at=1, ao_row=240, link_back=176, link_part=32, pace_row=32,
    pace_step=32, use_a=1, h0=0, body_chunks=123456, kv_top=51473, kv_bot=26, s_ord=5147236,
    o_ord=5241736, p_ord=1234567, o_link=32, o_half=6, q_jobs=(2, 4, 4, 4, 1, 3, 1, 3, 5, 6, 6, 1, 2, 1), xs_from=3, s_link=48, s_due=6, s_row=120, q_pin=2,
    seq="K0 Q0 K1 Q1 V0 F P0 K2@1112 Q2 O0 V1!4 P1 K3@2116 Q3 O1 V2@4016 P2!6 V3@3116 O2 P3!13 I O3")


def _build(**kw):
    cfg = dict(_DEFAULT)
    cfg.update(kw)
    kernel, scratch = _make_kernel(cfg)

    def run(A_q, A_k, A_v, A_shift_k, A_ssm_k, A_ssm_D, B_x, B_c_kv, B_w_q, B_w_uk,
            B_w_uv, B_w_o):
        tr = lambda a: jnp.swapaxes(a, 1, 2).reshape(M, S)
        args = (
            tr(A_q), tr(A_k), tr(A_v), A_shift_k.T, A_ssm_k, A_ssm_D, tr(B_x),
            B_c_kv.reshape(S, C),
            B_w_q.reshape(M // 2, 2 * H, D), B_w_uk.reshape(C // 2, 2 * H, D),
            B_w_uv.reshape(C // 2, 2 * H, D),
            jnp.swapaxes(B_w_o, 1, 2),
        )
        out = pl.pallas_call(
            kernel,
            in_specs=[pl.BlockSpec(memory_space=pl.ANY)] * len(args),
            out_specs=pl.BlockSpec(memory_space=pl.ANY),
            out_shape=jax.ShapeDtypeStruct((S, 2 * M), BF16),
            scratch_shapes=scratch,
            compiler_params=pltpu.CompilerParams(
                vmem_limit_bytes=126 * 1024 * 1024,
                disable_bounds_checks=True),
        )(*args)
        return out.reshape(1, S, 2 * M)

    return run


_run = _build()


@jax.jit
def pallas_concat_heads__ssm_conv_h3__compressed_kv_cla__prompt_kernel(
    A_q: jax.Array,
    A_k: jax.Array,
    A_v: jax.Array,
    A_shift_k: jax.Array,
    A_ssm_k: jax.Array,
    A_ssm_D: jax.Array,
    B_x: jax.Array,
    B_c_kv: jax.Array,
    B_w_q: jax.Array,
    B_w_uk: jax.Array,
    B_w_uv: jax.Array,
    B_w_o: jax.Array,
):
    return _run(A_q, A_k, A_v, A_shift_k, A_ssm_k, A_ssm_D, B_x, B_c_kv, B_w_q,
                B_w_uk, B_w_uv, B_w_o)
```

```python
import functools

import jax
import jax.numpy as jnp
from jax import lax
import jax.experimental.pallas as pl
import jax.experimental.pallas.tpu as pltpu

F32 = jnp.float32
BF16 = jnp.bfloat16
U32 = jnp.uint32

S = 2048
M = 448
MP = 512
C = 1024
H = 16
D = 256
KS = 4
LANE = 128
NB = S // LANE
AR = 32
A_STEPS = M // AR
LOG2E = 1.4426950408889634
QSCALE = D ** -0.5 * LOG2E
NEG = -1e30

NT = (((1,), (1,)), ((), ()))


def _dot(a, b):
    return jnp.dot(a, b, preferred_element_type=F32)


def _dot_nt(a, b):
    return lax.dot_general(a, b, NT, preferred_element_type=F32)


def _bf(x):
    return pltpu.bitcast(x, BF16)


def _u32(x):
    return pltpu.bitcast(x, U32)


def _h(r0, n):
    return pl.ds(r0 // 2, n // 2)


def _repack(ev, od):
    lo = (ev & jnp.uint32(0xFFFF)) | (od << 16)
    hi = (ev >> 16) | (od & jnp.uint32(0xFFFF0000))
    return lo, hi


def _split(w):
    return (pltpu.bitcast(w << 16, F32), pltpu.bitcast(w & jnp.uint32(0xFFFF0000), F32))


def _join(lo, hi):
    half = jnp.uint32(0x8000)
    lo = (pltpu.bitcast(lo, U32) + half) >> 16
    hi = (pltpu.bitcast(hi, U32) + half) & jnp.uint32(0xFFFF0000)
    return lo | hi


def _add(a, b):
    return _join(a[0] + b[0], a[1] + b[1])


def _sub(a, b):
    return _join(a[0] - b[0], a[1] - b[1])


def _opaque_zero(vals):
    acc = None
    for v in vals:
        b = v if v.dtype == U32 else pltpu.bitcast(v, U32)
        for r in range(0, b.shape[0], 8):
            for c in range(0, b.shape[1], LANE):
                t = b[r:r + 8, c:c + LANE]
                acc = t if acc is None else acc | t
    return jnp.minimum((acc >> 1).astype(jnp.int32), 0)


def _pin(x, zero, r=0, c=0):
    t = pltpu.bitcast(pltpu.bitcast(x[r:r + 8, c:c + LANE], jnp.int32) + zero, x.dtype)
    row = ([x[r:r + 8, :c]] if c > 0 else []) + [t] + (
        [x[r:r + 8, c + LANE:]] if c + LANE < x.shape[1] else [])
    row = jnp.concatenate(row, axis=1) if len(row) > 1 else row[0]
    col = ([x[:r, :]] if r > 0 else []) + [row] + ([x[r + 8:, :]] if r + 8 < x.shape[0] else [])
    return jnp.concatenate(col, axis=0) if len(col) > 1 else col[0]


def _digits(n):
    return [int(c) for c in str(n)]


def _rowcat(xs):
    return jnp.concatenate(xs, axis=0) if len(xs) > 1 else xs[0]


def _lanecat(xs):
    return jnp.concatenate(xs, axis=1) if len(xs) > 1 else xs[0]


def _make_kernel(cfg):
    tq = cfg["tq"]
    nq = S // tq
    nsub = tq // LANE
    KT = MP // LANE
    TP = LANE // 2
    XC = 4
    x_cols = S // XC
    QP = 2
    QIT = H // 2 // QP
    XH = (S - x_cols) // 2
    CP = 176
    AT = 3

    def kernel(aq_hbm, ak_hbm, av_hbm, sh_hbm, ssm_hbm, dd_hbm, x_hbm, c_hbm,
               wq_hbm, wk_hbm, wv_hbm, wo_hbm,
               out_hbm,
               a_v, sh_v, dd_v, par_v, f_v,
               xt_v, x_v, xs_v, c_v, wqs_v, wq_v, qacc, ws_v, wkv_v, wo_v,
               q_all, k_s, v_s, kb_s, vb_s, pd_s, pa_s, ra_t, rb_t, oa_v, out_v,
               sem_x, sem_wq, sem_w, sem_c, sem_s, sem_a, sem_out):
        x32, c32, wq32, wk32, wv32, wo32 = (
            r.bitcast(U32) for r in (x_hbm, c_hbm, wq_hbm, wk_hbm, wv_hbm, wo_hbm))
        a32 = [r.bitcast(U32) for r in (ak_hbm, av_hbm, ssm_hbm, aq_hbm)]

        sa_v = qacc

        def x_copy(i):
            cs = pl.ds(i * x_cols, x_cols)
            return pltpu.make_async_copy(x32.at[:, cs], xt_v.at[:, cs], sem_x.at[i])

        def wq_pairs(kt):
            return min(TP, M // 2 - kt * TP)

        def wq_copies(kt):
            n = wq_pairs(kt)
            dst = wqs_v[kt].reshape(4, n, 8, LANE)
            return [pltpu.make_async_copy(
                wq32.at[pl.ds(kt * TP, n), pl.ds(8 * (k // 2), 8), pl.ds((k % 2) * LANE, LANE)],
                dst.at[k], sem_wq.at[kt]) for k in range(4)]

        def wq_wait(kt):
            pltpu.make_async_copy(wqs_v[kt], wqs_v[kt], sem_wq.at[kt]).wait()

        def w_copies(g):
            dst = ws_v.reshape(8, C // 2, 8, LANE)
            src = (wk32, wv32)[g // 2]
            return [pltpu.make_async_copy(
                src.at[:, pl.ds(8 * par, 8), pl.ds((g % 2) * LANE, LANE)],
                dst.at[2 * g + par], sem_w.at[g]) for par in range(2)]

        def w_wait(g):
            pltpu.make_async_copy(ws_v.at[g], ws_v.at[g], sem_w.at[g]).wait()

        c_bounds = [0, CP, 2 * CP, S // 4]

        def c_copies(p):
            r0, n = c_bounds[p], c_bounds[p + 1] - c_bounds[p]
            return [pltpu.make_async_copy(c32.at[rs], c_v.at[rs], sem_c.at[p])
                    for rs in (pl.ds(r0, n), pl.ds(S // 4 + r0, n))]

        wo_copy = pltpu.make_async_copy(wo32, wo_v, sem_a.at[0])

        a_parts = [pl.ds(0, AR // 2), pl.ds(AR // 2, M // 2 - AR // 2)]

        def a_start(part):
            rs = a_parts[part]
            for k in range(4):
                pltpu.make_async_copy(
                    a32[k].at[rs], a_v.at[k, rs], sem_a.at[1 + part]).start()

        def a_wait(part):
            view = a_v.at[:, a_parts[part]]
            pltpu.make_async_copy(view, view, sem_a.at[1 + part]).wait()

        small = [pltpu.make_async_copy(sh_hbm, sh_v, sem_s.at[0]),
                 pltpu.make_async_copy(dd_hbm, dd_v, sem_s.at[1])]

        link = [None]
        pace = [None]

        def set_link(res, row=None, pacer=None):
            if row is None:
                row = res.shape[0] - cfg["link_back"]
            link[0] = _opaque_zero([res[row:row + 8, res.shape[1] - LANE:]])
            pace[0] = res if pacer is None else pacer

        def linked(x):
            return x if link[0] is None else _pin(x, link[0])

        def paced(w):
            res = pace[0]
            if res is None or link[0] is None or not cfg["pace_step"]:
                return w
            rows = []
            r0, step = cfg["pace_row"], cfg["pace_step"]
            if res.shape[0] < 400:
                r0, step = 0, 8
            if res.shape[0] < 200:
                return w
            zs = [_opaque_zero([res[r:r + 8, res.shape[1] - LANE:]])
                  for r in range(r0, r0 + 8 * step, step)]
            for r in range(0, w.shape[0], 8):
                z = zs[7 - (r // 8) % 8]
                t = pltpu.bitcast(w[r:r + 8, :], jnp.int32)
                rows.append(pltpu.bitcast(t + _lanecat([z] * (w.shape[1] // LANE)), U32))
            return _rowcat(rows)

        for cp in small:
            cp.start()
        x_copy(0).start()
        for cp in wq_copies(0):
            cp.start()

        def zero_body(k, carry):
            n = LANE // (S // D)
            bi = lax.broadcasted_iota(jnp.int32, (n, LANE), 0) + k * n
            mi = lax.broadcasted_iota(jnp.int32, (n, LANE), 1)
            ph = ((4 * mi + 1) * bi) & 511
            ang = ph.astype(F32) * (2.0 * 3.141592653589793 / 512.0)
            rs = pl.ds(pl.multiple_of(k * (n // 2), n // 2), n // 2)
            f_v[rs, 0:LANE] = _u32(jnp.cos(ang).astype(BF16))
            f_v[rs, LANE:] = _u32((-jnp.sin(ang)).astype(BF16))

            rb_t[k] = jnp.zeros((M, D), F32)
            cs = pl.ds(pl.multiple_of((k % 4) * D, D), D)
            ra_t[k // 4, 0:LANE, cs] = jnp.zeros((LANE, D), F32)
            ra_t[k // 4, AT * LANE:, cs] = jnp.zeros((M - AT * LANE, D), F32)
            return carry

        lax.fori_loop(0, S // D, zero_body, 0)
        c_v[S // 2:, :] = jnp.zeros((8, C), U32)

        for kt in range(1, KT):
            for cp in wq_copies(kt):
                cp.start()
        with jax.named_scope("small_wait"):
            for cp in small:
                cp.wait()
        sh = sh_v[...].astype(F32)
        for j in range(KS):
            par_v[j] = jnp.broadcast_to(sh[j:j + 1, :], (LANE, M)).T
        dd = dd_v[...].astype(F32).reshape(1, M)
        par_v[KS] = jnp.broadcast_to(dd, (LANE, M)).T

        def x_transpose(i):
            xt = xt_v[:, pl.ds(i * x_cols, x_cols)]
            xt = _rowcat([xt, jnp.zeros((MP // 2 - M // 2, x_cols), U32)])
            x_v[_h(i * x_cols, x_cols), :] = _u32(_bf(xt).astype(F32).T.astype(BF16))

        def q_early(kt, keep=False, jobs=()):
            first, last = kt == 0, kt == KT - 1
            n = wq_pairs(kt)
            cols = pl.ds(kt * LANE, LANE)
            if not keep:
                link[0] = None
            for j in range(H // 2):
                ws = []
                for half in range(2):
                    ev, od = (wqs_v[kt][pl.ds((2 * par + half) * n * 8 + j, n, stride=8), :]
                              for par in range(2))
                    ws.append(_repack(ev, od))
                w = _lanecat([ws[0][0], ws[1][0], ws[0][1], ws[1][1]])
                if n < TP:
                    w = _rowcat([w, jnp.zeros((TP - n, 2 * D), U32)])
                wq_v[j, pl.ds(kt * TP, TP), :] = w
                lhs = linked(x_v[_h(0, x_cols), cols])
                j0 = cfg["xs_from"]
                if jobs and j >= j0:
                    nj = H // 2 - j0
                    mine = jobs[(j - j0) * len(jobs) // nj:(j - j0 + 1) * len(jobs) // nj]
                    for k, job in enumerate(mine):
                        lhs = _pin(lhs, _opaque_zero(job()), 8 * (1 + k * 30 // len(mine)))
                d = _dot(_bf(lhs), _bf(w))
                set_link(d)
                if not first:
                    d = d + pltpu.bitcast(qacc[j], F32)
                if last:
                    d = (d * QSCALE).astype(BF16)
                    for t in range(2):
                        q_all[2 * j + t, _h(0, x_cols), :] = _u32(d[:, t * D:(t + 1) * D])
                else:
                    qacc[j] = pltpu.bitcast(d, U32)

        with jax.named_scope("x_wait"):
            x_copy(0).wait()
        x_transpose(0)
        for i in range(1, XC):
            x_copy(i).start()
        for g in range(QIT):
            for cp in w_copies(g) + (c_copies(g) if g < QIT - 1 else []):
                cp.start()
        wo_copy.start()
        a_start(0)
        a_start(1)
        with jax.named_scope("wq_wait"):
            wq_wait(0)
        q_early(0)
        with jax.named_scope("wq_wait"):
            wq_wait(1)
        q_early(1)
        with jax.named_scope("wq_wait"):
            wq_wait(2)
            wq_wait(3)
            for i in range(1, XC):
                x_copy(i).wait()
        for i in range(1, XC):
            x_transpose(i)

        def x_sums(u):
            a11, a12, a21, a22 = (
                _split(x_v[pl.ds((x_cols + rb * XH) // 2 + 8 * u, 8), cb * D:(cb + 1) * D])
                for rb in range(2) for cb in range(2))
            outs = [_add(a11, a22), _add(a21, a22), _add(a11, a12), _sub(a21, a11),
                    _sub(a12, a22)]
            for k, o in enumerate(outs):
                xs_v[k, 8 * u:8 * u + 8, :] = o
            return outs

        q_early(2, jobs=[functools.partial(x_sums, u) for u in range(XH // 16)])
        q_early(3, keep=True)

        def unpack(it, sub, j):
            g = it
            ev, od = (ws_v[g, pl.ds((par * (C // 2) + sub * TP) * 8 + j, TP, stride=8), :]
                      for par in range(2))
            lo, hi = _repack(ev, od)
            rows = pl.ds(sub * TP, TP)
            cols = pl.ds(pl.multiple_of(g * LANE, LANE), LANE)
            wkv_v[2 * j, rows, cols] = lo
            wkv_v[2 * j + 1, rows, cols] = hi
            return [lo, hi]

        def a_sums(it, u):
            r0 = jnp.clip((it - 1) * CP, 0, S // 4 - CP) + 8 * u
            src = [jnp.where(it == 0, S // 2, r0 + rb * (S // 4)) for rb in range(2)]
            r0 = pl.multiple_of(r0, 8)
            kw = C // 2
            a11, a12, a21, a22 = (
                _split(c_v[pl.ds(pl.multiple_of(src[rb], 8), 8), pl.ds(cb * kw, kw)])
                for rb in range(2) for cb in range(2))
            outs = [_add(a11, a22), _add(a21, a22), _add(a11, a12), _sub(a21, a11),
                    _sub(a12, a22)]
            for k, o in enumerate(outs):
                sa_v[k, pl.ds(r0, 8), :] = o
            return outs

        units = [functools.partial(unpack, sub=s_, j=j_)
                 for s_ in range(C // 2 // TP) for j_ in range(H // 2)]
        for u_ in range(CP // 8):
            units.insert(4 * u_ + 1, functools.partial(a_sums, u=u_))

        def q_pair(pair, todo):
            raw = lambda r, c: _lanecat([
                wq_v[pair, r * LANE:(r + 1) * LANE, pl.ds(t * D + c * LANE, LANE)]
                for t in range(2)])
            b = lambda r, c: _split(raw(r, c))
            sb = {1: _add(b(0, 0), b(1, 1)), 2: raw(0, 0), 3: _sub(b(0, 1), b(1, 1)),
                  4: _sub(b(1, 0), b(0, 0)), 5: raw(1, 1), 6: _add(b(0, 0), b(0, 1)),
                  7: _add(b(1, 0), b(1, 1))}
            n = XH // 2
            for rho in range(2):
                def sa(m):
                    if m == 3:
                        return x_v[_h(x_cols + rho * n, n), 0:D]
                    if m == 4:
                        return x_v[_h(x_cols + XH + rho * n, n), D:]
                    return xs_v[{1: 0, 2: 1, 5: 2, 6: 3, 7: 4}[m], _h(rho * n, n), :]

                def put(half, c0, c1):
                    rows = _h(x_cols + half * XH + rho * n, n)
                    for t in range(2):
                        q = _lanecat([c[:, t * LANE:(t + 1) * LANE] for c in (c0, c1)])
                        q_all[2 * pair + t, rows, :] = _u32((q * QSCALE).astype(BF16))

                p = {}
                for pos, m in enumerate((5, 1, 4, 7, 3, 2, 6)):
                    lhs = linked(sa(m))
                    nj = min(len(todo), cfg["q_jobs"][7 * rho + pos])
                    jobs = [todo.pop()(it=pair // QP) for _ in range(nj)]
                    for k, job in enumerate(jobs):
                        lhs = _pin(lhs, _opaque_zero(job), 8 * (1 + k * (n // 16 - 1) // nj))
                    p[m] = _dot(_bf(lhs), _bf(sb[m]))
                    set_link(p[m])
                    if m == 3:
                        put(0, (p[1] + p[4]) + (p[7] - p[5]), p[3] + p[5])
                put(1, p[2] + p[4], (p[1] + p[3]) + (p[6] - p[2]))

        def q_body(it, carry):
            with jax.named_scope("w_wait"):
                w_wait(it)
                for p in range(QIT - 1):
                    @pl.when(it == p + 1)
                    def _():
                        for cp in c_copies(p):
                            cp.wait()
            link[0] = None
            todo = units[::-1]
            for p in range(QP):
                q_pair(QP * it + p, todo)
            assert not todo
            return carry

        with jax.named_scope("q_loop"):
            lax.fori_loop(0, QIT, q_body, 0)
        wo_copy.wait()
        a_wait(0)

        tri = (lax.broadcasted_iota(jnp.int32, (LANE, LANE), 1)
               <= lax.broadcasted_iota(jnp.int32, (LANE, LANE), 0))

        NOUT = S // D

        def out_copy(i):
            if i >= NOUT:
                t = i - NOUT
                return pltpu.make_async_copy(
                    oa_v.at[t], out_hbm.at[:, pl.ds(t * LANE, LANE)], sem_out.at[i])
            rs = pl.ds(i * D, D)
            return pltpu.make_async_copy(
                out_v.at[rs], out_hbm.at[rs, pl.ds(AT * LANE, 2 * M - AT * LANE)], sem_out.at[i])

        body_chunks = _digits(cfg["body_chunks"])

        def b_out(k, tot):
            c0 = (k * D) % (S // 2)
            full = _rowcat([ra_t[k * D // (S // 2), AT * LANE:, c0:c0 + D], tot]).T
            out_v[k * D:(k + 1) * D, :] = full.astype(BF16)
            return full

        def head_step(h, carry):
            with jax.named_scope("step"):
                return head_step_(h, carry)

        def head_step_(h, carry):
            with_a = cfg["use_a"]

            @pl.when(h == A_STEPS)
            def _():
                for t in range(AT):
                    out_copy(NOUT + t).start()

            @pl.when(h == cfg["h0"] + 1)
            def _():
                a_wait(1)

            link[0] = None
            n2 = AR // 2
            a_rows2 = pl.ds(pl.multiple_of(jnp.minimum(h, A_STEPS - 1) * n2, n2), n2)
            a_rows = pl.ds(pl.multiple_of(jnp.minimum(h, A_STEPS - 1) * AR, AR), AR)

            kw = C // 2
            pending = []
            chains = {i: [] for i in range(nq + 1)}
            deadline = [None]

            def flush_pending(x, row):
                done = list(pending)
                del pending[:]
                if not done:
                    return x
                x = _pin(x, _opaque_zero([f for _, f in done]), row)

                @pl.when(h == H - 1)
                def _():
                    for k, _f in done:
                        out_copy(k).start()
                return x

            def a_fwd():
                kk = _bf(a_v[0, a_rows2, :]).astype(F32)
                lane = lax.broadcasted_iota(jnp.int32, (AR, LANE), 1)
                coef = [par_v[j, a_rows, :] for j in range(KS)]
                rolled = [kk] + [pltpu.roll(kk, j, 1) for j in range(1, KS)]
                vv = _bf(a_v[1, a_rows2, :]).astype(F32)
                kv_blocks = []
                for a in range(NB):
                    cs = slice(a * LANE, (a + 1) * LANE)
                    acc = rolled[0][:, cs] * coef[0]
                    for j in range(1, KS):
                        t = rolled[j][:, cs]
                        if a == 0:
                            t = jnp.where(lane >= j, t, 0.0)
                        acc = acc + t * coef[j]
                    kv_blocks.append(acc * vv[:, cs])
                hk = a_v[2, a_rows2, :]
                hk = _rowcat([hk[:, a * LANE:(a + 1) * LANE] for a in range(NB)])
                fm = _bf(f_v[...])
                hs = _dot(_bf(linked(hk)), fm)
                kv = linked(_rowcat(kv_blocks)).astype(BF16)
                xs = _dot(kv, fm)
                set_link(xs)
                return kv, xs, hs

            def a_conv(xs, hs):
                def tile(v, a, g, part):
                    r = a * AR + 8 * g
                    return v[r:r + 8, part * LANE:(part + 1) * LANE]

                z = {}
                gate = None
                width = cfg["a_width"]
                for g in range(AR // 8):
                    hr = [tile(hs, 0, g, 0)] + [
                        tile(hs, j, g, 0) - tile(hs, j - 1, g, 1) for j in range(1, NB)]
                    hi = [tile(hs, 0, g, 1)] + [
                        tile(hs, j, g, 1) + tile(hs, j - 1, g, 0) for j in range(1, NB)]
                    for c0 in range(0, NB, width):
                        for a in range(c0 + width):
                            xr, xi = tile(xs, a, g, 0), tile(xs, a, g, 1)
                            if gate is not None:
                                xr, xi = _pin(xr, gate), _pin(xi, gate)
                            for c in range(max(c0, a), c0 + width):
                                j = c - a
                                tr = xr * hr[j] - xi * hi[j]
                                ti = xr * hi[j] + xi * hr[j]
                                z[c, g] = (tr, ti) if a == 0 else (z[c, g][0] + tr, z[c, g][1] + ti)
                            gate = _opaque_zero(list(z[c0 + width - 1, g]))
                            chains[nq].append(gate)
                return z

            def a_inv(kv, z, flush=False):
                fm = _bf(f_v[...])
                ng = AR // 8
                ys = []
                for u in range(2):
                    rows = [_lanecat(z[c, g]) for g in range(u * ng // 2, (u + 1) * ng // 2)
                            for c in range(NB)]
                    lhs = linked(_rowcat(rows))
                    if flush:
                        lhs = flush_pending(lhs, 8)
                    ys.append(_dot_nt(lhs.astype(BF16), fm))
                y = _rowcat(ys)
                dd = par_v[KS, a_rows, :]
                for c in range(NB):
                    cs = slice(c * LANE, (c + 1) * LANE)
                    yc = _rowcat([y[(g * NB + c) * 8:(g * NB + c + 1) * 8, :] for g in range(ng)])
                    qq = _bf(a_v[3, a_rows2, cs]).astype(F32)
                    kvf = kv[c * AR:(c + 1) * AR, :].astype(F32)
                    c2 = (c % (NB // 2)) * LANE
                    ra_t[c // (NB // 2), a_rows, c2:c2 + LANE] = qq * (yc * (1.0 / LANE) + kvf * dd)

            def a_out():
                slab = jnp.clip(h // 4 - 1, 0, AT - 1)
                half = h % 2
                x = ra_t[half, pl.ds(pl.multiple_of(slab * LANE, LANE), LANE), :]
                xt = x.T
                dst = jnp.where(h >= A_STEPS, AT, slab)
                oa_v[dst, pl.ds(pl.multiple_of(half * (S // 2), S // 2), S // 2), :] = xt.astype(BF16)
                return xt

            def w_blk(r, c):
                return wkv_v[h, _h(r * kw, kw), pl.ds(c * LANE, LANE)]

            def one_pass(lhs, w, flush):
                lhs = linked(lhs)
                if flush:
                    lhs = flush_pending(lhs, cfg["ao_row"])
                if deadline[0] is not None:
                    if deadline[0][0] == 0:
                        lhs = _pin(lhs, deadline[0][1], cfg["ao_row"] - 8)
                        deadline[0] = None
                    else:
                        deadline[0] = (deadline[0][0] - 1, deadline[0][1])
                d = _dot(_bf(lhs), _bf(paced(w)))
                set_link(d)
                return d

            def b_op(which, m):
                raw = lambda r, c: w_blk(r, 2 * which + c)
                blk = lambda r, c: _split(raw(r, c))
                return {1: lambda: _add(blk(0, 0), blk(1, 1)),
                        2: lambda: raw(0, 0),
                        3: lambda: _sub(blk(0, 1), blk(1, 1)),
                        4: lambda: _sub(blk(1, 0), blk(0, 0)),
                        5: lambda: raw(1, 1),
                        6: lambda: _add(blk(0, 0), blk(0, 1)),
                        7: lambda: _add(blk(1, 0), blk(1, 1))}[m]()

            def a_op(m, rho):
                rs = _h(rho * tq, tq)
                if m == 3:
                    return c_v[rs, 0:kw]
                if m == 4:
                    return c_v[_h(S // 2 + rho * tq, tq), kw:]
                return sa_v[{1: 0, 2: 1, 5: 2, 6: 3, 7: 4}[m], rs, :]

            b_cache, prod = {}, {}

            def kv_proj(which, blk, flush):
                rho = blk % 2
                for k, m in enumerate(_digits(cfg["kv_top" if blk < 2 else "kv_bot"])):
                    if (which, m) not in b_cache:
                        b_cache[which, m] = b_op(which, m)
                    prod[which, m, rho] = one_pass(a_op(m, rho), b_cache[which, m], k == flush)
                p = lambda m: prod[which, m, rho]
                if blk < 2:
                    return [(p(1) + p(4)) + (p(7) - p(5)), p(3) + p(5)]
                return [p(2) + p(4), (p(1) + p(3)) + (p(6) - p(2))]

            def k_proj(blk, flush=-1):
                k = kv_proj(0, blk, flush)
                k_s[_h(blk * tq, tq), :] = _u32(_lanecat(k).astype(BF16))
                if blk < nq - 1:
                    b = lambda r, c: k[r][c * D:(c + 1) * D, :]
                    sums = [b(0, 0) + b(1, 1), b(0, 1) - b(1, 1), b(1, 0) - b(0, 0),
                            b(0, 0) + b(0, 1), b(1, 0) + b(1, 1)]
                    for n, x in enumerate(sums):
                        kb_s[n, _h(blk * D, D), :] = _u32(x.astype(BF16))

            def v_proj(blk, flush=-1):
                v = kv_proj(1, blk, flush)
                v_s[_h(blk * tq, tq), :] = _u32(_lanecat(v).astype(BF16))
                if blk < nq - 1:
                    b = lambda r, c: v[c][r * D:(r + 1) * D, :]
                    sums = [b(0, 0) + b(1, 1), b(0, 1) - b(1, 1), b(1, 0) - b(0, 0),
                            b(0, 0) + b(0, 1), b(1, 0) + b(1, 1)]
                    for k, x in enumerate(sums):
                        vb_s[k, _h(blk * D, D), :] = _u32(x.astype(BF16))

            def qk(i, dep=None, flush=False):
                r0 = i * tq
                off = None
                if i > 0:
                    raw = lambda r, c: q_all[h, _h(r0 + r * D, D), c * LANE:(c + 1) * LANE]
                    a = lambda r, c: _split(raw(r, c))
                    sa = {1: _add(a(0, 0), a(1, 1)), 2: _add(a(1, 0), a(1, 1)), 3: raw(0, 0),
                          4: raw(1, 1), 5: _add(a(0, 0), a(0, 1)), 6: _sub(a(1, 0), a(0, 0)),
                          7: _sub(a(0, 1), a(1, 1))}

                    def sb(m, j, t):
                        if m in (2, 5):
                            c = 0 if m == 2 else 1
                            rows = _h(j * tq + c * D + t * LANE, LANE)
                            return k_s[rows, c * LANE:(c + 1) * LANE]
                        n = {1: 0, 3: 1, 4: 2, 6: 3, 7: 4}[m]
                        return kb_s[n, _h(j * D + t * LANE, LANE), :]

                    top, bot, due = {}, {}, []
                    n_dot = 0
                    for j in range(i):
                        for t in range(2):
                            p = {}
                            for n, m in enumerate(_digits(cfg["s_ord"])):
                                lhs = linked(sa[m])
                                if due and n == cfg["s_due"]:
                                    lhs = _pin(lhs, due.pop(), cfg["s_row"])
                                p[m] = _dot_nt(_bf(lhs), _bf(sb(m, j, t)))
                                n_dot += 1
                                if n_dot % 4 == 0:
                                    set_link(p[m], cfg["s_link"])
                            top[4 * j + t] = (p[1] + p[4]) + (p[7] - p[5])
                            top[4 * j + 2 + t] = p[3] + p[5]
                            bot[4 * j + t] = p[2] + p[4]
                            bot[4 * j + 2 + t] = (p[1] + p[3]) + (p[6] - p[2])
                            due.append(_opaque_zero(
                                [x[4 * j + c + t] for x in (top, bot) for c in (0, 2)]))
                    off = _rowcat([_lanecat([x[c] for c in range(4 * i)]) for x in (top, bot)])
                q = linked(q_all[h, _h(r0, tq), :])
                if off is not None:
                    q = _pin(q, due.pop(), cfg["ao_row"] - 8)
                if dep is not None:
                    q = _pin(q, _opaque_zero([dep]), cfg["ao_row"])
                main = _dot_nt(_bf(q), _bf(k_s[_h(r0, LANE), :]))
                parts = [main if off is None else _lanecat([off, main])]
                for j in range(1, nsub):
                    q = linked(q_all[h, _h(r0 + LANE * j, tq - LANE * j), :])
                    if flush and j == cfg["q_pin"]:
                        q = flush_pending(q, 8)
                    parts.append(_dot_nt(_bf(q), _bf(k_s[_h(r0 + LANE * j, LANE), :])))
                set_link(parts[2], cfg["link_part"], main)
                return parts

            def exps(i, parts):
                sas, mbs = [], []
                for a in range(nsub):
                    blocks = [parts[j][LANE * (a - j):LANE * (a - j + 1), :] for j in range(a + 1)]
                    last = blocks[-1]
                    w = last.shape[1]
                    dg = jnp.where(tri, last[:, w - LANE:], NEG)
                    blocks[-1] = dg if w == LANE else _lanecat([last[:, :w - LANE], dg])
                    sas.append(_lanecat(blocks))
                    lane_max = functools.reduce(jnp.maximum, [
                        sas[a][:, t:t + LANE] for t in range(0, sas[a].shape[1], LANE)])
                    mx = jnp.max(lane_max, axis=1, keepdims=True)
                    if i > 0:
                        mx = mx + jnp.log2(jnp.sum(jnp.exp2(lane_max - mx), axis=1, keepdims=True))
                    mbs.append(jnp.broadcast_to(mx, (LANE, LANE)))
                chain = _opaque_zero([b[b.shape[0] - 8:, b.shape[1] - LANE:] for b in parts])
                pg, psums = {}, {}
                for r in range(0, tq // 2, 8):
                    for row in (r, r + tq // 2):
                        a, g = divmod(row, LANE)
                        mg = _pin(mbs[a][g:g + 8, :], chain)
                        pg[row] = [jnp.exp2(sas[a][g:g + 8, t:t + LANE] - mg)
                                   for t in range(0, sas[a].shape[1], LANE)]
                        psums[row] = functools.reduce(jnp.add, pg[row])
                        chain = _opaque_zero([psums[row]])
                        chains[i].append(chain)
                return pg, psums

            def softmax(i, pg, psums):
                r0 = i * tq
                pd, pa = pd_s.at[i % 2], pa_s[i % 2]
                first = lambda x, c=0: _pin(x, link[0], 0, c).astype(BF16)
                nt0 = r0 // LANE
                ls = []
                for a in range(nsub):
                    rows = range(LANE * a, LANE * (a + 1), 8)
                    ls.append(jnp.sum(_rowcat([psums[r] for r in rows]), axis=1, keepdims=True))
                    pd[LANE * a:LANE * (a + 1), 0:LANE * (a + 1)] = first(
                        _rowcat([_lanecat(pg[r][nt0:]) for r in rows]), LANE * a)
                if i > 0:
                    quad = lambda rh, ch: _rowcat([
                        _lanecat([pg[rh * (tq // 2) + r][4 * j + 2 * ch + t]
                                  for j in range(i) for t in range(2)])
                        for r in range(0, tq // 2, 8)])
                    a11, a12, a21, a22 = quad(0, 0), quad(0, 1), quad(1, 0), quad(1, 1)
                    ops = [a11 + a22, a21 + a22, a11, a22, a11 + a12, a21 - a11, a12 - a22]
                    for m, x in enumerate(ops):
                        if i == 3:
                            x = _pin(x, link[0], 0, 2 * D)
                        pa[m, :, 0:i * D] = first(x)
                return ls

            def pv(i, ls, flush=-1):
                r0 = i * tq
                pd, pa = pd_s.at[i % 2], pa_s[i % 2]
                off = None
                if i > 0:
                    def b_rows(m, j0, j1):
                        if m in (2, 5):
                            q = 0 if m == 2 else 1
                            return _rowcat([
                                v_s[_h(j * tq + q * D, D), q * LANE:(q + 1) * LANE]
                                for j in range(j0, j1)])
                        k = {1: 0, 3: 1, 4: 2, 6: 3, 7: 4}[m]
                        return vb_s[k, _h(j0 * D, (j1 - j0) * D), :]

                    p, n_dot = {}, 0
                    for j0, j1 in {1: [(0, 1)], 2: [(0, 2)], 3: [(0, 2), (2, 3)]}[i]:
                        for m in _digits(cfg["p_ord"]):
                            cols = slice(j0 * D, j1 * D)
                            rhs = b_rows(m, j0, j1)
                            if n_dot == flush:
                                rhs = flush_pending(rhs, 0)
                            rhs = _bf(rhs)
                            n_dot += 1
                            if j1 - j0 == 1 and m == cfg["p_ord"] % 10:
                                d = _rowcat([_dot(pa[m - 1, r:r + LANE, cols], rhs)
                                             for r in (0, LANE)])
                            else:
                                d = _dot(pa[m - 1, :, cols], rhs)
                            p[m] = d if m not in p else p[m] + d
                    off = _rowcat([
                        _lanecat([(p[1] + p[4]) + (p[7] - p[5]), p[3] + p[5]]),
                        _lanecat([p[2] + p[4], (p[1] + p[3]) + (p[6] - p[2])])])
                ctx = []
                for j in range(nsub):
                    c0 = LANE * j
                    ctx.append(_dot(pd[c0:, c0:c0 + LANE], _bf(v_s[_h(r0 + c0, LANE), :])))
                set_link(ctx[2], cfg["link_part"], ctx[0])
                cs = []
                for a in range(nsub):
                    sl = lambda j: slice(LANE * (a - j), LANE * (a - j + 1))
                    r = pl.reciprocal(ls[a], approx=True)
                    terms = [ctx[j][sl(j)] for j in range(a + 1)]
                    if off is not None:
                        terms.append(off[sl(0)])
                    cs.append(functools.reduce(jnp.add, terms) * r)
                return _rowcat(cs)

            wo_cache = {}

            def oproj(i, ctx):
                mh = M // 4
                raw = lambda r, c: wo_v[h, r * mh:(r + 1) * mh, c * LANE:(c + 1) * LANE]
                a = lambda r, c: _split(raw(r, c))
                a_ops = {1: lambda: _add(a(0, 0), a(1, 1)), 2: lambda: _add(a(1, 0), a(1, 1)),
                         3: lambda: raw(0, 0), 4: lambda: raw(1, 1),
                         5: lambda: _add(a(0, 0), a(0, 1)), 6: lambda: _sub(a(1, 0), a(0, 0)),
                         7: lambda: _sub(a(0, 1), a(1, 1))}
                b = lambda r, c: ctx[c * D:(c + 1) * D, r * LANE:(r + 1) * LANE]
                b_ops = {1: lambda: b(0, 0) + b(1, 1), 2: lambda: b(0, 0),
                         3: lambda: b(0, 1) - b(1, 1), 4: lambda: b(1, 0) - b(0, 0),
                         5: lambda: b(1, 1), 6: lambda: b(0, 0) + b(0, 1),
                         7: lambda: b(1, 0) + b(1, 1)}
                p = {}
                order = _digits(cfg["o_ord"])
                mm = M // 2
                old = lambda r, c: rb_t[2 * i + c, r * mm:(r + 1) * mm, :]
                terms = {(0, 0): (1, 4, -5, 7), (0, 1): (3, 5), (1, 0): (2, 4), (1, 1): (1, -2, 3, 6)}

                def total(q):
                    acc = old(*q)
                    for m in sorted(terms[q], key=lambda m: order.index(abs(m))):
                        acc = acc + p[m] if m > 0 else acc - p[-m]
                    return acc

                for n, m in enumerate(order):
                    if m not in wo_cache:
                        wo_cache[m] = a_ops[m]()
                    rhs = b_ops[m]().astype(BF16)
                    if n == cfg["o_half"]:
                        lhs = [linked(wo_cache[m][r:r + mh // 2]) for r in (0, mh // 2)]
                        halves = [_dot_nt(_bf(x), rhs) for x in lhs]
                        p[m] = _rowcat(halves)
                        set_link(halves[1], 0)
                    else:
                        p[m] = _dot_nt(_bf(linked(wo_cache[m])), rhs)
                        if (n - (n > cfg["o_half"])) % 2 == 1:
                            set_link(p[m], cfg["o_link"])
                for c in range(2):
                    k = 2 * i + c
                    tot = _rowcat([total((r, c)) for r in range(2)])
                    rb_t[k] = tot
                    if k + 1 in body_chunks:
                        pending.append((k, b_out(k, tot)))

            st = {}
            for op in cfg["seq"].split():
                op, _, dl = op.partition("@")
                if dl:
                    ch = chains[int(dl[0])]
                    deadline[0] = (int(dl[1]), ch[int(dl[2:]) * len(ch) // 16 - 1])
                op, _, fl = op.partition("!")
                fl = int(fl) if fl else -1
                kind, i = op[0], int(op[1:] or 0)
                if kind == "K":
                    k_proj(i, fl)
                elif kind == "V":
                    v_proj(i, fl)
                elif kind == "Q":
                    st["e", i] = exps(
                        i, qk(i, a_out() if i == cfg["ao_at"] else None, fl >= 0))
                elif kind == "P":
                    st["ctx", i] = pv(i, softmax(i, *st["e", i]), fl)
                elif kind == "O":
                    oproj(i, st["ctx", i])
                elif kind == "F" and with_a:
                    st["kv"], xs, hs = a_fwd()
                    st["z"] = a_conv(xs, hs)
                elif kind == "I" and with_a:
                    a_inv(st["kv"], st["z"], fl >= 0)
            assert not pending and deadline[0] is None
            return carry

        with jax.named_scope("loop_a"):
            lax.fori_loop(cfg["h0"], H, head_step, 0)
        with jax.named_scope("tail"):
            for i in [k for k in range(NOUT) if k + 1 not in body_chunks]:
                b_out(i, rb_t[i])
                out_copy(i).start()
            for i in range(NOUT + AT):
                out_copy(i).wait()

    scratch = [
        pltpu.VMEM((4, M // 2, S), U32),
        pltpu.VMEM((KS, M), BF16),
        pltpu.VMEM((M,), BF16),
        pltpu.VMEM((KS + 1, M, LANE), F32),
        pltpu.VMEM((LANE // 2, 2 * LANE), U32),
        pltpu.VMEM((M // 2, S), U32),
        pltpu.VMEM((S // 2, MP), U32),
        pltpu.VMEM((5, XH // 2, D), U32),
        pltpu.VMEM((S // 2 + 8, C), U32),
        [pltpu.VMEM((4 * min(TP, M // 2 - kt * TP) * 8, LANE), U32)
         for kt in range(KT)],
        pltpu.VMEM((H // 2, MP // 2, 2 * D), U32),
        pltpu.VMEM((H // 2, x_cols, 2 * D), U32),
        pltpu.VMEM((QIT, C * 8, LANE), U32),
        pltpu.VMEM((H, C // 2, 2 * D), U32),
        pltpu.VMEM((H, M // 2, D), U32),
        pltpu.VMEM((H, S // 2, D), U32),
        pltpu.VMEM((S // 2, D), U32),
        pltpu.VMEM((S // 2, D), U32),
        pltpu.VMEM((5, (nq - 1) * D // 2, LANE), U32),
        pltpu.VMEM((5, (nq - 1) * D // 2, LANE), U32),
        pltpu.VMEM((2, tq, tq), BF16),
        [pltpu.VMEM((7, tq // 2, n * D), BF16) for n in (2, 3)],
        pltpu.VMEM((2, M, S // 2), F32),
        pltpu.VMEM((S // D, M, D), F32),
        pltpu.VMEM((AT + 1, S, LANE), BF16),
        pltpu.VMEM((S, 2 * M - AT * LANE), BF16),
        pltpu.SemaphoreType.DMA((XC,)),
        pltpu.SemaphoreType.DMA((KT,)),
        pltpu.SemaphoreType.DMA((QIT,)),
        pltpu.SemaphoreType.DMA((QIT,)),
        pltpu.SemaphoreType.DMA((2,)),
        pltpu.SemaphoreType.DMA((3,)),
        pltpu.SemaphoreType.DMA((S // D + AT,)),
    ]
    return kernel, scratch


_DEFAULT = dict(
    tq=512, a_width=8, ao_at=1, ao_row=240, link_back=176, link_part=32, pace_row=16,
    pace_step=32, use_a=1, h0=0, body_chunks=123456, kv_top=51473, kv_bot=26, s_ord=5147236,
    o_ord=5241736, p_ord=1234567, o_link=32, o_half=6,
    q_jobs=(2, 4, 4, 4, 1, 3, 1, 3, 5, 6, 6, 1, 2, 1),
    xs_from=3, s_link=48, s_due=6, s_row=120, q_pin=2,
    seq="K0 Q0 K1 Q1 V0 F P0 K2@1112 Q2 O0 V1!4 P1 K3@2116 Q3 O1 V2@4016 P2!6 V3@3114 O2 P3!13 I O3")


def _build(**kw):
    cfg = dict(_DEFAULT)
    cfg.update(kw)
    kernel, scratch = _make_kernel(cfg)

    def run(A_q, A_k, A_v, A_shift_k, A_ssm_k, A_ssm_D, B_x, B_c_kv, B_w_q, B_w_uk,
            B_w_uv, B_w_o):
        tr = lambda a: jnp.swapaxes(a, 1, 2).reshape(M, S)
        args = (
            tr(A_q), tr(A_k), tr(A_v), A_shift_k.T, A_ssm_k, A_ssm_D, tr(B_x),
            B_c_kv.reshape(S, C),
            B_w_q.reshape(M // 2, 2 * H, D), B_w_uk.reshape(C // 2, 2 * H, D),
            B_w_uv.reshape(C // 2, 2 * H, D),
            jnp.swapaxes(B_w_o, 1, 2),
        )
        out = pl.pallas_call(
            kernel,
            in_specs=[pl.BlockSpec(memory_space=pl.ANY)] * len(args),
            out_specs=pl.BlockSpec(memory_space=pl.ANY),
            out_shape=jax.ShapeDtypeStruct((S, 2 * M), BF16),
            scratch_shapes=scratch,
            compiler_params=pltpu.CompilerParams(
                vmem_limit_bytes=126 * 1024 * 1024,
                disable_bounds_checks=True),
        )(*args)
        return out.reshape(1, S, 2 * M)

    return run


_run = _build()


@jax.jit
def pallas_concat_heads__ssm_conv_h3__compressed_kv_cla__prompt_kernel(
    A_q: jax.Array,
    A_k: jax.Array,
    A_v: jax.Array,
    A_shift_k: jax.Array,
    A_ssm_k: jax.Array,
    A_ssm_D: jax.Array,
    B_x: jax.Array,
    B_c_kv: jax.Array,
    B_w_q: jax.Array,
    B_w_uk: jax.Array,
    B_w_uv: jax.Array,
    B_w_o: jax.Array,
):
    return _run(A_q, A_k, A_v, A_shift_k, A_ssm_k, A_ssm_D, B_x, B_c_kv, B_w_q,
                B_w_uk, B_w_uv, B_w_o)
```

```python
import functools

import jax
import jax.numpy as jnp
from jax import lax
import jax.experimental.pallas as pl
import jax.experimental.pallas.tpu as pltpu

F32 = jnp.float32
BF16 = jnp.bfloat16
U32 = jnp.uint32

S = 2048
M = 448
MP = 512
C = 1024
H = 16
D = 256
KS = 4
LANE = 128
NB = S // LANE
AR = 32
A_STEPS = M // AR
LOG2E = 1.4426950408889634
QSCALE = D ** -0.5 * LOG2E
NEG = -1e30

NT = (((1,), (1,)), ((), ()))


def _dot(a, b):
    return jnp.dot(a, b, preferred_element_type=F32)


def _dot_nt(a, b):
    return lax.dot_general(a, b, NT, preferred_element_type=F32)


def _bf(x):
    return pltpu.bitcast(x, BF16)


def _u32(x):
    return pltpu.bitcast(x, U32)


def _h(r0, n):
    return pl.ds(r0 // 2, n // 2)


def _repack(ev, od):
    lo = (ev & jnp.uint32(0xFFFF)) | (od << 16)
    hi = (ev >> 16) | (od & jnp.uint32(0xFFFF0000))
    return lo, hi


def _split(w):
    return (pltpu.bitcast(w << 16, F32), pltpu.bitcast(w & jnp.uint32(0xFFFF0000), F32))


def _join(lo, hi):
    half = jnp.uint32(0x8000)
    lo = (pltpu.bitcast(lo, U32) + half) >> 16
    hi = (pltpu.bitcast(hi, U32) + half) & jnp.uint32(0xFFFF0000)
    return lo | hi


def _add(a, b):
    return _join(a[0] + b[0], a[1] + b[1])


def _sub(a, b):
    return _join(a[0] - b[0], a[1] - b[1])


def _opaque_zero(vals):
    acc = None
    for v in vals:
        b = v if v.dtype == U32 else pltpu.bitcast(v, U32)
        for r in range(0, b.shape[0], 8):
            for c in range(0, b.shape[1], LANE):
                t = b[r:r + 8, c:c + LANE]
                acc = t if acc is None else acc | t
    return jnp.minimum((acc >> 1).astype(jnp.int32), 0)


def _pin(x, zero, r=0, c=0):
    t = pltpu.bitcast(pltpu.bitcast(x[r:r + 8, c:c + LANE], jnp.int32) + zero, x.dtype)
    row = ([x[r:r + 8, :c]] if c > 0 else []) + [t] + (
        [x[r:r + 8, c + LANE:]] if c + LANE < x.shape[1] else [])
    row = jnp.concatenate(row, axis=1) if len(row) > 1 else row[0]
    col = ([x[:r, :]] if r > 0 else []) + [row] + ([x[r + 8:, :]] if r + 8 < x.shape[0] else [])
    return jnp.concatenate(col, axis=0) if len(col) > 1 else col[0]


def _digits(n):
    return [int(c) for c in str(n)]


def _rowcat(xs):
    return jnp.concatenate(xs, axis=0) if len(xs) > 1 else xs[0]


def _lanecat(xs):
    return jnp.concatenate(xs, axis=1) if len(xs) > 1 else xs[0]


def _make_kernel(cfg):
    tq = cfg["tq"]
    nq = S // tq
    nsub = tq // LANE
    KT = MP // LANE
    TP = LANE // 2
    XC = 4
    x_cols = S // XC
    QP = 2
    QIT = H // 2 // QP
    XH = (S - x_cols) // 2
    CP = 176
    AT = 3

    def kernel(aq_hbm, ak_hbm, av_hbm, sh_hbm, ssm_hbm, dd_hbm, x_hbm, c_hbm,
               wq_hbm, wk_hbm, wv_hbm, wo_hbm,
               out_hbm,
               a_v, sh_v, dd_v, par_v, f_v,
               xt_v, x_v, xs_v, c_v, wqs_v, wq_v, qacc, ws_v, wkv_v, wo_v,
               q_all, k_s, v_s, kb_s, vb_s, pd_s, pa_s, ra_t, rb_t, oa_v, out_v,
               sem_x, sem_wq, sem_w, sem_c, sem_s, sem_a, sem_out):
        x32, c32, wq32, wk32, wv32, wo32 = (
            r.bitcast(U32) for r in (x_hbm, c_hbm, wq_hbm, wk_hbm, wv_hbm, wo_hbm))
        a32 = [r.bitcast(U32) for r in (ak_hbm, av_hbm, ssm_hbm, aq_hbm)]

        sa_v = qacc

        def x_copy(i):
            cs = pl.ds(i * x_cols, x_cols)
            return pltpu.make_async_copy(x32.at[:, cs], xt_v.at[:, cs], sem_x.at[i])

        def wq_pairs(kt):
            return min(TP, M // 2 - kt * TP)

        def wq_copies(kt):
            n = wq_pairs(kt)
            dst = wqs_v[kt].reshape(4, n, 8, LANE)
            return [pltpu.make_async_copy(
                wq32.at[pl.ds(kt * TP, n), pl.ds(8 * (k // 2), 8), pl.ds((k % 2) * LANE, LANE)],
                dst.at[k], sem_wq.at[kt]) for k in range(4)]

        def wq_wait(kt):
            pltpu.make_async_copy(wqs_v[kt], wqs_v[kt], sem_wq.at[kt]).wait()

        def w_copies(g):
            dst = ws_v.reshape(8, C // 2, 8, LANE)
            src = (wk32, wv32)[g // 2]
            return [pltpu.make_async_copy(
                src.at[:, pl.ds(8 * par, 8), pl.ds((g % 2) * LANE, LANE)],
                dst.at[2 * g + par], sem_w.at[g]) for par in range(2)]

        def w_wait(g):
            pltpu.make_async_copy(ws_v.at[g], ws_v.at[g], sem_w.at[g]).wait()

        c_bounds = [0, CP, 2 * CP, S // 4]

        def c_copies(p):
            r0, n = c_bounds[p], c_bounds[p + 1] - c_bounds[p]
            return [pltpu.make_async_copy(c32.at[rs], c_v.at[rs], sem_c.at[p])
                    for rs in (pl.ds(r0, n), pl.ds(S // 4 + r0, n))]

        wo_copy = pltpu.make_async_copy(wo32, wo_v, sem_a.at[0])

        a_parts = [pl.ds(0, AR // 2), pl.ds(AR // 2, M // 2 - AR // 2)]

        def a_start(part):
            rs = a_parts[part]
            for k in range(4):
                pltpu.make_async_copy(
                    a32[k].at[rs], a_v.at[k, rs], sem_a.at[1 + part]).start()

        def a_wait(part):
            view = a_v.at[:, a_parts[part]]
            pltpu.make_async_copy(view, view, sem_a.at[1 + part]).wait()

        small = [pltpu.make_async_copy(sh_hbm, sh_v, sem_s.at[0]),
                 pltpu.make_async_copy(dd_hbm, dd_v, sem_s.at[1])]

        link = [None]
        pace = [None]

        def set_link(res, row=None, pacer=None):
            if row is None:
                row = res.shape[0] - cfg["link_back"]
            link[0] = _opaque_zero([res[row:row + 8, res.shape[1] - LANE:]])
            pace[0] = res if pacer is None else pacer

        def linked(x):
            return x if link[0] is None else _pin(x, link[0])

        def paced(w):
            res = pace[0]
            if res is None or link[0] is None or not cfg["pace_step"]:
                return w
            rows = []
            r0, step = cfg["pace_row"], cfg["pace_step"]
            if res.shape[0] < 400:
                r0, step = 0, 8
            if res.shape[0] < 200:
                return w
            zs = [_opaque_zero([res[r:r + 8, res.shape[1] - LANE:]])
                  for r in range(r0, r0 + 8 * step, step)]
            for r in range(0, w.shape[0], 8):
                z = zs[7 - (r // 8) % 8]
                t = pltpu.bitcast(w[r:r + 8, :], jnp.int32)
                rows.append(pltpu.bitcast(t + _lanecat([z] * (w.shape[1] // LANE)), U32))
            return _rowcat(rows)

        for cp in small:
            cp.start()
        x_copy(0).start()
        for cp in wq_copies(0):
            cp.start()

        def zero_body(k, carry):
            n = LANE // (S // D)
            bi = lax.broadcasted_iota(jnp.int32, (n, LANE), 0) + k * n
            mi = lax.broadcasted_iota(jnp.int32, (n, LANE), 1)
            ph = ((4 * mi + 1) * bi) & 511
            ang = ph.astype(F32) * (2.0 * 3.141592653589793 / 512.0)
            rs = pl.ds(pl.multiple_of(k * (n // 2), n // 2), n // 2)
            f_v[rs, 0:LANE] = _u32(jnp.cos(ang).astype(BF16))
            f_v[rs, LANE:] = _u32((-jnp.sin(ang)).astype(BF16))

            rb_t[k] = jnp.zeros((M, D), F32)
            cs = pl.ds(pl.multiple_of((k % 4) * D, D), D)
            ra_t[k // 4, 0:LANE, cs] = jnp.zeros((LANE, D), F32)
            ra_t[k // 4, AT * LANE:, cs] = jnp.zeros((M - AT * LANE, D), F32)
            return carry

        lax.fori_loop(0, S // D, zero_body, 0)
        c_v[S // 2:, :] = jnp.zeros((8, C), U32)

        for kt in range(1, KT):
            for cp in wq_copies(kt):
                cp.start()
        with jax.named_scope("small_wait"):
            for cp in small:
                cp.wait()
        sh = sh_v[...].astype(F32)
        for j in range(KS):
            par_v[j] = jnp.broadcast_to(sh[j:j + 1, :], (LANE, M)).T
        dd = dd_v[...].astype(F32).reshape(1, M)
        par_v[KS] = jnp.broadcast_to(dd, (LANE, M)).T

        def x_transpose(i):
            xt = xt_v[:, pl.ds(i * x_cols, x_cols)]
            xt = _rowcat([xt, jnp.zeros((MP // 2 - M // 2, x_cols), U32)])
            x_v[_h(i * x_cols, x_cols), :] = _u32(_bf(xt).astype(F32).T.astype(BF16))

        def q_early(kt, keep=False, jobs=()):
            first, last = kt == 0, kt == KT - 1
            n = wq_pairs(kt)
            cols = pl.ds(kt * LANE, LANE)
            if not keep:
                link[0] = None
            for j in range(H // 2):
                ws = []
                for half in range(2):
                    ev, od = (wqs_v[kt][pl.ds((2 * par + half) * n * 8 + j, n, stride=8), :]
                              for par in range(2))
                    ws.append(_repack(ev, od))
                w = _lanecat([ws[0][0], ws[1][0], ws[0][1], ws[1][1]])
                if n < TP:
                    w = _rowcat([w, jnp.zeros((TP - n, 2 * D), U32)])
                wq_v[j, pl.ds(kt * TP, TP), :] = w
                lhs = linked(x_v[_h(0, x_cols), cols])
                j0 = cfg["xs_from"]
                if jobs and j >= j0:
                    nj = H // 2 - j0
                    mine = jobs[(j - j0) * len(jobs) // nj:(j - j0 + 1) * len(jobs) // nj]
                    for k, job in enumerate(mine):
                        lhs = _pin(lhs, _opaque_zero(job()), 8 * (1 + k * 30 // len(mine)))
                d = _dot(_bf(lhs), _bf(w))
                set_link(d)
                if not first:
                    d = d + pltpu.bitcast(qacc[j], F32)
                if last:
                    d = (d * QSCALE).astype(BF16)
                    for t in range(2):
                        q_all[2 * j + t, _h(0, x_cols), :] = _u32(d[:, t * D:(t + 1) * D])
                else:
                    qacc[j] = pltpu.bitcast(d, U32)

        with jax.named_scope("x_wait"):
            x_copy(0).wait()
        x_transpose(0)
        for i in range(1, XC):
            x_copy(i).start()
        for g in range(QIT):
            for cp in w_copies(g) + (c_copies(g) if g < QIT - 1 else []):
                cp.start()
        wo_copy.start()
        a_start(0)
        a_start(1)
        with jax.named_scope("wq_wait"):
            wq_wait(0)
        q_early(0)
        with jax.named_scope("wq_wait"):
            wq_wait(1)
        q_early(1)
        with jax.named_scope("wq_wait"):
            wq_wait(2)
            wq_wait(3)
            for i in range(1, XC):
                x_copy(i).wait()
        for i in range(1, XC):
            x_transpose(i)

        def x_sums(u):
            a11, a12, a21, a22 = (
                _split(x_v[pl.ds((x_cols + rb * XH) // 2 + 8 * u, 8), cb * D:(cb + 1) * D])
                for rb in range(2) for cb in range(2))
            outs = [_add(a11, a22), _add(a21, a22), _add(a11, a12), _sub(a21, a11),
                    _sub(a12, a22)]
            for k, o in enumerate(outs):
                xs_v[k, 8 * u:8 * u + 8, :] = o
            return outs

        q_early(2, jobs=[functools.partial(x_sums, u) for u in range(XH // 16)])
        q_early(3, keep=True)

        def unpack(it, sub, j):
            g = it
            ev, od = (ws_v[g, pl.ds((par * (C // 2) + sub * TP) * 8 + j, TP, stride=8), :]
                      for par in range(2))
            lo, hi = _repack(ev, od)
            rows = pl.ds(sub * TP, TP)
            cols = pl.ds(pl.multiple_of(g * LANE, LANE), LANE)
            wkv_v[2 * j, rows, cols] = lo
            wkv_v[2 * j + 1, rows, cols] = hi
            return [lo, hi]

        def a_sums(it, u):
            r0 = jnp.clip((it - 1) * CP, 0, S // 4 - CP) + 8 * u
            src = [jnp.where(it == 0, S // 2, r0 + rb * (S // 4)) for rb in range(2)]
            r0 = pl.multiple_of(r0, 8)
            kw = C // 2
            a11, a12, a21, a22 = (
                _split(c_v[pl.ds(pl.multiple_of(src[rb], 8), 8), pl.ds(cb * kw, kw)])
                for rb in range(2) for cb in range(2))
            outs = [_add(a11, a22), _add(a21, a22), _add(a11, a12), _sub(a21, a11),
                    _sub(a12, a22)]
            for k, o in enumerate(outs):
                sa_v[k, pl.ds(r0, 8), :] = o
            return outs

        units = [functools.partial(unpack, sub=s_, j=j_)
                 for s_ in range(C // 2 // TP) for j_ in range(H // 2)]
        for u_ in range(CP // 8):
            units.insert(4 * u_ + 1, functools.partial(a_sums, u=u_))

        def q_pair(pair, todo):
            raw = lambda r, c: _lanecat([
                wq_v[pair, r * LANE:(r + 1) * LANE, pl.ds(t * D + c * LANE, LANE)]
                for t in range(2)])
            b = lambda r, c: _split(raw(r, c))
            sb = {1: _add(b(0, 0), b(1, 1)), 2: raw(0, 0), 3: _sub(b(0, 1), b(1, 1)),
                  4: _sub(b(1, 0), b(0, 0)), 5: raw(1, 1), 6: _add(b(0, 0), b(0, 1)),
                  7: _add(b(1, 0), b(1, 1))}
            n = XH // 2
            for rho in range(2):
                def sa(m):
                    if m == 3:
                        return x_v[_h(x_cols + rho * n, n), 0:D]
                    if m == 4:
                        return x_v[_h(x_cols + XH + rho * n, n), D:]
                    return xs_v[{1: 0, 2: 1, 5: 2, 6: 3, 7: 4}[m], _h(rho * n, n), :]

                def put(half, c0, c1):
                    rows = _h(x_cols + half * XH + rho * n, n)
                    for t in range(2):
                        q = _lanecat([c[:, t * LANE:(t + 1) * LANE] for c in (c0, c1)])
                        q_all[2 * pair + t, rows, :] = _u32((q * QSCALE).astype(BF16))

                p = {}
                for pos, m in enumerate((5, 1, 4, 7, 3, 2, 6)):
                    lhs = linked(sa(m))
                    nj = min(len(todo), cfg["q_jobs"][7 * rho + pos])
                    jobs = [todo.pop()(it=pair // QP) for _ in range(nj)]
                    for k, job in enumerate(jobs):
                        lhs = _pin(lhs, _opaque_zero(job), 8 * (1 + k * (n // 16 - 1) // nj))
                    p[m] = _dot(_bf(lhs), _bf(sb[m]))
                    set_link(p[m])
                    if m == 3:
                        put(0, (p[1] + p[4]) + (p[7] - p[5]), p[3] + p[5])
                put(1, p[2] + p[4], (p[1] + p[3]) + (p[6] - p[2]))

        def q_body(it, carry):
            with jax.named_scope("w_wait"):
                w_wait(it)
                for p in range(QIT - 1):
                    @pl.when(it == p + 1)
                    def _():
                        for cp in c_copies(p):
                            cp.wait()
            link[0] = None
            todo = units[::-1]
            for p in range(QP):
                q_pair(QP * it + p, todo)
            assert not todo
            return carry

        with jax.named_scope("q_loop"):
            lax.fori_loop(0, QIT, q_body, 0)
        wo_copy.wait()
        a_wait(0)

        tri = (lax.broadcasted_iota(jnp.int32, (LANE, LANE), 1)
               <= lax.broadcasted_iota(jnp.int32, (LANE, LANE), 0))

        NOUT = S // D

        def out_copy(i):
            if i >= NOUT:
                t = i - NOUT
                return pltpu.make_async_copy(
                    oa_v.at[t], out_hbm.at[:, pl.ds(t * LANE, LANE)], sem_out.at[i])
            rs = pl.ds(i * D, D)
            return pltpu.make_async_copy(
                out_v.at[rs], out_hbm.at[rs, pl.ds(AT * LANE, 2 * M - AT * LANE)], sem_out.at[i])

        body_chunks = _digits(cfg["body_chunks"])

        def b_out(k, tot):
            c0 = (k * D) % (S // 2)
            full = _rowcat([ra_t[k * D // (S // 2), AT * LANE:, c0:c0 + D], tot]).T
            out_v[k * D:(k + 1) * D, :] = full.astype(BF16)
            return full

        def head_step(h, carry):
            with jax.named_scope("step"):
                return head_step_(h, carry)

        def head_step_(h, carry):
            with_a = cfg["use_a"]

            @pl.when(h == A_STEPS)
            def _():
                for t in range(AT):
                    out_copy(NOUT + t).start()

            @pl.when(h == cfg["h0"] + 1)
            def _():
                a_wait(1)

            link[0] = None
            n2 = AR // 2
            a_rows2 = pl.ds(pl.multiple_of(jnp.minimum(h, A_STEPS - 1) * n2, n2), n2)
            a_rows = pl.ds(pl.multiple_of(jnp.minimum(h, A_STEPS - 1) * AR, AR), AR)

            kw = C // 2
            pending = []
            chains = {i: [] for i in range(nq + 1)}
            deadline = [None]

            def flush_pending(x, row):
                done = list(pending)
                del pending[:]
                if not done:
                    return x
                x = _pin(x, _opaque_zero([f for _, f in done]), row)

                if any(k is not None for k, _ in done):
                    @pl.when(h == H - 1)
                    def _():
                        for k, _f in done:
                            if k is not None:
                                out_copy(k).start()
                return x

            def a_fwd():
                kk = _bf(a_v[0, a_rows2, :]).astype(F32)
                lane = lax.broadcasted_iota(jnp.int32, (AR, LANE), 1)
                coef = [par_v[j, a_rows, :] for j in range(KS)]
                rolled = [kk] + [pltpu.roll(kk, j, 1) for j in range(1, KS)]
                vv = _bf(a_v[1, a_rows2, :]).astype(F32)
                kv_blocks = []
                for a in range(NB):
                    cs = slice(a * LANE, (a + 1) * LANE)
                    acc = rolled[0][:, cs] * coef[0]
                    for j in range(1, KS):
                        t = rolled[j][:, cs]
                        if a == 0:
                            t = jnp.where(lane >= j, t, 0.0)
                        acc = acc + t * coef[j]
                    kv_blocks.append(acc * vv[:, cs])
                hk = a_v[2, a_rows2, :]
                hk = _rowcat([hk[:, a * LANE:(a + 1) * LANE] for a in range(NB)])
                fm = _bf(f_v[...])
                hs = _dot(_bf(linked(hk)), fm)
                kv = linked(_rowcat(kv_blocks)).astype(BF16)
                xs = _dot(kv, fm)
                set_link(xs)
                return kv, xs, hs

            def a_conv(xs, hs):
                def tile(v, a, g, part):
                    r = a * AR + 8 * g
                    return v[r:r + 8, part * LANE:(part + 1) * LANE]

                z = {}
                gate = None
                width = cfg["a_width"]
                for g in range(AR // 8):
                    hr = [tile(hs, 0, g, 0)] + [
                        tile(hs, j, g, 0) - tile(hs, j - 1, g, 1) for j in range(1, NB)]
                    hi = [tile(hs, 0, g, 1)] + [
                        tile(hs, j, g, 1) + tile(hs, j - 1, g, 0) for j in range(1, NB)]
                    for c0 in range(0, NB, width):
                        for a in range(c0 + width):
                            xr, xi = tile(xs, a, g, 0), tile(xs, a, g, 1)
                            if gate is not None:
                                xr, xi = _pin(xr, gate), _pin(xi, gate)
                            for c in range(max(c0, a), c0 + width):
                                j = c - a
                                tr = xr * hr[j] - xi * hi[j]
                                ti = xr * hi[j] + xi * hr[j]
                                z[c, g] = (tr, ti) if a == 0 else (z[c, g][0] + tr, z[c, g][1] + ti)
                            gate = _opaque_zero(list(z[c0 + width - 1, g]))
                            chains[nq].append(gate)
                return z

            def a_inv(kv, z, flush=False):
                fm = _bf(f_v[...])
                ng = AR // 8
                ys = []
                for u in range(2):
                    rows = [_lanecat(z[c, g]) for g in range(u * ng // 2, (u + 1) * ng // 2)
                            for c in range(NB)]
                    lhs = linked(_rowcat(rows))
                    if flush:
                        lhs = flush_pending(lhs, 8)
                    ys.append(_dot_nt(lhs.astype(BF16), fm))
                y = _rowcat(ys)
                dd = par_v[KS, a_rows, :]
                for c in range(NB):
                    cs = slice(c * LANE, (c + 1) * LANE)
                    yc = _rowcat([y[(g * NB + c) * 8:(g * NB + c + 1) * 8, :] for g in range(ng)])
                    qq = _bf(a_v[3, a_rows2, cs]).astype(F32)
                    kvf = kv[c * AR:(c + 1) * AR, :].astype(F32)
                    c2 = (c % (NB // 2)) * LANE
                    ra_t[c // (NB // 2), a_rows, c2:c2 + LANE] = qq * (yc * (1.0 / LANE) + kvf * dd)

            def a_out():
                slab = jnp.clip(h // 4 - 1, 0, AT - 1)
                half = h % 2
                x = ra_t[half, pl.ds(pl.multiple_of(slab * LANE, LANE), LANE), :]
                xt = x.T
                dst = jnp.where(h >= A_STEPS, AT, slab)
                oa_v[dst, pl.ds(pl.multiple_of(half * (S // 2), S // 2), S // 2), :] = xt.astype(BF16)
                return xt

            def w_blk(r, c):
                return wkv_v[h, _h(r * kw, kw), pl.ds(c * LANE, LANE)]

            def one_pass(lhs, w, flush):
                lhs = linked(lhs)
                if flush:
                    lhs = flush_pending(lhs, cfg["ao_row"])
                if deadline[0] is not None:
                    if deadline[0][0] == 0:
                        lhs = _pin(lhs, deadline[0][1], cfg["ao_row"] - 8)
                        deadline[0] = None
                    else:
                        deadline[0] = (deadline[0][0] - 1, deadline[0][1])
                d = _dot(_bf(lhs), _bf(paced(w)))
                set_link(d)
                return d

            def b_op(which, m):
                raw = lambda r, c: w_blk(r, 2 * which + c)
                blk = lambda r, c: _split(raw(r, c))
                return {1: lambda: _add(blk(0, 0), blk(1, 1)),
                        2: lambda: raw(0, 0),
                        3: lambda: _sub(blk(0, 1), blk(1, 1)),
                        4: lambda: _sub(blk(1, 0), blk(0, 0)),
                        5: lambda: raw(1, 1),
                        6: lambda: _add(blk(0, 0), blk(0, 1)),
                        7: lambda: _add(blk(1, 0), blk(1, 1))}[m]()

            def a_op(m, rho):
                rs = _h(rho * tq, tq)
                if m == 3:
                    return c_v[rs, 0:kw]
                if m == 4:
                    return c_v[_h(S // 2 + rho * tq, tq), kw:]
                return sa_v[{1: 0, 2: 1, 5: 2, 6: 3, 7: 4}[m], rs, :]

            b_cache, prod = {}, {}

            def kv_proj(which, blk, flush):
                rho = blk % 2
                for k, m in enumerate(_digits(cfg["kv_top" if blk < 2 else "kv_bot"])):
                    if (which, m) not in b_cache:
                        b_cache[which, m] = b_op(which, m)
                    prod[which, m, rho] = one_pass(a_op(m, rho), b_cache[which, m], k == flush)
                p = lambda m: prod[which, m, rho]
                if blk < 2:
                    return [(p(1) + p(4)) + (p(7) - p(5)), p(3) + p(5)]
                return [p(2) + p(4), (p(1) + p(3)) + (p(6) - p(2))]

            def k_proj(blk, flush=-1):
                k = kv_proj(0, blk, flush)
                k_s[_h(blk * tq, tq), :] = _u32(_lanecat(k).astype(BF16))
                if blk < nq - 1:
                    b = lambda r, c: k[r][c * D:(c + 1) * D, :]
                    sums = [b(0, 0) + b(1, 1), b(0, 1) - b(1, 1), b(1, 0) - b(0, 0),
                            b(0, 0) + b(0, 1), b(1, 0) + b(1, 1)]
                    for n, x in enumerate(sums):
                        kb_s[n, _h(blk * D, D), :] = _u32(x.astype(BF16))

            def v_proj(blk, flush=-1):
                v = kv_proj(1, blk, flush)
                v_s[_h(blk * tq, tq), :] = _u32(_lanecat(v).astype(BF16))
                if blk < nq - 1:
                    b = lambda r, c: v[c][r * D:(r + 1) * D, :]
                    sums = [b(0, 0) + b(1, 1), b(0, 1) - b(1, 1), b(1, 0) - b(0, 0),
                            b(0, 0) + b(0, 1), b(1, 0) + b(1, 1)]
                    for k, x in enumerate(sums):
                        vb_s[k, _h(blk * D, D), :] = _u32(x.astype(BF16))

            def qk(i, flush=False):
                r0 = i * tq
                off = None
                if i > 0:
                    raw = lambda r, c: q_all[h, _h(r0 + r * D, D), c * LANE:(c + 1) * LANE]
                    a = lambda r, c: _split(raw(r, c))
                    sa = {1: _add(a(0, 0), a(1, 1)), 2: _add(a(1, 0), a(1, 1)), 3: raw(0, 0),
                          4: raw(1, 1), 5: _add(a(0, 0), a(0, 1)), 6: _sub(a(1, 0), a(0, 0)),
                          7: _sub(a(0, 1), a(1, 1))}

                    def sb(m, j, t):
                        if m in (2, 5):
                            c = 0 if m == 2 else 1
                            rows = _h(j * tq + c * D + t * LANE, LANE)
                            return k_s[rows, c * LANE:(c + 1) * LANE]
                        n = {1: 0, 3: 1, 4: 2, 6: 3, 7: 4}[m]
                        return kb_s[n, _h(j * D + t * LANE, LANE), :]

                    top, bot, due = {}, {}, []
                    n_dot = 0
                    for j in range(i):
                        for t in range(2):
                            p = {}
                            for n, m in enumerate(_digits(cfg["s_ord"])):
                                lhs = linked(sa[m])
                                if due and n == cfg["s_due"]:
                                    lhs = _pin(lhs, due.pop(), cfg["s_row"])
                                p[m] = _dot_nt(_bf(lhs), _bf(sb(m, j, t)))
                                n_dot += 1
                                if n_dot % 4 == 0:
                                    set_link(p[m], cfg["s_link"])
                            top[4 * j + t] = (p[1] + p[4]) + (p[7] - p[5])
                            top[4 * j + 2 + t] = p[3] + p[5]
                            bot[4 * j + t] = p[2] + p[4]
                            bot[4 * j + 2 + t] = (p[1] + p[3]) + (p[6] - p[2])
                            due.append(_opaque_zero(
                                [x[4 * j + c + t] for x in (top, bot) for c in (0, 2)]))
                    off = _rowcat([_lanecat([x[c] for c in range(4 * i)]) for x in (top, bot)])
                q = linked(q_all[h, _h(r0, tq), :])
                if off is not None:
                    q = _pin(q, due.pop(), cfg["ao_row"] - 8)
                main = _dot_nt(_bf(q), _bf(k_s[_h(r0, LANE), :]))
                parts = [main if off is None else _lanecat([off, main])]
                for j in range(1, nsub):
                    q = linked(q_all[h, _h(r0 + LANE * j, tq - LANE * j), :])
                    if flush and j == cfg["q_pin"]:
                        q = flush_pending(q, 8)
                    parts.append(_dot_nt(_bf(q), _bf(k_s[_h(r0 + LANE * j, LANE), :])))
                set_link(parts[2], cfg["link_part"], main)
                return parts

            def exps(i, parts):
                sas, mbs = [], []
                for a in range(nsub):
                    blocks = [parts[j][LANE * (a - j):LANE * (a - j + 1), :] for j in range(a + 1)]
                    last = blocks[-1]
                    w = last.shape[1]
                    dg = jnp.where(tri, last[:, w - LANE:], NEG)
                    blocks[-1] = dg if w == LANE else _lanecat([last[:, :w - LANE], dg])
                    sas.append(_lanecat(blocks))
                    lane_max = functools.reduce(jnp.maximum, [
                        sas[a][:, t:t + LANE] for t in range(0, sas[a].shape[1], LANE)])
                    mx = jnp.max(lane_max, axis=1, keepdims=True)
                    if i > 0:
                        mx = mx + jnp.log2(jnp.sum(jnp.exp2(lane_max - mx), axis=1, keepdims=True))
                    mbs.append(jnp.broadcast_to(mx, (LANE, LANE)))
                chain = _opaque_zero([b[b.shape[0] - 8:, b.shape[1] - LANE:] for b in parts])
                pg, psums = {}, {}
                for r in range(0, tq // 2, 8):
                    for row in (r, r + tq // 2):
                        a, g = divmod(row, LANE)
                        mg = _pin(mbs[a][g:g + 8, :], chain)
                        pg[row] = [jnp.exp2(sas[a][g:g + 8, t:t + LANE] - mg)
                                   for t in range(0, sas[a].shape[1], LANE)]
                        psums[row] = functools.reduce(jnp.add, pg[row])
                        chain = _opaque_zero([psums[row]])
                        chains[i].append(chain)
                return pg, psums

            def softmax(i, pg, psums):
                r0 = i * tq
                pd, pa = pd_s.at[i % 2], pa_s[i % 2]
                first = lambda x, c=0: _pin(x, link[0], 0, c).astype(BF16)
                nt0 = r0 // LANE
                ls = []
                for a in range(nsub):
                    rows = range(LANE * a, LANE * (a + 1), 8)
                    ls.append(jnp.sum(_rowcat([psums[r] for r in rows]), axis=1, keepdims=True))
                    pd[LANE * a:LANE * (a + 1), 0:LANE * (a + 1)] = first(
                        _rowcat([_lanecat(pg[r][nt0:]) for r in rows]), LANE * a)
                if i > 0:
                    quad = lambda rh, ch: _rowcat([
                        _lanecat([pg[rh * (tq // 2) + r][4 * j + 2 * ch + t]
                                  for j in range(i) for t in range(2)])
                        for r in range(0, tq // 2, 8)])
                    a11, a12, a21, a22 = quad(0, 0), quad(0, 1), quad(1, 0), quad(1, 1)
                    ops = [a11 + a22, a21 + a22, a11, a22, a11 + a12, a21 - a11, a12 - a22]
                    for m, x in enumerate(ops):
                        if i == 3:
                            x = _pin(x, link[0], 0, 2 * D)
                        pa[m, :, 0:i * D] = first(x)
                return ls

            def pv(i, ls, flush=-1):
                r0 = i * tq
                pd, pa = pd_s.at[i % 2], pa_s[i % 2]
                off = None
                if i > 0:
                    def b_rows(m, j0, j1):
                        if m in (2, 5):
                            q = 0 if m == 2 else 1
                            return _rowcat([
                                v_s[_h(j * tq + q * D, D), q * LANE:(q + 1) * LANE]
                                for j in range(j0, j1)])
                        k = {1: 0, 3: 1, 4: 2, 6: 3, 7: 4}[m]
                        return vb_s[k, _h(j0 * D, (j1 - j0) * D), :]

                    p, n_dot = {}, 0
                    for j0, j1 in {1: [(0, 1)], 2: [(0, 2)], 3: [(0, 2), (2, 3)]}[i]:
                        for m in _digits(cfg["p_ord"]):
                            cols = slice(j0 * D, j1 * D)
                            rhs = b_rows(m, j0, j1)
                            if n_dot == flush:
                                rhs = flush_pending(rhs, 0)
                            rhs = _bf(rhs)
                            n_dot += 1
                            if j1 - j0 == 1 and m == cfg["p_ord"] % 10:
                                d = _rowcat([_dot(pa[m - 1, r:r + LANE, cols], rhs)
                                             for r in (0, LANE)])
                            else:
                                d = _dot(pa[m - 1, :, cols], rhs)
                            p[m] = d if m not in p else p[m] + d
                    off = _rowcat([
                        _lanecat([(p[1] + p[4]) + (p[7] - p[5]), p[3] + p[5]]),
                        _lanecat([p[2] + p[4], (p[1] + p[3]) + (p[6] - p[2])])])
                ctx = []
                for j in range(nsub):
                    c0 = LANE * j
                    ctx.append(_dot(pd[c0:, c0:c0 + LANE], _bf(v_s[_h(r0 + c0, LANE), :])))
                set_link(ctx[2], cfg["link_part"], ctx[0])
                cs = []
                for a in range(nsub):
                    sl = lambda j: slice(LANE * (a - j), LANE * (a - j + 1))
                    r = pl.reciprocal(ls[a], approx=True)
                    terms = [ctx[j][sl(j)] for j in range(a + 1)]
                    if off is not None:
                        terms.append(off[sl(0)])
                    cs.append(functools.reduce(jnp.add, terms) * r)
                return _rowcat(cs)

            wo_cache = {}

            def oproj(i, ctx):
                mh = M // 4
                raw = lambda r, c: wo_v[h, r * mh:(r + 1) * mh, c * LANE:(c + 1) * LANE]
                a = lambda r, c: _split(raw(r, c))
                a_ops = {1: lambda: _add(a(0, 0), a(1, 1)), 2: lambda: _add(a(1, 0), a(1, 1)),
                         3: lambda: raw(0, 0), 4: lambda: raw(1, 1),
                         5: lambda: _add(a(0, 0), a(0, 1)), 6: lambda: _sub(a(1, 0), a(0, 0)),
                         7: lambda: _sub(a(0, 1), a(1, 1))}
                b = lambda r, c: ctx[c * D:(c + 1) * D, r * LANE:(r + 1) * LANE]
                b_ops = {1: lambda: b(0, 0) + b(1, 1), 2: lambda: b(0, 0),
                         3: lambda: b(0, 1) - b(1, 1), 4: lambda: b(1, 0) - b(0, 0),
                         5: lambda: b(1, 1), 6: lambda: b(0, 0) + b(0, 1),
                         7: lambda: b(1, 0) + b(1, 1)}
                p = {}
                order = _digits(cfg["o_ord"])
                mm = M // 2
                old = lambda r, c: rb_t[2 * i + c, r * mm:(r + 1) * mm, :]
                terms = {(0, 0): (1, 4, -5, 7), (0, 1): (3, 5), (1, 0): (2, 4), (1, 1): (1, -2, 3, 6)}

                def total(q):
                    acc = old(*q)
                    for m in sorted(terms[q], key=lambda m: order.index(abs(m))):
                        acc = acc + p[m] if m > 0 else acc - p[-m]
                    return acc

                for n, m in enumerate(order):
                    if m not in wo_cache:
                        wo_cache[m] = a_ops[m]()
                    rhs = b_ops[m]().astype(BF16)
                    if n == cfg["o_half"]:
                        lhs = [linked(wo_cache[m][r:r + mh // 2]) for r in (0, mh // 2)]
                        halves = [_dot_nt(_bf(x), rhs) for x in lhs]
                        p[m] = _rowcat(halves)
                        set_link(halves[1], 0)
                    else:
                        p[m] = _dot_nt(_bf(linked(wo_cache[m])), rhs)
                        if (n - (n > cfg["o_half"])) % 2 == 1:
                            set_link(p[m], cfg["o_link"])
                for c in range(2):
                    k = 2 * i + c
                    tot = _rowcat([total((r, c)) for r in range(2)])
                    rb_t[k] = tot
                    if k + 1 in body_chunks:
                        pending.append((k, b_out(k, tot)))

            st = {}
            for op in cfg["seq"].split():
                op, _, dl = op.partition("@")
                if dl:
                    ch = chains[int(dl[0])]
                    deadline[0] = (int(dl[1]), ch[int(dl[2:]) * len(ch) // 16 - 1])
                op, _, fl = op.partition("!")
                fl = int(fl) if fl else -1
                kind, i = op[0], int(op[1:] or 0)
                if kind == "K":
                    k_proj(i, fl)
                elif kind == "V":
                    v_proj(i, fl)
                elif kind == "Q":
                    st["e", i] = exps(i, qk(i, fl >= 0))
                elif kind == "P":
                    st["ctx", i] = pv(i, softmax(i, *st["e", i]), fl)
                elif kind == "O":
                    oproj(i, st["ctx", i])
                elif kind == "T":
                    pending.append((None, a_out()))
                elif kind == "F" and with_a:
                    st["kv"], xs, hs = a_fwd()
                    st["z"] = a_conv(xs, hs)
                elif kind == "I" and with_a:
                    a_inv(st["kv"], st["z"], fl >= 0)
            assert not pending and deadline[0] is None
            return carry

        with jax.named_scope("loop_a"):
            lax.fori_loop(cfg["h0"], H, head_step, 0)
        with jax.named_scope("tail"):
            for i in [k for k in range(NOUT) if k + 1 not in body_chunks]:
                b_out(i, rb_t[i])
                out_copy(i).start()
            for i in range(NOUT + AT):
                out_copy(i).wait()

    scratch = [
        pltpu.VMEM((4, M // 2, S), U32),
        pltpu.VMEM((KS, M), BF16),
        pltpu.VMEM((M,), BF16),
        pltpu.VMEM((KS + 1, M, LANE), F32),
        pltpu.VMEM((LANE // 2, 2 * LANE), U32),
        pltpu.VMEM((M // 2, S), U32),
        pltpu.VMEM((S // 2, MP), U32),
        pltpu.VMEM((5, XH // 2, D), U32),
        pltpu.VMEM((S // 2 + 8, C), U32),
        [pltpu.VMEM((4 * min(TP, M // 2 - kt * TP) * 8, LANE), U32)
         for kt in range(KT)],
        pltpu.VMEM((H // 2, MP // 2, 2 * D), U32),
        pltpu.VMEM((H // 2, x_cols, 2 * D), U32),
        pltpu.VMEM((QIT, C * 8, LANE), U32),
        pltpu.VMEM((H, C // 2, 2 * D), U32),
        pltpu.VMEM((H, M // 2, D), U32),
        pltpu.VMEM((H, S // 2, D), U32),
        pltpu.VMEM((S // 2, D), U32),
        pltpu.VMEM((S // 2, D), U32),
        pltpu.VMEM((5, (nq - 1) * D // 2, LANE), U32),
        pltpu.VMEM((5, (nq - 1) * D // 2, LANE), U32),
        pltpu.VMEM((2, tq, tq), BF16),
        [pltpu.VMEM((7, tq // 2, n * D), BF16) for n in (2, 3)],
        pltpu.VMEM((2, M, S // 2), F32),
        pltpu.VMEM((S // D, M, D), F32),
        pltpu.VMEM((AT + 1, S, LANE), BF16),
        pltpu.VMEM((S, 2 * M - AT * LANE), BF16),
        pltpu.SemaphoreType.DMA((XC,)),
        pltpu.SemaphoreType.DMA((KT,)),
        pltpu.SemaphoreType.DMA((QIT,)),
        pltpu.SemaphoreType.DMA((QIT,)),
        pltpu.SemaphoreType.DMA((2,)),
        pltpu.SemaphoreType.DMA((3,)),
        pltpu.SemaphoreType.DMA((S // D + AT,)),
    ]
    return kernel, scratch


_DEFAULT = dict(
    tq=512, a_width=16, ao_row=240, link_back=176, link_part=32, pace_row=16,
    pace_step=32, use_a=1, h0=0, body_chunks=123456, kv_top=51473, kv_bot=26, s_ord=5147236,
    o_ord=5241736, p_ord=1234567, o_link=32, o_half=6,
    q_jobs=(2, 4, 4, 4, 1, 3, 1, 3, 5, 6, 6, 1, 2, 1),
    xs_from=3, s_link=48, s_due=6, s_row=120, q_pin=2,
    seq="K0 Q0 T K1!4 Q1 V0 F P0 K2@1112 Q2 O0 V1!4 P1 K3@2116 Q3 O1 V2@4016 P2!6 V3@3114 O2 P3!13 I O3")


def _build(**kw):
    cfg = dict(_DEFAULT)
    cfg.update(kw)
    kernel, scratch = _make_kernel(cfg)

    def run(A_q, A_k, A_v, A_shift_k, A_ssm_k, A_ssm_D, B_x, B_c_kv, B_w_q, B_w_uk,
            B_w_uv, B_w_o):
        tr = lambda a: jnp.swapaxes(a, 1, 2).reshape(M, S)
        args = (
            tr(A_q), tr(A_k), tr(A_v), A_shift_k.T, A_ssm_k, A_ssm_D, tr(B_x),
            B_c_kv.reshape(S, C),
            B_w_q.reshape(M // 2, 2 * H, D), B_w_uk.reshape(C // 2, 2 * H, D),
            B_w_uv.reshape(C // 2, 2 * H, D),
            jnp.swapaxes(B_w_o, 1, 2),
        )
        out = pl.pallas_call(
            kernel,
            in_specs=[pl.BlockSpec(memory_space=pl.ANY)] * len(args),
            out_specs=pl.BlockSpec(memory_space=pl.ANY),
            out_shape=jax.ShapeDtypeStruct((S, 2 * M), BF16),
            scratch_shapes=scratch,
            compiler_params=pltpu.CompilerParams(
                vmem_limit_bytes=126 * 1024 * 1024,
                disable_bounds_checks=True),
        )(*args)
        return out.reshape(1, S, 2 * M)

    return run


_run = _build()


@jax.jit
def pallas_concat_heads__ssm_conv_h3__compressed_kv_cla__prompt_kernel(
    A_q: jax.Array,
    A_k: jax.Array,
    A_v: jax.Array,
    A_shift_k: jax.Array,
    A_ssm_k: jax.Array,
    A_ssm_D: jax.Array,
    B_x: jax.Array,
    B_c_kv: jax.Array,
    B_w_q: jax.Array,
    B_w_uk: jax.Array,
    B_w_uv: jax.Array,
    B_w_o: jax.Array,
):
    return _run(A_q, A_k, A_v, A_shift_k, A_ssm_k, A_ssm_D, B_x, B_c_kv, B_w_q,
                B_w_uk, B_w_uv, B_w_o)
```

```python
import functools

import jax
import jax.numpy as jnp
from jax import lax
import jax.experimental.pallas as pl
import jax.experimental.pallas.tpu as pltpu

F32 = jnp.float32
BF16 = jnp.bfloat16
U32 = jnp.uint32

S = 2048
M = 448
MP = 512
C = 1024
H = 16
D = 256
KS = 4
LANE = 128
NB = S // LANE
AR = 32
A_STEPS = M // AR
LOG2E = 1.4426950408889634
QSCALE = D ** -0.5 * LOG2E
NEG = -1e30

NT = (((1,), (1,)), ((), ()))


def _dot(a, b):
    return jnp.dot(a, b, preferred_element_type=F32)


def _dot_nt(a, b):
    return lax.dot_general(a, b, NT, preferred_element_type=F32)


def _bf(x):
    return pltpu.bitcast(x, BF16)


def _u32(x):
    return pltpu.bitcast(x, U32)


def _h(r0, n):
    return pl.ds(r0 // 2, n // 2)


def _repack(ev, od):
    lo = (ev & jnp.uint32(0xFFFF)) | (od << 16)
    hi = (ev >> 16) | (od & jnp.uint32(0xFFFF0000))
    return lo, hi


def _split(w):
    return (pltpu.bitcast(w << 16, F32), pltpu.bitcast(w & jnp.uint32(0xFFFF0000), F32))


def _join(lo, hi):
    half = jnp.uint32(0x8000)
    lo = (pltpu.bitcast(lo, U32) + half) >> 16
    hi = (pltpu.bitcast(hi, U32) + half) & jnp.uint32(0xFFFF0000)
    return lo | hi


def _add(a, b):
    return _join(a[0] + b[0], a[1] + b[1])


def _sub(a, b):
    return _join(a[0] - b[0], a[1] - b[1])


def _opaque_zero(vals):
    acc = None
    for v in vals:
        b = v if v.dtype == U32 else pltpu.bitcast(v, U32)
        for r in range(0, b.shape[0], 8):
            for c in range(0, b.shape[1], LANE):
                t = b[r:r + 8, c:c + LANE]
                acc = t if acc is None else acc | t
    return jnp.minimum((acc >> 1).astype(jnp.int32), 0)


def _pin(x, zero, r=0, c=0):
    t = pltpu.bitcast(pltpu.bitcast(x[r:r + 8, c:c + LANE], jnp.int32) + zero, x.dtype)
    row = ([x[r:r + 8, :c]] if c > 0 else []) + [t] + (
        [x[r:r + 8, c + LANE:]] if c + LANE < x.shape[1] else [])
    row = jnp.concatenate(row, axis=1) if len(row) > 1 else row[0]
    col = ([x[:r, :]] if r > 0 else []) + [row] + ([x[r + 8:, :]] if r + 8 < x.shape[0] else [])
    return jnp.concatenate(col, axis=0) if len(col) > 1 else col[0]


def _digits(n):
    return [int(c) for c in str(n)]


def _rowcat(xs):
    return jnp.concatenate(xs, axis=0) if len(xs) > 1 else xs[0]


def _lanecat(xs):
    return jnp.concatenate(xs, axis=1) if len(xs) > 1 else xs[0]


def _make_kernel(cfg):
    tq = cfg["tq"]
    nq = S // tq
    nsub = tq // LANE
    KT = MP // LANE
    TP = LANE // 2
    XC = 4
    x_cols = S // XC
    QP = 2
    QIT = H // 2 // QP
    XH = (S - x_cols) // 2
    CP = 176
    AT = 3

    def kernel(aq_hbm, ak_hbm, av_hbm, sh_hbm, ssm_hbm, dd_hbm, x_hbm, c_hbm,
               wq_hbm, wk_hbm, wv_hbm, wo_hbm,
               out_hbm,
               a_v, sh_v, dd_v, par_v, f_v,
               xt_v, x_v, xs_v, c_v, wqs_v, wq_v, qacc, ws_v, wkv_v, wo_v,
               q_all, k_s, v_s, kb_s, vb_s, pd_s, pa_s, ra_t, rb_t, oa_v, out_v,
               sem_x, sem_wq, sem_w, sem_c, sem_s, sem_a, sem_out):
        x32, c32, wq32, wk32, wv32, wo32 = (
            r.bitcast(U32) for r in (x_hbm, c_hbm, wq_hbm, wk_hbm, wv_hbm, wo_hbm))
        a32 = [r.bitcast(U32) for r in (ak_hbm, av_hbm, ssm_hbm, aq_hbm)]

        sa_v = qacc

        def x_copy(i):
            cs = pl.ds(i * x_cols, x_cols)
            return pltpu.make_async_copy(x32.at[:, cs], xt_v.at[:, cs], sem_x.at[i])

        def wq_pairs(kt):
            return min(TP, M // 2 - kt * TP)

        def wq_copies(kt):
            n = wq_pairs(kt)
            dst = wqs_v[kt].reshape(4, n, 8, LANE)
            return [pltpu.make_async_copy(
                wq32.at[pl.ds(kt * TP, n), pl.ds(8 * (k // 2), 8), pl.ds((k % 2) * LANE, LANE)],
                dst.at[k], sem_wq.at[kt]) for k in range(4)]

        def wq_wait(kt):
            pltpu.make_async_copy(wqs_v[kt], wqs_v[kt], sem_wq.at[kt]).wait()

        def w_copies(g):
            dst = ws_v.reshape(8, C // 2, 8, LANE)
            src = (wk32, wv32)[g // 2]
            return [pltpu.make_async_copy(
                src.at[:, pl.ds(8 * par, 8), pl.ds((g % 2) * LANE, LANE)],
                dst.at[2 * g + par], sem_w.at[g]) for par in range(2)]

        def w_wait(g):
            pltpu.make_async_copy(ws_v.at[g], ws_v.at[g], sem_w.at[g]).wait()

        c_bounds = [0, CP, 2 * CP, S // 4]

        def c_copies(p):
            r0, n = c_bounds[p], c_bounds[p + 1] - c_bounds[p]
            return [pltpu.make_async_copy(c32.at[rs], c_v.at[rs], sem_c.at[p])
                    for rs in (pl.ds(r0, n), pl.ds(S // 4 + r0, n))]

        wo_copy = pltpu.make_async_copy(wo32, wo_v, sem_a.at[0])

        a_parts = [pl.ds(0, AR // 2), pl.ds(AR // 2, M // 2 - AR // 2)]

        def a_start(part):
            rs = a_parts[part]
            for k in range(4):
                pltpu.make_async_copy(
                    a32[k].at[rs], a_v.at[k, rs], sem_a.at[1 + part]).start()

        def a_wait(part):
            view = a_v.at[:, a_parts[part]]
            pltpu.make_async_copy(view, view, sem_a.at[1 + part]).wait()

        small = [pltpu.make_async_copy(sh_hbm, sh_v, sem_s.at[0]),
                 pltpu.make_async_copy(dd_hbm, dd_v, sem_s.at[1])]

        link = [None]
        pace = [None]

        def set_link(res, row=None, pacer=None):
            if row is None:
                row = res.shape[0] - cfg["link_back"]
            link[0] = _opaque_zero([res[row:row + 8, res.shape[1] - LANE:]])
            pace[0] = res if pacer is None else pacer

        def linked(x):
            return x if link[0] is None else _pin(x, link[0])

        def paced(w):
            res = pace[0]
            if res is None or link[0] is None or not cfg["pace_step"]:
                return w
            rows = []
            r0, step = cfg["pace_row"], cfg["pace_step"]
            if res.shape[0] < 400:
                r0, step = 0, 8
            if res.shape[0] < 200:
                return w
            zs = [_opaque_zero([res[r:r + 8, res.shape[1] - LANE:]])
                  for r in range(r0, r0 + 8 * step, step)]
            for r in range(0, w.shape[0], 8):
                z = zs[7 - (r // 8) % 8]
                t = pltpu.bitcast(w[r:r + 8, :], jnp.int32)
                rows.append(pltpu.bitcast(t + _lanecat([z] * (w.shape[1] // LANE)), U32))
            return _rowcat(rows)

        for cp in small:
            cp.start()
        x_copy(0).start()
        for cp in wq_copies(0):
            cp.start()

        def zero_body(k, carry):
            n = LANE // (S // D)
            bi = lax.broadcasted_iota(jnp.int32, (n, LANE), 0) + k * n
            mi = lax.broadcasted_iota(jnp.int32, (n, LANE), 1)
            ph = ((4 * mi + 1) * bi) & 511
            ang = ph.astype(F32) * (2.0 * 3.141592653589793 / 512.0)
            rs = pl.ds(pl.multiple_of(k * (n // 2), n // 2), n // 2)
            f_v[rs, 0:LANE] = _u32(jnp.cos(ang).astype(BF16))
            f_v[rs, LANE:] = _u32((-jnp.sin(ang)).astype(BF16))

            rb_t[k] = jnp.zeros((M, D), F32)
            cs = pl.ds(pl.multiple_of((k % 4) * D, D), D)
            ra_t[k // 4, 0:LANE, cs] = jnp.zeros((LANE, D), F32)
            ra_t[k // 4, AT * LANE:, cs] = jnp.zeros((M - AT * LANE, D), F32)
            return carry

        lax.fori_loop(0, S // D, zero_body, 0)
        c_v[S // 2:, :] = jnp.zeros((8, C), U32)

        for kt in range(1, KT):
            for cp in wq_copies(kt):
                cp.start()
        with jax.named_scope("small_wait"):
            for cp in small:
                cp.wait()
        sh = sh_v[...].astype(F32)
        for j in range(KS):
            par_v[j] = jnp.broadcast_to(sh[j:j + 1, :], (LANE, M)).T
        dd = dd_v[...].astype(F32).reshape(1, M)
        par_v[KS] = jnp.broadcast_to(dd, (LANE, M)).T

        def x_transpose(i):
            xt = xt_v[:, pl.ds(i * x_cols, x_cols)]
            xt = _rowcat([xt, jnp.zeros((MP // 2 - M // 2, x_cols), U32)])
            x_v[_h(i * x_cols, x_cols), :] = _u32(_bf(xt).astype(F32).T.astype(BF16))

        def q_early(kt, keep=False, jobs=()):
            first, last = kt == 0, kt == KT - 1
            n = wq_pairs(kt)
            cols = pl.ds(kt * LANE, LANE)
            if not keep:
                link[0] = None
            for j in range(H // 2):
                ws = []
                for half in range(2):
                    ev, od = (wqs_v[kt][pl.ds((2 * par + half) * n * 8 + j, n, stride=8), :]
                              for par in range(2))
                    ws.append(_repack(ev, od))
                w = _lanecat([ws[0][0], ws[1][0], ws[0][1], ws[1][1]])
                if n < TP:
                    w = _rowcat([w, jnp.zeros((TP - n, 2 * D), U32)])
                wq_v[j, pl.ds(kt * TP, TP), :] = w
                lhs = linked(x_v[_h(0, x_cols), cols])
                j0 = cfg["xs_from"]
                if jobs and j >= j0:
                    nj = H // 2 - j0
                    mine = jobs[(j - j0) * len(jobs) // nj:(j - j0 + 1) * len(jobs) // nj]
                    for k, job in enumerate(mine):
                        lhs = _pin(lhs, _opaque_zero(job()), 8 * (1 + k * 30 // len(mine)))
                d = _dot(_bf(lhs), _bf(w))
                set_link(d)
                if not first:
                    d = d + pltpu.bitcast(qacc[j], F32)
                if last:
                    d = (d * QSCALE).astype(BF16)
                    for t in range(2):
                        q_all[2 * j + t, _h(0, x_cols), :] = _u32(d[:, t * D:(t + 1) * D])
                else:
                    qacc[j] = pltpu.bitcast(d, U32)

        with jax.named_scope("x_wait"):
            x_copy(0).wait()
        x_transpose(0)
        for i in range(1, XC):
            x_copy(i).start()
        for g in range(QIT):
            for cp in w_copies(g) + (c_copies(g) if g < QIT - 1 else []):
                cp.start()
        wo_copy.start()
        a_start(0)
        a_start(1)
        with jax.named_scope("wq_wait"):
            wq_wait(0)
        q_early(0)
        with jax.named_scope("wq_wait"):
            wq_wait(1)
        q_early(1)
        with jax.named_scope("wq_wait"):
            wq_wait(2)
            wq_wait(3)
            for i in range(1, XC):
                x_copy(i).wait()
        for i in range(1, XC):
            x_transpose(i)

        def x_sums(u):
            a11, a12, a21, a22 = (
                _split(x_v[pl.ds((x_cols + rb * XH) // 2 + 8 * u, 8), cb * D:(cb + 1) * D])
                for rb in range(2) for cb in range(2))
            outs = [_add(a11, a22), _add(a21, a22), _add(a11, a12), _sub(a21, a11),
                    _sub(a12, a22)]
            for k, o in enumerate(outs):
                xs_v[k, 8 * u:8 * u + 8, :] = o
            return outs

        q_early(2, jobs=[functools.partial(x_sums, u) for u in range(XH // 16)])
        q_early(3, keep=True)

        def unpack(it, sub, j):
            g = it
            ev, od = (ws_v[g, pl.ds((par * (C // 2) + sub * TP) * 8 + j, TP, stride=8), :]
                      for par in range(2))
            lo, hi = _repack(ev, od)
            rows = pl.ds(sub * TP, TP)
            cols = pl.ds(pl.multiple_of(g * LANE, LANE), LANE)
            wkv_v[2 * j, rows, cols] = lo
            wkv_v[2 * j + 1, rows, cols] = hi
            return [lo, hi]

        def a_sums(it, u, part):
            r0 = jnp.clip((it - 1) * CP, 0, S // 4 - CP) + 8 * u
            src = [jnp.where(it == 0, S // 2, r0 + rb * (S // 4)) for rb in range(2)]
            r0 = pl.multiple_of(r0, 8)
            kw = C // 2
            w = kw // cfg["c_split"]
            a11, a12, a21, a22 = (
                _split(c_v[pl.ds(pl.multiple_of(src[rb], 8), 8), pl.ds(cb * kw + part * w, w)])
                for rb in range(2) for cb in range(2))
            outs = [_add(a11, a22), _add(a21, a22), _add(a11, a12), _sub(a21, a11),
                    _sub(a12, a22)]
            for k, o in enumerate(outs):
                sa_v[k, pl.ds(r0, 8), pl.ds(part * w, w)] = o
            return outs

        units = [functools.partial(unpack, sub=s_, j=j_)
                 for s_ in range(C // 2 // TP) for j_ in range(H // 2)]
        extra = [functools.partial(a_sums, u=u_, part=p_)
                 for u_ in range(CP // 8) for p_ in range(cfg["c_split"])]
        total = len(units) + len(extra)
        for k_, job_ in enumerate(extra):
            units.insert((2 * k_ + 1) * total // (2 * len(extra)), job_)

        def q_pair(pair, todo):
            raw = lambda r, c: _lanecat([
                wq_v[pair, r * LANE:(r + 1) * LANE, pl.ds(t * D + c * LANE, LANE)]
                for t in range(2)])
            b = lambda r, c: _split(raw(r, c))
            sb = {1: _add(b(0, 0), b(1, 1)), 2: raw(0, 0), 3: _sub(b(0, 1), b(1, 1)),
                  4: _sub(b(1, 0), b(0, 0)), 5: raw(1, 1), 6: _add(b(0, 0), b(0, 1)),
                  7: _add(b(1, 0), b(1, 1))}
            n = XH // 2
            for rho in range(2):
                def sa(m):
                    if m == 3:
                        return x_v[_h(x_cols + rho * n, n), 0:D]
                    if m == 4:
                        return x_v[_h(x_cols + XH + rho * n, n), D:]
                    return xs_v[{1: 0, 2: 1, 5: 2, 6: 3, 7: 4}[m], _h(rho * n, n), :]

                def put(half, c0, c1):
                    rows = _h(x_cols + half * XH + rho * n, n)
                    for t in range(2):
                        q = _lanecat([c[:, t * LANE:(t + 1) * LANE] for c in (c0, c1)])
                        q_all[2 * pair + t, rows, :] = _u32((q * QSCALE).astype(BF16))

                p = {}
                for pos, m in enumerate((5, 1, 4, 7, 3, 2, 6)):
                    lhs = linked(sa(m))
                    nj = min(len(todo), cfg["q_jobs"][7 * rho + pos])
                    jobs = [todo.pop()(it=pair // QP) for _ in range(nj)]
                    for k, job in enumerate(jobs):
                        lhs = _pin(lhs, _opaque_zero(job), 8 * (1 + k * (n // 16 - 1) // nj))
                    p[m] = _dot(_bf(lhs), _bf(sb[m]))
                    set_link(p[m])
                    if m == 3:
                        put(0, (p[1] + p[4]) + (p[7] - p[5]), p[3] + p[5])
                put(1, p[2] + p[4], (p[1] + p[3]) + (p[6] - p[2]))

        def q_body(it, carry):
            with jax.named_scope("w_wait"):
                w_wait(it)
                for p in range(QIT - 1):
                    @pl.when(it == p + 1)
                    def _():
                        for cp in c_copies(p):
                            cp.wait()
            link[0] = None
            todo = units[::-1]
            for p in range(QP):
                q_pair(QP * it + p, todo)
            assert not todo
            return carry

        with jax.named_scope("q_loop"):
            lax.fori_loop(0, QIT, q_body, 0)
        wo_copy.wait()
        a_wait(0)

        tri = (lax.broadcasted_iota(jnp.int32, (LANE, LANE), 1)
               <= lax.broadcasted_iota(jnp.int32, (LANE, LANE), 0))

        NOUT = S // D

        def out_copy(i):
            if i >= NOUT:
                t = i - NOUT
                return pltpu.make_async_copy(
                    oa_v.at[t], out_hbm.at[:, pl.ds(t * LANE, LANE)], sem_out.at[i])
            rs = pl.ds(i * D, D)
            return pltpu.make_async_copy(
                out_v.at[rs], out_hbm.at[rs, pl.ds(AT * LANE, 2 * M - AT * LANE)], sem_out.at[i])

        body_chunks = _digits(cfg["body_chunks"])

        def b_out(k, tot):
            c0 = (k * D) % (S // 2)
            full = _rowcat([ra_t[k * D // (S // 2), AT * LANE:, c0:c0 + D], tot]).T
            out_v[k * D:(k + 1) * D, :] = full.astype(BF16)
            return full

        def head_step(h, carry):
            with jax.named_scope("step"):
                return head_step_(h, carry)

        def head_step_(h, carry):
            with_a = cfg["use_a"]

            @pl.when(h == A_STEPS)
            def _():
                for t in range(AT):
                    out_copy(NOUT + t).start()

            @pl.when(h == cfg["h0"] + 1)
            def _():
                a_wait(1)

            link[0] = None
            n2 = AR // 2
            a_rows2 = pl.ds(pl.multiple_of(jnp.minimum(h, A_STEPS - 1) * n2, n2), n2)
            a_rows = pl.ds(pl.multiple_of(jnp.minimum(h, A_STEPS - 1) * AR, AR), AR)

            kw = C // 2
            pending = []
            chains = {i: [] for i in range(nq + 1)}
            deadline = [None]

            def flush_pending(x, row):
                done = list(pending)
                del pending[:]
                if not done:
                    return x
                x = _pin(x, _opaque_zero([f for _, f in done]), row)

                if any(k is not None for k, _ in done):
                    @pl.when(h == H - 1)
                    def _():
                        for k, _f in done:
                            if k is not None:
                                out_copy(k).start()
                return x

            def a_fwd():
                kk = _bf(a_v[0, a_rows2, :]).astype(F32)
                lane = lax.broadcasted_iota(jnp.int32, (AR, LANE), 1)
                coef = [par_v[j, a_rows, :] for j in range(KS)]
                rolled = [kk] + [pltpu.roll(kk, j, 1) for j in range(1, KS)]
                vv = _bf(a_v[1, a_rows2, :]).astype(F32)
                kv_blocks = []
                for a in range(NB):
                    cs = slice(a * LANE, (a + 1) * LANE)
                    acc = rolled[0][:, cs] * coef[0]
                    for j in range(1, KS):
                        t = rolled[j][:, cs]
                        if a == 0:
                            t = jnp.where(lane >= j, t, 0.0)
                        acc = acc + t * coef[j]
                    kv_blocks.append(acc * vv[:, cs])
                hk = a_v[2, a_rows2, :]
                hk = _rowcat([hk[:, a * LANE:(a + 1) * LANE] for a in range(NB)])
                fm = _bf(f_v[...])
                hs = _dot(_bf(linked(hk)), fm)
                kv = linked(_rowcat(kv_blocks)).astype(BF16)
                xs = _dot(kv, fm)
                set_link(xs)
                return kv, xs, hs

            def a_conv(xs, hs):
                def tile(v, a, g, part):
                    r = a * AR + 8 * g
                    return v[r:r + 8, part * LANE:(part + 1) * LANE]

                z = {}
                gate = None
                width = cfg["a_width"]
                for g in range(AR // 8):
                    hr = [tile(hs, 0, g, 0)] + [
                        tile(hs, j, g, 0) - tile(hs, j - 1, g, 1) for j in range(1, NB)]
                    hi = [tile(hs, 0, g, 1)] + [
                        tile(hs, j, g, 1) + tile(hs, j - 1, g, 0) for j in range(1, NB)]
                    for c0 in range(0, NB, width):
                        for a in range(c0 + width):
                            xr, xi = tile(xs, a, g, 0), tile(xs, a, g, 1)
                            if gate is not None:
                                xr, xi = _pin(xr, gate), _pin(xi, gate)
                            for c in range(max(c0, a), c0 + width):
                                j = c - a
                                tr = xr * hr[j] - xi * hi[j]
                                ti = xr * hi[j] + xi * hr[j]
                                z[c, g] = (tr, ti) if a == 0 else (z[c, g][0] + tr, z[c, g][1] + ti)
                            gate = _opaque_zero(list(z[c0 + width - 1, g]))
                            chains[nq].append(gate)
                return z

            def a_inv(kv, z, flush=False):
                fm = _bf(f_v[...])
                ng = AR // 8
                ys = []
                for u in range(2):
                    rows = [_lanecat(z[c, g]) for g in range(u * ng // 2, (u + 1) * ng // 2)
                            for c in range(NB)]
                    lhs = linked(_rowcat(rows))
                    if flush:
                        lhs = flush_pending(lhs, 8)
                    ys.append(_dot_nt(lhs.astype(BF16), fm))
                y = _rowcat(ys)
                dd = par_v[KS, a_rows, :]
                for c in range(NB):
                    cs = slice(c * LANE, (c + 1) * LANE)
                    yc = _rowcat([y[(g * NB + c) * 8:(g * NB + c + 1) * 8, :] for g in range(ng)])
                    qq = _bf(a_v[3, a_rows2, cs]).astype(F32)
                    kvf = kv[c * AR:(c + 1) * AR, :].astype(F32)
                    c2 = (c % (NB // 2)) * LANE
                    ra_t[c // (NB // 2), a_rows, c2:c2 + LANE] = qq * (yc * (1.0 / LANE) + kvf * dd)

            def a_out():
                slab = jnp.clip(h // 4 - 1, 0, AT - 1)
                half = h % 2
                x = ra_t[half, pl.ds(pl.multiple_of(slab * LANE, LANE), LANE), :]
                xt = x.T
                dst = jnp.where(h >= A_STEPS, AT, slab)
                oa_v[dst, pl.ds(pl.multiple_of(half * (S // 2), S // 2), S // 2), :] = xt.astype(BF16)
                return xt

            def w_blk(r, c):
                return wkv_v[h, _h(r * kw, kw), pl.ds(c * LANE, LANE)]

            def one_pass(lhs, w, flush):
                lhs = linked(lhs)
                if flush:
                    lhs = flush_pending(lhs, cfg["ao_row"])
                if deadline[0] is not None:
                    if deadline[0][0] == 0:
                        lhs = _pin(lhs, deadline[0][1], cfg["ao_row"] - 8)
                        deadline[0] = None
                    else:
                        deadline[0] = (deadline[0][0] - 1, deadline[0][1])
                d = _dot(_bf(lhs), _bf(paced(w)))
                set_link(d)
                return d

            def b_op(which, m):
                raw = lambda r, c: w_blk(r, 2 * which + c)
                blk = lambda r, c: _split(raw(r, c))
                return {1: lambda: _add(blk(0, 0), blk(1, 1)),
                        2: lambda: raw(0, 0),
                        3: lambda: _sub(blk(0, 1), blk(1, 1)),
                        4: lambda: _sub(blk(1, 0), blk(0, 0)),
                        5: lambda: raw(1, 1),
                        6: lambda: _add(blk(0, 0), blk(0, 1)),
                        7: lambda: _add(blk(1, 0), blk(1, 1))}[m]()

            def a_op(m, rho):
                rs = _h(rho * tq, tq)
                if m == 3:
                    return c_v[rs, 0:kw]
                if m == 4:
                    return c_v[_h(S // 2 + rho * tq, tq), kw:]
                return sa_v[{1: 0, 2: 1, 5: 2, 6: 3, 7: 4}[m], rs, :]

            b_cache, prod = {}, {}

            def kv_proj(which, blk, flush):
                rho = blk % 2
                for k, m in enumerate(_digits(cfg["kv_top" if blk < 2 else "kv_bot"])):
                    if (which, m) not in b_cache:
                        b_cache[which, m] = b_op(which, m)
                    prod[which, m, rho] = one_pass(a_op(m, rho), b_cache[which, m], k == flush)
                p = lambda m: prod[which, m, rho]
                if blk < 2:
                    return [(p(1) + p(4)) + (p(7) - p(5)), p(3) + p(5)]
                return [p(2) + p(4), (p(1) + p(3)) + (p(6) - p(2))]

            def k_proj(blk, flush=-1):
                k = kv_proj(0, blk, flush)
                k_s[_h(blk * tq, tq), :] = _u32(_lanecat(k).astype(BF16))
                if blk < nq - 1:
                    b = lambda r, c: k[r][c * D:(c + 1) * D, :]
                    sums = [b(0, 0) + b(1, 1), b(0, 1) - b(1, 1), b(1, 0) - b(0, 0),
                            b(0, 0) + b(0, 1), b(1, 0) + b(1, 1)]
                    for n, x in enumerate(sums):
                        kb_s[n, _h(blk * D, D), :] = _u32(x.astype(BF16))

            def v_proj(blk, flush=-1):
                v = kv_proj(1, blk, flush)
                v_s[_h(blk * tq, tq), :] = _u32(_lanecat(v).astype(BF16))
                if blk < nq - 1:
                    b = lambda r, c: v[c][r * D:(r + 1) * D, :]
                    sums = [b(0, 0) + b(1, 1), b(0, 1) - b(1, 1), b(1, 0) - b(0, 0),
                            b(0, 0) + b(0, 1), b(1, 0) + b(1, 1)]
                    for k, x in enumerate(sums):
                        vb_s[k, _h(blk * D, D), :] = _u32(x.astype(BF16))

            def qk(i, flush=False):
                r0 = i * tq
                off = None
                if i > 0:
                    raw = lambda r, c: q_all[h, _h(r0 + r * D, D), c * LANE:(c + 1) * LANE]
                    a = lambda r, c: _split(raw(r, c))
                    sa = {1: _add(a(0, 0), a(1, 1)), 2: _add(a(1, 0), a(1, 1)), 3: raw(0, 0),
                          4: raw(1, 1), 5: _add(a(0, 0), a(0, 1)), 6: _sub(a(1, 0), a(0, 0)),
                          7: _sub(a(0, 1), a(1, 1))}

                    def sb(m, j, t):
                        if m in (2, 5):
                            c = 0 if m == 2 else 1
                            rows = _h(j * tq + c * D + t * LANE, LANE)
                            return k_s[rows, c * LANE:(c + 1) * LANE]
                        n = {1: 0, 3: 1, 4: 2, 6: 3, 7: 4}[m]
                        return kb_s[n, _h(j * D + t * LANE, LANE), :]

                    top, bot, due = {}, {}, []
                    n_dot = 0
                    for j in range(i):
                        for t in range(2):
                            p = {}
                            for n, m in enumerate(_digits(cfg["s_ord"])):
                                lhs = linked(sa[m])
                                if due and n == cfg["s_due"]:
                                    lhs = _pin(lhs, due.pop(), cfg["s_row"])
                                p[m] = _dot_nt(_bf(lhs), _bf(sb(m, j, t)))
                                n_dot += 1
                                if n_dot % 4 == 0:
                                    set_link(p[m], cfg["s_link"])
                            top[4 * j + t] = (p[1] + p[4]) + (p[7] - p[5])
                            top[4 * j + 2 + t] = p[3] + p[5]
                            bot[4 * j + t] = p[2] + p[4]
                            bot[4 * j + 2 + t] = (p[1] + p[3]) + (p[6] - p[2])
                            due.append(_opaque_zero(
                                [x[4 * j + c + t] for x in (top, bot) for c in (0, 2)]))
                    off = _rowcat([_lanecat([x[c] for c in range(4 * i)]) for x in (top, bot)])
                q = linked(q_all[h, _h(r0, tq), :])
                if off is not None:
                    q = _pin(q, due.pop(), cfg["ao_row"] - 8)
                main = _dot_nt(_bf(q), _bf(k_s[_h(r0, LANE), :]))
                parts = [main if off is None else _lanecat([off, main])]
                for j in range(1, nsub):
                    q = linked(q_all[h, _h(r0 + LANE * j, tq - LANE * j), :])
                    if flush and j == cfg["q_pin"]:
                        q = flush_pending(q, 8)
                    parts.append(_dot_nt(_bf(q), _bf(k_s[_h(r0 + LANE * j, LANE), :])))
                set_link(parts[2], cfg["link_part"], main)
                return parts

            def exps(i, parts):
                sas, mbs = [], []
                for a in range(nsub):
                    blocks = [parts[j][LANE * (a - j):LANE * (a - j + 1), :] for j in range(a + 1)]
                    last = blocks[-1]
                    w = last.shape[1]
                    dg = jnp.where(tri, last[:, w - LANE:], NEG)
                    blocks[-1] = dg if w == LANE else _lanecat([last[:, :w - LANE], dg])
                    sas.append(_lanecat(blocks))
                    lane_max = functools.reduce(jnp.maximum, [
                        sas[a][:, t:t + LANE] for t in range(0, sas[a].shape[1], LANE)])
                    mx = jnp.max(lane_max, axis=1, keepdims=True)
                    if i > 0:
                        mx = mx + jnp.log2(jnp.sum(jnp.exp2(lane_max - mx), axis=1, keepdims=True))
                    mbs.append(jnp.broadcast_to(mx, (LANE, LANE)))
                chain = _opaque_zero([b[b.shape[0] - 8:, b.shape[1] - LANE:] for b in parts])
                pg, psums = {}, {}
                for r in range(0, tq // 2, 8):
                    for row in (r, r + tq // 2):
                        a, g = divmod(row, LANE)
                        mg = _pin(mbs[a][g:g + 8, :], chain)
                        pg[row] = [jnp.exp2(sas[a][g:g + 8, t:t + LANE] - mg)
                                   for t in range(0, sas[a].shape[1], LANE)]
                        psums[row] = functools.reduce(jnp.add, pg[row])
                        chain = _opaque_zero([psums[row]])
                        chains[i].append(chain)
                return pg, psums

            def softmax(i, pg, psums):
                r0 = i * tq
                pd, pa = pd_s.at[i % 2], pa_s[i % 2]
                first = lambda x, c=0: _pin(x, link[0], 0, c).astype(BF16)
                nt0 = r0 // LANE
                ls = []
                for a in range(nsub):
                    rows = range(LANE * a, LANE * (a + 1), 8)
                    ls.append(jnp.sum(_rowcat([psums[r] for r in rows]), axis=1, keepdims=True))
                    pd[LANE * a:LANE * (a + 1), 0:LANE * (a + 1)] = first(
                        _rowcat([_lanecat(pg[r][nt0:]) for r in rows]), LANE * a)
                if i > 0:
                    quad = lambda rh, ch: _rowcat([
                        _lanecat([pg[rh * (tq // 2) + r][4 * j + 2 * ch + t]
                                  for j in range(i) for t in range(2)])
                        for r in range(0, tq // 2, 8)])
                    a11, a12, a21, a22 = quad(0, 0), quad(0, 1), quad(1, 0), quad(1, 1)
                    ops = [a11 + a22, a21 + a22, a11, a22, a11 + a12, a21 - a11, a12 - a22]
                    for m, x in enumerate(ops):
                        if i == 3:
                            x = _pin(x, link[0], 0, 2 * D)
                        pa[m, :, 0:i * D] = first(x)
                return ls

            def pv(i, ls, flush=-1):
                r0 = i * tq
                pd, pa = pd_s.at[i % 2], pa_s[i % 2]
                off = None
                if i > 0:
                    def b_rows(m, j0, j1):
                        if m in (2, 5):
                            q = 0 if m == 2 else 1
                            return _rowcat([
                                v_s[_h(j * tq + q * D, D), q * LANE:(q + 1) * LANE]
                                for j in range(j0, j1)])
                        k = {1: 0, 3: 1, 4: 2, 6: 3, 7: 4}[m]
                        return vb_s[k, _h(j0 * D, (j1 - j0) * D), :]

                    p, n_dot = {}, 0
                    for j0, j1 in {1: [(0, 1)], 2: [(0, 2)], 3: [(0, 2), (2, 3)]}[i]:
                        for m in _digits(cfg["p_ord"]):
                            cols = slice(j0 * D, j1 * D)
                            rhs = b_rows(m, j0, j1)
                            if n_dot == flush:
                                rhs = flush_pending(rhs, 0)
                            rhs = _bf(rhs)
                            n_dot += 1
                            if j1 - j0 == 1 and m == cfg["p_ord"] % 10:
                                d = _rowcat([_dot(pa[m - 1, r:r + LANE, cols], rhs)
                                             for r in (0, LANE)])
                            else:
                                d = _dot(pa[m - 1, :, cols], rhs)
                            p[m] = d if m not in p else p[m] + d
                    off = _rowcat([
                        _lanecat([(p[1] + p[4]) + (p[7] - p[5]), p[3] + p[5]]),
                        _lanecat([p[2] + p[4], (p[1] + p[3]) + (p[6] - p[2])])])
                ctx = []
                for j in range(nsub):
                    c0 = LANE * j
                    ctx.append(_dot(pd[c0:, c0:c0 + LANE], _bf(v_s[_h(r0 + c0, LANE), :])))
                set_link(ctx[2], cfg["link_part"], ctx[0])
                cs = []
                for a in range(nsub):
                    sl = lambda j: slice(LANE * (a - j), LANE * (a - j + 1))
                    r = pl.reciprocal(ls[a], approx=True)
                    terms = [ctx[j][sl(j)] for j in range(a + 1)]
                    if off is not None:
                        terms.append(off[sl(0)])
                    cs.append(functools.reduce(jnp.add, terms) * r)
                return _rowcat(cs)

            wo_cache = {}

            def oproj(i, ctx):
                mh = M // 4
                raw = lambda r, c: wo_v[h, r * mh:(r + 1) * mh, c * LANE:(c + 1) * LANE]
                a = lambda r, c: _split(raw(r, c))
                a_ops = {1: lambda: _add(a(0, 0), a(1, 1)), 2: lambda: _add(a(1, 0), a(1, 1)),
                         3: lambda: raw(0, 0), 4: lambda: raw(1, 1),
                         5: lambda: _add(a(0, 0), a(0, 1)), 6: lambda: _sub(a(1, 0), a(0, 0)),
                         7: lambda: _sub(a(0, 1), a(1, 1))}
                b = lambda r, c: ctx[c * D:(c + 1) * D, r * LANE:(r + 1) * LANE]
                b_ops = {1: lambda: b(0, 0) + b(1, 1), 2: lambda: b(0, 0),
                         3: lambda: b(0, 1) - b(1, 1), 4: lambda: b(1, 0) - b(0, 0),
                         5: lambda: b(1, 1), 6: lambda: b(0, 0) + b(0, 1),
                         7: lambda: b(1, 0) + b(1, 1)}
                p = {}
                order = _digits(cfg["o_ord"])
                mm = M // 2
                old = lambda r, c: rb_t[2 * i + c, r * mm:(r + 1) * mm, :]
                terms = {(0, 0): (1, 4, -5, 7), (0, 1): (3, 5), (1, 0): (2, 4), (1, 1): (1, -2, 3, 6)}

                def total(q):
                    acc = old(*q)
                    for m in sorted(terms[q], key=lambda m: order.index(abs(m))):
                        acc = acc + p[m] if m > 0 else acc - p[-m]
                    return acc

                for n, m in enumerate(order):
                    if m not in wo_cache:
                        wo_cache[m] = a_ops[m]()
                    rhs = b_ops[m]().astype(BF16)
                    if n == cfg["o_half"]:
                        lhs = [linked(wo_cache[m][r:r + mh // 2]) for r in (0, mh // 2)]
                        halves = [_dot_nt(_bf(x), rhs) for x in lhs]
                        p[m] = _rowcat(halves)
                        set_link(halves[1], 0)
                    else:
                        p[m] = _dot_nt(_bf(linked(wo_cache[m])), rhs)
                        if (n - (n > cfg["o_half"])) % 2 == 1:
                            set_link(p[m], cfg["o_link"])
                for c in range(2):
                    k = 2 * i + c
                    tot = _rowcat([total((r, c)) for r in range(2)])
                    rb_t[k] = tot
                    if k + 1 in body_chunks:
                        pending.append((k, b_out(k, tot)))

            st = {}
            for op in cfg["seq"].split():
                op, _, dl = op.partition("@")
                if dl:
                    ch = chains[int(dl[0])]
                    deadline[0] = (int(dl[1]), ch[int(dl[2:]) * len(ch) // 16 - 1])
                op, _, fl = op.partition("!")
                fl = int(fl) if fl else -1
                kind, i = op[0], int(op[1:] or 0)
                if kind == "K":
                    k_proj(i, fl)
                elif kind == "V":
                    v_proj(i, fl)
                elif kind == "Q":
                    st["e", i] = exps(i, qk(i, fl >= 0))
                elif kind == "P":
                    st["ctx", i] = pv(i, softmax(i, *st["e", i]), fl)
                elif kind == "O":
                    oproj(i, st["ctx", i])
                elif kind == "T":
                    pending.append((None, a_out()))
                elif kind == "F" and with_a:
                    st["kv"], xs, hs = a_fwd()
                    st["z"] = a_conv(xs, hs)
                elif kind == "I" and with_a:
                    a_inv(st["kv"], st["z"], fl >= 0)
            assert not pending and deadline[0] is None
            return carry

        with jax.named_scope("loop_a"):
            lax.fori_loop(cfg["h0"], H, head_step, 0)
        with jax.named_scope("tail"):
            for i in [k for k in range(NOUT) if k + 1 not in body_chunks]:
                b_out(i, rb_t[i])
                out_copy(i).start()
            for i in range(NOUT + AT):
                out_copy(i).wait()

    scratch = [
        pltpu.VMEM((4, M // 2, S), U32),
        pltpu.VMEM((KS, M), BF16),
        pltpu.VMEM((M,), BF16),
        pltpu.VMEM((KS + 1, M, LANE), F32),
        pltpu.VMEM((LANE // 2, 2 * LANE), U32),
        pltpu.VMEM((M // 2, S), U32),
        pltpu.VMEM((S // 2, MP), U32),
        pltpu.VMEM((5, XH // 2, D), U32),
        pltpu.VMEM((S // 2 + 8, C), U32),
        [pltpu.VMEM((4 * min(TP, M // 2 - kt * TP) * 8, LANE), U32)
         for kt in range(KT)],
        pltpu.VMEM((H // 2, MP // 2, 2 * D), U32),
        pltpu.VMEM((H // 2, x_cols, 2 * D), U32),
        pltpu.VMEM((QIT, C * 8, LANE), U32),
        pltpu.VMEM((H, C // 2, 2 * D), U32),
        pltpu.VMEM((H, M // 2, D), U32),
        pltpu.VMEM((H, S // 2, D), U32),
        pltpu.VMEM((S // 2, D), U32),
        pltpu.VMEM((S // 2, D), U32),
        pltpu.VMEM((5, (nq - 1) * D // 2, LANE), U32),
        pltpu.VMEM((5, (nq - 1) * D // 2, LANE), U32),
        pltpu.VMEM((2, tq, tq), BF16),
        [pltpu.VMEM((7, tq // 2, n * D), BF16) for n in (2, 3)],
        pltpu.VMEM((2, M, S // 2), F32),
        pltpu.VMEM((S // D, M, D), F32),
        pltpu.VMEM((AT + 1, S, LANE), BF16),
        pltpu.VMEM((S, 2 * M - AT * LANE), BF16),
        pltpu.SemaphoreType.DMA((XC,)),
        pltpu.SemaphoreType.DMA((KT,)),
        pltpu.SemaphoreType.DMA((QIT,)),
        pltpu.SemaphoreType.DMA((QIT,)),
        pltpu.SemaphoreType.DMA((2,)),
        pltpu.SemaphoreType.DMA((3,)),
        pltpu.SemaphoreType.DMA((S // D + AT,)),
    ]
    return kernel, scratch


_DEFAULT = dict(
    tq=512, a_width=16, ao_row=240, link_back=176, link_part=32, pace_row=16,
    pace_step=32, use_a=1, h0=0, body_chunks=123456, kv_top=51473, kv_bot=26, s_ord=5147236,
    o_ord=5241736, p_ord=1234567, o_link=32, o_half=6,
    q_jobs=(5, 6, 6, 6, 4, 5, 4, 6, 7, 7, 7, 4, 5, 4),
    xs_from=3, s_link=48, s_due=6, s_row=120, q_pin=2, c_split=4,
    seq="K0 Q0 T K1!4 Q1 V0 F P0 K2@1112 Q2 O0 V1!4 P1 K3@2116 Q3 O1 V2@4016 P2!6 V3@3114 O2 P3!13 I O3")


def _build(**kw):
    cfg = dict(_DEFAULT)
    cfg.update(kw)
    kernel, scratch = _make_kernel(cfg)

    def run(A_q, A_k, A_v, A_shift_k, A_ssm_k, A_ssm_D, B_x, B_c_kv, B_w_q, B_w_uk,
            B_w_uv, B_w_o):
        tr = lambda a: jnp.swapaxes(a, 1, 2).reshape(M, S)
        args = (
            tr(A_q), tr(A_k), tr(A_v), A_shift_k.T, A_ssm_k, A_ssm_D, tr(B_x),
            B_c_kv.reshape(S, C),
            B_w_q.reshape(M // 2, 2 * H, D), B_w_uk.reshape(C // 2, 2 * H, D),
            B_w_uv.reshape(C // 2, 2 * H, D),
            jnp.swapaxes(B_w_o, 1, 2),
        )
        out = pl.pallas_call(
            kernel,
            in_specs=[pl.BlockSpec(memory_space=pl.ANY)] * len(args),
            out_specs=pl.BlockSpec(memory_space=pl.ANY),
            out_shape=jax.ShapeDtypeStruct((S, 2 * M), BF16),
            scratch_shapes=scratch,
            compiler_params=pltpu.CompilerParams(
                vmem_limit_bytes=126 * 1024 * 1024,
                disable_bounds_checks=True),
        )(*args)
        return out.reshape(1, S, 2 * M)

    return run


_run = _build()


@jax.jit
def pallas_concat_heads__ssm_conv_h3__compressed_kv_cla__prompt_kernel(
    A_q: jax.Array,
    A_k: jax.Array,
    A_v: jax.Array,
    A_shift_k: jax.Array,
    A_ssm_k: jax.Array,
    A_ssm_D: jax.Array,
    B_x: jax.Array,
    B_c_kv: jax.Array,
    B_w_q: jax.Array,
    B_w_uk: jax.Array,
    B_w_uv: jax.Array,
    B_w_o: jax.Array,
):
    return _run(A_q, A_k, A_v, A_shift_k, A_ssm_k, A_ssm_D, B_x, B_c_kv, B_w_q,
                B_w_uk, B_w_uv, B_w_o)
```
